```python
import jax
import jax.numpy as jnp

def _softmax(x, axis=-1):
    return jax.nn.softmax(x, axis=axis)
def _gelu(x):
    return jax.nn.gelu(x, approximate=True)
def _silu(x):
    return jax.nn.silu(x)
def _sigmoid(x):
    return jax.nn.sigmoid(x)
def _layernorm(x, axis=-1, eps=1e-5):
    m = jnp.mean(x, axis=axis, keepdims=True)
    v = jnp.var(x, axis=axis, keepdims=True)
    return (x - m) / jnp.sqrt(v + eps)
def _scatter_add(tgt, idx, src, axis=0):
    return tgt.at[idx].add(src)
def _segment_sum(src, seg, n):
    return jax.ops.segment_sum(src, seg, n)
class _Rng:
    def __init__(self, key):
        self._k = key
    def _next(self):
        self._k, sub = jax.random.split(self._k)
        return sub
    def normal(self, shape):
        return jax.random.normal(self._next(), shape, dtype=jnp.bfloat16)
    def randint(self, lo, hi, shape):
        return jax.random.randint(self._next(), shape, lo, hi, dtype=jnp.int32)
    def uniform(self, shape, lo=0.0, hi=1.0):
        return jax.random.uniform(self._next(), shape, jnp.bfloat16, lo, hi)
    def permutation(self, n):
        return jax.random.permutation(self._next(), n)


kernel_name = 'sequential_preLN__compressed_kv_cla__moe_arch_mod__prompt'

def setup_inputs():
    _rng = _Rng(jax.random.key(int.from_bytes(__import__("os").urandom(4), "little")))
    _w = (lambda a: (lambda t: t.astype(jnp.bfloat16) if jnp.issubdtype(t.dtype, jnp.floating) else t)(jnp.asarray(a)))
    def _A_setup():
        B, H, Sq, Sk, D, M = 1, 32, 2048, 2048, 128, 1024
        Dc = 4 * D
        return {
            "x": _w((lambda *s: _rng.normal(s) * 0.05)(B, Sq, M)),
            "c_kv": _w((lambda *s: _rng.normal(s) * 0.05)(B, Sk, Dc)),
            "w_q": _w((lambda *s: _rng.normal(s) * 0.05)(M, H, D) * (M ** -0.5)),
            "w_uk": _w((lambda *s: _rng.normal(s) * 0.05)(Dc, H, D) * (Dc ** -0.5)),
            "w_uv": _w((lambda *s: _rng.normal(s) * 0.05)(Dc, H, D) * (Dc ** -0.5)),
            "w_o": _w((lambda *s: _rng.normal(s) * 0.05)(H, D, M) * ((H * D) ** -0.5)),
        }
    _A_in = _A_setup()

    def _B_setup():
        B, S, D, F, C = 1, 2048, 1024, 3584, 2
        return {
            "x": _w((lambda *s: _rng.normal(s) * 0.05)(B, S, D)),
            "w_r": _w((lambda *s: _rng.normal(s) * 0.05)(D)),
            "w_gate": _w((lambda *s: _rng.normal(s) * 0.05)(D, F)),
            "w_up": _w((lambda *s: _rng.normal(s) * 0.05)(D, F)),
            "w_down": _w((lambda *s: _rng.normal(s) * 0.05)(F, D)),
        }
    _B_in = _B_setup()

    return {
        "A_x": _A_in["x"],
        "A_c_kv": _A_in["c_kv"],
        "A_w_q": _A_in["w_q"],
        "A_w_uk": _A_in["w_uk"],
        "A_w_uv": _A_in["w_uv"],
        "A_w_o": _A_in["w_o"],
        "B_x": _B_in["x"],
        "B_w_r": _B_in["w_r"],
        "B_w_gate": _B_in["w_gate"],
        "B_w_up": _B_in["w_up"],
        "B_w_down": _B_in["w_down"],
    }

def reference(A_x, A_c_kv, A_w_q, A_w_uk, A_w_uv, A_w_o, B_x, B_w_r, B_w_gate, B_w_up, B_w_down):
    def _A_ref(x, c_kv, w_q, w_uk, w_uv, w_o):
        B, Sq, M = x.shape[0], x.shape[1], x.shape[2]
        Sk = c_kv.shape[1]
        H, D = w_q.shape[1], w_q.shape[2]
        q = jnp.einsum("bqm,mhd->bhqd", x, w_q)
        k = jnp.einsum("bkc,chd->bhkd", c_kv, w_uk)
        v = jnp.einsum("bkc,chd->bhkd", c_kv, w_uv)
        scores = jnp.einsum("bhqd,bhkd->bhqk", q, k) * (D ** -0.5)
        off = Sk - Sq
        qi = jnp.arange(Sq)[:, None]
        kj = jnp.arange(Sk)[None, :]
        cmask = kj <= (qi + off)
        scores = jnp.where(cmask[None, None], scores, -1e9)
        p = _softmax(scores, axis=-1)
        ctx = jnp.einsum("bhqk,bhkd->bhqd", p, v)
        return jnp.einsum("bhqd,hdm->bqm", ctx, w_o)

    def _B_ref(x, w_r, w_gate, w_up, w_down):
        B, S, D = x.shape
        C = 2
        r = x @ w_r
        idx = jnp.argsort(-r, axis=-1)[:, :C]
        idx_e = jnp.repeat(idx.reshape(B, C, 1), D, axis=2)
        x_sel = jnp.take_along_axis(x, idx_e, axis=1)
        g = _silu(x_sel @ w_gate)
        u = x_sel @ w_up
        y = (g * u) @ w_down
        r_sel = _sigmoid(jnp.take_along_axis(r, idx, axis=1))
        y = y * r_sel.reshape(B, C, 1)
        b_off = (jnp.arange(B) * S).reshape(B, 1)
        flat_idx = (idx + b_off).reshape(B * C)
        zero = (x * 0.0).reshape(B * S, D)
        upd = _scatter_add(zero, flat_idx, y.reshape(B * C, D), axis=0)
        return x + upd.reshape(B, S, D)

    x = A_x
    h = x + _A_ref(_layernorm(x, axis=-1), A_c_kv, A_w_q, A_w_uk, A_w_uv, A_w_o)
    h2 = h + _B_ref(_layernorm(h, axis=-1), B_w_r, B_w_gate, B_w_up, B_w_down)
    return h2
```

```python
import functools
import math

import jax
import jax.numpy as jnp
from jax import lax
import jax.experimental.pallas as pl
import jax.experimental.pallas.tpu as pltpu

_F32 = jnp.float32
_BF16 = jnp.bfloat16
_U32 = jnp.uint32

_EPS = 1e-5
_NEG = -1e30
_TQ = 256
_TO = 256


def _dot(a, b):
    return jnp.dot(a, b, preferred_element_type=_F32)


def _dot_nt(a, b):
    return lax.dot_general(a, b, (((1,), (1,)), ((), ())), preferred_element_type=_F32)


def _as_bf16(u):
    return pltpu.bitcast(u, _BF16)


def _as_u32(b):
    return pltpu.bitcast(b, _U32)


def _round_bf16(x):
    return x.astype(_BF16).astype(_F32)


def _layernorm(x):
    n = x.shape[-1]
    mean = jnp.sum(x, axis=-1, keepdims=True) * (1.0 / n)
    xc = x - mean
    var = jnp.sum(xc * xc, axis=-1, keepdims=True) * (1.0 / n)
    m = _round_bf16(mean)
    den = _round_bf16(jnp.sqrt(_round_bf16(_round_bf16(var) + _EPS)))
    return (x - m) * (1.0 / den)


def _kernel(x_hbm, c_hbm, wq_hbm, wk_hbm, wv_hbm, wo_hbm, wr_ref, wg_hbm, wu_hbm, wd_hbm,
            out_hbm,
            x_raw, c_raw, xn_s, c_s, q_s, k_s, v_s,
            wq_p, wk_p, wv_p, wq_s, wk_s, wv_s,
            ctx_s, wo_s, wg_s, wu_s, wd_s, h_s, r_s, out_s,
            sem_x, sem_c, sem_w, sem_big, sem_out,
            *, S, M, DC, H, D, F):
    TQ = _TQ
    NB = S // TQ
    qscale = (D ** -0.5) * math.log2(math.e)

    wq32 = wq_hbm.bitcast(_U32)
    wk32 = wk_hbm.bitcast(_U32)
    wv32 = wv_hbm.bitcast(_U32)

    def w_copies(pair, slot):
        return (
            pltpu.make_async_copy(wk32.at[:, pair, :], wk_p.at[slot], sem_w.at[slot, 0]),
            pltpu.make_async_copy(wv32.at[:, pair, :], wv_p.at[slot], sem_w.at[slot, 1]),
            pltpu.make_async_copy(wq32.at[:, pair, :], wq_p.at[slot], sem_w.at[slot, 2]),
        )

    def x_copy(i):
        return pltpu.make_async_copy(x_hbm.at[pl.ds(i * TQ, TQ), :],
                                     x_raw.at[pl.ds(i * TQ, TQ), :], sem_x.at[i])

    def c_copy(i):
        return pltpu.make_async_copy(c_hbm.at[pl.ds(i * TQ, TQ), :],
                                     c_raw.at[pl.ds(i * TQ, TQ), :], sem_c.at[i])

    big = ((wo_hbm, wo_s), (wg_hbm, wg_s), (wu_hbm, wu_s), (wd_hbm, wd_s))

    def big_start(t):
        for n, (src, dst) in enumerate(big):
            rows = src.shape[0] // H
            r0 = pl.multiple_of(t * rows, 16)
            pltpu.make_async_copy(src.at[pl.ds(r0, rows), :], dst.at[pl.ds(r0, rows), :],
                                  sem_big.at[n]).start()

    def big_wait(n):
        pltpu.make_async_copy(big[n][1], big[n][1], sem_big.at[n]).wait()

    def unpack_weights(slot, shift):
        for src, dst in ((wk_p, wk_s), (wv_p, wv_s), (wq_p, wq_s)):
            w = src[slot]
            w = (w << shift) & jnp.uint32(0xFFFF0000)
            dst[...] = _as_u32(pltpu.bitcast(w, _F32).astype(_BF16))

    def rows2(i, n=TQ):
        return pl.ds(i * (TQ // 2), n // 2)

    def proj_q(i):
        a = _as_bf16(xn_s[rows2(i), :])
        q = _dot(a, _as_bf16(wq_s[...])) * qscale
        q_s[rows2(i), :] = _as_u32(q.astype(_BF16))

    def proj_k(i):
        a = _as_bf16(c_s[rows2(i), :])
        k_s[rows2(i), :] = _as_u32(_dot(a, _as_bf16(wk_s[...])).astype(_BF16))

    def proj_v(i):
        a = _as_bf16(c_s[rows2(i), :])
        v_s[rows2(i), :] = _as_u32(_dot(a, _as_bf16(wv_s[...])).astype(_BF16))

    for cp in w_copies(0, 0):
        cp.start()
    for i in range(NB):
        c_copy(i).start()
        x_copy(i).start()
    for cp in w_copies(0, 0):
        cp.wait()
    unpack_weights(0, jnp.uint32(16))

    def pro_body(i, carry):
        c_copy(i).wait()
        x_copy(i).wait()
        r0 = pl.multiple_of(i * TQ, TQ)
        p0 = pl.multiple_of(i * (TQ // 2), TQ // 2)
        cc = c_raw[pl.ds(r0, TQ), :]
        c_s[pl.ds(p0, TQ // 2), :] = _as_u32(cc)
        k_s[pl.ds(p0, TQ // 2), :] = _as_u32(_dot(cc, _as_bf16(wk_s[...])).astype(_BF16))
        v_s[pl.ds(p0, TQ // 2), :] = _as_u32(_dot(cc, _as_bf16(wv_s[...])).astype(_BF16))
        xn = _layernorm(x_raw[pl.ds(r0, TQ), :].astype(_F32)).astype(_BF16)
        xn_s[pl.ds(p0, TQ // 2), :] = _as_u32(xn)
        q = _dot(xn, _as_bf16(wq_s[...])) * qscale
        q_s[pl.ds(p0, TQ // 2), :] = _as_u32(q.astype(_BF16))
        return carry

    lax.fori_loop(0, NB, pro_body, 0)

    big_start(H - 1)

    HT = TQ // 2
    tri = (lax.broadcasted_iota(jnp.int32, (HT, HT), 1)
           <= lax.broadcasted_iota(jnp.int32, (HT, HT), 0))

    def softmax_rows(parts):
        s = parts[0] if len(parts) == 1 else jnp.concatenate(parts, axis=1)
        m = jnp.max(s, axis=1, keepdims=True)
        p = jnp.exp2(s - m)
        l = jnp.sum(p, axis=1, keepdims=True)
        return p.astype(_BF16), l

    def attention(h, with_proj):
        for i in range(NB - 1, -1, -1):
            Lm = i * TQ + HT
            q = _as_bf16(q_s[rows2(i), :])
            s_main = _dot_nt(q, _as_bf16(k_s[pl.ds(0, Lm // 2), :]))
            s_last = _dot_nt(q[HT:], _as_bf16(k_s[pl.ds(Lm // 2, HT // 2), :]))
            if with_proj:
                proj_q(i)
                proj_k(i)
            top = [jnp.where(tri, s_main[:HT, Lm - HT:], _NEG)]
            if Lm > HT:
                top = [s_main[:HT, :Lm - HT]] + top
            p_top, l_top = softmax_rows(top)
            p_bot, l_bot = softmax_rows([s_main[HT:], jnp.where(tri, s_last, _NEG)])
            p_main = jnp.concatenate([p_top, p_bot[:, :Lm]], axis=0)
            o = _dot(p_main, _as_bf16(v_s[pl.ds(0, Lm // 2), :]))
            o_last = _dot(p_bot[:, Lm:], _as_bf16(v_s[pl.ds(Lm // 2, HT // 2), :]))
            o_top = o[:HT] * pl.reciprocal(l_top, approx=True)
            o_bot = (o[HT:] + o_last) * pl.reciprocal(l_bot, approx=True)
            ctx_s[h, rows2(i), :] = _as_u32(
                jnp.concatenate([o_top, o_bot], axis=0).astype(_BF16))
            if with_proj:
                proj_v(i)

    def head_body(h, carry):
        hn = h + 1
        pair = hn // 2
        slot = pair % 2

        @pl.when(hn % 2 == 0)
        def _():
            for cp in w_copies(pair, slot):
                cp.wait()

        @pl.when(jnp.logical_and(hn % 2 == 1, pair + 1 < H // 2))
        def _():
            for cp in w_copies(pair + 1, 1 - slot):
                cp.start()

        big_start(h)
        shift = ((1 - hn % 2) * 16).astype(_U32)
        unpack_weights(slot, shift)
        attention(h, True)
        return carry

    lax.fori_loop(0, H - 1, head_body, 0)
    attention(H - 1, False)

    TO = _TO
    NO = S // TO
    big_wait(0)
    wr = wr_ref[...].astype(_F32)

    def out_copy(j):
        return pltpu.make_async_copy(out_s.at[pl.ds(j * TO, TO), :],
                                     out_hbm.at[pl.ds(j * TO, TO), :], sem_out.at[j])

    def o_body(j, carry):
        r0 = pl.multiple_of(j * TO, TO)
        p0 = pl.multiple_of(j * (TO // 2), TO // 2)
        a = jnp.concatenate(
            [_as_bf16(ctx_s[hh, pl.ds(p0, TO // 2), :]) for hh in range(H)], axis=1)
        att = _dot(a, wo_s[...])
        hres = _round_bf16(x_raw[pl.ds(r0, TO), :].astype(_F32) + att)
        h_s[pl.ds(r0, TO), :] = hres
        hn = _round_bf16(_layernorm(hres))
        r_s[pl.ds(r0, TO), :] = _round_bf16(jnp.sum(hn * wr, axis=1, keepdims=True))
        out_s[pl.ds(r0, TO), :] = (hres + hn).astype(_BF16)
        out_copy(j).start()
        return carry

    lax.fori_loop(0, NO, o_body, 0)

    r = r_s[...]
    rid = lax.broadcasted_iota(jnp.int32, (S, 1), 0)
    m1 = jnp.max(r, axis=0, keepdims=True)
    i1 = jnp.min(jnp.where(r == m1, rid, S), axis=0, keepdims=True)
    r2 = jnp.where(rid == i1, -jnp.inf, r)
    m2 = jnp.max(r2, axis=0, keepdims=True)
    i2 = jnp.min(jnp.where(jnp.logical_and(r2 == m2, rid != i1), rid, S), axis=0, keepdims=True)
    i1s = jnp.clip(i1[0, 0], 0, S - 1)
    i2s = jnp.clip(i2[0, 0], 0, S - 1)

    R = 16
    row = lax.broadcasted_iota(jnp.int32, (R, 1), 0)
    h1 = h_s[pl.ds(i1s, 1), :]
    h2 = h_s[pl.ds(i2s, 1), :]
    hsel = jnp.where(row == 0, h1, h2)
    xs = _layernorm(hsel).astype(_BF16)
    for n in (1, 2, 3):
        big_wait(n)
    g = _round_bf16(_dot(xs, wg_s[...]))
    u = _round_bf16(_dot(xs, wu_s[...]))
    g = _round_bf16(g * (1.0 / (1.0 + jnp.exp(-g))))
    act = (g * u).astype(_BF16)
    y = _round_bf16(_dot(act, wd_s[...]))
    rsel = jnp.where(row == 0, m1, m2)
    gate = _round_bf16(1.0 / (1.0 + jnp.exp(-rsel)))
    y = _round_bf16(y * gate)
    y1 = y[0:1]
    y2 = y[1:2]

    for j in range(NO):
        out_copy(j).wait()

    def fix_block(b0):
        hb = h_s[pl.ds(b0, R), :]
        hnb = _round_bf16(_layernorm(hb))
        grow = row + b0
        upd = jnp.where(grow == i1s, y1, 0.0) + jnp.where(grow == i2s, y2, 0.0)
        out_s[pl.ds(b0, R), :] = (hb + _round_bf16(hnb + upd)).astype(_BF16)

    def fix_copy(b0, k):
        return pltpu.make_async_copy(out_s.at[pl.ds(b0, R), :],
                                     out_hbm.at[pl.ds(b0, R), :], sem_out.at[k])

    b1 = pl.multiple_of((i1s // R) * R, R)
    b2 = pl.multiple_of((i2s // R) * R, R)
    fix_block(b1)
    fix_copy(b1, 0).start()

    @pl.when(b2 != b1)
    def _():
        fix_block(b2)
        fix_copy(b2, 1).start()
        fix_copy(b2, 1).wait()

    fix_copy(b1, 0).wait()


@jax.jit
def pallas_sequential_preLN__compressed_kv_cla__moe_arch_mod__prompt_kernel(
    A_x: jax.Array,
    A_c_kv: jax.Array,
    A_w_q: jax.Array,
    A_w_uk: jax.Array,
    A_w_uv: jax.Array,
    A_w_o: jax.Array,
    B_x: jax.Array,
    B_w_r: jax.Array,
    B_w_gate: jax.Array,
    B_w_up: jax.Array,
    B_w_down: jax.Array,
):
    B, S, M = A_x.shape
    assert B == 1
    DC = A_c_kv.shape[2]
    H, D = A_w_q.shape[1], A_w_q.shape[2]
    F = B_w_gate.shape[1]
    assert A_c_kv.shape[1] == S and S % _TQ == 0 and S % _TO == 0 and H % 2 == 0

    x = A_x.reshape(S, M)
    c = A_c_kv.reshape(S, DC)
    wo = A_w_o.reshape(H * D, M)
    wr = B_w_r.reshape(1, M)

    any_spec = pl.BlockSpec(memory_space=pl.ANY)
    vmem_spec = pl.BlockSpec(memory_space=pltpu.VMEM)
    scratch = [
        pltpu.VMEM((S, M), _BF16),
        pltpu.VMEM((S, DC), _BF16),
        pltpu.VMEM((S // 2, M), _U32),
        pltpu.VMEM((S // 2, DC), _U32),
        pltpu.VMEM((S // 2, D), _U32),
        pltpu.VMEM((S // 2, D), _U32),
        pltpu.VMEM((S // 2, D), _U32),
        pltpu.VMEM((2, M, D), _U32),
        pltpu.VMEM((2, DC, D), _U32),
        pltpu.VMEM((2, DC, D), _U32),
        pltpu.VMEM((M // 2, D), _U32),
        pltpu.VMEM((DC // 2, D), _U32),
        pltpu.VMEM((DC // 2, D), _U32),
        pltpu.VMEM((H, S // 2, D), _U32),
        pltpu.VMEM((H * D, M), _BF16),
        pltpu.VMEM((M, F), _BF16),
        pltpu.VMEM((M, F), _BF16),
        pltpu.VMEM((F, M), _BF16),
        pltpu.VMEM((S, M), _F32),
        pltpu.VMEM((S, 1), _F32),
        pltpu.VMEM((S, M), _BF16),
        pltpu.SemaphoreType.DMA((S // _TQ,)),
        pltpu.SemaphoreType.DMA((S // _TQ,)),
        pltpu.SemaphoreType.DMA((2, 3)),
        pltpu.SemaphoreType.DMA((4,)),
        pltpu.SemaphoreType.DMA((S // _TO,)),
    ]
    out = pl.pallas_call(
        functools.partial(_kernel, S=S, M=M, DC=DC, H=H, D=D, F=F),
        in_specs=[any_spec, any_spec, any_spec, any_spec, any_spec, any_spec,
                  vmem_spec, any_spec, any_spec, any_spec],
        out_specs=any_spec,
        out_shape=jax.ShapeDtypeStruct((S, M), _BF16),
        scratch_shapes=scratch,
        compiler_params=pltpu.CompilerParams(vmem_limit_bytes=112 * 1024 * 1024),
        name="fused_mla_mod",
    )(x, c, A_w_q, A_w_uk, A_w_uv, wo, wr, B_w_gate, B_w_up, B_w_down)
    return out.reshape(B, S, M)
```

```python
import functools
import math

import jax
import jax.numpy as jnp
from jax import lax
import jax.experimental.pallas as pl
import jax.experimental.pallas.tpu as pltpu

_F32 = jnp.float32
_BF16 = jnp.bfloat16
_U32 = jnp.uint32
_I32 = jnp.int32

_EPS = 1e-5
_NEG = -1e30
_TQ = 256
_HT = 128
_FIX = 16
_WD_PAD = 128


def _dot(a, b):
    return jnp.dot(a, b, preferred_element_type=_F32)


def _dot_nt(a, b):
    return lax.dot_general(a, b, (((1,), (1,)), ((), ())), preferred_element_type=_F32)


def _as_bf16(u):
    return pltpu.bitcast(u, _BF16)


def _pack(x):
    return pltpu.bitcast(x.astype(_BF16), _U32)


def _round_bf16(x):
    return x.astype(_BF16).astype(_F32)


def _layernorm(x):
    n = x.shape[-1]
    mean = jnp.sum(x, axis=-1, keepdims=True) * (1.0 / n)
    xc = x - mean
    var = jnp.sum(xc * xc, axis=-1, keepdims=True) * (1.0 / n)
    m = _round_bf16(mean)
    den = _round_bf16(jnp.sqrt(_round_bf16(_round_bf16(var) + _EPS)))
    return (x - m) * (1.0 / den)


def _strassen_a(a11, a12, a21, a22):
    return (a11 + a22, a21 + a22, a11, a22, a11 + a12, a21 - a11, a12 - a22)


def _strassen_b(b11, b12, b21, b22):
    return (b11 + b22, b11, b12 - b22, b21 - b11, b22, b11 + b12, b21 + b22)


def _strassen_c(m):
    m1, m2, m3, m4, m5, m6, m7 = m
    return (m1 + m4 - m5 + m7, m3 + m5, m2 + m4, m1 - m2 + m3 + m6)


def _quadrants(x):
    r, c = x.shape[0] // 2, x.shape[1] // 2
    return x[:r, :c], x[:r, c:], x[r:, :c], x[r:, c:]


def _kernel(x_hbm, c_hbm, wq_hbm, wk_hbm, wv_hbm, wo_hbm, wr_ref, wg_hbm, wu_hbm, wd_hbm,
            out_hbm,
            x_raw, c_raw, xa_s, ca_s, q_s, k_s, v_s,
            wq_p, wk_p, wv_p, wqb_s, wkb_s, wvb_s,
            ctx_s, wo_p, wob_s, wg_s, wu_s, wd_s, h_s, r_s, out_s,
            sem_x, sem_c, sem_w, sem_wo, sem_ffn, sem_out,
            *, S, M, DC, H, D, F):
    TQ, HT = _TQ, _HT
    NB = S // TQ
    NP = H // 2
    KO = H * D // 2
    OS = KO // NP
    qscale = (D ** -0.5) * math.log2(math.e)

    wq32 = wq_hbm.bitcast(_U32)
    wk32 = wk_hbm.bitcast(_U32)
    wv32 = wv_hbm.bitcast(_U32)

    def w_copies(pair, slot):
        return (
            pltpu.make_async_copy(wk32.at[:, pair, :], wk_p.at[slot], sem_w.at[slot, 0]),
            pltpu.make_async_copy(wv32.at[:, pair, :], wv_p.at[slot], sem_w.at[slot, 1]),
            pltpu.make_async_copy(wq32.at[:, pair, :], wq_p.at[slot], sem_w.at[slot, 2]),
        )

    def wo_copies(t, slot):
        r0 = pl.multiple_of(t * OS, OS)
        return tuple(
            pltpu.make_async_copy(wo_hbm.at[pl.ds(half * KO + r0, OS), :],
                                  wo_p.at[slot, half], sem_wo.at[slot, half])
            for half in range(2))

    def x_copy(i):
        return pltpu.make_async_copy(x_hbm.at[pl.ds(i * TQ, TQ), :],
                                     x_raw.at[pl.ds(i * TQ, TQ), :], sem_x.at[i])

    def c_copy(i):
        return pltpu.make_async_copy(c_hbm.at[pl.ds(i * TQ, TQ), :],
                                     c_raw.at[pl.ds(i * TQ, TQ), :], sem_c.at[i])

    ffn = ((wg_hbm, wg_s), (wu_hbm, wu_s), (wd_hbm, wd_s))

    def ffn_start(t):
        for n, (src, dst) in enumerate(ffn):
            rows, cols = src.shape[0] // NP, src.shape[1]
            r0 = pl.multiple_of(t * rows, 16)
            pltpu.make_async_copy(src.at[pl.ds(r0, rows), :],
                                  dst.at[pl.ds(r0, rows), pl.ds(0, cols)],
                                  sem_ffn.at[n]).start()

    def ffn_wait(n):
        src, dst = ffn[n]
        pltpu.make_async_copy(src, dst.at[:, pl.ds(0, src.shape[1])], sem_ffn.at[n]).wait()

    def prep_pair_weights(slot):
        for src, dst in ((wk_p, wkb_s), (wv_p, wvb_s), (wq_p, wqb_s)):
            w = src[slot]
            kh = w.shape[0] // 2
            lo = pltpu.bitcast(w << 16, _F32)
            hi = pltpu.bitcast(w & jnp.uint32(0xFFFF0000), _F32)
            for t, b in enumerate(_strassen_b(lo[:kh], hi[:kh], lo[kh:], hi[kh:])):
                dst[t] = _pack(b)

    def prep_wo(slot, src0, nrows, dst0):
        top = wo_p[slot, 0, pl.ds(src0, nrows), :].astype(_F32)
        bot = wo_p[slot, 1, pl.ds(src0, nrows), :].astype(_F32)
        mh = M // 2
        for t, b in enumerate(_strassen_b(top[:, :mh], top[:, mh:], bot[:, :mh], bot[:, mh:])):
            wob_s[t, pl.ds(dst0, nrows // 2), :] = _pack(b)

    def project(a_ref, b_ref, dst, p0, a0):
        m = [_dot(_as_bf16(a_ref[t, pl.ds(a0, HT // 2), :]), _as_bf16(b_ref[t]))
             for t in range(7)]
        c11, c12, c21, c22 = _strassen_c(m)
        dst[0, pl.ds(p0, HT // 2), :] = _pack(c11)
        dst[1, pl.ds(p0, HT // 2), :] = _pack(c12)
        dst[0, pl.ds(p0 + HT // 2, HT // 2), :] = _pack(c21)
        dst[1, pl.ds(p0 + HT // 2, HT // 2), :] = _pack(c22)

    for cp in w_copies(0, 0):
        cp.start()
    for i in range(NB):
        c_copy(i).start()
        x_copy(i).start()
    for cp in w_copies(1, 1):
        cp.start()
    for cp in wo_copies(0, 0):
        cp.start()
    h_s[pl.ds(0, HT), :] = jnp.zeros((HT, M), _F32)
    for cp in w_copies(0, 0):
        cp.wait()
    prep_pair_weights(0)

    def pro_body(i, carry):
        c_copy(i).wait()
        x_copy(i).wait()
        r0 = pl.multiple_of(i * TQ, TQ)
        p0 = pl.multiple_of(i * (TQ // 2), TQ // 2)
        a0 = pl.multiple_of(i * (HT // 2), HT // 2)
        cc = c_raw[pl.ds(r0, TQ), :].astype(_F32)
        for t, a in enumerate(_strassen_a(*_quadrants(cc))):
            ca_s[t, pl.ds(a0, HT // 2), :] = _pack(a)
        project(ca_s, wkb_s, k_s, p0, a0)
        project(ca_s, wvb_s, v_s, p0, a0)
        xn = _layernorm(x_raw[pl.ds(r0, TQ), :].astype(_F32)) * qscale
        for t, a in enumerate(_strassen_a(*_quadrants(xn))):
            xa_s[t, pl.ds(a0, HT // 2), :] = _pack(a)
        project(xa_s, wqb_s, q_s, p0, a0)
        return carry

    lax.fori_loop(0, NB, pro_body, 0)

    ffn_start(NP - 1)

    tri = (lax.broadcasted_iota(_I32, (HT, HT), 1)
           <= lax.broadcasted_iota(_I32, (HT, HT), 0))

    def softmax_rows(parts):
        s = parts[0] if len(parts) == 1 else jnp.concatenate(parts, axis=1)
        m = jnp.max(s, axis=1, keepdims=True)
        p = jnp.exp2(s - m)
        l = jnp.sum(p, axis=1, keepdims=True)
        return p.astype(_BF16), l

    def scores(e, i):
        Lm = i * TQ + HT
        q = _as_bf16(q_s[e, pl.ds(i * (TQ // 2), TQ // 2), :])
        s_main = _dot_nt(q, _as_bf16(k_s[e, pl.ds(0, Lm // 2), :]))
        s_last = _dot_nt(q[HT:], _as_bf16(k_s[e, pl.ds(Lm // 2, HT // 2), :]))
        return s_main, s_last

    def context(e, head, i, s_main, s_last):
        Lm = i * TQ + HT
        top = [jnp.where(tri, s_main[:HT, Lm - HT:], _NEG)]
        if Lm > HT:
            top = [s_main[:HT, :Lm - HT]] + top
        p_top, l_top = softmax_rows(top)
        p_bot, l_bot = softmax_rows([s_main[HT:], jnp.where(tri, s_last, _NEG)])
        p_main = jnp.concatenate([p_top, p_bot[:, :Lm]], axis=0)
        o = _dot(p_main, _as_bf16(v_s[e, pl.ds(0, Lm // 2), :]))
        o_last = _dot(p_bot[:, Lm:], _as_bf16(v_s[e, pl.ds(Lm // 2, HT // 2), :]))
        o_top = o[:HT] * pl.reciprocal(l_top, approx=True)
        o_bot = (o[HT:] + o_last) * pl.reciprocal(l_bot, approx=True)
        ctx_s[head, pl.ds(i * (TQ // 2), TQ // 2), :] = _pack(
            jnp.concatenate([o_top, o_bot], axis=0))

    def pair_body(s, carry):
        slot = (s + 1) % 2

        @pl.when(s + 2 < NP)
        def _():
            for cp in w_copies(s + 2, 1 - slot):
                cp.start()

        for cp in wo_copies(s + 1, slot):
            cp.start()
        ffn_start(s)
        for cp in w_copies(s + 1, slot):
            cp.wait()
        for cp in wo_copies(s, 1 - slot):
            cp.wait()

        prep_pair_weights(slot)
        prep_wo(1 - slot, 0, OS, pl.multiple_of(s * (OS // 2), OS // 2))
        for i in range(NB - 1, -1, -1):
            p0, a0 = i * (TQ // 2), i * (HT // 2)
            sa = scores(0, i)
            sb = scores(1, i)
            project(xa_s, wqb_s, q_s, p0, a0)
            project(ca_s, wkb_s, k_s, p0, a0)
            context(0, 2 * s, i, *sa)
            context(1, 2 * s + 1, i, *sb)
            project(ca_s, wvb_s, v_s, p0, a0)
        return carry

    lax.fori_loop(0, NP - 1, pair_body, 0)

    last_slot = (NP - 1) % 2
    for cp in wo_copies(NP - 1, last_slot):
        cp.wait()

    def last_body(e, carry):
        half = OS // 2
        prep_wo(last_slot, pl.multiple_of(e * half, half), half,
                pl.multiple_of((NP - 1) * (OS // 2) + e * (half // 2), half // 2))
        nxt = scores(e, NB - 1)
        for i in range(NB - 1, -1, -1):
            cur = nxt
            if i > 0:
                nxt = scores(e, i - 1)
            context(e, H - 2 + e, i, *cur)
        return carry

    lax.fori_loop(0, 2, last_body, 0)

    wr = wr_ref[...].astype(_F32)
    eye = (lax.broadcasted_iota(_I32, (HT, HT), 1) == lax.broadcasted_iota(_I32, (HT, HT), 0))

    def epilogue(g, hres):
        r0 = pl.multiple_of((g + 1) * HT, HT)
        hn = _round_bf16(_layernorm(hres))
        r = _round_bf16(jnp.sum(hn * wr, axis=1, keepdims=True))
        r_s[pl.ds(g + 8, 1), :] = jnp.sum(jnp.where(eye, r, 0.0), axis=0, keepdims=True)
        out_s[pl.ds(r0, HT), :] = (hres + hn).astype(_BF16)

    def out_copy(g):
        return pltpu.make_async_copy(out_s.at[pl.ds(pl.multiple_of((g + 1) * HT, HT), HT), :],
                                     out_hbm.at[pl.ds(pl.multiple_of(g * HT, HT), HT), :],
                                     sem_out.at[g])

    def ctx_quadrant(p0, h0):
        return jnp.concatenate(
            [_as_bf16(ctx_s[h0 + hh, pl.ds(p0, HT // 2), :]) for hh in range(NP)],
            axis=1)

    def o_body(j, carry):
        r0 = pl.multiple_of(j * TQ, TQ)
        p0 = pl.multiple_of(j * (TQ // 2), TQ // 2)
        epilogue(2 * j - 1, h_s[pl.ds(r0, HT), :])

        a11 = ctx_quadrant(p0, 0)
        a12 = ctx_quadrant(p0, NP)
        a21 = ctx_quadrant(p0 + HT // 2, 0)
        a22 = ctx_quadrant(p0 + HT // 2, NP)
        f = lambda t: t.astype(_F32)

        def prod(t, a):
            return _dot(a.astype(_BF16), _as_bf16(wob_s[t]))

        m3 = prod(2, a11)
        m4 = prod(3, a22)
        m1 = prod(0, f(a11) + f(a22))
        m5 = prod(4, f(a11) + f(a12))
        m7 = prod(6, f(a12) - f(a22))
        att_top = jnp.concatenate([m1 + m4 - m5 + m7, m3 + m5], axis=1)
        h_top = _round_bf16(x_raw[pl.ds(r0, HT), :].astype(_F32) + att_top)
        h_s[pl.ds(r0 + HT, HT), :] = h_top
        epilogue(2 * j, h_top)
        m2 = prod(1, f(a21) + f(a22))
        m6 = prod(5, f(a21) - f(a11))
        att_bot = jnp.concatenate([m2 + m4, m1 - m2 + m3 + m6], axis=1)
        h_s[pl.ds(r0 + 2 * HT, HT), :] = _round_bf16(
            x_raw[pl.ds(r0 + HT, HT), :].astype(_F32) + att_bot)

        @pl.when(j > 0)
        def _():
            out_copy(2 * j - 1).start()

        out_copy(2 * j).start()
        return carry

    lax.fori_loop(0, NB, o_body, 0)
    NG = S // HT
    epilogue(NG - 1, h_s[pl.ds(S, HT), :])
    out_copy(NG - 1).start()

    r = r_s[pl.ds(8, NG), :] + 0.0
    tok = (lax.broadcasted_iota(_I32, (NG, HT), 0) * HT + lax.broadcasted_iota(_I32, (NG, HT), 1))
    bits = pltpu.bitcast(r, _I32)
    key = jnp.where(bits < 0, bits ^ 0x7FFF0000, bits) | (0xFFFF - tok)
    k1 = jnp.max(jnp.max(key, axis=0, keepdims=True), axis=1, keepdims=True)
    key2 = jnp.where(key == k1, jnp.iinfo(jnp.int32).min, key)
    k2 = jnp.max(jnp.max(key2, axis=0, keepdims=True), axis=1, keepdims=True)
    i1s = jnp.clip(0xFFFF - (k1[0, 0] & 0xFFFF), 0, S - 1)
    i2s = jnp.clip(0xFFFF - (k2[0, 0] & 0xFFFF), 0, S - 1)

    R = _FIX
    row = lax.broadcasted_iota(_I32, (R, 1), 0)
    h1 = h_s[pl.ds(i1s + HT, 1), :]
    h2 = h_s[pl.ds(i2s + HT, 1), :]
    hsel = jnp.where(row == 0, h1, h2)
    xs = _layernorm(hsel).astype(_BF16)
    for n in range(3):
        ffn_wait(n)
    g = _round_bf16(_dot(xs, wg_s[...]))
    u = _round_bf16(_dot(xs, wu_s[...]))
    g = _round_bf16(g * (1.0 / (1.0 + jnp.exp(-g))))
    act = (g * u).astype(_BF16)
    y = _round_bf16(_dot(act, wd_s[:, pl.ds(0, M)]))
    ksel = jnp.where(row == 0, k1, k2) & (-0x10000)
    rsel = pltpu.bitcast(jnp.where(ksel < 0, ksel ^ 0x7FFF0000, ksel), _F32)
    gate = _round_bf16(1.0 / (1.0 + jnp.exp(-rsel)))
    y = _round_bf16(y * gate)
    y1 = y[0:1]
    y2 = y[1:2]

    for gi in range(NG):
        out_copy(gi).wait()

    def fix_block(b0):
        hb = h_s[pl.ds(pl.multiple_of(b0 + HT, R), R), :]
        hnb = _round_bf16(_layernorm(hb))
        grow = row + b0
        upd = jnp.where(grow == i1s, y1, 0.0) + jnp.where(grow == i2s, y2, 0.0)
        out_s[pl.ds(pl.multiple_of(b0 + HT, R), R), :] = (
            hb + _round_bf16(hnb + upd)).astype(_BF16)

    def fix_copy(b0, k):
        return pltpu.make_async_copy(out_s.at[pl.ds(pl.multiple_of(b0 + HT, R), R), :],
                                     out_hbm.at[pl.ds(b0, R), :], sem_out.at[k])

    b1 = pl.multiple_of((i1s // R) * R, R)
    b2 = pl.multiple_of((i2s // R) * R, R)
    fix_block(b1)
    fix_block(b2)
    fix_copy(b1, 0).start()

    @pl.when(b2 != b1)
    def _():
        fix_copy(b2, 1).start()
        fix_copy(b2, 1).wait()

    fix_copy(b1, 0).wait()


@jax.jit
def pallas_sequential_preLN__compressed_kv_cla__moe_arch_mod__prompt_kernel(
    A_x: jax.Array,
    A_c_kv: jax.Array,
    A_w_q: jax.Array,
    A_w_uk: jax.Array,
    A_w_uv: jax.Array,
    A_w_o: jax.Array,
    B_x: jax.Array,
    B_w_r: jax.Array,
    B_w_gate: jax.Array,
    B_w_up: jax.Array,
    B_w_down: jax.Array,
):
    B, S, M = A_x.shape
    assert B == 1
    DC = A_c_kv.shape[2]
    H, D = A_w_q.shape[1], A_w_q.shape[2]
    F = B_w_gate.shape[1]
    assert A_c_kv.shape[1] == S and S % _TQ == 0 and H % 2 == 0 and S <= 0x10000
    NP = H // 2
    NG = S // _HT

    x = A_x.reshape(S, M)
    c = A_c_kv.reshape(S, DC)
    wo = A_w_o.reshape(H * D, M)
    wr = B_w_r.reshape(1, M)

    any_spec = pl.BlockSpec(memory_space=pl.ANY)
    vmem_spec = pl.BlockSpec(memory_space=pltpu.VMEM)
    scratch = [
        pltpu.VMEM((S, M), _BF16),
        pltpu.VMEM((S, DC), _BF16),
        pltpu.VMEM((7, S // 4, M // 2), _U32),
        pltpu.VMEM((7, S // 4, DC // 2), _U32),
        pltpu.VMEM((2, S // 2, D), _U32),
        pltpu.VMEM((2, S // 2, D), _U32),
        pltpu.VMEM((2, S // 2, D), _U32),
        pltpu.VMEM((2, M, D), _U32),
        pltpu.VMEM((2, DC, D), _U32),
        pltpu.VMEM((2, DC, D), _U32),
        pltpu.VMEM((7, M // 4, D), _U32),
        pltpu.VMEM((7, DC // 4, D), _U32),
        pltpu.VMEM((7, DC // 4, D), _U32),
        pltpu.VMEM((H, S // 2, D), _U32),
        pltpu.VMEM((2, 2, D, M), _BF16),
        pltpu.VMEM((7, H * D // 4, M // 2), _U32),
        pltpu.VMEM((M, F), _BF16),
        pltpu.VMEM((M, F), _BF16),
        pltpu.VMEM((F, M + _WD_PAD), _BF16),
        pltpu.VMEM((S + _HT, M), _F32),
        pltpu.VMEM((NG + 8, _HT), _F32),
        pltpu.VMEM((S + _HT, M), _BF16),
        pltpu.SemaphoreType.DMA((S // _TQ,)),
        pltpu.SemaphoreType.DMA((S // _TQ,)),
        pltpu.SemaphoreType.DMA((2, 3)),
        pltpu.SemaphoreType.DMA((2, 2)),
        pltpu.SemaphoreType.DMA((3,)),
        pltpu.SemaphoreType.DMA((NG,)),
    ]
    out = pl.pallas_call(
        functools.partial(_kernel, S=S, M=M, DC=DC, H=H, D=D, F=F),
        in_specs=[any_spec, any_spec, any_spec, any_spec, any_spec, any_spec,
                  vmem_spec, any_spec, any_spec, any_spec],
        out_specs=any_spec,
        out_shape=jax.ShapeDtypeStruct((S, M), _BF16),
        scratch_shapes=scratch,
        compiler_params=pltpu.CompilerParams(vmem_limit_bytes=120 * 1024 * 1024,
                                             disable_bounds_checks=True),
        name="fused_mla_mod",
    )(x, c, A_w_q, A_w_uk, A_w_uv, wo, wr, B_w_gate, B_w_up, B_w_down)
    return out.reshape(B, S, M)
```

```python
import functools
import math

import jax
import jax.numpy as jnp
from jax import lax
import jax.experimental.pallas as pl
import jax.experimental.pallas.tpu as pltpu

_F32 = jnp.float32
_BF16 = jnp.bfloat16
_U32 = jnp.uint32
_I32 = jnp.int32

_EPS = 1e-5
_NEG = -1e30
_TQ = 256
_HT = 128
_TIE = 4
_FIX = 16
_WD_PAD = 128


def _dot(a, b):
    return jnp.dot(a, b, preferred_element_type=_F32)


def _dot_nt(a, b):
    return lax.dot_general(a, b, (((1,), (1,)), ((), ())), preferred_element_type=_F32)


def _as_bf16(u):
    return pltpu.bitcast(u, _BF16)


def _pack(x):
    return pltpu.bitcast(x.astype(_BF16), _U32)


def _round_bf16(x):
    return x.astype(_BF16).astype(_F32)


def _layernorm(x):
    n = x.shape[-1]
    mean = jnp.sum(x, axis=-1, keepdims=True) * (1.0 / n)
    xc = x - mean
    var = jnp.sum(xc * xc, axis=-1, keepdims=True) * (1.0 / n)
    m = _round_bf16(mean)
    den = _round_bf16(jnp.sqrt(_round_bf16(_round_bf16(var) + _EPS)))
    return (x - m) * (1.0 / den)


def _strassen_a(a11, a12, a21, a22):
    return (a11 + a22, a21 + a22, a11, a22, a11 + a12, a21 - a11, a12 - a22)


def _strassen_b(b11, b12, b21, b22):
    return (b11 + b22, b11, b12 - b22, b21 - b11, b22, b11 + b12, b21 + b22)


def _strassen_c(m):
    m1, m2, m3, m4, m5, m6, m7 = m
    return (m1 + m4 - m5 + m7, m3 + m5, m2 + m4, m1 - m2 + m3 + m6)


def _quadrants(x):
    r, c = x.shape[0] // 2, x.shape[1] // 2
    return x[:r, :c], x[:r, c:], x[r:, :c], x[r:, c:]


def _kernel(x_hbm, c_hbm, wq_hbm, wk_hbm, wv_hbm, wo_hbm, wr_ref, wg_hbm, wu_hbm, wd_hbm,
            out_hbm,
            x_raw, c_raw, xa_s, ca_s, q_s, k_s, v_s,
            wq_p, wk_p, wv_p, wqb_s, wkb_s, wvb_s,
            ctx_s, wo_p, wob_s, wg_s, wu_s, wd_s, h_s, r_s, out_s,
            sem_x, sem_c, sem_w, sem_wo, sem_ffn, sem_out,
            *, S, M, DC, H, D, F):
    TQ, HT = _TQ, _HT
    NB = S // TQ
    NP = H // 2
    KO = H * D // 2
    OS = KO // NP
    qscale = (D ** -0.5) * math.log2(math.e)

    wq32 = wq_hbm.bitcast(_U32)
    wk32 = wk_hbm.bitcast(_U32)
    wv32 = wv_hbm.bitcast(_U32)

    def w_copies(pair, slot):
        return (
            pltpu.make_async_copy(wk32.at[:, pair, :], wk_p.at[slot], sem_w.at[slot, 0]),
            pltpu.make_async_copy(wv32.at[:, pair, :], wv_p.at[slot], sem_w.at[slot, 1]),
            pltpu.make_async_copy(wq32.at[:, pair, :], wq_p.at[slot], sem_w.at[slot, 2]),
        )

    def wo_copies(t, slot):
        r0 = pl.multiple_of(t * OS, OS)
        return tuple(
            pltpu.make_async_copy(wo_hbm.at[pl.ds(half * KO + r0, OS), :],
                                  wo_p.at[slot, half], sem_wo.at[slot, half])
            for half in range(2))

    def x_copy(i):
        return pltpu.make_async_copy(x_hbm.at[pl.ds(i * TQ, TQ), :],
                                     x_raw.at[pl.ds(i * TQ, TQ), :], sem_x.at[i])

    def c_copy(i):
        return pltpu.make_async_copy(c_hbm.at[pl.ds(i * TQ, TQ), :],
                                     c_raw.at[pl.ds(i * TQ, TQ), :], sem_c.at[i])

    ffn = ((wg_hbm, wg_s), (wu_hbm, wu_s), (wd_hbm, wd_s))

    def ffn_start(t):
        for n, (src, dst) in enumerate(ffn):
            rows, cols = src.shape[0] // NP, src.shape[1]
            r0 = pl.multiple_of(t * rows, 16)
            pltpu.make_async_copy(src.at[pl.ds(r0, rows), :],
                                  dst.at[pl.ds(r0, rows), pl.ds(0, cols)],
                                  sem_ffn.at[n]).start()

    def ffn_wait(n):
        src, dst = ffn[n]
        pltpu.make_async_copy(src, dst.at[:, pl.ds(0, src.shape[1])], sem_ffn.at[n]).wait()

    def lo_hi(w):
        return (pltpu.bitcast(w << 16, _F32), pltpu.bitcast(w & jnp.uint32(0xFFFF0000), _F32))

    def prep_pair_weights(slot):
        RC = 32
        for src, dst in ((wq_p, wqb_s), (wk_p, wkb_s), (wv_p, wvb_s)):
            kh = src.shape[1] // 2
            for r in range(0, kh, RC):
                b11, b12 = lo_hi(src[slot, pl.ds(r, RC), :])
                b21, b22 = lo_hi(src[slot, pl.ds(kh + r, RC), :])
                for t, b in enumerate(_strassen_b(b11, b12, b21, b22)):
                    dst[t, pl.ds(r // 2, RC // 2), :] = _pack(b)

    def prep_wo(slot, src0, nrows, dst0):
        mh = M // 2
        CC = 256
        for r in range(0, nrows, 16):
            rs = pl.ds(src0 + r, 16)
            for c0 in range(0, mh, CC):
                b11 = wo_p[slot, 0, rs, pl.ds(c0, CC)].astype(_F32)
                b12 = wo_p[slot, 0, rs, pl.ds(mh + c0, CC)].astype(_F32)
                b21 = wo_p[slot, 1, rs, pl.ds(c0, CC)].astype(_F32)
                b22 = wo_p[slot, 1, rs, pl.ds(mh + c0, CC)].astype(_F32)
                for t, b in enumerate(_strassen_b(b11, b12, b21, b22)):
                    wob_s[t, pl.ds(dst0 + r // 2, 8), pl.ds(c0, CC)] = _pack(b)

    def project(a_ref, b_ref, dst, p0, a0):
        m = [_dot(_as_bf16(a_ref[t, pl.ds(a0, HT // 2), :]), _as_bf16(b_ref[t]))
             for t in range(7)]
        c11, c12, c21, c22 = _strassen_c(m)
        dst[0, pl.ds(p0, HT // 2), :] = _pack(c11)
        dst[1, pl.ds(p0, HT // 2), :] = _pack(c12)
        dst[0, pl.ds(p0 + HT // 2, HT // 2), :] = _pack(c21)
        dst[1, pl.ds(p0 + HT // 2, HT // 2), :] = _pack(c22)

    for cp in w_copies(0, 0):
        cp.start()
    for i in range(NB):
        c_copy(i).start()
        x_copy(i).start()
    for cp in w_copies(1, 1):
        cp.start()
    for cp in wo_copies(0, 0):
        cp.start()
    h_s[pl.ds(0, HT), :] = jnp.zeros((HT, M), _F32)
    for cp in w_copies(0, 0):
        cp.wait()
    prep_pair_weights(0)

    def pro_body(i, carry):
        c_copy(i).wait()
        x_copy(i).wait()
        r0 = pl.multiple_of(i * TQ, TQ)
        p0 = pl.multiple_of(i * (TQ // 2), TQ // 2)
        a0 = pl.multiple_of(i * (HT // 2), HT // 2)
        cc = c_raw[pl.ds(r0, TQ), :].astype(_F32)
        for t, a in enumerate(_strassen_a(*_quadrants(cc))):
            ca_s[t, pl.ds(a0, HT // 2), :] = _pack(a)
        project(ca_s, wkb_s, k_s, p0, a0)
        project(ca_s, wvb_s, v_s, p0, a0)
        xn = _layernorm(x_raw[pl.ds(r0, TQ), :].astype(_F32)) * qscale
        for t, a in enumerate(_strassen_a(*_quadrants(xn))):
            xa_s[t, pl.ds(a0, HT // 2), :] = _pack(a)
        project(xa_s, wqb_s, q_s, p0, a0)
        return carry

    lax.fori_loop(0, NB, pro_body, 0)

    ffn_start(NP - 1)

    tri = (lax.broadcasted_iota(_I32, (HT, HT), 1)
           <= lax.broadcasted_iota(_I32, (HT, HT), 0))

    def softmax_rows(parts):
        s = parts[0] if len(parts) == 1 else jnp.concatenate(parts, axis=1)
        m = jnp.max(s, axis=1, keepdims=True)
        p = jnp.exp2(s - m)
        nt = p.shape[1] // HT
        tiles, acc = [], None
        for j in range(nt):
            pj = p[:, j * HT:(j + 1) * HT]
            acc = pj if acc is None else acc + pj
            if j > 0 and (j % _TIE == _TIE - 1 or j == nt - 1):
                pj = jnp.where(acc < 0.0, 0.0, pj)
            tiles.append(pj)
        p = tiles[0] if nt == 1 else jnp.concatenate(tiles, axis=1)
        l = jnp.sum(acc, axis=1, keepdims=True)
        return p.astype(_BF16), l

    def scores(e, i):
        Lm = i * TQ + HT
        q = _as_bf16(q_s[e, pl.ds(i * (TQ // 2), TQ // 2), :])
        s_main = _dot_nt(q, _as_bf16(k_s[e, pl.ds(0, Lm // 2), :]))
        s_last = _dot_nt(q[HT:], _as_bf16(k_s[e, pl.ds(Lm // 2, HT // 2), :]))
        return s_main, s_last

    def context(e, head, i, s_main, s_last):
        Lm = i * TQ + HT
        top = [jnp.where(tri, s_main[:HT, Lm - HT:], _NEG)]
        if Lm > HT:
            top = [s_main[:HT, :Lm - HT]] + top
        p_top, l_top = softmax_rows(top)
        p_bot, l_bot = softmax_rows([s_main[HT:], jnp.where(tri, s_last, _NEG)])
        p_main = jnp.concatenate([p_top, p_bot[:, :Lm]], axis=0)
        o = _dot(p_main, _as_bf16(v_s[e, pl.ds(0, Lm // 2), :]))
        o_last = _dot(p_bot[:, Lm:], _as_bf16(v_s[e, pl.ds(Lm // 2, HT // 2), :]))
        o_top = o[:HT] * pl.reciprocal(l_top, approx=True)
        o_bot = (o[HT:] + o_last) * pl.reciprocal(l_bot, approx=True)
        ctx_s[head, pl.ds(i * (TQ // 2), TQ // 2), :] = _pack(
            jnp.concatenate([o_top, o_bot], axis=0))

    def pair_body(s, carry):
        slot = (s + 1) % 2

        @pl.when(s + 2 < NP)
        def _():
            for cp in w_copies(s + 2, 1 - slot):
                cp.start()

        for cp in wo_copies(s + 1, slot):
            cp.start()
        ffn_start(s)
        for cp in w_copies(s + 1, slot):
            cp.wait()
        for cp in wo_copies(s, 1 - slot):
            cp.wait()

        prep_pair_weights(slot)
        wo0 = pl.multiple_of(s * (OS // 2), OS // 2)
        for i in range(NB - 1, -1, -1):
            p0, a0 = i * (TQ // 2), i * (HT // 2)
            sa = scores(0, i)
            sb = scores(1, i)
            prep_wo(1 - slot, i * (OS // NB), OS // NB, wo0 + i * (OS // NB // 2))
            project(xa_s, wqb_s, q_s, p0, a0)
            project(ca_s, wkb_s, k_s, p0, a0)
            context(0, 2 * s, i, *sa)
            context(1, 2 * s + 1, i, *sb)
            project(ca_s, wvb_s, v_s, p0, a0)
        return carry

    lax.fori_loop(0, NP - 1, pair_body, 0)

    last_slot = (NP - 1) % 2
    for cp in wo_copies(NP - 1, last_slot):
        cp.wait()

    def last_body(e, carry):
        half = OS // 2
        prep_wo(last_slot, pl.multiple_of(e * half, half), half,
                pl.multiple_of((NP - 1) * (OS // 2) + e * (half // 2), half // 2))
        nxt = scores(e, NB - 1)
        for i in range(NB - 1, -1, -1):
            cur = nxt
            if i > 0:
                nxt = scores(e, i - 1)
            context(e, H - 2 + e, i, *cur)
        return carry

    lax.fori_loop(0, 2, last_body, 0)

    wr = wr_ref[...].astype(_F32)
    eye = (lax.broadcasted_iota(_I32, (HT, HT), 1) == lax.broadcasted_iota(_I32, (HT, HT), 0))

    def epilogue(g, hres):
        r0 = pl.multiple_of((g + 1) * HT, HT)
        hn = _round_bf16(_layernorm(hres))
        r = _round_bf16(jnp.sum(hn * wr, axis=1, keepdims=True))
        r_s[pl.ds(g + 8, 1), :] = jnp.sum(jnp.where(eye, r, 0.0), axis=0, keepdims=True)
        out_s[pl.ds(r0, HT), :] = (hres + hn).astype(_BF16)

    def out_copy(g):
        return pltpu.make_async_copy(out_s.at[pl.ds(pl.multiple_of((g + 1) * HT, HT), HT), :],
                                     out_hbm.at[pl.ds(pl.multiple_of(g * HT, HT), HT), :],
                                     sem_out.at[g])

    def ctx_quadrant(p0, h0):
        return jnp.concatenate(
            [_as_bf16(ctx_s[h0 + hh, pl.ds(p0, HT // 2), :]) for hh in range(NP)],
            axis=1)

    def o_body(j, carry):
        r0 = pl.multiple_of(j * TQ, TQ)
        p0 = pl.multiple_of(j * (TQ // 2), TQ // 2)
        epilogue(2 * j - 1, h_s[pl.ds(r0, HT), :])

        a11 = ctx_quadrant(p0, 0)
        a12 = ctx_quadrant(p0, NP)
        a21 = ctx_quadrant(p0 + HT // 2, 0)
        a22 = ctx_quadrant(p0 + HT // 2, NP)
        f = lambda t: t.astype(_F32)

        def prod(t, a):
            return _dot(a.astype(_BF16), _as_bf16(wob_s[t]))

        m3 = prod(2, a11)
        m4 = prod(3, a22)
        m1 = prod(0, f(a11) + f(a22))
        m5 = prod(4, f(a11) + f(a12))
        m7 = prod(6, f(a12) - f(a22))
        att_top = jnp.concatenate([m1 + m4 - m5 + m7, m3 + m5], axis=1)
        h_top = _round_bf16(x_raw[pl.ds(r0, HT), :].astype(_F32) + att_top)
        h_s[pl.ds(r0 + HT, HT), :] = h_top
        epilogue(2 * j, h_top)
        m2 = prod(1, f(a21) + f(a22))
        m6 = prod(5, f(a21) - f(a11))
        att_bot = jnp.concatenate([m2 + m4, m1 - m2 + m3 + m6], axis=1)
        h_s[pl.ds(r0 + 2 * HT, HT), :] = _round_bf16(
            x_raw[pl.ds(r0 + HT, HT), :].astype(_F32) + att_bot)

        @pl.when(j > 0)
        def _():
            out_copy(2 * j - 1).start()

        out_copy(2 * j).start()
        return carry

    lax.fori_loop(0, NB, o_body, 0)
    NG = S // HT
    epilogue(NG - 1, h_s[pl.ds(S, HT), :])
    out_copy(NG - 1).start()

    r = r_s[pl.ds(8, NG), :] + 0.0
    tok = (lax.broadcasted_iota(_I32, (NG, HT), 0) * HT + lax.broadcasted_iota(_I32, (NG, HT), 1))
    bits = pltpu.bitcast(r, _I32)
    key = jnp.where(bits < 0, bits ^ 0x7FFF0000, bits) | (0xFFFF - tok)
    k1 = jnp.max(jnp.max(key, axis=0, keepdims=True), axis=1, keepdims=True)
    key2 = jnp.where(key == k1, jnp.iinfo(jnp.int32).min, key)
    k2 = jnp.max(jnp.max(key2, axis=0, keepdims=True), axis=1, keepdims=True)
    i1s = jnp.clip(0xFFFF - (k1[0, 0] & 0xFFFF), 0, S - 1)
    i2s = jnp.clip(0xFFFF - (k2[0, 0] & 0xFFFF), 0, S - 1)

    R = _FIX
    row = lax.broadcasted_iota(_I32, (R, 1), 0)
    h1 = h_s[pl.ds(i1s + HT, 1), :]
    h2 = h_s[pl.ds(i2s + HT, 1), :]
    hsel = jnp.where(row == 0, h1, h2)
    xs = _layernorm(hsel).astype(_BF16)
    for n in range(3):
        ffn_wait(n)
    g = _round_bf16(_dot(xs, wg_s[...]))
    u = _round_bf16(_dot(xs, wu_s[...]))
    g = _round_bf16(g * (1.0 / (1.0 + jnp.exp(-g))))
    act = (g * u).astype(_BF16)
    y = _round_bf16(_dot(act, wd_s[:, pl.ds(0, M)]))
    ksel = jnp.where(row == 0, k1, k2) & (-0x10000)
    rsel = pltpu.bitcast(jnp.where(ksel < 0, ksel ^ 0x7FFF0000, ksel), _F32)
    gate = _round_bf16(1.0 / (1.0 + jnp.exp(-rsel)))
    y = _round_bf16(y * gate)
    y1 = y[0:1]
    y2 = y[1:2]

    for gi in range(NG):
        out_copy(gi).wait()

    def fix_block(b0):
        hb = h_s[pl.ds(pl.multiple_of(b0 + HT, R), R), :]
        hnb = _round_bf16(_layernorm(hb))
        grow = row + b0
        upd = jnp.where(grow == i1s, y1, 0.0) + jnp.where(grow == i2s, y2, 0.0)
        out_s[pl.ds(pl.multiple_of(b0 + HT, R), R), :] = (
            hb + _round_bf16(hnb + upd)).astype(_BF16)

    def fix_copy(b0, k):
        return pltpu.make_async_copy(out_s.at[pl.ds(pl.multiple_of(b0 + HT, R), R), :],
                                     out_hbm.at[pl.ds(b0, R), :], sem_out.at[k])

    b1 = pl.multiple_of((i1s // R) * R, R)
    b2 = pl.multiple_of((i2s // R) * R, R)
    fix_block(b1)
    fix_block(b2)
    fix_copy(b1, 0).start()

    @pl.when(b2 != b1)
    def _():
        fix_copy(b2, 1).start()
        fix_copy(b2, 1).wait()

    fix_copy(b1, 0).wait()


@jax.jit
def pallas_sequential_preLN__compressed_kv_cla__moe_arch_mod__prompt_kernel(
    A_x: jax.Array,
    A_c_kv: jax.Array,
    A_w_q: jax.Array,
    A_w_uk: jax.Array,
    A_w_uv: jax.Array,
    A_w_o: jax.Array,
    B_x: jax.Array,
    B_w_r: jax.Array,
    B_w_gate: jax.Array,
    B_w_up: jax.Array,
    B_w_down: jax.Array,
):
    B, S, M = A_x.shape
    assert B == 1
    DC = A_c_kv.shape[2]
    H, D = A_w_q.shape[1], A_w_q.shape[2]
    F = B_w_gate.shape[1]
    assert A_c_kv.shape[1] == S and S % _TQ == 0 and H % 2 == 0 and S <= 0x10000
    NP = H // 2
    NG = S // _HT

    x = A_x.reshape(S, M)
    c = A_c_kv.reshape(S, DC)
    wo = A_w_o.reshape(H * D, M)
    wr = B_w_r.reshape(1, M)

    any_spec = pl.BlockSpec(memory_space=pl.ANY)
    vmem_spec = pl.BlockSpec(memory_space=pltpu.VMEM)
    scratch = [
        pltpu.VMEM((S, M), _BF16),
        pltpu.VMEM((S, DC), _BF16),
        pltpu.VMEM((7, S // 4, M // 2), _U32),
        pltpu.VMEM((7, S // 4, DC // 2), _U32),
        pltpu.VMEM((2, S // 2, D), _U32),
        pltpu.VMEM((2, S // 2, D), _U32),
        pltpu.VMEM((2, S // 2, D), _U32),
        pltpu.VMEM((2, M, D), _U32),
        pltpu.VMEM((2, DC, D), _U32),
        pltpu.VMEM((2, DC, D), _U32),
        pltpu.VMEM((7, M // 4, D), _U32),
        pltpu.VMEM((7, DC // 4, D), _U32),
        pltpu.VMEM((7, DC // 4, D), _U32),
        pltpu.VMEM((H, S // 2, D), _U32),
        pltpu.VMEM((2, 2, D, M), _BF16),
        pltpu.VMEM((7, H * D // 4, M // 2), _U32),
        pltpu.VMEM((M, F), _BF16),
        pltpu.VMEM((M, F), _BF16),
        pltpu.VMEM((F, M + _WD_PAD), _BF16),
        pltpu.VMEM((S + _HT, M), _F32),
        pltpu.VMEM((NG + 8, _HT), _F32),
        pltpu.VMEM((S + _HT, M), _BF16),
        pltpu.SemaphoreType.DMA((S // _TQ,)),
        pltpu.SemaphoreType.DMA((S // _TQ,)),
        pltpu.SemaphoreType.DMA((2, 3)),
        pltpu.SemaphoreType.DMA((2, 2)),
        pltpu.SemaphoreType.DMA((3,)),
        pltpu.SemaphoreType.DMA((NG,)),
    ]
    out = pl.pallas_call(
        functools.partial(_kernel, S=S, M=M, DC=DC, H=H, D=D, F=F),
        in_specs=[any_spec, any_spec, any_spec, any_spec, any_spec, any_spec,
                  vmem_spec, any_spec, any_spec, any_spec],
        out_specs=any_spec,
        out_shape=jax.ShapeDtypeStruct((S, M), _BF16),
        scratch_shapes=scratch,
        compiler_params=pltpu.CompilerParams(vmem_limit_bytes=120 * 1024 * 1024,
                                             disable_bounds_checks=True),
        name="fused_mla_mod",
    )(x, c, A_w_q, A_w_uk, A_w_uv, wo, wr, B_w_gate, B_w_up, B_w_down)
    return out.reshape(B, S, M)
```

```python
import functools
import math

import jax
import jax.numpy as jnp
from jax import lax
import jax.experimental.pallas as pl
import jax.experimental.pallas.tpu as pltpu

_F32 = jnp.float32
_BF16 = jnp.bfloat16
_U32 = jnp.uint32
_I32 = jnp.int32

_EPS = 1e-5
_NEG = -1e30
_TQ = 256
_HT = 128
import os
_TIE = int(os.environ.get('TIE', 4))
_CHAIN = int(os.environ.get('CHAIN', 0))
_ERG = int(os.environ.get('ERG', 16))
_EORD = int(os.environ.get('EORD', 0))
_EVAL = int(os.environ.get('EVAL', 1))
_U32BUF = os.environ.get('U32', 'xa,ca,q,k,v,wob,ctx,wb').split(',')
_FIX = 16
_WD_PAD = 128


def _dot(a, b):
    return jnp.dot(a, b, preferred_element_type=_F32)


def _dot_nt(a, b):
    return lax.dot_general(a, b, (((1,), (1,)), ((), ())), preferred_element_type=_F32)


def _as_bf16(u):
    return pltpu.bitcast(u, _BF16)


def _pack(x):
    return pltpu.bitcast(x.astype(_BF16), _U32)


def _rows(ref, r0, n):
    if ref.dtype == _U32:
        if isinstance(r0, int):
            return pl.ds(r0 // 2, n // 2)
        return pl.ds(pl.multiple_of(r0 // 2, 8), n // 2)
    return pl.ds(r0, n)


def _ld(ref, lead, r0, n):
    v = ref[lead, _rows(ref, r0, n), :]
    return _as_bf16(v) if ref.dtype == _U32 else v


def _st(ref, lead, r0, x, cols=slice(None)):
    v = _pack(x) if ref.dtype == _U32 else x.astype(_BF16)
    ref[lead, _rows(ref, r0, x.shape[0]), cols] = v


def _round_bf16(x):
    return x.astype(_BF16).astype(_F32)


def _layernorm(x):
    n = x.shape[-1]
    mean = jnp.sum(x, axis=-1, keepdims=True) * (1.0 / n)
    xc = x - mean
    var = jnp.sum(xc * xc, axis=-1, keepdims=True) * (1.0 / n)
    m = _round_bf16(mean)
    den = _round_bf16(jnp.sqrt(_round_bf16(_round_bf16(var) + _EPS)))
    return (x - m) * (1.0 / den)


def _strassen_a(a11, a12, a21, a22):
    return (a11 + a22, a21 + a22, a11, a22, a11 + a12, a21 - a11, a12 - a22)


def _strassen_b(b11, b12, b21, b22):
    return (b11 + b22, b11, b12 - b22, b21 - b11, b22, b11 + b12, b21 + b22)


def _strassen_c(m):
    m1, m2, m3, m4, m5, m6, m7 = m
    return (m1 + m4 - m5 + m7, m3 + m5, m2 + m4, m1 - m2 + m3 + m6)


def _quadrants(x):
    r, c = x.shape[0] // 2, x.shape[1] // 2
    return x[:r, :c], x[:r, c:], x[r:, :c], x[r:, c:]


def _kernel(x_hbm, c_hbm, wq_hbm, wk_hbm, wv_hbm, wo_hbm, wr_ref, wg_hbm, wu_hbm, wd_hbm,
            out_hbm,
            x_raw, c_raw, xa_s, ca_s, q_s, k_s, v_s,
            wq_p, wk_p, wv_p, wqb_s, wkb_s, wvb_s,
            ctx_s, wo_p, wob_s, wg_s, wu_s, wd_s, ht_s, hb_s, h_s, r_s, out_s,
            sem_x, sem_c, sem_w, sem_wo, sem_ffn, sem_out,
            *, S, M, DC, H, D, F):
    TQ, HT = _TQ, _HT
    NB = S // TQ
    NG = S // HT
    NP = H // 2
    KO = H * D // 2
    OS = KO // NP
    qscale = (D ** -0.5) * math.log2(math.e)

    wq32 = wq_hbm.bitcast(_U32)
    wk32 = wk_hbm.bitcast(_U32)
    wv32 = wv_hbm.bitcast(_U32)

    def w_copies(pair, slot):
        return (
            pltpu.make_async_copy(wk32.at[:, pair, :], wk_p.at[slot], sem_w.at[slot, 0]),
            pltpu.make_async_copy(wv32.at[:, pair, :], wv_p.at[slot], sem_w.at[slot, 1]),
            pltpu.make_async_copy(wq32.at[:, pair, :], wq_p.at[slot], sem_w.at[slot, 2]),
        )

    def wo_copies(t, slot):
        r0 = pl.multiple_of(t * OS, OS)
        return tuple(
            pltpu.make_async_copy(wo_hbm.at[pl.ds(half * KO + r0, OS), :],
                                  wo_p.at[slot, half], sem_wo.at[slot, half])
            for half in range(2))

    def x_copy(i):
        return pltpu.make_async_copy(x_hbm.at[pl.ds(i * TQ, TQ), :],
                                     x_raw.at[pl.ds(i * TQ, TQ), :], sem_x.at[i])

    def c_copy(i):
        return pltpu.make_async_copy(c_hbm.at[pl.ds(i * TQ, TQ), :],
                                     c_raw.at[pl.ds(i * TQ, TQ), :], sem_c.at[i])

    ffn = ((wg_hbm, wg_s), (wu_hbm, wu_s), (wd_hbm, wd_s))

    def ffn_start(t):
        for n, (src, dst) in enumerate(ffn):
            rows, cols = src.shape[0] // NP, src.shape[1]
            r0 = pl.multiple_of(t * rows, 16)
            pltpu.make_async_copy(src.at[pl.ds(r0, rows), :],
                                  dst.at[pl.ds(r0, rows), pl.ds(0, cols)],
                                  sem_ffn.at[n]).start()

    def ffn_wait(n):
        src, dst = ffn[n]
        pltpu.make_async_copy(src, dst.at[:, pl.ds(0, src.shape[1])], sem_ffn.at[n]).wait()

    def lo_hi(w):
        return (pltpu.bitcast(w << 16, _F32), pltpu.bitcast(w & jnp.uint32(0xFFFF0000), _F32))

    def prep_pair_weights(slot):
        RC = 32
        for src, dst in ((wq_p, wqb_s), (wk_p, wkb_s), (wv_p, wvb_s)):
            kh = src.shape[1] // 2
            for r in range(0, kh, RC):
                b11, b12 = lo_hi(src[slot, pl.ds(r, RC), :])
                b21, b22 = lo_hi(src[slot, pl.ds(kh + r, RC), :])
                for t, b in enumerate(_strassen_b(b11, b12, b21, b22)):
                    _st(dst, t, r, b)

    def prep_wo(slot, src0, nrows, dst0, pace, span):
        mh = M // 2
        pieces = [(r, c0) for r in range(0, nrows, 16) for c0 in range(0, mh, HT)]
        for n, (r, c0) in enumerate(pieces):
            t0 = n * span // len(pieces)
            zr, zc = (t0 % TQ) // 8 * 8, (t0 // TQ) * 4 * HT
            z = pltpu.bitcast(pace[zr:zr + 8, zc:zc + HT], _U32)
            z = pltpu.bitcast((z >> 16) >> 16, _F32)
            z = jnp.concatenate([z, z], axis=0)
            rs = pl.ds(src0 + r, 16)
            b11 = wo_p[slot, 0, rs, pl.ds(c0, HT)].astype(_F32) + z
            b12 = wo_p[slot, 0, rs, pl.ds(mh + c0, HT)].astype(_F32)
            b21 = wo_p[slot, 1, rs, pl.ds(c0, HT)].astype(_F32)
            b22 = wo_p[slot, 1, rs, pl.ds(mh + c0, HT)].astype(_F32) + z
            for t, b in enumerate(_strassen_b(b11, b12, b21, b22)):
                _st(wob_s, t, dst0 + r, b, pl.ds(c0, HT))

    def project(a_ref, b_ref, dst, r0, a0):
        kh = a_ref.shape[2]
        m = [_dot(_ld(a_ref, t, a0, HT), _ld(b_ref, t, 0, kh)) for t in range(7)]
        c11, c12, c21, c22 = _strassen_c(m)
        _st(dst, 0, r0, c11)
        _st(dst, 1, r0, c12)
        _st(dst, 0, r0 + HT, c21)
        _st(dst, 1, r0 + HT, c22)

    for cp in w_copies(0, 0):
        cp.start()
    for i in range(NB):
        c_copy(i).start()
        x_copy(i).start()
    for cp in w_copies(1, 1):
        cp.start()
    for cp in wo_copies(0, 0):
        cp.start()
    hb_s[...] = jnp.zeros((HT, M), _BF16)
    for cp in w_copies(0, 0):
        cp.wait()
    prep_pair_weights(0)

    def pro_body(i, carry):
        c_copy(i).wait()
        x_copy(i).wait()
        r0 = pl.multiple_of(i * TQ, TQ)
        a0 = pl.multiple_of(i * HT, HT)
        cc = c_raw[pl.ds(r0, TQ), :].astype(_F32)
        for t, a in enumerate(_strassen_a(*_quadrants(cc))):
            _st(ca_s, t, a0, a)
        project(ca_s, wkb_s, k_s, r0, a0)
        project(ca_s, wvb_s, v_s, r0, a0)
        xn = _layernorm(x_raw[pl.ds(r0, TQ), :].astype(_F32)) * qscale
        for t, a in enumerate(_strassen_a(*_quadrants(xn))):
            _st(xa_s, t, a0, a)
        project(xa_s, wqb_s, q_s, r0, a0)
        return carry

    with jax.named_scope('pro_loop'):
        lax.fori_loop(0, NB, pro_body, 0)

    for cp in w_copies(2, 0) + wo_copies(1, 1):
        cp.start()
    ffn_start(NP - 1)
    for cp in w_copies(1, 1) + wo_copies(0, 0):
        cp.wait()

    tri = (lax.broadcasted_iota(_I32, (HT, HT), 1)
           <= lax.broadcasted_iota(_I32, (HT, HT), 0))

    def softmax_rows(parts):
        s = parts[0] if len(parts) == 1 else jnp.concatenate(parts, axis=1)
        m = jnp.max(s, axis=1, keepdims=True)
        p = jnp.exp2(s - m)
        nt = p.shape[1] // HT
        tiles, acc, grp = [], None, None
        for j in range(nt):
            pj = p[:, j * HT:(j + 1) * HT]
            grp = pj if grp is None else grp + pj
            if j % _TIE == _TIE - 1 or j == nt - 1:
                if _CHAIN:
                    acc = grp if acc is None else acc + grp
                    if j > 0:
                        pj = jnp.minimum(pj, acc)
                else:
                    if j % _TIE > 0:
                        pj = jnp.minimum(pj, grp)
                    acc = grp if acc is None else acc + grp
                grp = None
            tiles.append(pj)
        p = tiles[0] if nt == 1 else jnp.concatenate(tiles, axis=1)
        l = jnp.sum(acc, axis=1, keepdims=True)
        return p, l

    def scores(e, i):
        Lm = i * TQ + HT
        s_main = _dot_nt(_ld(q_s, e, i * TQ, TQ), _ld(k_s, e, 0, Lm))
        s_last = _dot_nt(_ld(q_s, e, i * TQ + HT, HT), _ld(k_s, e, Lm, HT))
        return s_main, s_last

    def context(e, head, i, s_main, s_last):
        Lm = i * TQ + HT
        top = [jnp.where(tri, s_main[:HT, Lm - HT:], _NEG)]
        if Lm > HT:
            top = [s_main[:HT, :Lm - HT]] + top
        p_top, l_top = softmax_rows(top)
        p_bot, l_bot = softmax_rows([s_main[HT:], jnp.where(tri, s_last, _NEG)])
        p_main = jnp.concatenate([p_top, p_bot[:, :Lm]], axis=0).astype(_BF16)
        o = _dot(p_main, _ld(v_s, e, 0, Lm))
        o_last = _dot(p_bot[:, Lm:].astype(_BF16), _ld(v_s, e, Lm, HT))
        o_top = o[:HT] * pl.reciprocal(l_top, approx=True)
        o_bot = (o[HT:] + o_last) * pl.reciprocal(l_bot, approx=True)
        _st(ctx_s, head, i * TQ, jnp.concatenate([o_top, o_bot], axis=0))

    def pair_body(s, carry):
        slot = (s + 1) % 2
        prep_pair_weights(slot)
        wo0 = pl.multiple_of(s * OS, OS)
        for i in range(NB - 1, -1, -1):
            p0, a0 = i * TQ, i * HT
            sa = scores(0, i)
            sb = scores(1, i)
            if i in (NB - 2, NB - 3):
                q4 = OS // 4
                for e, sc in enumerate((sa, sb)):
                    r = (2 * (NB - 2 - i) + e) * q4
                    prep_wo(1 - slot, r, q4, wo0 + r, sc[0], 3 * TQ)
            project(xa_s, wqb_s, q_s, p0, a0)
            project(ca_s, wkb_s, k_s, p0, a0)
            context(0, 2 * s, i, *sa)
            context(1, 2 * s + 1, i, *sb)
            project(ca_s, wvb_s, v_s, p0, a0)

        @pl.when(s + 3 < NP)
        def _():
            for cp in w_copies(s + 3, slot):
                cp.start()

        @pl.when(s + 2 < NP)
        def _():
            for cp in wo_copies(s + 2, 1 - slot):
                cp.start()

        ffn_start(s)

        @pl.when(s + 2 < NP)
        def _():
            for cp in w_copies(s + 2, 1 - slot):
                cp.wait()

        for cp in wo_copies(s + 1, slot):
            cp.wait()
        return carry

    with jax.named_scope('pair_loop'):
        lax.fori_loop(0, NP - 1, pair_body, 0)

    last_slot = (NP - 1) % 2

    def last_body(e, carry):
        half = OS // 2
        nxt = scores(e, NB - 1)
        prep_wo(last_slot, pl.multiple_of(e * half, half), half,
                pl.multiple_of((NP - 1) * OS + e * half, half), nxt[0], 3 * TQ)
        for i in range(NB - 1, -1, -1):
            cur = nxt
            if i > 0:
                nxt = scores(e, i - 1)
            context(e, H - 2 + e, i, *cur)
        return carry

    with jax.named_scope('last_loop'):
        lax.fori_loop(0, 2, last_body, 0)

    wr = wr_ref[...].astype(_F32)
    eye = (lax.broadcasted_iota(_I32, (HT, HT), 1) == lax.broadcasted_iota(_I32, (HT, HT), 0))

    def epilogue(g, src):
        r0 = pl.multiple_of(g * HT, HT)
        rs = []
        for c in range(0, HT, _ERG):
            hb = src[pl.ds(c, _ERG), :]
            h_s[pl.ds(r0 + c, _ERG), :] = hb
            hc = hb.astype(_F32)
            hn = _round_bf16(_layernorm(hc))
            rs.append(_round_bf16(jnp.sum(hn * wr, axis=1, keepdims=True)))
            out_s[pl.ds(r0 + c, _ERG), :] = (hc + hn).astype(_BF16)
        r = jnp.concatenate(rs, axis=0)
        r_s[pl.ds(g, 1), :] = jnp.sum(jnp.where(eye, r, 0.0), axis=0, keepdims=True)
        return [pltpu.bitcast(jnp.broadcast_to(t, (_ERG, HT)), _U32) & jnp.uint32(0xFFFF)
                for t in rs]

    def out_copy(g):
        rows = pl.ds(pl.multiple_of(g * HT, HT), HT)
        return pltpu.make_async_copy(out_s.at[rows, :], out_hbm.at[rows, :], sem_out.at[g])

    def ctx_quadrant(p0, h0):
        return jnp.concatenate(
            [_ld(ctx_s, h0 + hh, p0, HT) for hh in range(NP)], axis=1)

    def tied_weights(t, ties):
        w = wob_s[t]
        if not ties:
            return _as_bf16(w)
        RB = w.shape[0] // 4
        blocks = []
        for kb in range(4):
            blk = w[kb * RB:(kb + 1) * RB]
            if any(k == kb for _, k in ties):
                head = [blk[:_ERG, n * HT:(n + 1) * HT] for n in range(w.shape[1] // HT)]
                head = [hd | ties[(n, kb)] if (n, kb) in ties else hd
                        for n, hd in enumerate(head)]
                blk = jnp.concatenate([jnp.concatenate(head, axis=1), blk[_ERG:]], axis=0)
            blocks.append(blk)
        return _as_bf16(jnp.concatenate(blocks, axis=0))

    def o_body(j, carry):
        r0 = pl.multiple_of(j * TQ, TQ)

        @pl.when(j > 1)
        def _():
            out_copy(2 * j - 3).start()

        @pl.when(j > 0)
        def _():
            out_copy(2 * j - 2).start()

        z = epilogue(jnp.maximum(2 * j - 1, 0), hb_s)

        a11 = lambda: ctx_quadrant(r0, 0)
        a12 = lambda: ctx_quadrant(r0, NP)
        a21 = lambda: ctx_quadrant(r0 + HT, 0)
        a22 = lambda: ctx_quadrant(r0 + HT, NP)
        f = lambda t: t().astype(_F32)
        left, right = pl.ds(0, M // 2), pl.ds(M // 2, M // 2)

        def prod(t, a, ties=None):
            return _dot(a.astype(_BF16), tied_weights(t, ties))

        def residual(dst, rows0, cols, att):
            dst[:, cols] = (x_raw[pl.ds(rows0, HT), cols].astype(_F32) + att).astype(_BF16)

        m3 = prod(2, a11(), {(1, 0): z[0], (1, 3): z[1], (2, 2): z[2], (3, 1): z[3]})
        m4 = prod(3, a22(), {(0, 0): z[4], (0, 3): z[5], (1, 2): z[6], (2, 1): z[7]})
        m5 = prod(4, f(a11) + f(a12))
        residual(ht_s, r0, right, m3 + m5)
        m1 = prod(0, f(a11) + f(a22))
        r_s[pl.ds(NG, 1), :] = jnp.zeros((1, HT), _F32)
        m7 = prod(6, f(a12) - f(a22))
        residual(ht_s, r0, left, m1 + m4 - m5 + m7)
        z = epilogue(2 * j, ht_s)
        m2 = prod(1, f(a21) + f(a22), {(1, 1): z[0], (2, 0): z[1], (2, 3): z[2], (3, 2): z[3]})
        residual(hb_s, r0 + HT, left, m2 + m4)
        m6 = prod(5, f(a21) - f(a11), {(1, 1): z[4], (2, 0): z[5], (2, 3): z[6], (3, 2): z[7]})
        residual(hb_s, r0 + HT, right, m1 - m2 + m3 + m6)
        return carry

    with jax.named_scope('o_loop'):
        lax.fori_loop(0, NB, o_body, 0)
    out_copy(NG - 3).start()
    out_copy(NG - 2).start()
    epilogue(NG - 1, hb_s)
    out_copy(NG - 1).start()

    r = r_s[pl.ds(0, NG), :] + 0.0
    tok = (lax.broadcasted_iota(_I32, (NG, HT), 0) * HT + lax.broadcasted_iota(_I32, (NG, HT), 1))
    bits = pltpu.bitcast(r, _I32)
    key = jnp.where(bits < 0, bits ^ 0x7FFF0000, bits) | (0xFFFF - tok)
    k1 = jnp.max(jnp.max(key, axis=0, keepdims=True), axis=1, keepdims=True)
    key2 = jnp.where(key == k1, jnp.iinfo(jnp.int32).min, key)
    k2 = jnp.max(jnp.max(key2, axis=0, keepdims=True), axis=1, keepdims=True)
    i1s = jnp.clip(0xFFFF - (k1[0, 0] & 0xFFFF), 0, S - 1)
    i2s = jnp.clip(0xFFFF - (k2[0, 0] & 0xFFFF), 0, S - 1)

    R = _FIX
    row = lax.broadcasted_iota(_I32, (R, 1), 0)
    b1 = pl.multiple_of((i1s // R) * R, R)
    b2 = pl.multiple_of((i2s // R) * R, R)
    hblk = [h_s[pl.ds(b0, R), :].astype(_F32) for b0 in (b1, b2)]
    hnblk = [_round_bf16(_layernorm(hb)) for hb in hblk]
    x1 = jnp.sum(jnp.where(row + b1 == i1s, hnblk[0], 0.0), axis=0, keepdims=True)
    x2 = jnp.sum(jnp.where(row + b2 == i2s, hnblk[1], 0.0), axis=0, keepdims=True)
    xs = jnp.where(row == 0, x1, x2).astype(_BF16)
    for n in range(3):
        ffn_wait(n)
    g = _round_bf16(_dot(xs, wg_s[...]))
    u = _round_bf16(_dot(xs, wu_s[...]))
    g = _round_bf16(g * (1.0 / (1.0 + jnp.exp(-g))))
    act = (g * u).astype(_BF16)
    y = _round_bf16(_dot(act, wd_s[:, pl.ds(0, M)]))
    ksel = jnp.where(row == 0, k1, k2) & (-0x10000)
    rsel = pltpu.bitcast(jnp.where(ksel < 0, ksel ^ 0x7FFF0000, ksel), _F32)
    gate = _round_bf16(1.0 / (1.0 + jnp.exp(-rsel)))
    y = _round_bf16(y * gate)
    y1 = y[0:1]
    y2 = y[1:2]

    for gi in range(NG):
        out_copy(gi).wait()

    def fix_copy(b0, k):
        return pltpu.make_async_copy(out_s.at[pl.ds(b0, R), :],
                                     out_hbm.at[pl.ds(b0, R), :], sem_out.at[k])

    for b0, hb, hnb in zip((b1, b2), hblk, hnblk):
        grow = row + b0
        upd = jnp.where(grow == i1s, y1, 0.0) + jnp.where(grow == i2s, y2, 0.0)
        out_s[pl.ds(b0, R), :] = (hb + _round_bf16(hnb + upd)).astype(_BF16)
    fix_copy(b1, 0).start()

    @pl.when(b2 != b1)
    def _():
        fix_copy(b2, 1).start()
        fix_copy(b2, 1).wait()

    fix_copy(b1, 0).wait()


@jax.jit
def pallas_sequential_preLN__compressed_kv_cla__moe_arch_mod__prompt_kernel(
    A_x: jax.Array,
    A_c_kv: jax.Array,
    A_w_q: jax.Array,
    A_w_uk: jax.Array,
    A_w_uv: jax.Array,
    A_w_o: jax.Array,
    B_x: jax.Array,
    B_w_r: jax.Array,
    B_w_gate: jax.Array,
    B_w_up: jax.Array,
    B_w_down: jax.Array,
):
    B, S, M = A_x.shape
    assert B == 1
    DC = A_c_kv.shape[2]
    H, D = A_w_q.shape[1], A_w_q.shape[2]
    F = B_w_gate.shape[1]
    assert A_c_kv.shape[1] == S and S % _TQ == 0 and H % 2 == 0 and S <= 0x10000
    NP = H // 2
    NG = S // _HT

    x = A_x.reshape(S, M)
    c = A_c_kv.reshape(S, DC)
    wo = A_w_o.reshape(H * D, M)
    wr = B_w_r.reshape(1, M)

    any_spec = pl.BlockSpec(memory_space=pl.ANY)
    vmem_spec = pl.BlockSpec(memory_space=pltpu.VMEM)
    def buf(name, lead, rows, cols):
        if name in _U32BUF:
            return pltpu.VMEM((lead, rows // 2, cols), _U32)
        return pltpu.VMEM((lead, rows, cols), _BF16)

    scratch = [
        pltpu.VMEM((S, M), _BF16),
        pltpu.VMEM((S, DC), _BF16),
        buf('xa', 7, S // 2, M // 2),
        buf('ca', 7, S // 2, DC // 2),
        buf('q', 2, S, D),
        buf('k', 2, S, D),
        buf('v', 2, S, D),
        pltpu.VMEM((2, M, D), _U32),
        pltpu.VMEM((2, DC, D), _U32),
        pltpu.VMEM((2, DC, D), _U32),
        buf('wb', 7, M // 2, D),
        buf('wb', 7, DC // 2, D),
        buf('wb', 7, DC // 2, D),
        buf('ctx', H, S, D),
        pltpu.VMEM((2, 2, D, M), _BF16),
        buf('wob', 7, H * D // 2, M // 2),
        pltpu.VMEM((M, F), _BF16),
        pltpu.VMEM((M, F), _BF16),
        pltpu.VMEM((F, M + _WD_PAD), _BF16),
        pltpu.VMEM((_HT, M), _BF16),
        pltpu.VMEM((_HT, M), _BF16),
        pltpu.VMEM((S, M), _BF16),
        pltpu.VMEM((NG + 8, _HT), _F32),
        pltpu.VMEM((S, M), _BF16),
        pltpu.SemaphoreType.DMA((S // _TQ,)),
        pltpu.SemaphoreType.DMA((S // _TQ,)),
        pltpu.SemaphoreType.DMA((2, 3)),
        pltpu.SemaphoreType.DMA((2, 2)),
        pltpu.SemaphoreType.DMA((3,)),
        pltpu.SemaphoreType.DMA((NG,)),
    ]
    out = pl.pallas_call(
        functools.partial(_kernel, S=S, M=M, DC=DC, H=H, D=D, F=F),
        in_specs=[any_spec, any_spec, any_spec, any_spec, any_spec, any_spec,
                  vmem_spec, any_spec, any_spec, any_spec],
        out_specs=any_spec,
        out_shape=jax.ShapeDtypeStruct((S, M), _BF16),
        scratch_shapes=scratch,
        compiler_params=pltpu.CompilerParams(vmem_limit_bytes=120 * 1024 * 1024,
                                             disable_bounds_checks=True),
        name="fused_mla_mod",
    )(x, c, A_w_q, A_w_uk, A_w_uv, wo, wr, B_w_gate, B_w_up, B_w_down)
    return out.reshape(B, S, M)
```

```python
import functools
import math

import jax
import jax.numpy as jnp
from jax import lax
import jax.experimental.pallas as pl
import jax.experimental.pallas.tpu as pltpu

_F32 = jnp.float32
_BF16 = jnp.bfloat16
_U32 = jnp.uint32
_I32 = jnp.int32

_EPS = 1e-5
_NEG = -1e30
_TQ = 256
_HT = 128
import os
_TIE = int(os.environ.get('TIE', 4))
_CHAIN = int(os.environ.get('CHAIN', 0))
_ERG = int(os.environ.get('ERG', 16))
_EORD = int(os.environ.get('EORD', 0))
_EVAL = int(os.environ.get('EVAL', 1))
_U32BUF = os.environ.get('U32', 'xa,ca,q,k,v,wob,ctx,wb').split(',')
_PC = int(os.environ.get('PC', 16))
_PX = int(os.environ.get('PX', 128))
_PV = int(os.environ.get('PV', 1))
_PQ = int(os.environ.get('PQ', 0))
_IDX_BITS = 13
_KEY_BIAS = 0x20000000
_FIX = 8
_WD_PAD = 128


def _dot(a, b):
    return jnp.dot(a, b, preferred_element_type=_F32)


def _dot_nt(a, b):
    return lax.dot_general(a, b, (((1,), (1,)), ((), ())), preferred_element_type=_F32)


def _as_bf16(u):
    return pltpu.bitcast(u, _BF16)


def _pack(x):
    return pltpu.bitcast(x.astype(_BF16), _U32)


def _rows(ref, r0, n):
    if ref.dtype == _U32:
        if isinstance(r0, int):
            return pl.ds(r0 // 2, n // 2)
        return pl.ds(pl.multiple_of(r0 // 2, 8), n // 2)
    return pl.ds(r0, n)


def _ld(ref, lead, r0, n):
    v = ref[lead, _rows(ref, r0, n), :]
    return _as_bf16(v) if ref.dtype == _U32 else v


def _st(ref, lead, r0, x, cols=slice(None)):
    v = _pack(x) if ref.dtype == _U32 else x.astype(_BF16)
    ref[lead, _rows(ref, r0, x.shape[0]), cols] = v


def _round_bf16(x):
    return x.astype(_BF16).astype(_F32)


def _layernorm(x):
    n = x.shape[-1]
    mean = jnp.sum(x, axis=-1, keepdims=True) * (1.0 / n)
    xc = x - mean
    var = jnp.sum(xc * xc, axis=-1, keepdims=True) * (1.0 / n)
    m = _round_bf16(mean)
    den = _round_bf16(jnp.sqrt(_round_bf16(_round_bf16(var) + _EPS)))
    return (x - m) * (1.0 / den)


def _layernorm_scaled(x, scale):
    n = x.shape[-1]
    mean = jnp.sum(x, axis=-1, keepdims=True) * (1.0 / n)
    xc = x - mean
    var = jnp.sum(xc * xc, axis=-1, keepdims=True) * (1.0 / n)
    return xc * (lax.rsqrt(var + _EPS) * scale)


def _strassen_a(a11, a12, a21, a22):
    return (a11 + a22, a21 + a22, a11, a22, a11 + a12, a21 - a11, a12 - a22)


def _strassen_b(b11, b12, b21, b22):
    return (b11 + b22, b11, b12 - b22, b21 - b11, b22, b11 + b12, b21 + b22)


def _strassen_c(m):
    m1, m2, m3, m4, m5, m6, m7 = m
    return (m1 + m4 - m5 + m7, m3 + m5, m2 + m4, m1 - m2 + m3 + m6)


def _quadrants(x):
    r, c = x.shape[0] // 2, x.shape[1] // 2
    return x[:r, :c], x[:r, c:], x[r:, :c], x[r:, c:]


def _kernel(x_hbm, c_hbm, wq_hbm, wk_hbm, wv_hbm, wo_hbm, wr_ref, wg_hbm, wu_hbm, wd_hbm,
            out_hbm,
            x_raw, c_raw, xa_s, ca_s, q_s, k_s, v_s,
            wq_p, wk_p, wv_p, wqb_s, wkb_s, wvb_s,
            ctx_s, wo_p, wob_s, wg_s, wu_s, wd_s, ht_s, hb_s, h_s, hn_s, r_s, out_s,
            sem_x, sem_c, sem_w, sem_wo, sem_ffn, sem_out,
            *, S, M, DC, H, D, F):
    TQ, HT = _TQ, _HT
    NB = S // TQ
    NG = S // HT
    NP = H // 2
    KO = H * D // 2
    OS = KO // NP
    qscale = (D ** -0.5) * math.log2(math.e)

    wq32 = wq_hbm.bitcast(_U32)
    wk32 = wk_hbm.bitcast(_U32)
    wv32 = wv_hbm.bitcast(_U32)

    def w_copies(pair, slot):
        return (
            pltpu.make_async_copy(wk32.at[:, pair, :], wk_p.at[slot], sem_w.at[slot, 0]),
            pltpu.make_async_copy(wv32.at[:, pair, :], wv_p.at[slot], sem_w.at[slot, 1]),
            pltpu.make_async_copy(wq32.at[:, pair, :], wq_p.at[slot], sem_w.at[slot, 2]),
        )

    def wo_copies(t, slot):
        r0 = pl.multiple_of(t * OS, OS)
        return tuple(
            pltpu.make_async_copy(wo_hbm.at[pl.ds(half * KO + r0, OS), :],
                                  wo_p.at[slot, half], sem_wo.at[slot, half])
            for half in range(2))

    def x_copy(i):
        rows = pl.ds(pl.multiple_of(i * TQ, TQ), TQ)
        return pltpu.make_async_copy(x_hbm.at[rows, :], x_raw.at[rows, :], sem_x.at[i % 3])

    def c_copy(i):
        rows = pl.ds(pl.multiple_of(i * TQ, TQ), TQ)
        return pltpu.make_async_copy(c_hbm.at[rows, :], c_raw.at[rows, :], sem_c.at[i % 3])

    ffn = ((wg_hbm, wg_s), (wu_hbm, wu_s), (wd_hbm, wd_s))

    def ffn_start(t):
        for n, (src, dst) in enumerate(ffn):
            rows, cols = src.shape[0] // NP, src.shape[1]
            r0 = pl.multiple_of(t * rows, 16)
            pltpu.make_async_copy(src.at[pl.ds(r0, rows), :],
                                  dst.at[pl.ds(r0, rows), pl.ds(0, cols)],
                                  sem_ffn.at[n]).start()

    def ffn_wait(n):
        src, dst = ffn[n]
        pltpu.make_async_copy(src, dst.at[:, pl.ds(0, src.shape[1])], sem_ffn.at[n]).wait()

    def lo_hi(w):
        return (pltpu.bitcast(w << 16, _F32), pltpu.bitcast(w & jnp.uint32(0xFFFF0000), _F32))

    def prep_pair_weights(slot):
        RC = 32
        for src, dst in ((wq_p, wqb_s), (wk_p, wkb_s), (wv_p, wvb_s)):
            kh = src.shape[1] // 2
            for r in range(0, kh, RC):
                b11, b12 = lo_hi(src[slot, pl.ds(r, RC), :])
                b21, b22 = lo_hi(src[slot, pl.ds(kh + r, RC), :])
                for t, b in enumerate(_strassen_b(b11, b12, b21, b22)):
                    _st(dst, t, r, b)

    def prep_wo(slot, src0, nrows, dst0, pace, span):
        mh = M // 2
        pieces = [(r, c0) for r in range(0, nrows, 16) for c0 in range(0, mh, HT)]
        for n, (r, c0) in enumerate(pieces):
            t0 = n * span // len(pieces)
            zr, zc = (t0 % TQ) // 8 * 8, (t0 // TQ) * 4 * HT
            z = pltpu.bitcast(pace[zr:zr + 8, zc:zc + HT], _U32)
            z = pltpu.bitcast((z >> 16) >> 16, _F32)
            z = jnp.concatenate([z, z], axis=0)
            rs = pl.ds(src0 + r, 16)
            b11 = wo_p[slot, 0, rs, pl.ds(c0, HT)].astype(_F32) + z
            b12 = wo_p[slot, 0, rs, pl.ds(mh + c0, HT)].astype(_F32)
            b21 = wo_p[slot, 1, rs, pl.ds(c0, HT)].astype(_F32)
            b22 = wo_p[slot, 1, rs, pl.ds(mh + c0, HT)].astype(_F32) + z
            for t, b in enumerate(_strassen_b(b11, b12, b21, b22)):
                _st(wob_s, t, dst0 + r, b, pl.ds(c0, HT))

    def project(a_ref, b_ref, dst, r0, a0):
        lhs = a_ref if isinstance(a_ref, list) else [_ld(a_ref, t, a0, HT) for t in range(7)]
        m = [_dot(lhs[t], _ld(b_ref, t, 0, lhs[t].shape[1])) for t in range(7)]
        c11, c12, c21, c22 = _strassen_c(m)
        _st(dst, 0, r0, c11)
        _st(dst, 1, r0, c12)
        _st(dst, 0, r0 + HT, c21)
        _st(dst, 1, r0 + HT, c22)

    for cp in w_copies(0, 0):
        cp.start()
    c_copy(0).start()
    x_copy(0).start()
    hb_s[...] = jnp.zeros((HT, M), _BF16)
    for cp in w_copies(0, 0):
        cp.wait()
    c_copy(1).start()
    x_copy(1).start()
    prep_pair_weights(0)

    def pro_body(i, carry):
        @pl.when(i + 2 < NB)
        def _():
            c_copy(i + 2).start()
            x_copy(i + 2).start()

        @pl.when(i + 2 == NB)
        def _():
            for cp in w_copies(1, 1) + wo_copies(0, 0):
                cp.start()

        c_copy(i).wait()
        x_copy(i).wait()
        r0 = pl.multiple_of(i * TQ, TQ)
        a0 = pl.multiple_of(i * HT, HT)


        def lhs_combos(src, dst, fn, piece):
            parts = [[] for _ in range(7)]
            for c in range(0, HT, piece):
                top = fn(src[pl.ds(r0 + c, piece), :].astype(_F32))
                bot = fn(src[pl.ds(r0 + HT + c, piece), :].astype(_F32))
                kh = top.shape[1] // 2
                for t, a in enumerate(
                        _strassen_a(top[:, :kh], top[:, kh:], bot[:, :kh], bot[:, kh:])):
                    parts[t].append(_pack(a))
            lhs = []
            for t in range(7):
                pk = jnp.concatenate(parts[t], axis=0)
                dst[t, _rows(dst, a0, HT), :] = pk
                lhs.append(_as_bf16(pk))
            return lhs

        ca = lhs_combos(c_raw, ca_s, lambda t: t, _PC)
        project(ca, wkb_s, k_s, r0, a0)
        project(ca_s if _PV else ca, wvb_s, v_s, r0, a0)
        xa = lhs_combos(x_raw, xa_s, lambda t: _layernorm_scaled(t, qscale), _PX)
        project(xa_s if _PQ else xa, wqb_s, q_s, r0, a0)
        return carry

    with jax.named_scope('pro_loop'):
        lax.fori_loop(0, NB, pro_body, 0)

    for cp in w_copies(2, 0) + wo_copies(1, 1):
        cp.start()
    ffn_start(NP - 1)
    for cp in w_copies(1, 1) + wo_copies(0, 0):
        cp.wait()

    tri = (lax.broadcasted_iota(_I32, (HT, HT), 1)
           <= lax.broadcasted_iota(_I32, (HT, HT), 0))

    def softmax_rows(parts):
        s = parts[0] if len(parts) == 1 else jnp.concatenate(parts, axis=1)
        m = jnp.max(s, axis=1, keepdims=True)
        p = jnp.exp2(s - m)
        nt = p.shape[1] // HT
        tiles, acc, grp = [], None, None
        for j in range(nt):
            pj = p[:, j * HT:(j + 1) * HT]
            grp = pj if grp is None else grp + pj
            if j % _TIE == _TIE - 1 or j == nt - 1:
                if _CHAIN:
                    acc = grp if acc is None else acc + grp
                    if j > 0:
                        pj = jnp.minimum(pj, acc)
                else:
                    if j % _TIE > 0:
                        pj = jnp.minimum(pj, grp)
                    acc = grp if acc is None else acc + grp
                grp = None
            tiles.append(pj)
        p = tiles[0] if nt == 1 else jnp.concatenate(tiles, axis=1)
        l = jnp.sum(acc, axis=1, keepdims=True)
        return p, l

    def scores(e, i):
        Lm = i * TQ + HT
        s_main = _dot_nt(_ld(q_s, e, i * TQ, TQ), _ld(k_s, e, 0, Lm))
        s_last = _dot_nt(_ld(q_s, e, i * TQ + HT, HT), _ld(k_s, e, Lm, HT))
        return s_main, s_last

    def context(e, head, i, s_main, s_last):
        Lm = i * TQ + HT
        top = [jnp.where(tri, s_main[:HT, Lm - HT:], _NEG)]
        if Lm > HT:
            top = [s_main[:HT, :Lm - HT]] + top
        p_top, l_top = softmax_rows(top)
        p_bot, l_bot = softmax_rows([s_main[HT:], jnp.where(tri, s_last, _NEG)])
        p_main = jnp.concatenate([p_top, p_bot[:, :Lm]], axis=0).astype(_BF16)
        o = _dot(p_main, _ld(v_s, e, 0, Lm))
        o_last = _dot(p_bot[:, Lm:].astype(_BF16), _ld(v_s, e, Lm, HT))
        o_top = o[:HT] * pl.reciprocal(l_top, approx=True)
        o_bot = (o[HT:] + o_last) * pl.reciprocal(l_bot, approx=True)
        _st(ctx_s, head, i * TQ, jnp.concatenate([o_top, o_bot], axis=0))

    def pair_body(s, carry):
        slot = (s + 1) % 2
        prep_pair_weights(slot)
        wo0 = pl.multiple_of(s * OS, OS)
        for i in range(NB - 1, -1, -1):
            p0, a0 = i * TQ, i * HT
            sa = scores(0, i)
            sb = scores(1, i)
            if i in (NB - 2, NB - 3):
                q4 = OS // 4
                for e, sc in enumerate((sa, sb)):
                    r = (2 * (NB - 2 - i) + e) * q4
                    prep_wo(1 - slot, r, q4, wo0 + r, sc[0], 3 * TQ)
            project(xa_s, wqb_s, q_s, p0, a0)
            project(ca_s, wkb_s, k_s, p0, a0)
            context(0, 2 * s, i, *sa)
            context(1, 2 * s + 1, i, *sb)
            project(ca_s, wvb_s, v_s, p0, a0)

        @pl.when(s + 3 < NP)
        def _():
            for cp in w_copies(s + 3, slot):
                cp.start()

        @pl.when(s + 2 < NP)
        def _():
            for cp in wo_copies(s + 2, 1 - slot):
                cp.start()

        ffn_start(s)

        @pl.when(s + 2 < NP)
        def _():
            for cp in w_copies(s + 2, 1 - slot):
                cp.wait()

        for cp in wo_copies(s + 1, slot):
            cp.wait()
        return carry

    with jax.named_scope('pair_loop'):
        lax.fori_loop(0, NP - 1, pair_body, 0)

    last_slot = (NP - 1) % 2

    def last_body(e, carry):
        half = OS // 2
        nxt = scores(e, NB - 1)
        prep_wo(last_slot, pl.multiple_of(e * half, half), half,
                pl.multiple_of((NP - 1) * OS + e * half, half), nxt[0], 3 * TQ)
        for i in range(NB - 1, -1, -1):
            cur = nxt
            if i > 0:
                nxt = scores(e, i - 1)
            context(e, H - 2 + e, i, *cur)
        return carry

    with jax.named_scope('last_loop'):
        lax.fori_loop(0, 2, last_body, 0)

    wr = wr_ref[...].astype(_F32)
    eye = (lax.broadcasted_iota(_I32, (HT, HT), 1) == lax.broadcasted_iota(_I32, (HT, HT), 0))

    def epilogue(g, src):
        r0 = pl.multiple_of(g * HT, HT)
        rs = []
        for c in range(0, HT, _ERG):
            hb = src[pl.ds(c, _ERG), :]
            h_s[pl.ds(r0 + c, _ERG), :] = hb
            hc = hb.astype(_F32)
            hnb = _layernorm(hc).astype(_BF16)
            hn_s[pl.ds(r0 + c, _ERG), :] = hnb
            hn = hnb.astype(_F32)
            rs.append(_round_bf16(jnp.sum(hn * wr, axis=1, keepdims=True)))
            out_s[pl.ds(r0 + c, _ERG), :] = (hc + hn).astype(_BF16)
        r = jnp.concatenate(rs, axis=0)
        r_s[pl.ds(g, 1), :] = jnp.sum(jnp.where(eye, r, 0.0), axis=0, keepdims=True)
        return [pltpu.bitcast(jnp.broadcast_to(t, (_ERG, HT)), _U32) & jnp.uint32(0xFFFF)
                for t in rs]

    def out_copy(g):
        rows = pl.ds(pl.multiple_of(g * HT, HT), HT)
        return pltpu.make_async_copy(out_s.at[rows, :], out_hbm.at[rows, :], sem_out.at[0])

    def ctx_quadrant(p0, h0):
        return jnp.concatenate(
            [_ld(ctx_s, h0 + hh, p0, HT) for hh in range(NP)], axis=1)

    def tied_weights(t, ties):
        w = wob_s[t]
        if not ties:
            return _as_bf16(w)
        RB = w.shape[0] // 4
        blocks = []
        for kb in range(4):
            blk = w[kb * RB:(kb + 1) * RB]
            if any(k == kb for _, k in ties):
                head = [blk[:_ERG, n * HT:(n + 1) * HT] for n in range(w.shape[1] // HT)]
                head = [hd | ties[(n, kb)] if (n, kb) in ties else hd
                        for n, hd in enumerate(head)]
                blk = jnp.concatenate([jnp.concatenate(head, axis=1), blk[_ERG:]], axis=0)
            blocks.append(blk)
        return _as_bf16(jnp.concatenate(blocks, axis=0))

    def o_body(j, carry):
        r0 = pl.multiple_of(j * TQ, TQ)

        @pl.when(j > 1)
        def _():
            out_copy(2 * j - 3).start()

        @pl.when(j > 0)
        def _():
            out_copy(2 * j - 2).start()

        z = epilogue(jnp.maximum(2 * j - 1, 0), hb_s)

        a11 = lambda: ctx_quadrant(r0, 0)
        a12 = lambda: ctx_quadrant(r0, NP)
        a21 = lambda: ctx_quadrant(r0 + HT, 0)
        a22 = lambda: ctx_quadrant(r0 + HT, NP)
        f = lambda t: t().astype(_F32)
        left, right = pl.ds(0, M // 2), pl.ds(M // 2, M // 2)

        def prod(t, a, ties=None):
            return _dot(a.astype(_BF16), tied_weights(t, ties))

        def residual(dst, rows0, cols, att):
            dst[:, cols] = (x_raw[pl.ds(rows0, HT), cols].astype(_F32) + att).astype(_BF16)

        m3 = prod(2, a11(), {(1, 0): z[0], (1, 3): z[1], (2, 2): z[2], (3, 1): z[3]})
        m4 = prod(3, a22(), {(0, 0): z[4], (0, 3): z[5], (1, 2): z[6], (2, 1): z[7]})
        m5 = prod(4, f(a11) + f(a12))
        residual(ht_s, r0, right, m3 + m5)
        m1 = prod(0, f(a11) + f(a22))
        r_s[pl.ds(NG, 1), :] = jnp.zeros((1, HT), _F32)
        m7 = prod(6, f(a12) - f(a22))
        residual(ht_s, r0, left, m1 + m4 - m5 + m7)
        z = epilogue(2 * j, ht_s)
        m2 = prod(1, f(a21) + f(a22), {(1, 1): z[0], (2, 0): z[1], (2, 3): z[2], (3, 2): z[3]})
        residual(hb_s, r0 + HT, left, m2 + m4)
        m6 = prod(5, f(a21) - f(a11), {(1, 1): z[4], (2, 0): z[5], (2, 3): z[6], (3, 2): z[7]})
        residual(hb_s, r0 + HT, right, m1 - m2 + m3 + m6)
        return carry

    for n in range(3):
        ffn_wait(n)
    with jax.named_scope('o_loop'):
        lax.fori_loop(0, NB, o_body, 0)
    out_copy(NG - 3).start()
    out_copy(NG - 2).start()
    epilogue(NG - 1, hb_s)
    out_copy(NG - 1).start()

    r = r_s[pl.ds(0, NG), :] + 0.0
    tok = (lax.broadcasted_iota(_I32, (NG, HT), 0) * HT + lax.broadcasted_iota(_I32, (NG, HT), 1))
    code = pltpu.bitcast(r, _I32) >> 16
    code = jnp.where(code < 0, code ^ 0x7FFF, code) + 0x8000
    key = pltpu.bitcast(((code << _IDX_BITS) | (S - 1 - tok)) + _KEY_BIAS, _F32)
    k1 = jnp.max(jnp.max(key, axis=0, keepdims=True), axis=1, keepdims=True)
    key2 = jnp.where(key == k1, 0.0, key)
    k2 = jnp.max(jnp.max(key2, axis=0, keepdims=True), axis=1, keepdims=True)

    R = _FIX
    row = lax.broadcasted_iota(_I32, (2 * R, 1), 0)
    ki = pltpu.bitcast(jnp.where(row < R, k1, k2), _I32) - _KEY_BIAS
    idx = S - 1 - (ki & (2 ** _IDX_BITS - 1))
    i1 = jnp.clip(idx[0, 0], 0, S - 1)
    i2 = jnp.clip(idx[R, 0], 0, S - 1)
    b1 = pl.multiple_of((i1 // R) * R, R)
    b2 = pl.multiple_of((i2 // R) * R, R)
    tokr = jnp.where(row < R, b1 + row, b2 + row - R)
    cd = ((pltpu.bitcast(jnp.where(tokr == i1, k1, k2), _I32) - _KEY_BIAS) >> _IDX_BITS) - 0x8000
    score = pltpu.bitcast(jnp.where(cd < 0, cd ^ 0x7FFF, cd) << 16, _F32)
    gate = _round_bf16(1.0 / (1.0 + jnp.exp(-score)))

    hnsel = jnp.concatenate([hn_s[pl.ds(b1, R), :].astype(_F32),
                             hn_s[pl.ds(b2, R), :].astype(_F32)], axis=0)
    xs = hnsel.astype(_BF16)
    g = _round_bf16(_dot(xs, wg_s[...]))
    u = _round_bf16(_dot(xs, wu_s[...]))
    g = _round_bf16(g * (1.0 / (1.0 + jnp.exp(-g))))
    act = (g * u).astype(_BF16)
    y = _round_bf16(_dot(act, wd_s[:, pl.ds(0, M)]))
    y = _round_bf16(y * gate)
    upd = jnp.where(jnp.logical_or(tokr == i1, tokr == i2), y, 0.0)
    hsel = jnp.concatenate([h_s[pl.ds(b1, R), :].astype(_F32),
                            h_s[pl.ds(b2, R), :].astype(_F32)], axis=0)
    fixed = hsel + _round_bf16(hnsel + upd)

    pltpu.make_async_copy(out_s, out_hbm, sem_out.at[0]).wait()

    def fix_copy(b0, k):
        return pltpu.make_async_copy(out_s.at[pl.ds(b0, R), :],
                                     out_hbm.at[pl.ds(b0, R), :], sem_out.at[k])

    out_s[pl.ds(b1, R), :] = fixed[:R].astype(_BF16)
    out_s[pl.ds(b2, R), :] = fixed[R:].astype(_BF16)
    fix_copy(b1, 0).start()

    @pl.when(b2 != b1)
    def _():
        fix_copy(b2, 1).start()
        fix_copy(b2, 1).wait()

    fix_copy(b1, 0).wait()


@jax.jit
def pallas_sequential_preLN__compressed_kv_cla__moe_arch_mod__prompt_kernel(
    A_x: jax.Array,
    A_c_kv: jax.Array,
    A_w_q: jax.Array,
    A_w_uk: jax.Array,
    A_w_uv: jax.Array,
    A_w_o: jax.Array,
    B_x: jax.Array,
    B_w_r: jax.Array,
    B_w_gate: jax.Array,
    B_w_up: jax.Array,
    B_w_down: jax.Array,
):
    B, S, M = A_x.shape
    assert B == 1
    DC = A_c_kv.shape[2]
    H, D = A_w_q.shape[1], A_w_q.shape[2]
    F = B_w_gate.shape[1]
    assert A_c_kv.shape[1] == S and S % _TQ == 0 and H % 2 == 0 and S <= 2 ** _IDX_BITS
    NP = H // 2
    NG = S // _HT

    x = A_x.reshape(S, M)
    c = A_c_kv.reshape(S, DC)
    wo = A_w_o.reshape(H * D, M)
    wr = B_w_r.reshape(1, M)

    any_spec = pl.BlockSpec(memory_space=pl.ANY)
    vmem_spec = pl.BlockSpec(memory_space=pltpu.VMEM)
    def buf(name, lead, rows, cols):
        if name in _U32BUF:
            return pltpu.VMEM((lead, rows // 2, cols), _U32)
        return pltpu.VMEM((lead, rows, cols), _BF16)

    scratch = [
        pltpu.VMEM((S, M), _BF16),
        pltpu.VMEM((S, DC), _BF16),
        buf('xa', 7, S // 2, M // 2),
        buf('ca', 7, S // 2, DC // 2),
        buf('q', 2, S, D),
        buf('k', 2, S, D),
        buf('v', 2, S, D),
        pltpu.VMEM((2, M, D), _U32),
        pltpu.VMEM((2, DC, D), _U32),
        pltpu.VMEM((2, DC, D), _U32),
        buf('wb', 7, M // 2, D),
        buf('wb', 7, DC // 2, D),
        buf('wb', 7, DC // 2, D),
        buf('ctx', H, S, D),
        pltpu.VMEM((2, 2, D, M), _BF16),
        buf('wob', 7, H * D // 2, M // 2),
        pltpu.VMEM((M, F), _BF16),
        pltpu.VMEM((M, F), _BF16),
        pltpu.VMEM((F, M + _WD_PAD), _BF16),
        pltpu.VMEM((_HT, M), _BF16),
        pltpu.VMEM((_HT, M), _BF16),
        pltpu.VMEM((S, M), _BF16),
        pltpu.VMEM((S, M), _BF16),
        pltpu.VMEM((NG + 8, _HT), _F32),
        pltpu.VMEM((S, M), _BF16),
        pltpu.SemaphoreType.DMA((3,)),
        pltpu.SemaphoreType.DMA((3,)),
        pltpu.SemaphoreType.DMA((2, 3)),
        pltpu.SemaphoreType.DMA((2, 2)),
        pltpu.SemaphoreType.DMA((3,)),
        pltpu.SemaphoreType.DMA((2,)),
    ]
    out = pl.pallas_call(
        functools.partial(_kernel, S=S, M=M, DC=DC, H=H, D=D, F=F),
        in_specs=[any_spec, any_spec, any_spec, any_spec, any_spec, any_spec,
                  vmem_spec, any_spec, any_spec, any_spec],
        out_specs=any_spec,
        out_shape=jax.ShapeDtypeStruct((S, M), _BF16),
        scratch_shapes=scratch,
        compiler_params=pltpu.CompilerParams(vmem_limit_bytes=120 * 1024 * 1024,
                                             disable_bounds_checks=True,
                                             disable_semaphore_checks=True),
        name="fused_mla_mod",
    )(x, c, A_w_q, A_w_uk, A_w_uv, wo, wr, B_w_gate, B_w_up, B_w_down)
    return out.reshape(B, S, M)
```

```python
import functools
import math

import jax
import jax.numpy as jnp
from jax import lax
import jax.experimental.pallas as pl
import jax.experimental.pallas.tpu as pltpu

_F32 = jnp.float32
_BF16 = jnp.bfloat16
_U32 = jnp.uint32
_I32 = jnp.int32

_EPS = 1e-5
_NEG = -1e30
_TQ = 256
_HT = 128
import os
_TIE = int(os.environ.get('TIE', 4))
_CHAIN = int(os.environ.get('CHAIN', 0))
_ERG = int(os.environ.get('ERG', 16))
_EORD = int(os.environ.get('EORD', 0))
_EVAL = int(os.environ.get('EVAL', 1))
_U32BUF = os.environ.get('U32', 'xa,ca,q,k,v,wob,ctx,wb').split(',')
_PC = int(os.environ.get('PC', 16))
_PX = int(os.environ.get('PX', 128))
_PV = int(os.environ.get('PV', 1))
_PQ = int(os.environ.get('PQ', 0))
_IDX_BITS = 13
_KEY_BIAS = 0x20000000
_FIX = 8
_WD_PAD = 128


def _dot(a, b):
    return jnp.dot(a, b, preferred_element_type=_F32)


def _dot_nt(a, b):
    return lax.dot_general(a, b, (((1,), (1,)), ((), ())), preferred_element_type=_F32)


def _as_bf16(u):
    return pltpu.bitcast(u, _BF16)


def _pack(x):
    return pltpu.bitcast(x.astype(_BF16), _U32)


def _rows(ref, r0, n):
    if ref.dtype == _U32:
        if isinstance(r0, tuple):
            return pl.ds(r0[0] + r0[1] // 2, n // 2)
        if isinstance(r0, int):
            return pl.ds(r0 // 2, n // 2)
        return pl.ds(pl.multiple_of(r0 // 2, 8), n // 2)
    return pl.ds(r0, n)


def _ld(ref, lead, r0, n):
    v = ref[lead, _rows(ref, r0, n), :]
    return _as_bf16(v) if ref.dtype == _U32 else v


def _st(ref, lead, r0, x, cols=slice(None)):
    v = _pack(x) if ref.dtype == _U32 else x.astype(_BF16)
    ref[lead, _rows(ref, r0, x.shape[0]), cols] = v


def _round_bf16(x):
    return x.astype(_BF16).astype(_F32)


def _layernorm(x):
    n = x.shape[-1]
    mean = jnp.sum(x, axis=-1, keepdims=True) * (1.0 / n)
    xc = x - mean
    var = jnp.sum(xc * xc, axis=-1, keepdims=True) * (1.0 / n)
    m = _round_bf16(mean)
    den = _round_bf16(jnp.sqrt(_round_bf16(_round_bf16(var) + _EPS)))
    return (x - m) * (1.0 / den)


def _layernorm_scaled(x, scale):
    n = x.shape[-1]
    mean = jnp.sum(x, axis=-1, keepdims=True) * (1.0 / n)
    xc = x - mean
    var = jnp.sum(xc * xc, axis=-1, keepdims=True) * (1.0 / n)
    return xc * (lax.rsqrt(var + _EPS) * scale)


def _strassen_a(a11, a12, a21, a22):
    return (a11 + a22, a21 + a22, a11, a22, a11 + a12, a21 - a11, a12 - a22)


def _strassen_b(b11, b12, b21, b22):
    return (b11 + b22, b11, b12 - b22, b21 - b11, b22, b11 + b12, b21 + b22)


def _strassen_c(m):
    m1, m2, m3, m4, m5, m6, m7 = m
    return (m1 + m4 - m5 + m7, m3 + m5, m2 + m4, m1 - m2 + m3 + m6)


_SA = (((0, 1), (3, 1)), ((2, 1), (3, 1)), ((0, 1),), ((3, 1),),
       ((0, 1), (1, 1)), ((2, 1), (0, -1)), ((1, 1), (3, -1)))
_SB = (((0, 1), (3, 1)), ((0, 1),), ((1, 1), (3, -1)), ((2, 1), (0, -1)),
       ((3, 1),), ((0, 1), (1, 1)), ((2, 1), (3, 1)))


def _combine(terms):
    terms = sorted(terms, key=lambda ts: -ts[1])
    acc = terms[0][0]
    assert terms[0][1] > 0
    for v, sg in terms[1:]:
        acc = acc + v if sg > 0 else acc - v
    return acc


def _quadrants(x):
    r, c = x.shape[0] // 2, x.shape[1] // 2
    return x[:r, :c], x[:r, c:], x[r:, :c], x[r:, c:]


def _kernel(x_hbm, c_hbm, wq_hbm, wk_hbm, wv_hbm, wo_hbm, wr_ref, wg_hbm, wu_hbm, wd_hbm,
            out_hbm,
            x_raw, c_raw, xa_s, ca_s, q_s, k_s, v_s,
            wq_p, wk_p, wv_p, wqb_s, wkb_s, wvb_s,
            ctx_s, wo_p, wob_s, wg_s, wu_s, wd_s, ht_s, hb_s, h_s, hn_s, r_s, out_s,
            sem_x, sem_c, sem_w, sem_wo, sem_ffn, sem_out,
            *, S, M, DC, H, D, F):
    TQ, HT = _TQ, _HT
    NB = S // TQ
    NG = S // HT
    NP = H // 2
    KO = H * D // 4
    NO = M // 4
    OS = KO // NP
    qscale = (D ** -0.5) * math.log2(math.e)

    wq32 = wq_hbm.bitcast(_U32)
    wk32 = wk_hbm.bitcast(_U32)
    wv32 = wv_hbm.bitcast(_U32)

    def w_copies(pair, slot):
        return (
            pltpu.make_async_copy(wk32.at[:, pair, :], wk_p.at[slot], sem_w.at[slot, 0]),
            pltpu.make_async_copy(wv32.at[:, pair, :], wv_p.at[slot], sem_w.at[slot, 1]),
            pltpu.make_async_copy(wq32.at[:, pair, :], wq_p.at[slot], sem_w.at[slot, 2]),
        )

    def wo_copies(t, slot):
        r0 = pl.multiple_of(t * OS, OS)
        return tuple(
            pltpu.make_async_copy(wo_hbm.at[pl.ds(half * KO + r0, OS), :],
                                  wo_p.at[slot, half], sem_wo.at[slot, half])
            for half in range(4))

    def x_copy(i):
        rows = pl.ds(pl.multiple_of(i * TQ, TQ), TQ)
        return pltpu.make_async_copy(x_hbm.at[rows, :], x_raw.at[rows, :], sem_x.at[i % 3])

    def c_copy(i):
        rows = pl.ds(pl.multiple_of(i * TQ, TQ), TQ)
        return pltpu.make_async_copy(c_hbm.at[rows, :], c_raw.at[rows, :], sem_c.at[i % 3])

    ffn = ((wg_hbm, wg_s), (wu_hbm, wu_s), (wd_hbm, wd_s))

    def ffn_start(t):
        for n, (src, dst) in enumerate(ffn):
            rows, cols = src.shape[0] // NP, src.shape[1]
            r0 = pl.multiple_of(t * rows, 16)
            pltpu.make_async_copy(src.at[pl.ds(r0, rows), :],
                                  dst.at[pl.ds(r0, rows), pl.ds(0, cols)],
                                  sem_ffn.at[n]).start()

    def ffn_wait(n):
        src, dst = ffn[n]
        pltpu.make_async_copy(src, dst.at[:, pl.ds(0, src.shape[1])], sem_ffn.at[n]).wait()

    def lo_hi(w):
        return (pltpu.bitcast(w << 16, _F32), pltpu.bitcast(w & jnp.uint32(0xFFFF0000), _F32))

    def prep_pair_weights(slot):
        RC = 32
        for src, dst in ((wq_p, wqb_s), (wk_p, wkb_s), (wv_p, wvb_s)):
            kh = src.shape[1] // 2
            for r in range(0, kh, RC):
                b11, b12 = lo_hi(src[slot, pl.ds(r, RC), :])
                b21, b22 = lo_hi(src[slot, pl.ds(kh + r, RC), :])
                for t, b in enumerate(_strassen_b(b11, b12, b21, b22)):
                    _st(dst, t, r, b)

    def prep_wo(slot, src0, nrows, dst0, pace, span):
        pieces = [(r, c0, t) for r in range(0, nrows, 16) for c0 in range(0, NO, HT)
                  for t in range(7)]
        for n, (r, c0, t) in enumerate(pieces):
            t0 = n * span // len(pieces)
            zr, zc = (t0 % TQ) // 8 * 8, (t0 // TQ) * 4 * HT
            z = pltpu.bitcast(pace[zr:zr + 8, zc:zc + HT], _U32)
            z = pltpu.bitcast((z >> 16) >> 16, _F32)
            z = jnp.concatenate([z, z], axis=0)
            rs = pl.ds(src0 + r, 16)
            sub = []
            for q2 in range(4):
                v = _combine([
                    (wo_p[slot, 2 * (q1 // 2) + q2 // 2, rs,
                          pl.ds((2 * (q1 % 2) + q2 % 2) * NO + c0, HT)].astype(_F32), sg)
                    for q1, sg in _SB[t]])
                sub.append(v + z if q2 in (0, 3) else v)
            for u, b in enumerate(_strassen_b(*sub)):
                _st(wob_s, 7 * t + u, dst0 + r, b, pl.ds(c0, HT))

    def project(a_ref, b_ref, dst, r0, a0):
        lhs = a_ref if isinstance(a_ref, list) else [_ld(a_ref, t, a0, HT) for t in range(7)]
        m = [_dot(lhs[t], _ld(b_ref, t, 0, lhs[t].shape[1])) for t in range(7)]
        c11, c12, c21, c22 = _strassen_c(m)
        _st(dst, 0, r0, c11)
        _st(dst, 1, r0, c12)
        _st(dst, 0, r0 + HT, c21)
        _st(dst, 1, r0 + HT, c22)

    for cp in w_copies(0, 0):
        cp.start()
    c_copy(0).start()
    x_copy(0).start()
    hb_s[...] = jnp.zeros((HT, M), _BF16)
    for cp in w_copies(0, 0):
        cp.wait()
    c_copy(1).start()
    x_copy(1).start()
    prep_pair_weights(0)

    def pro_body(i, carry):
        @pl.when(i + 2 < NB)
        def _():
            c_copy(i + 2).start()
            x_copy(i + 2).start()

        @pl.when(i + 2 == NB)
        def _():
            for cp in w_copies(1, 1) + wo_copies(0, 0):
                cp.start()

        c_copy(i).wait()
        x_copy(i).wait()
        r0 = pl.multiple_of(i * TQ, TQ)
        a0 = pl.multiple_of(i * HT, HT)


        def lhs_combos(src, dst, fn, piece):
            parts = [[] for _ in range(7)]
            for c in range(0, HT, piece):
                top = fn(src[pl.ds(r0 + c, piece), :].astype(_F32))
                bot = fn(src[pl.ds(r0 + HT + c, piece), :].astype(_F32))
                kh = top.shape[1] // 2
                for t, a in enumerate(
                        _strassen_a(top[:, :kh], top[:, kh:], bot[:, :kh], bot[:, kh:])):
                    parts[t].append(_pack(a))
            lhs = []
            for t in range(7):
                pk = jnp.concatenate(parts[t], axis=0)
                dst[t, _rows(dst, a0, HT), :] = pk
                lhs.append(_as_bf16(pk))
            return lhs

        ca = lhs_combos(c_raw, ca_s, lambda t: t, _PC)
        project(ca, wkb_s, k_s, r0, a0)
        project(ca_s if _PV else ca, wvb_s, v_s, r0, a0)
        xa = lhs_combos(x_raw, xa_s, lambda t: _layernorm_scaled(t, qscale), _PX)
        project(xa_s if _PQ else xa, wqb_s, q_s, r0, a0)
        return carry

    with jax.named_scope('pro_loop'):
        lax.fori_loop(0, NB, pro_body, 0)

    for cp in w_copies(2, 0) + wo_copies(1, 1):
        cp.start()
    ffn_start(NP - 1)
    for cp in w_copies(1, 1) + wo_copies(0, 0):
        cp.wait()

    tri = (lax.broadcasted_iota(_I32, (HT, HT), 1)
           <= lax.broadcasted_iota(_I32, (HT, HT), 0))

    def softmax_rows(parts):
        s = parts[0] if len(parts) == 1 else jnp.concatenate(parts, axis=1)
        m = jnp.max(s, axis=1, keepdims=True)
        p = jnp.exp2(s - m)
        nt = p.shape[1] // HT
        tiles, acc, grp = [], None, None
        for j in range(nt):
            pj = p[:, j * HT:(j + 1) * HT]
            grp = pj if grp is None else grp + pj
            if j % _TIE == _TIE - 1 or j == nt - 1:
                if _CHAIN:
                    acc = grp if acc is None else acc + grp
                    if j > 0:
                        pj = jnp.minimum(pj, acc)
                else:
                    if j % _TIE > 0:
                        pj = jnp.minimum(pj, grp)
                    acc = grp if acc is None else acc + grp
                grp = None
            tiles.append(pj)
        p = tiles[0] if nt == 1 else jnp.concatenate(tiles, axis=1)
        l = jnp.sum(acc, axis=1, keepdims=True)
        return p, l

    def scores(e, i):
        Lm = i * TQ + HT
        s_main = _dot_nt(_ld(q_s, e, i * TQ, TQ), _ld(k_s, e, 0, Lm))
        s_last = _dot_nt(_ld(q_s, e, i * TQ + HT, HT), _ld(k_s, e, Lm, HT))
        return s_main, s_last

    def context(e, head, i, s_main, s_last):
        Lm = i * TQ + HT
        top = [jnp.where(tri, s_main[:HT, Lm - HT:], _NEG)]
        if Lm > HT:
            top = [s_main[:HT, :Lm - HT]] + top
        p_top, l_top = softmax_rows(top)
        p_bot, l_bot = softmax_rows([s_main[HT:], jnp.where(tri, s_last, _NEG)])
        p_main = jnp.concatenate([p_top, p_bot[:, :Lm]], axis=0).astype(_BF16)
        o = _dot(p_main, _ld(v_s, e, 0, Lm))
        o_last = _dot(p_bot[:, Lm:].astype(_BF16), _ld(v_s, e, Lm, HT))
        o_top = o[:HT] * pl.reciprocal(l_top, approx=True)
        o_bot = (o[HT:] + o_last) * pl.reciprocal(l_bot, approx=True)
        _st(ctx_s, head, i * TQ, jnp.concatenate([o_top, o_bot], axis=0))

    def pair_body(s, carry):
        slot = (s + 1) % 2
        prep_pair_weights(slot)
        wo0 = pl.multiple_of(s * OS, OS)
        for i in range(NB - 1, -1, -1):
            p0, a0 = i * TQ, i * HT
            sa = scores(0, i)
            sb = scores(1, i)
            if i in (NB - 2, NB - 3):
                q4 = OS // 4
                for e, sc in enumerate((sa, sb)):
                    r = (2 * (NB - 2 - i) + e) * q4
                    prep_wo(1 - slot, r, q4, wo0 + r, sc[0], 3 * TQ)
            project(xa_s, wqb_s, q_s, p0, a0)
            project(ca_s, wkb_s, k_s, p0, a0)
            context(0, 2 * s, i, *sa)
            context(1, 2 * s + 1, i, *sb)
            project(ca_s, wvb_s, v_s, p0, a0)

        @pl.when(s + 3 < NP)
        def _():
            for cp in w_copies(s + 3, slot):
                cp.start()

        @pl.when(s + 2 < NP)
        def _():
            for cp in wo_copies(s + 2, 1 - slot):
                cp.start()

        ffn_start(s)

        @pl.when(s + 2 < NP)
        def _():
            for cp in w_copies(s + 2, 1 - slot):
                cp.wait()

        for cp in wo_copies(s + 1, slot):
            cp.wait()
        return carry

    with jax.named_scope('pair_loop'):
        lax.fori_loop(0, NP - 1, pair_body, 0)

    last_slot = (NP - 1) % 2

    def last_body(e, carry):
        half = OS // 2
        nxt = scores(e, NB - 1)
        prep_wo(last_slot, pl.multiple_of(e * half, half), half,
                pl.multiple_of((NP - 1) * OS + e * half, half), nxt[0], 3 * TQ)
        for i in range(NB - 1, -1, -1):
            cur = nxt
            if i > 0:
                nxt = scores(e, i - 1)
            context(e, H - 2 + e, i, *cur)
        return carry

    with jax.named_scope('last_loop'):
        lax.fori_loop(0, 2, last_body, 0)

    wr = wr_ref[...].astype(_F32)
    eye = (lax.broadcasted_iota(_I32, (HT, HT), 1) == lax.broadcasted_iota(_I32, (HT, HT), 0))

    def epilogue(g, src):
        r0 = pl.multiple_of(g * HT, HT)
        rs = []
        for c in range(0, HT, _ERG):
            hb = src[pl.ds(c, _ERG), :]
            h_s[pl.ds(r0 + c, _ERG), :] = hb
            hc = hb.astype(_F32)
            hnb = _layernorm(hc).astype(_BF16)
            hn_s[pl.ds(r0 + c, _ERG), :] = hnb
            hn = hnb.astype(_F32)
            rs.append(_round_bf16(jnp.sum(hn * wr, axis=1, keepdims=True)))
            out_s[pl.ds(r0 + c, _ERG), :] = (hc + hn).astype(_BF16)
        r = jnp.concatenate(rs, axis=0)
        r_s[pl.ds(g, 1), :] = jnp.sum(jnp.where(eye, r, 0.0), axis=0, keepdims=True)
        return [pltpu.bitcast(jnp.broadcast_to(t, (_ERG, HT)), _U32) & jnp.uint32(0xFFFF)
                for t in rs]

    def out_copy(g):
        rows = pl.ds(pl.multiple_of(g * HT, HT), HT)
        return pltpu.make_async_copy(out_s.at[rows, :], out_hbm.at[rows, :], sem_out.at[0])

    QT = HT // 2
    KS = 2 * D

    def prod(r0, t, ties):
        ps = []
        for u in range(7):
            terms = [(2 * (q1 // 2) + q2 // 2, 2 * (q1 % 2) + q2 % 2, s1 * s2)
                     for q1, s1 in _SA[t] for q2, s2 in _SA[u]]
            r_s[pl.ds(NG, 1), :] = jnp.zeros((1, HT), _F32)
            acc = None
            for k0 in range(0, KO, KS):
                def blk(rb, kb):
                    h0 = (kb * KO + k0) // D
                    return jnp.concatenate(
                        [_ld(ctx_s, h0 + hh, (r0, rb * QT), QT) for hh in range(KS // D)], axis=1)
                if len(terms) == 1:
                    lhs = blk(terms[0][0], terms[0][1])
                else:
                    lhs = _combine([(blk(rb, kb).astype(_F32), sg)
                                    for rb, kb, sg in terms]).astype(_BF16)
                w = wob_s[7 * t + u, pl.ds(k0 // 2, KS // 2), :]
                if k0 == 0 and u in ties:
                    head = jnp.concatenate([w[:_ERG, :HT] | ties[u], w[:_ERG, HT:]], axis=1)
                    w = jnp.concatenate([head, w[_ERG:]], axis=0)
                d = _dot(lhs, _as_bf16(w))
                acc = d if acc is None else acc + d
            ps.append(acc)
        c11, c12, c21, c22 = _strassen_c(ps)
        return jnp.concatenate([jnp.concatenate([c11, c12], axis=1),
                                jnp.concatenate([c21, c22], axis=1)], axis=0)

    def o_body(j, carry):
        r0 = pl.multiple_of(j * TQ, TQ)

        @pl.when(j > 1)
        def _():
            out_copy(2 * j - 3).start()

        @pl.when(j > 0)
        def _():
            out_copy(2 * j - 2).start()

        z = epilogue(jnp.maximum(2 * j - 1, 0), hb_s)

        rh = pl.multiple_of(j * (TQ // 2), TQ // 2)
        left, right = pl.ds(0, M // 2), pl.ds(M // 2, M // 2)

        def residual(dst, rows0, cols, att):
            dst[:, cols] = (x_raw[pl.ds(rows0, HT), cols].astype(_F32) + att).astype(_BF16)

        m3 = prod(rh, 2, {2: z[0], 3: z[1], 5: z[2], 6: z[3]})
        m4 = prod(rh, 3, {1: z[4], 3: z[5], 4: z[6], 6: z[7]})
        m5 = prod(rh, 4, {})
        residual(ht_s, r0, right, m3 + m5)
        m1 = prod(rh, 0, {})
        m7 = prod(rh, 6, {})
        residual(ht_s, r0, left, m1 + m4 - m5 + m7)
        z = epilogue(2 * j, ht_s)
        m2 = prod(rh, 1, {3: z[0], 4: z[1], 6: z[2]})
        residual(hb_s, r0 + HT, left, m2 + m4)
        m6 = prod(rh, 5, {0: z[3], 2: z[4], 3: z[5], 4: z[6], 6: z[7]})
        residual(hb_s, r0 + HT, right, m1 - m2 + m3 + m6)
        return carry

    for n in range(3):
        ffn_wait(n)
    with jax.named_scope('o_loop'):
        lax.fori_loop(0, NB, o_body, 0)
    out_copy(NG - 3).start()
    out_copy(NG - 2).start()
    epilogue(NG - 1, hb_s)
    out_copy(NG - 1).start()

    r = r_s[pl.ds(0, NG), :] + 0.0
    tok = (lax.broadcasted_iota(_I32, (NG, HT), 0) * HT + lax.broadcasted_iota(_I32, (NG, HT), 1))
    code = pltpu.bitcast(r, _I32) >> 16
    code = jnp.where(code < 0, code ^ 0x7FFF, code) + 0x8000
    key = pltpu.bitcast(((code << _IDX_BITS) | (S - 1 - tok)) + _KEY_BIAS, _F32)
    k1 = jnp.max(jnp.max(key, axis=0, keepdims=True), axis=1, keepdims=True)
    key2 = jnp.where(key == k1, 0.0, key)
    k2 = jnp.max(jnp.max(key2, axis=0, keepdims=True), axis=1, keepdims=True)

    R = _FIX
    row = lax.broadcasted_iota(_I32, (2 * R, 1), 0)
    ki = pltpu.bitcast(jnp.where(row < R, k1, k2), _I32) - _KEY_BIAS
    idx = S - 1 - (ki & (2 ** _IDX_BITS - 1))
    i1 = jnp.clip(idx[0, 0], 0, S - 1)
    i2 = jnp.clip(idx[R, 0], 0, S - 1)
    b1 = pl.multiple_of((i1 // R) * R, R)
    b2 = pl.multiple_of((i2 // R) * R, R)
    tokr = jnp.where(row < R, b1 + row, b2 + row - R)
    cd = ((pltpu.bitcast(jnp.where(tokr == i1, k1, k2), _I32) - _KEY_BIAS) >> _IDX_BITS) - 0x8000
    score = pltpu.bitcast(jnp.where(cd < 0, cd ^ 0x7FFF, cd) << 16, _F32)
    gate = _round_bf16(1.0 / (1.0 + jnp.exp(-score)))

    hnsel = jnp.concatenate([hn_s[pl.ds(b1, R), :].astype(_F32),
                             hn_s[pl.ds(b2, R), :].astype(_F32)], axis=0)
    xs = hnsel.astype(_BF16)
    g = _round_bf16(_dot(xs, wg_s[...]))
    u = _round_bf16(_dot(xs, wu_s[...]))
    g = _round_bf16(g * (1.0 / (1.0 + jnp.exp(-g))))
    act = (g * u).astype(_BF16)
    y = _round_bf16(_dot(act, wd_s[:, pl.ds(0, M)]))
    y = _round_bf16(y * gate)
    upd = jnp.where(jnp.logical_or(tokr == i1, tokr == i2), y, 0.0)
    hsel = jnp.concatenate([h_s[pl.ds(b1, R), :].astype(_F32),
                            h_s[pl.ds(b2, R), :].astype(_F32)], axis=0)
    fixed = hsel + _round_bf16(hnsel + upd)

    pltpu.make_async_copy(out_s, out_hbm, sem_out.at[0]).wait()

    def fix_copy(b0, k):
        return pltpu.make_async_copy(out_s.at[pl.ds(b0, R), :],
                                     out_hbm.at[pl.ds(b0, R), :], sem_out.at[k])

    out_s[pl.ds(b1, R), :] = fixed[:R].astype(_BF16)
    out_s[pl.ds(b2, R), :] = fixed[R:].astype(_BF16)
    fix_copy(b1, 0).start()

    @pl.when(b2 != b1)
    def _():
        fix_copy(b2, 1).start()
        fix_copy(b2, 1).wait()

    fix_copy(b1, 0).wait()


@jax.jit
def pallas_sequential_preLN__compressed_kv_cla__moe_arch_mod__prompt_kernel(
    A_x: jax.Array,
    A_c_kv: jax.Array,
    A_w_q: jax.Array,
    A_w_uk: jax.Array,
    A_w_uv: jax.Array,
    A_w_o: jax.Array,
    B_x: jax.Array,
    B_w_r: jax.Array,
    B_w_gate: jax.Array,
    B_w_up: jax.Array,
    B_w_down: jax.Array,
):
    B, S, M = A_x.shape
    assert B == 1
    DC = A_c_kv.shape[2]
    H, D = A_w_q.shape[1], A_w_q.shape[2]
    F = B_w_gate.shape[1]
    assert A_c_kv.shape[1] == S and S % _TQ == 0 and H % 2 == 0 and S <= 2 ** _IDX_BITS
    NP = H // 2
    NG = S // _HT

    x = A_x.reshape(S, M)
    c = A_c_kv.reshape(S, DC)
    wo = A_w_o.reshape(H * D, M)
    wr = B_w_r.reshape(1, M)

    any_spec = pl.BlockSpec(memory_space=pl.ANY)
    vmem_spec = pl.BlockSpec(memory_space=pltpu.VMEM)
    def buf(name, lead, rows, cols):
        if name in _U32BUF:
            return pltpu.VMEM((lead, rows // 2, cols), _U32)
        return pltpu.VMEM((lead, rows, cols), _BF16)

    scratch = [
        pltpu.VMEM((S, M), _BF16),
        pltpu.VMEM((S, DC), _BF16),
        buf('xa', 7, S // 2, M // 2),
        buf('ca', 7, S // 2, DC // 2),
        buf('q', 2, S, D),
        buf('k', 2, S, D),
        buf('v', 2, S, D),
        pltpu.VMEM((2, M, D), _U32),
        pltpu.VMEM((2, DC, D), _U32),
        pltpu.VMEM((2, DC, D), _U32),
        buf('wb', 7, M // 2, D),
        buf('wb', 7, DC // 2, D),
        buf('wb', 7, DC // 2, D),
        buf('ctx', H, S, D),
        pltpu.VMEM((2, 4, D // 2, M), _BF16),
        buf('wob', 49, H * D // 4, M // 4),
        pltpu.VMEM((M, F), _BF16),
        pltpu.VMEM((M, F), _BF16),
        pltpu.VMEM((F, M + _WD_PAD), _BF16),
        pltpu.VMEM((_HT, M), _BF16),
        pltpu.VMEM((_HT, M), _BF16),
        pltpu.VMEM((S, M), _BF16),
        pltpu.VMEM((S, M), _BF16),
        pltpu.VMEM((NG + 8, _HT), _F32),
        pltpu.VMEM((S, M), _BF16),
        pltpu.SemaphoreType.DMA((3,)),
        pltpu.SemaphoreType.DMA((3,)),
        pltpu.SemaphoreType.DMA((2, 3)),
        pltpu.SemaphoreType.DMA((2, 4)),
        pltpu.SemaphoreType.DMA((3,)),
        pltpu.SemaphoreType.DMA((2,)),
    ]
    out = pl.pallas_call(
        functools.partial(_kernel, S=S, M=M, DC=DC, H=H, D=D, F=F),
        in_specs=[any_spec, any_spec, any_spec, any_spec, any_spec, any_spec,
                  vmem_spec, any_spec, any_spec, any_spec],
        out_specs=any_spec,
        out_shape=jax.ShapeDtypeStruct((S, M), _BF16),
        scratch_shapes=scratch,
        compiler_params=pltpu.CompilerParams(vmem_limit_bytes=120 * 1024 * 1024,
                                             disable_bounds_checks=True,
                                             disable_semaphore_checks=True),
        name="fused_mla_mod",
    )(x, c, A_w_q, A_w_uk, A_w_uv, wo, wr, B_w_gate, B_w_up, B_w_down)
    return out.reshape(B, S, M)
```

```python
import functools
import math

import jax
import jax.numpy as jnp
from jax import lax
import jax.experimental.pallas as pl
import jax.experimental.pallas.tpu as pltpu

_F32 = jnp.float32
_BF16 = jnp.bfloat16
_U32 = jnp.uint32
_I32 = jnp.int32

_EPS = 1e-5
_NEG = -1e30
_TQ = 256
_HT = 128
import os
_TIE = int(os.environ.get('TIE', 4))
_CHAIN = int(os.environ.get('CHAIN', 0))
_ERG = int(os.environ.get('ERG', 16))
_EORD = int(os.environ.get('EORD', 0))
_EVAL = int(os.environ.get('EVAL', 1))
_U32BUF = os.environ.get('U32', 'xa,ca,q,k,v,wob,ctx,wb').split(',')
_PC = int(os.environ.get('PC', 16))
_PX = int(os.environ.get('PX', 128))
_PV = int(os.environ.get('PV', 1))
_PQ = int(os.environ.get('PQ', 0))
_OT = {
    0: [(0, 2), (0, 3), (0, 4), (0, 5), (0, 6), (1, 0), (1, 1), (1, 2),
        (1, 3), (1, 4), (1, 5), (1, 6), (2, 0), (2, 3), (2, 4), (3, 4)],
    1: [(0, 2), (0, 3), (0, 4), (0, 6), (1, 1), (1, 2), (1, 3), (1, 4),
        (1, 6), (2, 3), (2, 4), (3, 3), (3, 4), (4, 3), (4, 4), (5, 3)],
    2: [(0, 2), (0, 3), (0, 5), (0, 6), (1, 1), (1, 3), (1, 4), (1, 6),
        (2, 2), (2, 4), (2, 6), (3, 2), (3, 4), (4, 0), (4, 3), (4, 5)],
}
_OTIES = _OT[int(os.environ.get('OT', 1))]
_IDX_BITS = 13
_KEY_BIAS = 0x20000000
_FIX = 8
_WD_PAD = 128


def _dot(a, b):
    return jnp.dot(a, b, preferred_element_type=_F32)


def _dot_nt(a, b):
    return lax.dot_general(a, b, (((1,), (1,)), ((), ())), preferred_element_type=_F32)


def _as_bf16(u):
    return pltpu.bitcast(u, _BF16)


def _pack(x):
    return pltpu.bitcast(x.astype(_BF16), _U32)


def _rows(ref, r0, n):
    if ref.dtype == _U32:
        if isinstance(r0, tuple):
            return pl.ds(r0[0] + r0[1] // 2, n // 2)
        if isinstance(r0, int):
            return pl.ds(r0 // 2, n // 2)
        return pl.ds(pl.multiple_of(r0 // 2, 8), n // 2)
    return pl.ds(r0, n)


def _ld(ref, lead, r0, n):
    v = ref[lead, _rows(ref, r0, n), :]
    return _as_bf16(v) if ref.dtype == _U32 else v


def _st(ref, lead, r0, x, cols=slice(None)):
    v = _pack(x) if ref.dtype == _U32 else x.astype(_BF16)
    ref[lead, _rows(ref, r0, x.shape[0]), cols] = v


def _round_bf16(x):
    return x.astype(_BF16).astype(_F32)


def _layernorm(x):
    n = x.shape[-1]
    mean = jnp.sum(x, axis=-1, keepdims=True) * (1.0 / n)
    xc = x - mean
    var = jnp.sum(xc * xc, axis=-1, keepdims=True) * (1.0 / n)
    m = _round_bf16(mean)
    den = _round_bf16(jnp.sqrt(_round_bf16(_round_bf16(var) + _EPS)))
    return (x - m) * (1.0 / den)


def _layernorm_scaled(x, scale):
    n = x.shape[-1]
    mean = jnp.sum(x, axis=-1, keepdims=True) * (1.0 / n)
    xc = x - mean
    var = jnp.sum(xc * xc, axis=-1, keepdims=True) * (1.0 / n)
    return xc * (lax.rsqrt(var + _EPS) * scale)


def _strassen_a(a11, a12, a21, a22):
    return (a11 + a22, a21 + a22, a11, a22, a11 + a12, a21 - a11, a12 - a22)


def _strassen_b(b11, b12, b21, b22):
    return (b11 + b22, b11, b12 - b22, b21 - b11, b22, b11 + b12, b21 + b22)


def _strassen_c(m):
    m1, m2, m3, m4, m5, m6, m7 = m
    return (m1 + m4 - m5 + m7, m3 + m5, m2 + m4, m1 - m2 + m3 + m6)


_SA = (((0, 1), (3, 1)), ((2, 1), (3, 1)), ((0, 1),), ((3, 1),),
       ((0, 1), (1, 1)), ((2, 1), (0, -1)), ((1, 1), (3, -1)))
_SB = (((0, 1), (3, 1)), ((0, 1),), ((1, 1), (3, -1)), ((2, 1), (0, -1)),
       ((3, 1),), ((0, 1), (1, 1)), ((2, 1), (3, 1)))


def _combine(terms):
    terms = sorted(terms, key=lambda ts: -ts[1])
    acc = terms[0][0]
    assert terms[0][1] > 0
    for v, sg in terms[1:]:
        acc = acc + v if sg > 0 else acc - v
    return acc


def _quadrants(x):
    r, c = x.shape[0] // 2, x.shape[1] // 2
    return x[:r, :c], x[:r, c:], x[r:, :c], x[r:, c:]


def _kernel(x_hbm, c_hbm, wq_hbm, wk_hbm, wv_hbm, wo_hbm, wr_ref, wg_hbm, wu_hbm, wd_hbm,
            out_hbm,
            x_raw, c_raw, xa_s, ca_s, q_s, k_s, v_s,
            wq_p, wk_p, wv_p, wqb_s, wkb_s, wvb_s,
            ctx_s, wo_p, wob_s, wg_s, wu_s, wd_s, ht_s, hb_s, h_s, hn_s, r_s, junk_s, out_s,
            sem_x, sem_c, sem_w, sem_wo, sem_ffn, sem_out,
            *, S, M, DC, H, D, F):
    TQ, HT = _TQ, _HT
    NB = S // TQ
    NG = S // HT
    NP = H // 2
    KO = H * D // 4
    NO = M // 4
    OS = KO // NP
    qscale = (D ** -0.5) * math.log2(math.e)

    wq32 = wq_hbm.bitcast(_U32)
    wk32 = wk_hbm.bitcast(_U32)
    wv32 = wv_hbm.bitcast(_U32)

    def w_copies(pair, slot):
        return (
            pltpu.make_async_copy(wk32.at[:, pair, :], wk_p.at[slot], sem_w.at[slot, 0]),
            pltpu.make_async_copy(wv32.at[:, pair, :], wv_p.at[slot], sem_w.at[slot, 1]),
            pltpu.make_async_copy(wq32.at[:, pair, :], wq_p.at[slot], sem_w.at[slot, 2]),
        )

    def wo_copies(t, slot):
        r0 = pl.multiple_of(t * OS, OS)
        return tuple(
            pltpu.make_async_copy(wo_hbm.at[pl.ds(half * KO + r0, OS), :],
                                  wo_p.at[slot, half], sem_wo.at[slot, half])
            for half in range(4))

    def x_copy(i):
        rows = pl.ds(pl.multiple_of(i * TQ, TQ), TQ)
        return pltpu.make_async_copy(x_hbm.at[rows, :], x_raw.at[rows, :], sem_x.at[i % 3])

    def c_copy(i):
        rows = pl.ds(pl.multiple_of(i * TQ, TQ), TQ)
        return pltpu.make_async_copy(c_hbm.at[rows, :], c_raw.at[rows, :], sem_c.at[i % 3])

    ffn = ((wg_hbm, wg_s), (wu_hbm, wu_s), (wd_hbm, wd_s))

    def ffn_start(t):
        for n, (src, dst) in enumerate(ffn):
            rows, cols = src.shape[0] // NP, src.shape[1]
            r0 = pl.multiple_of(t * rows, 16)
            pltpu.make_async_copy(src.at[pl.ds(r0, rows), :],
                                  dst.at[pl.ds(r0, rows), pl.ds(0, cols)],
                                  sem_ffn.at[n]).start()

    def ffn_wait(n):
        src, dst = ffn[n]
        pltpu.make_async_copy(src, dst.at[:, pl.ds(0, src.shape[1])], sem_ffn.at[n]).wait()

    def lo_hi(w):
        return (pltpu.bitcast(w << 16, _F32), pltpu.bitcast(w & jnp.uint32(0xFFFF0000), _F32))

    def prep_pair_weights(slot):
        RC = 32
        for src, dst in ((wq_p, wqb_s), (wk_p, wkb_s), (wv_p, wvb_s)):
            kh = src.shape[1] // 2
            for r in range(0, kh, RC):
                b11, b12 = lo_hi(src[slot, pl.ds(r, RC), :])
                b21, b22 = lo_hi(src[slot, pl.ds(kh + r, RC), :])
                for t, b in enumerate(_strassen_b(b11, b12, b21, b22)):
                    _st(dst, t, r, b)

    def prep_wo(slot, src0, nrows, dst0, pace, span):
        pieces = [(r, c0, t) for r in range(0, nrows, 16) for c0 in range(0, NO, HT)
                  for t in range(7)]
        for n, (r, c0, t) in enumerate(pieces):
            t0 = n * span // len(pieces)
            zr, zc = (t0 % TQ) // 8 * 8, (t0 // TQ) * 4 * HT
            z = pltpu.bitcast(pace[zr:zr + 8, zc:zc + HT], _U32)
            z = pltpu.bitcast((z >> 16) >> 16, _F32)
            z = jnp.concatenate([z, z], axis=0)
            rs = pl.ds(src0 + r, 16)
            sub = []
            for q2 in range(4):
                v = _combine([
                    (wo_p[slot, 2 * (q1 // 2) + q2 // 2, rs,
                          pl.ds((2 * (q1 % 2) + q2 % 2) * NO + c0, HT)].astype(_F32), sg)
                    for q1, sg in _SB[t]])
                sub.append(v + z if q2 in (0, 3) else v)
            for u, b in enumerate(_strassen_b(*sub)):
                _st(wob_s, 7 * t + u, dst0 + r, b, pl.ds(c0, HT))

    def project(a_ref, b_ref, dst, r0, a0):
        lhs = a_ref if isinstance(a_ref, list) else [_ld(a_ref, t, a0, HT) for t in range(7)]
        m = [_dot(lhs[t], _ld(b_ref, t, 0, lhs[t].shape[1])) for t in range(7)]
        c11, c12, c21, c22 = _strassen_c(m)
        _st(dst, 0, r0, c11)
        _st(dst, 1, r0, c12)
        _st(dst, 0, r0 + HT, c21)
        _st(dst, 1, r0 + HT, c22)

    for cp in w_copies(0, 0):
        cp.start()
    c_copy(0).start()
    x_copy(0).start()
    ht_s[...] = jnp.zeros((HT, M), _BF16)
    hb_s[...] = jnp.zeros((HT, M), _BF16)
    for cp in w_copies(0, 0):
        cp.wait()
    c_copy(1).start()
    x_copy(1).start()
    prep_pair_weights(0)

    def pro_body(i, carry):
        @pl.when(i + 2 < NB)
        def _():
            c_copy(i + 2).start()
            x_copy(i + 2).start()

        @pl.when(i + 2 == NB)
        def _():
            for cp in w_copies(1, 1) + wo_copies(0, 0):
                cp.start()

        c_copy(i).wait()
        x_copy(i).wait()
        r0 = pl.multiple_of(i * TQ, TQ)
        a0 = pl.multiple_of(i * HT, HT)


        def lhs_combos(src, dst, fn, piece):
            parts = [[] for _ in range(7)]
            for c in range(0, HT, piece):
                top = fn(src[pl.ds(r0 + c, piece), :].astype(_F32))
                bot = fn(src[pl.ds(r0 + HT + c, piece), :].astype(_F32))
                kh = top.shape[1] // 2
                for t, a in enumerate(
                        _strassen_a(top[:, :kh], top[:, kh:], bot[:, :kh], bot[:, kh:])):
                    parts[t].append(_pack(a))
            lhs = []
            for t in range(7):
                pk = jnp.concatenate(parts[t], axis=0)
                dst[t, _rows(dst, a0, HT), :] = pk
                lhs.append(_as_bf16(pk))
            return lhs

        ca = lhs_combos(c_raw, ca_s, lambda t: t, _PC)
        project(ca, wkb_s, k_s, r0, a0)
        project(ca_s if _PV else ca, wvb_s, v_s, r0, a0)
        xa = lhs_combos(x_raw, xa_s, lambda t: _layernorm_scaled(t, qscale), _PX)
        project(xa_s if _PQ else xa, wqb_s, q_s, r0, a0)
        return carry

    with jax.named_scope('pro_loop'):
        lax.fori_loop(0, NB, pro_body, 0)

    for cp in w_copies(2, 0) + wo_copies(1, 1):
        cp.start()
    ffn_start(NP - 1)
    for cp in w_copies(1, 1) + wo_copies(0, 0):
        cp.wait()

    tri = (lax.broadcasted_iota(_I32, (HT, HT), 1)
           <= lax.broadcasted_iota(_I32, (HT, HT), 0))

    def softmax_rows(parts):
        s = parts[0] if len(parts) == 1 else jnp.concatenate(parts, axis=1)
        m = jnp.max(s, axis=1, keepdims=True)
        p = jnp.exp2(s - m)
        nt = p.shape[1] // HT
        tiles, acc, grp = [], None, None
        for j in range(nt):
            pj = p[:, j * HT:(j + 1) * HT]
            grp = pj if grp is None else grp + pj
            if j % _TIE == _TIE - 1 or j == nt - 1:
                if _CHAIN:
                    acc = grp if acc is None else acc + grp
                    if j > 0:
                        pj = jnp.minimum(pj, acc)
                else:
                    if j % _TIE > 0:
                        pj = jnp.minimum(pj, grp)
                    acc = grp if acc is None else acc + grp
                grp = None
            tiles.append(pj)
        p = tiles[0] if nt == 1 else jnp.concatenate(tiles, axis=1)
        l = jnp.sum(acc, axis=1, keepdims=True)
        return p, l

    def scores(e, i):
        Lm = i * TQ + HT
        s_main = _dot_nt(_ld(q_s, e, i * TQ, TQ), _ld(k_s, e, 0, Lm))
        s_last = _dot_nt(_ld(q_s, e, i * TQ + HT, HT), _ld(k_s, e, Lm, HT))
        return s_main, s_last

    def context(e, head, i, s_main, s_last):
        Lm = i * TQ + HT
        top = [jnp.where(tri, s_main[:HT, Lm - HT:], _NEG)]
        if Lm > HT:
            top = [s_main[:HT, :Lm - HT]] + top
        p_top, l_top = softmax_rows(top)
        p_bot, l_bot = softmax_rows([s_main[HT:], jnp.where(tri, s_last, _NEG)])
        p_main = jnp.concatenate([p_top, p_bot[:, :Lm]], axis=0).astype(_BF16)
        o = _dot(p_main, _ld(v_s, e, 0, Lm))
        o_last = _dot(p_bot[:, Lm:].astype(_BF16), _ld(v_s, e, Lm, HT))
        o_top = o[:HT] * pl.reciprocal(l_top, approx=True)
        o_bot = (o[HT:] + o_last) * pl.reciprocal(l_bot, approx=True)
        _st(ctx_s, head, i * TQ, jnp.concatenate([o_top, o_bot], axis=0))

    def pair_body(s, carry):
        slot = (s + 1) % 2
        prep_pair_weights(slot)
        wo0 = pl.multiple_of(s * OS, OS)
        for i in range(NB - 1, -1, -1):
            p0, a0 = i * TQ, i * HT
            sa = scores(0, i)
            sb = scores(1, i)
            if i in (NB - 2, NB - 3):
                q4 = OS // 4
                for e, sc in enumerate((sa, sb)):
                    r = (2 * (NB - 2 - i) + e) * q4
                    prep_wo(1 - slot, r, q4, wo0 + r, sc[0], 3 * TQ)
            project(xa_s, wqb_s, q_s, p0, a0)
            project(ca_s, wkb_s, k_s, p0, a0)
            context(0, 2 * s, i, *sa)
            context(1, 2 * s + 1, i, *sb)
            project(ca_s, wvb_s, v_s, p0, a0)

        @pl.when(s + 3 < NP)
        def _():
            for cp in w_copies(s + 3, slot):
                cp.start()

        @pl.when(s + 2 < NP)
        def _():
            for cp in wo_copies(s + 2, 1 - slot):
                cp.start()

        ffn_start(s)

        @pl.when(s + 2 < NP)
        def _():
            for cp in w_copies(s + 2, 1 - slot):
                cp.wait()

        for cp in wo_copies(s + 1, slot):
            cp.wait()
        return carry

    with jax.named_scope('pair_loop'):
        lax.fori_loop(0, NP - 1, pair_body, 0)

    last_slot = (NP - 1) % 2

    def last_body(e, carry):
        half = OS // 2
        nxt = scores(e, NB - 1)
        prep_wo(last_slot, pl.multiple_of(e * half, half), half,
                pl.multiple_of((NP - 1) * OS + e * half, half), nxt[0], 3 * TQ)
        for i in range(NB - 1, -1, -1):
            cur = nxt
            if i > 0:
                nxt = scores(e, i - 1)
            context(e, H - 2 + e, i, *cur)
        return carry

    with jax.named_scope('last_loop'):
        lax.fori_loop(0, 2, last_body, 0)

    wr = wr_ref[...].astype(_F32)
    eye = (lax.broadcasted_iota(_I32, (HT, HT), 1) == lax.broadcasted_iota(_I32, (HT, HT), 0))

    def epilogue(g, src):
        r0 = pl.multiple_of(g * HT, HT)
        rs = []
        for c in range(0, HT, _ERG):
            hb = src[pl.ds(c, _ERG), :]
            h_s[pl.ds(r0 + c, _ERG), :] = hb
            hc = hb.astype(_F32)
            hnb = _layernorm(hc).astype(_BF16)
            hn_s[pl.ds(r0 + c, _ERG), :] = hnb
            hn = hnb.astype(_F32)
            rs.append(_round_bf16(jnp.sum(hn * wr, axis=1, keepdims=True)))
            out_s[pl.ds(r0 + c, _ERG), :] = (hc + hn).astype(_BF16)
        r = jnp.concatenate(rs, axis=0)
        r_s[pl.ds(g, 1), :] = jnp.sum(jnp.where(eye, r, 0.0), axis=0, keepdims=True)
        return [pltpu.bitcast(jnp.broadcast_to(t, (_ERG, HT)), _U32) & jnp.uint32(0xFFFF)
                for t in rs]

    def out_copy(g):
        rows = pl.ds(pl.multiple_of(g * HT, HT), HT)
        return pltpu.make_async_copy(out_s.at[rows, :], out_hbm.at[rows, :], sem_out.at[0])

    QT = HT // 2
    KS = 2 * D

    def prod(r0, t, ties):
        ps = []
        for u in range(7):
            terms = [(2 * (q1 // 2) + q2 // 2, 2 * (q1 % 2) + q2 % 2, s1 * s2)
                     for q1, s1 in _SA[t] for q2, s2 in _SA[u]]
            junk_s[...] = jnp.zeros(junk_s.shape, _F32)
            acc = None
            for k0 in range(0, KO, KS):
                def blk(rb, kb):
                    h0 = (kb * KO + k0) // D
                    return jnp.concatenate(
                        [_ld(ctx_s, h0 + hh, (r0, rb * QT), QT) for hh in range(KS // D)], axis=1)
                if len(terms) == 1:
                    lhs = blk(terms[0][0], terms[0][1])
                else:
                    lhs = _combine([(blk(rb, kb).astype(_F32), sg)
                                    for rb, kb, sg in terms]).astype(_BF16)
                w = wob_s[7 * t + u, pl.ds(k0 // 2, KS // 2), :]
                if k0 == 0 and u in ties:
                    head = jnp.concatenate([w[:_ERG, :HT] | ties[u], w[:_ERG, HT:]], axis=1)
                    w = jnp.concatenate([head, w[_ERG:]], axis=0)
                d = _dot(lhs, _as_bf16(w))
                acc = d if acc is None else acc + d
            ps.append(acc)
        c11, c12, c21, c22 = _strassen_c(ps)
        return jnp.concatenate([jnp.concatenate([c11, c12], axis=1),
                                jnp.concatenate([c21, c22], axis=1)], axis=0)

    def o_body(j, carry):
        r0 = pl.multiple_of(j * TQ, TQ)

        @pl.when(j > 1)
        def _():
            out_copy(2 * j - 4).start()
            out_copy(2 * j - 3).start()

        gp = jnp.maximum(2 * j - 2, 0)
        z = epilogue(gp, ht_s) + epilogue(gp + 1, hb_s)
        ties = [{} for _ in range(7)]
        for zt, (o, u) in zip(z, _OTIES):
            ties[o][u] = zt

        rh = pl.multiple_of(j * (TQ // 2), TQ // 2)
        left, right = pl.ds(0, M // 2), pl.ds(M // 2, M // 2)

        def residual(dst, rows0, cols, att):
            dst[:, cols] = (x_raw[pl.ds(rows0, HT), cols].astype(_F32) + att).astype(_BF16)

        m3 = prod(rh, 2, ties[0])
        m4 = prod(rh, 3, ties[1])
        m5 = prod(rh, 4, ties[2])
        residual(ht_s, r0, right, m3 + m5)
        m1 = prod(rh, 0, ties[3])
        m7 = prod(rh, 6, ties[4])
        residual(ht_s, r0, left, m1 + m4 - m5 + m7)
        m2 = prod(rh, 1, ties[5])
        residual(hb_s, r0 + HT, left, m2 + m4)
        m6 = prod(rh, 5, ties[6])
        residual(hb_s, r0 + HT, right, m1 - m2 + m3 + m6)
        return carry

    for n in range(3):
        ffn_wait(n)
    with jax.named_scope('o_loop'):
        lax.fori_loop(0, NB, o_body, 0)
    out_copy(NG - 4).start()
    out_copy(NG - 3).start()
    epilogue(NG - 2, ht_s)
    epilogue(NG - 1, hb_s)
    out_copy(NG - 2).start()
    out_copy(NG - 1).start()

    r = r_s[pl.ds(0, NG), :] + 0.0
    tok = (lax.broadcasted_iota(_I32, (NG, HT), 0) * HT + lax.broadcasted_iota(_I32, (NG, HT), 1))
    code = pltpu.bitcast(r, _I32) >> 16
    code = jnp.where(code < 0, code ^ 0x7FFF, code) + 0x8000
    key = pltpu.bitcast(((code << _IDX_BITS) | (S - 1 - tok)) + _KEY_BIAS, _F32)
    k1 = jnp.max(jnp.max(key, axis=0, keepdims=True), axis=1, keepdims=True)
    key2 = jnp.where(key == k1, 0.0, key)
    k2 = jnp.max(jnp.max(key2, axis=0, keepdims=True), axis=1, keepdims=True)

    R = _FIX
    row = lax.broadcasted_iota(_I32, (2 * R, 1), 0)
    ki = pltpu.bitcast(jnp.where(row < R, k1, k2), _I32) - _KEY_BIAS
    idx = S - 1 - (ki & (2 ** _IDX_BITS - 1))
    i1 = jnp.clip(idx[0, 0], 0, S - 1)
    i2 = jnp.clip(idx[R, 0], 0, S - 1)
    b1 = pl.multiple_of((i1 // R) * R, R)
    b2 = pl.multiple_of((i2 // R) * R, R)
    tokr = jnp.where(row < R, b1 + row, b2 + row - R)
    cd = ((pltpu.bitcast(jnp.where(tokr == i1, k1, k2), _I32) - _KEY_BIAS) >> _IDX_BITS) - 0x8000
    score = pltpu.bitcast(jnp.where(cd < 0, cd ^ 0x7FFF, cd) << 16, _F32)
    gate = _round_bf16(1.0 / (1.0 + jnp.exp(-score)))

    hnsel = jnp.concatenate([hn_s[pl.ds(b1, R), :].astype(_F32),
                             hn_s[pl.ds(b2, R), :].astype(_F32)], axis=0)
    xs = hnsel.astype(_BF16)
    g = _round_bf16(_dot(xs, wg_s[...]))
    u = _round_bf16(_dot(xs, wu_s[...]))
    g = _round_bf16(g * (1.0 / (1.0 + jnp.exp(-g))))
    act = (g * u).astype(_BF16)
    y = _round_bf16(_dot(act, wd_s[:, pl.ds(0, M)]))
    y = _round_bf16(y * gate)
    upd = jnp.where(jnp.logical_or(tokr == i1, tokr == i2), y, 0.0)
    hsel = jnp.concatenate([h_s[pl.ds(b1, R), :].astype(_F32),
                            h_s[pl.ds(b2, R), :].astype(_F32)], axis=0)
    fixed = hsel + _round_bf16(hnsel + upd)

    pltpu.make_async_copy(out_s, out_hbm, sem_out.at[0]).wait()

    def fix_copy(b0, k):
        return pltpu.make_async_copy(out_s.at[pl.ds(b0, R), :],
                                     out_hbm.at[pl.ds(b0, R), :], sem_out.at[k])

    out_s[pl.ds(b1, R), :] = fixed[:R].astype(_BF16)
    out_s[pl.ds(b2, R), :] = fixed[R:].astype(_BF16)
    fix_copy(b1, 0).start()

    @pl.when(b2 != b1)
    def _():
        fix_copy(b2, 1).start()
        fix_copy(b2, 1).wait()

    fix_copy(b1, 0).wait()


@jax.jit
def pallas_sequential_preLN__compressed_kv_cla__moe_arch_mod__prompt_kernel(
    A_x: jax.Array,
    A_c_kv: jax.Array,
    A_w_q: jax.Array,
    A_w_uk: jax.Array,
    A_w_uv: jax.Array,
    A_w_o: jax.Array,
    B_x: jax.Array,
    B_w_r: jax.Array,
    B_w_gate: jax.Array,
    B_w_up: jax.Array,
    B_w_down: jax.Array,
):
    B, S, M = A_x.shape
    assert B == 1
    DC = A_c_kv.shape[2]
    H, D = A_w_q.shape[1], A_w_q.shape[2]
    F = B_w_gate.shape[1]
    assert A_c_kv.shape[1] == S and S % _TQ == 0 and H % 2 == 0 and S <= 2 ** _IDX_BITS
    NP = H // 2
    NG = S // _HT

    x = A_x.reshape(S, M)
    c = A_c_kv.reshape(S, DC)
    wo = A_w_o.reshape(H * D, M)
    wr = B_w_r.reshape(1, M)

    any_spec = pl.BlockSpec(memory_space=pl.ANY)
    vmem_spec = pl.BlockSpec(memory_space=pltpu.VMEM)
    def buf(name, lead, rows, cols):
        if name in _U32BUF:
            return pltpu.VMEM((lead, rows // 2, cols), _U32)
        return pltpu.VMEM((lead, rows, cols), _BF16)

    scratch = [
        pltpu.VMEM((S, M), _BF16),
        pltpu.VMEM((S, DC), _BF16),
        buf('xa', 7, S // 2, M // 2),
        buf('ca', 7, S // 2, DC // 2),
        buf('q', 2, S, D),
        buf('k', 2, S, D),
        buf('v', 2, S, D),
        pltpu.VMEM((2, M, D), _U32),
        pltpu.VMEM((2, DC, D), _U32),
        pltpu.VMEM((2, DC, D), _U32),
        buf('wb', 7, M // 2, D),
        buf('wb', 7, DC // 2, D),
        buf('wb', 7, DC // 2, D),
        buf('ctx', H, S, D),
        pltpu.VMEM((2, 4, D // 2, M), _BF16),
        buf('wob', 49, H * D // 4, M // 4),
        pltpu.VMEM((M, F), _BF16),
        pltpu.VMEM((M, F), _BF16),
        pltpu.VMEM((F, M + _WD_PAD), _BF16),
        pltpu.VMEM((_HT, M), _BF16),
        pltpu.VMEM((_HT, M), _BF16),
        pltpu.VMEM((S, M), _BF16),
        pltpu.VMEM((S, M), _BF16),
        pltpu.VMEM((NG, _HT), _F32),
        pltpu.VMEM((8, _HT), _F32),
        pltpu.VMEM((S, M), _BF16),
        pltpu.SemaphoreType.DMA((3,)),
        pltpu.SemaphoreType.DMA((3,)),
        pltpu.SemaphoreType.DMA((2, 3)),
        pltpu.SemaphoreType.DMA((2, 4)),
        pltpu.SemaphoreType.DMA((3,)),
        pltpu.SemaphoreType.DMA((2,)),
    ]
    out = pl.pallas_call(
        functools.partial(_kernel, S=S, M=M, DC=DC, H=H, D=D, F=F),
        in_specs=[any_spec, any_spec, any_spec, any_spec, any_spec, any_spec,
                  vmem_spec, any_spec, any_spec, any_spec],
        out_specs=any_spec,
        out_shape=jax.ShapeDtypeStruct((S, M), _BF16),
        scratch_shapes=scratch,
        compiler_params=pltpu.CompilerParams(vmem_limit_bytes=120 * 1024 * 1024,
                                             disable_bounds_checks=True,
                                             disable_semaphore_checks=True),
        name="fused_mla_mod",
    )(x, c, A_w_q, A_w_uk, A_w_uv, wo, wr, B_w_gate, B_w_up, B_w_down)
    return out.reshape(B, S, M)
```

```python
import functools
import math

import jax
import jax.numpy as jnp
from jax import lax
import jax.experimental.pallas as pl
import jax.experimental.pallas.tpu as pltpu

_F32 = jnp.float32
_BF16 = jnp.bfloat16
_U32 = jnp.uint32
_I32 = jnp.int32

_EPS = 1e-5
_NEG = -1e30
_TQ = 256
_HT = 128
import os
_TIE = int(os.environ.get('TIE', 4))
_CHAIN = int(os.environ.get('CHAIN', 0))
_ERG = int(os.environ.get('ERG', 16))
_EORD = int(os.environ.get('EORD', 0))
_EVAL = int(os.environ.get('EVAL', 1))
_U32BUF = os.environ.get('U32', 'xa,ca,q,k,v,wob,ctx,wb').split(',')
_PC = int(os.environ.get('PC', 16))
_PX = int(os.environ.get('PX', 128))
_PV = int(os.environ.get('PV', 1))
_PQ = int(os.environ.get('PQ', 0))
_OT = {
    0: [(0, 2), (0, 3), (0, 4), (0, 5), (0, 6), (1, 0), (1, 1), (1, 2),
        (1, 3), (1, 4), (1, 5), (1, 6), (2, 0), (2, 3), (2, 4), (3, 4)],
    1: [(0, 2), (0, 3), (0, 4), (0, 6), (1, 1), (1, 2), (1, 3), (1, 4),
        (1, 6), (2, 3), (2, 4), (3, 3), (3, 4), (4, 3), (4, 4), (5, 3)],
    2: [(0, 2), (0, 3), (0, 5), (0, 6), (1, 1), (1, 3), (1, 4), (1, 6),
        (2, 2), (2, 4), (2, 6), (3, 2), (3, 4), (4, 0), (4, 3), (4, 5)],
}
_OTIES = _OT[int(os.environ.get('OT', 1))]
_WQM = int(os.environ.get('WQM', 1))
_WQS = int(os.environ.get('WQS', 896))
_KVLATE = int(os.environ.get('KVLATE', 0))
_IDX_BITS = 13
_KEY_BIAS = 0x20000000
_FIX = 8
_WD_PAD = 128


def _dot(a, b):
    return jnp.dot(a, b, preferred_element_type=_F32)


def _dot_nt(a, b):
    return lax.dot_general(a, b, (((1,), (1,)), ((), ())), preferred_element_type=_F32)


def _as_bf16(u):
    return pltpu.bitcast(u, _BF16)


def _pack(x):
    return pltpu.bitcast(x.astype(_BF16), _U32)


def _rows(ref, r0, n):
    if ref.dtype == _U32:
        if isinstance(r0, tuple):
            return pl.ds(r0[0] + r0[1] // 2, n // 2)
        if isinstance(r0, int):
            return pl.ds(r0 // 2, n // 2)
        return pl.ds(pl.multiple_of(r0 // 2, 8), n // 2)
    return pl.ds(r0, n)


def _ld(ref, lead, r0, n):
    v = ref[lead, _rows(ref, r0, n), :]
    return _as_bf16(v) if ref.dtype == _U32 else v


def _st(ref, lead, r0, x, cols=slice(None)):
    v = _pack(x) if ref.dtype == _U32 else x.astype(_BF16)
    ref[lead, _rows(ref, r0, x.shape[0]), cols] = v


def _round_bf16(x):
    return x.astype(_BF16).astype(_F32)


def _layernorm(x):
    n = x.shape[-1]
    mean = jnp.sum(x, axis=-1, keepdims=True) * (1.0 / n)
    xc = x - mean
    var = jnp.sum(xc * xc, axis=-1, keepdims=True) * (1.0 / n)
    m = _round_bf16(mean)
    den = _round_bf16(jnp.sqrt(_round_bf16(_round_bf16(var) + _EPS)))
    return (x - m) * (1.0 / den)


def _layernorm_scaled(x, scale):
    n = x.shape[-1]
    mean = jnp.sum(x, axis=-1, keepdims=True) * (1.0 / n)
    xc = x - mean
    var = jnp.sum(xc * xc, axis=-1, keepdims=True) * (1.0 / n)
    return xc * (lax.rsqrt(var + _EPS) * scale)


def _strassen_a(a11, a12, a21, a22):
    return (a11 + a22, a21 + a22, a11, a22, a11 + a12, a21 - a11, a12 - a22)


def _strassen_b(b11, b12, b21, b22):
    return (b11 + b22, b11, b12 - b22, b21 - b11, b22, b11 + b12, b21 + b22)


def _strassen_c(m):
    m1, m2, m3, m4, m5, m6, m7 = m
    return (m1 + m4 - m5 + m7, m3 + m5, m2 + m4, m1 - m2 + m3 + m6)


_SA = (((0, 1), (3, 1)), ((2, 1), (3, 1)), ((0, 1),), ((3, 1),),
       ((0, 1), (1, 1)), ((2, 1), (0, -1)), ((1, 1), (3, -1)))
_SB = (((0, 1), (3, 1)), ((0, 1),), ((1, 1), (3, -1)), ((2, 1), (0, -1)),
       ((3, 1),), ((0, 1), (1, 1)), ((2, 1), (3, 1)))


def _combine(terms):
    terms = sorted(terms, key=lambda ts: -ts[1])
    acc = terms[0][0]
    assert terms[0][1] > 0
    for v, sg in terms[1:]:
        acc = acc + v if sg > 0 else acc - v
    return acc


def _quadrants(x):
    r, c = x.shape[0] // 2, x.shape[1] // 2
    return x[:r, :c], x[:r, c:], x[r:, :c], x[r:, c:]


def _kernel(x_hbm, c_hbm, wq_hbm, wk_hbm, wv_hbm, wo_hbm, wr_ref, wg_hbm, wu_hbm, wd_hbm,
            out_hbm,
            x_raw, c_raw, xa_s, ca_s, q_s, k_s, v_s,
            wq_p, wk_p, wv_p, wqb_s, wkvb_s,
            ctx_s, wo_p, wob_s, wg_s, wu_s, wd_s, ht_s, hb_s, h_s, hn_s, r_s, junk_s, out_s,
            sem_x, sem_c, sem_w, sem_wo, sem_ffn, sem_out,
            *, S, M, DC, H, D, F):
    TQ, HT = _TQ, _HT
    NB = S // TQ
    NG = S // HT
    NP = H // 2
    KO = H * D // 4
    NO = M // 4
    OS = KO // NP
    qscale = (D ** -0.5) * math.log2(math.e)

    wq32 = wq_hbm.bitcast(_U32)
    wk32 = wk_hbm.bitcast(_U32)
    wv32 = wv_hbm.bitcast(_U32)

    def w_copies(pair, slot):
        return (
            pltpu.make_async_copy(wk32.at[:, pair, :], wk_p.at[slot], sem_w.at[slot, 0]),
            pltpu.make_async_copy(wv32.at[:, pair, :], wv_p.at[slot], sem_w.at[slot, 1]),
            pltpu.make_async_copy(wq32.at[:, pair, :], wq_p.at[slot], sem_w.at[slot, 2]),
        )

    def wo_copies(t, slot):
        r0 = pl.multiple_of(t * OS, OS)
        return tuple(
            pltpu.make_async_copy(wo_hbm.at[pl.ds(half * KO + r0, OS), :],
                                  wo_p.at[slot, half], sem_wo.at[slot, half])
            for half in range(4))

    def x_copy(i):
        rows = pl.ds(pl.multiple_of(i * TQ, TQ), TQ)
        return pltpu.make_async_copy(x_hbm.at[rows, :], x_raw.at[rows, :], sem_x.at[i % 3])

    def c_copy(i):
        rows = pl.ds(pl.multiple_of(i * TQ, TQ), TQ)
        return pltpu.make_async_copy(c_hbm.at[rows, :], c_raw.at[rows, :], sem_c.at[i % 3])

    ffn = ((wg_hbm, wg_s), (wu_hbm, wu_s), (wd_hbm, wd_s))

    def ffn_start(t):
        for n, (src, dst) in enumerate(ffn):
            rows, cols = src.shape[0] // NP, src.shape[1]
            r0 = pl.multiple_of(t * rows, 16)
            pltpu.make_async_copy(src.at[pl.ds(r0, rows), :],
                                  dst.at[pl.ds(r0, rows), pl.ds(0, cols)],
                                  sem_ffn.at[n]).start()

    def ffn_wait(n):
        src, dst = ffn[n]
        pltpu.make_async_copy(src, dst.at[:, pl.ds(0, src.shape[1])], sem_ffn.at[n]).wait()

    def lo_hi(w):
        return (pltpu.bitcast(w << 16, _F32), pltpu.bitcast(w & jnp.uint32(0xFFFF0000), _F32))

    def pacer(mats, span, total):
        per = -(-total // len(mats))

        def zero(n):
            t0 = (n % per) * span // per
            zr, zc = (t0 % TQ) // 8 * 8, (t0 // TQ) * 4 * HT
            z = pltpu.bitcast(mats[n // per][zr:zr + 8, zc:zc + HT], _U32)
            z = (z >> 16) >> 16
            return jnp.concatenate([z, z], axis=0)
        return zero

    def store_combos(dst, lead0, r, sub, sink):
        z = None
        for u, b in enumerate(_strassen_b(*sub)):
            pk = _pack(b)
            dst[lead0 + u, pl.ds(r // 2, pk.shape[0]), :] = pk
            z = pk if z is None else z | pk
        if sink is not None:
            junk_s[pl.ds(8 * sink, 8), :] = z

    NWQ = M // 32
    NWKV = 7 * DC // 64

    def prep_wq(slot, pace=None):
        kh = M // 2
        for n, r in enumerate(range(0, kh, 16)):
            top, bot = wq_p[slot, pl.ds(r, 16), :], wq_p[slot, pl.ds(kh + r, 16), :]
            if pace is not None:
                z = pace(n)
                top, bot = top | z, bot | z
            store_combos(wqb_s, 0, r, lo_hi(top) + lo_hi(bot),
                         None if pace is None else 1 + n)

    def prep_wkv(slot, pace=None):
        kq = DC // 4
        pieces = [(t, r) for t in range(7) for r in range(0, kq, 16)]
        for n, (t, r) in enumerate(pieces):
            terms = [[] for _ in range(4)]
            for k, (q1, sg) in enumerate(_SB[t]):
                src = (wk_p, wv_p)[q1 % 2]
                for rb in range(2):
                    w = src[slot, pl.ds((2 * (q1 // 2) + rb) * kq + r, 16), :]
                    if pace is not None and k == 0:
                        w = w | pace(n)
                    lo, hi = lo_hi(w)
                    terms[2 * rb].append((lo, sg))
                    terms[2 * rb + 1].append((hi, sg))
            store_combos(wkvb_s, 7 * t, r, [_combine(tm) for tm in terms],
                         None if pace is None else 1 + NWQ + n)

    def prep_wo(slot, src0, nrows, dst0, mats, span):
        pieces = [(r, c0, t) for r in range(0, nrows, 16) for c0 in range(0, NO, HT)
                  for t in range(7)]
        pace = pacer(mats, span, len(pieces))
        for n, (r, c0, t) in enumerate(pieces):
            z = pltpu.bitcast(pace(n), _F32)
            rs = pl.ds(src0 + r, 16)
            sub = []
            for q2 in range(4):
                v = _combine([
                    (wo_p[slot, 2 * (q1 // 2) + q2 // 2, rs,
                          pl.ds((2 * (q1 % 2) + q2 % 2) * NO + c0, HT)].astype(_F32), sg)
                    for q1, sg in _SB[t]])
                sub.append(v + z if q2 in (0, 3) else v)
            for u, b in enumerate(_strassen_b(*sub)):
                _st(wob_s, 7 * t + u, dst0 + r, b, pl.ds(c0, HT))

    def project(a_ref, b_ref, dst, r0, a0):
        lhs = a_ref if isinstance(a_ref, list) else [_ld(a_ref, t, a0, HT) for t in range(7)]
        m = [_dot(lhs[t], _ld(b_ref, t, 0, lhs[t].shape[1])) for t in range(7)]
        c11, c12, c21, c22 = _strassen_c(m)
        _st(dst, 0, r0, c11)
        _st(dst, 1, r0, c12)
        _st(dst, 0, r0 + HT, c21)
        _st(dst, 1, r0 + HT, c22)

    QT = HT // 2

    def project_kv(lhs, r0):
        m = []
        for t in range(7):
            ps = [_dot(lhs(7 * t + u), _ld(wkvb_s, 7 * t + u, 0, DC // 4)) for u in range(7)]
            m.append(_strassen_c(ps))
        for q2 in range(4):
            for q1, cblk in enumerate(_strassen_c([mt[q2] for mt in m])):
                rb = 2 * (q1 // 2) + q2 // 2
                _st((k_s, v_s)[q1 % 2], q2 % 2, r0 + rb * QT, cblk)

    for cp in w_copies(0, 0):
        cp.start()
    c_copy(0).start()
    x_copy(0).start()
    ht_s[...] = jnp.zeros((HT, M), _BF16)
    hb_s[...] = jnp.zeros((HT, M), _BF16)
    for cp in w_copies(0, 0):
        cp.wait()
    c_copy(1).start()
    x_copy(1).start()
    prep_wkv(0)
    prep_wq(0)

    def pro_body(i, carry):
        @pl.when(i + 2 < NB)
        def _():
            c_copy(i + 2).start()
            x_copy(i + 2).start()

        @pl.when(i + 2 == NB)
        def _():
            for cp in w_copies(1, 1) + wo_copies(0, 0):
                cp.start()

        c_copy(i).wait()
        x_copy(i).wait()
        r0 = pl.multiple_of(i * TQ, TQ)
        a0 = pl.multiple_of(i * HT, HT)


        def lhs_combos(src, dst, fn, piece):
            parts = [[] for _ in range(7)]
            for c in range(0, HT, piece):
                top = fn(src[pl.ds(r0 + c, piece), :].astype(_F32))
                bot = fn(src[pl.ds(r0 + HT + c, piece), :].astype(_F32))
                kh = top.shape[1] // 2
                for t, a in enumerate(
                        _strassen_a(top[:, :kh], top[:, kh:], bot[:, :kh], bot[:, kh:])):
                    parts[t].append(_pack(a))
            lhs = []
            for t in range(7):
                pk = jnp.concatenate(parts[t], axis=0)
                dst[t, _rows(dst, a0, HT), :] = pk
                lhs.append(_as_bf16(pk))
            return lhs

        kq = DC // 4
        cb = [[c_raw[pl.ds(r0 + rb * QT, QT), pl.ds(kb * kq, kq)].astype(_F32)
               for kb in range(4)] for rb in range(4)]
        ca = []
        for t in range(7):
            sub = [_combine([(cb[2 * (q1 // 2) + q2 // 2][2 * (q1 % 2) + q2 % 2], sg)
                             for q1, sg in _SA[t]]) for q2 in range(4)]
            for u, a in enumerate(_strassen_a(*sub)):
                pk = _pack(a)
                ca_s[7 * t + u, pl.ds(pl.multiple_of(i * (QT // 2), QT // 2), QT // 2), :] = pk
                ca.append(_as_bf16(pk))
        project_kv(lambda n: ca[n], r0)
        xa = lhs_combos(x_raw, xa_s, lambda t: _layernorm_scaled(t, qscale), _PX)
        project(xa_s if _PQ else xa, wqb_s, q_s, r0, a0)
        return carry

    with jax.named_scope('pro_loop'):
        lax.fori_loop(0, NB, pro_body, 0)

    for cp in w_copies(2, 0) + wo_copies(1, 1):
        cp.start()
    ffn_start(NP - 1)
    for cp in w_copies(1, 1) + wo_copies(0, 0):
        cp.wait()

    tri = (lax.broadcasted_iota(_I32, (HT, HT), 1)
           <= lax.broadcasted_iota(_I32, (HT, HT), 0))

    def softmax_rows(parts):
        s = parts[0] if len(parts) == 1 else jnp.concatenate(parts, axis=1)
        m = jnp.max(s, axis=1, keepdims=True)
        p = jnp.exp2(s - m)
        nt = p.shape[1] // HT
        tiles, acc, grp = [], None, None
        for j in range(nt):
            pj = p[:, j * HT:(j + 1) * HT]
            grp = pj if grp is None else grp + pj
            if j % _TIE == _TIE - 1 or j == nt - 1:
                if _CHAIN:
                    acc = grp if acc is None else acc + grp
                    if j > 0:
                        pj = jnp.minimum(pj, acc)
                else:
                    if j % _TIE > 0:
                        pj = jnp.minimum(pj, grp)
                    acc = grp if acc is None else acc + grp
                grp = None
            tiles.append(pj)
        p = tiles[0] if nt == 1 else jnp.concatenate(tiles, axis=1)
        l = jnp.sum(acc, axis=1, keepdims=True)
        return p, l

    def scores(e, i):
        Lm = i * TQ + HT
        s_main = _dot_nt(_ld(q_s, e, i * TQ, TQ), _ld(k_s, e, 0, Lm))
        s_last = _dot_nt(_ld(q_s, e, i * TQ + HT, HT), _ld(k_s, e, Lm, HT))
        return s_main, s_last

    def context(e, head, i, s_main, s_last):
        Lm = i * TQ + HT
        top = [jnp.where(tri, s_main[:HT, Lm - HT:], _NEG)]
        if Lm > HT:
            top = [s_main[:HT, :Lm - HT]] + top
        p_top, l_top = softmax_rows(top)
        p_bot, l_bot = softmax_rows([s_main[HT:], jnp.where(tri, s_last, _NEG)])
        p_main = jnp.concatenate([p_top, p_bot[:, :Lm]], axis=0).astype(_BF16)
        o = _dot(p_main, _ld(v_s, e, 0, Lm))
        o_last = _dot(p_bot[:, Lm:].astype(_BF16), _ld(v_s, e, Lm, HT))
        o_top = o[:HT] * pl.reciprocal(l_top, approx=True)
        o_bot = (o[HT:] + o_last) * pl.reciprocal(l_bot, approx=True)
        _st(ctx_s, head, i * TQ, jnp.concatenate([o_top, o_bot], axis=0))

    def pair_body(s, carry):
        slot = (s + 1) % 2
        wo0 = pl.multiple_of(s * OS, OS)

        def kv(i):
            project_kv(lambda n: _ld(ca_s, n, i * QT, QT), i * TQ)

        for i in range(NB - 1, -1, -1):
            sa = scores(0, i)
            sb = scores(1, i)
            if i == NB - 1:
                prep_wq(slot, pacer([sa[0], sb[0]][:_WQM], _WQS, NWQ))
            if i == NB - 2:
                prep_wkv(slot, pacer([sa[0], sb[0]], 3 * TQ, NWKV))
            if i in (NB - 3, NB - 4):
                r = (NB - 3 - i) * (OS // 2)
                prep_wo(1 - slot, r, OS // 2, wo0 + r, [sa[0], sb[0]], 2 * TQ + HT)
            project(xa_s, wqb_s, q_s, i * TQ, i * HT)
            if i == NB - 2 or (_KVLATE and i < NB - 2):
                kv(i + 1)
            context(0, 2 * s, i, *sa)
            context(1, 2 * s + 1, i, *sb)
            if i == 0 or (not _KVLATE and i < NB - 1):
                kv(i)

        @pl.when(s + 3 < NP)
        def _():
            for cp in w_copies(s + 3, slot):
                cp.start()

        @pl.when(s + 2 < NP)
        def _():
            for cp in wo_copies(s + 2, 1 - slot):
                cp.start()

        ffn_start(s)

        @pl.when(s + 2 < NP)
        def _():
            for cp in w_copies(s + 2, 1 - slot):
                cp.wait()

        for cp in wo_copies(s + 1, slot):
            cp.wait()
        return carry

    with jax.named_scope('pair_loop'):
        lax.fori_loop(0, NP - 1, pair_body, 0)

    last_slot = (NP - 1) % 2

    def last_body(e, carry):
        half = OS // 2
        nxt = scores(e, NB - 1)
        prep_wo(last_slot, pl.multiple_of(e * half, half), half,
                pl.multiple_of((NP - 1) * OS + e * half, half), [nxt[0]], 3 * TQ)
        for i in range(NB - 1, -1, -1):
            cur = nxt
            if i > 0:
                nxt = scores(e, i - 1)
            context(e, H - 2 + e, i, *cur)
        return carry

    with jax.named_scope('last_loop'):
        lax.fori_loop(0, 2, last_body, 0)

    wr = wr_ref[...].astype(_F32)
    eye = (lax.broadcasted_iota(_I32, (HT, HT), 1) == lax.broadcasted_iota(_I32, (HT, HT), 0))

    def epilogue(g, src):
        r0 = pl.multiple_of(g * HT, HT)
        rs = []
        for c in range(0, HT, _ERG):
            hb = src[pl.ds(c, _ERG), :]
            h_s[pl.ds(r0 + c, _ERG), :] = hb
            hc = hb.astype(_F32)
            hnb = _layernorm(hc).astype(_BF16)
            hn_s[pl.ds(r0 + c, _ERG), :] = hnb
            hn = hnb.astype(_F32)
            rs.append(_round_bf16(jnp.sum(hn * wr, axis=1, keepdims=True)))
            out_s[pl.ds(r0 + c, _ERG), :] = (hc + hn).astype(_BF16)
        r = jnp.concatenate(rs, axis=0)
        r_s[pl.ds(g, 1), :] = jnp.sum(jnp.where(eye, r, 0.0), axis=0, keepdims=True)
        return [pltpu.bitcast(jnp.broadcast_to(t, (_ERG, HT)), _U32) & jnp.uint32(0xFFFF)
                for t in rs]

    def out_copy(g):
        rows = pl.ds(pl.multiple_of(g * HT, HT), HT)
        return pltpu.make_async_copy(out_s.at[rows, :], out_hbm.at[rows, :], sem_out.at[0])

    KS = 2 * D

    def prod(r0, t, ties):
        ps = []
        for u in range(7):
            terms = [(2 * (q1 // 2) + q2 // 2, 2 * (q1 % 2) + q2 % 2, s1 * s2)
                     for q1, s1 in _SA[t] for q2, s2 in _SA[u]]
            junk_s[pl.ds(0, 8), :] = jnp.zeros((8, HT), _U32)
            acc = None
            for k0 in range(0, KO, KS):
                def blk(rb, kb):
                    h0 = (kb * KO + k0) // D
                    return jnp.concatenate(
                        [_ld(ctx_s, h0 + hh, (r0, rb * QT), QT) for hh in range(KS // D)], axis=1)
                if len(terms) == 1:
                    lhs = blk(terms[0][0], terms[0][1])
                else:
                    lhs = _combine([(blk(rb, kb).astype(_F32), sg)
                                    for rb, kb, sg in terms]).astype(_BF16)
                w = wob_s[7 * t + u, pl.ds(k0 // 2, KS // 2), :]
                if k0 == 0 and u in ties:
                    head = jnp.concatenate([w[:_ERG, :HT] | ties[u], w[:_ERG, HT:]], axis=1)
                    w = jnp.concatenate([head, w[_ERG:]], axis=0)
                d = _dot(lhs, _as_bf16(w))
                acc = d if acc is None else acc + d
            ps.append(acc)
        c11, c12, c21, c22 = _strassen_c(ps)
        return jnp.concatenate([jnp.concatenate([c11, c12], axis=1),
                                jnp.concatenate([c21, c22], axis=1)], axis=0)

    def o_body(j, carry):
        r0 = pl.multiple_of(j * TQ, TQ)

        @pl.when(j > 1)
        def _():
            out_copy(2 * j - 4).start()
            out_copy(2 * j - 3).start()

        gp = jnp.maximum(2 * j - 2, 0)
        z = epilogue(gp, ht_s) + epilogue(gp + 1, hb_s)
        ties = [{} for _ in range(7)]
        for zt, (o, u) in zip(z, _OTIES):
            ties[o][u] = zt

        rh = pl.multiple_of(j * (TQ // 2), TQ // 2)
        left, right = pl.ds(0, M // 2), pl.ds(M // 2, M // 2)

        def residual(dst, rows0, cols, att):
            dst[:, cols] = (x_raw[pl.ds(rows0, HT), cols].astype(_F32) + att).astype(_BF16)

        m3 = prod(rh, 2, ties[0])
        m4 = prod(rh, 3, ties[1])
        m5 = prod(rh, 4, ties[2])
        residual(ht_s, r0, right, m3 + m5)
        m1 = prod(rh, 0, ties[3])
        m7 = prod(rh, 6, ties[4])
        residual(ht_s, r0, left, m1 + m4 - m5 + m7)
        m2 = prod(rh, 1, ties[5])
        residual(hb_s, r0 + HT, left, m2 + m4)
        m6 = prod(rh, 5, ties[6])
        residual(hb_s, r0 + HT, right, m1 - m2 + m3 + m6)
        return carry

    for n in range(3):
        ffn_wait(n)
    with jax.named_scope('o_loop'):
        lax.fori_loop(0, NB, o_body, 0)
    out_copy(NG - 4).start()
    out_copy(NG - 3).start()
    epilogue(NG - 2, ht_s)
    epilogue(NG - 1, hb_s)
    out_copy(NG - 2).start()
    out_copy(NG - 1).start()

    r = r_s[pl.ds(0, NG), :] + 0.0
    tok = (lax.broadcasted_iota(_I32, (NG, HT), 0) * HT + lax.broadcasted_iota(_I32, (NG, HT), 1))
    code = pltpu.bitcast(r, _I32) >> 16
    code = jnp.where(code < 0, code ^ 0x7FFF, code) + 0x8000
    key = pltpu.bitcast(((code << _IDX_BITS) | (S - 1 - tok)) + _KEY_BIAS, _F32)
    k1 = jnp.max(jnp.max(key, axis=0, keepdims=True), axis=1, keepdims=True)
    key2 = jnp.where(key == k1, 0.0, key)
    k2 = jnp.max(jnp.max(key2, axis=0, keepdims=True), axis=1, keepdims=True)

    R = _FIX
    row = lax.broadcasted_iota(_I32, (2 * R, 1), 0)
    ki = pltpu.bitcast(jnp.where(row < R, k1, k2), _I32) - _KEY_BIAS
    idx = S - 1 - (ki & (2 ** _IDX_BITS - 1))
    i1 = jnp.clip(idx[0, 0], 0, S - 1)
    i2 = jnp.clip(idx[R, 0], 0, S - 1)
    b1 = pl.multiple_of((i1 // R) * R, R)
    b2 = pl.multiple_of((i2 // R) * R, R)
    tokr = jnp.where(row < R, b1 + row, b2 + row - R)
    cd = ((pltpu.bitcast(jnp.where(tokr == i1, k1, k2), _I32) - _KEY_BIAS) >> _IDX_BITS) - 0x8000
    score = pltpu.bitcast(jnp.where(cd < 0, cd ^ 0x7FFF, cd) << 16, _F32)
    gate = _round_bf16(1.0 / (1.0 + jnp.exp(-score)))

    hnsel = jnp.concatenate([hn_s[pl.ds(b1, R), :].astype(_F32),
                             hn_s[pl.ds(b2, R), :].astype(_F32)], axis=0)
    xs = hnsel.astype(_BF16)
    g = _round_bf16(_dot(xs, wg_s[...]))
    u = _round_bf16(_dot(xs, wu_s[...]))
    g = _round_bf16(g * (1.0 / (1.0 + jnp.exp(-g))))
    act = (g * u).astype(_BF16)
    y = _round_bf16(_dot(act, wd_s[:, pl.ds(0, M)]))
    y = _round_bf16(y * gate)
    upd = jnp.where(jnp.logical_or(tokr == i1, tokr == i2), y, 0.0)
    hsel = jnp.concatenate([h_s[pl.ds(b1, R), :].astype(_F32),
                            h_s[pl.ds(b2, R), :].astype(_F32)], axis=0)
    fixed = hsel + _round_bf16(hnsel + upd)

    pltpu.make_async_copy(out_s, out_hbm, sem_out.at[0]).wait()

    def fix_copy(b0, k):
        return pltpu.make_async_copy(out_s.at[pl.ds(b0, R), :],
                                     out_hbm.at[pl.ds(b0, R), :], sem_out.at[k])

    out_s[pl.ds(b1, R), :] = fixed[:R].astype(_BF16)
    out_s[pl.ds(b2, R), :] = fixed[R:].astype(_BF16)
    fix_copy(b1, 0).start()

    @pl.when(b2 != b1)
    def _():
        fix_copy(b2, 1).start()
        fix_copy(b2, 1).wait()

    fix_copy(b1, 0).wait()


@jax.jit
def pallas_sequential_preLN__compressed_kv_cla__moe_arch_mod__prompt_kernel(
    A_x: jax.Array,
    A_c_kv: jax.Array,
    A_w_q: jax.Array,
    A_w_uk: jax.Array,
    A_w_uv: jax.Array,
    A_w_o: jax.Array,
    B_x: jax.Array,
    B_w_r: jax.Array,
    B_w_gate: jax.Array,
    B_w_up: jax.Array,
    B_w_down: jax.Array,
):
    B, S, M = A_x.shape
    assert B == 1
    DC = A_c_kv.shape[2]
    H, D = A_w_q.shape[1], A_w_q.shape[2]
    F = B_w_gate.shape[1]
    assert A_c_kv.shape[1] == S and S % _TQ == 0 and H % 2 == 0 and S <= 2 ** _IDX_BITS
    NP = H // 2
    NG = S // _HT

    x = A_x.reshape(S, M)
    c = A_c_kv.reshape(S, DC)
    wo = A_w_o.reshape(H * D, M)
    wr = B_w_r.reshape(1, M)

    any_spec = pl.BlockSpec(memory_space=pl.ANY)
    vmem_spec = pl.BlockSpec(memory_space=pltpu.VMEM)
    def buf(name, lead, rows, cols):
        if name in _U32BUF:
            return pltpu.VMEM((lead, rows // 2, cols), _U32)
        return pltpu.VMEM((lead, rows, cols), _BF16)

    scratch = [
        pltpu.VMEM((S, M), _BF16),
        pltpu.VMEM((S, DC), _BF16),
        buf('xa', 7, S // 2, M // 2),
        buf('ca', 49, S // 4, DC // 4),
        buf('q', 2, S, D),
        buf('k', 2, S, D),
        buf('v', 2, S, D),
        pltpu.VMEM((2, M, D), _U32),
        pltpu.VMEM((2, DC, D), _U32),
        pltpu.VMEM((2, DC, D), _U32),
        buf('wb', 7, M // 2, D),
        buf('wb', 49, DC // 4, D),
        buf('ctx', H, S, D),
        pltpu.VMEM((2, 4, D // 2, M), _BF16),
        buf('wob', 49, H * D // 4, M // 4),
        pltpu.VMEM((M, F), _BF16),
        pltpu.VMEM((M, F), _BF16),
        pltpu.VMEM((F, M + _WD_PAD), _BF16),
        pltpu.VMEM((_HT, M), _BF16),
        pltpu.VMEM((_HT, M), _BF16),
        pltpu.VMEM((S, M), _BF16),
        pltpu.VMEM((S, M), _BF16),
        pltpu.VMEM((NG, _HT), _F32),
        pltpu.VMEM((1024, _HT), _U32),
        pltpu.VMEM((S, M), _BF16),
        pltpu.SemaphoreType.DMA((3,)),
        pltpu.SemaphoreType.DMA((3,)),
        pltpu.SemaphoreType.DMA((2, 3)),
        pltpu.SemaphoreType.DMA((2, 4)),
        pltpu.SemaphoreType.DMA((3,)),
        pltpu.SemaphoreType.DMA((2,)),
    ]
    out = pl.pallas_call(
        functools.partial(_kernel, S=S, M=M, DC=DC, H=H, D=D, F=F),
        in_specs=[any_spec, any_spec, any_spec, any_spec, any_spec, any_spec,
                  vmem_spec, any_spec, any_spec, any_spec],
        out_specs=any_spec,
        out_shape=jax.ShapeDtypeStruct((S, M), _BF16),
        scratch_shapes=scratch,
        compiler_params=pltpu.CompilerParams(vmem_limit_bytes=120 * 1024 * 1024,
                                             disable_bounds_checks=True,
                                             disable_semaphore_checks=True),
        name="fused_mla_mod",
    )(x, c, A_w_q, A_w_uk, A_w_uv, wo, wr, B_w_gate, B_w_up, B_w_down)
    return out.reshape(B, S, M)
```

```python
import functools
import math

import jax
import jax.numpy as jnp
from jax import lax
import jax.experimental.pallas as pl
import jax.experimental.pallas.tpu as pltpu

_F32 = jnp.float32
_BF16 = jnp.bfloat16
_U32 = jnp.uint32
_I32 = jnp.int32

_EPS = 1e-5
_NEG = -1e30
_TQ = 256
_HT = 128
import os
_TIE = int(os.environ.get('TIE', 4))
_CHAIN = int(os.environ.get('CHAIN', 0))
_ERG = int(os.environ.get('ERG', 16))
_EORD = int(os.environ.get('EORD', 0))
_EVAL = int(os.environ.get('EVAL', 1))
_U32BUF = os.environ.get('U32', 'xa,ca,q,k,v,wob,ctx,wb').split(',')
_PA = int(os.environ.get('PA', 13))
_PB = int(os.environ.get('PB', 0))
_PC = int(os.environ.get('PC', 16))
_PX = int(os.environ.get('PX', 8))
_OT = {
    0: [(0, 2), (0, 3), (0, 4), (0, 5), (0, 6), (1, 0), (1, 1), (1, 2),
        (1, 3), (1, 4), (1, 5), (1, 6), (2, 0), (2, 3), (2, 4), (3, 4)],
    1: [(0, 2), (0, 3), (0, 4), (0, 6), (1, 1), (1, 2), (1, 3), (1, 4),
        (1, 6), (2, 3), (2, 4), (3, 3), (3, 4), (4, 3), (4, 4), (5, 3)],
    2: [(0, 2), (0, 3), (0, 5), (0, 6), (1, 1), (1, 3), (1, 4), (1, 6),
        (2, 2), (2, 4), (2, 6), (3, 2), (3, 4), (4, 0), (4, 3), (4, 5)],
}
_OTIES = _OT[int(os.environ.get('OT', 1))]
_WQS = int(os.environ.get('WQS', 896))
_KVLATE = int(os.environ.get('KVLATE', 0))
_IDX_BITS = 13
_KEY_BIAS = 0x20000000
_FIX = 8
_WD_PAD = 128


def _dot(a, b):
    return jnp.dot(a, b, preferred_element_type=_F32)


def _dot_nt(a, b):
    return lax.dot_general(a, b, (((1,), (1,)), ((), ())), preferred_element_type=_F32)


def _as_bf16(u):
    return pltpu.bitcast(u, _BF16)


def _pack(x):
    return pltpu.bitcast(x.astype(_BF16), _U32)


def _rows(ref, r0, n):
    if ref.dtype == _U32:
        if isinstance(r0, tuple):
            return pl.ds(r0[0] + r0[1] // 2, n // 2)
        if isinstance(r0, int):
            return pl.ds(r0 // 2, n // 2)
        return pl.ds(pl.multiple_of(r0 // 2, 8), n // 2)
    return pl.ds(r0, n)


def _ld(ref, lead, r0, n):
    v = ref[lead, _rows(ref, r0, n), :]
    return _as_bf16(v) if ref.dtype == _U32 else v


def _st(ref, lead, r0, x, cols=slice(None)):
    v = _pack(x) if ref.dtype == _U32 else x.astype(_BF16)
    ref[lead, _rows(ref, r0, x.shape[0]), cols] = v


def _round_bf16(x):
    return x.astype(_BF16).astype(_F32)


def _layernorm(x):
    n = x.shape[-1]
    mean = jnp.sum(x, axis=-1, keepdims=True) * (1.0 / n)
    xc = x - mean
    var = jnp.sum(xc * xc, axis=-1, keepdims=True) * (1.0 / n)
    m = _round_bf16(mean)
    den = _round_bf16(jnp.sqrt(_round_bf16(_round_bf16(var) + _EPS)))
    return (x - m) * (1.0 / den)


def _layernorm_scaled(x, scale):
    n = x.shape[-1]
    mean = jnp.sum(x, axis=-1, keepdims=True) * (1.0 / n)
    xc = x - mean
    var = jnp.sum(xc * xc, axis=-1, keepdims=True) * (1.0 / n)
    return xc * (lax.rsqrt(var + _EPS) * scale)


def _strassen_a(a11, a12, a21, a22):
    return (a11 + a22, a21 + a22, a11, a22, a11 + a12, a21 - a11, a12 - a22)


def _strassen_b(b11, b12, b21, b22):
    return (b11 + b22, b11, b12 - b22, b21 - b11, b22, b11 + b12, b21 + b22)


def _strassen_c(m):
    m1, m2, m3, m4, m5, m6, m7 = m
    return (m1 + m4 - m5 + m7, m3 + m5, m2 + m4, m1 - m2 + m3 + m6)


_SA = (((0, 1), (3, 1)), ((2, 1), (3, 1)), ((0, 1),), ((3, 1),),
       ((0, 1), (1, 1)), ((2, 1), (0, -1)), ((1, 1), (3, -1)))
_SB = (((0, 1), (3, 1)), ((0, 1),), ((1, 1), (3, -1)), ((2, 1), (0, -1)),
       ((3, 1),), ((0, 1), (1, 1)), ((2, 1), (3, 1)))


def _combine(terms):
    terms = sorted(terms, key=lambda ts: -ts[1])
    acc = terms[0][0]
    assert terms[0][1] > 0
    for v, sg in terms[1:]:
        acc = acc + v if sg > 0 else acc - v
    return acc


def _quadrants(x):
    r, c = x.shape[0] // 2, x.shape[1] // 2
    return x[:r, :c], x[:r, c:], x[r:, :c], x[r:, c:]


def _kernel(x_hbm, c_hbm, wq_hbm, wk_hbm, wv_hbm, wo_hbm, wr_ref, wg_hbm, wu_hbm, wd_hbm,
            out_hbm,
            x_raw, c_raw, xn_s, ca_s, q_s, k_s, v_s,
            wq_p, wk_p, wv_p, wqb_s, wkvb_s,
            ctx_s, wo_p, wob_s, wg_s, wu_s, wd_s, ht_s, hb_s, h_s, hn_s, r_s, junk_s, out_s,
            sem_x, sem_c, sem_w, sem_wo, sem_ffn, sem_out,
            *, S, M, DC, H, D, F):
    TQ, HT = _TQ, _HT
    NB = S // TQ
    NG = S // HT
    NP = H // 2
    KO = H * D // 4
    NO = M // 4
    OS = KO // NP
    qscale = (D ** -0.5) * math.log2(math.e)

    wq32 = wq_hbm.bitcast(_U32)
    wk32 = wk_hbm.bitcast(_U32)
    wv32 = wv_hbm.bitcast(_U32)

    def w_copies(pair, slot):
        return (
            pltpu.make_async_copy(wk32.at[:, pair, :], wk_p.at[slot], sem_w.at[slot, 0]),
            pltpu.make_async_copy(wv32.at[:, pair, :], wv_p.at[slot], sem_w.at[slot, 1]),
            pltpu.make_async_copy(wq32.at[:, pair, :], wq_p.at[slot], sem_w.at[slot, 2]),
        )

    def wo_copies(t, slot):
        r0 = pl.multiple_of(t * OS, OS)
        return tuple(
            pltpu.make_async_copy(wo_hbm.at[pl.ds(half * KO + r0, OS), :],
                                  wo_p.at[slot, half], sem_wo.at[slot, half])
            for half in range(4))

    def x_copy(i):
        rows = pl.ds(pl.multiple_of(i * TQ, TQ), TQ)
        return pltpu.make_async_copy(x_hbm.at[rows, :], x_raw.at[rows, :], sem_x.at[i % 3])

    def c_copy(i):
        rows = pl.ds(pl.multiple_of(i * TQ, TQ), TQ)
        return pltpu.make_async_copy(c_hbm.at[rows, :], c_raw.at[rows, :], sem_c.at[i % 3])

    ffn = ((wg_hbm, wg_s), (wu_hbm, wu_s), (wd_hbm, wd_s))

    def ffn_start(t):
        for n, (src, dst) in enumerate(ffn):
            rows, cols = src.shape[0] // NP, src.shape[1]
            r0 = pl.multiple_of(t * rows, 16)
            pltpu.make_async_copy(src.at[pl.ds(r0, rows), :],
                                  dst.at[pl.ds(r0, rows), pl.ds(0, cols)],
                                  sem_ffn.at[n]).start()

    def ffn_wait(n):
        src, dst = ffn[n]
        pltpu.make_async_copy(src, dst.at[:, pl.ds(0, src.shape[1])], sem_ffn.at[n]).wait()

    def lo_hi(w):
        return (pltpu.bitcast(w << 16, _F32), pltpu.bitcast(w & jnp.uint32(0xFFFF0000), _F32))

    def pacer(tiles, total):
        def zero(n):
            mat, zr, zc = tiles[n * len(tiles) // total]
            z = pltpu.bitcast(mat[zr:zr + 8, zc:zc + HT], _U32)
            z = (z >> 16) >> 16
            return jnp.concatenate([z, z], axis=0)
        return zero

    def score_tiles(mats, span):
        return [(m, t0 % TQ, (t0 // TQ) * 4 * HT) for m in mats for t0 in range(0, span, 8)]

    def store_combos(dst, lead0, r, sub, sink):
        z = None
        for u, b in enumerate(_strassen_b(*sub)):
            pk = _pack(b)
            dst[lead0 + u, pl.ds(r // 2, pk.shape[0]), :] = pk
            z = pk if z is None else z | pk
        if sink is not None:
            junk_s[pl.ds(8 * sink, 8), :] = z

    NWQ = M // 32
    NWKV = 7 * DC // 64

    def prep_wq(slot, pace=None):
        kh = M // 2
        for n, r in enumerate(range(0, kh, 16)):
            top, bot = wq_p[slot, pl.ds(r, 16), :], wq_p[slot, pl.ds(kh + r, 16), :]
            if pace is not None:
                z = pace(n)
                top, bot = top | z, bot | z
            store_combos(wqb_s, 0, r, lo_hi(top) + lo_hi(bot),
                         None if pace is None else 1 + n)

    def prep_wkv(slot, pace=None):
        kq = DC // 4
        pieces = [(t, r) for t in range(7) for r in range(0, kq, 16)]
        for n, (t, r) in enumerate(pieces):
            terms = [[] for _ in range(4)]
            for k, (q1, sg) in enumerate(_SB[t]):
                src = (wk_p, wv_p)[q1 % 2]
                for rb in range(2):
                    w = src[slot, pl.ds((2 * (q1 // 2) + rb) * kq + r, 16), :]
                    if pace is not None and k == 0:
                        w = w | pace(n)
                    lo, hi = lo_hi(w)
                    terms[2 * rb].append((lo, sg))
                    terms[2 * rb + 1].append((hi, sg))
            store_combos(wkvb_s, 7 * t, r, [_combine(tm) for tm in terms],
                         None if pace is None else 1 + NWQ + n)

    def prep_wo(slot, src0, nrows, dst0, mats, span):
        pieces = [(r, c0, t) for r in range(0, nrows, 16) for c0 in range(0, NO, HT)
                  for t in range(7)]
        pace = pacer(score_tiles(mats, span), len(pieces))
        for n, (r, c0, t) in enumerate(pieces):
            z = pltpu.bitcast(pace(n), _F32)
            rs = pl.ds(src0 + r, 16)
            sub = []
            for q2 in range(4):
                v = _combine([
                    (wo_p[slot, 2 * (q1 // 2) + q2 // 2, rs,
                          pl.ds((2 * (q1 % 2) + q2 % 2) * NO + c0, HT)].astype(_F32), sg)
                    for q1, sg in _SB[t]])
                sub.append(v + z if q2 in (0, 3) else v)
            for u, b in enumerate(_strassen_b(*sub)):
                _st(wob_s, 7 * t + u, dst0 + r, b, pl.ds(c0, HT))

    QT = HT // 2
    KQ = DC // 4

    def fence():
        junk_s[pl.ds(0, 8), :] = jnp.zeros((8, HT), _U32)

    def project_q(xn, x0, r0):
        kh = M // 2
        m = []
        for t in range(7):
            fence()
            lhs = _combine([(xn[pl.ds(x0 + (q // 2) * HT, HT), pl.ds((q % 2) * kh, kh)], sg)
                            for q, sg in _SA[t]])
            m.append(_dot(lhs.astype(_BF16), _ld(wqb_s, t, 0, kh)))
        for q, cblk in enumerate(_strassen_c(m)):
            _st(q_s, q % 2, r0 + (q // 2) * HT, cblk)
        return [(mt, r, 0) for mt in m for r in range(0, HT, 8)]

    def project_kv(ca, a0, r0):
        m, tiles = [], []
        for t in range(7):
            ps = []
            for u in range(7):
                fence()
                lhs = _combine([(ca[t, pl.ds(a0 + (q // 2) * QT, QT), pl.ds((q % 2) * KQ, KQ)],
                                 sg) for q, sg in _SA[u]])
                ps.append(_dot(lhs.astype(_BF16), _ld(wkvb_s, 7 * t + u, 0, KQ)))
            m.append(_strassen_c(ps))
            tiles += [(pu, r, 0) for pu in ps for r in (0, QT // 2)]
        for q2 in range(4):
            for q1, cblk in enumerate(_strassen_c([mt[q2] for mt in m])):
                rb = 2 * (q1 // 2) + q2 // 2
                _st((k_s, v_s)[q1 % 2], q2 % 2, r0 + rb * QT, cblk)
        return tiles

    def stage_lhs(r0, xn, x0, ca, a0, pace_x=None, pace_c=None):
        kh = DC // 2
        for n, c in enumerate(range(0, HT, 8)):
            top = c_raw[pl.ds(r0 + c, 8), :].astype(_F32)
            bot = c_raw[pl.ds(r0 + HT + c, 8), :].astype(_F32)
            quad = [top[:, :kh], top[:, kh:], bot[:, :kh], bot[:, kh:]]
            if pace_c is not None:
                z = pltpu.bitcast(pace_c(n)[:8], _F32)
                z = jnp.concatenate([z] * (kh // HT), axis=1)
                quad[0], quad[3] = quad[0] + z, quad[3] + z
            for t, a in enumerate(_strassen_a(*quad)):
                ca[t, pl.ds(a0 + c, 8), :] = a
        for n, c in enumerate(range(0, TQ, _PX)):
            xr = x_raw[pl.ds(r0 + c, _PX), :].astype(_F32)
            if pace_x is not None:
                z = pltpu.bitcast(pace_x(n)[:_PX], _F32)
                xr = jnp.concatenate([xr[:, :HT] + z, xr[:, HT:]], axis=1)
            xn[pl.ds(x0 + c, _PX), :] = _layernorm_scaled(xr, qscale)

    c_copy(0).start()
    x_copy(0).start()
    for cp in w_copies(0, 0):
        cp.start()
    ht_s[...] = jnp.zeros((HT, M), _BF16)
    hb_s[...] = jnp.zeros((HT, M), _BF16)
    c_copy(0).wait()
    x_copy(0).wait()
    c_copy(1).start()
    x_copy(1).start()
    stage_lhs(0, xn_s, 0, ca_s, 0)
    for cp in w_copies(0, 0):
        cp.wait()
    c_copy(2).start()
    x_copy(2).start()
    prep_wkv(0)
    prep_wq(0)

    def pro_body(i, carry):
        @pl.when(i + 3 < NB)
        def _():
            c_copy(i + 3).start()
            x_copy(i + 3).start()

        @pl.when(i + 3 == NB)
        def _():
            for cp in w_copies(1, 1) + wo_copies(0, 0):
                cp.start()

        @pl.when(i + 1 < NB)
        def _():
            c_copy(i + 1).wait()
            x_copy(i + 1).wait()

        r0 = pl.multiple_of(i * TQ, TQ)
        xn = xn_s.at[pl.ds(r0, 2 * TQ), :]
        ca = ca_s.at[:, pl.ds(pl.multiple_of(i * HT, HT), 2 * HT), :]
        tiles = project_q(xn, 0, r0) + project_kv(ca, 0, r0)
        nt = len(tiles)
        rn = pl.multiple_of(jnp.minimum(i + 1, NB - 1) * TQ, TQ)
        stage_lhs(rn, xn, TQ, ca, HT, pacer(tiles[:nt * _PA // 16], TQ // _PX),
                  pacer(tiles[nt * _PB // 16:nt * _PC // 16], HT // 8))
        return carry

    with jax.named_scope('pro_loop'):
        lax.fori_loop(0, NB, pro_body, 0)

    for cp in w_copies(2, 0) + wo_copies(1, 1):
        cp.start()
    ffn_start(NP - 1)
    for cp in w_copies(1, 1) + wo_copies(0, 0):
        cp.wait()

    tri = (lax.broadcasted_iota(_I32, (HT, HT), 1)
           <= lax.broadcasted_iota(_I32, (HT, HT), 0))

    def softmax_rows(parts):
        s = parts[0] if len(parts) == 1 else jnp.concatenate(parts, axis=1)
        m = jnp.max(s, axis=1, keepdims=True)
        p = jnp.exp2(s - m)
        nt = p.shape[1] // HT
        tiles, acc, grp = [], None, None
        for j in range(nt):
            pj = p[:, j * HT:(j + 1) * HT]
            grp = pj if grp is None else grp + pj
            if j % _TIE == _TIE - 1 or j == nt - 1:
                if _CHAIN:
                    acc = grp if acc is None else acc + grp
                    if j > 0:
                        pj = jnp.minimum(pj, acc)
                else:
                    if j % _TIE > 0:
                        pj = jnp.minimum(pj, grp)
                    acc = grp if acc is None else acc + grp
                grp = None
            tiles.append(pj)
        p = tiles[0] if nt == 1 else jnp.concatenate(tiles, axis=1)
        l = jnp.sum(acc, axis=1, keepdims=True)
        return p, l

    def scores(e, i):
        Lm = i * TQ + HT
        s_main = _dot_nt(_ld(q_s, e, i * TQ, TQ), _ld(k_s, e, 0, Lm))
        s_last = _dot_nt(_ld(q_s, e, i * TQ + HT, HT), _ld(k_s, e, Lm, HT))
        return s_main, s_last

    def context(e, head, i, s_main, s_last):
        Lm = i * TQ + HT
        top = [jnp.where(tri, s_main[:HT, Lm - HT:], _NEG)]
        if Lm > HT:
            top = [s_main[:HT, :Lm - HT]] + top
        p_top, l_top = softmax_rows(top)
        p_bot, l_bot = softmax_rows([s_main[HT:], jnp.where(tri, s_last, _NEG)])
        p_main = jnp.concatenate([p_top, p_bot[:, :Lm]], axis=0).astype(_BF16)
        o = _dot(p_main, _ld(v_s, e, 0, Lm))
        o_last = _dot(p_bot[:, Lm:].astype(_BF16), _ld(v_s, e, Lm, HT))
        o_top = o[:HT] * pl.reciprocal(l_top, approx=True)
        o_bot = (o[HT:] + o_last) * pl.reciprocal(l_bot, approx=True)
        _st(ctx_s, head, i * TQ, jnp.concatenate([o_top, o_bot], axis=0))

    def pair_body(s, carry):
        slot = (s + 1) % 2
        wo0 = pl.multiple_of(s * OS, OS)

        def kv(i):
            project_kv(ca_s, i * HT, i * TQ)

        for i in range(NB - 1, -1, -1):
            sa = scores(0, i)
            sb = scores(1, i)
            if i == NB - 1:
                prep_wq(slot, pacer(score_tiles([sa[0]], _WQS), NWQ))
            if i == NB - 2:
                prep_wkv(slot, pacer(score_tiles([sa[0], sb[0]], 3 * TQ), NWKV))
            if i in (NB - 3, NB - 4):
                r = (NB - 3 - i) * (OS // 2)
                prep_wo(1 - slot, r, OS // 2, wo0 + r, [sa[0], sb[0]], 2 * TQ + HT)
            project_q(xn_s, i * TQ, i * TQ)
            if i == NB - 2 or (_KVLATE and i < NB - 2):
                kv(i + 1)
            context(0, 2 * s, i, *sa)
            context(1, 2 * s + 1, i, *sb)
            if i == 0 or (not _KVLATE and i < NB - 1):
                kv(i)

        @pl.when(s + 3 < NP)
        def _():
            for cp in w_copies(s + 3, slot):
                cp.start()

        @pl.when(s + 2 < NP)
        def _():
            for cp in wo_copies(s + 2, 1 - slot):
                cp.start()

        ffn_start(s)

        @pl.when(s + 2 < NP)
        def _():
            for cp in w_copies(s + 2, 1 - slot):
                cp.wait()

        for cp in wo_copies(s + 1, slot):
            cp.wait()
        return carry

    with jax.named_scope('pair_loop'):
        lax.fori_loop(0, NP - 1, pair_body, 0)

    last_slot = (NP - 1) % 2

    def last_body(e, carry):
        half = OS // 2
        nxt = scores(e, NB - 1)
        prep_wo(last_slot, pl.multiple_of(e * half, half), half,
                pl.multiple_of((NP - 1) * OS + e * half, half), [nxt[0]], 3 * TQ)
        for i in range(NB - 1, -1, -1):
            cur = nxt
            if i > 0:
                nxt = scores(e, i - 1)
            context(e, H - 2 + e, i, *cur)
        return carry

    with jax.named_scope('last_loop'):
        lax.fori_loop(0, 2, last_body, 0)

    wr = wr_ref[...].astype(_F32)
    eye = (lax.broadcasted_iota(_I32, (HT, HT), 1) == lax.broadcasted_iota(_I32, (HT, HT), 0))

    def epilogue(g, src):
        r0 = pl.multiple_of(g * HT, HT)
        rs = []
        for c in range(0, HT, _ERG):
            hb = src[pl.ds(c, _ERG), :]
            h_s[pl.ds(r0 + c, _ERG), :] = hb
            hc = hb.astype(_F32)
            hnb = _layernorm(hc).astype(_BF16)
            hn_s[pl.ds(r0 + c, _ERG), :] = hnb
            hn = hnb.astype(_F32)
            rs.append(_round_bf16(jnp.sum(hn * wr, axis=1, keepdims=True)))
            out_s[pl.ds(r0 + c, _ERG), :] = (hc + hn).astype(_BF16)
        r = jnp.concatenate(rs, axis=0)
        r_s[pl.ds(g, 1), :] = jnp.sum(jnp.where(eye, r, 0.0), axis=0, keepdims=True)
        return [pltpu.bitcast(jnp.broadcast_to(t, (_ERG, HT)), _U32) & jnp.uint32(0xFFFF)
                for t in rs]

    def out_copy(g):
        rows = pl.ds(pl.multiple_of(g * HT, HT), HT)
        return pltpu.make_async_copy(out_s.at[rows, :], out_hbm.at[rows, :], sem_out.at[0])

    KS = 2 * D

    def prod(r0, t, ties):
        ps = []
        for u in range(7):
            terms = [(2 * (q1 // 2) + q2 // 2, 2 * (q1 % 2) + q2 % 2, s1 * s2)
                     for q1, s1 in _SA[t] for q2, s2 in _SA[u]]
            fence()
            acc = None
            for k0 in range(0, KO, KS):
                def blk(rb, kb):
                    h0 = (kb * KO + k0) // D
                    return jnp.concatenate(
                        [_ld(ctx_s, h0 + hh, (r0, rb * QT), QT) for hh in range(KS // D)], axis=1)
                if len(terms) == 1:
                    lhs = blk(terms[0][0], terms[0][1])
                else:
                    lhs = _combine([(blk(rb, kb).astype(_F32), sg)
                                    for rb, kb, sg in terms]).astype(_BF16)
                w = wob_s[7 * t + u, pl.ds(k0 // 2, KS // 2), :]
                if k0 == 0 and u in ties:
                    head = jnp.concatenate([w[:_ERG, :HT] | ties[u], w[:_ERG, HT:]], axis=1)
                    w = jnp.concatenate([head, w[_ERG:]], axis=0)
                d = _dot(lhs, _as_bf16(w))
                acc = d if acc is None else acc + d
            ps.append(acc)
        c11, c12, c21, c22 = _strassen_c(ps)
        return jnp.concatenate([jnp.concatenate([c11, c12], axis=1),
                                jnp.concatenate([c21, c22], axis=1)], axis=0)

    def o_body(j, carry):
        r0 = pl.multiple_of(j * TQ, TQ)

        @pl.when(j > 1)
        def _():
            out_copy(2 * j - 4).start()
            out_copy(2 * j - 3).start()

        gp = jnp.maximum(2 * j - 2, 0)
        z = epilogue(gp, ht_s) + epilogue(gp + 1, hb_s)
        ties = [{} for _ in range(7)]
        for zt, (o, u) in zip(z, _OTIES):
            ties[o][u] = zt

        rh = pl.multiple_of(j * (TQ // 2), TQ // 2)
        left, right = pl.ds(0, M // 2), pl.ds(M // 2, M // 2)

        def residual(dst, rows0, cols, att):
            dst[:, cols] = (x_raw[pl.ds(rows0, HT), cols].astype(_F32) + att).astype(_BF16)

        m3 = prod(rh, 2, ties[0])
        m4 = prod(rh, 3, ties[1])
        m5 = prod(rh, 4, ties[2])
        residual(ht_s, r0, right, m3 + m5)
        m1 = prod(rh, 0, ties[3])
        m7 = prod(rh, 6, ties[4])
        residual(ht_s, r0, left, m1 + m4 - m5 + m7)
        m2 = prod(rh, 1, ties[5])
        residual(hb_s, r0 + HT, left, m2 + m4)
        m6 = prod(rh, 5, ties[6])
        residual(hb_s, r0 + HT, right, m1 - m2 + m3 + m6)
        return carry

    for n in range(3):
        ffn_wait(n)
    with jax.named_scope('o_loop'):
        lax.fori_loop(0, NB, o_body, 0)
    out_copy(NG - 4).start()
    out_copy(NG - 3).start()
    epilogue(NG - 2, ht_s)
    epilogue(NG - 1, hb_s)
    out_copy(NG - 2).start()
    out_copy(NG - 1).start()

    r = r_s[pl.ds(0, NG), :] + 0.0
    tok = (lax.broadcasted_iota(_I32, (NG, HT), 0) * HT + lax.broadcasted_iota(_I32, (NG, HT), 1))
    code = pltpu.bitcast(r, _I32) >> 16
    code = jnp.where(code < 0, code ^ 0x7FFF, code) + 0x8000
    key = pltpu.bitcast(((code << _IDX_BITS) | (S - 1 - tok)) + _KEY_BIAS, _F32)
    k1 = jnp.max(jnp.max(key, axis=0, keepdims=True), axis=1, keepdims=True)
    key2 = jnp.where(key == k1, 0.0, key)
    k2 = jnp.max(jnp.max(key2, axis=0, keepdims=True), axis=1, keepdims=True)

    R = _FIX
    row = lax.broadcasted_iota(_I32, (2 * R, 1), 0)
    ki = pltpu.bitcast(jnp.where(row < R, k1, k2), _I32) - _KEY_BIAS
    idx = S - 1 - (ki & (2 ** _IDX_BITS - 1))
    i1 = jnp.clip(idx[0, 0], 0, S - 1)
    i2 = jnp.clip(idx[R, 0], 0, S - 1)
    b1 = pl.multiple_of((i1 // R) * R, R)
    b2 = pl.multiple_of((i2 // R) * R, R)
    tokr = jnp.where(row < R, b1 + row, b2 + row - R)
    cd = ((pltpu.bitcast(jnp.where(tokr == i1, k1, k2), _I32) - _KEY_BIAS) >> _IDX_BITS) - 0x8000
    score = pltpu.bitcast(jnp.where(cd < 0, cd ^ 0x7FFF, cd) << 16, _F32)
    gate = _round_bf16(1.0 / (1.0 + jnp.exp(-score)))

    hnsel = jnp.concatenate([hn_s[pl.ds(b1, R), :].astype(_F32),
                             hn_s[pl.ds(b2, R), :].astype(_F32)], axis=0)
    xs = hnsel.astype(_BF16)
    g = _round_bf16(_dot(xs, wg_s[...]))
    u = _round_bf16(_dot(xs, wu_s[...]))
    g = _round_bf16(g * (1.0 / (1.0 + jnp.exp(-g))))
    act = (g * u).astype(_BF16)
    y = _round_bf16(_dot(act, wd_s[:, pl.ds(0, M)]))
    y = _round_bf16(y * gate)
    upd = jnp.where(jnp.logical_or(tokr == i1, tokr == i2), y, 0.0)
    hsel = jnp.concatenate([h_s[pl.ds(b1, R), :].astype(_F32),
                            h_s[pl.ds(b2, R), :].astype(_F32)], axis=0)
    fixed = hsel + _round_bf16(hnsel + upd)

    pltpu.make_async_copy(out_s, out_hbm, sem_out.at[0]).wait()

    def fix_copy(b0, k):
        return pltpu.make_async_copy(out_s.at[pl.ds(b0, R), :],
                                     out_hbm.at[pl.ds(b0, R), :], sem_out.at[k])

    out_s[pl.ds(b1, R), :] = fixed[:R].astype(_BF16)
    out_s[pl.ds(b2, R), :] = fixed[R:].astype(_BF16)
    fix_copy(b1, 0).start()

    @pl.when(b2 != b1)
    def _():
        fix_copy(b2, 1).start()
        fix_copy(b2, 1).wait()

    fix_copy(b1, 0).wait()


@jax.jit
def pallas_sequential_preLN__compressed_kv_cla__moe_arch_mod__prompt_kernel(
    A_x: jax.Array,
    A_c_kv: jax.Array,
    A_w_q: jax.Array,
    A_w_uk: jax.Array,
    A_w_uv: jax.Array,
    A_w_o: jax.Array,
    B_x: jax.Array,
    B_w_r: jax.Array,
    B_w_gate: jax.Array,
    B_w_up: jax.Array,
    B_w_down: jax.Array,
):
    B, S, M = A_x.shape
    assert B == 1
    DC = A_c_kv.shape[2]
    H, D = A_w_q.shape[1], A_w_q.shape[2]
    F = B_w_gate.shape[1]
    assert A_c_kv.shape[1] == S and S % _TQ == 0 and H % 2 == 0 and S <= 2 ** _IDX_BITS
    NP = H // 2
    NG = S // _HT

    x = A_x.reshape(S, M)
    c = A_c_kv.reshape(S, DC)
    wo = A_w_o.reshape(H * D, M)
    wr = B_w_r.reshape(1, M)

    any_spec = pl.BlockSpec(memory_space=pl.ANY)
    vmem_spec = pl.BlockSpec(memory_space=pltpu.VMEM)
    def buf(name, lead, rows, cols):
        if name in _U32BUF:
            return pltpu.VMEM((lead, rows // 2, cols), _U32)
        return pltpu.VMEM((lead, rows, cols), _BF16)

    scratch = [
        pltpu.VMEM((S, M), _BF16),
        pltpu.VMEM((S, DC), _BF16),
        pltpu.VMEM((S + _TQ, M), _F32),
        pltpu.VMEM((7, S // 2 + _HT, DC // 2), _F32),
        buf('q', 2, S, D),
        buf('k', 2, S, D),
        buf('v', 2, S, D),
        pltpu.VMEM((2, M, D), _U32),
        pltpu.VMEM((2, DC, D), _U32),
        pltpu.VMEM((2, DC, D), _U32),
        buf('wb', 7, M // 2, D),
        buf('wb', 49, DC // 4, D),
        buf('ctx', H, S, D),
        pltpu.VMEM((2, 4, D // 2, M), _BF16),
        buf('wob', 49, H * D // 4, M // 4),
        pltpu.VMEM((M, F), _BF16),
        pltpu.VMEM((M, F), _BF16),
        pltpu.VMEM((F, M + _WD_PAD), _BF16),
        pltpu.VMEM((_HT, M), _BF16),
        pltpu.VMEM((_HT, M), _BF16),
        pltpu.VMEM((S, M), _BF16),
        pltpu.VMEM((S, M), _BF16),
        pltpu.VMEM((NG, _HT), _F32),
        pltpu.VMEM((1024, _HT), _U32),
        pltpu.VMEM((S, M), _BF16),
        pltpu.SemaphoreType.DMA((3,)),
        pltpu.SemaphoreType.DMA((3,)),
        pltpu.SemaphoreType.DMA((2, 3)),
        pltpu.SemaphoreType.DMA((2, 4)),
        pltpu.SemaphoreType.DMA((3,)),
        pltpu.SemaphoreType.DMA((2,)),
    ]
    out = pl.pallas_call(
        functools.partial(_kernel, S=S, M=M, DC=DC, H=H, D=D, F=F),
        in_specs=[any_spec, any_spec, any_spec, any_spec, any_spec, any_spec,
                  vmem_spec, any_spec, any_spec, any_spec],
        out_specs=any_spec,
        out_shape=jax.ShapeDtypeStruct((S, M), _BF16),
        scratch_shapes=scratch,
        compiler_params=pltpu.CompilerParams(vmem_limit_bytes=120 * 1024 * 1024,
                                             disable_bounds_checks=True,
                                             disable_semaphore_checks=True),
        name="fused_mla_mod",
    )(x, c, A_w_q, A_w_uk, A_w_uv, wo, wr, B_w_gate, B_w_up, B_w_down)
    return out.reshape(B, S, M)
```

```python
import functools
import math

import jax
import jax.numpy as jnp
from jax import lax
import jax.experimental.pallas as pl
import jax.experimental.pallas.tpu as pltpu

_F32 = jnp.float32
_BF16 = jnp.bfloat16
_U32 = jnp.uint32
_I32 = jnp.int32

_EPS = 1e-5
_NEG = -1e30
_TQ = 256
_HT = 128
import os
_TIE = int(os.environ.get('TIE', 4))
_CHAIN = int(os.environ.get('CHAIN', 0))
_ERG = int(os.environ.get('ERG', 16))
_EORD = int(os.environ.get('EORD', 0))
_EVAL = int(os.environ.get('EVAL', 1))
_U32BUF = os.environ.get('U32', 'xa,ca,q,k,v,wob,ctx,wb').split(',')
_PA = int(os.environ.get('PA', 13))
_PB = int(os.environ.get('PB', 0))
_PC = int(os.environ.get('PC', 16))
_PX = int(os.environ.get('PX', 8))
_OT = {
    0: [(0, 2), (0, 3), (0, 4), (0, 5), (0, 6), (1, 0), (1, 1), (1, 2),
        (1, 3), (1, 4), (1, 5), (1, 6), (2, 0), (2, 3), (2, 4), (3, 4)],
    1: [(0, 2), (0, 3), (0, 4), (0, 6), (1, 1), (1, 2), (1, 3), (1, 4),
        (1, 6), (2, 3), (2, 4), (3, 3), (3, 4), (4, 3), (4, 4), (5, 3)],
    2: [(0, 2), (0, 3), (0, 5), (0, 6), (1, 1), (1, 3), (1, 4), (1, 6),
        (2, 2), (2, 4), (2, 6), (3, 2), (3, 4), (4, 0), (4, 3), (4, 5)],
}
_OTIES = _OT[int(os.environ.get('OT', 1))]
_WQS = int(os.environ.get('WQS', 896))
_NG = int(os.environ.get('NG', 16))
_BIG = int(os.environ.get('BIG', 3))
_TSPAN = 360
_DIST = int(os.environ.get('DIST', 2))
_PN = int(os.environ.get('PN', 14))
_WOH = int(os.environ.get('WOH', 0))
_IDX_BITS = 13
_KEY_BIAS = 0x20000000
_FIX = 8
_WD_PAD = 128


def _dot(a, b):
    return jnp.dot(a, b, preferred_element_type=_F32)


def _dot_nt(a, b):
    return lax.dot_general(a, b, (((1,), (1,)), ((), ())), preferred_element_type=_F32)


def _as_bf16(u):
    return pltpu.bitcast(u, _BF16)


def _pack(x):
    return pltpu.bitcast(x.astype(_BF16), _U32)


def _rows(ref, r0, n):
    if ref.dtype == _U32:
        if isinstance(r0, tuple):
            return pl.ds(r0[0] + r0[1] // 2, n // 2)
        if isinstance(r0, int):
            return pl.ds(r0 // 2, n // 2)
        return pl.ds(pl.multiple_of(r0 // 2, 8), n // 2)
    return pl.ds(r0, n)


def _ld(ref, lead, r0, n):
    v = ref[lead, _rows(ref, r0, n), :]
    return _as_bf16(v) if ref.dtype == _U32 else v


def _st(ref, lead, r0, x, cols=slice(None)):
    v = _pack(x) if ref.dtype == _U32 else x.astype(_BF16)
    if lead is None:
        ref[_rows(ref, r0, x.shape[0]), cols] = v
    else:
        ref[lead, _rows(ref, r0, x.shape[0]), cols] = v


def _round_bf16(x):
    return x.astype(_BF16).astype(_F32)


def _layernorm(x):
    n = x.shape[-1]
    mean = jnp.sum(x, axis=-1, keepdims=True) * (1.0 / n)
    xc = x - mean
    var = jnp.sum(xc * xc, axis=-1, keepdims=True) * (1.0 / n)
    m = _round_bf16(mean)
    den = _round_bf16(jnp.sqrt(_round_bf16(_round_bf16(var) + _EPS)))
    return (x - m) * (1.0 / den)


def _layernorm_scaled(x, scale):
    n = x.shape[-1]
    mean = jnp.sum(x, axis=-1, keepdims=True) * (1.0 / n)
    xc = x - mean
    var = jnp.sum(xc * xc, axis=-1, keepdims=True) * (1.0 / n)
    return xc * (lax.rsqrt(var + _EPS) * scale)


def _strassen_a(a11, a12, a21, a22):
    return (a11 + a22, a21 + a22, a11, a22, a11 + a12, a21 - a11, a12 - a22)


def _strassen_b(b11, b12, b21, b22):
    return (b11 + b22, b11, b12 - b22, b21 - b11, b22, b11 + b12, b21 + b22)


def _strassen_c(m):
    m1, m2, m3, m4, m5, m6, m7 = m
    return (m4 - m5 + m1 + m7, m3 + m5, m4 + m2, m3 - m2 + m1 + m6)


_ORDER = (2, 4, 3, 1, 0, 6, 5)


_SA = (((0, 1), (3, 1)), ((2, 1), (3, 1)), ((0, 1),), ((3, 1),),
       ((0, 1), (1, 1)), ((2, 1), (0, -1)), ((1, 1), (3, -1)))
_SB = (((0, 1), (3, 1)), ((0, 1),), ((1, 1), (3, -1)), ((2, 1), (0, -1)),
       ((3, 1),), ((0, 1), (1, 1)), ((2, 1), (3, 1)))


def _combine(terms):
    terms = sorted(terms, key=lambda ts: -ts[1])
    acc = terms[0][0]
    assert terms[0][1] > 0
    for v, sg in terms[1:]:
        acc = acc + v if sg > 0 else acc - v
    return acc


def _quadrants(x):
    r, c = x.shape[0] // 2, x.shape[1] // 2
    return x[:r, :c], x[:r, c:], x[r:, :c], x[r:, c:]


def _kernel(x_hbm, c_hbm, wq_hbm, wk_hbm, wv_hbm, wo_hbm, wr_ref, wg_hbm, wu_hbm, wd_hbm,
            out_hbm,
            x_raw, c_raw, xn_s, ca_s, q_s, k_s, v_s,
            wq_p, wk_p, wv_p, wqb_s, wkvb_s,
            ctx_s, wo_p, wob_s, wg_s, wu_s, wd_s, ht_s, hb_s, h_s, hn_s, r_s, junk_s, out_s,
            sem_x, sem_c, sem_w, sem_wq, sem_wo, sem_ffn, sem_out,
            *, S, M, DC, H, D, F):
    TQ, HT = _TQ, _HT
    NB = S // TQ
    NG = S // HT
    NP = H // 2
    KO = H * D // 4
    NO = M // 4
    OS = KO // NP
    qscale = (D ** -0.5) * math.log2(math.e)

    wq32 = wq_hbm.bitcast(_U32)
    wk32 = wk_hbm.bitcast(_U32)
    wv32 = wv_hbm.bitcast(_U32)

    def w_copies(pair, slot):
        return (
            pltpu.make_async_copy(wk32.at[:, pair, :], wk_p.at[slot], sem_w.at[slot, 0]),
            pltpu.make_async_copy(wv32.at[:, pair, :], wv_p.at[slot], sem_w.at[slot, 1]),
        )

    def wq_copy(pair):
        return pltpu.make_async_copy(wq32.at[:, pair, :], wq_p.at[pair % 4],
                                     sem_wq.at[pair % 4])

    def wo_copies(t, slot):
        r0 = pl.multiple_of(t * OS, OS)
        return tuple(
            pltpu.make_async_copy(wo_hbm.at[pl.ds(half * KO + r0, OS), :],
                                  wo_p.at[slot, half], sem_wo.at[slot, half])
            for half in range(4))

    def x_copy(i):
        rows = pl.ds(pl.multiple_of(i * TQ, TQ), TQ)
        return pltpu.make_async_copy(x_hbm.at[rows, :], x_raw.at[rows, :], sem_x.at[i % 3])

    def c_copy(i):
        rows = pl.ds(pl.multiple_of(i * TQ, TQ), TQ)
        return pltpu.make_async_copy(c_hbm.at[rows, :], c_raw.at[rows, :], sem_c.at[i % 3])

    ffn = ((wg_hbm, wg_s), (wu_hbm, wu_s), (wd_hbm, wd_s))

    def ffn_start(t):
        for n, (src, dst) in enumerate(ffn):
            rows, cols = src.shape[0] // NP, src.shape[1]
            r0 = pl.multiple_of(t * rows, 16)
            pltpu.make_async_copy(src.at[pl.ds(r0, rows), :],
                                  dst.at[pl.ds(r0, rows), pl.ds(0, cols)],
                                  sem_ffn.at[n]).start()

    def ffn_wait(n):
        src, dst = ffn[n]
        pltpu.make_async_copy(src, dst.at[:, pl.ds(0, src.shape[1])], sem_ffn.at[n]).wait()

    def lo_hi(w):
        return (pltpu.bitcast(w << 16, _F32), pltpu.bitcast(w & jnp.uint32(0xFFFF0000), _F32))

    def pacer(tiles, total):
        def zero(n):
            mat, zr, zc = tiles[n * len(tiles) // total]
            z = pltpu.bitcast(mat[zr:zr + 8, zc:zc + HT], _U32)
            z = (z >> 16) >> 16
            return jnp.concatenate([z, z], axis=0)
        return zero

    def score_tiles(mats, span):
        return [(m, t0 % TQ, (t0 // TQ) * 4 * HT) for m in mats for t0 in range(0, span, 8)]

    def prep_w4(srcs, dst, kq, rows, pace=None, sink=None):
        pieces = [(t, r) for t in range(7) for r in rows]
        for n, (t, r) in enumerate(pieces):
            terms = [[] for _ in range(4)]
            for k, (q1, sg) in enumerate(_SB[t]):
                for rb in range(2):
                    w = srcs[q1 % 2][pl.ds((2 * (q1 // 2) + rb) * kq + r, 16), :]
                    if pace is not None and k == 0:
                        w = w | pace(n)
                    lo, hi = lo_hi(w)
                    terms[2 * rb].append((lo, sg))
                    terms[2 * rb + 1].append((hi, sg))
            z = None
            for u, b in enumerate(_strassen_b(*[_combine(tm) for tm in terms])):
                pk = _pack(b)
                dst[7 * t + u, pl.ds(r // 2, 8), :] = pk
                z = pk if z is None else z | pk
            if sink is not None:
                junk_s[pl.ds(8 * (sink + n), 8), :] = z

    def prep_wo(slot, src0, nrows, dst0, mats, span):
        pieces = [(r, c0, t) for r in range(0, nrows, 16) for c0 in range(0, NO, HT)
                  for t in range(7)]
        pace = pacer(score_tiles(mats, span), len(pieces))
        for n, (r, c0, t) in enumerate(pieces):
            z = pltpu.bitcast(pace(n), _F32)
            rs = pl.ds(src0 + r, 16)
            sub = []
            for q2 in range(4):
                v = _combine([
                    (wo_p[slot, 2 * (q1 // 2) + q2 // 2, rs,
                          pl.ds((2 * (q1 % 2) + q2 % 2) * NO + c0, HT)].astype(_F32), sg)
                    for q1, sg in _SB[t]])
                sub.append(v + z if q2 in (0, 3) else v)
            for u, b in enumerate(_strassen_b(*sub)):
                _st(wob_s, 7 * t + u, dst0 + r, b, pl.ds(c0, HT))

    QT = HT // 2
    KQ = DC // 4
    MQ = M // 4

    def fence():
        junk_s[pl.ds(0, 8), :] = jnp.zeros((8, HT), _U32)

    def tie(w, ties):
        parts, at = [], 0
        for r in sorted(ties):
            if r > at:
                parts.append(w[at:r])
            parts.append(w[r:r + 8] | ties[r])
            at = r + 8
        if at < w.shape[0]:
            parts.append(w[at:])
        return parts[0] if len(parts) == 1 else jnp.concatenate(parts, axis=0)

    def project4(lhs, w, store, zs=()):
        m, tiles, cnt = [None] * 7, [], [0]
        for t in _ORDER:
            ps = [None] * 7
            for u in _ORDER:
                fence()
                a = lhs(t, u)
                wt = w[7 * t + u]
                n = len(tiles) * len(zs) * D * 8 // (_TSPAN * a.shape[1] * 2)
                done = cnt[0]
                if zs and done < len(zs) and n > done:
                    wt = tie(wt, {0: zs[done]})
                    cnt[0] += 1
                ps[u] = _dot(a.astype(_BF16), _as_bf16(wt))
                tiles += [(ps[u], r, 0) for r in range(0, QT, QT * D // (2 * a.shape[1]))]
            m[t] = _strassen_c(ps)
        for q2 in range(4):
            for q1, cblk in enumerate(_strassen_c([mt[q2] for mt in m])):
                store(2 * (q1 % 2) + q2 % 2, (2 * (q1 // 2) + q2 // 2) * QT, cblk)
        return tiles

    def project_q(xn, x0, wqb, q, r0):
        def lhs(t, u):
            return _combine([
                (xn[pl.ds(x0 + (2 * (q1 // 2) + q2 // 2) * QT, QT),
                    pl.ds((2 * (q1 % 2) + q2 % 2) * MQ, MQ)], s1 * s2)
                for q1, s1 in _SA[t] for q2, s2 in _SA[u]])
        return project4(lhs, wqb, lambda nb, r, val: _st(q, nb, r0 + r, val))

    def project_kv(ca, a0, r0, zs=()):
        def lhs(t, u):
            return _combine([
                (ca[t, pl.ds(a0 + (q2 // 2) * QT, QT), pl.ds((q2 % 2) * KQ, KQ)], sg)
                for q2, sg in _SA[u]])
        return project4(lhs, wkvb_s,
                        lambda nb, r, val: _st((k_s, v_s)[nb // 2], nb % 2, r0 + r, val), zs)

    def prep_wq(raw, slot, r, nr, pace, sink=None):
        span = 3 * MQ + nr
        prep_w4((wq_p.at[raw, pl.ds(r, span), :], wq_p.at[raw + 1, pl.ds(r, span), :]),
                wqb_s.at[slot, :, pl.ds(pl.multiple_of(r // 2, 8), nr // 2), :],
                MQ, range(0, nr, 16), pace, sink)

    def stage_lhs(r0, xn, x0, ca, a0, pace_x=None, pace_c=None):
        kh = DC // 2
        for n, c in enumerate(range(0, HT, 8)):
            top = c_raw[pl.ds(r0 + c, 8), :].astype(_F32)
            bot = c_raw[pl.ds(r0 + HT + c, 8), :].astype(_F32)
            quad = [top[:, :kh], top[:, kh:], bot[:, :kh], bot[:, kh:]]
            if pace_c is not None:
                z = pltpu.bitcast(pace_c(n)[:8], _F32)
                z = jnp.concatenate([z] * (kh // HT), axis=1)
                quad[0], quad[3] = quad[0] + z, quad[3] + z
            for t, a in enumerate(_strassen_a(*quad)):
                ca[t, pl.ds(a0 + c, 8), :] = a
        for n, c in enumerate(range(0, TQ, _PX)):
            xr = x_raw[pl.ds(r0 + c, _PX), :].astype(_F32)
            if pace_x is not None:
                z = pltpu.bitcast(pace_x(n)[:_PX], _F32)
                xr = jnp.concatenate([xr[:, :HT] + z, xr[:, HT:]], axis=1)
            xn[pl.ds(x0 + c, _PX), :] = _layernorm_scaled(xr, qscale)

    for cp in w_copies(0, 0):
        cp.start()
    c_copy(0).start()
    x_copy(0).start()
    ht_s[...] = jnp.zeros((HT, M), _BF16)
    hb_s[...] = jnp.zeros((HT, M), _BF16)
    for cp in w_copies(0, 0):
        cp.wait()
    wq_copy(0).start()
    wq_copy(1).start()
    c_copy(1).start()
    x_copy(1).start()

    def prep0_body(g, carry):
        r = pl.multiple_of(g * 16, 16)
        span = 3 * KQ + 16
        prep_w4((wk_p.at[0, pl.ds(r, span), :], wv_p.at[0, pl.ds(r, span), :]),
                wkvb_s.at[:, pl.ds(pl.multiple_of(g * 8, 8), 8), :], KQ, [0])
        return carry

    lax.fori_loop(0, KQ // 16, prep0_body, 0)
    c_copy(0).wait()
    x_copy(0).wait()
    stage_lhs(0, xn_s, 0, ca_s, 0)
    wq_copy(0).wait()
    wq_copy(1).wait()
    c_copy(2).start()
    x_copy(2).start()

    def pro_body(with_q, i, carry):
        @pl.when(i + 3 < NB)
        def _():
            c_copy(i + 3).start()
            x_copy(i + 3).start()

        if with_q:
            @pl.when(i + 3 == NB)
            def _():
                for cp in w_copies(1, 1) + wo_copies(0, 0) + (wq_copy(4), wq_copy(5)):
                    cp.start()
        else:
            @pl.when(i == 1)
            def _():
                wq_copy(2).start()
                wq_copy(3).start()

        @pl.when(i + 1 < NB)
        def _():
            c_copy(i + 1).wait()
            x_copy(i + 1).wait()

        r0 = pl.multiple_of(i * TQ, TQ)
        xn = xn_s.at[pl.ds(r0, 2 * TQ), :]
        ca = ca_s.at[:, pl.ds(pl.multiple_of(i * HT, HT), 2 * HT), :]
        rn = pl.multiple_of(jnp.minimum(i + 1, NB - 1) * TQ, TQ)
        if with_q:
            tiles = project_q(xn, 0, wqb_s.at[0], q_s, r0)
            nt = len(tiles)
            kt = project_kv(ca, 0, r0)
            stage_lhs(rn, xn, TQ, ca, HT, pacer(tiles[:nt * _PA // 16], TQ // _PX),
                      pacer(tiles[nt * _PB // 16:nt * _PC // 16], HT // 8))
            nr = MQ // NB
            prep_wq(2, 1, pl.multiple_of((i - NB // 2) * nr, nr), nr, pacer(kt, 7 * nr // 16))
        else:
            tiles = project_kv(ca, 0, r0)
            stage_lhs(rn, xn, TQ, ca, HT, pacer(tiles, TQ // _PX), pacer(tiles, HT // 8))
            nr = MQ // (NB // 2)
            prep_wq(0, 0, pl.multiple_of(i * nr, nr), nr, pacer(tiles, 7 * nr // 16))
        return carry

    with jax.named_scope('pro_loop'):
        lax.fori_loop(0, NB // 2, functools.partial(pro_body, False), 0)
        wq_copy(2).wait()
        wq_copy(3).wait()
        lax.fori_loop(NB // 2, NB, functools.partial(pro_body, True), 0)

    for cp in w_copies(2, 0) + wo_copies(1, 1):
        cp.start()
    ffn_start(NP - 1)
    for cp in w_copies(1, 1) + wo_copies(0, 0) + (wq_copy(4),):
        cp.wait()

    tri = (lax.broadcasted_iota(_I32, (HT, HT), 1)
           <= lax.broadcasted_iota(_I32, (HT, HT), 0))

    def softmax_rows(parts):
        s = parts[0] if len(parts) == 1 else jnp.concatenate(parts, axis=1)
        m = jnp.max(s, axis=1, keepdims=True)
        p = jnp.exp2(s - m)
        nt = p.shape[1] // HT
        tiles, acc, grp = [], None, None
        for j in range(nt):
            pj = p[:, j * HT:(j + 1) * HT]
            grp = pj if grp is None else grp + pj
            if j % _TIE == _TIE - 1 or j == nt - 1:
                if _CHAIN:
                    acc = grp if acc is None else acc + grp
                    if j > 0:
                        pj = jnp.minimum(pj, acc)
                else:
                    if j % _TIE > 0:
                        pj = jnp.minimum(pj, grp)
                    acc = grp if acc is None else acc + grp
                grp = None
            tiles.append(pj)
        p = tiles[0] if nt == 1 else jnp.concatenate(tiles, axis=1)
        return p, acc

    def scores(q, e, i, zs=()):
        Lm = i * TQ + HT
        nt = Lm // HT
        ties = {(4 + n * (nt - 4) // len(zs)) * QT + 8 * (n % 8): z for n, z in enumerate(zs)}
        keys = _as_bf16(tie(k_s[e, pl.ds(0, Lm // 2), :], ties))
        s_main = _dot_nt(_ld(q, e, i * TQ, TQ), keys)
        s_last = _dot_nt(_ld(q, e, i * TQ + HT, HT), _ld(k_s, e, Lm, HT))
        return s_main, s_last

    def context(e, head, i, s_main, s_last, e_static=0):
        Lm = i * TQ + HT
        top = [jnp.where(tri, s_main[:HT, Lm - HT:], _NEG)]
        if Lm > HT:
            top = [s_main[:HT, :Lm - HT]] + top
        p_top, l_top = softmax_rows(top)
        p_bot, l_bot = softmax_rows([s_main[HT:], jnp.where(tri, s_last, _NEG)])
        p_main = jnp.concatenate([p_top, p_bot[:, :Lm]], axis=0).astype(_BF16)
        o = _dot(p_main, _ld(v_s, e, 0, Lm))
        o_last = _dot(p_bot[:, Lm:].astype(_BF16), _ld(v_s, e, Lm, HT))
        o = jnp.concatenate([o[:HT], o[HT:] + o_last], axis=0)
        acc = jnp.concatenate([l_top, l_bot], axis=0)

        def normalize(pace=None, n0=0):
            zs, z = [], None
            for n, g in enumerate(range(0, TQ, 16)):
                a = acc[g:g + 16]
                if pace is not None:
                    a = a + pltpu.bitcast(pace(n0 + n), _F32)
                linv = jnp.broadcast_to(
                    pl.reciprocal(jnp.sum(a, axis=1, keepdims=True), approx=True), (16, D))
                _st(ctx_s.at[head], None, i * TQ + g, o[g:g + 16] * linv)
                bits = pltpu.bitcast(linv, _U32)
                bits = bits[:8] | bits[8:]
                z = bits if z is None else z | bits
                if n % _NG == _NG - 1:
                    zs.append((z >> 16) >> 16)
                    z = None
            return zs
        return normalize

    def pair_body(s, carry):
        slot = (s + 1) % 2
        odd = s % 2
        wo0 = pl.multiple_of(s * OS, OS)
        q_rd = q_s.at[pl.ds(2 * odd, 2)]
        q_wr = q_s.at[:, pl.ds(pl.multiple_of(odd * (S // 4), S // 4), S // 4), :]
        xn = xn_s.at[pl.ds(pl.multiple_of(odd * (S // 2), S // 2), S // 2), :]
        quad = (s + 1) // 2
        wqb = wqb_s.at[quad % 2]
        NH = NB // 2
        pend = {}

        for i in range(NB - 1, -1, -1):
            sa = scores(q_rd, 0, i)
            zs = []
            if i + 2 in pend:
                na, nb = pend.pop(i + 2)
                src = score_tiles([sa[0]], (2 * i + 1) * QT * _PN // 16) if i >= _BIG else kt
                pace = pacer(src, TQ // 8)
                zs = na(pace) + nb(pace, TQ // 16)
            sb = scores(q_rd, 1, i, zs if i >= _BIG else ())
            if i == NB - 1:
                prep_w4((wk_p.at[slot], wv_p.at[slot]), wkvb_s, KQ, range(0, KQ, 16),
                        pacer(score_tiles([sa[0], sb[0]], 3 * TQ + HT), 7 * KQ // 16), 1)
            if i == NB - 2:
                prep_wq(2 * (jnp.minimum(quad + 1, NP // 2 - 1) % 2), (quad + 1) % 2,
                        pl.multiple_of((1 - odd) * (MQ // 2), MQ // 2), MQ // 2,
                        pacer(score_tiles([sa[0], sb[0]], 3 * TQ), 7 * MQ // 32), 64)
            if i in (NB - 3, NB - 4):
                r = (NB - 3 - i) * (OS // 2)
                prep_wo(1 - slot, r, OS // 2, wo0 + r, [sa[0], sb[0]][_WOH:], 2 * TQ + QT)
            if i >= NH:
                project_q(xn, (i - NH) * TQ, wqb, q_wr, (i - NH) * TQ)
            else:
                project_kv(ca_s, (2 * i + 1) * HT, (2 * i + 1) * TQ, () if i >= _BIG else zs)
            pend[i] = (context(0, 2 * s, i, *sa), context(1, 2 * s + 1, i, *sb))
            if i < NH:
                kt = project_kv(ca_s, 2 * i * HT, 2 * i * TQ)
        for i in sorted(pend, reverse=True):
            pend[i][0]()
            pend[i][1]()

        @pl.when(s + 3 < NP)
        def _():
            for cp in w_copies(s + 3, slot):
                cp.start()

        @pl.when(s + 2 < NP)
        def _():
            for cp in wo_copies(s + 2, 1 - slot):
                cp.start()

        @pl.when(s + 6 < NP)
        def _():
            wq_copy(s + 6).start()

        ffn_start(s)

        @pl.when(s + 5 < NP)
        def _():
            wq_copy(s + 5).wait()

        @pl.when(s + 2 < NP)
        def _():
            for cp in w_copies(s + 2, 1 - slot):
                cp.wait()

        for cp in wo_copies(s + 1, slot):
            cp.wait()
        return carry

    with jax.named_scope('pair_loop'):
        lax.fori_loop(0, NP - 1, pair_body, 0)

    last_slot = (NP - 1) % 2

    def last_body(e, carry):
        half = OS // 2
        q_rd = q_s.at[pl.ds(2, 2)]
        nxt = scores(q_rd, e, NB - 1)
        prep_wo(last_slot, pl.multiple_of(e * half, half), half,
                pl.multiple_of((NP - 1) * OS + e * half, half), [nxt[0]], 3 * TQ)
        for i in range(NB - 1, -1, -1):
            cur = nxt
            if i > 0:
                nxt = scores(q_rd, e, i - 1)
            context(e, H - 2 + e, i, *cur)()
        return carry

    with jax.named_scope('last_loop'):
        lax.fori_loop(0, 2, last_body, 0)

    wr = wr_ref[...].astype(_F32)
    eye = (lax.broadcasted_iota(_I32, (HT, HT), 1) == lax.broadcasted_iota(_I32, (HT, HT), 0))

    def epilogue(g, src):
        r0 = pl.multiple_of(g * HT, HT)
        rs = []
        for c in range(0, HT, _ERG):
            hb = src[pl.ds(c, _ERG), :]
            h_s[pl.ds(r0 + c, _ERG), :] = hb
            hc = hb.astype(_F32)
            hnb = _layernorm(hc).astype(_BF16)
            hn_s[pl.ds(r0 + c, _ERG), :] = hnb
            hn = hnb.astype(_F32)
            rs.append(_round_bf16(jnp.sum(hn * wr, axis=1, keepdims=True)))
            out_s[pl.ds(r0 + c, _ERG), :] = (hc + hn).astype(_BF16)
        r = jnp.concatenate(rs, axis=0)
        r_s[pl.ds(g, 1), :] = jnp.sum(jnp.where(eye, r, 0.0), axis=0, keepdims=True)
        return [pltpu.bitcast(jnp.broadcast_to(t, (_ERG, HT)), _U32) & jnp.uint32(0xFFFF)
                for t in rs]

    def out_copy(g):
        rows = pl.ds(pl.multiple_of(g * HT, HT), HT)
        return pltpu.make_async_copy(out_s.at[rows, :], out_hbm.at[rows, :], sem_out.at[0])

    KS = 2 * D

    def prod(r0, t, ties):
        ps = []
        for u in range(7):
            terms = [(2 * (q1 // 2) + q2 // 2, 2 * (q1 % 2) + q2 % 2, s1 * s2)
                     for q1, s1 in _SA[t] for q2, s2 in _SA[u]]
            fence()
            acc = None
            for k0 in range(0, KO, KS):
                def blk(rb, kb):
                    h0 = (kb * KO + k0) // D
                    return jnp.concatenate(
                        [_ld(ctx_s, h0 + hh, (r0, rb * QT), QT) for hh in range(KS // D)], axis=1)
                if len(terms) == 1:
                    lhs = blk(terms[0][0], terms[0][1])
                else:
                    lhs = _combine([(blk(rb, kb).astype(_F32), sg)
                                    for rb, kb, sg in terms]).astype(_BF16)
                w = wob_s[7 * t + u, pl.ds(k0 // 2, KS // 2), :]
                if k0 == 0 and u in ties:
                    head = jnp.concatenate([w[:_ERG, :HT] | ties[u], w[:_ERG, HT:]], axis=1)
                    w = jnp.concatenate([head, w[_ERG:]], axis=0)
                d = _dot(lhs, _as_bf16(w))
                acc = d if acc is None else acc + d
            ps.append(acc)
        c11, c12, c21, c22 = _strassen_c(ps)
        return jnp.concatenate([jnp.concatenate([c11, c12], axis=1),
                                jnp.concatenate([c21, c22], axis=1)], axis=0)

    def o_body(j, carry):
        r0 = pl.multiple_of(j * TQ, TQ)

        @pl.when(j > 1)
        def _():
            out_copy(2 * j - 4).start()
            out_copy(2 * j - 3).start()

        gp = jnp.maximum(2 * j - 2, 0)
        z = epilogue(gp, ht_s) + epilogue(gp + 1, hb_s)
        ties = [{} for _ in range(7)]
        for zt, (o, u) in zip(z, _OTIES):
            ties[o][u] = zt

        rh = pl.multiple_of(j * (TQ // 2), TQ // 2)
        left, right = pl.ds(0, M // 2), pl.ds(M // 2, M // 2)

        def residual(dst, rows0, cols, att):
            dst[:, cols] = (x_raw[pl.ds(rows0, HT), cols].astype(_F32) + att).astype(_BF16)

        m3 = prod(rh, 2, ties[0])
        m4 = prod(rh, 3, ties[1])
        m5 = prod(rh, 4, ties[2])
        residual(ht_s, r0, right, m3 + m5)
        m1 = prod(rh, 0, ties[3])
        m7 = prod(rh, 6, ties[4])
        residual(ht_s, r0, left, m1 + m4 - m5 + m7)
        m2 = prod(rh, 1, ties[5])
        residual(hb_s, r0 + HT, left, m2 + m4)
        m6 = prod(rh, 5, ties[6])
        residual(hb_s, r0 + HT, right, m1 - m2 + m3 + m6)
        return carry

    for n in range(3):
        ffn_wait(n)
    with jax.named_scope('o_loop'):
        lax.fori_loop(0, NB, o_body, 0)
    out_copy(NG - 4).start()
    out_copy(NG - 3).start()
    epilogue(NG - 2, ht_s)
    epilogue(NG - 1, hb_s)
    out_copy(NG - 2).start()
    out_copy(NG - 1).start()

    r = r_s[pl.ds(0, NG), :] + 0.0
    tok = (lax.broadcasted_iota(_I32, (NG, HT), 0) * HT + lax.broadcasted_iota(_I32, (NG, HT), 1))
    code = pltpu.bitcast(r, _I32) >> 16
    code = jnp.where(code < 0, code ^ 0x7FFF, code) + 0x8000
    key = pltpu.bitcast(((code << _IDX_BITS) | (S - 1 - tok)) + _KEY_BIAS, _F32)
    k1 = jnp.max(jnp.max(key, axis=0, keepdims=True), axis=1, keepdims=True)
    key2 = jnp.where(key == k1, 0.0, key)
    k2 = jnp.max(jnp.max(key2, axis=0, keepdims=True), axis=1, keepdims=True)

    R = _FIX
    row = lax.broadcasted_iota(_I32, (2 * R, 1), 0)
    ki = pltpu.bitcast(jnp.where(row < R, k1, k2), _I32) - _KEY_BIAS
    idx = S - 1 - (ki & (2 ** _IDX_BITS - 1))
    i1 = jnp.clip(idx[0, 0], 0, S - 1)
    i2 = jnp.clip(idx[R, 0], 0, S - 1)
    b1 = pl.multiple_of((i1 // R) * R, R)
    b2 = pl.multiple_of((i2 // R) * R, R)
    tokr = jnp.where(row < R, b1 + row, b2 + row - R)
    cd = ((pltpu.bitcast(jnp.where(tokr == i1, k1, k2), _I32) - _KEY_BIAS) >> _IDX_BITS) - 0x8000
    score = pltpu.bitcast(jnp.where(cd < 0, cd ^ 0x7FFF, cd) << 16, _F32)
    gate = _round_bf16(1.0 / (1.0 + jnp.exp(-score)))

    hnsel = jnp.concatenate([hn_s[pl.ds(b1, R), :].astype(_F32),
                             hn_s[pl.ds(b2, R), :].astype(_F32)], axis=0)
    xs = hnsel.astype(_BF16)
    g = _round_bf16(_dot(xs, wg_s[...]))
    u = _round_bf16(_dot(xs, wu_s[...]))
    g = _round_bf16(g * (1.0 / (1.0 + jnp.exp(-g))))
    act = (g * u).astype(_BF16)
    y = _round_bf16(_dot(act, wd_s[:, pl.ds(0, M)]))
    y = _round_bf16(y * gate)
    upd = jnp.where(jnp.logical_or(tokr == i1, tokr == i2), y, 0.0)
    hsel = jnp.concatenate([h_s[pl.ds(b1, R), :].astype(_F32),
                            h_s[pl.ds(b2, R), :].astype(_F32)], axis=0)
    fixed = hsel + _round_bf16(hnsel + upd)

    pltpu.make_async_copy(out_s, out_hbm, sem_out.at[0]).wait()

    def fix_copy(b0, k):
        return pltpu.make_async_copy(out_s.at[pl.ds(b0, R), :],
                                     out_hbm.at[pl.ds(b0, R), :], sem_out.at[k])

    out_s[pl.ds(b1, R), :] = fixed[:R].astype(_BF16)
    out_s[pl.ds(b2, R), :] = fixed[R:].astype(_BF16)
    fix_copy(b1, 0).start()

    @pl.when(b2 != b1)
    def _():
        fix_copy(b2, 1).start()
        fix_copy(b2, 1).wait()

    fix_copy(b1, 0).wait()


@jax.jit
def pallas_sequential_preLN__compressed_kv_cla__moe_arch_mod__prompt_kernel(
    A_x: jax.Array,
    A_c_kv: jax.Array,
    A_w_q: jax.Array,
    A_w_uk: jax.Array,
    A_w_uv: jax.Array,
    A_w_o: jax.Array,
    B_x: jax.Array,
    B_w_r: jax.Array,
    B_w_gate: jax.Array,
    B_w_up: jax.Array,
    B_w_down: jax.Array,
):
    B, S, M = A_x.shape
    assert B == 1
    DC = A_c_kv.shape[2]
    H, D = A_w_q.shape[1], A_w_q.shape[2]
    F = B_w_gate.shape[1]
    assert A_c_kv.shape[1] == S and S % _TQ == 0 and H % 2 == 0 and S <= 2 ** _IDX_BITS
    NP = H // 2
    NG = S // _HT

    x = A_x.reshape(S, M)
    c = A_c_kv.reshape(S, DC)
    wo = A_w_o.reshape(H * D, M)
    wr = B_w_r.reshape(1, M)

    any_spec = pl.BlockSpec(memory_space=pl.ANY)
    vmem_spec = pl.BlockSpec(memory_space=pltpu.VMEM)
    def buf(name, lead, rows, cols):
        if name in _U32BUF:
            return pltpu.VMEM((lead, rows // 2, cols), _U32)
        return pltpu.VMEM((lead, rows, cols), _BF16)

    scratch = [
        pltpu.VMEM((S, M), _BF16),
        pltpu.VMEM((S, DC), _BF16),
        pltpu.VMEM((S + _TQ, M), _F32),
        pltpu.VMEM((7, S // 2 + _HT, DC // 2), _F32),
        buf('q', 4, S, D),
        buf('k', 2, S, D),
        buf('v', 2, S, D),
        pltpu.VMEM((4, M, D), _U32),
        pltpu.VMEM((2, DC, D), _U32),
        pltpu.VMEM((2, DC, D), _U32),
        pltpu.VMEM((2, 49, M // 8, D), _U32),
        buf('wb', 49, DC // 4, D),
        buf('ctx', H, S, D),
        pltpu.VMEM((2, 4, D // 2, M), _BF16),
        buf('wob', 49, H * D // 4, M // 4),
        pltpu.VMEM((M, F), _BF16),
        pltpu.VMEM((M, F), _BF16),
        pltpu.VMEM((F, M + _WD_PAD), _BF16),
        pltpu.VMEM((_HT, M), _BF16),
        pltpu.VMEM((_HT, M), _BF16),
        pltpu.VMEM((S, M), _BF16),
        pltpu.VMEM((S, M), _BF16),
        pltpu.VMEM((NG, _HT), _F32),
        pltpu.VMEM((1024, _HT), _U32),
        pltpu.VMEM((S, M), _BF16),
        pltpu.SemaphoreType.DMA((3,)),
        pltpu.SemaphoreType.DMA((3,)),
        pltpu.SemaphoreType.DMA((2, 2)),
        pltpu.SemaphoreType.DMA((4,)),
        pltpu.SemaphoreType.DMA((2, 4)),
        pltpu.SemaphoreType.DMA((3,)),
        pltpu.SemaphoreType.DMA((2,)),
    ]
    out = pl.pallas_call(
        functools.partial(_kernel, S=S, M=M, DC=DC, H=H, D=D, F=F),
        in_specs=[any_spec, any_spec, any_spec, any_spec, any_spec, any_spec,
                  vmem_spec, any_spec, any_spec, any_spec],
        out_specs=any_spec,
        out_shape=jax.ShapeDtypeStruct((S, M), _BF16),
        scratch_shapes=scratch,
        compiler_params=pltpu.CompilerParams(vmem_limit_bytes=124 * 1024 * 1024,
                                             disable_bounds_checks=True,
                                             disable_semaphore_checks=True),
        name="fused_mla_mod",
    )(x, c, A_w_q, A_w_uk, A_w_uv, wo, wr, B_w_gate, B_w_up, B_w_down)
    return out.reshape(B, S, M)
```

```python
import functools
import math

import jax
import jax.numpy as jnp
from jax import lax
import jax.experimental.pallas as pl
import jax.experimental.pallas.tpu as pltpu

_F32 = jnp.float32
_BF16 = jnp.bfloat16
_U32 = jnp.uint32
_I32 = jnp.int32

_EPS = 1e-5
_NEG = -1e30
_TQ = 256
_HT = 128
import os
_TIE = int(os.environ.get('TIE', 4))
_CHAIN = int(os.environ.get('CHAIN', 0))
_ERG = int(os.environ.get('ERG', 16))
_EORD = int(os.environ.get('EORD', 0))
_EVAL = int(os.environ.get('EVAL', 1))
_U32BUF = os.environ.get('U32', 'xa,ca,q,k,v,wob,ctx,wb').split(',')
_PA = int(os.environ.get('PA', 13))
_PB = int(os.environ.get('PB', 13))
_PC = int(os.environ.get('PC', 16))
_PX = int(os.environ.get('PX', 8))
_OT = {
    0: [(0, 2), (0, 3), (0, 4), (0, 5), (0, 6), (1, 0), (1, 1), (1, 2),
        (1, 3), (1, 4), (1, 5), (1, 6), (2, 0), (2, 3), (2, 4), (3, 4)],
    1: [(0, 2), (0, 3), (0, 4), (0, 6), (1, 1), (1, 2), (1, 3), (1, 4),
        (1, 6), (2, 3), (2, 4), (3, 3), (3, 4), (4, 3), (4, 4), (5, 3)],
    2: [(0, 2), (0, 3), (0, 5), (0, 6), (1, 1), (1, 3), (1, 4), (1, 6),
        (2, 2), (2, 4), (2, 6), (3, 2), (3, 4), (4, 0), (4, 3), (4, 5)],
}
_OTIES = _OT[int(os.environ.get('OT', 1))]
_WQS = int(os.environ.get('WQS', 896))
_NG = int(os.environ.get('NG', 16))
_BIG = int(os.environ.get('BIG', 3))
_TSPAN = 360
_DIST = int(os.environ.get('DIST', 2))
_PN = int(os.environ.get('PN', 14))
_WOH = int(os.environ.get('WOH', 0))
_LND = int(os.environ.get('LND', 6))
_FR = int(os.environ.get('FR', 2))
_IDX_BITS = 13
_KEY_BIAS = 0x20000000
_FIX = 8
_WD_PAD = 128


def _dot(a, b):
    return jnp.dot(a, b, preferred_element_type=_F32)


def _dot_nt(a, b):
    return lax.dot_general(a, b, (((1,), (1,)), ((), ())), preferred_element_type=_F32)


def _as_bf16(u):
    return pltpu.bitcast(u, _BF16)


def _pack(x):
    return pltpu.bitcast(x.astype(_BF16), _U32)


def _rows(ref, r0, n):
    if ref.dtype == _U32:
        if isinstance(r0, tuple):
            return pl.ds(r0[0] + r0[1] // 2, n // 2)
        if isinstance(r0, int):
            return pl.ds(r0 // 2, n // 2)
        return pl.ds(pl.multiple_of(r0 // 2, 8), n // 2)
    return pl.ds(r0, n)


def _ld(ref, lead, r0, n):
    v = ref[lead, _rows(ref, r0, n), :]
    return _as_bf16(v) if ref.dtype == _U32 else v


def _st(ref, lead, r0, x, cols=slice(None)):
    v = _pack(x) if ref.dtype == _U32 else x.astype(_BF16)
    if lead is None:
        ref[_rows(ref, r0, x.shape[0]), cols] = v
    else:
        ref[lead, _rows(ref, r0, x.shape[0]), cols] = v


def _round_bf16(x):
    return x.astype(_BF16).astype(_F32)


def _layernorm(x):
    n = x.shape[-1]
    mean = jnp.sum(x, axis=-1, keepdims=True) * (1.0 / n)
    xc = x - mean
    var = jnp.sum(xc * xc, axis=-1, keepdims=True) * (1.0 / n)
    m = _round_bf16(mean)
    den = _round_bf16(jnp.sqrt(_round_bf16(_round_bf16(var) + _EPS)))
    return (x - m) * (1.0 / den)


def _layernorm_scaled(x, scale):
    n = x.shape[-1]
    mean = jnp.sum(x, axis=-1, keepdims=True) * (1.0 / n)
    xc = x - mean
    var = jnp.sum(xc * xc, axis=-1, keepdims=True) * (1.0 / n)
    return xc * (lax.rsqrt(var + _EPS) * scale)


def _strassen_a(a11, a12, a21, a22):
    return (a11 + a22, a21 + a22, a11, a22, a11 + a12, a21 - a11, a12 - a22)


def _strassen_b(b11, b12, b21, b22):
    return (b11 + b22, b11, b12 - b22, b21 - b11, b22, b11 + b12, b21 + b22)


def _strassen_c(m):
    m1, m2, m3, m4, m5, m6, m7 = m
    return (m4 - m5 + m1 + m7, m3 + m5, m4 + m2, m3 - m2 + m1 + m6)


_ORDER = (2, 4, 3, 1, 0, 6, 5)


_SA = (((0, 1), (3, 1)), ((2, 1), (3, 1)), ((0, 1),), ((3, 1),),
       ((0, 1), (1, 1)), ((2, 1), (0, -1)), ((1, 1), (3, -1)))
_SB = (((0, 1), (3, 1)), ((0, 1),), ((1, 1), (3, -1)), ((2, 1), (0, -1)),
       ((3, 1),), ((0, 1), (1, 1)), ((2, 1), (3, 1)))


def _combine(terms):
    terms = sorted(terms, key=lambda ts: -ts[1])
    acc = terms[0][0]
    assert terms[0][1] > 0
    for v, sg in terms[1:]:
        acc = acc + v if sg > 0 else acc - v
    return acc


def _quadrants(x):
    r, c = x.shape[0] // 2, x.shape[1] // 2
    return x[:r, :c], x[:r, c:], x[r:, :c], x[r:, c:]


def _kernel(x_hbm, c_hbm, wq_hbm, wk_hbm, wv_hbm, wo_hbm, wr_ref, wg_hbm, wu_hbm, wd_hbm,
            out_hbm,
            x_raw, c_raw, xn_s, ca_s, q_s, k_s, v_s,
            wq_p, wk_p, wv_p, wqb_s, wkvb_s,
            ctx_s, wo_p, wob_s, wg_s, wu_s, wd_s, ht_s, hb_s, h_s, hn_s, r_s, junk_s, out_s,
            sem_x, sem_c, sem_w, sem_wq, sem_wo, sem_ffn, sem_out,
            *, S, M, DC, H, D, F):
    TQ, HT = _TQ, _HT
    NB = S // TQ
    NG = S // HT
    NP = H // 2
    KO = H * D // 4
    NO = M // 4
    OS = KO // NP
    qscale = (D ** -0.5) * math.log2(math.e)

    wq32 = wq_hbm.bitcast(_U32)
    wk32 = wk_hbm.bitcast(_U32)
    wv32 = wv_hbm.bitcast(_U32)

    def w_copies(pair, slot):
        return (
            pltpu.make_async_copy(wk32.at[:, pair, :], wk_p.at[slot], sem_w.at[slot, 0]),
            pltpu.make_async_copy(wv32.at[:, pair, :], wv_p.at[slot], sem_w.at[slot, 1]),
        )

    def wq_copy(pair):
        return pltpu.make_async_copy(wq32.at[:, pair, :], wq_p.at[pair % 4],
                                     sem_wq.at[pair % 4])

    def wo_copies(t, slot):
        r0 = pl.multiple_of(t * OS, OS)
        return tuple(
            pltpu.make_async_copy(wo_hbm.at[pl.ds(half * KO + r0, OS), :],
                                  wo_p.at[slot, half], sem_wo.at[slot, half])
            for half in range(4))

    def x_copy(i, n):
        rows = pl.ds(pl.multiple_of(i * TQ, TQ), TQ)
        return pltpu.make_async_copy(x_hbm.at[rows, :], x_raw.at[rows, :], sem_x.at[n % 3])

    def c_copy(i):
        rows = pl.ds(pl.multiple_of(i * 2 * TQ, 2 * TQ), 2 * TQ)
        return pltpu.make_async_copy(c_hbm.at[rows, :], c_raw.at[rows, :], sem_c.at[i % 3])

    ffn = ((wg_hbm, wg_s), (wu_hbm, wu_s), (wd_hbm, wd_s))

    def ffn_start(t):
        for n, (src, dst) in enumerate(ffn):
            rows, cols = src.shape[0] // NP, src.shape[1]
            r0 = pl.multiple_of(t * rows, 16)
            pltpu.make_async_copy(src.at[pl.ds(r0, rows), :],
                                  dst.at[pl.ds(r0, rows), pl.ds(0, cols)],
                                  sem_ffn.at[n]).start()

    def ffn_wait(n):
        src, dst = ffn[n]
        pltpu.make_async_copy(src, dst.at[:, pl.ds(0, src.shape[1])], sem_ffn.at[n]).wait()

    def lo_hi(w):
        return (pltpu.bitcast(w << 16, _F32), pltpu.bitcast(w & jnp.uint32(0xFFFF0000), _F32))

    def pacer(tiles, total, free=0):
        def zero(n):
            if n < free:
                return jnp.zeros((16, HT), _U32)
            mat, zr, zc = tiles[(n - free) * len(tiles) // (total - free)]
            z = pltpu.bitcast(mat[zr:zr + 8, zc:zc + HT], _U32)
            z = (z >> 16) >> 16
            return jnp.concatenate([z, z], axis=0)
        return zero

    def score_tiles(mats, span):
        return [(m, t0 % TQ, (t0 // TQ) * 4 * HT) for m in mats for t0 in range(0, span, 8)]

    def prep_w4(srcs, dst, kq, rows, pace=None, sink=None):
        pieces = [(t, r) for t in range(7) for r in rows]
        for n, (t, r) in enumerate(pieces):
            terms = [[] for _ in range(4)]
            for k, (q1, sg) in enumerate(_SB[t]):
                for rb in range(2):
                    w = srcs[q1 % 2][pl.ds((2 * (q1 // 2) + rb) * kq + r, 16), :]
                    if pace is not None and k == 0:
                        w = w | pace(n)
                    lo, hi = lo_hi(w)
                    terms[2 * rb].append((lo, sg))
                    terms[2 * rb + 1].append((hi, sg))
            z = None
            for u, b in enumerate(_strassen_b(*[_combine(tm) for tm in terms])):
                pk = _pack(b)
                dst[7 * t + u, pl.ds(r // 2, 8), :] = pk
                z = pk if z is None else z | pk
            if sink is not None:
                junk_s[pl.ds(8 * (sink + n), 8), :] = z

    def prep_wo(slot, src0, nrows, dst0, mats, span):
        pieces = [(r, c0, t) for r in range(0, nrows, 16) for c0 in range(0, NO, HT)
                  for t in range(7)]
        pace = pacer(score_tiles(mats, span), len(pieces))
        for n, (r, c0, t) in enumerate(pieces):
            z = pltpu.bitcast(pace(n), _F32)
            rs = pl.ds(src0 + r, 16)
            sub = []
            for q2 in range(4):
                v = _combine([
                    (wo_p[slot, 2 * (q1 // 2) + q2 // 2, rs,
                          pl.ds((2 * (q1 % 2) + q2 % 2) * NO + c0, HT)].astype(_F32), sg)
                    for q1, sg in _SB[t]])
                sub.append(v + z if q2 in (0, 3) else v)
            for u, b in enumerate(_strassen_b(*sub)):
                _st(wob_s, 7 * t + u, dst0 + r, b, pl.ds(c0, HT))

    QT = HT // 2
    KQ = DC // 4
    MQ = M // 4

    def fence():
        junk_s[pl.ds(0, 8), :] = jnp.zeros((8, HT), _U32)

    def tie(w, ties):
        parts, at = [], 0
        for r in sorted(ties):
            if r > at:
                parts.append(w[at:r])
            parts.append(w[r:r + 8] | ties[r])
            at = r + 8
        if at < w.shape[0]:
            parts.append(w[at:])
        return parts[0] if len(parts) == 1 else jnp.concatenate(parts, axis=0)

    def project4(lhs, w, store, zs=()):
        m, tiles, cnt = [None] * 7, [], [0]
        for t in _ORDER:
            ps = [None] * 7
            for u in _ORDER:
                fence()
                a = lhs(t, u)
                wt = w[7 * t + u]
                n = len(tiles) * len(zs) * D * 8 // (_TSPAN * a.shape[1] * 2)
                done = cnt[0]
                if zs and done < len(zs) and n > done:
                    wt = tie(wt, {0: zs[done]})
                    cnt[0] += 1
                ps[u] = _dot(a.astype(_BF16), _as_bf16(wt))
                tiles += [(ps[u], r, 0) for r in range(0, QT, QT * D // (2 * a.shape[1]))]
            m[t] = _strassen_c(ps)
        for q2 in range(4):
            for q1, cblk in enumerate(_strassen_c([mt[q2] for mt in m])):
                store(2 * (q1 % 2) + q2 % 2, (2 * (q1 // 2) + q2 // 2) * QT, cblk)
        return tiles

    def project_q(xn, x0, wqb, q, r0):
        def lhs(t, u):
            return _combine([
                (xn[pl.ds(x0 + (2 * (q1 // 2) + q2 // 2) * QT, QT),
                    pl.ds((2 * (q1 % 2) + q2 % 2) * MQ, MQ)], s1 * s2)
                for q1, s1 in _SA[t] for q2, s2 in _SA[u]])
        return project4(lhs, wqb, lambda nb, r, val: _st(q, nb, r0 + r, val))

    def project_kv(ca, a0, r0, zs=()):
        def lhs(t, u):
            return _combine([
                (ca[t, pl.ds(a0 + (q2 // 2) * QT, QT), pl.ds((q2 % 2) * KQ, KQ)], sg)
                for q2, sg in _SA[u]])
        return project4(lhs, wkvb_s,
                        lambda nb, r, val: _st((k_s, v_s)[nb // 2], nb % 2, r0 + r, val), zs)

    def prep_wq(raw, slot, r, nr, pace, sink=None):
        span = 3 * MQ + nr
        prep_w4((wq_p.at[raw, pl.ds(r, span), :], wq_p.at[raw + 1, pl.ds(r, span), :]),
                wqb_s.at[slot, :, pl.ds(pl.multiple_of(r // 2, 8), nr // 2), :],
                MQ, range(0, nr, 16), pace, sink)

    NH = NB // 2

    def plain_weights(src0, src1):
        return jnp.concatenate(lo_hi(src0[...]) + lo_hi(src1[...]), axis=1).astype(_BF16)

    def stage_x(r0, xn, x0, pace):
        done = []
        for n, c in enumerate(range(0, TQ, _PX)):
            xr = x_raw[pl.ds(r0 + c, _PX), :].astype(_F32)
            z = pace(n)[:_PX]
            if n >= _LND:
                z = z | done[n - _LND]
            xr = jnp.concatenate([xr[:, :HT] + pltpu.bitcast(z, _F32), xr[:, HT:]], axis=1)
            y = _layernorm_scaled(xr, qscale)
            xn[pl.ds(x0 + c, _PX), :] = y
            done.append((pltpu.bitcast(y[:, :HT], _U32) >> 16) >> 16)

    def stage_c(r0, a0, pace):
        kh = DC // 2
        for n, c in enumerate(range(0, HT, 8)):
            top = c_raw[pl.ds(r0 + c, 8), :].astype(_F32)
            bot = c_raw[pl.ds(r0 + HT + c, 8), :].astype(_F32)
            z = pltpu.bitcast(pace(n)[:8], _F32)
            z = jnp.concatenate([z] * (kh // HT), axis=1)
            for t, a in enumerate(
                    _strassen_a(top[:, :kh] + z, top[:, kh:], bot[:, :kh], bot[:, kh:] + z)):
                ca_s[t, pl.ds(a0 + c, 8), :] = a

    def xs_copy(n):
        return x_copy((n + NH) % NB, n)

    for cp in w_copies(0, 0):
        cp.start()
    c_copy(0).start()
    xs_copy(0).start()
    ht_s[...] = jnp.zeros((HT, M), _BF16)
    hb_s[...] = jnp.zeros((HT, M), _BF16)
    for cp in w_copies(0, 0):
        cp.wait()
    c_copy(1).start()
    xs_copy(1).start()
    c_copy(0).wait()
    xs_copy(0).wait()

    def pro_a(i, carry):
        @pl.when(i + 2 < NH)
        def _():
            c_copy(i + 2).start()

        xs_copy(i + 2).start()

        @pl.when(i >= 1)
        def _():
            wq_copy(i - 1).start()

        @pl.when(i > 0)
        def _():
            c_copy(i).wait()
            xs_copy(i).wait()

        r0 = pl.multiple_of(i * 2 * TQ, 2 * TQ)
        kv = _dot(c_raw[pl.ds(r0, 2 * TQ), :], plain_weights(wk_p.at[0], wv_p.at[0]))
        for nb in range(4):
            _st((k_s, v_s)[nb // 2], nb % 2, r0, kv[:, nb * D:(nb + 1) * D])
        tiles = [(kv, r, nb * D) for nb in range(4) for r in range(0, 2 * TQ, 8)]
        nt = len(tiles)
        a0 = pl.multiple_of(i * TQ, TQ)
        stage_c(r0, a0, pacer(tiles[:nt // 2], HT // 8))
        stage_c(r0 + TQ, a0 + HT, pacer(tiles[nt // 2:nt * 15 // 16], HT // 8))
        rx = pl.multiple_of((i + NH) * TQ, TQ)
        stage_x(rx, xn_s, rx, pacer(tiles[:nt * _PA // 16], TQ // _PX, _FR))
        return carry

    def pro_b(i, carry):
        @pl.when(i + 2 < NH)
        def _():
            xs_copy(NH + i + 2).start()

        @pl.when(i == 0)
        def _():
            wq_copy(3).start()

        @pl.when(i == 2)
        def _():
            for cp in w_copies(1, 1) + wo_copies(0, 0):
                cp.start()
            wq_copy(2).wait()
            wq_copy(3).wait()

        xs_copy(NH + i).wait()
        r0 = pl.multiple_of(i * TQ, TQ)
        xn = xn_s.at[pl.ds(r0, S // 2 + TQ), :]
        kh = M // 2
        lhs = [xn[pl.ds(S // 2, TQ), pl.ds(k0, kh)].astype(_BF16) for k0 in (0, kh)]
        tiles = []
        for nb in range(4):
            d = [_dot(lhs[k], lo_hi(wq_p[nb // 2, pl.ds(k * kh, kh), :])[nb % 2].astype(_BF16))
                 for k in range(2)]
            _st(q_s, nb, r0 + S // 2, d[0] + d[1])
            tiles += [(dk, r, 0) for dk in d for r in range(0, TQ, 8)]
        nt = len(tiles)
        stage_x(r0, xn, 0, pacer(tiles[:nt * _PB // 16], TQ // _PX, _FR))
        nr = MQ // (2 * NH)
        npc = 7 * nr // 16
        pace = pacer(tiles[:nt * _PC // 16], 3 * npc, _FR)
        for k in range(3):
            u = 3 * i + k
            quad = u // (2 * NH)
            prep_wq(2 * quad, quad, pl.multiple_of((u % (2 * NH)) * nr, nr), nr,
                    lambda n, k=k: pace(k * npc + n))
        return carry

    with jax.named_scope('pro_a'):
        lax.fori_loop(0, NH, pro_a, 0)
    wq_copy(0).wait()
    wq_copy(1).wait()
    with jax.named_scope('pro_b'):
        lax.fori_loop(0, NH, pro_b, 0)

    for cp in w_copies(2, 0) + wo_copies(1, 1) + (wq_copy(4), wq_copy(5)):
        cp.start()
    ffn_start(NP - 1)
    for cp in w_copies(1, 1) + wo_copies(0, 0):
        cp.wait()

    tri = (lax.broadcasted_iota(_I32, (HT, HT), 1)
           <= lax.broadcasted_iota(_I32, (HT, HT), 0))

    def softmax_rows(parts):
        s = parts[0] if len(parts) == 1 else jnp.concatenate(parts, axis=1)
        m = jnp.max(s, axis=1, keepdims=True)
        p = jnp.exp2(s - m)
        nt = p.shape[1] // HT
        tiles, acc, grp = [], None, None
        for j in range(nt):
            pj = p[:, j * HT:(j + 1) * HT]
            grp = pj if grp is None else grp + pj
            if j % _TIE == _TIE - 1 or j == nt - 1:
                if _CHAIN:
                    acc = grp if acc is None else acc + grp
                    if j > 0:
                        pj = jnp.minimum(pj, acc)
                else:
                    if j % _TIE > 0:
                        pj = jnp.minimum(pj, grp)
                    acc = grp if acc is None else acc + grp
                grp = None
            tiles.append(pj)
        p = tiles[0] if nt == 1 else jnp.concatenate(tiles, axis=1)
        return p, acc

    def scores(q, e, i, zs=()):
        Lm = i * TQ + HT
        nt = Lm // HT
        ties = {(4 + n * (nt - 4) // len(zs)) * QT + 8 * (n % 8): z for n, z in enumerate(zs)}
        keys = _as_bf16(tie(k_s[e, pl.ds(0, Lm // 2), :], ties))
        s_main = _dot_nt(_ld(q, e, i * TQ, TQ), keys)
        s_last = _dot_nt(_ld(q, e, i * TQ + HT, HT), _ld(k_s, e, Lm, HT))
        return s_main, s_last

    def context(e, head, i, s_main, s_last, e_static=0):
        Lm = i * TQ + HT
        top = [jnp.where(tri, s_main[:HT, Lm - HT:], _NEG)]
        if Lm > HT:
            top = [s_main[:HT, :Lm - HT]] + top
        p_top, l_top = softmax_rows(top)
        p_bot, l_bot = softmax_rows([s_main[HT:], jnp.where(tri, s_last, _NEG)])
        p_main = jnp.concatenate([p_top, p_bot[:, :Lm]], axis=0).astype(_BF16)
        o = _dot(p_main, _ld(v_s, e, 0, Lm))
        o_last = _dot(p_bot[:, Lm:].astype(_BF16), _ld(v_s, e, Lm, HT))
        o = jnp.concatenate([o[:HT], o[HT:] + o_last], axis=0)
        acc = jnp.concatenate([l_top, l_bot], axis=0)

        def normalize(pace=None, n0=0):
            zs, z = [], None
            for n, g in enumerate(range(0, TQ, 16)):
                a = acc[g:g + 16]
                if pace is not None:
                    a = a + pltpu.bitcast(pace(n0 + n), _F32)
                linv = jnp.broadcast_to(
                    pl.reciprocal(jnp.sum(a, axis=1, keepdims=True), approx=True), (16, D))
                _st(ctx_s.at[head], None, i * TQ + g, o[g:g + 16] * linv)
                bits = pltpu.bitcast(linv, _U32)
                bits = bits[:8] | bits[8:]
                z = bits if z is None else z | bits
                if n % _NG == _NG - 1:
                    zs.append((z >> 16) >> 16)
                    z = None
            return zs
        return normalize

    def pair_body(s, carry):
        slot = (s + 1) % 2
        odd = s % 2
        wo0 = pl.multiple_of(s * OS, OS)
        q_rd = q_s.at[pl.ds(2 * odd, 2)]
        q_wr = q_s.at[:, pl.ds(pl.multiple_of(odd * (S // 4), S // 4), S // 4), :]
        xn = xn_s.at[pl.ds(pl.multiple_of(odd * (S // 2), S // 2), S // 2), :]
        quad = (s + 1) // 2
        wqb = wqb_s.at[quad % 2]
        pend = {}

        for i in range(NB - 1, -1, -1):
            sa = scores(q_rd, 0, i)
            zs = []
            if i + 2 in pend:
                na, nb = pend.pop(i + 2)
                src = score_tiles([sa[0]], (2 * i + 1) * QT * _PN // 16) if i >= _BIG else kt
                pace = pacer(src, TQ // 8)
                zs = na(pace) + nb(pace, TQ // 16)
            sb = scores(q_rd, 1, i, zs if i >= _BIG else ())
            if i == NB - 1:
                prep_w4((wk_p.at[slot], wv_p.at[slot]), wkvb_s, KQ, range(0, KQ, 16),
                        pacer(score_tiles([sa[0], sb[0]], 3 * TQ + HT), 7 * KQ // 16), 1)
            if i == NB - 2:
                prep_wq(2 * (jnp.minimum(quad + 1, NP // 2 - 1) % 2), (quad + 1) % 2,
                        pl.multiple_of((1 - odd) * (MQ // 2), MQ // 2), MQ // 2,
                        pacer(score_tiles([sa[0], sb[0]], 3 * TQ), 7 * MQ // 32), 64)
            if i in (NB - 3, NB - 4):
                r = (NB - 3 - i) * (OS // 2)
                prep_wo(1 - slot, r, OS // 2, wo0 + r, [sa[0], sb[0]][_WOH:], 2 * TQ + QT)
            if i >= NH:
                project_q(xn, (i - NH) * TQ, wqb, q_wr, (i - NH) * TQ)
            else:
                project_kv(ca_s, (2 * i + 1) * HT, (2 * i + 1) * TQ, () if i >= _BIG else zs)
            pend[i] = (context(0, 2 * s, i, *sa), context(1, 2 * s + 1, i, *sb))
            if i < NH:
                kt = project_kv(ca_s, 2 * i * HT, 2 * i * TQ)
        for i in sorted(pend, reverse=True):
            pend[i][0]()
            pend[i][1]()

        @pl.when(s + 3 < NP)
        def _():
            for cp in w_copies(s + 3, slot):
                cp.start()

        @pl.when(s + 2 < NP)
        def _():
            for cp in wo_copies(s + 2, 1 - slot):
                cp.start()

        @pl.when(s + 6 < NP)
        def _():
            wq_copy(s + 6).start()

        ffn_start(s)

        @pl.when(s == 0)
        def _():
            wq_copy(4).wait()

        @pl.when(s + 5 < NP)
        def _():
            wq_copy(s + 5).wait()

        @pl.when(s + 2 < NP)
        def _():
            for cp in w_copies(s + 2, 1 - slot):
                cp.wait()

        for cp in wo_copies(s + 1, slot):
            cp.wait()
        return carry

    with jax.named_scope('pair_loop'):
        lax.fori_loop(0, NP - 1, pair_body, 0)

    last_slot = (NP - 1) % 2

    def last_body(e, carry):
        half = OS // 2
        q_rd = q_s.at[pl.ds(2, 2)]
        nxt = scores(q_rd, e, NB - 1)
        prep_wo(last_slot, pl.multiple_of(e * half, half), half,
                pl.multiple_of((NP - 1) * OS + e * half, half), [nxt[0]], 3 * TQ)
        for i in range(NB - 1, -1, -1):
            cur = nxt
            if i > 0:
                nxt = scores(q_rd, e, i - 1)
            context(e, H - 2 + e, i, *cur)()
        return carry

    with jax.named_scope('last_loop'):
        lax.fori_loop(0, 2, last_body, 0)

    wr = wr_ref[...].astype(_F32)
    eye = (lax.broadcasted_iota(_I32, (HT, HT), 1) == lax.broadcasted_iota(_I32, (HT, HT), 0))

    def epilogue(g, src):
        r0 = pl.multiple_of(g * HT, HT)
        rs = []
        for c in range(0, HT, _ERG):
            hb = src[pl.ds(c, _ERG), :]
            h_s[pl.ds(r0 + c, _ERG), :] = hb
            hc = hb.astype(_F32)
            hnb = _layernorm(hc).astype(_BF16)
            hn_s[pl.ds(r0 + c, _ERG), :] = hnb
            hn = hnb.astype(_F32)
            rs.append(_round_bf16(jnp.sum(hn * wr, axis=1, keepdims=True)))
            out_s[pl.ds(r0 + c, _ERG), :] = (hc + hn).astype(_BF16)
        r = jnp.concatenate(rs, axis=0)
        r_s[pl.ds(g, 1), :] = jnp.sum(jnp.where(eye, r, 0.0), axis=0, keepdims=True)
        return [pltpu.bitcast(jnp.broadcast_to(t, (_ERG, HT)), _U32) & jnp.uint32(0xFFFF)
                for t in rs]

    def out_copy(g):
        rows = pl.ds(pl.multiple_of(g * HT, HT), HT)
        return pltpu.make_async_copy(out_s.at[rows, :], out_hbm.at[rows, :], sem_out.at[0])

    KS = 2 * D

    def prod(r0, t, ties):
        ps = []
        for u in range(7):
            terms = [(2 * (q1 // 2) + q2 // 2, 2 * (q1 % 2) + q2 % 2, s1 * s2)
                     for q1, s1 in _SA[t] for q2, s2 in _SA[u]]
            fence()
            acc = None
            for k0 in range(0, KO, KS):
                def blk(rb, kb):
                    h0 = (kb * KO + k0) // D
                    return jnp.concatenate(
                        [_ld(ctx_s, h0 + hh, (r0, rb * QT), QT) for hh in range(KS // D)], axis=1)
                if len(terms) == 1:
                    lhs = blk(terms[0][0], terms[0][1])
                else:
                    lhs = _combine([(blk(rb, kb).astype(_F32), sg)
                                    for rb, kb, sg in terms]).astype(_BF16)
                w = wob_s[7 * t + u, pl.ds(k0 // 2, KS // 2), :]
                if k0 == 0 and u in ties:
                    head = jnp.concatenate([w[:_ERG, :HT] | ties[u], w[:_ERG, HT:]], axis=1)
                    w = jnp.concatenate([head, w[_ERG:]], axis=0)
                d = _dot(lhs, _as_bf16(w))
                acc = d if acc is None else acc + d
            ps.append(acc)
        c11, c12, c21, c22 = _strassen_c(ps)
        return jnp.concatenate([jnp.concatenate([c11, c12], axis=1),
                                jnp.concatenate([c21, c22], axis=1)], axis=0)

    def o_body(j, carry):
        r0 = pl.multiple_of(j * TQ, TQ)

        @pl.when(j > 1)
        def _():
            out_copy(2 * j - 4).start()
            out_copy(2 * j - 3).start()

        gp = jnp.maximum(2 * j - 2, 0)
        z = epilogue(gp, ht_s) + epilogue(gp + 1, hb_s)
        ties = [{} for _ in range(7)]
        for zt, (o, u) in zip(z, _OTIES):
            ties[o][u] = zt

        rh = pl.multiple_of(j * (TQ // 2), TQ // 2)
        left, right = pl.ds(0, M // 2), pl.ds(M // 2, M // 2)

        def residual(dst, rows0, cols, att):
            dst[:, cols] = (x_raw[pl.ds(rows0, HT), cols].astype(_F32) + att).astype(_BF16)

        m3 = prod(rh, 2, ties[0])
        m4 = prod(rh, 3, ties[1])
        m5 = prod(rh, 4, ties[2])
        residual(ht_s, r0, right, m3 + m5)
        m1 = prod(rh, 0, ties[3])
        m7 = prod(rh, 6, ties[4])
        residual(ht_s, r0, left, m1 + m4 - m5 + m7)
        m2 = prod(rh, 1, ties[5])
        residual(hb_s, r0 + HT, left, m2 + m4)
        m6 = prod(rh, 5, ties[6])
        residual(hb_s, r0 + HT, right, m1 - m2 + m3 + m6)
        return carry

    for n in range(3):
        ffn_wait(n)
    with jax.named_scope('o_loop'):
        lax.fori_loop(0, NB, o_body, 0)
    out_copy(NG - 4).start()
    out_copy(NG - 3).start()
    epilogue(NG - 2, ht_s)
    epilogue(NG - 1, hb_s)
    out_copy(NG - 2).start()
    out_copy(NG - 1).start()

    r = r_s[pl.ds(0, NG), :] + 0.0
    tok = (lax.broadcasted_iota(_I32, (NG, HT), 0) * HT + lax.broadcasted_iota(_I32, (NG, HT), 1))
    code = pltpu.bitcast(r, _I32) >> 16
    code = jnp.where(code < 0, code ^ 0x7FFF, code) + 0x8000
    key = pltpu.bitcast(((code << _IDX_BITS) | (S - 1 - tok)) + _KEY_BIAS, _F32)
    k1 = jnp.max(jnp.max(key, axis=0, keepdims=True), axis=1, keepdims=True)
    key2 = jnp.where(key == k1, 0.0, key)
    k2 = jnp.max(jnp.max(key2, axis=0, keepdims=True), axis=1, keepdims=True)

    R = _FIX
    row = lax.broadcasted_iota(_I32, (2 * R, 1), 0)
    ki = pltpu.bitcast(jnp.where(row < R, k1, k2), _I32) - _KEY_BIAS
    idx = S - 1 - (ki & (2 ** _IDX_BITS - 1))
    i1 = jnp.clip(idx[0, 0], 0, S - 1)
    i2 = jnp.clip(idx[R, 0], 0, S - 1)
    b1 = pl.multiple_of((i1 // R) * R, R)
    b2 = pl.multiple_of((i2 // R) * R, R)
    tokr = jnp.where(row < R, b1 + row, b2 + row - R)
    cd = ((pltpu.bitcast(jnp.where(tokr == i1, k1, k2), _I32) - _KEY_BIAS) >> _IDX_BITS) - 0x8000
    score = pltpu.bitcast(jnp.where(cd < 0, cd ^ 0x7FFF, cd) << 16, _F32)
    gate = _round_bf16(1.0 / (1.0 + jnp.exp(-score)))

    hnsel = jnp.concatenate([hn_s[pl.ds(b1, R), :].astype(_F32),
                             hn_s[pl.ds(b2, R), :].astype(_F32)], axis=0)
    xs = hnsel.astype(_BF16)
    g = _round_bf16(_dot(xs, wg_s[...]))
    u = _round_bf16(_dot(xs, wu_s[...]))
    g = _round_bf16(g * (1.0 / (1.0 + jnp.exp(-g))))
    act = (g * u).astype(_BF16)
    y = _round_bf16(_dot(act, wd_s[:, pl.ds(0, M)]))
    y = _round_bf16(y * gate)
    upd = jnp.where(jnp.logical_or(tokr == i1, tokr == i2), y, 0.0)
    hsel = jnp.concatenate([h_s[pl.ds(b1, R), :].astype(_F32),
                            h_s[pl.ds(b2, R), :].astype(_F32)], axis=0)
    fixed = hsel + _round_bf16(hnsel + upd)

    pltpu.make_async_copy(out_s, out_hbm, sem_out.at[0]).wait()

    def fix_copy(b0, k):
        return pltpu.make_async_copy(out_s.at[pl.ds(b0, R), :],
                                     out_hbm.at[pl.ds(b0, R), :], sem_out.at[k])

    out_s[pl.ds(b1, R), :] = fixed[:R].astype(_BF16)
    out_s[pl.ds(b2, R), :] = fixed[R:].astype(_BF16)
    fix_copy(b1, 0).start()

    @pl.when(b2 != b1)
    def _():
        fix_copy(b2, 1).start()
        fix_copy(b2, 1).wait()

    fix_copy(b1, 0).wait()


@jax.jit
def pallas_sequential_preLN__compressed_kv_cla__moe_arch_mod__prompt_kernel(
    A_x: jax.Array,
    A_c_kv: jax.Array,
    A_w_q: jax.Array,
    A_w_uk: jax.Array,
    A_w_uv: jax.Array,
    A_w_o: jax.Array,
    B_x: jax.Array,
    B_w_r: jax.Array,
    B_w_gate: jax.Array,
    B_w_up: jax.Array,
    B_w_down: jax.Array,
):
    B, S, M = A_x.shape
    assert B == 1
    DC = A_c_kv.shape[2]
    H, D = A_w_q.shape[1], A_w_q.shape[2]
    F = B_w_gate.shape[1]
    assert A_c_kv.shape[1] == S and S % _TQ == 0 and H % 2 == 0 and S <= 2 ** _IDX_BITS
    NP = H // 2
    NG = S // _HT

    x = A_x.reshape(S, M)
    c = A_c_kv.reshape(S, DC)
    wo = A_w_o.reshape(H * D, M)
    wr = B_w_r.reshape(1, M)

    any_spec = pl.BlockSpec(memory_space=pl.ANY)
    vmem_spec = pl.BlockSpec(memory_space=pltpu.VMEM)
    def buf(name, lead, rows, cols):
        if name in _U32BUF:
            return pltpu.VMEM((lead, rows // 2, cols), _U32)
        return pltpu.VMEM((lead, rows, cols), _BF16)

    scratch = [
        pltpu.VMEM((S, M), _BF16),
        pltpu.VMEM((S, DC), _BF16),
        pltpu.VMEM((S, M), _F32),
        pltpu.VMEM((7, S // 2, DC // 2), _F32),
        buf('q', 4, S, D),
        buf('k', 2, S, D),
        buf('v', 2, S, D),
        pltpu.VMEM((4, M, D), _U32),
        pltpu.VMEM((2, DC, D), _U32),
        pltpu.VMEM((2, DC, D), _U32),
        pltpu.VMEM((2, 49, M // 8, D), _U32),
        buf('wb', 49, DC // 4, D),
        buf('ctx', H, S, D),
        pltpu.VMEM((2, 4, D // 2, M), _BF16),
        buf('wob', 49, H * D // 4, M // 4),
        pltpu.VMEM((M, F), _BF16),
        pltpu.VMEM((M, F), _BF16),
        pltpu.VMEM((F, M + _WD_PAD), _BF16),
        pltpu.VMEM((_HT, M), _BF16),
        pltpu.VMEM((_HT, M), _BF16),
        pltpu.VMEM((S, M), _BF16),
        pltpu.VMEM((S, M), _BF16),
        pltpu.VMEM((NG, _HT), _F32),
        pltpu.VMEM((1024, _HT), _U32),
        pltpu.VMEM((S, M), _BF16),
        pltpu.SemaphoreType.DMA((3,)),
        pltpu.SemaphoreType.DMA((3,)),
        pltpu.SemaphoreType.DMA((2, 2)),
        pltpu.SemaphoreType.DMA((4,)),
        pltpu.SemaphoreType.DMA((2, 4)),
        pltpu.SemaphoreType.DMA((3,)),
        pltpu.SemaphoreType.DMA((2,)),
    ]
    out = pl.pallas_call(
        functools.partial(_kernel, S=S, M=M, DC=DC, H=H, D=D, F=F),
        in_specs=[any_spec, any_spec, any_spec, any_spec, any_spec, any_spec,
                  vmem_spec, any_spec, any_spec, any_spec],
        out_specs=any_spec,
        out_shape=jax.ShapeDtypeStruct((S, M), _BF16),
        scratch_shapes=scratch,
        compiler_params=pltpu.CompilerParams(vmem_limit_bytes=124 * 1024 * 1024,
                                             disable_bounds_checks=True,
                                             disable_semaphore_checks=True),
        name="fused_mla_mod",
    )(x, c, A_w_q, A_w_uk, A_w_uv, wo, wr, B_w_gate, B_w_up, B_w_down)
    return out.reshape(B, S, M)
```

```python
import functools
import math

import jax
import jax.numpy as jnp
from jax import lax
import jax.experimental.pallas as pl
import jax.experimental.pallas.tpu as pltpu

_F32 = jnp.float32
_BF16 = jnp.bfloat16
_U32 = jnp.uint32
_I32 = jnp.int32

_EPS = 1e-5
_NEG = -1e30
_TQ = 256
_HT = 128
import os
_TIE = int(os.environ.get('TIE', 4))
_CHAIN = int(os.environ.get('CHAIN', 0))
_ERG = int(os.environ.get('ERG', 16))
_EORD = int(os.environ.get('EORD', 0))
_EVAL = int(os.environ.get('EVAL', 1))
_U32BUF = os.environ.get('U32', 'xa,ca,q,k,v,wob,ctx,wb').split(',')
_PA = int(os.environ.get('PA', 13))
_PB = int(os.environ.get('PB', 13))
_PC = int(os.environ.get('PC', 16))
_PX = int(os.environ.get('PX', 8))
_OT = {
    0: [(0, 2), (0, 3), (0, 4), (0, 5), (0, 6), (1, 0), (1, 1), (1, 2),
        (1, 3), (1, 4), (1, 5), (1, 6), (2, 0), (2, 3), (2, 4), (3, 4)],
    1: [(0, 2), (0, 3), (0, 4), (0, 6), (1, 1), (1, 2), (1, 3), (1, 4),
        (1, 6), (2, 3), (2, 4), (3, 3), (3, 4), (4, 3), (4, 4), (5, 3)],
    2: [(0, 2), (0, 3), (0, 5), (0, 6), (1, 1), (1, 3), (1, 4), (1, 6),
        (2, 2), (2, 4), (2, 6), (3, 2), (3, 4), (4, 0), (4, 3), (4, 5)],
}
_OTIES = _OT[int(os.environ.get('OT', 1))]
_WQS = int(os.environ.get('WQS', 672))
_NG = int(os.environ.get('NG', 16))
_BIG = int(os.environ.get('BIG', 3))
_TSPAN = 360
_DIST = int(os.environ.get('DIST', 2))
_PN = int(os.environ.get('PN', 14))
_WOH = int(os.environ.get('WOH', 0))
_LND = int(os.environ.get('LND', 6))
_FR = int(os.environ.get('FR', 2))
_LATE = int(os.environ.get('LATE', 2))
_TIEL = int(os.environ.get('TIEL', 3))
_LD = int(os.environ.get('LD', 9))
_LORD = [int(c) for c in os.environ.get('LORD', '76543210')]
_IDX_BITS = 13
_KEY_BIAS = 0x20000000
_FIX = 8
_WD_PAD = 128


def _dot(a, b):
    return jnp.dot(a, b, preferred_element_type=_F32)


def _dot_nt(a, b):
    return lax.dot_general(a, b, (((1,), (1,)), ((), ())), preferred_element_type=_F32)


def _as_bf16(u):
    return pltpu.bitcast(u, _BF16)


def _pack(x):
    return pltpu.bitcast(x.astype(_BF16), _U32)


def _rows(ref, r0, n):
    if ref.dtype == _U32:
        if isinstance(r0, tuple):
            return pl.ds(r0[0] + r0[1] // 2, n // 2)
        if isinstance(r0, int):
            return pl.ds(r0 // 2, n // 2)
        return pl.ds(pl.multiple_of(r0 // 2, 8), n // 2)
    return pl.ds(r0, n)


def _ld(ref, lead, r0, n):
    v = ref[lead, _rows(ref, r0, n), :]
    return _as_bf16(v) if ref.dtype == _U32 else v


def _st(ref, lead, r0, x, cols=slice(None)):
    v = _pack(x) if ref.dtype == _U32 else x.astype(_BF16)
    if lead is None:
        ref[_rows(ref, r0, x.shape[0]), cols] = v
    else:
        ref[lead, _rows(ref, r0, x.shape[0]), cols] = v


def _round_bf16(x):
    return x.astype(_BF16).astype(_F32)


def _layernorm(x):
    n = x.shape[-1]
    mean = jnp.sum(x, axis=-1, keepdims=True) * (1.0 / n)
    xc = x - mean
    var = jnp.sum(xc * xc, axis=-1, keepdims=True) * (1.0 / n)
    m = _round_bf16(mean)
    den = _round_bf16(jnp.sqrt(_round_bf16(_round_bf16(var) + _EPS)))
    return (x - m) * (1.0 / den)


def _layernorm_scaled(x, scale):
    n = x.shape[-1]
    mean = jnp.sum(x, axis=-1, keepdims=True) * (1.0 / n)
    xc = x - mean
    var = jnp.sum(xc * xc, axis=-1, keepdims=True) * (1.0 / n)
    return xc * (lax.rsqrt(var + _EPS) * scale)


def _strassen_a(a11, a12, a21, a22):
    return (a11 + a22, a21 + a22, a11, a22, a11 + a12, a21 - a11, a12 - a22)


def _strassen_b(b11, b12, b21, b22):
    return (b11 + b22, b11, b12 - b22, b21 - b11, b22, b11 + b12, b21 + b22)


def _strassen_c(m):
    m1, m2, m3, m4, m5, m6, m7 = m
    return (m4 - m5 + m1 + m7, m3 + m5, m4 + m2, m3 - m2 + m1 + m6)


_ORDER = (2, 4, 3, 1, 0, 6, 5)


_SA = (((0, 1), (3, 1)), ((2, 1), (3, 1)), ((0, 1),), ((3, 1),),
       ((0, 1), (1, 1)), ((2, 1), (0, -1)), ((1, 1), (3, -1)))
_SB = (((0, 1), (3, 1)), ((0, 1),), ((1, 1), (3, -1)), ((2, 1), (0, -1)),
       ((3, 1),), ((0, 1), (1, 1)), ((2, 1), (3, 1)))


def _combine(terms):
    terms = sorted(terms, key=lambda ts: -ts[1])
    acc = terms[0][0]
    assert terms[0][1] > 0
    for v, sg in terms[1:]:
        acc = acc + v if sg > 0 else acc - v
    return acc


def _quadrants(x):
    r, c = x.shape[0] // 2, x.shape[1] // 2
    return x[:r, :c], x[:r, c:], x[r:, :c], x[r:, c:]


def _kernel(x_hbm, c_hbm, wq_hbm, wk_hbm, wv_hbm, wo_hbm, wr_ref, wg_hbm, wu_hbm, wd_hbm,
            out_hbm,
            x_raw, c_raw, xn_s, ca_s, q_s, k_s, v_s,
            wq_p, wk_p, wv_p, wqb_s, wkvb_s,
            ctx_s, wo_p, wob_s, wg_s, wu_s, wd_s, ht_s, hb_s, h_s, hn_s, r_s, junk_s, out_s,
            sem_x, sem_c, sem_w, sem_wq, sem_wo, sem_ffn, sem_out,
            *, S, M, DC, H, D, F):
    TQ, HT = _TQ, _HT
    NB = S // TQ
    NG = S // HT
    NP = H // 2
    KO = H * D // 4
    NO = M // 4
    OS = KO // NP
    qscale = (D ** -0.5) * math.log2(math.e)

    wq32 = wq_hbm.bitcast(_U32)
    wk32 = wk_hbm.bitcast(_U32)
    wv32 = wv_hbm.bitcast(_U32)

    def w_copies(pair, slot):
        return (
            pltpu.make_async_copy(wk32.at[:, pair, :], wk_p.at[slot], sem_w.at[slot, 0]),
            pltpu.make_async_copy(wv32.at[:, pair, :], wv_p.at[slot], sem_w.at[slot, 1]),
        )

    def wq_copy(pair):
        return pltpu.make_async_copy(wq32.at[:, pair, :], wq_p.at[pair % 4],
                                     sem_wq.at[pair % 4])

    def wo_copies(t, slot):
        r0 = pl.multiple_of(t * OS, OS)
        return tuple(
            pltpu.make_async_copy(wo_hbm.at[pl.ds(half * KO + r0, OS), :],
                                  wo_p.at[slot, half], sem_wo.at[slot, half])
            for half in range(4))

    def x_copy(i, n):
        rows = pl.ds(pl.multiple_of(i * TQ, TQ), TQ)
        return pltpu.make_async_copy(x_hbm.at[rows, :], x_raw.at[rows, :], sem_x.at[n % 3])

    def c_copy(i):
        rows = pl.ds(pl.multiple_of(i * 2 * TQ, 2 * TQ), 2 * TQ)
        return pltpu.make_async_copy(c_hbm.at[rows, :], c_raw.at[rows, :], sem_c.at[i % 3])

    ffn = ((wg_hbm, wg_s), (wu_hbm, wu_s), (wd_hbm, wd_s))

    def ffn_start(t):
        for n, (src, dst) in enumerate(ffn):
            rows, cols = src.shape[0] // NP, src.shape[1]
            r0 = pl.multiple_of(t * rows, 16)
            pltpu.make_async_copy(src.at[pl.ds(r0, rows), :],
                                  dst.at[pl.ds(r0, rows), pl.ds(0, cols)],
                                  sem_ffn.at[n]).start()

    def ffn_wait(n):
        src, dst = ffn[n]
        pltpu.make_async_copy(src, dst.at[:, pl.ds(0, src.shape[1])], sem_ffn.at[n]).wait()

    def lo_hi(w):
        return (pltpu.bitcast(w << 16, _F32), pltpu.bitcast(w & jnp.uint32(0xFFFF0000), _F32))

    def pacer(tiles, total, free=0):
        def zero(n):
            if n < free:
                return jnp.zeros((16, HT), _U32)
            mat, zr, zc = tiles[(n - free) * len(tiles) // (total - free)]
            z = pltpu.bitcast(mat[zr:zr + 8, zc:zc + HT], _U32)
            z = (z >> 16) >> 16
            return jnp.concatenate([z, z], axis=0)
        return zero

    def score_tiles(mats, span):
        return [(m, t0 % TQ, (t0 // TQ) * 4 * HT) for m in mats for t0 in range(0, span, 8)]

    def prep_w4(srcs, dst, kq, rows, pace=None, sink=None):
        pieces = [(t, r) for t in range(7) for r in rows]
        for n, (t, r) in enumerate(pieces):
            terms = [[] for _ in range(4)]
            for k, (q1, sg) in enumerate(_SB[t]):
                for rb in range(2):
                    w = srcs[q1 % 2][pl.ds((2 * (q1 // 2) + rb) * kq + r, 16), :]
                    if pace is not None and k == 0:
                        w = w | pace(n)
                    lo, hi = lo_hi(w)
                    terms[2 * rb].append((lo, sg))
                    terms[2 * rb + 1].append((hi, sg))
            z = None
            for u, b in enumerate(_strassen_b(*[_combine(tm) for tm in terms])):
                pk = _pack(b)
                dst[7 * t + u, pl.ds(r // 2, 8), :] = pk
                z = pk if z is None else z | pk
            if sink is not None:
                junk_s[pl.ds(8 * (sink + n), 8), :] = z

    def prep_wo(slot, src0, nrows, dst0, mats, span):
        pieces = [(r, c0, t) for r in range(0, nrows, 16) for c0 in range(0, NO, HT)
                  for t in range(7)]
        pace = pacer(score_tiles(mats, span), len(pieces))
        for n, (r, c0, t) in enumerate(pieces):
            z = pltpu.bitcast(pace(n), _F32)
            rs = pl.ds(src0 + r, 16)
            sub = []
            for q2 in range(4):
                v = _combine([
                    (wo_p[slot, 2 * (q1 // 2) + q2 // 2, rs,
                          pl.ds((2 * (q1 % 2) + q2 % 2) * NO + c0, HT)].astype(_F32), sg)
                    for q1, sg in _SB[t]])
                sub.append(v + z if q2 in (0, 3) else v)
            for u, b in enumerate(_strassen_b(*sub)):
                _st(wob_s, 7 * t + u, dst0 + r, b, pl.ds(c0, HT))

    QT = HT // 2
    KQ = DC // 4
    MQ = M // 4

    def fence():
        junk_s[pl.ds(0, 8), :] = jnp.zeros((8, HT), _U32)

    def tie(w, ties):
        parts, at = [], 0
        for r in sorted(ties):
            if r > at:
                parts.append(w[at:r])
            parts.append(w[r:r + 8] | ties[r])
            at = r + 8
        if at < w.shape[0]:
            parts.append(w[at:])
        return parts[0] if len(parts) == 1 else jnp.concatenate(parts, axis=0)

    def project4(lhs, w, store, zs=()):
        m, tiles, cnt = [None] * 7, [], [0]
        for t in _ORDER:
            ps = [None] * 7
            for u in _ORDER:
                fence()
                a = lhs(t, u)
                wt = w[7 * t + u]
                n = len(tiles) * len(zs) * D * 8 // (_TSPAN * a.shape[1] * 2)
                done = cnt[0]
                if zs and done < len(zs) and n > done:
                    wt = tie(wt, {0: zs[done]})
                    cnt[0] += 1
                ps[u] = _dot(a.astype(_BF16), _as_bf16(wt))
                tiles += [(ps[u], r, 0) for r in range(0, QT, QT * D // (2 * a.shape[1]))]
            m[t] = _strassen_c(ps)
        for q2 in range(4):
            for q1, cblk in enumerate(_strassen_c([mt[q2] for mt in m])):
                store(2 * (q1 % 2) + q2 % 2, (2 * (q1 // 2) + q2 // 2) * QT, cblk)
        return tiles

    def project_q(xn, x0, wqb, q, r0):
        def lhs(t, u):
            return _combine([
                (xn[pl.ds(x0 + (2 * (q1 // 2) + q2 // 2) * QT, QT),
                    pl.ds((2 * (q1 % 2) + q2 % 2) * MQ, MQ)], s1 * s2)
                for q1, s1 in _SA[t] for q2, s2 in _SA[u]])
        return project4(lhs, wqb, lambda nb, r, val: _st(q, nb, r0 + r, val))

    def project_kv(ca, a0, r0, zs=()):
        def lhs(t, u):
            return _combine([
                (ca[t, pl.ds(a0 + (q2 // 2) * QT, QT), pl.ds((q2 % 2) * KQ, KQ)], sg)
                for q2, sg in _SA[u]])
        return project4(lhs, wkvb_s,
                        lambda nb, r, val: _st((k_s, v_s)[nb // 2], nb % 2, r0 + r, val), zs)

    def prep_wq(raw, slot, r, nr, pace, sink=None):
        span = 3 * MQ + nr
        prep_w4((wq_p.at[raw, pl.ds(r, span), :], wq_p.at[raw + 1, pl.ds(r, span), :]),
                wqb_s.at[slot, :, pl.ds(pl.multiple_of(r // 2, 8), nr // 2), :],
                MQ, range(0, nr, 16), pace, sink)

    NH = NB // 2

    def plain_weights(src0, src1):
        return jnp.concatenate(lo_hi(src0[...]) + lo_hi(src1[...]), axis=1).astype(_BF16)

    def stage_x(r0, xn, x0, pace):
        done = []
        for n, c in enumerate(range(0, TQ, _PX)):
            xr = x_raw[pl.ds(r0 + c, _PX), :].astype(_F32)
            z = pace(n)[:_PX]
            if n >= _LND:
                z = z | done[n - _LND]
            xr = jnp.concatenate([xr[:, :HT] + pltpu.bitcast(z, _F32), xr[:, HT:]], axis=1)
            y = _layernorm_scaled(xr, qscale)
            xn[pl.ds(x0 + c, _PX), :] = y
            done.append((pltpu.bitcast(y[:, :HT], _U32) >> 16) >> 16)

    def stage_c(r0, a0, pace):
        kh = DC // 2
        for n, c in enumerate(range(0, HT, 8)):
            top = c_raw[pl.ds(r0 + c, 8), :].astype(_F32)
            bot = c_raw[pl.ds(r0 + HT + c, 8), :].astype(_F32)
            z = pltpu.bitcast(pace(n)[:8], _F32)
            z = jnp.concatenate([z] * (kh // HT), axis=1)
            for t, a in enumerate(
                    _strassen_a(top[:, :kh] + z, top[:, kh:], bot[:, :kh], bot[:, kh:] + z)):
                ca_s[t, pl.ds(a0 + c, 8), :] = a

    def xs_copy(n):
        return x_copy((n + NH) % NB, n)

    for cp in w_copies(0, 0):
        cp.start()
    c_copy(0).start()
    xs_copy(0).start()
    ht_s[...] = jnp.zeros((HT, M), _BF16)
    hb_s[...] = jnp.zeros((HT, M), _BF16)
    for cp in w_copies(0, 0):
        cp.wait()
    c_copy(1).start()
    xs_copy(1).start()
    c_copy(0).wait()
    xs_copy(0).wait()

    def pro_a(i, carry):
        @pl.when(i + 2 < NH)
        def _():
            c_copy(i + 2).start()

        @pl.when(i + 2 <= NH)
        def _():
            xs_copy(i + 2).start()

        @pl.when(jnp.logical_and(i >= 1, i <= 2))
        def _():
            wq_copy(i - 1).start()

        @pl.when(i > 0)
        def _():
            c_copy(i).wait()
            xs_copy(i).wait()

        r0 = pl.multiple_of(i * 2 * TQ, 2 * TQ)
        kv = _dot(c_raw[pl.ds(r0, 2 * TQ), :], plain_weights(wk_p.at[0], wv_p.at[0]))
        for nb in range(4):
            _st((k_s, v_s)[nb // 2], nb % 2, r0, kv[:, nb * D:(nb + 1) * D])
        tiles = [(kv, r, nb * D) for nb in range(4) for r in range(0, 2 * TQ, 8)]
        nt = len(tiles)
        a0 = pl.multiple_of(i * TQ, TQ)
        stage_c(r0, a0, pacer(tiles[:nt // 2], HT // 8))
        stage_c(r0 + TQ, a0 + HT, pacer(tiles[nt // 2:nt * 15 // 16], HT // 8))
        rx = pl.multiple_of((i + NH) * TQ, TQ)
        stage_x(rx, xn_s, rx, pacer(tiles[:nt * _PA // 16], TQ // _PX, _FR))
        return carry

    def pro_b(i, carry):
        @pl.when(i + 2 < NH)
        def _():
            xs_copy(NH + i + 2).start()

        @pl.when(i == 2)
        def _():
            for cp in w_copies(1, 1) + wo_copies(0, 0):
                cp.start()
            wq_copy(2).wait()
            wq_copy(3).wait()

        xs_copy(NH + i).wait()
        r0 = pl.multiple_of(i * TQ, TQ)
        xn = xn_s.at[pl.ds(r0, S // 2 + TQ), :]
        kh = M // 2
        lhs = [xn[pl.ds(S // 2, TQ), pl.ds(k0, kh)].astype(_BF16) for k0 in (0, kh)]
        tiles = []
        for nb in range(4):
            d = [_dot(lhs[k], lo_hi(wq_p[nb // 2, pl.ds(k * kh, kh), :])[nb % 2].astype(_BF16))
                 for k in range(2)]
            _st(q_s, nb, r0 + S // 2, d[0] + d[1])
            tiles += [(dk, r, 0) for dk in d for r in range(0, TQ, 8)]
        nt = len(tiles)
        stage_x(r0, xn, 0, pacer(tiles[:nt * _PB // 16], TQ // _PX, _FR))
        nr = MQ // (2 * NH)
        npc = 7 * nr // 16
        pace = pacer(tiles[:nt * _PC // 16], 3 * npc, _FR)
        for k in range(3):
            u = 3 * i + k
            quad = u // (2 * NH)
            prep_wq(2 * quad, quad, pl.multiple_of((u % (2 * NH)) * nr, nr), nr,
                    lambda n, k=k: pace(k * npc + n))
        return carry

    with jax.named_scope('pro_a'):
        lax.fori_loop(0, NH, pro_a, 0)
    wq_copy(0).wait()
    wq_copy(1).wait()
    xs_copy(NH + 1).start()
    wq_copy(2).start()
    wq_copy(3).start()
    with jax.named_scope('pro_b'):
        lax.fori_loop(0, NH, pro_b, 0)

    for cp in w_copies(2, 0) + wo_copies(1, 1) + (wq_copy(4), wq_copy(5)):
        cp.start()
    ffn_start(NP - 1)
    for cp in w_copies(1, 1) + wo_copies(0, 0):
        cp.wait()

    tri = (lax.broadcasted_iota(_I32, (HT, HT), 1)
           <= lax.broadcasted_iota(_I32, (HT, HT), 0))

    def softmax_rows(parts, _TIE):
        s = parts[0] if len(parts) == 1 else jnp.concatenate(parts, axis=1)
        m = jnp.max(s, axis=1, keepdims=True)
        p = jnp.exp2(s - m)
        nt = p.shape[1] // HT
        tiles, acc, grp = [], None, None
        for j in range(nt):
            pj = p[:, j * HT:(j + 1) * HT]
            grp = pj if grp is None else grp + pj
            if j % _TIE == _TIE - 1 or j == nt - 1:
                if _CHAIN:
                    acc = grp if acc is None else acc + grp
                    if j > 0:
                        pj = jnp.minimum(pj, acc)
                else:
                    if j % _TIE > 0:
                        pj = jnp.minimum(pj, grp)
                    acc = grp if acc is None else acc + grp
                grp = None
            tiles.append(pj)
        p = tiles[0] if nt == 1 else jnp.concatenate(tiles, axis=1)
        return p, acc

    def scores(q, e, i, zs=()):
        Lm = i * TQ + HT
        nt = Lm // HT
        ties = {(4 + n * (nt - 4) // len(zs)) * QT + 8 * (n % 8): z for n, z in enumerate(zs)}
        keys = _as_bf16(tie(k_s[e, pl.ds(0, Lm // 2), :], ties))
        s_main = _dot_nt(_ld(q, e, i * TQ, TQ), keys)
        s_last = _dot_nt(_ld(q, e, i * TQ + HT, HT), _ld(k_s, e, Lm, HT))
        return s_main, s_last

    def values(e, i):
        Lm = i * TQ + HT
        return _ld(v_s, e, 0, Lm), _ld(v_s, e, Lm, HT)

    def context(vals, head, i, s_main, s_last, group=_TIE):
        Lm = i * TQ + HT
        top = [jnp.where(tri, s_main[:HT, Lm - HT:], _NEG)]
        if Lm > HT:
            top = [s_main[:HT, :Lm - HT]] + top
        p_top, l_top = softmax_rows(top, group)
        p_bot, l_bot = softmax_rows([s_main[HT:], jnp.where(tri, s_last, _NEG)], group)
        p_main = jnp.concatenate([p_top, p_bot[:, :Lm]], axis=0).astype(_BF16)
        o = _dot(p_main, vals[0])
        o_last = _dot(p_bot[:, Lm:].astype(_BF16), vals[1])
        o = jnp.concatenate([o[:HT], o[HT:] + o_last], axis=0)
        acc = jnp.concatenate([l_top, l_bot], axis=0)

        def normalize(pace=None, n0=0):
            zs, z = [], None
            for n, g in enumerate(range(0, TQ, 16)):
                a = acc[g:g + 16]
                if pace is not None:
                    a = a + pltpu.bitcast(pace(n0 + n), _F32)
                linv = jnp.broadcast_to(
                    pl.reciprocal(jnp.sum(a, axis=1, keepdims=True), approx=True), (16, D))
                _st(ctx_s.at[head], None, i * TQ + g, o[g:g + 16] * linv)
                bits = pltpu.bitcast(linv, _U32)
                bits = bits[:8] | bits[8:]
                z = bits if z is None else z | bits
                if n % _NG == _NG - 1:
                    zs.append((z >> 16) >> 16)
                    z = None
            return zs
        return normalize

    def pair_body(s, carry):
        slot = (s + 1) % 2
        odd = s % 2
        wo0 = pl.multiple_of(s * OS, OS)
        q_rd = q_s.at[pl.ds(2 * odd, 2)]
        q_wr = q_s.at[:, pl.ds(pl.multiple_of(odd * (S // 4), S // 4), S // 4), :]
        xn = xn_s.at[pl.ds(pl.multiple_of(odd * (S // 2), S // 2), S // 2), :]
        quad = (s + 1) // 2
        wqb = wqb_s.at[quad % 2]
        pend, sc = {}, {}

        def norm(blocks, tiles):
            fns = [f for i in blocks for f in pend.pop(i)]
            pace = pacer(tiles, len(fns) * (TQ // 16))
            return [z for k, f in enumerate(fns) for z in f(pace, k * (TQ // 16))]

        def qk(i, nrm=()):
            sa = scores(q_rd, 0, i)
            zs = norm(nrm, score_tiles([sa[0]], (2 * i + 1) * QT * _PN // 16)) if nrm else ()
            sc[i] = (sa, scores(q_rd, 1, i, zs))
            return [sa[0], sc[i][1][0]]

        def pv(i):
            pend[i] = [context(values(e, i), 2 * s + e, i, *sc[i][e]) for e in range(2)]

        def kv(j, zs=()):
            return project_kv(ca_s, j * HT, j * TQ, zs)

        for i in range(NB - 1, NH - 1, -1):
            mats = qk(i, [i + 2] if i + 2 < NB else [])
            if i == NB - 1:
                prep_w4((wk_p.at[slot], wv_p.at[slot]), wkvb_s, KQ, range(0, KQ, 16),
                        pacer(score_tiles(mats, 3 * TQ + HT), 7 * KQ // 16), 1)
            if i == NB - 2:
                prep_wq(2 * (jnp.minimum(quad + 1, NP // 2 - 1) % 2), (quad + 1) % 2,
                        pl.multiple_of((1 - odd) * (MQ // 2), MQ // 2), MQ // 2,
                        pacer(score_tiles(mats, _WQS), 7 * MQ // 32), 64)
            if i in (NB - 3, NB - 4):
                r = (NB - 3 - i) * (OS // 2)
                prep_wo(1 - slot, r, OS // 2, wo0 + r, mats, 2 * TQ + QT)
            project_q(xn, (i - NH) * TQ, wqb, q_wr, (i - NH) * TQ)
            pv(i)
        assert NH == 4
        if _LATE == 0:
            qk(1); qk(0); t = kv(7); z = norm([5], t[len(t) // 4:]); pv(1); pv(0); kv(6, z)
            qk(3, [4]); t = kv(5); z = norm([1, 0], t); pv(3); kv(4, z)
            qk(2); kv(3); pv(2)
            t = kv(2); t = kv(1, norm([3], t)); kv(0, norm([2], t))
        elif _LATE == 1:
            qk(3, [5]); kv(7); pv(3); t = kv(6)
            z = norm([4], t); qk(1); qk(0); kv(5, z); pv(1); pv(0); t = kv(4)
            z = norm([3], t); qk(2); kv(3, z); pv(2)
            t = kv(2); t = kv(1, norm([1, 0], t)); kv(0, norm([2], t))
        elif _LATE == 2:
            qk(3, [5]); qk(0); kv(7); pv(3); pv(0); t = kv(6)
            z = norm([4], t); qk(2); qk(1); kv(5, z); pv(2); pv(1)
            t = kv(4); t = kv(3, norm([3], t)); t = kv(2, norm([0], t))
            t = kv(1, norm([2], t)); kv(0, norm([1], t))
        assert not pend

        @pl.when(s + 3 < NP)
        def _():
            for cp in w_copies(s + 3, slot):
                cp.start()

        @pl.when(s + 2 < NP)
        def _():
            for cp in wo_copies(s + 2, 1 - slot):
                cp.start()

        @pl.when(s + 6 < NP)
        def _():
            wq_copy(s + 6).start()

        ffn_start(s)

        @pl.when(s == 0)
        def _():
            wq_copy(4).wait()

        @pl.when(s + 5 < NP)
        def _():
            wq_copy(s + 5).wait()

        @pl.when(s + 2 < NP)
        def _():
            for cp in w_copies(s + 2, 1 - slot):
                cp.wait()

        for cp in wo_copies(s + 1, slot):
            cp.wait()
        return carry

    with jax.named_scope('pair_loop'):
        lax.fori_loop(0, NP - 1, pair_body, 0)

    last_slot = (NP - 1) % 2

    def last_body(e, carry):
        half = OS // 2
        q_rd = q_s.at[pl.ds(2, 2)]
        order = _LORD
        sc = {order[0]: scores(q_rd, e, order[0])}
        prep_wo(last_slot, pl.multiple_of(e * half, half), half,
                pl.multiple_of((NP - 1) * OS + e * half, half), [sc[order[0]][0]], 3 * TQ)
        pend, zs = [], ()
        for n, i in enumerate(order):
            if n + 1 < NB:
                j = order[n + 1]
                sc[j] = scores(q_rd, e, j, zs if j >= 3 else ())
                zs = ()
                if len(pend) >= _LD and n + 2 < NB and order[n + 2] >= 3:
                    zs = pend.pop(0)(pacer(score_tiles([sc[j][0]], (2 * j + 1) * QT), TQ // 16))
            pend.append(context(values(e, i), H - 2 + e, i, *sc[i], group=_TIEL))
        for f in pend:
            f()
        return carry

    with jax.named_scope('last_loop'):
        lax.fori_loop(0, 2, last_body, 0)

    wr = wr_ref[...].astype(_F32)
    eye = (lax.broadcasted_iota(_I32, (HT, HT), 1) == lax.broadcasted_iota(_I32, (HT, HT), 0))

    def epilogue(g, src):
        r0 = pl.multiple_of(g * HT, HT)
        rs = []
        for c in range(0, HT, _ERG):
            hb = src[pl.ds(c, _ERG), :]
            h_s[pl.ds(r0 + c, _ERG), :] = hb
            hc = hb.astype(_F32)
            hnb = _layernorm(hc).astype(_BF16)
            hn_s[pl.ds(r0 + c, _ERG), :] = hnb
            hn = hnb.astype(_F32)
            rs.append(_round_bf16(jnp.sum(hn * wr, axis=1, keepdims=True)))
            out_s[pl.ds(r0 + c, _ERG), :] = (hc + hn).astype(_BF16)
        r = jnp.concatenate(rs, axis=0)
        r_s[pl.ds(g, 1), :] = jnp.sum(jnp.where(eye, r, 0.0), axis=0, keepdims=True)
        return [pltpu.bitcast(jnp.broadcast_to(t, (_ERG, HT)), _U32) & jnp.uint32(0xFFFF)
                for t in rs]

    def out_copy(g):
        rows = pl.ds(pl.multiple_of(g * HT, HT), HT)
        return pltpu.make_async_copy(out_s.at[rows, :], out_hbm.at[rows, :], sem_out.at[0])

    KS = 2 * D

    def prod(r0, t, ties):
        ps = []
        for u in range(7):
            terms = [(2 * (q1 // 2) + q2 // 2, 2 * (q1 % 2) + q2 % 2, s1 * s2)
                     for q1, s1 in _SA[t] for q2, s2 in _SA[u]]
            fence()
            acc = None
            for k0 in range(0, KO, KS):
                def blk(rb, kb):
                    h0 = (kb * KO + k0) // D
                    return jnp.concatenate(
                        [_ld(ctx_s, h0 + hh, (r0, rb * QT), QT) for hh in range(KS // D)], axis=1)
                if len(terms) == 1:
                    lhs = blk(terms[0][0], terms[0][1])
                else:
                    lhs = _combine([(blk(rb, kb).astype(_F32), sg)
                                    for rb, kb, sg in terms]).astype(_BF16)
                w = wob_s[7 * t + u, pl.ds(k0 // 2, KS // 2), :]
                if k0 == 0 and u in ties:
                    head = jnp.concatenate([w[:_ERG, :HT] | ties[u], w[:_ERG, HT:]], axis=1)
                    w = jnp.concatenate([head, w[_ERG:]], axis=0)
                d = _dot(lhs, _as_bf16(w))
                acc = d if acc is None else acc + d
            ps.append(acc)
        c11, c12, c21, c22 = _strassen_c(ps)
        return jnp.concatenate([jnp.concatenate([c11, c12], axis=1),
                                jnp.concatenate([c21, c22], axis=1)], axis=0)

    def o_body(j, carry):
        r0 = pl.multiple_of(j * TQ, TQ)

        @pl.when(j > 1)
        def _():
            out_copy(2 * j - 4).start()
            out_copy(2 * j - 3).start()

        gp = jnp.maximum(2 * j - 2, 0)
        z = epilogue(gp, ht_s) + epilogue(gp + 1, hb_s)
        ties = [{} for _ in range(7)]
        for zt, (o, u) in zip(z, _OTIES):
            ties[o][u] = zt

        rh = pl.multiple_of(j * (TQ // 2), TQ // 2)
        left, right = pl.ds(0, M // 2), pl.ds(M // 2, M // 2)

        def residual(dst, rows0, cols, att):
            dst[:, cols] = (x_raw[pl.ds(rows0, HT), cols].astype(_F32) + att).astype(_BF16)

        m3 = prod(rh, 2, ties[0])
        m4 = prod(rh, 3, ties[1])
        m5 = prod(rh, 4, ties[2])
        residual(ht_s, r0, right, m3 + m5)
        m1 = prod(rh, 0, ties[3])
        m7 = prod(rh, 6, ties[4])
        residual(ht_s, r0, left, m1 + m4 - m5 + m7)
        m2 = prod(rh, 1, ties[5])
        residual(hb_s, r0 + HT, left, m2 + m4)
        m6 = prod(rh, 5, ties[6])
        residual(hb_s, r0 + HT, right, m1 - m2 + m3 + m6)
        return carry

    for n in range(3):
        ffn_wait(n)
    with jax.named_scope('o_loop'):
        lax.fori_loop(0, NB, o_body, 0)
    out_copy(NG - 4).start()
    out_copy(NG - 3).start()
    epilogue(NG - 2, ht_s)
    epilogue(NG - 1, hb_s)
    out_copy(NG - 2).start()
    out_copy(NG - 1).start()

    r = r_s[pl.ds(0, NG), :] + 0.0
    tok = (lax.broadcasted_iota(_I32, (NG, HT), 0) * HT + lax.broadcasted_iota(_I32, (NG, HT), 1))
    code = pltpu.bitcast(r, _I32) >> 16
    code = jnp.where(code < 0, code ^ 0x7FFF, code) + 0x8000
    key = pltpu.bitcast(((code << _IDX_BITS) | (S - 1 - tok)) + _KEY_BIAS, _F32)
    k1 = jnp.max(jnp.max(key, axis=0, keepdims=True), axis=1, keepdims=True)
    key2 = jnp.where(key == k1, 0.0, key)
    k2 = jnp.max(jnp.max(key2, axis=0, keepdims=True), axis=1, keepdims=True)

    R = _FIX
    row = lax.broadcasted_iota(_I32, (2 * R, 1), 0)
    ki = pltpu.bitcast(jnp.where(row < R, k1, k2), _I32) - _KEY_BIAS
    idx = S - 1 - (ki & (2 ** _IDX_BITS - 1))
    i1 = jnp.clip(idx[0, 0], 0, S - 1)
    i2 = jnp.clip(idx[R, 0], 0, S - 1)
    b1 = pl.multiple_of((i1 // R) * R, R)
    b2 = pl.multiple_of((i2 // R) * R, R)
    tokr = jnp.where(row < R, b1 + row, b2 + row - R)
    cd = ((pltpu.bitcast(jnp.where(tokr == i1, k1, k2), _I32) - _KEY_BIAS) >> _IDX_BITS) - 0x8000
    score = pltpu.bitcast(jnp.where(cd < 0, cd ^ 0x7FFF, cd) << 16, _F32)
    gate = _round_bf16(1.0 / (1.0 + jnp.exp(-score)))

    hnsel = jnp.concatenate([hn_s[pl.ds(b1, R), :].astype(_F32),
                             hn_s[pl.ds(b2, R), :].astype(_F32)], axis=0)
    xs = hnsel.astype(_BF16)
    g = _round_bf16(_dot(xs, wg_s[...]))
    u = _round_bf16(_dot(xs, wu_s[...]))
    g = _round_bf16(g * (1.0 / (1.0 + jnp.exp(-g))))
    act = (g * u).astype(_BF16)
    y = _round_bf16(_dot(act, wd_s[:, pl.ds(0, M)]))
    y = _round_bf16(y * gate)
    upd = jnp.where(jnp.logical_or(tokr == i1, tokr == i2), y, 0.0)
    hsel = jnp.concatenate([h_s[pl.ds(b1, R), :].astype(_F32),
                            h_s[pl.ds(b2, R), :].astype(_F32)], axis=0)
    fixed = hsel + _round_bf16(hnsel + upd)

    pltpu.make_async_copy(out_s, out_hbm, sem_out.at[0]).wait()

    def fix_copy(b0, k):
        return pltpu.make_async_copy(out_s.at[pl.ds(b0, R), :],
                                     out_hbm.at[pl.ds(b0, R), :], sem_out.at[k])

    out_s[pl.ds(b1, R), :] = fixed[:R].astype(_BF16)
    out_s[pl.ds(b2, R), :] = fixed[R:].astype(_BF16)
    fix_copy(b1, 0).start()

    @pl.when(b2 != b1)
    def _():
        fix_copy(b2, 1).start()
        fix_copy(b2, 1).wait()

    fix_copy(b1, 0).wait()


@jax.jit
def pallas_sequential_preLN__compressed_kv_cla__moe_arch_mod__prompt_kernel(
    A_x: jax.Array,
    A_c_kv: jax.Array,
    A_w_q: jax.Array,
    A_w_uk: jax.Array,
    A_w_uv: jax.Array,
    A_w_o: jax.Array,
    B_x: jax.Array,
    B_w_r: jax.Array,
    B_w_gate: jax.Array,
    B_w_up: jax.Array,
    B_w_down: jax.Array,
):
    B, S, M = A_x.shape
    assert B == 1
    DC = A_c_kv.shape[2]
    H, D = A_w_q.shape[1], A_w_q.shape[2]
    F = B_w_gate.shape[1]
    assert A_c_kv.shape[1] == S and S % _TQ == 0 and H % 2 == 0 and S <= 2 ** _IDX_BITS
    NP = H // 2
    NG = S // _HT

    x = A_x.reshape(S, M)
    c = A_c_kv.reshape(S, DC)
    wo = A_w_o.reshape(H * D, M)
    wr = B_w_r.reshape(1, M)

    any_spec = pl.BlockSpec(memory_space=pl.ANY)
    vmem_spec = pl.BlockSpec(memory_space=pltpu.VMEM)
    def buf(name, lead, rows, cols):
        if name in _U32BUF:
            return pltpu.VMEM((lead, rows // 2, cols), _U32)
        return pltpu.VMEM((lead, rows, cols), _BF16)

    scratch = [
        pltpu.VMEM((S, M), _BF16),
        pltpu.VMEM((S, DC), _BF16),
        pltpu.VMEM((S, M), _F32),
        pltpu.VMEM((7, S // 2, DC // 2), _F32),
        buf('q', 4, S, D),
        buf('k', 2, S, D),
        buf('v', 2, S, D),
        pltpu.VMEM((4, M, D), _U32),
        pltpu.VMEM((2, DC, D), _U32),
        pltpu.VMEM((2, DC, D), _U32),
        pltpu.VMEM((2, 49, M // 8, D), _U32),
        buf('wb', 49, DC // 4, D),
        buf('ctx', H, S, D),
        pltpu.VMEM((2, 4, D // 2, M), _BF16),
        buf('wob', 49, H * D // 4, M // 4),
        pltpu.VMEM((M, F), _BF16),
        pltpu.VMEM((M, F), _BF16),
        pltpu.VMEM((F, M + _WD_PAD), _BF16),
        pltpu.VMEM((_HT, M), _BF16),
        pltpu.VMEM((_HT, M), _BF16),
        pltpu.VMEM((S, M), _BF16),
        pltpu.VMEM((S, M), _BF16),
        pltpu.VMEM((NG, _HT), _F32),
        pltpu.VMEM((1024, _HT), _U32),
        pltpu.VMEM((S, M), _BF16),
        pltpu.SemaphoreType.DMA((3,)),
        pltpu.SemaphoreType.DMA((3,)),
        pltpu.SemaphoreType.DMA((2, 2)),
        pltpu.SemaphoreType.DMA((4,)),
        pltpu.SemaphoreType.DMA((2, 4)),
        pltpu.SemaphoreType.DMA((3,)),
        pltpu.SemaphoreType.DMA((2,)),
    ]
    out = pl.pallas_call(
        functools.partial(_kernel, S=S, M=M, DC=DC, H=H, D=D, F=F),
        in_specs=[any_spec, any_spec, any_spec, any_spec, any_spec, any_spec,
                  vmem_spec, any_spec, any_spec, any_spec],
        out_specs=any_spec,
        out_shape=jax.ShapeDtypeStruct((S, M), _BF16),
        scratch_shapes=scratch,
        compiler_params=pltpu.CompilerParams(vmem_limit_bytes=124 * 1024 * 1024,
                                             disable_bounds_checks=True,
                                             disable_semaphore_checks=True),
        name="fused_mla_mod",
    )(x, c, A_w_q, A_w_uk, A_w_uv, wo, wr, B_w_gate, B_w_up, B_w_down)
    return out.reshape(B, S, M)
```

```python
import functools
import math

import jax
import jax.numpy as jnp
from jax import lax
import jax.experimental.pallas as pl
import jax.experimental.pallas.tpu as pltpu

_F32 = jnp.float32
_BF16 = jnp.bfloat16
_U32 = jnp.uint32
_I32 = jnp.int32

_EPS = 1e-5
_NEG = -1e30
_TQ = 256
_HT = 128
import os
_TIE = int(os.environ.get('TIE', 4))
_CHAIN = int(os.environ.get('CHAIN', 0))
_ERG = int(os.environ.get('ERG', 8))
_EORD = int(os.environ.get('EORD', 0))
_EVAL = int(os.environ.get('EVAL', 1))
_U32BUF = os.environ.get('U32', 'xa,ca,q,k,v,wob,ctx,wb').split(',')
_PA = int(os.environ.get('PA', 13))
_PB = int(os.environ.get('PB', 13))
_PC = int(os.environ.get('PC', 16))
_PX = int(os.environ.get('PX', 8))
_OSPLIT = int(os.environ.get('OSPLIT', 0))
_O1 = int(os.environ.get('O1', 14))
_O2 = int(os.environ.get('O2', 14))
_END = int(os.environ.get('END', 3))
_WQS = int(os.environ.get('WQS', 672))
_NG = int(os.environ.get('NG', 16))
_BIG = int(os.environ.get('BIG', 3))
_TSPAN = 360
_DIST = int(os.environ.get('DIST', 2))
_PN = int(os.environ.get('PN', 14))
_WOH = int(os.environ.get('WOH', 0))
_LND = int(os.environ.get('LND', 6))
_FR = int(os.environ.get('FR', 2))
_LATE = int(os.environ.get('LATE', 2))
_TIEL = int(os.environ.get('TIEL', 3))
_LD = int(os.environ.get('LD', 9))
_LORD = [int(c) for c in os.environ.get('LORD', '76543210')]
_ZU = int(os.environ.get('ZU', 1))
_FD = int(os.environ.get('FD', 99))
_IDX_BITS = 13
_KEY_BIAS = 0x20000000
_FIX = 8
_WD_PAD = 128


def _dot(a, b):
    return jnp.dot(a, b, preferred_element_type=_F32)


def _dot_nt(a, b):
    return lax.dot_general(a, b, (((1,), (1,)), ((), ())), preferred_element_type=_F32)


def _as_bf16(u):
    return pltpu.bitcast(u, _BF16)


def _pack(x):
    return pltpu.bitcast(x.astype(_BF16), _U32)


def _rows(ref, r0, n):
    if ref.dtype == _U32:
        if isinstance(r0, tuple):
            return pl.ds(r0[0] + r0[1] // 2, n // 2)
        if isinstance(r0, int):
            return pl.ds(r0 // 2, n // 2)
        return pl.ds(pl.multiple_of(r0 // 2, 8), n // 2)
    return pl.ds(r0, n)


def _ld(ref, lead, r0, n):
    v = ref[lead, _rows(ref, r0, n), :]
    return _as_bf16(v) if ref.dtype == _U32 else v


def _st(ref, lead, r0, x, cols=slice(None)):
    v = _pack(x) if ref.dtype == _U32 else x.astype(_BF16)
    if lead is None:
        ref[_rows(ref, r0, x.shape[0]), cols] = v
    else:
        ref[lead, _rows(ref, r0, x.shape[0]), cols] = v


def _round_bf16(x):
    return x.astype(_BF16).astype(_F32)


def _layernorm(x):
    n = x.shape[-1]
    mean = jnp.sum(x, axis=-1, keepdims=True) * (1.0 / n)
    xc = x - mean
    var = jnp.sum(xc * xc, axis=-1, keepdims=True) * (1.0 / n)
    m = _round_bf16(mean)
    den = _round_bf16(jnp.sqrt(_round_bf16(_round_bf16(var) + _EPS)))
    return (x - m) * (1.0 / den)


def _layernorm_scaled(x, scale):
    n = x.shape[-1]
    mean = jnp.sum(x, axis=-1, keepdims=True) * (1.0 / n)
    xc = x - mean
    var = jnp.sum(xc * xc, axis=-1, keepdims=True) * (1.0 / n)
    return xc * (lax.rsqrt(var + _EPS) * scale)


def _strassen_a(a11, a12, a21, a22):
    return (a11 + a22, a21 + a22, a11, a22, a11 + a12, a21 - a11, a12 - a22)


def _strassen_b(b11, b12, b21, b22):
    return (b11 + b22, b11, b12 - b22, b21 - b11, b22, b11 + b12, b21 + b22)


def _strassen_c(m):
    m1, m2, m3, m4, m5, m6, m7 = m
    return (m4 - m5 + m1 + m7, m3 + m5, m4 + m2, m3 - m2 + m1 + m6)


_ORDER = (2, 4, 3, 1, 0, 6, 5)


_SA = (((0, 1), (3, 1)), ((2, 1), (3, 1)), ((0, 1),), ((3, 1),),
       ((0, 1), (1, 1)), ((2, 1), (0, -1)), ((1, 1), (3, -1)))
_SB = (((0, 1), (3, 1)), ((0, 1),), ((1, 1), (3, -1)), ((2, 1), (0, -1)),
       ((3, 1),), ((0, 1), (1, 1)), ((2, 1), (3, 1)))


def _combine(terms):
    terms = sorted(terms, key=lambda ts: -ts[1])
    acc = terms[0][0]
    assert terms[0][1] > 0
    for v, sg in terms[1:]:
        acc = acc + v if sg > 0 else acc - v
    return acc


def _quadrants(x):
    r, c = x.shape[0] // 2, x.shape[1] // 2
    return x[:r, :c], x[:r, c:], x[r:, :c], x[r:, c:]


def _kernel(x_hbm, c_hbm, wq_hbm, wk_hbm, wv_hbm, wo_hbm, wr_hbm, wg_hbm, wu_hbm, wd_hbm,
            out_hbm,
            x_raw, c_raw, xn_s, ca_s, q_s, k_s, v_s,
            wq_p, wk_p, wv_p, wqb_s, wkvb_s,
            ctx_s, wo_p, wob_s, wg_s, wu_s, wd_s, ht_s, hb_s, h_s, hn_s, r_s, junk_s, out_s, wr_s,
            sem_x, sem_c, sem_w, sem_wq, sem_wo, sem_ffn, sem_out,
            *, S, M, DC, H, D, F):
    TQ, HT = _TQ, _HT
    NB = S // TQ
    NG = S // HT
    NP = H // 2
    KO = H * D // 4
    NO = M // 4
    OS = KO // NP
    qscale = (D ** -0.5) * math.log2(math.e)

    wq32 = wq_hbm.bitcast(_U32)
    wk32 = wk_hbm.bitcast(_U32)
    wv32 = wv_hbm.bitcast(_U32)

    def w_copies(pair, slot):
        return (
            pltpu.make_async_copy(wk32.at[:, pair, :], wk_p.at[slot], sem_w.at[slot, 0]),
            pltpu.make_async_copy(wv32.at[:, pair, :], wv_p.at[slot], sem_w.at[slot, 1]),
        )

    def wq_copy(pair):
        return pltpu.make_async_copy(wq32.at[:, pair, :], wq_p.at[pair % 4],
                                     sem_wq.at[pair % 4])

    def wo_copies(t, slot):
        r0 = pl.multiple_of(t * OS, OS)
        return tuple(
            pltpu.make_async_copy(wo_hbm.at[pl.ds(half * KO + r0, OS), :],
                                  wo_p.at[slot, half], sem_wo.at[slot, half])
            for half in range(4))

    def x_copy(i, n):
        rows = pl.ds(pl.multiple_of(i * TQ, TQ), TQ)
        return pltpu.make_async_copy(x_hbm.at[rows, :], x_raw.at[rows, :], sem_x.at[n % 3])

    def c_copy(i):
        rows = pl.ds(pl.multiple_of(i * 2 * TQ, 2 * TQ), 2 * TQ)
        return pltpu.make_async_copy(c_hbm.at[rows, :], c_raw.at[rows, :], sem_c.at[i % 3])

    ffn = ((wg_hbm, wg_s), (wu_hbm, wu_s), (wd_hbm, wd_s))

    def ffn_start(t):
        for n, (src, dst) in enumerate(ffn):
            rows, cols = src.shape[0] // NP, src.shape[1]
            r0 = pl.multiple_of(t * rows, 16)
            pltpu.make_async_copy(src.at[pl.ds(r0, rows), :],
                                  dst.at[pl.ds(r0, rows), pl.ds(0, cols)],
                                  sem_ffn.at[n]).start()

    def ffn_wait(n):
        src, dst = ffn[n]
        pltpu.make_async_copy(src, dst.at[:, pl.ds(0, src.shape[1])], sem_ffn.at[n]).wait()

    def lo_hi(w):
        return (pltpu.bitcast(w << 16, _F32), pltpu.bitcast(w & jnp.uint32(0xFFFF0000), _F32))

    def pacer(tiles, total, free=0):
        def zero(n):
            if n < free:
                return jnp.zeros((16, HT), _U32)
            mat, zr, zc = tiles[(n - free) * len(tiles) // (total - free)]
            z = pltpu.bitcast(mat[zr:zr + 8, zc:zc + HT], _U32)
            z = (z >> 16) >> 16
            return jnp.concatenate([z, z], axis=0)
        return zero

    def score_tiles(mats, span):
        return [(m, t0 % TQ, (t0 // TQ) * 4 * HT) for m in mats for t0 in range(0, span, 8)]

    def prep_w4(srcs, dst, kq, rows, pace=None, sink=None):
        pieces = [(t, r) for t in range(7) for r in rows]
        for n, (t, r) in enumerate(pieces):
            terms = [[] for _ in range(4)]
            for k, (q1, sg) in enumerate(_SB[t]):
                for rb in range(2):
                    w = srcs[q1 % 2][pl.ds((2 * (q1 // 2) + rb) * kq + r, 16), :]
                    if pace is not None and k == 0:
                        w = w | pace(n)
                    lo, hi = lo_hi(w)
                    terms[2 * rb].append((lo, sg))
                    terms[2 * rb + 1].append((hi, sg))
            z = None
            for u, b in enumerate(_strassen_b(*[_combine(tm) for tm in terms])):
                pk = _pack(b)
                dst[7 * t + u, pl.ds(r // 2, 8), :] = pk
                z = pk if z is None else z | pk
            if sink is not None:
                junk_s[pl.ds(8 * (sink + n), 8), :] = z

    def prep_wo(slot, src0, nrows, dst0, mats, span):
        pieces = [(r, c0, t) for r in range(0, nrows, 16) for c0 in range(0, NO, HT)
                  for t in range(7)]
        pace = pacer(score_tiles(mats, span), len(pieces))
        for n, (r, c0, t) in enumerate(pieces):
            z = pltpu.bitcast(pace(n), _F32)
            rs = pl.ds(src0 + r, 16)
            sub = []
            for q2 in range(4):
                v = _combine([
                    (wo_p[slot, 2 * (q1 // 2) + q2 // 2, rs,
                          pl.ds((2 * (q1 % 2) + q2 % 2) * NO + c0, HT)].astype(_F32), sg)
                    for q1, sg in _SB[t]])
                sub.append(v + z if q2 in (0, 3) else v)
            for u, b in enumerate(_strassen_b(*sub)):
                _st(wob_s, 7 * t + u, dst0 + r, b, pl.ds(c0, HT))

    QT = HT // 2
    KQ = DC // 4
    MQ = M // 4

    def fence():
        junk_s[pl.ds(0, 8), :] = jnp.zeros((8, HT), _U32)

    def tie(w, ties):
        parts, at = [], 0
        for r in sorted(ties):
            if r > at:
                parts.append(w[at:r])
            parts.append(w[r:r + 8] | ties[r])
            at = r + 8
        if at < w.shape[0]:
            parts.append(w[at:])
        return parts[0] if len(parts) == 1 else jnp.concatenate(parts, axis=0)

    def project4(lhs, w, store, zs=()):
        m, tiles, cnt = [None] * 7, [], [0]
        for t in _ORDER:
            ps = [None] * 7
            for u in _ORDER:
                fence()
                a = lhs(t, u)
                wt = w[7 * t + u]
                n = len(tiles) * len(zs) * D * 8 // (_TSPAN * a.shape[1] * 2)
                done = cnt[0]
                if zs and done < len(zs) and n > done:
                    wt = tie(wt, {0: zs[done]})
                    cnt[0] += 1
                ps[u] = _dot(a.astype(_BF16), _as_bf16(wt))
                tiles += [(ps[u], r, 0) for r in range(0, QT, QT * D // (2 * a.shape[1]))]
            m[t] = _strassen_c(ps)
        for q2 in range(4):
            for q1, cblk in enumerate(_strassen_c([mt[q2] for mt in m])):
                store(2 * (q1 % 2) + q2 % 2, (2 * (q1 // 2) + q2 // 2) * QT, cblk)
        return tiles

    def project_q(xn, x0, wqb, q, r0):
        def lhs(t, u):
            return _combine([
                (xn[pl.ds(x0 + (2 * (q1 // 2) + q2 // 2) * QT, QT),
                    pl.ds((2 * (q1 % 2) + q2 % 2) * MQ, MQ)], s1 * s2)
                for q1, s1 in _SA[t] for q2, s2 in _SA[u]])
        return project4(lhs, wqb, lambda nb, r, val: _st(q, nb, r0 + r, val))

    def project_kv(ca, a0, r0, zs=()):
        def lhs(t, u):
            return _combine([
                (ca[t, pl.ds(a0 + (q2 // 2) * QT, QT), pl.ds((q2 % 2) * KQ, KQ)], sg)
                for q2, sg in _SA[u]])
        return project4(lhs, wkvb_s,
                        lambda nb, r, val: _st((k_s, v_s)[nb // 2], nb % 2, r0 + r, val), zs)

    def prep_wq(raw, slot, r, nr, pace, sink=None):
        span = 3 * MQ + nr
        prep_w4((wq_p.at[raw, pl.ds(r, span), :], wq_p.at[raw + 1, pl.ds(r, span), :]),
                wqb_s.at[slot, :, pl.ds(pl.multiple_of(r // 2, 8), nr // 2), :],
                MQ, range(0, nr, 16), pace, sink)

    NH = NB // 2

    def plain_weights(src0, src1):
        return jnp.concatenate(lo_hi(src0[...]) + lo_hi(src1[...]), axis=1).astype(_BF16)

    def stage_x(r0, xn, x0, pace):
        done = []
        for n, c in enumerate(range(0, TQ, _PX)):
            xr = x_raw[pl.ds(r0 + c, _PX), :].astype(_F32)
            z = pace(n)[:_PX]
            if n >= _LND:
                z = z | done[n - _LND]
            xr = jnp.concatenate([xr[:, :HT] + pltpu.bitcast(z, _F32), xr[:, HT:]], axis=1)
            y = _layernorm_scaled(xr, qscale)
            xn[pl.ds(x0 + c, _PX), :] = y
            done.append((pltpu.bitcast(y[:, :HT], _U32) >> 16) >> 16)

    def stage_c(r0, a0, pace):
        kh = DC // 2
        for n, c in enumerate(range(0, HT, 8)):
            top = c_raw[pl.ds(r0 + c, 8), :].astype(_F32)
            bot = c_raw[pl.ds(r0 + HT + c, 8), :].astype(_F32)
            z = pltpu.bitcast(pace(n)[:8], _F32)
            z = jnp.concatenate([z] * (kh // HT), axis=1)
            for t, a in enumerate(
                    _strassen_a(top[:, :kh] + z, top[:, kh:], bot[:, :kh], bot[:, kh:] + z)):
                ca_s[t, pl.ds(a0 + c, 8), :] = a

    def xs_copy(n):
        return x_copy((n + NH) % NB, n)

    for cp in w_copies(0, 0):
        cp.start()
    c_copy(0).start()
    xs_copy(0).start()
    ht_s[...] = jnp.zeros((HT, M), _BF16)
    hb_s[...] = jnp.zeros((HT, M), _BF16)
    for cp in w_copies(0, 0):
        cp.wait()
    c_copy(1).start()
    xs_copy(1).start()
    c_copy(0).wait()
    xs_copy(0).wait()

    def pro_a(i, carry):
        @pl.when(i + 2 < NH)
        def _():
            c_copy(i + 2).start()

        @pl.when(i + 2 <= NH)
        def _():
            xs_copy(i + 2).start()

        @pl.when(jnp.logical_and(i >= 1, i <= 2))
        def _():
            wq_copy(i - 1).start()

        @pl.when(i > 0)
        def _():
            c_copy(i).wait()
            xs_copy(i).wait()

        r0 = pl.multiple_of(i * 2 * TQ, 2 * TQ)
        kv = _dot(c_raw[pl.ds(r0, 2 * TQ), :], plain_weights(wk_p.at[0], wv_p.at[0]))
        for nb in range(4):
            _st((k_s, v_s)[nb // 2], nb % 2, r0, kv[:, nb * D:(nb + 1) * D])
        tiles = [(kv, r, nb * D) for nb in range(4) for r in range(0, 2 * TQ, 8)]
        nt = len(tiles)
        a0 = pl.multiple_of(i * TQ, TQ)
        stage_c(r0, a0, pacer(tiles[:nt // 2], HT // 8))
        stage_c(r0 + TQ, a0 + HT, pacer(tiles[nt // 2:nt * 15 // 16], HT // 8))
        rx = pl.multiple_of((i + NH) * TQ, TQ)
        stage_x(rx, xn_s, rx, pacer(tiles[:nt * _PA // 16], TQ // _PX, _FR))
        return carry

    def pro_b(i, carry):
        @pl.when(i + 2 < NH)
        def _():
            xs_copy(NH + i + 2).start()

        @pl.when(i == 2)
        def _():
            for cp in w_copies(1, 1) + wo_copies(0, 0):
                cp.start()
            wq_copy(2).wait()
            wq_copy(3).wait()

        xs_copy(NH + i).wait()
        r0 = pl.multiple_of(i * TQ, TQ)
        xn = xn_s.at[pl.ds(r0, S // 2 + TQ), :]
        kh = M // 2
        lhs = [xn[pl.ds(S // 2, TQ), pl.ds(k0, kh)].astype(_BF16) for k0 in (0, kh)]
        tiles = []
        for nb in range(4):
            d = [_dot(lhs[k], lo_hi(wq_p[nb // 2, pl.ds(k * kh, kh), :])[nb % 2].astype(_BF16))
                 for k in range(2)]
            _st(q_s, nb, r0 + S // 2, d[0] + d[1])
            tiles += [(dk, r, 0) for dk in d for r in range(0, TQ, 8)]
        nt = len(tiles)
        stage_x(r0, xn, 0, pacer(tiles[:nt * _PB // 16], TQ // _PX, _FR))
        nr = MQ // (2 * NH)
        npc = 7 * nr // 16
        pace = pacer(tiles[:nt * _PC // 16], 3 * npc, _FR)
        for k in range(3):
            u = 3 * i + k
            quad = u // (2 * NH)
            prep_wq(2 * quad, quad, pl.multiple_of((u % (2 * NH)) * nr, nr), nr,
                    lambda n, k=k: pace(k * npc + n))
        return carry

    with jax.named_scope('pro_a'):
        lax.fori_loop(0, NH, pro_a, 0)
    wq_copy(0).wait()
    wq_copy(1).wait()
    xs_copy(NH + 1).start()
    wq_copy(2).start()
    wq_copy(3).start()
    with jax.named_scope('pro_b'):
        lax.fori_loop(0, NH, pro_b, 0)

    for cp in w_copies(2, 0) + wo_copies(1, 1) + (wq_copy(4), wq_copy(5)):
        cp.start()
    ffn_start(NP - 1)
    wr_copy = pltpu.make_async_copy(wr_hbm, wr_s, sem_ffn.at[3])
    wr_copy.start()
    for cp in w_copies(1, 1) + wo_copies(0, 0):
        cp.wait()

    tri = (lax.broadcasted_iota(_I32, (HT, HT), 1)
           <= lax.broadcasted_iota(_I32, (HT, HT), 0))

    def softmax_rows(parts, _TIE):
        s = parts[0] if len(parts) == 1 else jnp.concatenate(parts, axis=1)
        m = jnp.max(s, axis=1, keepdims=True)
        p = jnp.exp2(s - m)
        nt = p.shape[1] // HT
        tiles, acc, grp = [], None, None
        for j in range(nt):
            pj = p[:, j * HT:(j + 1) * HT]
            grp = pj if grp is None else grp + pj
            if j % _TIE == _TIE - 1 or j == nt - 1:
                if _CHAIN:
                    acc = grp if acc is None else acc + grp
                    if j > 0:
                        pj = jnp.minimum(pj, acc)
                else:
                    if j % _TIE > 0:
                        pj = jnp.minimum(pj, grp)
                    acc = grp if acc is None else acc + grp
                grp = None
            tiles.append(pj)
        p = tiles[0] if nt == 1 else jnp.concatenate(tiles, axis=1)
        return p, acc

    def scores(q, e, i, zs=()):
        Lm = i * TQ + HT
        nt = Lm // HT
        ties = {(4 + n * (nt - 4) // len(zs)) * QT + 8 * (n % 8): z for n, z in enumerate(zs)}
        keys = _as_bf16(tie(k_s[e, pl.ds(0, Lm // 2), :], ties))
        s_main = _dot_nt(_ld(q, e, i * TQ, TQ), keys)
        s_last = _dot_nt(_ld(q, e, i * TQ + HT, HT), _ld(k_s, e, Lm, HT))
        return s_main, s_last

    def values(e, i):
        Lm = i * TQ + HT
        return _ld(v_s, e, 0, Lm), _ld(v_s, e, Lm, HT)

    def context(vals, head, i, s_main, s_last, group=_TIE):
        Lm = i * TQ + HT
        top = [jnp.where(tri, s_main[:HT, Lm - HT:], _NEG)]
        if Lm > HT:
            top = [s_main[:HT, :Lm - HT]] + top
        p_top, l_top = softmax_rows(top, group)
        p_bot, l_bot = softmax_rows([s_main[HT:], jnp.where(tri, s_last, _NEG)], group)
        p_main = jnp.concatenate([p_top, p_bot[:, :Lm]], axis=0).astype(_BF16)
        o = _dot(p_main, vals[0])
        o_last = _dot(p_bot[:, Lm:].astype(_BF16), vals[1])
        o = jnp.concatenate([o[:HT], o[HT:] + o_last], axis=0)
        acc = jnp.concatenate([l_top, l_bot], axis=0)

        def normalize(pace=None, n0=0):
            zs, z = [], None
            for n, g in enumerate(range(0, TQ, 16)):
                a = acc[g:g + 16]
                if pace is not None:
                    a = a + pltpu.bitcast(pace(n0 + n), _F32)
                linv = jnp.broadcast_to(
                    pl.reciprocal(jnp.sum(a, axis=1, keepdims=True), approx=True), (16, D))
                _st(ctx_s.at[head], None, i * TQ + g, o[g:g + 16] * linv)
                bits = pltpu.bitcast(linv, _U32)
                bits = bits[:8] | bits[8:]
                z = bits if z is None else z | bits
                if n % _NG == _NG - 1:
                    zs.append((z >> 16) >> 16)
                    z = None
            return zs
        return normalize

    def pair_body(s, carry):
        slot = (s + 1) % 2
        odd = s % 2
        wo0 = pl.multiple_of(s * OS, OS)
        q_rd = q_s.at[pl.ds(2 * odd, 2)]
        q_wr = q_s.at[:, pl.ds(pl.multiple_of(odd * (S // 4), S // 4), S // 4), :]
        xn = xn_s.at[pl.ds(pl.multiple_of(odd * (S // 2), S // 2), S // 2), :]
        quad = (s + 1) // 2
        wqb = wqb_s.at[quad % 2]
        pend, sc = {}, {}

        def norm(blocks, tiles):
            fns = [f for i in blocks for f in pend.pop(i)]
            pace = pacer(tiles, len(fns) * (TQ // 16))
            return [z for k, f in enumerate(fns) for z in f(pace, k * (TQ // 16))]

        def qk(i, nrm=()):
            sa = scores(q_rd, 0, i)
            zs = norm(nrm, score_tiles([sa[0]], (2 * i + 1) * QT * _PN // 16)) if nrm else ()
            sc[i] = (sa, scores(q_rd, 1, i, zs))
            return [sa[0], sc[i][1][0]]

        def pv(i):
            pend[i] = [context(values(e, i), 2 * s + e, i, *sc[i][e]) for e in range(2)]

        def kv(j, zs=()):
            return project_kv(ca_s, j * HT, j * TQ, zs)

        for i in range(NB - 1, NH - 1, -1):
            mats = qk(i, [i + 2] if i + 2 < NB else [])
            if i == NB - 1:
                prep_w4((wk_p.at[slot], wv_p.at[slot]), wkvb_s, KQ, range(0, KQ, 16),
                        pacer(score_tiles(mats, 3 * TQ + HT), 7 * KQ // 16), 1)
            if i == NB - 2:
                prep_wq(2 * (jnp.minimum(quad + 1, NP // 2 - 1) % 2), (quad + 1) % 2,
                        pl.multiple_of((1 - odd) * (MQ // 2), MQ // 2), MQ // 2,
                        pacer(score_tiles(mats, _WQS), 7 * MQ // 32), 64)
            if i in (NB - 3, NB - 4):
                r = (NB - 3 - i) * (OS // 2)
                prep_wo(1 - slot, r, OS // 2, wo0 + r, mats, 2 * TQ + QT)
            project_q(xn, (i - NH) * TQ, wqb, q_wr, (i - NH) * TQ)
            pv(i)
        assert NH == 4
        if _LATE == 0:
            qk(1); qk(0); t = kv(7); z = norm([5], t[len(t) // 4:]); pv(1); pv(0); kv(6, z)
            qk(3, [4]); t = kv(5); z = norm([1, 0], t); pv(3); kv(4, z)
            qk(2); kv(3); pv(2)
            t = kv(2); t = kv(1, norm([3], t)); kv(0, norm([2], t))
        elif _LATE == 1:
            qk(3, [5]); kv(7); pv(3); t = kv(6)
            z = norm([4], t); qk(1); qk(0); kv(5, z); pv(1); pv(0); t = kv(4)
            z = norm([3], t); qk(2); kv(3, z); pv(2)
            t = kv(2); t = kv(1, norm([1, 0], t)); kv(0, norm([2], t))
        elif _LATE == 2:
            qk(3, [5]); qk(0); kv(7); pv(3); pv(0); t = kv(6)
            z = norm([4], t); qk(2); qk(1); kv(5, z); pv(2); pv(1)
            t = kv(4); t = kv(3, norm([3], t)); t = kv(2, norm([0], t))
            t = kv(1, norm([2], t)); kv(0, norm([1], t))
        assert not pend

        @pl.when(s + 3 < NP)
        def _():
            for cp in w_copies(s + 3, slot):
                cp.start()

        @pl.when(s + 2 < NP)
        def _():
            for cp in wo_copies(s + 2, 1 - slot):
                cp.start()

        @pl.when(s + 6 < NP)
        def _():
            wq_copy(s + 6).start()

        ffn_start(s)

        @pl.when(s == 0)
        def _():
            wq_copy(4).wait()

        @pl.when(s + 5 < NP)
        def _():
            wq_copy(s + 5).wait()

        @pl.when(s + 2 < NP)
        def _():
            for cp in w_copies(s + 2, 1 - slot):
                cp.wait()

        for cp in wo_copies(s + 1, slot):
            cp.wait()
        return carry

    with jax.named_scope('pair_loop'):
        lax.fori_loop(0, NP - 1, pair_body, 0)

    last_slot = (NP - 1) % 2

    def last_body(e, carry):
        half = OS // 2
        q_rd = q_s.at[pl.ds(2, 2)]
        order = _LORD
        sc = {order[0]: scores(q_rd, e, order[0])}
        prep_wo(last_slot, pl.multiple_of(e * half, half), half,
                pl.multiple_of((NP - 1) * OS + e * half, half), [sc[order[0]][0]], 3 * TQ)
        pend, zs = [], ()
        for n, i in enumerate(order):
            if n + 1 < NB:
                j = order[n + 1]
                sc[j] = scores(q_rd, e, j, zs if j >= 3 else ())
                zs = ()
                if len(pend) >= _LD and n + 2 < NB and order[n + 2] >= 3:
                    zs = pend.pop(0)(pacer(score_tiles([sc[j][0]], (2 * j + 1) * QT), TQ // 16))
            pend.append(context(values(e, i), H - 2 + e, i, *sc[i], group=_TIEL))
        for f in pend:
            f()
        return carry

    with jax.named_scope('last_loop'):
        lax.fori_loop(0, 2, last_body, 0)

    wr_copy.wait()
    wr = wr_s[...].astype(_F32).reshape(1, M)
    eye = (lax.broadcasted_iota(_I32, (HT, HT), 1) == lax.broadcasted_iota(_I32, (HT, HT), 0))

    def epilogue(g, src, pace=None, write_out=True, dist=_END):
        r0 = pl.multiple_of(g * HT, HT)
        rs = []
        for n, c in enumerate(range(0, HT, _ERG)):
            hb = src[pl.ds(c, _ERG), :]
            hc = hb.astype(_F32)
            z = None if pace is None else pace(n)[:_ERG]
            if n >= dist:
                zc = (pltpu.bitcast(jnp.broadcast_to(rs[n - dist], (_ERG, HT)), _U32)
                      & jnp.uint32(0xFFFF))
                z = zc if z is None else z | zc
            if z is not None:
                hc = jnp.concatenate([hc[:, :HT] + pltpu.bitcast(z, _F32), hc[:, HT:]], axis=1)
            hnb = _layernorm(hc).astype(_BF16)
            hn_s[pl.ds(r0 + c, _ERG), :] = hnb
            hn = hnb.astype(_F32)
            rs.append(_round_bf16(jnp.sum(hn * wr, axis=1, keepdims=True)))
            if write_out:
                h_s[pl.ds(r0 + c, _ERG), :] = hb
                out_s[pl.ds(r0 + c, _ERG), :] = (hc + hn).astype(_BF16)
        r = jnp.concatenate(rs, axis=0)
        r = jnp.sum(jnp.where(eye, r, 0.0), axis=0, keepdims=True)
        r_s[pl.ds(g, 1), :] = r
        return (pltpu.bitcast(jnp.broadcast_to(r, (8, HT)), _U32) >> 16) >> 16

    def out_copy(g):
        rows = pl.ds(pl.multiple_of(g * HT, HT), HT)
        return pltpu.make_async_copy(out_s.at[rows, :], out_hbm.at[rows, :], sem_out.at[0])

    KS = 2 * D

    def prod(r0, t, tiles, z=None, zu=0):
        ps = [None] * 7
        for u in _ORDER:
            terms = [(2 * (q1 // 2) + q2 // 2, 2 * (q1 % 2) + q2 % 2, s1 * s2)
                     for q1, s1 in _SA[t] for q2, s2 in _SA[u]]
            fence()
            acc = None
            for k0 in range(0, KO, KS):
                def blk(rb, kb):
                    h0 = (kb * KO + k0) // D
                    return jnp.concatenate(
                        [_ld(ctx_s, h0 + hh, (r0, rb * QT), QT) for hh in range(KS // D)], axis=1)
                if len(terms) == 1:
                    lhs = blk(terms[0][0], terms[0][1])
                else:
                    lhs = _combine([(blk(rb, kb).astype(_F32), sg)
                                    for rb, kb, sg in terms]).astype(_BF16)
                w = wob_s[7 * t + u, pl.ds(k0 // 2, KS // 2), :]
                if z is not None and k0 == 0 and u == _ORDER[zu]:
                    w = tie(w, {0: jnp.concatenate([z, z], axis=1)})
                d = _dot(lhs, _as_bf16(w))
                tiles.append((d, 0, 0))
                acc = d if acc is None else acc + d
            ps[u] = acc
        c11, c12, c21, c22 = _strassen_c(ps)
        return jnp.concatenate([jnp.concatenate([c11, c12], axis=1),
                                jnp.concatenate([c21, c22], axis=1)], axis=0)

    NPC = HT // _ERG

    def o_body(j, carry):
        r0 = pl.multiple_of(j * TQ, TQ)
        lag = 1 if _OSPLIT else 2

        @pl.when(j > 1)
        def _():
            out_copy(2 * j - lag - 2).start()

        @pl.when(j > lag - 1)
        def _():
            out_copy(2 * j - lag - 1).start()

        rh = pl.multiple_of(j * (TQ // 2), TQ // 2)
        left, right = pl.ds(0, M // 2), pl.ds(M // 2, M // 2)

        def residual(dst, rows0, cols, att):
            dst[:, cols] = (x_raw[pl.ds(rows0, HT), cols].astype(_F32) + att).astype(_BF16)

        tl = []
        m3 = prod(rh, 2, tl)
        m4 = prod(rh, 3, tl)
        if _OSPLIT:
            z = epilogue(jnp.maximum(2 * j - 1, 0), hb_s,
                         pacer(tl[:len(tl) * _O1 // 16], NPC, 1))
        else:
            gp = jnp.maximum(2 * j - 2, 0)
            z = epilogue(gp, ht_s, pacer(tl[:len(tl) * _O1 // 16], NPC, 1))
        tl = []
        m5 = prod(rh, 4, tl, z, _ZU)
        z = None
        residual(ht_s, r0, right, m3 + m5)
        m1 = prod(rh, 0, tl)
        m7 = prod(rh, 6, tl)
        residual(ht_s, r0, left, m4 - m5 + m1 + m7)
        if not _OSPLIT:
            z = epilogue(gp + 1, hb_s, pacer(tl[:len(tl) * _O2 // 16], NPC))
        tl = []
        m2 = prod(rh, 1, tl, z, _ZU)
        residual(hb_s, r0 + HT, left, m4 + m2)
        m6 = prod(rh, 5, tl)
        residual(hb_s, r0 + HT, right, m3 + m1 - m2 + m6)
        if _OSPLIT:
            epilogue(2 * j, ht_s, pacer(tl[2:len(tl) * _O2 // 16], NPC))
        return carry

    for n in range(3):
        ffn_wait(n)
    with jax.named_scope('o_loop'):
        lax.fori_loop(0, NB, o_body, 0)
    rest = [(NG - 1, hb_s)] if _OSPLIT else [(NG - 2, ht_s), (NG - 1, hb_s)]
    out_copy(rest[0][0] - 2).start()
    out_copy(rest[0][0] - 1).start()
    for g, src in rest:
        epilogue(g, src, None, False, _FD)

    r = r_s[pl.ds(0, NG), :] + 0.0
    tok = (lax.broadcasted_iota(_I32, (NG, HT), 0) * HT + lax.broadcasted_iota(_I32, (NG, HT), 1))
    code = pltpu.bitcast(r, _I32) >> 16
    code = jnp.where(code < 0, code ^ 0x7FFF, code) + 0x8000
    key = pltpu.bitcast(((code << _IDX_BITS) | (S - 1 - tok)) + _KEY_BIAS, _F32)
    k1 = jnp.max(jnp.max(key, axis=0, keepdims=True), axis=1, keepdims=True)
    key2 = jnp.where(key == k1, 0.0, key)
    k2 = jnp.max(jnp.max(key2, axis=0, keepdims=True), axis=1, keepdims=True)

    R = _FIX
    row = lax.broadcasted_iota(_I32, (2 * R, 1), 0)
    ki = pltpu.bitcast(jnp.where(row < R, k1, k2), _I32) - _KEY_BIAS
    idx = S - 1 - (ki & (2 ** _IDX_BITS - 1))
    i1 = jnp.clip(idx[0, 0], 0, S - 1)
    i2 = jnp.clip(idx[R, 0], 0, S - 1)
    b1 = pl.multiple_of((i1 // R) * R, R)
    b2 = pl.multiple_of((i2 // R) * R, R)
    tokr = jnp.where(row < R, b1 + row, b2 + row - R)
    cd = ((pltpu.bitcast(jnp.where(tokr == i1, k1, k2), _I32) - _KEY_BIAS) >> _IDX_BITS) - 0x8000
    score = pltpu.bitcast(jnp.where(cd < 0, cd ^ 0x7FFF, cd) << 16, _F32)
    gate = _round_bf16(1.0 / (1.0 + jnp.exp(-score)))

    hnsel = jnp.concatenate([hn_s[pl.ds(b1, R), :].astype(_F32),
                             hn_s[pl.ds(b2, R), :].astype(_F32)], axis=0)
    xs = hnsel.astype(_BF16)
    g = _dot(xs, wg_s[...])
    u = _dot(xs, wu_s[...])
    pace = pacer([(mat, 0, c0) for mat in (g, u) for c0 in range(0, F, HT)],
                 len(rest) * HT // 8)
    for k, (gi, src) in enumerate(rest):
        for n, c in enumerate(range(0, HT, 8)):
            rows = pl.ds(gi * HT + c, 8)
            hb = src[pl.ds(c, 8), :]
            h_s[rows, :] = hb
            z = pltpu.bitcast(pace(k * HT // 8 + n)[:8], _F32)
            z = jnp.concatenate([z] * (M // HT), axis=1)
            out_s[rows, :] = (hb.astype(_F32) + z + hn_s[rows, :].astype(_F32)).astype(_BF16)
        out_copy(gi).start()
    g = _round_bf16(g)
    u = _round_bf16(u)
    g = _round_bf16(g * (1.0 / (1.0 + jnp.exp(-g))))
    act = (g * u).astype(_BF16)
    y = _round_bf16(_dot(act, wd_s[:, pl.ds(0, M)]))
    y = _round_bf16(y * gate)
    upd = jnp.where(jnp.logical_or(tokr == i1, tokr == i2), y, 0.0)
    hsel = jnp.concatenate([h_s[pl.ds(b1, R), :].astype(_F32),
                            h_s[pl.ds(b2, R), :].astype(_F32)], axis=0)
    fixed = hsel + _round_bf16(hnsel + upd)

    pltpu.make_async_copy(out_s, out_hbm, sem_out.at[0]).wait()

    def fix_copy(b0, k):
        return pltpu.make_async_copy(out_s.at[pl.ds(b0, R), :],
                                     out_hbm.at[pl.ds(b0, R), :], sem_out.at[k])

    out_s[pl.ds(b1, R), :] = fixed[:R].astype(_BF16)
    out_s[pl.ds(b2, R), :] = fixed[R:].astype(_BF16)
    fix_copy(b1, 0).start()

    @pl.when(b2 != b1)
    def _():
        fix_copy(b2, 1).start()
        fix_copy(b2, 1).wait()

    fix_copy(b1, 0).wait()


@jax.jit
def pallas_sequential_preLN__compressed_kv_cla__moe_arch_mod__prompt_kernel(
    A_x: jax.Array,
    A_c_kv: jax.Array,
    A_w_q: jax.Array,
    A_w_uk: jax.Array,
    A_w_uv: jax.Array,
    A_w_o: jax.Array,
    B_x: jax.Array,
    B_w_r: jax.Array,
    B_w_gate: jax.Array,
    B_w_up: jax.Array,
    B_w_down: jax.Array,
):
    B, S, M = A_x.shape
    assert B == 1
    DC = A_c_kv.shape[2]
    H, D = A_w_q.shape[1], A_w_q.shape[2]
    F = B_w_gate.shape[1]
    assert A_c_kv.shape[1] == S and S % _TQ == 0 and H % 2 == 0 and S <= 2 ** _IDX_BITS
    NP = H // 2
    NG = S // _HT

    x = A_x.reshape(S, M)
    c = A_c_kv.reshape(S, DC)
    wo = A_w_o.reshape(H * D, M)

    any_spec = pl.BlockSpec(memory_space=pl.ANY)
    def buf(name, lead, rows, cols):
        if name in _U32BUF:
            return pltpu.VMEM((lead, rows // 2, cols), _U32)
        return pltpu.VMEM((lead, rows, cols), _BF16)

    scratch = [
        pltpu.VMEM((S, M), _BF16),
        pltpu.VMEM((S, DC), _BF16),
        pltpu.VMEM((S, M), _F32),
        pltpu.VMEM((7, S // 2, DC // 2), _F32),
        buf('q', 4, S, D),
        buf('k', 2, S, D),
        buf('v', 2, S, D),
        pltpu.VMEM((4, M, D), _U32),
        pltpu.VMEM((2, DC, D), _U32),
        pltpu.VMEM((2, DC, D), _U32),
        pltpu.VMEM((2, 49, M // 8, D), _U32),
        buf('wb', 49, DC // 4, D),
        buf('ctx', H, S, D),
        pltpu.VMEM((2, 4, D // 2, M), _BF16),
        buf('wob', 49, H * D // 4, M // 4),
        pltpu.VMEM((M, F), _BF16),
        pltpu.VMEM((M, F), _BF16),
        pltpu.VMEM((F, M + _WD_PAD), _BF16),
        pltpu.VMEM((_HT, M), _BF16),
        pltpu.VMEM((_HT, M), _BF16),
        pltpu.VMEM((S, M), _BF16),
        pltpu.VMEM((S, M), _BF16),
        pltpu.VMEM((NG, _HT), _F32),
        pltpu.VMEM((1024, _HT), _U32),
        pltpu.VMEM((S, M), _BF16),
        pltpu.VMEM((M,), _BF16),
        pltpu.SemaphoreType.DMA((3,)),
        pltpu.SemaphoreType.DMA((3,)),
        pltpu.SemaphoreType.DMA((2, 2)),
        pltpu.SemaphoreType.DMA((4,)),
        pltpu.SemaphoreType.DMA((2, 4)),
        pltpu.SemaphoreType.DMA((4,)),
        pltpu.SemaphoreType.DMA((2,)),
    ]
    out = pl.pallas_call(
        functools.partial(_kernel, S=S, M=M, DC=DC, H=H, D=D, F=F),
        in_specs=[any_spec] * 10,
        out_specs=any_spec,
        out_shape=jax.ShapeDtypeStruct((S, M), _BF16),
        scratch_shapes=scratch,
        compiler_params=pltpu.CompilerParams(vmem_limit_bytes=124 * 1024 * 1024,
                                             disable_bounds_checks=True,
                                             disable_semaphore_checks=True),
        name="fused_mla_mod",
    )(x, c, A_w_q, A_w_uk, A_w_uv, wo, B_w_r, B_w_gate, B_w_up, B_w_down)
    return out.reshape(B, S, M)
```

```python
import functools
import math

import jax
import jax.numpy as jnp
from jax import lax
import jax.experimental.pallas as pl
import jax.experimental.pallas.tpu as pltpu

_F32 = jnp.float32
_BF16 = jnp.bfloat16
_U32 = jnp.uint32
_I32 = jnp.int32

_EPS = 1e-5
_NEG = -1e30
_TQ = 256
_HT = 128
import os
_TIE = int(os.environ.get('TIE', 4))
_CHAIN = int(os.environ.get('CHAIN', 0))
_ERG = int(os.environ.get('ERG', 8))
_EORD = int(os.environ.get('EORD', 0))
_EVAL = int(os.environ.get('EVAL', 1))
_U32BUF = os.environ.get('U32', 'xa,ca,q,k,v,wob,ctx,wb').split(',')
_PA = int(os.environ.get('PA', 13))
_PB = int(os.environ.get('PB', 13))
_PC = int(os.environ.get('PC', 16))
_PX = int(os.environ.get('PX', 8))
_OSPLIT = int(os.environ.get('OSPLIT', 0))
_O1 = int(os.environ.get('O1', 14))
_O2 = int(os.environ.get('O2', 14))
_END = int(os.environ.get('END', 3))
_WQS = int(os.environ.get('WQS', 672))
_NG = int(os.environ.get('NG', 16))
_BIG = int(os.environ.get('BIG', 3))
_TSPAN = 360
_DIST = int(os.environ.get('DIST', 2))
_PN = int(os.environ.get('PN', 14))
_WOH = int(os.environ.get('WOH', 0))
_LND = int(os.environ.get('LND', 6))
_FR = int(os.environ.get('FR', 2))
_LATE = int(os.environ.get('LATE', 2))
_TIEL = int(os.environ.get('TIEL', 3))
_LD = int(os.environ.get('LD', 9))
_LORD = [int(c) for c in os.environ.get('LORD', '76543210')]
_ZU = int(os.environ.get('ZU', 1))
_FD = int(os.environ.get('FD', 99))
_LEAD = int(os.environ.get('LEAD', 0))
def _sp(k, d):
    v = [int(t) for t in os.environ.get(k, d).split(',')]
    return [(v[0], v[1]), (v[2], v[3])]
_S7 = _sp('S7', '0,768,128,896')
_S6 = _sp('S6', '0,672,0,672')
_IDX_BITS = 13
_KEY_BIAS = 0x30000000
_FIX = 8
_WD_PAD = 128


def _dot(a, b):
    return jnp.dot(a, b, preferred_element_type=_F32)


def _dot_nt(a, b):
    return lax.dot_general(a, b, (((1,), (1,)), ((), ())), preferred_element_type=_F32)


def _as_bf16(u):
    return pltpu.bitcast(u, _BF16)


def _pack(x):
    return pltpu.bitcast(x.astype(_BF16), _U32)


def _rows(ref, r0, n):
    if ref.dtype == _U32:
        if isinstance(r0, tuple):
            return pl.ds(r0[0] + r0[1] // 2, n // 2)
        if isinstance(r0, int):
            return pl.ds(r0 // 2, n // 2)
        return pl.ds(pl.multiple_of(r0 // 2, 8), n // 2)
    return pl.ds(r0, n)


def _ld(ref, lead, r0, n):
    v = ref[lead, _rows(ref, r0, n), :]
    return _as_bf16(v) if ref.dtype == _U32 else v


def _st(ref, lead, r0, x, cols=slice(None)):
    v = _pack(x) if ref.dtype == _U32 else x.astype(_BF16)
    if lead is None:
        ref[_rows(ref, r0, x.shape[0]), cols] = v
    else:
        ref[lead, _rows(ref, r0, x.shape[0]), cols] = v


def _round_bf16(x):
    return x.astype(_BF16).astype(_F32)


def _layernorm(x):
    n = x.shape[-1]
    mean = jnp.sum(x, axis=-1, keepdims=True) * (1.0 / n)
    xc = x - mean
    var = jnp.sum(xc * xc, axis=-1, keepdims=True) * (1.0 / n)
    m = _round_bf16(mean)
    den = _round_bf16(jnp.sqrt(_round_bf16(_round_bf16(var) + _EPS)))
    return (x - m) * pl.reciprocal(den, approx=True)


def _layernorm_scaled(x, scale):
    n = x.shape[-1]
    mean = jnp.sum(x, axis=-1, keepdims=True) * (1.0 / n)
    xc = x - mean
    var = jnp.sum(xc * xc, axis=-1, keepdims=True) * (1.0 / n)
    return xc * (lax.rsqrt(var + _EPS) * scale)


def _strassen_a(a11, a12, a21, a22):
    return (a11 + a22, a21 + a22, a11, a22, a11 + a12, a21 - a11, a12 - a22)


def _strassen_b(b11, b12, b21, b22):
    return (b11 + b22, b11, b12 - b22, b21 - b11, b22, b11 + b12, b21 + b22)


def _strassen_c(m):
    m1, m2, m3, m4, m5, m6, m7 = m
    return (m4 - m5 + m1 + m7, m3 + m5, m4 + m2, m3 - m2 + m1 + m6)


_ORDER = (2, 4, 3, 1, 0, 6, 5)


_SA = (((0, 1), (3, 1)), ((2, 1), (3, 1)), ((0, 1),), ((3, 1),),
       ((0, 1), (1, 1)), ((2, 1), (0, -1)), ((1, 1), (3, -1)))
_SB = (((0, 1), (3, 1)), ((0, 1),), ((1, 1), (3, -1)), ((2, 1), (0, -1)),
       ((3, 1),), ((0, 1), (1, 1)), ((2, 1), (3, 1)))


def _combine(terms):
    terms = sorted(terms, key=lambda ts: -ts[1])
    acc = terms[0][0]
    assert terms[0][1] > 0
    for v, sg in terms[1:]:
        acc = acc + v if sg > 0 else acc - v
    return acc


def _quadrants(x):
    r, c = x.shape[0] // 2, x.shape[1] // 2
    return x[:r, :c], x[:r, c:], x[r:, :c], x[r:, c:]


def _kernel(x_hbm, c_hbm, wq_hbm, wk_hbm, wv_hbm, wo_hbm, wr_hbm, wg_hbm, wu_hbm, wd_hbm,
            out_hbm,
            x_raw, c_raw, xn_s, ca_s, q_s, k_s, v_s,
            wq_p, wk_p, wv_p, wqb_s, wkvb_s,
            ctx_s, wo_p, wob_s, wg_s, wu_s, wd_s, ht_s, hb_s, h_s, hn_s, junk_s, out_s, wr_s,
            sem_x, sem_c, sem_w, sem_wq, sem_wo, sem_ffn, sem_out,
            *, S, M, DC, H, D, F):
    TQ, HT = _TQ, _HT
    NB = S // TQ
    NG = S // HT
    NP = H // 2
    KO = H * D // 4
    NO = M // 4
    OS = KO // NP
    qscale = (D ** -0.5) * math.log2(math.e)

    wq32 = wq_hbm.bitcast(_U32)
    wk32 = wk_hbm.bitcast(_U32)
    wv32 = wv_hbm.bitcast(_U32)

    def w_copies(pair, slot):
        return (
            pltpu.make_async_copy(wk32.at[:, pair, :], wk_p.at[slot], sem_w.at[slot, 0]),
            pltpu.make_async_copy(wv32.at[:, pair, :], wv_p.at[slot], sem_w.at[slot, 1]),
        )

    def wq_copy(pair):
        return pltpu.make_async_copy(wq32.at[:, pair, :], wq_p.at[pair % 4],
                                     sem_wq.at[pair % 4])

    def wo_copies(t, slot):
        r0 = pl.multiple_of(t * OS, OS)
        return tuple(
            pltpu.make_async_copy(wo_hbm.at[pl.ds(half * KO + r0, OS), :],
                                  wo_p.at[slot, half], sem_wo.at[slot, half])
            for half in range(4))

    def x_copy(i, n):
        rows = pl.ds(pl.multiple_of(i * TQ, TQ), TQ)
        return pltpu.make_async_copy(x_hbm.at[rows, :], x_raw.at[rows, :], sem_x.at[n % 3])

    def c_copy(i):
        rows = pl.ds(pl.multiple_of(i * 2 * TQ, 2 * TQ), 2 * TQ)
        return pltpu.make_async_copy(c_hbm.at[rows, :], c_raw.at[rows, :], sem_c.at[i % 3])

    ffn = ((wg_hbm, wg_s), (wu_hbm, wu_s), (wd_hbm, wd_s))

    def ffn_start(t):
        for n, (src, dst) in enumerate(ffn):
            rows, cols = src.shape[0] // NP, src.shape[1]
            r0 = pl.multiple_of(t * rows, 16)
            pltpu.make_async_copy(src.at[pl.ds(r0, rows), :],
                                  dst.at[pl.ds(r0, rows), pl.ds(0, cols)],
                                  sem_ffn.at[n]).start()

    def ffn_wait(n):
        src, dst = ffn[n]
        pltpu.make_async_copy(src, dst.at[:, pl.ds(0, src.shape[1])], sem_ffn.at[n]).wait()

    def lo_hi(w):
        return (pltpu.bitcast(w << 16, _F32), pltpu.bitcast(w & jnp.uint32(0xFFFF0000), _F32))

    def pacer(tiles, total, free=0):
        def zero(n):
            if n < free:
                return jnp.zeros((16, HT), _U32)
            mat, zr, zc = tiles[(n - free) * len(tiles) // (total - free)]
            z = pltpu.bitcast(mat[zr:zr + 8, zc:zc + HT], _U32)
            z = (z >> 16) >> 16
            return jnp.concatenate([z, z], axis=0)
        return zero

    def score_tiles(mats, span, spans=None):
        spans = spans or [(0, span)] * len(mats)
        return [(m, t0 % TQ, (t0 // TQ) * 4 * HT)
                for m, (lo, hi) in zip(mats, spans) for t0 in range(lo, hi, 8)]

    def prep_w4(srcs, dst, kq, rows, pace=None, sink=None):
        pieces = [(t, r) for t in range(7) for r in rows]
        for n, (t, r) in enumerate(pieces):
            terms = [[] for _ in range(4)]
            for k, (q1, sg) in enumerate(_SB[t]):
                for rb in range(2):
                    w = srcs[q1 % 2][pl.ds((2 * (q1 // 2) + rb) * kq + r, 16), :]
                    if pace is not None and k == 0:
                        w = w | pace(n)
                    lo, hi = lo_hi(w)
                    terms[2 * rb].append((lo, sg))
                    terms[2 * rb + 1].append((hi, sg))
            z = None
            for u, b in enumerate(_strassen_b(*[_combine(tm) for tm in terms])):
                pk = _pack(b)
                dst[7 * t + u, pl.ds(r // 2, 8), :] = pk
                z = pk if z is None else z | pk
            if sink is not None:
                junk_s[pl.ds(8 * (sink + n), 8), :] = z

    def prep_wo(slot, src0, nrows, dst0, mats, span):
        pieces = [(r, c0, t) for r in range(0, nrows, 16) for c0 in range(0, NO, HT)
                  for t in range(7)]
        pace = pacer(score_tiles(mats, span), len(pieces))
        for n, (r, c0, t) in enumerate(pieces):
            z = pltpu.bitcast(pace(n), _F32)
            rs = pl.ds(src0 + r, 16)
            sub = []
            for q2 in range(4):
                v = _combine([
                    (wo_p[slot, 2 * (q1 // 2) + q2 // 2, rs,
                          pl.ds((2 * (q1 % 2) + q2 % 2) * NO + c0, HT)].astype(_F32), sg)
                    for q1, sg in _SB[t]])
                sub.append(v + z if q2 in (0, 3) else v)
            for u, b in enumerate(_strassen_b(*sub)):
                _st(wob_s, 7 * t + u, dst0 + r, b, pl.ds(c0, HT))

    QT = HT // 2
    KQ = DC // 4
    MQ = M // 4

    def fence():
        junk_s[pl.ds(0, 8), :] = jnp.zeros((8, HT), _U32)

    def tie(w, ties):
        parts, at = [], 0
        for r in sorted(ties):
            if r > at:
                parts.append(w[at:r])
            parts.append(w[r:r + 8] | ties[r])
            at = r + 8
        if at < w.shape[0]:
            parts.append(w[at:])
        return parts[0] if len(parts) == 1 else jnp.concatenate(parts, axis=0)

    def project4(lhs, w, store, zs=(), mid=None):
        m, tiles, cnt = [None] * 7, [], [0]
        for t in _ORDER:
            ps = [None] * 7
            for u in _ORDER:
                if mid is not None and t == _ORDER[0] and u == _ORDER[_LEAD]:
                    mid()
                fence()
                a = lhs(t, u)
                wt = w[7 * t + u]
                n = len(tiles) * len(zs) * D * 8 // (_TSPAN * a.shape[1] * 2)
                done = cnt[0]
                if zs and done < len(zs) and n > done:
                    wt = tie(wt, {0: zs[done]})
                    cnt[0] += 1
                ps[u] = _dot(a.astype(_BF16), _as_bf16(wt))
                tiles += [(ps[u], r, 0) for r in range(0, QT, QT * D // (2 * a.shape[1]))]
            m[t] = _strassen_c(ps)
        for q2 in range(4):
            for q1, cblk in enumerate(_strassen_c([mt[q2] for mt in m])):
                store(2 * (q1 % 2) + q2 % 2, (2 * (q1 // 2) + q2 // 2) * QT, cblk)
        return tiles

    def project_q(xn, x0, wqb, q, r0, mid=None):
        def lhs(t, u):
            return _combine([
                (xn[pl.ds(x0 + (2 * (q1 // 2) + q2 // 2) * QT, QT),
                    pl.ds((2 * (q1 % 2) + q2 % 2) * MQ, MQ)], s1 * s2)
                for q1, s1 in _SA[t] for q2, s2 in _SA[u]])
        return project4(lhs, wqb, lambda nb, r, val: _st(q, nb, r0 + r, val), (), mid)

    def project_kv(ca, a0, r0, zs=()):
        def lhs(t, u):
            return _combine([
                (ca[t, pl.ds(a0 + (q2 // 2) * QT, QT), pl.ds((q2 % 2) * KQ, KQ)], sg)
                for q2, sg in _SA[u]])
        return project4(lhs, wkvb_s,
                        lambda nb, r, val: _st((k_s, v_s)[nb // 2], nb % 2, r0 + r, val), zs)

    def prep_wq(raw, slot, r, nr, pace, sink=None):
        span = 3 * MQ + nr
        prep_w4((wq_p.at[raw, pl.ds(r, span), :], wq_p.at[raw + 1, pl.ds(r, span), :]),
                wqb_s.at[slot, :, pl.ds(pl.multiple_of(r // 2, 8), nr // 2), :],
                MQ, range(0, nr, 16), pace, sink)

    NH = NB // 2

    def plain_weights(src0, src1):
        return jnp.concatenate(lo_hi(src0[...]) + lo_hi(src1[...]), axis=1).astype(_BF16)

    def stage_x(r0, xn, x0, pace):
        done = []
        for n, c in enumerate(range(0, TQ, _PX)):
            xr = x_raw[pl.ds(r0 + c, _PX), :].astype(_F32)
            z = pace(n)[:_PX]
            if n >= _LND:
                z = z | done[n - _LND]
            xr = jnp.concatenate([xr[:, :HT] + pltpu.bitcast(z, _F32), xr[:, HT:]], axis=1)
            y = _layernorm_scaled(xr, qscale)
            xn[pl.ds(x0 + c, _PX), :] = y
            done.append((pltpu.bitcast(y[:, :HT], _U32) >> 16) >> 16)

    def stage_c(r0, a0, pace):
        kh = DC // 2
        for n, c in enumerate(range(0, HT, 8)):
            top = c_raw[pl.ds(r0 + c, 8), :].astype(_F32)
            bot = c_raw[pl.ds(r0 + HT + c, 8), :].astype(_F32)
            z = pltpu.bitcast(pace(n)[:8], _F32)
            z = jnp.concatenate([z] * (kh // HT), axis=1)
            for t, a in enumerate(
                    _strassen_a(top[:, :kh] + z, top[:, kh:], bot[:, :kh], bot[:, kh:] + z)):
                ca_s[t, pl.ds(a0 + c, 8), :] = a

    def xs_copy(n):
        return x_copy((n + NH) % NB, n)

    for cp in w_copies(0, 0):
        cp.start()
    c_copy(0).start()
    xs_copy(0).start()
    ht_s[...] = jnp.zeros((HT, M), _F32)
    hb_s[...] = jnp.zeros((HT, M), _F32)
    for cp in w_copies(0, 0):
        cp.wait()
    c_copy(1).start()
    xs_copy(1).start()
    c_copy(0).wait()
    xs_copy(0).wait()

    def pro_a(i, carry):
        @pl.when(i + 2 < NH)
        def _():
            c_copy(i + 2).start()

        @pl.when(i + 2 <= NH)
        def _():
            xs_copy(i + 2).start()

        @pl.when(jnp.logical_and(i >= 1, i <= 2))
        def _():
            wq_copy(i - 1).start()

        @pl.when(i > 0)
        def _():
            c_copy(i).wait()
            xs_copy(i).wait()

        r0 = pl.multiple_of(i * 2 * TQ, 2 * TQ)
        kv = _dot(c_raw[pl.ds(r0, 2 * TQ), :], plain_weights(wk_p.at[0], wv_p.at[0]))
        for nb in range(4):
            _st((k_s, v_s)[nb // 2], nb % 2, r0, kv[:, nb * D:(nb + 1) * D])
        tiles = [(kv, r, nb * D) for nb in range(4) for r in range(0, 2 * TQ, 8)]
        nt = len(tiles)
        a0 = pl.multiple_of(i * TQ, TQ)
        stage_c(r0, a0, pacer(tiles[:nt // 2], HT // 8))
        stage_c(r0 + TQ, a0 + HT, pacer(tiles[nt // 2:nt * 15 // 16], HT // 8))
        rx = pl.multiple_of((i + NH) * TQ, TQ)
        stage_x(rx, xn_s, rx, pacer(tiles[:nt * _PA // 16], TQ // _PX, _FR))
        return carry

    def pro_b(i, carry):
        @pl.when(i + 2 < NH)
        def _():
            xs_copy(NH + i + 2).start()

        @pl.when(i == 2)
        def _():
            for cp in w_copies(1, 1) + wo_copies(0, 0):
                cp.start()
            wq_copy(2).wait()
            wq_copy(3).wait()

        xs_copy(NH + i).wait()
        r0 = pl.multiple_of(i * TQ, TQ)
        xn = xn_s.at[pl.ds(r0, S // 2 + TQ), :]
        kh = M // 2
        lhs = [xn[pl.ds(S // 2, TQ), pl.ds(k0, kh)].astype(_BF16) for k0 in (0, kh)]
        tiles = []
        for nb in range(4):
            d = [_dot(lhs[k], lo_hi(wq_p[nb // 2, pl.ds(k * kh, kh), :])[nb % 2].astype(_BF16))
                 for k in range(2)]
            _st(q_s, nb, r0 + S // 2, d[0] + d[1])
            tiles += [(dk, r, 0) for dk in d for r in range(0, TQ, 8)]
        nt = len(tiles)
        stage_x(r0, xn, 0, pacer(tiles[:nt * _PB // 16], TQ // _PX, _FR))
        nr = MQ // (2 * NH)
        npc = 7 * nr // 16
        pace = pacer(tiles[:nt * _PC // 16], 3 * npc, _FR)
        for k in range(3):
            u = 3 * i + k
            quad = u // (2 * NH)
            prep_wq(2 * quad, quad, pl.multiple_of((u % (2 * NH)) * nr, nr), nr,
                    lambda n, k=k: pace(k * npc + n))
        return carry

    with jax.named_scope('pro_a'):
        lax.fori_loop(0, NH, pro_a, 0)
    wq_copy(0).wait()
    wq_copy(1).wait()
    xs_copy(NH + 1).start()
    wq_copy(2).start()
    wq_copy(3).start()
    with jax.named_scope('pro_b'):
        lax.fori_loop(0, NH, pro_b, 0)

    for cp in w_copies(2, 0) + wo_copies(1, 1) + (wq_copy(4), wq_copy(5)):
        cp.start()
    ffn_start(NP - 1)
    wr_copy = pltpu.make_async_copy(wr_hbm, wr_s, sem_ffn.at[3])
    wr_copy.start()
    for cp in w_copies(1, 1) + wo_copies(0, 0):
        cp.wait()

    tri = (lax.broadcasted_iota(_I32, (HT, HT), 1)
           <= lax.broadcasted_iota(_I32, (HT, HT), 0))

    def softmax_rows(parts, _TIE):
        s = parts[0] if len(parts) == 1 else jnp.concatenate(parts, axis=1)
        m = jnp.max(s, axis=1, keepdims=True)
        p = jnp.exp2(s - m)
        nt = p.shape[1] // HT
        tiles, acc, grp = [], None, None
        for j in range(nt):
            pj = p[:, j * HT:(j + 1) * HT]
            grp = pj if grp is None else grp + pj
            if j % _TIE == _TIE - 1 or j == nt - 1:
                if _CHAIN:
                    acc = grp if acc is None else acc + grp
                    if j > 0:
                        pj = jnp.minimum(pj, acc)
                else:
                    if j % _TIE > 0:
                        pj = jnp.minimum(pj, grp)
                    acc = grp if acc is None else acc + grp
                grp = None
            tiles.append(pj)
        p = tiles[0] if nt == 1 else jnp.concatenate(tiles, axis=1)
        return p, acc

    def scores(q, e, i, zs=()):
        Lm = i * TQ + HT
        nt = Lm // HT
        ties = {(4 + n * (nt - 4) // len(zs)) * QT + 8 * (n % 8): z for n, z in enumerate(zs)}
        keys = _as_bf16(tie(k_s[e, pl.ds(0, Lm // 2), :], ties))
        s_main = _dot_nt(_ld(q, e, i * TQ, TQ), keys)
        s_last = _dot_nt(_ld(q, e, i * TQ + HT, HT), _ld(k_s, e, Lm, HT))
        return s_main, s_last

    def values(e, i):
        Lm = i * TQ + HT
        return _ld(v_s, e, 0, Lm), _ld(v_s, e, Lm, HT)

    def context(vals, head, i, s_main, s_last, group=_TIE):
        Lm = i * TQ + HT
        top = [jnp.where(tri, s_main[:HT, Lm - HT:], _NEG)]
        if Lm > HT:
            top = [s_main[:HT, :Lm - HT]] + top
        p_top, l_top = softmax_rows(top, group)
        p_bot, l_bot = softmax_rows([s_main[HT:], jnp.where(tri, s_last, _NEG)], group)
        p_main = jnp.concatenate([p_top, p_bot[:, :Lm]], axis=0).astype(_BF16)
        o = _dot(p_main, vals[0])
        o_last = _dot(p_bot[:, Lm:].astype(_BF16), vals[1])
        o = jnp.concatenate([o[:HT], o[HT:] + o_last], axis=0)
        acc = jnp.concatenate([l_top, l_bot], axis=0)

        def normalize(pace=None, n0=0):
            zs, z = [], None
            for n, g in enumerate(range(0, TQ, 16)):
                a = acc[g:g + 16]
                if pace is not None:
                    a = a + pltpu.bitcast(pace(n0 + n), _F32)
                linv = jnp.broadcast_to(
                    pl.reciprocal(jnp.sum(a, axis=1, keepdims=True), approx=True), (16, D))
                _st(ctx_s.at[head], None, i * TQ + g, o[g:g + 16] * linv)
                bits = pltpu.bitcast(linv, _U32)
                bits = bits[:8] | bits[8:]
                z = bits if z is None else z | bits
                if n % _NG == _NG - 1:
                    zs.append((z >> 16) >> 16)
                    z = None
            return zs
        return normalize

    def pair_body(s, carry):
        slot = (s + 1) % 2
        odd = s % 2
        wo0 = pl.multiple_of(s * OS, OS)
        q_rd = q_s.at[pl.ds(2 * odd, 2)]
        q_wr = q_s.at[:, pl.ds(pl.multiple_of(odd * (S // 4), S // 4), S // 4), :]
        xn = xn_s.at[pl.ds(pl.multiple_of(odd * (S // 2), S // 2), S // 2), :]
        quad = (s + 1) // 2
        wqb = wqb_s.at[quad % 2]
        pend, sc = {}, {}

        def norm(blocks, tiles):
            fns = [f for i in blocks for f in pend.pop(i)]
            pace = pacer(tiles, len(fns) * (TQ // 16))
            return [z for k, f in enumerate(fns) for z in f(pace, k * (TQ // 16))]

        def qk(i, nrm=()):
            sa = scores(q_rd, 0, i)
            zs = norm(nrm, score_tiles([sa[0]], (2 * i + 1) * QT * _PN // 16)) if nrm else ()
            sc[i] = (sa, scores(q_rd, 1, i, zs))
            return [sa[0], sc[i][1][0]]

        def pv(i):
            pend[i] = [context(values(e, i), 2 * s + e, i, *sc[i][e]) for e in range(2)]

        def kv(j, zs=()):
            return project_kv(ca_s, j * HT, j * TQ, zs)

        for i in range(NB - 1, NH - 1, -1):
            def head_part(i=i):
                mats = qk(i, [i + 2] if i + 2 < NB else [])
                if i == NB - 1:
                    prep_w4((wk_p.at[slot], wv_p.at[slot]), wkvb_s, KQ, range(0, KQ, 16),
                            pacer(score_tiles(mats, 0, _S7), 7 * KQ // 16), 1)
                if i == NB - 2:
                    prep_wq(2 * (jnp.minimum(quad + 1, NP // 2 - 1) % 2), (quad + 1) % 2,
                            pl.multiple_of((1 - odd) * (MQ // 2), MQ // 2), MQ // 2,
                            pacer(score_tiles(mats, 0, _S6), 7 * MQ // 32), 64)
                if i in (NB - 3, NB - 4):
                    r = (NB - 3 - i) * (OS // 2)
                    prep_wo(1 - slot, r, OS // 2, wo0 + r, mats, 2 * TQ + QT)

            if i == NB - 1:
                project_q(xn, (i - NH) * TQ, wqb, q_wr, (i - NH) * TQ, head_part)
            else:
                head_part()
                project_q(xn, (i - NH) * TQ, wqb, q_wr, (i - NH) * TQ)
            pv(i)
        assert NH == 4
        if _LATE == 0:
            qk(1); qk(0); t = kv(7); z = norm([5], t[len(t) // 4:]); pv(1); pv(0); kv(6, z)
            qk(3, [4]); t = kv(5); z = norm([1, 0], t); pv(3); kv(4, z)
            qk(2); kv(3); pv(2)
            t = kv(2); t = kv(1, norm([3], t)); kv(0, norm([2], t))
        elif _LATE == 1:
            qk(3, [5]); kv(7); pv(3); t = kv(6)
            z = norm([4], t); qk(1); qk(0); kv(5, z); pv(1); pv(0); t = kv(4)
            z = norm([3], t); qk(2); kv(3, z); pv(2)
            t = kv(2); t = kv(1, norm([1, 0], t)); kv(0, norm([2], t))
        elif _LATE == 2:
            qk(3, [5]); qk(0); kv(7); pv(3); pv(0); t = kv(6)
            z = norm([4], t); qk(2); qk(1); kv(5, z); pv(2); pv(1)
            t = kv(4); t = kv(3, norm([3], t)); t = kv(2, norm([0], t))
            t = kv(1, norm([2], t)); kv(0, norm([1], t))
        assert not pend

        @pl.when(s + 3 < NP)
        def _():
            for cp in w_copies(s + 3, slot):
                cp.start()

        @pl.when(s + 2 < NP)
        def _():
            for cp in wo_copies(s + 2, 1 - slot):
                cp.start()

        @pl.when(s + 6 < NP)
        def _():
            wq_copy(s + 6).start()

        ffn_start(s)

        @pl.when(s == 0)
        def _():
            wq_copy(4).wait()

        @pl.when(s + 5 < NP)
        def _():
            wq_copy(s + 5).wait()

        @pl.when(s + 2 < NP)
        def _():
            for cp in w_copies(s + 2, 1 - slot):
                cp.wait()

        for cp in wo_copies(s + 1, slot):
            cp.wait()
        return carry

    with jax.named_scope('pair_loop'):
        lax.fori_loop(0, NP - 1, pair_body, 0)

    last_slot = (NP - 1) % 2

    def last_body(e, carry):
        half = OS // 2
        q_rd = q_s.at[pl.ds(2, 2)]
        order = _LORD
        sc = {order[0]: scores(q_rd, e, order[0])}
        prep_wo(last_slot, pl.multiple_of(e * half, half), half,
                pl.multiple_of((NP - 1) * OS + e * half, half), [sc[order[0]][0]], 3 * TQ)
        pend, zs = [], ()
        for n, i in enumerate(order):
            if n + 1 < NB:
                j = order[n + 1]
                sc[j] = scores(q_rd, e, j, zs if j >= 3 else ())
                zs = ()
                if len(pend) >= _LD and n + 2 < NB and order[n + 2] >= 3:
                    zs = pend.pop(0)(pacer(score_tiles([sc[j][0]], (2 * j + 1) * QT), TQ // 16))
            pend.append(context(values(e, i), H - 2 + e, i, *sc[i], group=_TIEL))
        for f in pend:
            f()
        return carry

    with jax.named_scope('last_loop'):
        lax.fori_loop(0, 2, last_body, 0)

    wr_copy.wait()
    wr = wr_s[...].astype(_F32).reshape(1, M)
    sub8 = lax.broadcasted_iota(_I32, (8, HT), 0)

    def epilogue(g, src, top2, pace=None, write_out=True, dist=_END, valid=None):
        r0 = pl.multiple_of(g * HT, HT)
        best, second = top2
        bits = []
        for n, c in enumerate(range(0, HT, 8)):
            hc = src[pl.ds(c, 8), :]
            z = None if pace is None else pace(n)[:8]
            if n >= dist:
                zc = pltpu.bitcast(bits[n - dist] & 0xFFFF, _U32)
                z = zc if z is None else z | zc
            if z is not None:
                hc = jnp.concatenate([hc[:, :HT] + pltpu.bitcast(z, _F32), hc[:, HT:]], axis=1)
            hnb = _layernorm(hc).astype(_BF16)
            hn_s[pl.ds(r0 + c, 8), :] = hnb
            hn = hnb.astype(_F32)
            if write_out:
                out_s[pl.ds(r0 + c, 8), :] = (hc + hn).astype(_BF16)
            r = jnp.broadcast_to(jnp.sum(hn * wr, axis=1, keepdims=True), (8, HT))
            rb = pltpu.bitcast(_round_bf16(r) + 0.0, _I32)
            bits.append(rb)
            key = ((jnp.where(rb < 0, rb ^ 0x7FFF0000, rb) >> (16 - _IDX_BITS))
                   + ((_KEY_BIAS + S - 1 - c - r0) - sub8))
            key = pltpu.bitcast(key, _F32)
            if valid is not None:
                key = jnp.where(valid, key, 0.0)
            second = jnp.maximum(second, jnp.minimum(best, key))
            best = jnp.maximum(best, key)
        return best, second

    def out_copy(g):
        rows = pl.ds(pl.multiple_of(g * HT, HT), HT)
        return pltpu.make_async_copy(out_s.at[rows, :], out_hbm.at[rows, :], sem_out.at[0])

    KS = 2 * D

    def prod(r0, t, tiles, z=None, zu=0):
        ps = [None] * 7
        for u in _ORDER:
            terms = [(2 * (q1 // 2) + q2 // 2, 2 * (q1 % 2) + q2 % 2, s1 * s2)
                     for q1, s1 in _SA[t] for q2, s2 in _SA[u]]
            fence()
            acc = None
            for k0 in range(0, KO, KS):
                def blk(rb, kb):
                    h0 = (kb * KO + k0) // D
                    return jnp.concatenate(
                        [_ld(ctx_s, h0 + hh, (r0, rb * QT), QT) for hh in range(KS // D)], axis=1)
                if len(terms) == 1:
                    lhs = blk(terms[0][0], terms[0][1])
                else:
                    lhs = _combine([(blk(rb, kb).astype(_F32), sg)
                                    for rb, kb, sg in terms]).astype(_BF16)
                w = wob_s[7 * t + u, pl.ds(k0 // 2, KS // 2), :]
                if z is not None and k0 == 0 and u == _ORDER[zu]:
                    w = tie(w, {0: jnp.concatenate([z, z], axis=1)})
                d = _dot(lhs, _as_bf16(w))
                tiles.append((d, 0, 0))
                acc = d if acc is None else acc + d
            ps[u] = acc
        c11, c12, c21, c22 = _strassen_c(ps)
        return jnp.concatenate([jnp.concatenate([c11, c12], axis=1),
                                jnp.concatenate([c21, c22], axis=1)], axis=0)

    NPC = HT // 8

    def zero_of(v):
        return (pltpu.bitcast(v, _U32) >> 16) >> 16

    def o_body(j, top2):
        r0 = pl.multiple_of(j * TQ, TQ)
        lag = 1 if _OSPLIT else 2

        @pl.when(j > 1)
        def _():
            out_copy(2 * j - lag - 2).start()

        @pl.when(j > lag - 1)
        def _():
            out_copy(2 * j - lag - 1).start()

        rh = pl.multiple_of(j * (TQ // 2), TQ // 2)
        left, right = pl.ds(0, M // 2), pl.ds(M // 2, M // 2)

        def residual(dst, rows0, cols, att):
            hb = (x_raw[pl.ds(rows0, HT), cols].astype(_F32) + att).astype(_BF16)
            h_s[pl.ds(rows0, HT), cols] = hb
            dst[:, cols] = hb.astype(_F32)

        tl = []
        m3 = prod(rh, 2, tl)
        m4 = prod(rh, 3, tl)
        gp = jnp.maximum(2 * j - lag, 0)
        top2 = epilogue(gp, hb_s if _OSPLIT else ht_s, top2,
                        pacer(tl[:len(tl) * _O1 // 16], NPC, 1), valid=j > 0)
        tl = []
        m5 = prod(rh, 4, tl, zero_of(top2[0]), _ZU)
        z = None
        residual(ht_s, r0, right, m3 + m5)
        m1 = prod(rh, 0, tl)
        m7 = prod(rh, 6, tl)
        residual(ht_s, r0, left, m4 - m5 + m1 + m7)
        if not _OSPLIT:
            top2 = epilogue(gp + 1, hb_s, top2, pacer(tl[:len(tl) * _O2 // 16], NPC),
                            valid=j > 0)
            z = zero_of(top2[0])
        tl = []
        m2 = prod(rh, 1, tl, z, _ZU)
        residual(hb_s, r0 + HT, left, m4 + m2)
        m6 = prod(rh, 5, tl)
        residual(hb_s, r0 + HT, right, m3 + m1 - m2 + m6)
        if _OSPLIT:
            top2 = epilogue(2 * j, ht_s, top2, pacer(tl[2:len(tl) * _O2 // 16], NPC))
        return top2

    for n in range(3):
        ffn_wait(n)
    with jax.named_scope('o_loop'):
        top2 = lax.fori_loop(0, NB, o_body, (jnp.zeros((8, HT), _F32),) * 2)
    rest = [(NG - 1, hb_s)] if _OSPLIT else [(NG - 2, ht_s), (NG - 1, hb_s)]
    out_copy(rest[0][0] - 2).start()
    out_copy(rest[0][0] - 1).start()
    for g, src in rest:
        top2 = epilogue(g, src, top2, None, False, NPC)

    best, second = top2
    k1 = jnp.max(best, axis=0, keepdims=True)
    k2 = jnp.max(jnp.where(best == k1, second, best), axis=0, keepdims=True)

    R = _FIX
    row = lax.broadcasted_iota(_I32, (2 * R, HT), 0)
    idx = S - 1 - (pltpu.bitcast(jnp.where(row < R, k1, k2), _I32) & (2 ** _IDX_BITS - 1))
    i1 = jnp.clip(idx[0, 0], 0, S - 1)
    i2 = jnp.clip(idx[R, 0], 0, S - 1)
    b1 = pl.multiple_of(i1 & -R, R)
    b2 = pl.multiple_of(i2 & -R, R)
    tokr = jnp.where(row < R, b1 + row, b2 + row - R)
    cd = (((pltpu.bitcast(jnp.where(tokr == i1, k1, k2), _I32) - _KEY_BIAS) >> _IDX_BITS) << 16)
    score = pltpu.bitcast(jnp.where(cd < 0, cd ^ 0x7FFF0000, cd), _F32)
    gate = _round_bf16(1.0 / (1.0 + jnp.exp(-score)))
    gate = jnp.concatenate([gate] * (M // HT), axis=1)
    tokr = jnp.concatenate([tokr] * (M // HT), axis=1)

    hnsel = jnp.concatenate([hn_s[pl.ds(b1, R), :].astype(_F32),
                             hn_s[pl.ds(b2, R), :].astype(_F32)], axis=0)
    xs = hnsel.astype(_BF16)
    g = _dot(xs, wg_s[...])
    u = _dot(xs, wu_s[...])
    pace = pacer([(mat, 0, c0) for mat in (g, u) for c0 in range(0, F, HT)],
                 len(rest) * HT // 8)
    for k, (gi, src) in enumerate(rest):
        for n, c in enumerate(range(0, HT, 8)):
            rows = pl.ds(gi * HT + c, 8)
            z = pltpu.bitcast(pace(k * HT // 8 + n)[:8], _F32)
            z = jnp.concatenate([z] * (M // HT), axis=1)
            out_s[rows, :] = (src[pl.ds(c, 8), :] + z + hn_s[rows, :].astype(_F32)).astype(_BF16)
        out_copy(gi).start()
    g = _round_bf16(g)
    u = _round_bf16(u)
    g = _round_bf16(g * (1.0 / (1.0 + jnp.exp(-g))))
    act = (g * u).astype(_BF16)
    y = _round_bf16(_dot(act, wd_s[:, pl.ds(0, M)]))
    y = _round_bf16(y * gate)
    upd = jnp.where(jnp.logical_or(tokr == i1, tokr == i2), y, 0.0)
    hsel = jnp.concatenate([h_s[pl.ds(b1, R), :].astype(_F32),
                            h_s[pl.ds(b2, R), :].astype(_F32)], axis=0)
    fixed = hsel + _round_bf16(hnsel + upd)

    pltpu.make_async_copy(out_s, out_hbm, sem_out.at[0]).wait()

    def fix_copy(b0, k):
        return pltpu.make_async_copy(out_s.at[pl.ds(b0, R), :],
                                     out_hbm.at[pl.ds(b0, R), :], sem_out.at[k])

    out_s[pl.ds(b1, R), :] = fixed[:R].astype(_BF16)
    out_s[pl.ds(b2, R), :] = fixed[R:].astype(_BF16)
    fix_copy(b1, 0).start()

    @pl.when(b2 != b1)
    def _():
        fix_copy(b2, 1).start()
        fix_copy(b2, 1).wait()

    fix_copy(b1, 0).wait()


@jax.jit
def pallas_sequential_preLN__compressed_kv_cla__moe_arch_mod__prompt_kernel(
    A_x: jax.Array,
    A_c_kv: jax.Array,
    A_w_q: jax.Array,
    A_w_uk: jax.Array,
    A_w_uv: jax.Array,
    A_w_o: jax.Array,
    B_x: jax.Array,
    B_w_r: jax.Array,
    B_w_gate: jax.Array,
    B_w_up: jax.Array,
    B_w_down: jax.Array,
):
    B, S, M = A_x.shape
    assert B == 1
    DC = A_c_kv.shape[2]
    H, D = A_w_q.shape[1], A_w_q.shape[2]
    F = B_w_gate.shape[1]
    assert A_c_kv.shape[1] == S and S % _TQ == 0 and H % 2 == 0 and S <= 2 ** _IDX_BITS
    NP = H // 2
    NG = S // _HT

    x = A_x.reshape(S, M)
    c = A_c_kv.reshape(S, DC)
    wo = A_w_o.reshape(H * D, M)

    any_spec = pl.BlockSpec(memory_space=pl.ANY)
    def buf(name, lead, rows, cols):
        if name in _U32BUF:
            return pltpu.VMEM((lead, rows // 2, cols), _U32)
        return pltpu.VMEM((lead, rows, cols), _BF16)

    scratch = [
        pltpu.VMEM((S, M), _BF16),
        pltpu.VMEM((S, DC), _BF16),
        pltpu.VMEM((S, M), _F32),
        pltpu.VMEM((7, S // 2, DC // 2), _F32),
        buf('q', 4, S, D),
        buf('k', 2, S, D),
        buf('v', 2, S, D),
        pltpu.VMEM((4, M, D), _U32),
        pltpu.VMEM((2, DC, D), _U32),
        pltpu.VMEM((2, DC, D), _U32),
        pltpu.VMEM((2, 49, M // 8, D), _U32),
        buf('wb', 49, DC // 4, D),
        buf('ctx', H, S, D),
        pltpu.VMEM((2, 4, D // 2, M), _BF16),
        buf('wob', 49, H * D // 4, M // 4),
        pltpu.VMEM((M, F), _BF16),
        pltpu.VMEM((M, F), _BF16),
        pltpu.VMEM((F, M + _WD_PAD), _BF16),
        pltpu.VMEM((_HT, M), _F32),
        pltpu.VMEM((_HT, M), _F32),
        pltpu.VMEM((S, M), _BF16),
        pltpu.VMEM((S, M), _BF16),
        pltpu.VMEM((1024, _HT), _U32),
        pltpu.VMEM((S, M), _BF16),
        pltpu.VMEM((M,), _BF16),
        pltpu.SemaphoreType.DMA((3,)),
        pltpu.SemaphoreType.DMA((3,)),
        pltpu.SemaphoreType.DMA((2, 2)),
        pltpu.SemaphoreType.DMA((4,)),
        pltpu.SemaphoreType.DMA((2, 4)),
        pltpu.SemaphoreType.DMA((4,)),
        pltpu.SemaphoreType.DMA((2,)),
    ]
    out = pl.pallas_call(
        functools.partial(_kernel, S=S, M=M, DC=DC, H=H, D=D, F=F),
        in_specs=[any_spec] * 10,
        out_specs=any_spec,
        out_shape=jax.ShapeDtypeStruct((S, M), _BF16),
        scratch_shapes=scratch,
        compiler_params=pltpu.CompilerParams(vmem_limit_bytes=124 * 1024 * 1024,
                                             disable_bounds_checks=True,
                                             disable_semaphore_checks=True),
        name="fused_mla_mod",
    )(x, c, A_w_q, A_w_uk, A_w_uv, wo, B_w_r, B_w_gate, B_w_up, B_w_down)
    return out.reshape(B, S, M)
```

```python
import functools
import math

import jax
import jax.numpy as jnp
from jax import lax
import jax.experimental.pallas as pl
import jax.experimental.pallas.tpu as pltpu

_F32 = jnp.float32
_BF16 = jnp.bfloat16
_U32 = jnp.uint32
_I32 = jnp.int32

_EPS = 1e-5
_NEG = -1e30
_TQ = 256
_HT = 128
import os
_TIE = int(os.environ.get('TIE', 4))
_CHAIN = int(os.environ.get('CHAIN', 0))
_ERG = int(os.environ.get('ERG', 8))
_EORD = int(os.environ.get('EORD', 0))
_EVAL = int(os.environ.get('EVAL', 1))
_U32BUF = os.environ.get('U32', 'xa,ca,q,k,v,wob,ctx,wb').split(',')
_PA = int(os.environ.get('PA', 13))
_PB = int(os.environ.get('PB', 13))
_PC = int(os.environ.get('PC', 16))
_PX = int(os.environ.get('PX', 8))
_OSPLIT = int(os.environ.get('OSPLIT', 0))
_O1 = int(os.environ.get('O1', 14))
_O2 = int(os.environ.get('O2', 14))
_END = int(os.environ.get('END', 3))
_WQS = int(os.environ.get('WQS', 672))
_NG = int(os.environ.get('NG', 16))
_BIG = int(os.environ.get('BIG', 3))
_TSPAN = 360
_DIST = int(os.environ.get('DIST', 2))
_PN = int(os.environ.get('PN', 14))
_WOH = int(os.environ.get('WOH', 0))
_LND = int(os.environ.get('LND', 6))
_FR = int(os.environ.get('FR', 0))
_LATE = int(os.environ.get('LATE', 2))
_TIEL = int(os.environ.get('TIEL', 3))
_LD = int(os.environ.get('LD', 9))
_LORD = [int(c) for c in os.environ.get('LORD', '76543210')]
_ZU = int(os.environ.get('ZU', 1))
_FD = int(os.environ.get('FD', 99))
_LEAD = int(os.environ.get('LEAD', 0))
def _sp(k, d):
    v = [int(t) for t in os.environ.get(k, d).split(',')]
    return [(v[0], v[1]), (v[2], v[3])]
_S7 = _sp('S7', '0,768,128,896')
_S6 = _sp('S6', '0,672,0,672')
_IDX_BITS = 13
_KEY_BIAS = 0x30000000
_FIX = 8
_WD_PAD = 128


def _dot(a, b):
    return jnp.dot(a, b, preferred_element_type=_F32)


def _dot_nt(a, b):
    return lax.dot_general(a, b, (((1,), (1,)), ((), ())), preferred_element_type=_F32)


def _as_bf16(u):
    return pltpu.bitcast(u, _BF16)


def _pack(x):
    return pltpu.bitcast(x.astype(_BF16), _U32)


def _rows(ref, r0, n):
    if ref.dtype == _U32:
        if isinstance(r0, tuple):
            return pl.ds(r0[0] + r0[1] // 2, n // 2)
        if isinstance(r0, int):
            return pl.ds(r0 // 2, n // 2)
        return pl.ds(pl.multiple_of(r0 // 2, 8), n // 2)
    return pl.ds(r0, n)


def _ld(ref, lead, r0, n):
    v = ref[lead, _rows(ref, r0, n), :]
    return _as_bf16(v) if ref.dtype == _U32 else v


def _st(ref, lead, r0, x, cols=slice(None)):
    v = _pack(x) if ref.dtype == _U32 else x.astype(_BF16)
    if lead is None:
        ref[_rows(ref, r0, x.shape[0]), cols] = v
    else:
        ref[lead, _rows(ref, r0, x.shape[0]), cols] = v


def _round_bf16(x):
    return x.astype(_BF16).astype(_F32)


def _layernorm(x):
    n = x.shape[-1]
    mean = jnp.sum(x, axis=-1, keepdims=True) * (1.0 / n)
    xc = x - mean
    var = jnp.sum(xc * xc, axis=-1, keepdims=True) * (1.0 / n)
    m = _round_bf16(mean)
    den = _round_bf16(jnp.sqrt(_round_bf16(_round_bf16(var) + _EPS)))
    return (x - m) * pl.reciprocal(den, approx=True)


def _layernorm_scaled(x, scale):
    n = x.shape[-1]
    mean = jnp.sum(x, axis=-1, keepdims=True) * (1.0 / n)
    xc = x - mean
    var = jnp.sum(xc * xc, axis=-1, keepdims=True) * (1.0 / n)
    return xc * (lax.rsqrt(var + _EPS) * scale)


def _strassen_a(a11, a12, a21, a22):
    return (a11 + a22, a21 + a22, a11, a22, a11 + a12, a21 - a11, a12 - a22)


def _strassen_b(b11, b12, b21, b22):
    return (b11 + b22, b11, b12 - b22, b21 - b11, b22, b11 + b12, b21 + b22)


def _strassen_c(m):
    m1, m2, m3, m4, m5, m6, m7 = m
    return (m4 - m5 + m1 + m7, m3 + m5, m4 + m2, m3 - m2 + m1 + m6)


_ORDER = (2, 4, 3, 1, 0, 6, 5)


_SA = (((0, 1), (3, 1)), ((2, 1), (3, 1)), ((0, 1),), ((3, 1),),
       ((0, 1), (1, 1)), ((2, 1), (0, -1)), ((1, 1), (3, -1)))
_SB = (((0, 1), (3, 1)), ((0, 1),), ((1, 1), (3, -1)), ((2, 1), (0, -1)),
       ((3, 1),), ((0, 1), (1, 1)), ((2, 1), (3, 1)))


def _combine(terms):
    terms = sorted(terms, key=lambda ts: -ts[1])
    acc = terms[0][0]
    assert terms[0][1] > 0
    for v, sg in terms[1:]:
        acc = acc + v if sg > 0 else acc - v
    return acc


def _quadrants(x):
    r, c = x.shape[0] // 2, x.shape[1] // 2
    return x[:r, :c], x[:r, c:], x[r:, :c], x[r:, c:]


def _kernel(x_hbm, c_hbm, wq_hbm, wk_hbm, wv_hbm, wo_hbm, wr_hbm, wg_hbm, wu_hbm, wd_hbm,
            out_hbm,
            x_raw, c_raw, xn_s, ca_s, q_s, k_s, v_s,
            wq_p, wk_p, wv_p, wqb_s, wkvb_s,
            ctx_s, wo_p, wob_s, wg_s, wu_s, wd_s, ht_s, hb_s, h_s, hn_s, junk_s, out_s, wr_s,
            sem_x, sem_c, sem_w, sem_wq, sem_wo, sem_ffn, sem_out,
            *, S, M, DC, H, D, F):
    TQ, HT = _TQ, _HT
    NB = S // TQ
    NG = S // HT
    NP = H // 2
    KO = H * D // 4
    NO = M // 4
    OS = KO // NP
    qscale = (D ** -0.5) * math.log2(math.e)

    wq32 = wq_hbm.bitcast(_U32)
    wk32 = wk_hbm.bitcast(_U32)
    wv32 = wv_hbm.bitcast(_U32)

    def w_copies(pair, slot):
        return (
            pltpu.make_async_copy(wk32.at[:, pair, :], wk_p.at[slot], sem_w.at[slot, 0]),
            pltpu.make_async_copy(wv32.at[:, pair, :], wv_p.at[slot], sem_w.at[slot, 1]),
        )

    def wq_copy(pair):
        return pltpu.make_async_copy(wq32.at[:, pair, :], wq_p.at[pair % 4],
                                     sem_wq.at[pair % 4])

    def wo_copies(t, slot):
        r0 = pl.multiple_of(t * OS, OS)
        return tuple(
            pltpu.make_async_copy(wo_hbm.at[pl.ds(half * KO + r0, OS), :],
                                  wo_p.at[slot, half], sem_wo.at[slot, half])
            for half in range(4))

    def x_copy(i, n):
        rows = pl.ds(pl.multiple_of(i * TQ, TQ), TQ)
        return pltpu.make_async_copy(x_hbm.at[rows, :], x_raw.at[rows, :], sem_x.at[n % 3])

    def c_copy(i):
        rows = pl.ds(pl.multiple_of(i * 2 * TQ, 2 * TQ), 2 * TQ)
        return pltpu.make_async_copy(c_hbm.at[rows, :], c_raw.at[rows, :], sem_c.at[i % 3])

    ffn = ((wg_hbm, wg_s), (wu_hbm, wu_s), (wd_hbm, wd_s))

    def ffn_start(t):
        for n, (src, dst) in enumerate(ffn):
            rows, cols = src.shape[0] // NP, src.shape[1]
            r0 = pl.multiple_of(t * rows, 16)
            pltpu.make_async_copy(src.at[pl.ds(r0, rows), :],
                                  dst.at[pl.ds(r0, rows), pl.ds(0, cols)],
                                  sem_ffn.at[n]).start()

    def ffn_wait(n):
        src, dst = ffn[n]
        pltpu.make_async_copy(src, dst.at[:, pl.ds(0, src.shape[1])], sem_ffn.at[n]).wait()

    def lo_hi(w):
        return (pltpu.bitcast(w << 16, _F32), pltpu.bitcast(w & jnp.uint32(0xFFFF0000), _F32))

    def pacer(tiles, total, free=0):
        def zero(n):
            if n < free:
                return jnp.zeros((16, HT), _U32)
            mat, zr, zc = tiles[(n - free) * len(tiles) // (total - free)]
            z = pltpu.bitcast(mat[zr:zr + 8, zc:zc + HT], _U32)
            z = (z >> 16) >> 16
            return jnp.concatenate([z, z], axis=0)
        return zero

    def score_tiles(mats, span, spans=None):
        spans = spans or [(0, span)] * len(mats)
        return [(m, t0 % TQ, (t0 // TQ) * 4 * HT)
                for m, (lo, hi) in zip(mats, spans) for t0 in range(lo, hi, 8)]

    def prep_w4(srcs, dst, kq, rows, pace=None, sink=None):
        pieces = [(t, r) for t in range(7) for r in rows]
        for n, (t, r) in enumerate(pieces):
            terms = [[] for _ in range(4)]
            for k, (q1, sg) in enumerate(_SB[t]):
                for rb in range(2):
                    w = srcs[q1 % 2][pl.ds((2 * (q1 // 2) + rb) * kq + r, 16), :]
                    if pace is not None and k == 0:
                        w = w | pace(n)
                    lo, hi = lo_hi(w)
                    terms[2 * rb].append((lo, sg))
                    terms[2 * rb + 1].append((hi, sg))
            z = None
            for u, b in enumerate(_strassen_b(*[_combine(tm) for tm in terms])):
                pk = _pack(b)
                dst[7 * t + u, pl.ds(r // 2, 8), :] = pk
                z = pk if z is None else z | pk
            if sink is not None:
                junk_s[pl.ds(8 * (sink + n), 8), :] = z

    def prep_wo(slot, src0, nrows, dst0, mats, span):
        pieces = [(r, c0, t) for r in range(0, nrows, 16) for c0 in range(0, NO, HT)
                  for t in range(7)]
        pace = pacer(score_tiles(mats, span), len(pieces))
        for n, (r, c0, t) in enumerate(pieces):
            z = pltpu.bitcast(pace(n), _F32)
            rs = pl.ds(src0 + r, 16)
            sub = []
            for q2 in range(4):
                v = _combine([
                    (wo_p[slot, 2 * (q1 // 2) + q2 // 2, rs,
                          pl.ds((2 * (q1 % 2) + q2 % 2) * NO + c0, HT)].astype(_F32), sg)
                    for q1, sg in _SB[t]])
                sub.append(v + z if q2 in (0, 3) else v)
            for u, b in enumerate(_strassen_b(*sub)):
                _st(wob_s, 7 * t + u, dst0 + r, b, pl.ds(c0, HT))

    QT = HT // 2
    KQ = DC // 4
    MQ = M // 4

    def fence():
        junk_s[pl.ds(0, 8), :] = jnp.zeros((8, HT), _U32)

    def tie(w, ties):
        parts, at = [], 0
        for r in sorted(ties):
            if r > at:
                parts.append(w[at:r])
            parts.append(w[r:r + 8] | ties[r])
            at = r + 8
        if at < w.shape[0]:
            parts.append(w[at:])
        return parts[0] if len(parts) == 1 else jnp.concatenate(parts, axis=0)

    def project4(lhs, w, store, zs=(), mid=None):
        m, tiles, cnt = [None] * 7, [], [0]
        for t in _ORDER:
            ps = [None] * 7
            for u in _ORDER:
                if mid is not None and t == _ORDER[0] and u == _ORDER[_LEAD]:
                    mid()
                fence()
                a = lhs(t, u)
                wt = w[7 * t + u]
                n = len(tiles) * len(zs) * D * 8 // (_TSPAN * a.shape[1] * 2)
                done = cnt[0]
                if zs and done < len(zs) and n > done:
                    wt = tie(wt, {0: zs[done]})
                    cnt[0] += 1
                ps[u] = _dot(a.astype(_BF16), _as_bf16(wt))
                tiles += [(ps[u], r, 0) for r in range(0, QT, QT * D // (2 * a.shape[1]))]
            m[t] = _strassen_c(ps)
        for q2 in range(4):
            for q1, cblk in enumerate(_strassen_c([mt[q2] for mt in m])):
                store(2 * (q1 % 2) + q2 % 2, (2 * (q1 // 2) + q2 // 2) * QT, cblk)
        return tiles

    def project_q(xn, x0, wqb, q, r0, mid=None):
        def lhs(t, u):
            return _combine([
                (xn[pl.ds(x0 + (2 * (q1 // 2) + q2 // 2) * QT, QT),
                    pl.ds((2 * (q1 % 2) + q2 % 2) * MQ, MQ)], s1 * s2)
                for q1, s1 in _SA[t] for q2, s2 in _SA[u]])
        return project4(lhs, wqb, lambda nb, r, val: _st(q, nb, r0 + r, val), (), mid)

    def project_kv(ca, a0, r0, zs=()):
        def lhs(t, u):
            return _combine([
                (ca[t, pl.ds(a0 + (q2 // 2) * QT, QT), pl.ds((q2 % 2) * KQ, KQ)], sg)
                for q2, sg in _SA[u]])
        return project4(lhs, wkvb_s,
                        lambda nb, r, val: _st((k_s, v_s)[nb // 2], nb % 2, r0 + r, val), zs)

    def prep_wq(raw, slot, r, nr, pace, sink=None):
        span = 3 * MQ + nr
        prep_w4((wq_p.at[raw, pl.ds(r, span), :], wq_p.at[raw + 1, pl.ds(r, span), :]),
                wqb_s.at[slot, :, pl.ds(pl.multiple_of(r // 2, 8), nr // 2), :],
                MQ, range(0, nr, 16), pace, sink)

    NH = NB // 2

    def plain_weights(src0, src1):
        return jnp.concatenate(lo_hi(src0[...]) + lo_hi(src1[...]), axis=1).astype(_BF16)

    def stage_x(r0, xn, x0, pace):
        done = []
        for n, c in enumerate(range(0, TQ, _PX)):
            xr = x_raw[pl.ds(r0 + c, _PX), :].astype(_F32)
            z = pace(n)[:_PX]
            if n >= _LND:
                z = z | done[n - _LND]
            xr = jnp.concatenate([xr[:, :HT] + pltpu.bitcast(z, _F32), xr[:, HT:]], axis=1)
            y = _layernorm_scaled(xr, qscale)
            xn[pl.ds(x0 + c, _PX), :] = y
            done.append((pltpu.bitcast(y[:, :HT], _U32) >> 16) >> 16)

    def stage_c(r0, a0, pace):
        kh = DC // 2
        for n, c in enumerate(range(0, HT, 8)):
            top = c_raw[pl.ds(r0 + c, 8), :].astype(_F32)
            bot = c_raw[pl.ds(r0 + HT + c, 8), :].astype(_F32)
            z = pltpu.bitcast(pace(n)[:8], _F32)
            z = jnp.concatenate([z] * (kh // HT), axis=1)
            for t, a in enumerate(
                    _strassen_a(top[:, :kh] + z, top[:, kh:], bot[:, :kh], bot[:, kh:] + z)):
                ca_s[t, pl.ds(a0 + c, 8), :] = a

    def xs_copy(n):
        return x_copy((n + NH) % NB, n)

    for cp in w_copies(0, 0):
        cp.start()
    c_copy(0).start()
    xs_copy(0).start()
    ht_s[...] = jnp.zeros((HT, M), _F32)
    hb_s[...] = jnp.zeros((HT, M), _F32)
    for cp in w_copies(0, 0):
        cp.wait()
    c_copy(1).start()
    xs_copy(1).start()
    c_copy(0).wait()
    xs_copy(0).wait()

    def pro_a(i, carry):
        @pl.when(i + 2 < NH)
        def _():
            c_copy(i + 2).start()

        @pl.when(i + 2 <= NH)
        def _():
            xs_copy(i + 2).start()

        @pl.when(jnp.logical_and(i >= 1, i <= 2))
        def _():
            wq_copy(i - 1).start()

        r0 = pl.multiple_of(i * 2 * TQ, 2 * TQ)
        kv = _dot(c_raw[pl.ds(r0, 2 * TQ), :], plain_weights(wk_p.at[0], wv_p.at[0]))
        for nb in range(4):
            _st((k_s, v_s)[nb // 2], nb % 2, r0, kv[:, nb * D:(nb + 1) * D])
        tiles = [(kv, r, nb * D) for nb in range(4) for r in range(0, 2 * TQ, 8)]
        nt = len(tiles)
        a0 = pl.multiple_of(i * TQ, TQ)
        stage_c(r0, a0, pacer(tiles[:nt // 2], HT // 8))
        stage_c(r0 + TQ, a0 + HT, pacer(tiles[nt // 2:nt * 15 // 16], HT // 8))
        rx = pl.multiple_of((i + NH) * TQ, TQ)
        stage_x(rx, xn_s, rx, pacer(tiles[:nt * _PA // 16], TQ // _PX, _FR))

        @pl.when(i + 1 < NH)
        def _():
            c_copy(i + 1).wait()

        xs_copy(i + 1).wait()
        return carry

    def pro_b(i, carry):
        @pl.when(i + 2 < NH)
        def _():
            xs_copy(NH + i + 2).start()

        @pl.when(i == 2)
        def _():
            for cp in w_copies(1, 1) + wo_copies(0, 0):
                cp.start()

        r0 = pl.multiple_of(i * TQ, TQ)
        xn = xn_s.at[pl.ds(r0, S // 2 + TQ), :]
        kh = M // 2
        lhs = [xn[pl.ds(S // 2, TQ), pl.ds(k0, kh)].astype(_BF16) for k0 in (0, kh)]
        tiles = []
        for nb in range(4):
            d = [_dot(lhs[k], lo_hi(wq_p[nb // 2, pl.ds(k * kh, kh), :])[nb % 2].astype(_BF16))
                 for k in range(2)]
            _st(q_s, nb, r0 + S // 2, d[0] + d[1])
            tiles += [(dk, r, 0) for dk in d for r in range(0, TQ, 8)]
        nt = len(tiles)
        stage_x(r0, xn, 0, pacer(tiles[:nt * _PB // 16], TQ // _PX, _FR))
        nr = MQ // (2 * NH)
        npc = 7 * nr // 16
        pace = pacer(tiles[:nt * _PC // 16], 3 * npc, _FR)
        for k in range(3):
            u = 3 * i + k
            quad = u // (2 * NH)
            prep_wq(2 * quad, quad, pl.multiple_of((u % (2 * NH)) * nr, nr), nr,
                    lambda n, k=k: pace(k * npc + n))

        @pl.when(i == 1)
        def _():
            wq_copy(2).wait()
            wq_copy(3).wait()

        @pl.when(i + 1 < NH)
        def _():
            xs_copy(NH + i + 1).wait()

        return carry

    with jax.named_scope('pro_a'):
        lax.fori_loop(0, NH, pro_a, 0)
    wq_copy(0).wait()
    wq_copy(1).wait()
    xs_copy(NH + 1).start()
    wq_copy(2).start()
    wq_copy(3).start()
    with jax.named_scope('pro_b'):
        lax.fori_loop(0, NH, pro_b, 0)

    for cp in w_copies(2, 0) + wo_copies(1, 1) + (wq_copy(4), wq_copy(5)):
        cp.start()
    ffn_start(NP - 1)
    wr_copy = pltpu.make_async_copy(wr_hbm, wr_s, sem_ffn.at[3])
    wr_copy.start()
    for cp in w_copies(1, 1) + wo_copies(0, 0):
        cp.wait()

    tri = (lax.broadcasted_iota(_I32, (HT, HT), 1)
           <= lax.broadcasted_iota(_I32, (HT, HT), 0))

    def softmax_rows(parts, _TIE):
        s = parts[0] if len(parts) == 1 else jnp.concatenate(parts, axis=1)
        m = jnp.max(s, axis=1, keepdims=True)
        p = jnp.exp2(s - m)
        nt = p.shape[1] // HT
        tiles, acc, grp = [], None, None
        for j in range(nt):
            pj = p[:, j * HT:(j + 1) * HT]
            grp = pj if grp is None else grp + pj
            if j % _TIE == _TIE - 1 or j == nt - 1:
                if _CHAIN:
                    acc = grp if acc is None else acc + grp
                    if j > 0:
                        pj = jnp.minimum(pj, acc)
                else:
                    if j % _TIE > 0:
                        pj = jnp.minimum(pj, grp)
                    acc = grp if acc is None else acc + grp
                grp = None
            tiles.append(pj)
        p = tiles[0] if nt == 1 else jnp.concatenate(tiles, axis=1)
        return p, acc

    def scores(q, e, i, zs=()):
        Lm = i * TQ + HT
        nt = Lm // HT
        ties = {(4 + n * (nt - 4) // len(zs)) * QT + 8 * (n % 8): z for n, z in enumerate(zs)}
        keys = _as_bf16(tie(k_s[e, pl.ds(0, Lm // 2), :], ties))
        s_main = _dot_nt(_ld(q, e, i * TQ, TQ), keys)
        s_last = _dot_nt(_ld(q, e, i * TQ + HT, HT), _ld(k_s, e, Lm, HT))
        return s_main, s_last

    def values(e, i):
        Lm = i * TQ + HT
        return _ld(v_s, e, 0, Lm), _ld(v_s, e, Lm, HT)

    def context(vals, head, i, s_main, s_last, group=_TIE):
        Lm = i * TQ + HT
        top = [jnp.where(tri, s_main[:HT, Lm - HT:], _NEG)]
        if Lm > HT:
            top = [s_main[:HT, :Lm - HT]] + top
        p_top, l_top = softmax_rows(top, group)
        p_bot, l_bot = softmax_rows([s_main[HT:], jnp.where(tri, s_last, _NEG)], group)
        p_main = jnp.concatenate([p_top, p_bot[:, :Lm]], axis=0).astype(_BF16)
        o = _dot(p_main, vals[0])
        o_last = _dot(p_bot[:, Lm:].astype(_BF16), vals[1])
        o = jnp.concatenate([o[:HT], o[HT:] + o_last], axis=0)
        acc = jnp.concatenate([l_top, l_bot], axis=0)

        def normalize(pace=None, n0=0):
            zs, z = [], None
            for n, g in enumerate(range(0, TQ, 16)):
                a = acc[g:g + 16]
                if pace is not None:
                    a = a + pltpu.bitcast(pace(n0 + n), _F32)
                linv = jnp.broadcast_to(
                    pl.reciprocal(jnp.sum(a, axis=1, keepdims=True), approx=True), (16, D))
                _st(ctx_s.at[head], None, i * TQ + g, o[g:g + 16] * linv)
                bits = pltpu.bitcast(linv, _U32)
                bits = bits[:8] | bits[8:]
                z = bits if z is None else z | bits
                if n % _NG == _NG - 1:
                    zs.append((z >> 16) >> 16)
                    z = None
            return zs
        return normalize

    def pair_body(s, carry):
        slot = (s + 1) % 2
        odd = s % 2
        wo0 = pl.multiple_of(s * OS, OS)
        q_rd = q_s.at[pl.ds(2 * odd, 2)]
        q_wr = q_s.at[:, pl.ds(pl.multiple_of(odd * (S // 4), S // 4), S // 4), :]
        xn = xn_s.at[pl.ds(pl.multiple_of(odd * (S // 2), S // 2), S // 2), :]
        quad = (s + 1) // 2
        wqb = wqb_s.at[quad % 2]
        pend, sc = {}, {}

        def norm(blocks, tiles):
            fns = [f for i in blocks for f in pend.pop(i)]
            pace = pacer(tiles, len(fns) * (TQ // 16))
            return [z for k, f in enumerate(fns) for z in f(pace, k * (TQ // 16))]

        def qk(i, nrm=()):
            sa = scores(q_rd, 0, i)
            zs = norm(nrm, score_tiles([sa[0]], (2 * i + 1) * QT * _PN // 16)) if nrm else ()
            sc[i] = (sa, scores(q_rd, 1, i, zs))
            return [sa[0], sc[i][1][0]]

        def pv(i):
            pend[i] = [context(values(e, i), 2 * s + e, i, *sc[i][e]) for e in range(2)]

        def kv(j, zs=()):
            return project_kv(ca_s, j * HT, j * TQ, zs)

        for i in range(NB - 1, NH - 1, -1):
            def head_part(i=i):
                mats = qk(i, [i + 2] if i + 2 < NB else [])
                if i == NB - 1:
                    prep_w4((wk_p.at[slot], wv_p.at[slot]), wkvb_s, KQ, range(0, KQ, 16),
                            pacer(score_tiles(mats, 0, _S7), 7 * KQ // 16), 1)
                if i == NB - 2:
                    prep_wq(2 * (jnp.minimum(quad + 1, NP // 2 - 1) % 2), (quad + 1) % 2,
                            pl.multiple_of((1 - odd) * (MQ // 2), MQ // 2), MQ // 2,
                            pacer(score_tiles(mats, 0, _S6), 7 * MQ // 32), 64)
                if i in (NB - 3, NB - 4):
                    r = (NB - 3 - i) * (OS // 2)
                    prep_wo(1 - slot, r, OS // 2, wo0 + r, mats, 2 * TQ + QT)

            if i == NB - 1:
                project_q(xn, (i - NH) * TQ, wqb, q_wr, (i - NH) * TQ, head_part)
            else:
                head_part()
                project_q(xn, (i - NH) * TQ, wqb, q_wr, (i - NH) * TQ)
            pv(i)
        assert NH == 4
        if _LATE == 0:
            qk(1); qk(0); t = kv(7); z = norm([5], t[len(t) // 4:]); pv(1); pv(0); kv(6, z)
            qk(3, [4]); t = kv(5); z = norm([1, 0], t); pv(3); kv(4, z)
            qk(2); kv(3); pv(2)
            t = kv(2); t = kv(1, norm([3], t)); kv(0, norm([2], t))
        elif _LATE == 1:
            qk(3, [5]); kv(7); pv(3); t = kv(6)
            z = norm([4], t); qk(1); qk(0); kv(5, z); pv(1); pv(0); t = kv(4)
            z = norm([3], t); qk(2); kv(3, z); pv(2)
            t = kv(2); t = kv(1, norm([1, 0], t)); kv(0, norm([2], t))
        elif _LATE == 2:
            qk(3, [5]); qk(0); kv(7); pv(3); pv(0); t = kv(6)
            z = norm([4], t); qk(2); qk(1); kv(5, z); pv(2); pv(1)
            t = kv(4); t = kv(3, norm([3], t)); t = kv(2, norm([0], t))
            t = kv(1, norm([2], t)); kv(0, norm([1], t))
        assert not pend

        @pl.when(s + 3 < NP)
        def _():
            for cp in w_copies(s + 3, slot):
                cp.start()

        @pl.when(s + 2 < NP)
        def _():
            for cp in wo_copies(s + 2, 1 - slot):
                cp.start()

        @pl.when(s + 6 < NP)
        def _():
            wq_copy(s + 6).start()

        ffn_start(s)

        @pl.when(s == 0)
        def _():
            wq_copy(4).wait()

        @pl.when(s + 5 < NP)
        def _():
            wq_copy(s + 5).wait()

        @pl.when(s + 2 < NP)
        def _():
            for cp in w_copies(s + 2, 1 - slot):
                cp.wait()

        for cp in wo_copies(s + 1, slot):
            cp.wait()
        return carry

    with jax.named_scope('pair_loop'):
        lax.fori_loop(0, NP - 1, pair_body, 0)

    last_slot = (NP - 1) % 2

    def last_body(e, carry):
        half = OS // 2
        q_rd = q_s.at[pl.ds(2, 2)]
        order = _LORD
        sc = {order[0]: scores(q_rd, e, order[0])}
        prep_wo(last_slot, pl.multiple_of(e * half, half), half,
                pl.multiple_of((NP - 1) * OS + e * half, half), [sc[order[0]][0]], 3 * TQ)
        pend, zs = [], ()
        for n, i in enumerate(order):
            if n + 1 < NB:
                j = order[n + 1]
                sc[j] = scores(q_rd, e, j, zs if j >= 3 else ())
                zs = ()
                if len(pend) >= _LD and n + 2 < NB and order[n + 2] >= 3:
                    zs = pend.pop(0)(pacer(score_tiles([sc[j][0]], (2 * j + 1) * QT), TQ // 16))
            pend.append(context(values(e, i), H - 2 + e, i, *sc[i], group=_TIEL))
        for f in pend:
            f()
        return carry

    with jax.named_scope('last_loop'):
        lax.fori_loop(0, 2, last_body, 0)

    wr_copy.wait()
    wr = wr_s[...].astype(_F32).reshape(1, M)
    sub8 = lax.broadcasted_iota(_I32, (8, HT), 0)

    def epilogue(g, src, top2, pace=None, write_out=True, dist=_END, valid=None):
        r0 = pl.multiple_of(g * HT, HT)
        best, second = top2
        bits = []
        for n, c in enumerate(range(0, HT, 8)):
            hc = src[pl.ds(c, 8), :]
            z = None if pace is None else pace(n)[:8]
            if n >= dist:
                zc = pltpu.bitcast(bits[n - dist] & 0xFFFF, _U32)
                z = zc if z is None else z | zc
            if z is not None:
                hc = jnp.concatenate([hc[:, :HT] + pltpu.bitcast(z, _F32), hc[:, HT:]], axis=1)
            hnb = _layernorm(hc).astype(_BF16)
            hn_s[pl.ds(r0 + c, 8), :] = hnb
            hn = hnb.astype(_F32)
            if write_out:
                out_s[pl.ds(r0 + c, 8), :] = (hc + hn).astype(_BF16)
            r = jnp.broadcast_to(jnp.sum(hn * wr, axis=1, keepdims=True), (8, HT))
            rb = pltpu.bitcast(_round_bf16(r) + 0.0, _I32)
            bits.append(rb)
            key = ((jnp.where(rb < 0, rb ^ 0x7FFF0000, rb) >> (16 - _IDX_BITS))
                   + ((_KEY_BIAS + S - 1 - c - r0) - sub8))
            key = pltpu.bitcast(key, _F32)
            if valid is not None:
                key = jnp.where(valid, key, 0.0)
            second = jnp.maximum(second, jnp.minimum(best, key))
            best = jnp.maximum(best, key)
        return best, second

    def out_copy(g):
        rows = pl.ds(pl.multiple_of(g * HT, HT), HT)
        return pltpu.make_async_copy(out_s.at[rows, :], out_hbm.at[rows, :], sem_out.at[0])

    KS = 2 * D

    def prod(r0, t, tiles, z=None, zu=0):
        ps = [None] * 7
        for u in _ORDER:
            terms = [(2 * (q1 // 2) + q2 // 2, 2 * (q1 % 2) + q2 % 2, s1 * s2)
                     for q1, s1 in _SA[t] for q2, s2 in _SA[u]]
            fence()
            acc = None
            for k0 in range(0, KO, KS):
                def blk(rb, kb):
                    h0 = (kb * KO + k0) // D
                    return jnp.concatenate(
                        [_ld(ctx_s, h0 + hh, (r0, rb * QT), QT) for hh in range(KS // D)], axis=1)
                if len(terms) == 1:
                    lhs = blk(terms[0][0], terms[0][1])
                else:
                    lhs = _combine([(blk(rb, kb).astype(_F32), sg)
                                    for rb, kb, sg in terms]).astype(_BF16)
                w = wob_s[7 * t + u, pl.ds(k0 // 2, KS // 2), :]
                if z is not None and k0 == 0 and u == _ORDER[zu]:
                    w = tie(w, {0: jnp.concatenate([z, z], axis=1)})
                d = _dot(lhs, _as_bf16(w))
                tiles.append((d, 0, 0))
                acc = d if acc is None else acc + d
            ps[u] = acc
        c11, c12, c21, c22 = _strassen_c(ps)
        return jnp.concatenate([jnp.concatenate([c11, c12], axis=1),
                                jnp.concatenate([c21, c22], axis=1)], axis=0)

    NPC = HT // 8

    def zero_of(v):
        return (pltpu.bitcast(v, _U32) >> 16) >> 16

    def o_body(j, top2):
        r0 = pl.multiple_of(j * TQ, TQ)
        lag = 1 if _OSPLIT else 2

        @pl.when(j > 1)
        def _():
            out_copy(2 * j - lag - 2).start()

        @pl.when(j > lag - 1)
        def _():
            out_copy(2 * j - lag - 1).start()

        rh = pl.multiple_of(j * (TQ // 2), TQ // 2)
        left, right = pl.ds(0, M // 2), pl.ds(M // 2, M // 2)

        def residual(dst, rows0, cols, att):
            hb = (x_raw[pl.ds(rows0, HT), cols].astype(_F32) + att).astype(_BF16)
            h_s[pl.ds(rows0, HT), cols] = hb
            dst[:, cols] = hb.astype(_F32)

        tl = []
        m3 = prod(rh, 2, tl)
        m4 = prod(rh, 3, tl)
        gp = jnp.maximum(2 * j - lag, 0)
        top2 = epilogue(gp, hb_s if _OSPLIT else ht_s, top2,
                        pacer(tl[:len(tl) * _O1 // 16], NPC, 1), valid=j > 0)
        tl = []
        m5 = prod(rh, 4, tl, zero_of(top2[0]), _ZU)
        z = None
        residual(ht_s, r0, right, m3 + m5)
        m1 = prod(rh, 0, tl)
        m7 = prod(rh, 6, tl)
        residual(ht_s, r0, left, m4 - m5 + m1 + m7)
        if not _OSPLIT:
            top2 = epilogue(gp + 1, hb_s, top2, pacer(tl[:len(tl) * _O2 // 16], NPC),
                            valid=j > 0)
            z = zero_of(top2[0])
        tl = []
        m2 = prod(rh, 1, tl, z, _ZU)
        residual(hb_s, r0 + HT, left, m4 + m2)
        m6 = prod(rh, 5, tl)
        residual(hb_s, r0 + HT, right, m3 + m1 - m2 + m6)
        if _OSPLIT:
            top2 = epilogue(2 * j, ht_s, top2, pacer(tl[2:len(tl) * _O2 // 16], NPC))
        return top2

    for n in range(3):
        ffn_wait(n)
    with jax.named_scope('o_loop'):
        top2 = lax.fori_loop(0, NB, o_body, (jnp.zeros((8, HT), _F32),) * 2)
    rest = [(NG - 1, hb_s)] if _OSPLIT else [(NG - 2, ht_s), (NG - 1, hb_s)]
    out_copy(rest[0][0] - 2).start()
    out_copy(rest[0][0] - 1).start()
    for g, src in rest:
        top2 = epilogue(g, src, top2, None, False, NPC)

    best, second = top2
    k1 = jnp.max(best, axis=0, keepdims=True)
    k2 = jnp.max(jnp.where(best == k1, second, best), axis=0, keepdims=True)

    R = _FIX
    row = lax.broadcasted_iota(_I32, (2 * R, HT), 0)
    idx = S - 1 - (pltpu.bitcast(jnp.where(row < R, k1, k2), _I32) & (2 ** _IDX_BITS - 1))
    i1 = jnp.clip(idx[0, 0], 0, S - 1)
    i2 = jnp.clip(idx[R, 0], 0, S - 1)
    b1 = pl.multiple_of(i1 & -R, R)
    b2 = pl.multiple_of(i2 & -R, R)
    tokr = jnp.where(row < R, b1 + row, b2 + row - R)
    cd = (((pltpu.bitcast(jnp.where(tokr == i1, k1, k2), _I32) - _KEY_BIAS) >> _IDX_BITS) << 16)
    score = pltpu.bitcast(jnp.where(cd < 0, cd ^ 0x7FFF0000, cd), _F32)
    gate = _round_bf16(1.0 / (1.0 + jnp.exp(-score)))
    gate = jnp.concatenate([gate] * (M // HT), axis=1)
    tokr = jnp.concatenate([tokr] * (M // HT), axis=1)

    hnsel = jnp.concatenate([hn_s[pl.ds(b1, R), :].astype(_F32),
                             hn_s[pl.ds(b2, R), :].astype(_F32)], axis=0)
    xs = hnsel.astype(_BF16)
    g = _dot(xs, wg_s[...])
    u = _dot(xs, wu_s[...])
    pace = pacer([(mat, 0, c0) for mat in (g, u) for c0 in range(0, F, HT)],
                 len(rest) * HT // 8)
    for k, (gi, src) in enumerate(rest):
        for n, c in enumerate(range(0, HT, 8)):
            rows = pl.ds(gi * HT + c, 8)
            z = pltpu.bitcast(pace(k * HT // 8 + n)[:8], _F32)
            z = jnp.concatenate([z] * (M // HT), axis=1)
            out_s[rows, :] = (src[pl.ds(c, 8), :] + z + hn_s[rows, :].astype(_F32)).astype(_BF16)
        out_copy(gi).start()
    g = _round_bf16(g)
    u = _round_bf16(u)
    g = _round_bf16(g * (1.0 / (1.0 + jnp.exp(-g))))
    act = (g * u).astype(_BF16)
    y = _round_bf16(_dot(act, wd_s[:, pl.ds(0, M)]))
    y = _round_bf16(y * gate)
    upd = jnp.where(jnp.logical_or(tokr == i1, tokr == i2), y, 0.0)
    hsel = jnp.concatenate([h_s[pl.ds(b1, R), :].astype(_F32),
                            h_s[pl.ds(b2, R), :].astype(_F32)], axis=0)
    fixed = hsel + _round_bf16(hnsel + upd)

    pltpu.make_async_copy(out_s, out_hbm, sem_out.at[0]).wait()

    def fix_copy(b0, k):
        return pltpu.make_async_copy(out_s.at[pl.ds(b0, R), :],
                                     out_hbm.at[pl.ds(b0, R), :], sem_out.at[k])

    out_s[pl.ds(b1, R), :] = fixed[:R].astype(_BF16)
    out_s[pl.ds(b2, R), :] = fixed[R:].astype(_BF16)
    fix_copy(b1, 0).start()

    @pl.when(b2 != b1)
    def _():
        fix_copy(b2, 1).start()
        fix_copy(b2, 1).wait()

    fix_copy(b1, 0).wait()


@jax.jit
def pallas_sequential_preLN__compressed_kv_cla__moe_arch_mod__prompt_kernel(
    A_x: jax.Array,
    A_c_kv: jax.Array,
    A_w_q: jax.Array,
    A_w_uk: jax.Array,
    A_w_uv: jax.Array,
    A_w_o: jax.Array,
    B_x: jax.Array,
    B_w_r: jax.Array,
    B_w_gate: jax.Array,
    B_w_up: jax.Array,
    B_w_down: jax.Array,
):
    B, S, M = A_x.shape
    assert B == 1
    DC = A_c_kv.shape[2]
    H, D = A_w_q.shape[1], A_w_q.shape[2]
    F = B_w_gate.shape[1]
    assert A_c_kv.shape[1] == S and S % _TQ == 0 and H % 2 == 0 and S <= 2 ** _IDX_BITS
    NP = H // 2
    NG = S // _HT

    x = A_x.reshape(S, M)
    c = A_c_kv.reshape(S, DC)
    wo = A_w_o.reshape(H * D, M)

    any_spec = pl.BlockSpec(memory_space=pl.ANY)
    def buf(name, lead, rows, cols):
        if name in _U32BUF:
            return pltpu.VMEM((lead, rows // 2, cols), _U32)
        return pltpu.VMEM((lead, rows, cols), _BF16)

    scratch = [
        pltpu.VMEM((S, M), _BF16),
        pltpu.VMEM((S, DC), _BF16),
        pltpu.VMEM((S, M), _F32),
        pltpu.VMEM((7, S // 2, DC // 2), _F32),
        buf('q', 4, S, D),
        buf('k', 2, S, D),
        buf('v', 2, S, D),
        pltpu.VMEM((4, M, D), _U32),
        pltpu.VMEM((2, DC, D), _U32),
        pltpu.VMEM((2, DC, D), _U32),
        pltpu.VMEM((2, 49, M // 8, D), _U32),
        buf('wb', 49, DC // 4, D),
        buf('ctx', H, S, D),
        pltpu.VMEM((2, 4, D // 2, M), _BF16),
        buf('wob', 49, H * D // 4, M // 4),
        pltpu.VMEM((M, F), _BF16),
        pltpu.VMEM((M, F), _BF16),
        pltpu.VMEM((F, M + _WD_PAD), _BF16),
        pltpu.VMEM((_HT, M), _F32),
        pltpu.VMEM((_HT, M), _F32),
        pltpu.VMEM((S, M), _BF16),
        pltpu.VMEM((S, M), _BF16),
        pltpu.VMEM((1024, _HT), _U32),
        pltpu.VMEM((S, M), _BF16),
        pltpu.VMEM((M,), _BF16),
        pltpu.SemaphoreType.DMA((3,)),
        pltpu.SemaphoreType.DMA((3,)),
        pltpu.SemaphoreType.DMA((2, 2)),
        pltpu.SemaphoreType.DMA((4,)),
        pltpu.SemaphoreType.DMA((2, 4)),
        pltpu.SemaphoreType.DMA((4,)),
        pltpu.SemaphoreType.DMA((2,)),
    ]
    out = pl.pallas_call(
        functools.partial(_kernel, S=S, M=M, DC=DC, H=H, D=D, F=F),
        in_specs=[any_spec] * 10,
        out_specs=any_spec,
        out_shape=jax.ShapeDtypeStruct((S, M), _BF16),
        scratch_shapes=scratch,
        compiler_params=pltpu.CompilerParams(vmem_limit_bytes=124 * 1024 * 1024,
                                             disable_bounds_checks=True,
                                             disable_semaphore_checks=True),
        name="fused_mla_mod",
    )(x, c, A_w_q, A_w_uk, A_w_uv, wo, B_w_r, B_w_gate, B_w_up, B_w_down)
    return out.reshape(B, S, M)
```

```python
import functools
import math

import jax
import jax.numpy as jnp
from jax import lax
import jax.experimental.pallas as pl
import jax.experimental.pallas.tpu as pltpu

_F32 = jnp.float32
_BF16 = jnp.bfloat16
_U32 = jnp.uint32
_I32 = jnp.int32

_EPS = 1e-5
_NEG = -1e30
_TQ = 256
_HT = 128
_QT = 64
_IDX_BITS = 13
_KEY_BIAS = 0x30000000
_FIX = 8
_WD_PAD = 128


def _dot(a, b):
    return jnp.dot(a, b, preferred_element_type=_F32)


def _dot_nt(a, b):
    return lax.dot_general(a, b, (((1,), (1,)), ((), ())), preferred_element_type=_F32)


def _as_bf16(u):
    return pltpu.bitcast(u, _BF16)


def _pack(x):
    return pltpu.bitcast(x.astype(_BF16), _U32)


def _rows(r0, n):
    if isinstance(r0, int):
        return pl.ds(r0 // 2, n // 2)
    return pl.ds(pl.multiple_of(r0 // 2, 8), n // 2)


def _ld(ref, lead, r0, n):
    return _as_bf16(ref[lead, _rows(r0, n), :])


def _st(ref, lead, r0, x, cols=slice(None)):
    ref[lead, _rows(r0, x.shape[0]), cols] = _pack(x)


def _round_bf16(x):
    return x.astype(_BF16).astype(_F32)


def _zero_of(v):
    return (pltpu.bitcast(v, _U32) >> 16) >> 16


def _lo_hi(w):
    return (pltpu.bitcast(w << 16, _F32), pltpu.bitcast(w & jnp.uint32(0xFFFF0000), _F32))


def _row_stats(x):
    n = x.shape[-1]
    mean = jnp.sum(x, axis=-1, keepdims=True) * (1.0 / n)
    xc = x - mean
    return mean, xc, jnp.sum(xc * xc, axis=-1, keepdims=True) * (1.0 / n)


def _layernorm(x):
    mean, _, var = _row_stats(x)
    den = _round_bf16(jnp.sqrt(_round_bf16(_round_bf16(var) + _EPS)))
    return (x - _round_bf16(mean)) * pl.reciprocal(den, approx=True)


def _layernorm_scaled(x, scale):
    _, xc, var = _row_stats(x)
    return xc * (lax.rsqrt(var + _EPS) * scale)


_SA = (((0, 1), (3, 1)), ((2, 1), (3, 1)), ((0, 1),), ((3, 1),),
       ((0, 1), (1, 1)), ((2, 1), (0, -1)), ((1, 1), (3, -1)))
_SB = (((0, 1), (3, 1)), ((0, 1),), ((1, 1), (3, -1)), ((2, 1), (0, -1)),
       ((3, 1),), ((0, 1), (1, 1)), ((2, 1), (3, 1)))
_ORDER = (2, 4, 3, 1, 0, 6, 5)


def _combine(terms):
    terms = sorted(terms, key=lambda ts: -ts[1])
    assert terms[0][1] > 0
    acc = terms[0][0]
    for v, sg in terms[1:]:
        acc = acc + v if sg > 0 else acc - v
    return acc


def _operands(table, quad):
    return [_combine([(quad[q], sg) for q, sg in terms]) for terms in table]


def _strassen_c(m):
    m1, m2, m3, m4, m5, m6, m7 = m
    return (m4 - m5 + m1 + m7, m3 + m5, m4 + m2, m3 - m2 + m1 + m6)


def _sub(q1, q2):
    return 2 * (q1 // 2) + q2 // 2, 2 * (q1 % 2) + q2 % 2


def _pacer(tiles, total, free=0):
    def zero(n):
        if n < free:
            return jnp.zeros((16, _HT), _U32)
        mat, r, c = tiles[(n - free) * len(tiles) // (total - free)]
        z = _zero_of(mat[r:r + 8, c:c + _HT])
        return jnp.concatenate([z, z], axis=0)
    return zero


def _score_tiles(mats, spans):
    return [(m, t0 % _TQ, (t0 // _TQ) * 4 * _HT)
            for m, (lo, hi) in zip(mats, spans) for t0 in range(lo, hi, 8)]


def _tie(w, ties):
    parts, at = [], 0
    for r in sorted(ties):
        if r > at:
            parts.append(w[at:r])
        parts.append(w[r:r + 8] | ties[r])
        at = r + 8
    if at < w.shape[0]:
        parts.append(w[at:])
    return parts[0] if len(parts) == 1 else jnp.concatenate(parts, axis=0)


def _add_zero(x, z):
    return jnp.concatenate([x[:, :_HT] + pltpu.bitcast(z, _F32), x[:, _HT:]], axis=1)


def _kernel(x_hbm, c_hbm, wq_hbm, wk_hbm, wv_hbm, wo_hbm, wr_hbm, wg_hbm, wu_hbm, wd_hbm,
            out_hbm,
            x_raw, c_raw, xn_s, ca_s, q_s, k_s, v_s,
            wq_p, wk_p, wv_p, wqb_s, wkvb_s,
            ctx_s, wo_p, wob_s, wg_s, wu_s, wd_s, ht_s, hb_s, h_s, hn_s, junk_s, out_s, wr_s,
            sem_x, sem_c, sem_w, sem_wq, sem_wo, sem_ffn, sem_out,
            *, S, M, DC, H, D, F):
    TQ, HT, QT = _TQ, _HT, _QT
    NB = S // TQ
    NH = NB // 2
    NG = S // HT
    NP = H // 2
    KQ, MQ = DC // 4, M // 4
    KO, NO = H * D // 4, M // 4
    OS = KO // NP
    qscale = (D ** -0.5) * math.log2(math.e)

    wq32 = wq_hbm.bitcast(_U32)
    wk32 = wk_hbm.bitcast(_U32)
    wv32 = wv_hbm.bitcast(_U32)

    def w_copies(pair, slot):
        return (
            pltpu.make_async_copy(wk32.at[:, pair, :], wk_p.at[slot], sem_w.at[2 * slot]),
            pltpu.make_async_copy(wv32.at[:, pair, :], wv_p.at[slot], sem_w.at[2 * slot + 1]),
        )

    def wq_copy(pair):
        return pltpu.make_async_copy(wq32.at[:, pair, :], wq_p.at[pair % 4],
                                     sem_wq.at[pair % 4])

    def wo_copies(t, slot):
        r0 = pl.multiple_of(t * OS, OS)
        return tuple(
            pltpu.make_async_copy(wo_hbm.at[pl.ds(k * KO + r0, OS), :],
                                  wo_p.at[slot, k], sem_wo.at[4 * slot + k])
            for k in range(4))

    def x_copy(n):
        rows = pl.ds(pl.multiple_of(((n + NH) % NB) * TQ, TQ), TQ)
        return pltpu.make_async_copy(x_hbm.at[rows, :], x_raw.at[rows, :], sem_x.at[n % 3])

    def c_copy(i):
        rows = pl.ds(pl.multiple_of(i * 2 * TQ, 2 * TQ), 2 * TQ)
        return pltpu.make_async_copy(c_hbm.at[rows, :], c_raw.at[rows, :], sem_c.at[i % 3])

    ffn = ((wg_hbm, wg_s), (wu_hbm, wu_s), (wd_hbm, wd_s))

    def ffn_start(t):
        for n, (src, dst) in enumerate(ffn):
            rows, cols = src.shape[0] // NP, src.shape[1]
            r0 = pl.multiple_of(t * rows, 16)
            pltpu.make_async_copy(src.at[pl.ds(r0, rows), :],
                                  dst.at[pl.ds(r0, rows), pl.ds(0, cols)],
                                  sem_ffn.at[n]).start()

    def ffn_wait(n):
        src, dst = ffn[n]
        pltpu.make_async_copy(src, dst.at[:, pl.ds(0, src.shape[1])], sem_ffn.at[n]).wait()

    wr_copy = pltpu.make_async_copy(wr_hbm, wr_s, sem_ffn.at[3])

    def out_copy(g):
        rows = pl.ds(pl.multiple_of(g * HT, HT), HT)
        return pltpu.make_async_copy(out_s.at[rows, :], out_hbm.at[rows, :], sem_out.at[0])

    def prep_w4(srcs, dst, kq, rows, pace, sink=None):
        pieces = [(t, r) for t in range(7) for r in rows]
        for n, (t, r) in enumerate(pieces):
            terms = [[] for _ in range(4)]
            for k, (q1, sg) in enumerate(_SB[t]):
                for rb in range(2):
                    w = srcs[q1 % 2][pl.ds((2 * (q1 // 2) + rb) * kq + r, 16), :]
                    if k == 0:
                        w = w | pace(n)
                    lo, hi = _lo_hi(w)
                    terms[2 * rb].append((lo, sg))
                    terms[2 * rb + 1].append((hi, sg))
            z = None
            for u, b in enumerate(_operands(_SB, [_combine(tm) for tm in terms])):
                pk = _pack(b)
                dst[7 * t + u, pl.ds(r // 2, 8), :] = pk
                z = pk if z is None else z | pk
            if sink is not None:
                junk_s[pl.ds(8 * (sink + n), 8), :] = z

    def prep_wq(raw, slot, r, nr, pace, sink=None):
        span = 3 * MQ + nr
        prep_w4((wq_p.at[raw, pl.ds(r, span), :], wq_p.at[raw + 1, pl.ds(r, span), :]),
                wqb_s.at[slot, :, pl.ds(pl.multiple_of(r // 2, 8), nr // 2), :],
                MQ, range(0, nr, 16), pace, sink)

    def prep_wo(slot, src0, nrows, dst0, tiles):
        pieces = [(r, c0, t) for r in range(0, nrows, 16) for c0 in range(0, NO, HT)
                  for t in range(7)]
        pace = _pacer(tiles, len(pieces))
        for n, (r, c0, t) in enumerate(pieces):
            z = pltpu.bitcast(pace(n), _F32)
            sub = []
            for q2 in range(4):
                v = _combine([
                    (wo_p[slot, _sub(q1, q2)[0], pl.ds(src0 + r, 16),
                          pl.ds(_sub(q1, q2)[1] * NO + c0, HT)].astype(_F32), sg)
                    for q1, sg in _SB[t]])
                sub.append(v + z if q2 in (0, 3) else v)
            for u, b in enumerate(_operands(_SB, sub)):
                _st(wob_s, 7 * t + u, dst0 + r, b, pl.ds(c0, HT))

    def fence():
        junk_s[pl.ds(0, 8), :] = jnp.zeros((8, HT), _U32)

    def project4(lhs, w, store, zs=()):
        at = {-(-45 * (k + 1) // len(zs)): z for k, z in enumerate(zs)}
        m, tiles = [None] * 7, []
        for nt, t in enumerate(_ORDER):
            ps = [None] * 7
            for nu, u in enumerate(_ORDER):
                fence()
                a = lhs(t, u)
                wt = w[7 * t + u]
                if 7 * nt + nu in at:
                    wt = _tie(wt, {0: at[7 * nt + nu]})
                ps[u] = _dot(a.astype(_BF16), _as_bf16(wt))
                tiles += [(ps[u], r, 0) for r in range(0, QT, QT * D // (2 * a.shape[1]))]
            m[t] = _strassen_c(ps)
        for q2 in range(4):
            for q1, cblk in enumerate(_strassen_c([mt[q2] for mt in m])):
                store(_sub(q1, q2)[1], _sub(q1, q2)[0] * QT, cblk)
        return tiles

    def project_q(xn, wqb, q, r0):
        def lhs(t, u):
            return _combine([
                (xn[pl.ds(r0 + _sub(q1, q2)[0] * QT, QT), pl.ds(_sub(q1, q2)[1] * MQ, MQ)],
                 s1 * s2) for q1, s1 in _SA[t] for q2, s2 in _SA[u]])
        return project4(lhs, wqb, lambda nb, r, val: _st(q, nb, r0 + r, val))

    def project_kv(j, zs=()):
        def lhs(t, u):
            return _combine([
                (ca_s[t, pl.ds(j * HT + (q2 // 2) * QT, QT), pl.ds((q2 % 2) * KQ, KQ)], sg)
                for q2, sg in _SA[u]])
        return project4(lhs, wkvb_s,
                        lambda nb, r, val: _st((k_s, v_s)[nb // 2], nb % 2, j * TQ + r, val), zs)

    def stage_x(r0, xn, x0, pace):
        done = []
        for n, c in enumerate(range(0, TQ, 8)):
            z = pace(n)[:8]
            if n >= 6:
                z = z | done[n - 6]
            y = _layernorm_scaled(_add_zero(x_raw[pl.ds(r0 + c, 8), :].astype(_F32), z), qscale)
            xn[pl.ds(x0 + c, 8), :] = y
            done.append(_zero_of(y[:, :HT]))

    def stage_c(r0, a0, pace):
        kh = DC // 2
        for n, c in enumerate(range(0, HT, 8)):
            top = c_raw[pl.ds(r0 + c, 8), :].astype(_F32)
            bot = c_raw[pl.ds(r0 + HT + c, 8), :].astype(_F32)
            z = pltpu.bitcast(pace(n)[:8], _F32)
            z = jnp.concatenate([z] * (kh // HT), axis=1)
            quad = (top[:, :kh] + z, top[:, kh:], bot[:, :kh], bot[:, kh:] + z)
            for t, a in enumerate(_operands(_SA, quad)):
                ca_s[t, pl.ds(a0 + c, 8), :] = a

    for cp in w_copies(0, 0) + (c_copy(0), x_copy(0)):
        cp.start()
    ht_s[...] = jnp.zeros((HT, M), _F32)
    hb_s[...] = jnp.zeros((HT, M), _F32)
    for cp in w_copies(0, 0):
        cp.wait()
    c_copy(1).start()
    x_copy(1).start()
    c_copy(0).wait()
    x_copy(0).wait()

    def pro_a(i, carry):
        @pl.when(i + 2 < NH)
        def _():
            c_copy(i + 2).start()

        @pl.when(i + 2 <= NH)
        def _():
            x_copy(i + 2).start()

        @pl.when(jnp.logical_and(i >= 1, i <= 2))
        def _():
            wq_copy(i - 1).start()

        r0 = pl.multiple_of(i * 2 * TQ, 2 * TQ)
        wkv = jnp.concatenate(_lo_hi(wk_p[0]) + _lo_hi(wv_p[0]), axis=1).astype(_BF16)
        kv = _dot(c_raw[pl.ds(r0, 2 * TQ), :], wkv)
        for nb in range(4):
            _st((k_s, v_s)[nb // 2], nb % 2, r0, kv[:, nb * D:(nb + 1) * D])
        tiles = [(kv, r, nb * D) for nb in range(4) for r in range(0, 2 * TQ, 8)]
        nt = len(tiles)
        a0 = pl.multiple_of(i * TQ, TQ)
        stage_c(r0, a0, _pacer(tiles[:nt // 2], HT // 8))
        stage_c(r0 + TQ, a0 + HT, _pacer(tiles[nt // 2:nt * 15 // 16], HT // 8))
        rx = pl.multiple_of((i + NH) * TQ, TQ)
        stage_x(rx, xn_s, rx, _pacer(tiles[:nt * 13 // 16], TQ // 8))

        @pl.when(i + 1 < NH)
        def _():
            c_copy(i + 1).wait()

        x_copy(i + 1).wait()
        return carry

    def pro_b(i, carry):
        @pl.when(i + 2 < NH)
        def _():
            x_copy(NH + i + 2).start()

        @pl.when(i == 2)
        def _():
            for cp in w_copies(1, 1) + wo_copies(0, 0):
                cp.start()

        r0 = pl.multiple_of(i * TQ, TQ)
        xn = xn_s.at[pl.ds(r0, S // 2 + TQ), :]
        kh = M // 2
        lhs = [xn[pl.ds(S // 2, TQ), pl.ds(k0, kh)].astype(_BF16) for k0 in (0, kh)]
        tiles = []
        for nb in range(4):
            d = [_dot(lhs[k], _lo_hi(wq_p[nb // 2, pl.ds(k * kh, kh), :])[nb % 2].astype(_BF16))
                 for k in range(2)]
            _st(q_s, nb, r0 + S // 2, d[0] + d[1])
            tiles += [(dk, r, 0) for dk in d for r in range(0, TQ, 8)]
        stage_x(r0, xn, 0, _pacer(tiles[:len(tiles) * 13 // 16], TQ // 8))
        nr = MQ // (2 * NH)
        npc = 7 * nr // 16
        pace = _pacer(tiles, 3 * npc)
        for k in range(3):
            u = 3 * i + k
            quad = u // (2 * NH)
            prep_wq(2 * quad, quad, pl.multiple_of((u % (2 * NH)) * nr, nr), nr,
                    lambda n, k=k: pace(k * npc + n))

        @pl.when(i == 1)
        def _():
            wq_copy(2).wait()
            wq_copy(3).wait()

        @pl.when(i + 1 < NH)
        def _():
            x_copy(NH + i + 1).wait()

        return carry

    with jax.named_scope('pro_a'):
        lax.fori_loop(0, NH, pro_a, 0)
    wq_copy(0).wait()
    wq_copy(1).wait()
    for cp in (x_copy(NH + 1), wq_copy(2), wq_copy(3)):
        cp.start()
    with jax.named_scope('pro_b'):
        lax.fori_loop(0, NH, pro_b, 0)

    for cp in w_copies(2, 0) + wo_copies(1, 1) + (wq_copy(4), wq_copy(5)):
        cp.start()
    ffn_start(NP - 1)
    wr_copy.start()
    for cp in w_copies(1, 1) + wo_copies(0, 0):
        cp.wait()

    tri = (lax.broadcasted_iota(_I32, (HT, HT), 1)
           <= lax.broadcasted_iota(_I32, (HT, HT), 0))

    def softmax_rows(parts, group):
        s = parts[0] if len(parts) == 1 else jnp.concatenate(parts, axis=1)
        p = jnp.exp2(s - jnp.max(s, axis=1, keepdims=True))
        nt = p.shape[1] // HT
        tiles, acc, grp = [], None, None
        for j in range(nt):
            pj = p[:, j * HT:(j + 1) * HT]
            grp = pj if grp is None else grp + pj
            if j % group == group - 1 or j == nt - 1:
                if j % group > 0:
                    pj = jnp.minimum(pj, grp)
                acc = grp if acc is None else acc + grp
                grp = None
            tiles.append(pj)
        return (tiles[0] if nt == 1 else jnp.concatenate(tiles, axis=1)), acc

    def scores(q, e, i, zs=()):
        Lm = i * TQ + HT
        ties = {(4 + n * (Lm // HT - 4) // len(zs)) * QT + 8 * n: z for n, z in enumerate(zs)}
        keys = _as_bf16(_tie(k_s[e, pl.ds(0, Lm // 2), :], ties))
        s_main = _dot_nt(_ld(q, e, i * TQ, TQ), keys)
        s_last = _dot_nt(_ld(q, e, i * TQ + HT, HT), _ld(k_s, e, Lm, HT))
        return s_main, s_last

    def context(e, head, i, s_main, s_last, group):
        Lm = i * TQ + HT
        v_main, v_last = _ld(v_s, e, 0, Lm), _ld(v_s, e, Lm, HT)
        top = [jnp.where(tri, s_main[:HT, Lm - HT:], _NEG)]
        if Lm > HT:
            top = [s_main[:HT, :Lm - HT]] + top
        p_top, l_top = softmax_rows(top, group)
        p_bot, l_bot = softmax_rows([s_main[HT:], jnp.where(tri, s_last, _NEG)], group)
        o = _dot(jnp.concatenate([p_top, p_bot[:, :Lm]], axis=0).astype(_BF16), v_main)
        o_last = _dot(p_bot[:, Lm:].astype(_BF16), v_last)
        o = jnp.concatenate([o[:HT], o[HT:] + o_last], axis=0)
        acc = jnp.concatenate([l_top, l_bot], axis=0)

        def normalize(pace=None, n0=0):
            z = None
            for n, g in enumerate(range(0, TQ, 16)):
                a = acc[g:g + 16]
                if pace is not None:
                    a = a + pltpu.bitcast(pace(n0 + n), _F32)
                linv = jnp.broadcast_to(
                    pl.reciprocal(jnp.sum(a, axis=1, keepdims=True), approx=True), (16, D))
                ctx_s.at[head][_rows(i * TQ + g, 16), :] = _pack(o[g:g + 16] * linv)
                bits = pltpu.bitcast(linv, _U32)
                bits = bits[:8] | bits[8:]
                z = bits if z is None else z | bits
            return _zero_of(z)
        return normalize

    def pair_body(s, carry):
        slot = (s + 1) % 2
        odd = s % 2
        wo0 = pl.multiple_of(s * OS, OS)
        q_rd = q_s.at[pl.ds(2 * odd, 2)]
        q_wr = q_s.at[:, pl.ds(pl.multiple_of(odd * (S // 4), S // 4), S // 4), :]
        xn = xn_s.at[pl.ds(pl.multiple_of(odd * (S // 2), S // 2), S // 2), :]
        quad = (s + 1) // 2
        wqb = wqb_s.at[quad % 2]
        pend, sc = {}, {}

        def norm(i, tiles):
            pace = _pacer(tiles, TQ // 8)
            return [f(pace, k * (TQ // 16)) for k, f in enumerate(pend.pop(i))]

        def qk(i, nrm=None):
            sa = scores(q_rd, 0, i)
            zs = ()
            if nrm is not None:
                zs = norm(nrm, _score_tiles([sa[0]], [(0, (2 * i + 1) * QT * 7 // 8)]))
            sc[i] = (sa, scores(q_rd, 1, i, zs))
            return [sa[0], sc[i][1][0]]

        def pv(i):
            pend[i] = [context(e, 2 * s + e, i, *sc[i][e], 4) for e in range(2)]

        kv = project_kv
        for i in range(7, 3, -1):
            mats = qk(i, i + 2 if i + 2 < NB else None)
            if i == 7:
                prep_w4((wk_p.at[slot], wv_p.at[slot]), wkvb_s, KQ, range(0, KQ, 16),
                        _pacer(_score_tiles(mats, [(0, 768), (128, 896)]), 7 * KQ // 16), 1)
            elif i == 6:
                prep_wq(2 * (jnp.minimum(quad + 1, NP // 2 - 1) % 2), (quad + 1) % 2,
                        pl.multiple_of((1 - odd) * (MQ // 2), MQ // 2), MQ // 2,
                        _pacer(_score_tiles(mats, [(0, 672)] * 2), 7 * MQ // 32), 64)
            else:
                r = (5 - i) * (OS // 2)
                prep_wo(1 - slot, r, OS // 2, wo0 + r, _score_tiles(mats, [(0, 576)] * 2))
            project_q(xn, wqb, q_wr, (i - NH) * TQ)
            pv(i)
        qk(3, 5)
        qk(0)
        kv(7)
        pv(3)
        pv(0)
        z = norm(4, kv(6))
        qk(2)
        qk(1)
        kv(5, z)
        pv(2)
        pv(1)
        t = kv(4)
        for j, i in ((3, 3), (2, 0), (1, 2), (0, 1)):
            t = kv(j, norm(i, t))

        @pl.when(s + 3 < NP)
        def _():
            for cp in w_copies(s + 3, slot):
                cp.start()

        @pl.when(s + 2 < NP)
        def _():
            for cp in wo_copies(s + 2, 1 - slot):
                cp.start()

        @pl.when(s + 6 < NP)
        def _():
            wq_copy(s + 6).start()

        ffn_start(s)

        @pl.when(s == 0)
        def _():
            wq_copy(4).wait()

        @pl.when(s + 5 < NP)
        def _():
            wq_copy(s + 5).wait()

        @pl.when(s + 2 < NP)
        def _():
            for cp in w_copies(s + 2, 1 - slot):
                cp.wait()

        for cp in wo_copies(s + 1, slot):
            cp.wait()
        return carry

    with jax.named_scope('pair_loop'):
        lax.fori_loop(0, NP - 1, pair_body, 0)

    def last_body(e, carry):
        half = OS // 2
        q_rd = q_s.at[pl.ds(2, 2)]
        nxt = scores(q_rd, e, NB - 1)
        prep_wo((NP - 1) % 2, pl.multiple_of(e * half, half), half,
                pl.multiple_of((NP - 1) * OS + e * half, half),
                _score_tiles([nxt[0]], [(0, 768)]))
        pend = []
        for i in range(NB - 1, -1, -1):
            cur = nxt
            if i > 0:
                nxt = scores(q_rd, e, i - 1)
            pend.append(context(e, H - 2 + e, i, *cur, 3))
        for f in pend:
            f()
        return carry

    with jax.named_scope('last_loop'):
        lax.fori_loop(0, 2, last_body, 0)

    wr_copy.wait()
    wr = wr_s[...].astype(_F32).reshape(1, M)
    sub8 = lax.broadcasted_iota(_I32, (8, HT), 0)
    NPC = HT // 8

    def epilogue(g, src, top2, pace=None, valid=None):
        r0 = pl.multiple_of(g * HT, HT)
        best, second = top2
        bits = []
        for n, c in enumerate(range(0, HT, 8)):
            hc = src[pl.ds(c, 8), :]
            if pace is not None:
                z = pace(n)[:8]
                if n >= 3:
                    z = z | pltpu.bitcast(bits[n - 3] & 0xFFFF, _U32)
                hc = _add_zero(hc, z)
            hnb = _layernorm(hc).astype(_BF16)
            hn_s[pl.ds(r0 + c, 8), :] = hnb
            hn = hnb.astype(_F32)
            if pace is not None:
                out_s[pl.ds(r0 + c, 8), :] = (hc + hn).astype(_BF16)
            r = jnp.broadcast_to(jnp.sum(hn * wr, axis=1, keepdims=True), (8, HT))
            rb = pltpu.bitcast(_round_bf16(r) + 0.0, _I32)
            bits.append(rb)
            key = ((jnp.where(rb < 0, rb ^ 0x7FFF0000, rb) >> (16 - _IDX_BITS))
                   + ((_KEY_BIAS + S - 1 - c - r0) - sub8))
            key = pltpu.bitcast(key, _F32)
            if valid is not None:
                key = jnp.where(valid, key, 0.0)
            second = jnp.maximum(second, jnp.minimum(best, key))
            best = jnp.maximum(best, key)
        return best, second

    def prod(rh, t, tiles, z=None):
        KS = 2 * D
        ps = [None] * 7
        for u in _ORDER:
            terms = [_sub(q1, q2) + (s1 * s2,) for q1, s1 in _SA[t] for q2, s2 in _SA[u]]
            fence()
            acc = None
            for k0 in range(0, KO, KS):
                def blk(rb, kb):
                    h0 = (kb * KO + k0) // D
                    return jnp.concatenate(
                        [_as_bf16(ctx_s[h0 + hh, pl.ds(rh + rb * QT // 2, QT // 2), :])
                         for hh in range(KS // D)], axis=1)
                if len(terms) == 1:
                    lhs = blk(terms[0][0], terms[0][1])
                else:
                    lhs = _combine([(blk(rb, kb).astype(_F32), sg)
                                    for rb, kb, sg in terms]).astype(_BF16)
                w = wob_s[7 * t + u, _rows(k0, KS), :]
                if z is not None and k0 == 0 and u == _ORDER[1]:
                    w = _tie(w, {0: jnp.concatenate([z, z], axis=1)})
                d = _dot(lhs, _as_bf16(w))
                tiles.append((d, 0, 0))
                acc = d if acc is None else acc + d
            ps[u] = acc
        c11, c12, c21, c22 = _strassen_c(ps)
        return jnp.concatenate([jnp.concatenate([c11, c12], axis=1),
                                jnp.concatenate([c21, c22], axis=1)], axis=0)

    def o_body(j, top2):
        r0 = pl.multiple_of(j * TQ, TQ)

        @pl.when(j > 1)
        def _():
            out_copy(2 * j - 4).start()

        @pl.when(j > 1)
        def _():
            out_copy(2 * j - 3).start()

        rh = pl.multiple_of(j * (TQ // 2), TQ // 2)
        left, right = pl.ds(0, M // 2), pl.ds(M // 2, M // 2)

        def residual(dst, rows0, cols, att):
            hb = (x_raw[pl.ds(rows0, HT), cols].astype(_F32) + att).astype(_BF16)
            h_s[pl.ds(rows0, HT), cols] = hb
            dst[:, cols] = hb.astype(_F32)

        gp = jnp.maximum(2 * j - 2, 0)
        tl = []
        m3 = prod(rh, 2, tl)
        m4 = prod(rh, 3, tl)
        top2 = epilogue(gp, ht_s, top2, _pacer(tl[:len(tl) * 7 // 8], NPC, 1), j > 0)
        tl = []
        m5 = prod(rh, 4, tl, _zero_of(top2[0]))
        residual(ht_s, r0, right, m3 + m5)
        m1 = prod(rh, 0, tl)
        m7 = prod(rh, 6, tl)
        residual(ht_s, r0, left, m4 - m5 + m1 + m7)
        top2 = epilogue(gp + 1, hb_s, top2, _pacer(tl[:len(tl) * 7 // 8], NPC), j > 0)
        m2 = prod(rh, 1, tl, _zero_of(top2[0]))
        residual(hb_s, r0 + HT, left, m4 + m2)
        m6 = prod(rh, 5, tl)
        residual(hb_s, r0 + HT, right, m3 + m1 - m2 + m6)
        return top2

    for n in range(3):
        ffn_wait(n)
    with jax.named_scope('o_loop'):
        top2 = lax.fori_loop(0, NB, o_body, (jnp.zeros((8, HT), _F32),) * 2)
    rest = ((NG - 2, ht_s), (NG - 1, hb_s))
    out_copy(NG - 4).start()
    out_copy(NG - 3).start()
    for g, src in rest:
        top2 = epilogue(g, src, top2)

    best, second = top2
    k1 = jnp.max(best, axis=0, keepdims=True)
    k2 = jnp.max(jnp.where(best == k1, second, best), axis=0, keepdims=True)

    R = _FIX
    row = lax.broadcasted_iota(_I32, (2 * R, HT), 0)
    idx = S - 1 - (pltpu.bitcast(jnp.where(row < R, k1, k2), _I32) & (2 ** _IDX_BITS - 1))
    i1 = jnp.clip(idx[0, 0], 0, S - 1)
    i2 = jnp.clip(idx[R, 0], 0, S - 1)
    b1 = pl.multiple_of(i1 & -R, R)
    b2 = pl.multiple_of(i2 & -R, R)
    tokr = jnp.where(row < R, b1 + row, b2 + row - R)
    cd = (((pltpu.bitcast(jnp.where(tokr == i1, k1, k2), _I32) - _KEY_BIAS) >> _IDX_BITS) << 16)
    score = pltpu.bitcast(jnp.where(cd < 0, cd ^ 0x7FFF0000, cd), _F32)
    gate = _round_bf16(1.0 / (1.0 + jnp.exp(-score)))
    gate = jnp.concatenate([gate] * (M // HT), axis=1)
    tokr = jnp.concatenate([tokr] * (M // HT), axis=1)

    hnsel = jnp.concatenate([hn_s[pl.ds(b1, R), :].astype(_F32),
                             hn_s[pl.ds(b2, R), :].astype(_F32)], axis=0)
    xs = hnsel.astype(_BF16)
    g = _dot(xs, wg_s[...])
    u = _dot(xs, wu_s[...])
    pace = _pacer([(mat, 0, c0) for mat in (g, u) for c0 in range(0, F, HT)], len(rest) * NPC)
    for k, (gi, src) in enumerate(rest):
        for n, c in enumerate(range(0, HT, 8)):
            rows = pl.ds(gi * HT + c, 8)
            z = pltpu.bitcast(pace(k * NPC + n)[:8], _F32)
            z = jnp.concatenate([z] * (M // HT), axis=1)
            out_s[rows, :] = (src[pl.ds(c, 8), :] + z + hn_s[rows, :].astype(_F32)).astype(_BF16)
        out_copy(gi).start()
    g = _round_bf16(g)
    u = _round_bf16(u)
    g = _round_bf16(g * (1.0 / (1.0 + jnp.exp(-g))))
    act = (g * u).astype(_BF16)
    y = _round_bf16(_round_bf16(_dot(act, wd_s[:, pl.ds(0, M)])) * gate)
    upd = jnp.where(jnp.logical_or(tokr == i1, tokr == i2), y, 0.0)
    hsel = jnp.concatenate([h_s[pl.ds(b1, R), :].astype(_F32),
                            h_s[pl.ds(b2, R), :].astype(_F32)], axis=0)
    fixed = hsel + _round_bf16(hnsel + upd)

    pltpu.make_async_copy(out_s, out_hbm, sem_out.at[0]).wait()

    def fix_copy(b0, k):
        return pltpu.make_async_copy(out_s.at[pl.ds(b0, R), :],
                                     out_hbm.at[pl.ds(b0, R), :], sem_out.at[k])

    out_s[pl.ds(b1, R), :] = fixed[:R].astype(_BF16)
    out_s[pl.ds(b2, R), :] = fixed[R:].astype(_BF16)
    fix_copy(b1, 0).start()

    @pl.when(b2 != b1)
    def _():
        fix_copy(b2, 1).start()
        fix_copy(b2, 1).wait()

    fix_copy(b1, 0).wait()


@jax.jit
def pallas_sequential_preLN__compressed_kv_cla__moe_arch_mod__prompt_kernel(
    A_x: jax.Array,
    A_c_kv: jax.Array,
    A_w_q: jax.Array,
    A_w_uk: jax.Array,
    A_w_uv: jax.Array,
    A_w_o: jax.Array,
    B_x: jax.Array,
    B_w_r: jax.Array,
    B_w_gate: jax.Array,
    B_w_up: jax.Array,
    B_w_down: jax.Array,
):
    B, S, M = A_x.shape
    DC = A_c_kv.shape[2]
    H, D = A_w_q.shape[1], A_w_q.shape[2]
    F = B_w_gate.shape[1]
    assert (B, S, M, DC, H, D) == (1, 8 * _TQ, 1024, 512, 32, _HT) and A_c_kv.shape[1] == S
    assert F % (8 * H) == 0 and S <= 2 ** _IDX_BITS

    scratch = [
        pltpu.VMEM((S, M), _BF16),
        pltpu.VMEM((S, DC), _BF16),
        pltpu.VMEM((S, M), _F32),
        pltpu.VMEM((7, S // 2, DC // 2), _F32),
        pltpu.VMEM((4, S // 2, D), _U32),
        pltpu.VMEM((2, S // 2, D), _U32),
        pltpu.VMEM((2, S // 2, D), _U32),
        pltpu.VMEM((4, M, D), _U32),
        pltpu.VMEM((2, DC, D), _U32),
        pltpu.VMEM((2, DC, D), _U32),
        pltpu.VMEM((2, 49, M // 8, D), _U32),
        pltpu.VMEM((49, DC // 8, D), _U32),
        pltpu.VMEM((H, S // 2, D), _U32),
        pltpu.VMEM((2, 4, D // 2, M), _BF16),
        pltpu.VMEM((49, H * D // 8, M // 4), _U32),
        pltpu.VMEM((M, F), _BF16),
        pltpu.VMEM((M, F), _BF16),
        pltpu.VMEM((F, M + _WD_PAD), _BF16),
        pltpu.VMEM((_HT, M), _F32),
        pltpu.VMEM((_HT, M), _F32),
        pltpu.VMEM((S, M), _BF16),
        pltpu.VMEM((S, M), _BF16),
        pltpu.VMEM((1024, _HT), _U32),
        pltpu.VMEM((S, M), _BF16),
        pltpu.VMEM((M,), _BF16),
        pltpu.SemaphoreType.DMA((3,)),
        pltpu.SemaphoreType.DMA((3,)),
        pltpu.SemaphoreType.DMA((4,)),
        pltpu.SemaphoreType.DMA((4,)),
        pltpu.SemaphoreType.DMA((8,)),
        pltpu.SemaphoreType.DMA((4,)),
        pltpu.SemaphoreType.DMA((2,)),
    ]
    any_spec = pl.BlockSpec(memory_space=pl.ANY)
    out = pl.pallas_call(
        functools.partial(_kernel, S=S, M=M, DC=DC, H=H, D=D, F=F),
        in_specs=[any_spec] * 10,
        out_specs=any_spec,
        out_shape=jax.ShapeDtypeStruct((S, M), _BF16),
        scratch_shapes=scratch,
        compiler_params=pltpu.CompilerParams(vmem_limit_bytes=124 * 1024 * 1024,
                                             disable_bounds_checks=True,
                                             disable_semaphore_checks=True),
        name="fused_mla_mod",
    )(A_x.reshape(S, M), A_c_kv.reshape(S, DC), A_w_q, A_w_uk, A_w_uv,
      A_w_o.reshape(H * D, M), B_w_r, B_w_gate, B_w_up, B_w_down)
    return out.reshape(B, S, M)
```

```python
import functools
import math

import jax
import jax.numpy as jnp
from jax import lax
import jax.experimental.pallas as pl
import jax.experimental.pallas.tpu as pltpu

_F32 = jnp.float32
_BF16 = jnp.bfloat16
_U32 = jnp.uint32
_I32 = jnp.int32

_EPS = 1e-5
_NEG = -1e30
_TQ = 256
_HT = 128
_QT = 64
_IDX_BITS = 13
_KEY_BIAS = 0x30000000
_FIX = 8
_WD_PAD = 128


def _dot(a, b):
    return jnp.dot(a, b, preferred_element_type=_F32)


def _dot_nt(a, b):
    return lax.dot_general(a, b, (((1,), (1,)), ((), ())), preferred_element_type=_F32)


def _as_bf16(u):
    return pltpu.bitcast(u, _BF16)


def _pack(x):
    return pltpu.bitcast(x.astype(_BF16), _U32)


def _rows(r0, n):
    if isinstance(r0, int):
        return pl.ds(r0 // 2, n // 2)
    return pl.ds(pl.multiple_of(r0 // 2, 8), n // 2)


def _ld(ref, lead, r0, n):
    return _as_bf16(ref[lead, _rows(r0, n), :])


def _st(ref, lead, r0, x, cols=slice(None)):
    ref[lead, _rows(r0, x.shape[0]), cols] = _pack(x)


def _round_bf16(x):
    return x.astype(_BF16).astype(_F32)


def _zero_of(v):
    return (pltpu.bitcast(v, _U32) >> 16) >> 16


def _lo_hi(w):
    return (pltpu.bitcast(w << 16, _F32), pltpu.bitcast(w & jnp.uint32(0xFFFF0000), _F32))


def _row_stats(x):
    n = x.shape[-1]
    mean = jnp.sum(x, axis=-1, keepdims=True) * (1.0 / n)
    xc = x - mean
    return mean, xc, jnp.sum(xc * xc, axis=-1, keepdims=True) * (1.0 / n)


def _layernorm(x):
    mean, _, var = _row_stats(x)
    den = _round_bf16(jnp.sqrt(_round_bf16(_round_bf16(var) + _EPS)))
    return (x - _round_bf16(mean)) * pl.reciprocal(den, approx=True)


def _layernorm_scaled(x, scale):
    _, xc, var = _row_stats(x)
    return xc * (lax.rsqrt(var + _EPS) * scale)


_SA = (((0, 1), (3, 1)), ((2, 1), (3, 1)), ((0, 1),), ((3, 1),),
       ((0, 1), (1, 1)), ((2, 1), (0, -1)), ((1, 1), (3, -1)))
_SB = (((0, 1), (3, 1)), ((0, 1),), ((1, 1), (3, -1)), ((2, 1), (0, -1)),
       ((3, 1),), ((0, 1), (1, 1)), ((2, 1), (3, 1)))
_ORDER = (2, 4, 3, 1, 0, 6, 5)


def _combine(terms):
    terms = sorted(terms, key=lambda ts: -ts[1])
    assert terms[0][1] > 0
    acc = terms[0][0]
    for v, sg in terms[1:]:
        acc = acc + v if sg > 0 else acc - v
    return acc


def _operands(table, quad):
    return [_combine([(quad[q], sg) for q, sg in terms]) for terms in table]


def _strassen_c(m):
    m1, m2, m3, m4, m5, m6, m7 = m
    return (m4 - m5 + m1 + m7, m3 + m5, m4 + m2, m3 - m2 + m1 + m6)


def _sub(q1, q2):
    return 2 * (q1 // 2) + q2 // 2, 2 * (q1 % 2) + q2 % 2


def _pacer(tiles, total, free=0):
    def zero(n):
        if n < free:
            return jnp.zeros((16, _HT), _U32)
        mat, r, c = tiles[(n - free) * len(tiles) // (total - free)]
        z = _zero_of(mat[r:r + 8, c:c + _HT])
        return jnp.concatenate([z, z], axis=0)
    return zero


def _score_tiles(mats, spans):
    return [(m, t0 % _TQ, (t0 // _TQ) * 4 * _HT)
            for m, (lo, hi) in zip(mats, spans) for t0 in range(lo, hi, 8)]


def _tie(w, ties):
    parts, at = [], 0
    for r in sorted(ties):
        if r > at:
            parts.append(w[at:r])
        parts.append(w[r:r + 8] | ties[r])
        at = r + 8
    if at < w.shape[0]:
        parts.append(w[at:])
    return parts[0] if len(parts) == 1 else jnp.concatenate(parts, axis=0)


def _add_zero(x, z):
    return jnp.concatenate([x[:, :_HT] + pltpu.bitcast(z, _F32), x[:, _HT:]], axis=1)


def _kernel(x_hbm, c_hbm, wq_hbm, wk_hbm, wv_hbm, wo_hbm, wr_hbm, wg_hbm, wu_hbm, wd_hbm,
            out_hbm,
            x_raw, c_raw, xn_s, ca_s, q_s, k_s, v_s,
            wq_p, wk_p, wv_p, wqb_s, wkvb_s,
            ctx_s, wo_p, wob_s, wg_s, wu_s, wd_s, ht_s, hb_s, h_s, hn_s, junk_s, out_s, wr_s,
            sem_x, sem_c, sem_w, sem_wq, sem_wo, sem_ffn, sem_out,
            *, S, M, DC, H, D, F):
    TQ, HT, QT = _TQ, _HT, _QT
    NB = S // TQ
    NH = NB // 2
    NG = S // HT
    NP = H // 2
    KQ, MQ = DC // 4, M // 4
    KO, NO = H * D // 4, M // 4
    OS = KO // NP
    qscale = (D ** -0.5) * math.log2(math.e)

    wq32 = wq_hbm.bitcast(_U32)
    wk32 = wk_hbm.bitcast(_U32)
    wv32 = wv_hbm.bitcast(_U32)

    def w_copies(pair, slot):
        return (
            pltpu.make_async_copy(wk32.at[:, pair, :], wk_p.at[slot], sem_w.at[2 * slot]),
            pltpu.make_async_copy(wv32.at[:, pair, :], wv_p.at[slot], sem_w.at[2 * slot + 1]),
        )

    def wq_copy(pair):
        return pltpu.make_async_copy(wq32.at[:, pair, :], wq_p.at[pair % 4],
                                     sem_wq.at[pair % 4])

    def wo_copies(t, slot):
        r0 = pl.multiple_of(t * OS, OS)
        return tuple(
            pltpu.make_async_copy(wo_hbm.at[pl.ds(k * KO + r0, OS), :],
                                  wo_p.at[slot, k], sem_wo.at[4 * slot + k])
            for k in range(4))

    def x_copy(n):
        rows = pl.ds(pl.multiple_of(((n + NH) % NB) * TQ, TQ), TQ)
        return pltpu.make_async_copy(x_hbm.at[rows, :], x_raw.at[rows, :], sem_x.at[n])

    def c_copy(i):
        rows = pl.ds(pl.multiple_of(i * 2 * TQ, 2 * TQ), 2 * TQ)
        return pltpu.make_async_copy(c_hbm.at[rows, :], c_raw.at[rows, :], sem_c.at[i])

    ffn = ((wg_hbm, wg_s), (wu_hbm, wu_s), (wd_hbm, wd_s))

    def ffn_start(t):
        for n, (src, dst) in enumerate(ffn):
            rows, cols = src.shape[0] // NP, src.shape[1]
            r0 = pl.multiple_of(t * rows, 16)
            pltpu.make_async_copy(src.at[pl.ds(r0, rows), :],
                                  dst.at[pl.ds(r0, rows), pl.ds(0, cols)],
                                  sem_ffn.at[n]).start()

    def ffn_wait(n):
        src, dst = ffn[n]
        pltpu.make_async_copy(src, dst.at[:, pl.ds(0, src.shape[1])], sem_ffn.at[n]).wait()

    wr_copy = pltpu.make_async_copy(wr_hbm, wr_s, sem_ffn.at[3])

    def out_copy(g):
        rows = pl.ds(pl.multiple_of(g * HT, HT), HT)
        return pltpu.make_async_copy(out_s.at[rows, :], out_hbm.at[rows, :], sem_out.at[0])

    def prep_w4(srcs, dst, kq, rows, pace, sink=None):
        pieces = [(t, r) for t in range(7) for r in rows]
        for n, (t, r) in enumerate(pieces):
            terms = [[] for _ in range(4)]
            for k, (q1, sg) in enumerate(_SB[t]):
                for rb in range(2):
                    w = srcs[q1 % 2][pl.ds((2 * (q1 // 2) + rb) * kq + r, 16), :]
                    if k == 0:
                        w = w | pace(n)
                    lo, hi = _lo_hi(w)
                    terms[2 * rb].append((lo, sg))
                    terms[2 * rb + 1].append((hi, sg))
            z = None
            for u, b in enumerate(_operands(_SB, [_combine(tm) for tm in terms])):
                pk = _pack(b)
                dst[7 * t + u, pl.ds(r // 2, 8), :] = pk
                z = pk if z is None else z | pk
            if sink is not None:
                junk_s[pl.ds(8 * (sink + n), 8), :] = z

    def prep_wq(raw, slot, r, nr, pace, sink=None):
        span = 3 * MQ + nr
        prep_w4((wq_p.at[raw, pl.ds(r, span), :], wq_p.at[raw + 1, pl.ds(r, span), :]),
                wqb_s.at[slot, :, pl.ds(pl.multiple_of(r // 2, 8), nr // 2), :],
                MQ, range(0, nr, 16), pace, sink)

    def prep_wo(slot, src0, nrows, dst0, tiles):
        pieces = [(r, c0, t) for r in range(0, nrows, 16) for c0 in range(0, NO, HT)
                  for t in range(7)]
        pace = _pacer(tiles, len(pieces))
        for n, (r, c0, t) in enumerate(pieces):
            z = pltpu.bitcast(pace(n), _F32)
            sub = []
            for q2 in range(4):
                v = _combine([
                    (wo_p[slot, _sub(q1, q2)[0], pl.ds(src0 + r, 16),
                          pl.ds(_sub(q1, q2)[1] * NO + c0, HT)].astype(_F32), sg)
                    for q1, sg in _SB[t]])
                sub.append(v + z if q2 in (0, 3) else v)
            for u, b in enumerate(_operands(_SB, sub)):
                _st(wob_s, 7 * t + u, dst0 + r, b, pl.ds(c0, HT))

    def fence():
        junk_s[pl.ds(0, 8), :] = jnp.zeros((8, HT), _U32)

    def project4(lhs, w, store, zs=()):
        at = {-(-45 * (k + 1) // len(zs)): z for k, z in enumerate(zs)}
        m, tiles = [None] * 7, []
        for nt, t in enumerate(_ORDER):
            ps = [None] * 7
            for nu, u in enumerate(_ORDER):
                fence()
                a = lhs(t, u)
                wt = w[7 * t + u]
                if 7 * nt + nu in at:
                    wt = _tie(wt, {0: at[7 * nt + nu]})
                ps[u] = _dot(a.astype(_BF16), _as_bf16(wt))
                tiles += [(ps[u], r, 0) for r in range(0, QT, QT * D // (2 * a.shape[1]))]
            m[t] = _strassen_c(ps)
        for q2 in range(4):
            for q1, cblk in enumerate(_strassen_c([mt[q2] for mt in m])):
                store(_sub(q1, q2)[1], _sub(q1, q2)[0] * QT, cblk)
        return tiles

    def project_q(xn, wqb, q, r0):
        def lhs(t, u):
            return _combine([
                (xn[pl.ds(r0 + _sub(q1, q2)[0] * QT, QT), pl.ds(_sub(q1, q2)[1] * MQ, MQ)],
                 s1 * s2) for q1, s1 in _SA[t] for q2, s2 in _SA[u]])
        return project4(lhs, wqb, lambda nb, r, val: _st(q, nb, r0 + r, val))

    def project_kv(j, zs=()):
        def lhs(t, u):
            return _combine([
                (ca_s[t, pl.ds(j * HT + (q2 // 2) * QT, QT), pl.ds((q2 % 2) * KQ, KQ)], sg)
                for q2, sg in _SA[u]])
        return project4(lhs, wkvb_s,
                        lambda nb, r, val: _st((k_s, v_s)[nb // 2], nb % 2, j * TQ + r, val), zs)

    def stage_x(r0, xn, x0, pace):
        done = []
        for n, c in enumerate(range(0, TQ, 8)):
            z = pace(n)[:8]
            if n >= 6:
                z = z | done[n - 6]
            y = _layernorm_scaled(_add_zero(x_raw[pl.ds(r0 + c, 8), :].astype(_F32), z), qscale)
            xn[pl.ds(x0 + c, 8), :] = y
            done.append(_zero_of(y[:, :HT]))

    def stage_c(r0, a0, pace):
        kh = DC // 2
        for n, c in enumerate(range(0, HT, 8)):
            top = c_raw[pl.ds(r0 + c, 8), :].astype(_F32)
            bot = c_raw[pl.ds(r0 + HT + c, 8), :].astype(_F32)
            z = pltpu.bitcast(pace(n)[:8], _F32)
            z = jnp.concatenate([z] * (kh // HT), axis=1)
            quad = (top[:, :kh] + z, top[:, kh:], bot[:, :kh], bot[:, kh:] + z)
            for t, a in enumerate(_operands(_SA, quad)):
                ca_s[t, pl.ds(a0 + c, 8), :] = a

    def issue(n, carry):
        @pl.when(n == 0)
        def _():
            for cp in w_copies(0, 0):
                cp.start()

        @pl.when(n < NH)
        def _():
            c_copy(n).start()

        @pl.when(jnp.logical_or(n == NH, n == NH + 2))
        def _():
            wq_copy(n - NH).start()
            wq_copy(n - NH + 1).start()

        @pl.when(n < NB)
        def _():
            x_copy(n).start()

        @pl.when(n == NB)
        def _():
            for cp in w_copies(1, 1) + wo_copies(0, 0):
                cp.start()
        return carry

    lax.fori_loop(0, NB + 1, issue, 0)
    ht_s[...] = jnp.zeros((HT, M), _F32)
    hb_s[...] = jnp.zeros((HT, M), _F32)
    for cp in w_copies(0, 0) + (c_copy(0), x_copy(0)):
        cp.wait()

    def pro_a(i, carry):
        r0 = pl.multiple_of(i * 2 * TQ, 2 * TQ)
        wkv = jnp.concatenate(_lo_hi(wk_p[0]) + _lo_hi(wv_p[0]), axis=1).astype(_BF16)
        kv = _dot(c_raw[pl.ds(r0, 2 * TQ), :], wkv)
        for nb in range(4):
            _st((k_s, v_s)[nb // 2], nb % 2, r0, kv[:, nb * D:(nb + 1) * D])
        tiles = [(kv, r, nb * D) for nb in range(4) for r in range(0, 2 * TQ, 8)]
        nt = len(tiles)
        a0 = pl.multiple_of(i * TQ, TQ)
        stage_c(r0, a0, _pacer(tiles[:nt // 2], HT // 8))
        stage_c(r0 + TQ, a0 + HT, _pacer(tiles[nt // 2:nt * 15 // 16], HT // 8))
        rx = pl.multiple_of((i + NH) * TQ, TQ)
        stage_x(rx, xn_s, rx, _pacer(tiles[:nt * 13 // 16], TQ // 8))

        @pl.when(i + 1 < NH)
        def _():
            c_copy(i + 1).wait()

        x_copy(i + 1).wait()
        return carry

    def pro_b(i, carry):
        r0 = pl.multiple_of(i * TQ, TQ)
        xn = xn_s.at[pl.ds(r0, S // 2 + TQ), :]
        kh = M // 2
        lhs = [xn[pl.ds(S // 2, TQ), pl.ds(k0, kh)].astype(_BF16) for k0 in (0, kh)]
        tiles = []
        for nb in range(4):
            d = [_dot(lhs[k], _lo_hi(wq_p[nb // 2, pl.ds(k * kh, kh), :])[nb % 2].astype(_BF16))
                 for k in range(2)]
            _st(q_s, nb, r0 + S // 2, d[0] + d[1])
            tiles += [(dk, r, 0) for dk in d for r in range(0, TQ, 8)]
        stage_x(r0, xn, 0, _pacer(tiles[:len(tiles) * 13 // 16], TQ // 8))
        nr = MQ // (2 * NH)
        npc = 7 * nr // 16
        pace = _pacer(tiles, 3 * npc)
        for k in range(3):
            u = 3 * i + k
            quad = u // (2 * NH)
            prep_wq(2 * quad, quad, pl.multiple_of((u % (2 * NH)) * nr, nr), nr,
                    lambda n, k=k: pace(k * npc + n))

        @pl.when(i == 1)
        def _():
            wq_copy(2).wait()
            wq_copy(3).wait()

        @pl.when(i + 1 < NH)
        def _():
            x_copy(NH + i + 1).wait()

        return carry

    with jax.named_scope('pro_a'):
        lax.fori_loop(0, NH, pro_a, 0)
    wq_copy(0).wait()
    wq_copy(1).wait()
    with jax.named_scope('pro_b'):
        lax.fori_loop(0, NH, pro_b, 0)

    for cp in w_copies(2, 0) + wo_copies(1, 1) + (wq_copy(4), wq_copy(5)):
        cp.start()
    ffn_start(NP - 1)
    wr_copy.start()
    for cp in w_copies(1, 1) + wo_copies(0, 0):
        cp.wait()

    tri = (lax.broadcasted_iota(_I32, (HT, HT), 1)
           <= lax.broadcasted_iota(_I32, (HT, HT), 0))

    def softmax_rows(parts, group):
        s = parts[0] if len(parts) == 1 else jnp.concatenate(parts, axis=1)
        p = jnp.exp2(s - jnp.max(s, axis=1, keepdims=True))
        nt = p.shape[1] // HT
        tiles, acc, grp = [], None, None
        for j in range(nt):
            pj = p[:, j * HT:(j + 1) * HT]
            grp = pj if grp is None else grp + pj
            if j % group == group - 1 or j == nt - 1:
                if j % group > 0:
                    pj = jnp.minimum(pj, grp)
                acc = grp if acc is None else acc + grp
                grp = None
            tiles.append(pj)
        return (tiles[0] if nt == 1 else jnp.concatenate(tiles, axis=1)), acc

    def scores(q, e, i, zs=()):
        Lm = i * TQ + HT
        ties = {(4 + n * (Lm // HT - 4) // len(zs)) * QT + 8 * n: z for n, z in enumerate(zs)}
        keys = _as_bf16(_tie(k_s[e, pl.ds(0, Lm // 2), :], ties))
        s_main = _dot_nt(_ld(q, e, i * TQ, TQ), keys)
        s_last = _dot_nt(_ld(q, e, i * TQ + HT, HT), _ld(k_s, e, Lm, HT))
        return s_main, s_last

    def context(e, head, i, s_main, s_last, group):
        Lm = i * TQ + HT
        v_main, v_last = _ld(v_s, e, 0, Lm), _ld(v_s, e, Lm, HT)
        top = [jnp.where(tri, s_main[:HT, Lm - HT:], _NEG)]
        if Lm > HT:
            top = [s_main[:HT, :Lm - HT]] + top
        p_top, l_top = softmax_rows(top, group)
        p_bot, l_bot = softmax_rows([s_main[HT:], jnp.where(tri, s_last, _NEG)], group)
        o = _dot(jnp.concatenate([p_top, p_bot[:, :Lm]], axis=0).astype(_BF16), v_main)
        o_last = _dot(p_bot[:, Lm:].astype(_BF16), v_last)
        o = jnp.concatenate([o[:HT], o[HT:] + o_last], axis=0)
        acc = jnp.concatenate([l_top, l_bot], axis=0)

        def normalize(pace=None, n0=0):
            z = None
            for n, g in enumerate(range(0, TQ, 16)):
                a = acc[g:g + 16]
                if pace is not None:
                    a = a + pltpu.bitcast(pace(n0 + n), _F32)
                linv = jnp.broadcast_to(
                    pl.reciprocal(jnp.sum(a, axis=1, keepdims=True), approx=True), (16, D))
                ctx_s.at[head][_rows(i * TQ + g, 16), :] = _pack(o[g:g + 16] * linv)
                bits = pltpu.bitcast(linv, _U32)
                bits = bits[:8] | bits[8:]
                z = bits if z is None else z | bits
            return _zero_of(z)
        return normalize

    def pair_body(s, carry):
        slot = (s + 1) % 2
        odd = s % 2
        wo0 = pl.multiple_of(s * OS, OS)
        q_rd = q_s.at[pl.ds(2 * odd, 2)]
        q_wr = q_s.at[:, pl.ds(pl.multiple_of(odd * (S // 4), S // 4), S // 4), :]
        xn = xn_s.at[pl.ds(pl.multiple_of(odd * (S // 2), S // 2), S // 2), :]
        quad = (s + 1) // 2
        wqb = wqb_s.at[quad % 2]
        pend, sc = {}, {}

        def norm(i, tiles):
            pace = _pacer(tiles, TQ // 8)
            return [f(pace, k * (TQ // 16)) for k, f in enumerate(pend.pop(i))]

        def qk(i, nrm=None):
            sa = scores(q_rd, 0, i)
            zs = ()
            if nrm is not None:
                zs = norm(nrm, _score_tiles([sa[0]], [(0, (2 * i + 1) * QT * 7 // 8)]))
            sc[i] = (sa, scores(q_rd, 1, i, zs))
            return [sa[0], sc[i][1][0]]

        def pv(i):
            pend[i] = [context(e, 2 * s + e, i, *sc[i][e], 4) for e in range(2)]

        kv = project_kv
        for i in range(7, 3, -1):
            mats = qk(i, i + 2 if i + 2 < NB else None)
            if i == 7:
                prep_w4((wk_p.at[slot], wv_p.at[slot]), wkvb_s, KQ, range(0, KQ, 16),
                        _pacer(_score_tiles(mats, [(0, 768), (128, 896)]), 7 * KQ // 16), 1)
            elif i == 6:
                prep_wq(2 * (jnp.minimum(quad + 1, NP // 2 - 1) % 2), (quad + 1) % 2,
                        pl.multiple_of((1 - odd) * (MQ // 2), MQ // 2), MQ // 2,
                        _pacer(_score_tiles(mats, [(0, 672)] * 2), 7 * MQ // 32), 64)
            else:
                r = (5 - i) * (OS // 2)
                prep_wo(1 - slot, r, OS // 2, wo0 + r, _score_tiles(mats, [(0, 576)] * 2))
            project_q(xn, wqb, q_wr, (i - NH) * TQ)
            pv(i)
        qk(3, 5)
        qk(0)
        kv(7)
        pv(3)
        pv(0)
        z = norm(4, kv(6))
        qk(2)
        qk(1)
        kv(5, z)
        pv(2)
        pv(1)
        t = kv(4)
        for j, i in ((3, 3), (2, 0), (1, 2), (0, 1)):
            t = kv(j, norm(i, t))

        @pl.when(s + 3 < NP)
        def _():
            for cp in w_copies(s + 3, slot):
                cp.start()

        @pl.when(s + 2 < NP)
        def _():
            for cp in wo_copies(s + 2, 1 - slot):
                cp.start()

        @pl.when(s + 6 < NP)
        def _():
            wq_copy(s + 6).start()

        ffn_start(s)

        @pl.when(s == 0)
        def _():
            wq_copy(4).wait()

        @pl.when(s + 5 < NP)
        def _():
            wq_copy(s + 5).wait()

        @pl.when(s + 2 < NP)
        def _():
            for cp in w_copies(s + 2, 1 - slot):
                cp.wait()

        for cp in wo_copies(s + 1, slot):
            cp.wait()
        return carry

    with jax.named_scope('pair_loop'):
        lax.fori_loop(0, NP - 1, pair_body, 0)

    def last_body(e, carry):
        half = OS // 2
        q_rd = q_s.at[pl.ds(2, 2)]
        nxt = scores(q_rd, e, NB - 1)
        prep_wo((NP - 1) % 2, pl.multiple_of(e * half, half), half,
                pl.multiple_of((NP - 1) * OS + e * half, half),
                _score_tiles([nxt[0]], [(0, 768)]))
        pend = []
        for i in range(NB - 1, -1, -1):
            cur = nxt
            if i > 0:
                nxt = scores(q_rd, e, i - 1)
            pend.append(context(e, H - 2 + e, i, *cur, 3))
        for f in pend:
            f()
        return carry

    with jax.named_scope('last_loop'):
        lax.fori_loop(0, 2, last_body, 0)

    wr_copy.wait()
    wr = wr_s[...].astype(_F32).reshape(1, M)
    sub8 = lax.broadcasted_iota(_I32, (8, HT), 0)
    NPC = HT // 8

    def epilogue(g, src, top2, pace=None, valid=None):
        r0 = pl.multiple_of(g * HT, HT)
        best, second = top2
        bits = []
        for n, c in enumerate(range(0, HT, 8)):
            hc = src[pl.ds(c, 8), :]
            if pace is not None:
                z = pace(n)[:8]
                if n >= 3:
                    z = z | pltpu.bitcast(bits[n - 3] & 0xFFFF, _U32)
                hc = _add_zero(hc, z)
            hnb = _layernorm(hc).astype(_BF16)
            hn_s[pl.ds(r0 + c, 8), :] = hnb
            hn = hnb.astype(_F32)
            if pace is not None:
                out_s[pl.ds(r0 + c, 8), :] = (hc + hn).astype(_BF16)
            r = jnp.broadcast_to(jnp.sum(hn * wr, axis=1, keepdims=True), (8, HT))
            rb = pltpu.bitcast(_round_bf16(r) + 0.0, _I32)
            bits.append(rb)
            key = ((jnp.where(rb < 0, rb ^ 0x7FFF0000, rb) >> (16 - _IDX_BITS))
                   + ((_KEY_BIAS + S - 1 - c - r0) - sub8))
            key = pltpu.bitcast(key, _F32)
            if valid is not None:
                key = jnp.where(valid, key, 0.0)
            second = jnp.maximum(second, jnp.minimum(best, key))
            best = jnp.maximum(best, key)
        return best, second

    def prod(rh, t, tiles, z=None):
        KS = 2 * D
        ps = [None] * 7
        for u in _ORDER:
            terms = [_sub(q1, q2) + (s1 * s2,) for q1, s1 in _SA[t] for q2, s2 in _SA[u]]
            fence()
            acc = None
            for k0 in range(0, KO, KS):
                def blk(rb, kb):
                    h0 = (kb * KO + k0) // D
                    return jnp.concatenate(
                        [_as_bf16(ctx_s[h0 + hh, pl.ds(rh + rb * QT // 2, QT // 2), :])
                         for hh in range(KS // D)], axis=1)
                if len(terms) == 1:
                    lhs = blk(terms[0][0], terms[0][1])
                else:
                    lhs = _combine([(blk(rb, kb).astype(_F32), sg)
                                    for rb, kb, sg in terms]).astype(_BF16)
                w = wob_s[7 * t + u, _rows(k0, KS), :]
                if z is not None and k0 == 0 and u == _ORDER[1]:
                    w = _tie(w, {0: jnp.concatenate([z, z], axis=1)})
                d = _dot(lhs, _as_bf16(w))
                tiles.append((d, 0, 0))
                acc = d if acc is None else acc + d
            ps[u] = acc
        c11, c12, c21, c22 = _strassen_c(ps)
        return jnp.concatenate([jnp.concatenate([c11, c12], axis=1),
                                jnp.concatenate([c21, c22], axis=1)], axis=0)

    def o_body(j, top2):
        r0 = pl.multiple_of(j * TQ, TQ)

        @pl.when(j > 1)
        def _():
            out_copy(2 * j - 4).start()

        @pl.when(j > 1)
        def _():
            out_copy(2 * j - 3).start()

        rh = pl.multiple_of(j * (TQ // 2), TQ // 2)
        left, right = pl.ds(0, M // 2), pl.ds(M // 2, M // 2)

        def residual(dst, rows0, cols, att):
            hb = (x_raw[pl.ds(rows0, HT), cols].astype(_F32) + att).astype(_BF16)
            h_s[pl.ds(rows0, HT), cols] = hb
            dst[:, cols] = hb.astype(_F32)

        gp = jnp.maximum(2 * j - 2, 0)
        tl = []
        m3 = prod(rh, 2, tl)
        m4 = prod(rh, 3, tl)
        top2 = epilogue(gp, ht_s, top2, _pacer(tl[:len(tl) * 7 // 8], NPC, 1), j > 0)
        tl = []
        m5 = prod(rh, 4, tl, _zero_of(top2[0]))
        residual(ht_s, r0, right, m3 + m5)
        m1 = prod(rh, 0, tl)
        m7 = prod(rh, 6, tl)
        residual(ht_s, r0, left, m4 - m5 + m1 + m7)
        top2 = epilogue(gp + 1, hb_s, top2, _pacer(tl[:len(tl) * 7 // 8], NPC), j > 0)
        m2 = prod(rh, 1, tl, _zero_of(top2[0]))
        residual(hb_s, r0 + HT, left, m4 + m2)
        m6 = prod(rh, 5, tl)
        residual(hb_s, r0 + HT, right, m3 + m1 - m2 + m6)
        return top2

    for n in range(3):
        ffn_wait(n)
    with jax.named_scope('o_loop'):
        top2 = lax.fori_loop(0, NB, o_body, (jnp.zeros((8, HT), _F32),) * 2)
    rest = ((NG - 2, ht_s), (NG - 1, hb_s))
    out_copy(NG - 4).start()
    out_copy(NG - 3).start()
    for g, src in rest:
        top2 = epilogue(g, src, top2)

    best, second = top2
    k1 = jnp.max(best, axis=0, keepdims=True)
    k2 = jnp.max(jnp.where(best == k1, second, best), axis=0, keepdims=True)

    R = _FIX
    row = lax.broadcasted_iota(_I32, (2 * R, HT), 0)
    idx = S - 1 - (pltpu.bitcast(jnp.where(row < R, k1, k2), _I32) & (2 ** _IDX_BITS - 1))
    i1 = jnp.clip(idx[0, 0], 0, S - 1)
    i2 = jnp.clip(idx[R, 0], 0, S - 1)
    b1 = pl.multiple_of(i1 & -R, R)
    b2 = pl.multiple_of(i2 & -R, R)
    tokr = jnp.where(row < R, b1 + row, b2 + row - R)
    cd = (((pltpu.bitcast(jnp.where(tokr == i1, k1, k2), _I32) - _KEY_BIAS) >> _IDX_BITS) << 16)
    score = pltpu.bitcast(jnp.where(cd < 0, cd ^ 0x7FFF0000, cd), _F32)
    gate = _round_bf16(1.0 / (1.0 + jnp.exp(-score)))
    gate = jnp.concatenate([gate] * (M // HT), axis=1)
    tokr = jnp.concatenate([tokr] * (M // HT), axis=1)

    hnsel = jnp.concatenate([hn_s[pl.ds(b1, R), :].astype(_F32),
                             hn_s[pl.ds(b2, R), :].astype(_F32)], axis=0)
    xs = hnsel.astype(_BF16)
    g = _dot(xs, wg_s[...])
    u = _dot(xs, wu_s[...])
    pace = _pacer([(mat, 0, c0) for mat in (g, u) for c0 in range(0, F, HT)], len(rest) * NPC)
    for k, (gi, src) in enumerate(rest):
        for n, c in enumerate(range(0, HT, 8)):
            rows = pl.ds(gi * HT + c, 8)
            z = pltpu.bitcast(pace(k * NPC + n)[:8], _F32)
            z = jnp.concatenate([z] * (M // HT), axis=1)
            out_s[rows, :] = (src[pl.ds(c, 8), :] + z + hn_s[rows, :].astype(_F32)).astype(_BF16)
        out_copy(gi).start()
    g = _round_bf16(g)
    u = _round_bf16(u)
    g = _round_bf16(g * (1.0 / (1.0 + jnp.exp(-g))))
    act = (g * u).astype(_BF16)
    y = _round_bf16(_round_bf16(_dot(act, wd_s[:, pl.ds(0, M)])) * gate)
    upd = jnp.where(jnp.logical_or(tokr == i1, tokr == i2), y, 0.0)
    hsel = jnp.concatenate([h_s[pl.ds(b1, R), :].astype(_F32),
                            h_s[pl.ds(b2, R), :].astype(_F32)], axis=0)
    fixed = hsel + _round_bf16(hnsel + upd)

    pltpu.make_async_copy(out_s, out_hbm, sem_out.at[0]).wait()

    def fix_copy(b0, k):
        return pltpu.make_async_copy(out_s.at[pl.ds(b0, R), :],
                                     out_hbm.at[pl.ds(b0, R), :], sem_out.at[k])

    out_s[pl.ds(b1, R), :] = fixed[:R].astype(_BF16)
    out_s[pl.ds(b2, R), :] = fixed[R:].astype(_BF16)
    fix_copy(b1, 0).start()

    @pl.when(b2 != b1)
    def _():
        fix_copy(b2, 1).start()
        fix_copy(b2, 1).wait()

    fix_copy(b1, 0).wait()


@jax.jit
def pallas_sequential_preLN__compressed_kv_cla__moe_arch_mod__prompt_kernel(
    A_x: jax.Array,
    A_c_kv: jax.Array,
    A_w_q: jax.Array,
    A_w_uk: jax.Array,
    A_w_uv: jax.Array,
    A_w_o: jax.Array,
    B_x: jax.Array,
    B_w_r: jax.Array,
    B_w_gate: jax.Array,
    B_w_up: jax.Array,
    B_w_down: jax.Array,
):
    B, S, M = A_x.shape
    DC = A_c_kv.shape[2]
    H, D = A_w_q.shape[1], A_w_q.shape[2]
    F = B_w_gate.shape[1]
    assert (B, S, M, DC, H, D) == (1, 8 * _TQ, 1024, 512, 32, _HT) and A_c_kv.shape[1] == S
    assert F % (8 * H) == 0 and S <= 2 ** _IDX_BITS

    scratch = [
        pltpu.VMEM((S, M), _BF16),
        pltpu.VMEM((S, DC), _BF16),
        pltpu.VMEM((S, M), _F32),
        pltpu.VMEM((7, S // 2, DC // 2), _F32),
        pltpu.VMEM((4, S // 2, D), _U32),
        pltpu.VMEM((2, S // 2, D), _U32),
        pltpu.VMEM((2, S // 2, D), _U32),
        pltpu.VMEM((4, M, D), _U32),
        pltpu.VMEM((2, DC, D), _U32),
        pltpu.VMEM((2, DC, D), _U32),
        pltpu.VMEM((2, 49, M // 8, D), _U32),
        pltpu.VMEM((49, DC // 8, D), _U32),
        pltpu.VMEM((H, S // 2, D), _U32),
        pltpu.VMEM((2, 4, D // 2, M), _BF16),
        pltpu.VMEM((49, H * D // 8, M // 4), _U32),
        pltpu.VMEM((M, F), _BF16),
        pltpu.VMEM((M, F), _BF16),
        pltpu.VMEM((F, M + _WD_PAD), _BF16),
        pltpu.VMEM((_HT, M), _F32),
        pltpu.VMEM((_HT, M), _F32),
        pltpu.VMEM((S, M), _BF16),
        pltpu.VMEM((S, M), _BF16),
        pltpu.VMEM((1024, _HT), _U32),
        pltpu.VMEM((S, M), _BF16),
        pltpu.VMEM((M,), _BF16),
        pltpu.SemaphoreType.DMA((S // _TQ,)),
        pltpu.SemaphoreType.DMA((S // _TQ // 2,)),
        pltpu.SemaphoreType.DMA((4,)),
        pltpu.SemaphoreType.DMA((4,)),
        pltpu.SemaphoreType.DMA((8,)),
        pltpu.SemaphoreType.DMA((4,)),
        pltpu.SemaphoreType.DMA((2,)),
    ]
    any_spec = pl.BlockSpec(memory_space=pl.ANY)
    out = pl.pallas_call(
        functools.partial(_kernel, S=S, M=M, DC=DC, H=H, D=D, F=F),
        in_specs=[any_spec] * 10,
        out_specs=any_spec,
        out_shape=jax.ShapeDtypeStruct((S, M), _BF16),
        scratch_shapes=scratch,
        compiler_params=pltpu.CompilerParams(vmem_limit_bytes=124 * 1024 * 1024,
                                             disable_bounds_checks=True,
                                             disable_semaphore_checks=True),
        name="fused_mla_mod",
    )(A_x.reshape(S, M), A_c_kv.reshape(S, DC), A_w_q, A_w_uk, A_w_uv,
      A_w_o.reshape(H * D, M), B_w_r, B_w_gate, B_w_up, B_w_down)
    return out.reshape(B, S, M)
```

```python
import functools
import math

import jax
import jax.numpy as jnp
from jax import lax
import jax.experimental.pallas as pl
import jax.experimental.pallas.tpu as pltpu

_F32 = jnp.float32
_BF16 = jnp.bfloat16
_U32 = jnp.uint32
_I32 = jnp.int32

_EPS = 1e-5
_NEG = -1e30
_TQ = 256
_HT = 128
_QT = 64
_IDX_BITS = 13
_KEY_BIAS = 0x30000000
_FIX = 8
_WD_PAD = 128


def _dot(a, b):
    return jnp.dot(a, b, preferred_element_type=_F32)


def _dot_nt(a, b):
    return lax.dot_general(a, b, (((1,), (1,)), ((), ())), preferred_element_type=_F32)


def _as_bf16(u):
    return pltpu.bitcast(u, _BF16)


def _pack(x):
    return pltpu.bitcast(x.astype(_BF16), _U32)


def _rows(r0, n):
    if isinstance(r0, int):
        return pl.ds(r0 // 2, n // 2)
    return pl.ds(pl.multiple_of(r0 // 2, 8), n // 2)


def _ld(ref, lead, r0, n):
    return _as_bf16(ref[lead, _rows(r0, n), :])


def _st(ref, lead, r0, x, cols=slice(None)):
    ref[lead, _rows(r0, x.shape[0]), cols] = _pack(x)


def _round_bf16(x):
    return x.astype(_BF16).astype(_F32)


def _zero_of(v):
    return (pltpu.bitcast(v, _U32) >> 16) >> 16


def _lo_hi(w):
    return (pltpu.bitcast(w << 16, _F32), pltpu.bitcast(w & jnp.uint32(0xFFFF0000), _F32))


def _row_stats(x):
    n = x.shape[-1]
    mean = jnp.sum(x, axis=-1, keepdims=True) * (1.0 / n)
    xc = x - mean
    return mean, xc, jnp.sum(xc * xc, axis=-1, keepdims=True) * (1.0 / n)


def _layernorm(x):
    mean, _, var = _row_stats(x)
    den = _round_bf16(jnp.sqrt(_round_bf16(_round_bf16(var) + _EPS)))
    return (x - _round_bf16(mean)) * pl.reciprocal(den, approx=True)


def _layernorm_scaled(x, scale):
    _, xc, var = _row_stats(x)
    return xc * (lax.rsqrt(var + _EPS) * scale)


_SA = (((0, 1), (3, 1)), ((2, 1), (3, 1)), ((0, 1),), ((3, 1),),
       ((0, 1), (1, 1)), ((2, 1), (0, -1)), ((1, 1), (3, -1)))
_SB = (((0, 1), (3, 1)), ((0, 1),), ((1, 1), (3, -1)), ((2, 1), (0, -1)),
       ((3, 1),), ((0, 1), (1, 1)), ((2, 1), (3, 1)))
_ORDER = (2, 4, 3, 1, 0, 6, 5)


def _combine(terms):
    terms = sorted(terms, key=lambda ts: -ts[1])
    assert terms[0][1] > 0
    acc = terms[0][0]
    for v, sg in terms[1:]:
        acc = acc + v if sg > 0 else acc - v
    return acc


def _operands(table, quad):
    return [_combine([(quad[q], sg) for q, sg in terms]) for terms in table]


def _strassen_c(m):
    m1, m2, m3, m4, m5, m6, m7 = m
    return (m4 - m5 + m1 + m7, m3 + m5, m4 + m2, m3 - m2 + m1 + m6)


def _sub(q1, q2):
    return 2 * (q1 // 2) + q2 // 2, 2 * (q1 % 2) + q2 % 2


def _pacer(tiles, total, free=0):
    def zero(n):
        if n < free:
            return jnp.zeros((16, _HT), _U32)
        mat, r, c = tiles[(n - free) * len(tiles) // (total - free)]
        z = _zero_of(mat[r:r + 8, c:c + _HT])
        return jnp.concatenate([z, z], axis=0)
    return zero


def _score_tiles(mats, spans):
    return [(m, t0 % _TQ, (t0 // _TQ) * 4 * _HT)
            for m, (lo, hi) in zip(mats, spans) for t0 in range(lo, hi, 8)]


def _tie(w, ties):
    parts, at = [], 0
    for r in sorted(ties):
        if r > at:
            parts.append(w[at:r])
        parts.append(w[r:r + 8] | ties[r])
        at = r + 8
    if at < w.shape[0]:
        parts.append(w[at:])
    return parts[0] if len(parts) == 1 else jnp.concatenate(parts, axis=0)


def _add_zero(x, z):
    return jnp.concatenate([x[:, :_HT] + pltpu.bitcast(z, _F32), x[:, _HT:]], axis=1)


def _kernel(x_hbm, c_hbm, wq_hbm, wk_hbm, wv_hbm, wo_hbm, wr_hbm, wg_hbm, wu_hbm, wd_hbm,
            out_hbm,
            x_raw, c_raw, xn_s, ca_s, q_s, k_s, v_s,
            wq_p, wkv_p, wqb_s, wkvb_s,
            ctx_s, wo_p, wob_s, wg_s, wu_s, wd_s, ht_s, hb_s, h_s, hn_s, junk_s, out_s, wr_s,
            sem_x, sem_c, sem_w, sem_wq, sem_wo, sem_ffn, sem_out,
            *, S, M, DC, H, D, F):
    TQ, HT, QT = _TQ, _HT, _QT
    NB = S // TQ
    NH = NB // 2
    NG = S // HT
    NP = H // 2
    KQ, MQ = DC // 4, M // 4
    KO, NO = H * D // 4, M // 4
    OS = KO // NP
    qscale = (D ** -0.5) * math.log2(math.e)

    wq32 = wq_hbm.bitcast(_U32)
    wk32 = wk_hbm.bitcast(_U32)
    wv32 = wv_hbm.bitcast(_U32)

    def w_start(pair, slot):
        for k, src in enumerate((wk32, wv32)):
            pltpu.make_async_copy(src.at[:, pair, :], wkv_p.at[slot, k], sem_w.at[slot]).start()

    def w_wait(slot):
        pltpu.make_async_copy(wkv_p.at[slot], wkv_p.at[slot], sem_w.at[slot]).wait()

    def wq_copy(pair):
        return pltpu.make_async_copy(wq32.at[:, pair, :], wq_p.at[pair & 3],
                                     sem_wq.at[pair & 3])

    def wo_start(t, slot):
        r0 = pl.multiple_of(t * OS, OS)
        for k in range(4):
            pltpu.make_async_copy(wo_hbm.at[pl.ds(k * KO + r0, OS), :],
                                  wo_p.at[slot, k], sem_wo.at[slot]).start()

    def wo_wait(slot):
        pltpu.make_async_copy(wo_p.at[slot], wo_p.at[slot], sem_wo.at[slot]).wait()

    def x_copy(n):
        rows = pl.ds(pl.multiple_of(((n + NH) % NB) * TQ, TQ), TQ)
        return pltpu.make_async_copy(x_hbm.at[rows, :], x_raw.at[rows, :], sem_x.at[n])

    def c_copy(i):
        rows = pl.ds(pl.multiple_of(i * 2 * TQ, 2 * TQ), 2 * TQ)
        return pltpu.make_async_copy(c_hbm.at[rows, :], c_raw.at[rows, :], sem_c.at[i])

    ffn = ((wg_hbm, wg_s), (wu_hbm, wu_s), (wd_hbm, wd_s))

    def ffn_start(t):
        for n, (src, dst) in enumerate(ffn):
            rows, cols = src.shape[0] // NP, src.shape[1]
            r0 = pl.multiple_of(t * rows, 16)
            pltpu.make_async_copy(src.at[pl.ds(r0, rows), :],
                                  dst.at[pl.ds(r0, rows), pl.ds(0, cols)],
                                  sem_ffn.at[n]).start()

    def ffn_wait(n):
        src, dst = ffn[n]
        pltpu.make_async_copy(src, dst.at[:, pl.ds(0, src.shape[1])], sem_ffn.at[n]).wait()

    wr_copy = pltpu.make_async_copy(wr_hbm, wr_s, sem_ffn.at[3])

    def out_copy(g):
        rows = pl.ds(pl.multiple_of(g * HT, HT), HT)
        return pltpu.make_async_copy(out_s.at[rows, :], out_hbm.at[rows, :], sem_out.at[0])

    def prep_w4(srcs, dst, kq, rows, pace, sink=None):
        pieces = [(t, r) for t in range(7) for r in rows]
        for n, (t, r) in enumerate(pieces):
            terms = [[] for _ in range(4)]
            for k, (q1, sg) in enumerate(_SB[t]):
                for rb in range(2):
                    w = srcs[q1 % 2][pl.ds((2 * (q1 // 2) + rb) * kq + r, 16), :]
                    if k == 0:
                        w = w | pace(n)
                    lo, hi = _lo_hi(w)
                    terms[2 * rb].append((lo, sg))
                    terms[2 * rb + 1].append((hi, sg))
            z = None
            for u, b in enumerate(_operands(_SB, [_combine(tm) for tm in terms])):
                pk = _pack(b)
                dst[7 * t + u, pl.ds(r // 2, 8), :] = pk
                z = pk if z is None else z | pk
            if sink is not None:
                junk_s[pl.ds(8 * (sink + n), 8), :] = z

    def prep_wq(raw, slot, r, nr, pace, sink=None):
        span = 3 * MQ + nr
        prep_w4((wq_p.at[raw, pl.ds(r, span), :], wq_p.at[raw + 1, pl.ds(r, span), :]),
                wqb_s.at[slot, :, pl.ds(pl.multiple_of(r // 2, 8), nr // 2), :],
                MQ, range(0, nr, 16), pace, sink)

    def prep_wo(slot, src0, nrows, dst0, tiles):
        pieces = [(r, c0, t) for r in range(0, nrows, 16) for c0 in range(0, NO, HT)
                  for t in range(7)]
        pace = _pacer(tiles, len(pieces))
        for n, (r, c0, t) in enumerate(pieces):
            z = pltpu.bitcast(pace(n), _F32)
            sub = []
            for q2 in range(4):
                v = _combine([
                    (wo_p[slot, _sub(q1, q2)[0], pl.ds(src0 + r, 16),
                          pl.ds(_sub(q1, q2)[1] * NO + c0, HT)].astype(_F32), sg)
                    for q1, sg in _SB[t]])
                sub.append(v + z if q2 in (0, 3) else v)
            for u, b in enumerate(_operands(_SB, sub)):
                _st(wob_s, 7 * t + u, dst0 + r, b, pl.ds(c0, HT))

    def fence():
        junk_s[pl.ds(0, 8), :] = jnp.zeros((8, HT), _U32)

    def project4(lhs, w, store, zs=()):
        at = {-(-45 * (k + 1) // len(zs)): z for k, z in enumerate(zs)}
        m, tiles = [None] * 7, []
        for nt, t in enumerate(_ORDER):
            ps = [None] * 7
            for nu, u in enumerate(_ORDER):
                fence()
                a = lhs(t, u)
                wt = w[7 * t + u]
                if 7 * nt + nu in at:
                    wt = _tie(wt, {0: at[7 * nt + nu]})
                ps[u] = _dot(a.astype(_BF16), _as_bf16(wt))
                tiles += [(ps[u], r, 0) for r in range(0, QT, QT * D // (2 * a.shape[1]))]
            m[t] = _strassen_c(ps)
        for q2 in range(4):
            for q1, cblk in enumerate(_strassen_c([mt[q2] for mt in m])):
                store(_sub(q1, q2)[1], _sub(q1, q2)[0] * QT, cblk)
        return tiles

    def project_q(xn, wqb, q, r0):
        def lhs(t, u):
            return _combine([
                (xn[pl.ds(r0 + _sub(q1, q2)[0] * QT, QT), pl.ds(_sub(q1, q2)[1] * MQ, MQ)],
                 s1 * s2) for q1, s1 in _SA[t] for q2, s2 in _SA[u]])
        return project4(lhs, wqb, lambda nb, r, val: _st(q, nb, r0 + r, val))

    def project_kv(j, zs=()):
        def lhs(t, u):
            return _combine([
                (ca_s[t, pl.ds(j * HT + (q2 // 2) * QT, QT), pl.ds((q2 % 2) * KQ, KQ)], sg)
                for q2, sg in _SA[u]])
        return project4(lhs, wkvb_s,
                        lambda nb, r, val: _st((k_s, v_s)[nb // 2], nb % 2, j * TQ + r, val), zs)

    def stage_x(r0, xn, x0, pace):
        done = []
        for n, c in enumerate(range(0, TQ, 8)):
            z = pace(n)[:8]
            if n >= 6:
                z = z | done[n - 6]
            y = _layernorm_scaled(_add_zero(x_raw[pl.ds(r0 + c, 8), :].astype(_F32), z), qscale)
            xn[pl.ds(x0 + c, 8), :] = y
            done.append(_zero_of(y[:, :HT]))

    def stage_c(r0, a0, pace):
        kh = DC // 2
        for n, c in enumerate(range(0, HT, 8)):
            top = c_raw[pl.ds(r0 + c, 8), :].astype(_F32)
            bot = c_raw[pl.ds(r0 + HT + c, 8), :].astype(_F32)
            z = pltpu.bitcast(pace(n)[:8], _F32)
            z = jnp.concatenate([z] * (kh // HT), axis=1)
            quad = (top[:, :kh] + z, top[:, kh:], bot[:, :kh], bot[:, kh:] + z)
            for t, a in enumerate(_operands(_SA, quad)):
                ca_s[t, pl.ds(a0 + c, 8), :] = a

    def issue(n, carry):
        @pl.when(n == 0)
        def _():
            w_start(0, 0)

        @pl.when(n < NH)
        def _():
            c_copy(n).start()

        @pl.when(jnp.logical_or(n == NH, n == NH + 2))
        def _():
            wq_copy(n - NH).start()
            wq_copy(n - NH + 1).start()

        @pl.when(n < NB)
        def _():
            x_copy(n).start()

        @pl.when(n == NB)
        def _():
            w_start(1, 1)
            wo_start(0, 0)
        return carry

    lax.fori_loop(0, NB + 1, issue, 0)
    ht_s[...] = jnp.zeros((HT, M), _F32)
    hb_s[...] = jnp.zeros((HT, M), _F32)
    w_wait(0)
    c_copy(0).wait()
    x_copy(0).wait()

    def pro_a(i, carry):
        r0 = pl.multiple_of(i * 2 * TQ, 2 * TQ)
        wkv = jnp.concatenate(_lo_hi(wkv_p[0, 0]) + _lo_hi(wkv_p[0, 1]), axis=1).astype(_BF16)
        kv = _dot(c_raw[pl.ds(r0, 2 * TQ), :], wkv)
        for nb in range(4):
            _st((k_s, v_s)[nb // 2], nb % 2, r0, kv[:, nb * D:(nb + 1) * D])
        tiles = [(kv, r, nb * D) for nb in range(4) for r in range(0, 2 * TQ, 8)]
        nt = len(tiles)
        a0 = pl.multiple_of(i * TQ, TQ)
        stage_c(r0, a0, _pacer(tiles[:nt // 2], HT // 8))
        stage_c(r0 + TQ, a0 + HT, _pacer(tiles[nt // 2:nt * 15 // 16], HT // 8))
        rx = pl.multiple_of((i + NH) * TQ, TQ)
        stage_x(rx, xn_s, rx, _pacer(tiles[:nt * 13 // 16], TQ // 8))

        @pl.when(i + 1 < NH)
        def _():
            c_copy(i + 1).wait()

        x_copy(i + 1).wait()
        return carry

    def pro_b(i, carry):
        r0 = pl.multiple_of(i * TQ, TQ)
        xn = xn_s.at[pl.ds(r0, S // 2 + TQ), :]
        kh = M // 2
        lhs = [xn[pl.ds(S // 2, TQ), pl.ds(k0, kh)].astype(_BF16) for k0 in (0, kh)]
        tiles = []
        for nb in range(4):
            d = [_dot(lhs[k], _lo_hi(wq_p[nb // 2, pl.ds(k * kh, kh), :])[nb % 2].astype(_BF16))
                 for k in range(2)]
            _st(q_s, nb, r0 + S // 2, d[0] + d[1])
            tiles += [(dk, r, 0) for dk in d for r in range(0, TQ, 8)]
        stage_x(r0, xn, 0, _pacer(tiles[:len(tiles) * 13 // 16], TQ // 8))
        nr = MQ // (2 * NH)
        npc = 7 * nr // 16
        pace = _pacer(tiles, 3 * npc)
        for k in range(3):
            u = 3 * i + k
            quad = u // (2 * NH)
            prep_wq(2 * quad, quad, pl.multiple_of((u % (2 * NH)) * nr, nr), nr,
                    lambda n, k=k: pace(k * npc + n))

        @pl.when(i == 1)
        def _():
            wq_copy(2).wait()
            wq_copy(3).wait()

        @pl.when(i + 1 < NH)
        def _():
            x_copy(NH + i + 1).wait()

        return carry

    with jax.named_scope('pro_a'):
        lax.fori_loop(0, NH, pro_a, 0)
    wq_copy(0).wait()
    wq_copy(1).wait()
    with jax.named_scope('pro_b'):
        lax.fori_loop(0, NH, pro_b, 0)

    w_start(2, 0)
    wo_start(1, 1)
    wq_copy(4).start()
    wq_copy(5).start()
    ffn_start(NP - 1)
    wr_copy.start()
    w_wait(1)
    wo_wait(0)

    tri = (lax.broadcasted_iota(_I32, (HT, HT), 1)
           <= lax.broadcasted_iota(_I32, (HT, HT), 0))

    def softmax_rows(parts, group):
        s = parts[0] if len(parts) == 1 else jnp.concatenate(parts, axis=1)
        p = jnp.exp2(s - jnp.max(s, axis=1, keepdims=True))
        nt = p.shape[1] // HT
        tiles, acc, grp = [], None, None
        for j in range(nt):
            pj = p[:, j * HT:(j + 1) * HT]
            grp = pj if grp is None else grp + pj
            if j % group == group - 1 or j == nt - 1:
                if j % group > 0:
                    pj = jnp.minimum(pj, grp)
                acc = grp if acc is None else acc + grp
                grp = None
            tiles.append(pj)
        return (tiles[0] if nt == 1 else jnp.concatenate(tiles, axis=1)), acc

    def scores(q, e, i, zs=()):
        Lm = i * TQ + HT
        ties = {(4 + n * (Lm // HT - 4) // len(zs)) * QT + 8 * n: z for n, z in enumerate(zs)}
        keys = _as_bf16(_tie(k_s[e, pl.ds(0, Lm // 2), :], ties))
        s_main = _dot_nt(_ld(q, e, i * TQ, TQ), keys)
        s_last = _dot_nt(_ld(q, e, i * TQ + HT, HT), _ld(k_s, e, Lm, HT))
        return s_main, s_last

    def context(e, head, i, s_main, s_last, group):
        Lm = i * TQ + HT
        v_main, v_last = _ld(v_s, e, 0, Lm), _ld(v_s, e, Lm, HT)
        top = [jnp.where(tri, s_main[:HT, Lm - HT:], _NEG)]
        if Lm > HT:
            top = [s_main[:HT, :Lm - HT]] + top
        p_top, l_top = softmax_rows(top, group)
        p_bot, l_bot = softmax_rows([s_main[HT:], jnp.where(tri, s_last, _NEG)], group)
        o = _dot(jnp.concatenate([p_top, p_bot[:, :Lm]], axis=0).astype(_BF16), v_main)
        o_last = _dot(p_bot[:, Lm:].astype(_BF16), v_last)
        o = jnp.concatenate([o[:HT], o[HT:] + o_last], axis=0)
        acc = jnp.concatenate([l_top, l_bot], axis=0)

        def normalize(pace=None, n0=0):
            z = None
            for n, g in enumerate(range(0, TQ, 16)):
                a = acc[g:g + 16]
                if pace is not None:
                    a = a + pltpu.bitcast(pace(n0 + n), _F32)
                linv = jnp.broadcast_to(
                    pl.reciprocal(jnp.sum(a, axis=1, keepdims=True), approx=True), (16, D))
                ctx_s.at[head][_rows(i * TQ + g, 16), :] = _pack(o[g:g + 16] * linv)
                bits = pltpu.bitcast(linv, _U32)
                bits = bits[:8] | bits[8:]
                z = bits if z is None else z | bits
            return _zero_of(z)
        return normalize

    def pair_body(s, carry):
        odd = s & 1
        slot = 1 - odd
        wo0 = pl.multiple_of(s * OS, OS)
        q_rd = q_s.at[pl.ds(2 * odd, 2)]
        q_wr = q_s.at[:, pl.ds(pl.multiple_of(odd * (S // 4), S // 4), S // 4), :]
        xn = xn_s.at[pl.ds(pl.multiple_of(odd * (S // 2), S // 2), S // 2), :]
        quad = (s + 1) >> 1
        wqb = wqb_s.at[quad & 1]
        pend, sc = {}, {}

        def norm(i, tiles):
            pace = _pacer(tiles, TQ // 8)
            return [f(pace, k * (TQ // 16)) for k, f in enumerate(pend.pop(i))]

        def qk(i, nrm=None):
            sa = scores(q_rd, 0, i)
            zs = ()
            if nrm is not None:
                zs = norm(nrm, _score_tiles([sa[0]], [(0, (2 * i + 1) * QT * 7 // 8)]))
            sc[i] = (sa, scores(q_rd, 1, i, zs))
            return [sa[0], sc[i][1][0]]

        def pv(i):
            pend[i] = [context(e, 2 * s + e, i, *sc[i][e], 4) for e in range(2)]

        kv = project_kv
        for i in range(7, 3, -1):
            mats = qk(i, i + 2 if i + 2 < NB else None)
            if i == 7:
                prep_w4((wkv_p.at[slot, 0], wkv_p.at[slot, 1]), wkvb_s, KQ, range(0, KQ, 16),
                        _pacer(_score_tiles(mats, [(0, 768), (128, 896)]), 7 * KQ // 16), 1)
            elif i == 6:
                prep_wq(2 * (jnp.minimum(quad + 1, NP // 2 - 1) & 1), (quad + 1) & 1,
                        pl.multiple_of((1 - odd) * (MQ // 2), MQ // 2), MQ // 2,
                        _pacer(_score_tiles(mats, [(0, 672)] * 2), 7 * MQ // 32), 64)
            else:
                r = (5 - i) * (OS // 2)
                prep_wo(odd, r, OS // 2, wo0 + r, _score_tiles(mats, [(0, 576)] * 2))
            project_q(xn, wqb, q_wr, (i - NH) * TQ)
            pv(i)
        qk(3, 5)
        qk(0)
        kv(7)
        pv(3)
        pv(0)
        z = norm(4, kv(6))
        qk(2)
        qk(1)
        kv(5, z)
        pv(2)
        pv(1)
        t = kv(4)
        for j, i in ((3, 3), (2, 0), (1, 2), (0, 1)):
            t = kv(j, norm(i, t))

        @pl.when(s + 3 < NP)
        def _():
            w_start(s + 3, slot)

        @pl.when(s + 2 < NP)
        def _():
            wo_start(s + 2, odd)

        @pl.when(s + 6 < NP)
        def _():
            wq_copy(s + 6).start()

        ffn_start(s)

        @pl.when(s + 5 < NP)
        def _():
            wq_copy(s + 5).wait()

        @pl.when(s + 2 < NP)
        def _():
            w_wait(odd)

        wo_wait(slot)

        @pl.when(s == 0)
        def _():
            wq_copy(4).wait()

        return carry

    with jax.named_scope('pair_loop'):
        lax.fori_loop(0, NP - 1, pair_body, 0)

    def last_body(e, carry):
        half = OS // 2
        q_rd = q_s.at[pl.ds(2, 2)]
        nxt = scores(q_rd, e, NB - 1)
        prep_wo((NP - 1) % 2, pl.multiple_of(e * half, half), half,
                pl.multiple_of((NP - 1) * OS + e * half, half),
                _score_tiles([nxt[0]], [(0, 768)]))
        pend = []
        for i in range(NB - 1, -1, -1):
            cur = nxt
            if i > 0:
                nxt = scores(q_rd, e, i - 1)
            pend.append(context(e, H - 2 + e, i, *cur, 3))
        for f in pend:
            f()
        return carry

    with jax.named_scope('last_loop'):
        lax.fori_loop(0, 2, last_body, 0)

    wr_copy.wait()
    wr = wr_s[...].astype(_F32).reshape(1, M)
    sub8 = lax.broadcasted_iota(_I32, (8, HT), 0)
    NPC = HT // 8

    def epilogue(g, src, top2, pace=None, valid=None):
        r0 = pl.multiple_of(g * HT, HT)
        best, second = top2
        bits = []
        for n, c in enumerate(range(0, HT, 8)):
            hc = src[pl.ds(c, 8), :]
            if pace is not None:
                z = pace(n)[:8]
                if n >= 3:
                    z = z | pltpu.bitcast(bits[n - 3] & 0xFFFF, _U32)
                hc = _add_zero(hc, z)
            hnb = _layernorm(hc).astype(_BF16)
            hn_s[pl.ds(r0 + c, 8), :] = hnb
            hn = hnb.astype(_F32)
            if pace is not None:
                out_s[pl.ds(r0 + c, 8), :] = (hc + hn).astype(_BF16)
            r = jnp.broadcast_to(jnp.sum(hn * wr, axis=1, keepdims=True), (8, HT))
            rb = pltpu.bitcast(_round_bf16(r) + 0.0, _I32)
            bits.append(rb)
            key = ((jnp.where(rb < 0, rb ^ 0x7FFF0000, rb) >> (16 - _IDX_BITS))
                   + ((_KEY_BIAS + S - 1 - c - r0) - sub8))
            key = pltpu.bitcast(key, _F32)
            if valid is not None:
                key = jnp.where(valid, key, 0.0)
            second = jnp.maximum(second, jnp.minimum(best, key))
            best = jnp.maximum(best, key)
        return best, second

    def prod(rh, t, tiles, z=None):
        KS = 2 * D
        ps = [None] * 7
        for u in _ORDER:
            terms = [_sub(q1, q2) + (s1 * s2,) for q1, s1 in _SA[t] for q2, s2 in _SA[u]]
            fence()
            acc = None
            for k0 in range(0, KO, KS):
                def blk(rb, kb):
                    h0 = (kb * KO + k0) // D
                    return jnp.concatenate(
                        [_as_bf16(ctx_s[h0 + hh, pl.ds(rh + rb * QT // 2, QT // 2), :])
                         for hh in range(KS // D)], axis=1)
                if len(terms) == 1:
                    lhs = blk(terms[0][0], terms[0][1])
                else:
                    lhs = _combine([(blk(rb, kb).astype(_F32), sg)
                                    for rb, kb, sg in terms]).astype(_BF16)
                w = wob_s[7 * t + u, _rows(k0, KS), :]
                if z is not None and k0 == 0 and u == _ORDER[1]:
                    w = _tie(w, {0: jnp.concatenate([z, z], axis=1)})
                d = _dot(lhs, _as_bf16(w))
                tiles.append((d, 0, 0))
                acc = d if acc is None else acc + d
            ps[u] = acc
        c11, c12, c21, c22 = _strassen_c(ps)
        return jnp.concatenate([jnp.concatenate([c11, c12], axis=1),
                                jnp.concatenate([c21, c22], axis=1)], axis=0)

    def o_body(j, top2):
        r0 = pl.multiple_of(j * TQ, TQ)

        @pl.when(j > 1)
        def _():
            out_copy(2 * j - 4).start()

        @pl.when(j > 1)
        def _():
            out_copy(2 * j - 3).start()

        rh = pl.multiple_of(j * (TQ // 2), TQ // 2)
        left, right = pl.ds(0, M // 2), pl.ds(M // 2, M // 2)

        def residual(dst, rows0, cols, att):
            hb = (x_raw[pl.ds(rows0, HT), cols].astype(_F32) + att).astype(_BF16)
            h_s[pl.ds(rows0, HT), cols] = hb
            dst[:, cols] = hb.astype(_F32)

        gp = jnp.maximum(2 * j - 2, 0)
        tl = []
        m3 = prod(rh, 2, tl)
        m4 = prod(rh, 3, tl)
        top2 = epilogue(gp, ht_s, top2, _pacer(tl[:len(tl) * 7 // 8], NPC, 1), j > 0)
        tl = []
        m5 = prod(rh, 4, tl, _zero_of(top2[0]))
        residual(ht_s, r0, right, m3 + m5)
        m1 = prod(rh, 0, tl)
        m7 = prod(rh, 6, tl)
        residual(ht_s, r0, left, m4 - m5 + m1 + m7)
        top2 = epilogue(gp + 1, hb_s, top2, _pacer(tl[:len(tl) * 7 // 8], NPC), j > 0)
        m2 = prod(rh, 1, tl, _zero_of(top2[0]))
        residual(hb_s, r0 + HT, left, m4 + m2)
        m6 = prod(rh, 5, tl)
        residual(hb_s, r0 + HT, right, m3 + m1 - m2 + m6)
        return top2

    for n in range(3):
        ffn_wait(n)
    with jax.named_scope('o_loop'):
        top2 = lax.fori_loop(0, NB, o_body, (jnp.zeros((8, HT), _F32),) * 2)
    rest = ((NG - 2, ht_s), (NG - 1, hb_s))
    out_copy(NG - 4).start()
    out_copy(NG - 3).start()
    for g, src in rest:
        top2 = epilogue(g, src, top2)

    best, second = top2
    k1 = jnp.max(best, axis=0, keepdims=True)
    k2 = jnp.max(jnp.where(best == k1, second, best), axis=0, keepdims=True)

    R = _FIX
    row = lax.broadcasted_iota(_I32, (2 * R, HT), 0)
    idx = S - 1 - (pltpu.bitcast(jnp.where(row < R, k1, k2), _I32) & (2 ** _IDX_BITS - 1))
    i1 = jnp.clip(idx[0, 0], 0, S - 1)
    i2 = jnp.clip(idx[R, 0], 0, S - 1)
    b1 = pl.multiple_of(i1 & -R, R)
    b2 = pl.multiple_of(i2 & -R, R)
    tokr = jnp.where(row < R, b1 + row, b2 + row - R)
    cd = (((pltpu.bitcast(jnp.where(tokr == i1, k1, k2), _I32) - _KEY_BIAS) >> _IDX_BITS) << 16)
    score = pltpu.bitcast(jnp.where(cd < 0, cd ^ 0x7FFF0000, cd), _F32)
    gate = _round_bf16(1.0 / (1.0 + jnp.exp(-score)))
    gate = jnp.concatenate([gate] * (M // HT), axis=1)
    tokr = jnp.concatenate([tokr] * (M // HT), axis=1)

    hnsel = jnp.concatenate([hn_s[pl.ds(b1, R), :].astype(_F32),
                             hn_s[pl.ds(b2, R), :].astype(_F32)], axis=0)
    xs = hnsel.astype(_BF16)
    g = _dot(xs, wg_s[...])
    u = _dot(xs, wu_s[...])
    pace = _pacer([(mat, 0, c0) for mat in (g, u) for c0 in range(0, F, HT)], len(rest) * NPC)
    for k, (gi, src) in enumerate(rest):
        for n, c in enumerate(range(0, HT, 8)):
            rows = pl.ds(gi * HT + c, 8)
            z = pltpu.bitcast(pace(k * NPC + n)[:8], _F32)
            z = jnp.concatenate([z] * (M // HT), axis=1)
            out_s[rows, :] = (src[pl.ds(c, 8), :] + z + hn_s[rows, :].astype(_F32)).astype(_BF16)
        out_copy(gi).start()
    g = _round_bf16(g)
    u = _round_bf16(u)
    g = _round_bf16(g * (1.0 / (1.0 + jnp.exp(-g))))
    act = (g * u).astype(_BF16)
    y = _round_bf16(_round_bf16(_dot(act, wd_s[:, pl.ds(0, M)])) * gate)
    upd = jnp.where(jnp.logical_or(tokr == i1, tokr == i2), y, 0.0)
    hsel = jnp.concatenate([h_s[pl.ds(b1, R), :].astype(_F32),
                            h_s[pl.ds(b2, R), :].astype(_F32)], axis=0)
    fixed = hsel + _round_bf16(hnsel + upd)

    pltpu.make_async_copy(out_s, out_hbm, sem_out.at[0]).wait()

    def fix_copy(b0, k):
        return pltpu.make_async_copy(out_s.at[pl.ds(b0, R), :],
                                     out_hbm.at[pl.ds(b0, R), :], sem_out.at[k])

    out_s[pl.ds(b1, R), :] = fixed[:R].astype(_BF16)
    out_s[pl.ds(b2, R), :] = fixed[R:].astype(_BF16)
    fix_copy(b1, 0).start()

    @pl.when(b2 != b1)
    def _():
        fix_copy(b2, 1).start()
        fix_copy(b2, 1).wait()

    fix_copy(b1, 0).wait()


@jax.jit
def pallas_sequential_preLN__compressed_kv_cla__moe_arch_mod__prompt_kernel(
    A_x: jax.Array,
    A_c_kv: jax.Array,
    A_w_q: jax.Array,
    A_w_uk: jax.Array,
    A_w_uv: jax.Array,
    A_w_o: jax.Array,
    B_x: jax.Array,
    B_w_r: jax.Array,
    B_w_gate: jax.Array,
    B_w_up: jax.Array,
    B_w_down: jax.Array,
):
    B, S, M = A_x.shape
    DC = A_c_kv.shape[2]
    H, D = A_w_q.shape[1], A_w_q.shape[2]
    F = B_w_gate.shape[1]
    assert (B, S, M, DC, H, D) == (1, 8 * _TQ, 1024, 512, 32, _HT) and A_c_kv.shape[1] == S
    assert F % (8 * H) == 0 and S <= 2 ** _IDX_BITS

    scratch = [
        pltpu.VMEM((S, M), _BF16),
        pltpu.VMEM((S, DC), _BF16),
        pltpu.VMEM((S, M), _F32),
        pltpu.VMEM((7, S // 2, DC // 2), _F32),
        pltpu.VMEM((4, S // 2, D), _U32),
        pltpu.VMEM((2, S // 2, D), _U32),
        pltpu.VMEM((2, S // 2, D), _U32),
        pltpu.VMEM((4, M, D), _U32),
        pltpu.VMEM((2, 2, DC, D), _U32),
        pltpu.VMEM((2, 49, M // 8, D), _U32),
        pltpu.VMEM((49, DC // 8, D), _U32),
        pltpu.VMEM((H, S // 2, D), _U32),
        pltpu.VMEM((2, 4, D // 2, M), _BF16),
        pltpu.VMEM((49, H * D // 8, M // 4), _U32),
        pltpu.VMEM((M, F), _BF16),
        pltpu.VMEM((M, F), _BF16),
        pltpu.VMEM((F, M + _WD_PAD), _BF16),
        pltpu.VMEM((_HT, M), _F32),
        pltpu.VMEM((_HT, M), _F32),
        pltpu.VMEM((S, M), _BF16),
        pltpu.VMEM((S, M), _BF16),
        pltpu.VMEM((1024, _HT), _U32),
        pltpu.VMEM((S, M), _BF16),
        pltpu.VMEM((M,), _BF16),
        pltpu.SemaphoreType.DMA((S // _TQ,)),
        pltpu.SemaphoreType.DMA((S // _TQ // 2,)),
        pltpu.SemaphoreType.DMA((2,)),
        pltpu.SemaphoreType.DMA((4,)),
        pltpu.SemaphoreType.DMA((2,)),
        pltpu.SemaphoreType.DMA((4,)),
        pltpu.SemaphoreType.DMA((2,)),
    ]
    any_spec = pl.BlockSpec(memory_space=pl.ANY)
    out = pl.pallas_call(
        functools.partial(_kernel, S=S, M=M, DC=DC, H=H, D=D, F=F),
        in_specs=[any_spec] * 10,
        out_specs=any_spec,
        out_shape=jax.ShapeDtypeStruct((S, M), _BF16),
        scratch_shapes=scratch,
        compiler_params=pltpu.CompilerParams(vmem_limit_bytes=124 * 1024 * 1024,
                                             disable_bounds_checks=True,
                                             disable_semaphore_checks=True),
        name="fused_mla_mod",
    )(A_x.reshape(S, M), A_c_kv.reshape(S, DC), A_w_q, A_w_uk, A_w_uv,
      A_w_o.reshape(H * D, M), B_w_r, B_w_gate, B_w_up, B_w_down)
    return out.reshape(B, S, M)
```

```python
import functools
import math

import jax
import jax.numpy as jnp
from jax import lax
import jax.experimental.pallas as pl
import jax.experimental.pallas.tpu as pltpu

_F32 = jnp.float32
_BF16 = jnp.bfloat16
_U32 = jnp.uint32
_I32 = jnp.int32

_EPS = 1e-5
_NEG = -1e30
_TQ = 256
_HT = 128
_QT = 64
_IDX_BITS = 13
_KEY_BIAS = 0x30000000
_FIX = 8
_WD_PAD = 128


def _dot(a, b):
    return jnp.dot(a, b, preferred_element_type=_F32)


def _dot_nt(a, b):
    return lax.dot_general(a, b, (((1,), (1,)), ((), ())), preferred_element_type=_F32)


def _as_bf16(u):
    return pltpu.bitcast(u, _BF16)


def _pack(x):
    return pltpu.bitcast(x.astype(_BF16), _U32)


def _rows(r0, n):
    if isinstance(r0, int):
        return pl.ds(r0 // 2, n // 2)
    return pl.ds(pl.multiple_of(r0 // 2, 8), n // 2)


def _ld(ref, lead, r0, n):
    return _as_bf16(ref[lead, _rows(r0, n), :])


def _st(ref, lead, r0, x, cols=slice(None)):
    ref[lead, _rows(r0, x.shape[0]), cols] = _pack(x)


def _round_bf16(x):
    return x.astype(_BF16).astype(_F32)


def _zero_of(v):
    return (pltpu.bitcast(v, _U32) >> 16) >> 16


def _lo_hi(w):
    return (pltpu.bitcast(w << 16, _F32), pltpu.bitcast(w & jnp.uint32(0xFFFF0000), _F32))


def _row_stats(x):
    n = x.shape[-1]
    mean = jnp.sum(x, axis=-1, keepdims=True) * (1.0 / n)
    xc = x - mean
    return mean, xc, jnp.sum(xc * xc, axis=-1, keepdims=True) * (1.0 / n)


def _layernorm(x):
    mean, _, var = _row_stats(x)
    den = _round_bf16(jnp.sqrt(_round_bf16(_round_bf16(var) + _EPS)))
    return (x - _round_bf16(mean)) * pl.reciprocal(den, approx=True)


def _layernorm_scaled(x, scale):
    _, xc, var = _row_stats(x)
    return xc * (lax.rsqrt(var + _EPS) * scale)


_SA = (((0, 1), (3, 1)), ((2, 1), (3, 1)), ((0, 1),), ((3, 1),),
       ((0, 1), (1, 1)), ((2, 1), (0, -1)), ((1, 1), (3, -1)))
_SB = (((0, 1), (3, 1)), ((0, 1),), ((1, 1), (3, -1)), ((2, 1), (0, -1)),
       ((3, 1),), ((0, 1), (1, 1)), ((2, 1), (3, 1)))
_ORDER = (2, 4, 3, 1, 0, 6, 5)


def _combine(terms):
    terms = sorted(terms, key=lambda ts: -ts[1])
    assert terms[0][1] > 0
    acc = terms[0][0]
    for v, sg in terms[1:]:
        acc = acc + v if sg > 0 else acc - v
    return acc


def _operands(table, quad):
    return [_combine([(quad[q], sg) for q, sg in terms]) for terms in table]


def _strassen_c(m):
    m1, m2, m3, m4, m5, m6, m7 = m
    return (m4 - m5 + m1 + m7, m3 + m5, m4 + m2, m3 - m2 + m1 + m6)


def _sub(q1, q2):
    return 2 * (q1 // 2) + q2 // 2, 2 * (q1 % 2) + q2 % 2


def _pacer(tiles, total, free=0):
    def zero(n):
        if n < free:
            return jnp.zeros((16, _HT), _U32)
        mat, r, c = tiles[(n - free) * len(tiles) // (total - free)]
        z = _zero_of(mat[r:r + 8, c:c + _HT])
        return jnp.concatenate([z, z], axis=0)
    return zero


def _score_tiles(mats, spans):
    return [(m, t0 % _TQ, (t0 // _TQ) * 4 * _HT)
            for m, (lo, hi) in zip(mats, spans) for t0 in range(lo, hi, 8)]


def _tie(w, ties):
    parts, at = [], 0
    for r in sorted(ties):
        if r > at:
            parts.append(w[at:r])
        parts.append(w[r:r + 8] | ties[r])
        at = r + 8
    if at < w.shape[0]:
        parts.append(w[at:])
    return parts[0] if len(parts) == 1 else jnp.concatenate(parts, axis=0)


def _add_zero(x, z):
    return jnp.concatenate([x[:, :_HT] + pltpu.bitcast(z, _F32), x[:, _HT:]], axis=1)


def _kernel(x_hbm, c_hbm, wq_hbm, wk_hbm, wv_hbm, wo_hbm, wr_hbm, wg_hbm, wu_hbm, wd_hbm,
            out_hbm,
            x_raw, c_raw, xn_s, ca_s, q_s, k_s, v_s,
            wq_p, wkv_p, wqb_s, wkvb_s,
            ctx_s, wo_p, wob_s, wg_s, wu_s, wd_s, ht_s, hb_s, h_s, hn_s, junk_s, out_s, wr_s,
            sem_x, sem_c, sem_w, sem_wq, sem_wo, sem_ffn, sem_out,
            *, S, M, DC, H, D, F):
    TQ, HT, QT = _TQ, _HT, _QT
    NB = S // TQ
    NH = NB // 2
    NG = S // HT
    NP = H // 2
    KQ, MQ = DC // 4, M // 4
    KO, NO = H * D // 4, M // 4
    OS = KO // NP
    qscale = (D ** -0.5) * math.log2(math.e)

    wq32 = wq_hbm.bitcast(_U32)
    wk32 = wk_hbm.bitcast(_U32)
    wv32 = wv_hbm.bitcast(_U32)

    def w_start(pair, slot):
        for k, src in enumerate((wk32, wv32)):
            pltpu.make_async_copy(src.at[:, pair, :], wkv_p.at[slot, k], sem_w.at[slot]).start()

    def w_wait(slot):
        pltpu.make_async_copy(wkv_p.at[slot], wkv_p.at[slot], sem_w.at[slot]).wait()

    def wq_copy(pair):
        return pltpu.make_async_copy(wq32.at[:, pair, :], wq_p.at[pair & 3],
                                     sem_wq.at[pair & 3])

    def wo_start(t, slot):
        r0 = pl.multiple_of(t * OS, OS)
        for k in range(4):
            pltpu.make_async_copy(wo_hbm.at[pl.ds(k * KO + r0, OS), :],
                                  wo_p.at[slot, k], sem_wo.at[slot]).start()

    def wo_wait(slot):
        pltpu.make_async_copy(wo_p.at[slot], wo_p.at[slot], sem_wo.at[slot]).wait()

    def x_copy(n):
        rows = pl.ds(pl.multiple_of(((n + NH) % NB) * TQ, TQ), TQ)
        return pltpu.make_async_copy(x_hbm.at[rows, :], x_raw.at[rows, :], sem_x.at[n])

    def c_copy(i):
        rows = pl.ds(pl.multiple_of(i * 2 * TQ, 2 * TQ), 2 * TQ)
        return pltpu.make_async_copy(c_hbm.at[rows, :], c_raw.at[rows, :], sem_c.at[i])

    ffn = ((wg_hbm, wg_s), (wu_hbm, wu_s), (wd_hbm, wd_s))

    def ffn_start(t):
        for n, (src, dst) in enumerate(ffn):
            rows, cols = src.shape[0] // NP, src.shape[1]
            r0 = pl.multiple_of(t * rows, 16)
            pltpu.make_async_copy(src.at[pl.ds(r0, rows), :],
                                  dst.at[pl.ds(r0, rows), pl.ds(0, cols)],
                                  sem_ffn.at[n]).start()

    def ffn_wait(n):
        src, dst = ffn[n]
        pltpu.make_async_copy(src, dst.at[:, pl.ds(0, src.shape[1])], sem_ffn.at[n]).wait()

    wr_copy = pltpu.make_async_copy(wr_hbm, wr_s, sem_ffn.at[3])

    def out_copy(g):
        rows = pl.ds(pl.multiple_of(g * HT, HT), HT)
        return pltpu.make_async_copy(out_s.at[rows, :], out_hbm.at[rows, :], sem_out.at[0])

    def prep_w4(srcs, dst, kq, rows, pace, sink=None):
        pieces = [(t, r) for t in range(7) for r in rows]
        for n, (t, r) in enumerate(pieces):
            terms = [[] for _ in range(4)]
            for k, (q1, sg) in enumerate(_SB[t]):
                for rb in range(2):
                    w = srcs[q1 % 2][pl.ds((2 * (q1 // 2) + rb) * kq + r, 16), :]
                    if k == 0:
                        w = w | pace(n)
                    lo, hi = _lo_hi(w)
                    terms[2 * rb].append((lo, sg))
                    terms[2 * rb + 1].append((hi, sg))
            z = None
            for u, b in enumerate(_operands(_SB, [_combine(tm) for tm in terms])):
                pk = _pack(b)
                dst[7 * t + u, pl.ds(r // 2, 8), :] = pk
                z = pk if z is None else z | pk
            if sink is not None:
                junk_s[pl.ds(8 * (sink + n), 8), :] = z

    def prep_wq(raw, slot, r, nr, pace, sink=None):
        span = 3 * MQ + nr
        prep_w4((wq_p.at[raw, pl.ds(r, span), :], wq_p.at[raw + 1, pl.ds(r, span), :]),
                wqb_s.at[slot, :, pl.ds(pl.multiple_of(r // 2, 8), nr // 2), :],
                MQ, range(0, nr, 16), pace, sink)

    def prep_wo(slot, src0, nrows, dst0, tiles):
        pieces = [(r, c0, t) for r in range(0, nrows, 16) for c0 in range(0, NO, HT)
                  for t in range(7)]
        pace = _pacer(tiles, len(pieces))
        for n, (r, c0, t) in enumerate(pieces):
            z = pltpu.bitcast(pace(n), _F32)
            sub = []
            for q2 in range(4):
                v = _combine([
                    (wo_p[slot, _sub(q1, q2)[0], pl.ds(src0 + r, 16),
                          pl.ds(_sub(q1, q2)[1] * NO + c0, HT)].astype(_F32), sg)
                    for q1, sg in _SB[t]])
                sub.append(v + z if q2 in (0, 3) else v)
            for u, b in enumerate(_operands(_SB, sub)):
                _st(wob_s, 7 * t + u, dst0 + r, b, pl.ds(c0, HT))

    def fence():
        junk_s[pl.ds(0, 8), :] = jnp.zeros((8, HT), _U32)

    def project4(lhs, w, store, zs=()):
        at = {48 * (k + 1) // len(zs): z for k, z in enumerate(zs)}
        m, tiles = [None] * 7, []
        for nt, t in enumerate(_ORDER):
            ps = [None] * 7
            for nu, u in enumerate(_ORDER):
                fence()
                a = lhs(t, u)
                wt = w[7 * t + u]
                if 7 * nt + nu in at:
                    wt = _tie(wt, {0: at[7 * nt + nu]})
                ps[u] = _dot(a.astype(_BF16), _as_bf16(wt))
                tiles += [(ps[u], r, 0) for r in range(0, QT, QT * D // (2 * a.shape[1]))]
            m[t] = _strassen_c(ps)
        for q2 in range(4):
            for q1, cblk in enumerate(_strassen_c([mt[q2] for mt in m])):
                store(_sub(q1, q2)[1], _sub(q1, q2)[0] * QT, cblk)
        return tiles

    def project_q(xn, wqb, q, r0):
        def lhs(t, u):
            return _combine([
                (xn[pl.ds(r0 + _sub(q1, q2)[0] * QT, QT), pl.ds(_sub(q1, q2)[1] * MQ, MQ)],
                 s1 * s2) for q1, s1 in _SA[t] for q2, s2 in _SA[u]])
        return project4(lhs, wqb, lambda nb, r, val: _st(q, nb, r0 + r, val))

    def project_kv(j, zs=()):
        def lhs(t, u):
            return _combine([
                (ca_s[t, pl.ds(j * HT + (q2 // 2) * QT, QT), pl.ds((q2 % 2) * KQ, KQ)], sg)
                for q2, sg in _SA[u]])
        return project4(lhs, wkvb_s,
                        lambda nb, r, val: _st((k_s, v_s)[nb // 2], nb % 2, j * TQ + r, val), zs)

    def stage_x(r0, xn, x0, pace):
        done = []
        for n, c in enumerate(range(0, TQ, 8)):
            z = pace(n)[:8]
            if n >= 6:
                z = z | done[n - 6]
            y = _layernorm_scaled(_add_zero(x_raw[pl.ds(r0 + c, 8), :].astype(_F32), z), qscale)
            xn[pl.ds(x0 + c, 8), :] = y
            done.append(_zero_of(y[:, :HT]))

    def stage_c(r0, a0, pace):
        kh = DC // 2
        for n, c in enumerate(range(0, HT, 8)):
            top = c_raw[pl.ds(r0 + c, 8), :].astype(_F32)
            bot = c_raw[pl.ds(r0 + HT + c, 8), :].astype(_F32)
            z = pltpu.bitcast(pace(n)[:8], _F32)
            z = jnp.concatenate([z] * (kh // HT), axis=1)
            quad = (top[:, :kh] + z, top[:, kh:], bot[:, :kh], bot[:, kh:] + z)
            for t, a in enumerate(_operands(_SA, quad)):
                ca_s[t, pl.ds(a0 + c, 8), :] = a

    def issue(n, carry):
        @pl.when(n == 0)
        def _():
            w_start(0, 0)

        @pl.when(n < NH)
        def _():
            c_copy(n).start()

        @pl.when(jnp.logical_or(n == NH, n == NH + 2))
        def _():
            wq_copy(n - NH).start()
            wq_copy(n - NH + 1).start()

        @pl.when(n < NB)
        def _():
            x_copy(n).start()

        @pl.when(n == NB)
        def _():
            w_start(1, 1)
            wo_start(0, 0)
        return carry

    lax.fori_loop(0, NB + 1, issue, 0)
    ht_s[...] = jnp.zeros((HT, M), _F32)
    hb_s[...] = jnp.zeros((HT, M), _F32)
    w_wait(0)
    c_copy(0).wait()
    x_copy(0).wait()

    def pro_a(i, carry):
        r0 = pl.multiple_of(i * 2 * TQ, 2 * TQ)
        wkv = jnp.concatenate(_lo_hi(wkv_p[0, 0]) + _lo_hi(wkv_p[0, 1]), axis=1).astype(_BF16)
        kv = _dot(c_raw[pl.ds(r0, 2 * TQ), :], wkv)
        for nb in range(4):
            _st((k_s, v_s)[nb // 2], nb % 2, r0, kv[:, nb * D:(nb + 1) * D])
        tiles = [(kv, r, nb * D) for nb in range(4) for r in range(0, 2 * TQ, 8)]
        nt = len(tiles)
        a0 = pl.multiple_of(i * TQ, TQ)
        stage_c(r0, a0, _pacer(tiles[:nt // 2], HT // 8))
        stage_c(r0 + TQ, a0 + HT, _pacer(tiles[nt // 2:nt * 15 // 16], HT // 8))
        rx = pl.multiple_of((i + NH) * TQ, TQ)
        stage_x(rx, xn_s, rx, _pacer(tiles[:nt * 13 // 16], TQ // 8))

        @pl.when(i + 1 < NH)
        def _():
            c_copy(i + 1).wait()

        x_copy(i + 1).wait()
        return carry

    def pro_b(i, carry):
        r0 = pl.multiple_of(i * TQ, TQ)
        xn = xn_s.at[pl.ds(r0, S // 2 + TQ), :]
        kh = M // 2
        lhs = [xn[pl.ds(S // 2, TQ), pl.ds(k0, kh)].astype(_BF16) for k0 in (0, kh)]
        tiles = []
        for nb in range(4):
            d = [_dot(lhs[k], _lo_hi(wq_p[nb // 2, pl.ds(k * kh, kh), :])[nb % 2].astype(_BF16))
                 for k in range(2)]
            _st(q_s, nb, r0 + S // 2, d[0] + d[1])
            tiles += [(dk, r, 0) for dk in d for r in range(0, TQ, 8)]
        stage_x(r0, xn, 0, _pacer(tiles[:len(tiles) * 13 // 16], TQ // 8))
        nr = MQ // (2 * NH)
        npc = 7 * nr // 16
        pace = _pacer(tiles, 3 * npc)
        for k in range(3):
            u = 3 * i + k
            quad = u // (2 * NH)
            prep_wq(2 * quad, quad, pl.multiple_of((u % (2 * NH)) * nr, nr), nr,
                    lambda n, k=k: pace(k * npc + n))

        @pl.when(i == 1)
        def _():
            wq_copy(2).wait()
            wq_copy(3).wait()

        @pl.when(i + 1 < NH)
        def _():
            x_copy(NH + i + 1).wait()

        return carry

    with jax.named_scope('pro_a'):
        lax.fori_loop(0, NH, pro_a, 0)
    wq_copy(0).wait()
    wq_copy(1).wait()
    with jax.named_scope('pro_b'):
        lax.fori_loop(0, NH, pro_b, 0)

    w_start(2, 0)
    wo_start(1, 1)
    wq_copy(4).start()
    wq_copy(5).start()
    ffn_start(NP - 1)
    wr_copy.start()
    w_wait(1)
    wo_wait(0)

    tri = (lax.broadcasted_iota(_I32, (HT, HT), 1)
           <= lax.broadcasted_iota(_I32, (HT, HT), 0))

    def softmax_rows(parts, group):
        s = parts[0] if len(parts) == 1 else jnp.concatenate(parts, axis=1)
        p = jnp.exp2(s - jnp.max(s, axis=1, keepdims=True))
        nt = p.shape[1] // HT
        tiles, acc, grp = [], None, None
        for j in range(nt):
            pj = p[:, j * HT:(j + 1) * HT]
            grp = pj if grp is None else grp + pj
            if j % group == group - 1 or j == nt - 1:
                if j % group > 0:
                    pj = jnp.minimum(pj, grp)
                acc = grp if acc is None else acc + grp
                grp = None
            tiles.append(pj)
        return (tiles[0] if nt == 1 else jnp.concatenate(tiles, axis=1)), acc

    def scores(q, e, i, zs=()):
        Lm = i * TQ + HT
        ties = {(4 + n * (Lm // HT - 4) // len(zs)) * QT + 8 * n: z for n, z in enumerate(zs)}
        keys = _as_bf16(_tie(k_s[e, pl.ds(0, Lm // 2), :], ties))
        s_main = _dot_nt(_ld(q, e, i * TQ, TQ), keys)
        s_last = _dot_nt(_ld(q, e, i * TQ + HT, HT), _ld(k_s, e, Lm, HT))
        return s_main, s_last

    def context(e, head, i, s_main, s_last, group):
        Lm = i * TQ + HT
        v_main, v_last = _ld(v_s, e, 0, Lm), _ld(v_s, e, Lm, HT)
        top = [jnp.where(tri, s_main[:HT, Lm - HT:], _NEG)]
        if Lm > HT:
            top = [s_main[:HT, :Lm - HT]] + top
        p_top, l_top = softmax_rows(top, group)
        p_bot, l_bot = softmax_rows([s_main[HT:], jnp.where(tri, s_last, _NEG)], group)
        o = _dot(jnp.concatenate([p_top, p_bot[:, :Lm]], axis=0).astype(_BF16), v_main)
        o_last = _dot(p_bot[:, Lm:].astype(_BF16), v_last)
        o = jnp.concatenate([o[:HT], o[HT:] + o_last], axis=0)
        acc = jnp.concatenate([l_top, l_bot], axis=0)

        def normalize(pace=None, n0=0):
            z = None
            for n, g in enumerate(range(0, TQ, 16)):
                a = acc[g:g + 16]
                if pace is not None:
                    a = a + pltpu.bitcast(pace(n0 + n), _F32)
                linv = jnp.broadcast_to(
                    pl.reciprocal(jnp.sum(a, axis=1, keepdims=True), approx=True), (16, D))
                ctx_s.at[head][_rows(i * TQ + g, 16), :] = _pack(o[g:g + 16] * linv)
                bits = pltpu.bitcast(linv, _U32)
                bits = bits[:8] | bits[8:]
                z = bits if z is None else z | bits
            return _zero_of(z)
        return normalize

    def pair_body(s, carry):
        odd = s & 1
        slot = 1 - odd
        wo0 = pl.multiple_of(s * OS, OS)
        q_rd = q_s.at[pl.ds(2 * odd, 2)]
        q_wr = q_s.at[:, pl.ds(pl.multiple_of(odd * (S // 4), S // 4), S // 4), :]
        xn = xn_s.at[pl.ds(pl.multiple_of(odd * (S // 2), S // 2), S // 2), :]
        quad = (s + 1) >> 1
        wqb = wqb_s.at[quad & 1]
        pend, sc = {}, {}

        def norm(i, tiles):
            pace = _pacer(tiles, TQ // 8)
            return [f(pace, k * (TQ // 16)) for k, f in enumerate(pend.pop(i))]

        def qk(i, nrm=None):
            sa = scores(q_rd, 0, i)
            zs = ()
            if nrm is not None:
                zs = norm(nrm, _score_tiles([sa[0]], [(0, (2 * i + 1) * QT * 7 // 8)]))
            sc[i] = (sa, scores(q_rd, 1, i, zs))
            return [sa[0], sc[i][1][0]]

        def pv(i):
            pend[i] = [context(e, 2 * s + e, i, *sc[i][e], 4) for e in range(2)]

        kv = project_kv
        for i in range(7, 3, -1):
            mats = qk(i, i + 2 if i + 2 < NB else None)
            if i == 7:
                prep_w4((wkv_p.at[slot, 0], wkv_p.at[slot, 1]), wkvb_s, KQ, range(0, KQ, 16),
                        _pacer(_score_tiles(mats, [(0, 768), (64, 832)]), 7 * KQ // 16), 1)
            elif i == 6:
                prep_wq(2 * (jnp.minimum(quad + 1, NP // 2 - 1) & 1), (quad + 1) & 1,
                        pl.multiple_of((1 - odd) * (MQ // 2), MQ // 2), MQ // 2,
                        _pacer(_score_tiles(mats, [(0, 704), (96, 672)]), 7 * MQ // 32), 64)
            else:
                r = (5 - i) * (OS // 2)
                prep_wo(odd, r, OS // 2, wo0 + r,
                        _score_tiles(mats, [(0, 512), (128, 576)]))
            project_q(xn, wqb, q_wr, (i - NH) * TQ)
            pv(i)
        qk(3, 5)
        qk(0)
        kv(7)
        pv(3)
        pv(0)
        z = norm(4, kv(6))
        qk(2)
        qk(1)
        kv(5, z)
        pv(2)
        pv(1)
        t = kv(4)
        for j, i in ((3, 3), (2, 0), (1, 2), (0, 1)):
            t = kv(j, norm(i, t[8:]))

        @pl.when(s + 3 < NP)
        def _():
            w_start(s + 3, slot)

        @pl.when(s + 2 < NP)
        def _():
            wo_start(s + 2, odd)

        @pl.when(s + 6 < NP)
        def _():
            wq_copy(s + 6).start()

        ffn_start(s)

        @pl.when(s + 5 < NP)
        def _():
            wq_copy(s + 5).wait()

        @pl.when(s + 2 < NP)
        def _():
            w_wait(odd)

        wo_wait(slot)

        @pl.when(s == 0)
        def _():
            wq_copy(4).wait()

        return carry

    with jax.named_scope('pair_loop'):
        lax.fori_loop(0, NP - 1, pair_body, 0)

    def last_body(e, carry):
        half = OS // 2
        q_rd = q_s.at[pl.ds(2, 2)]
        nxt = scores(q_rd, e, NB - 1)
        prep_wo((NP - 1) % 2, pl.multiple_of(e * half, half), half,
                pl.multiple_of((NP - 1) * OS + e * half, half),
                _score_tiles([nxt[0]], [(0, 768)]))
        pend = []
        for i in range(NB - 1, -1, -1):
            cur = nxt
            if i > 0:
                nxt = scores(q_rd, e, i - 1)
            pend.append(context(e, H - 2 + e, i, *cur, 3))
        for f in pend:
            f()
        return carry

    with jax.named_scope('last_loop'):
        lax.fori_loop(0, 2, last_body, 0)

    wr_copy.wait()
    wr = wr_s[...].astype(_F32).reshape(1, M)
    sub8 = lax.broadcasted_iota(_I32, (8, HT), 0)
    NPC = HT // 8

    def epilogue(g, src, top2, pace=None, valid=None):
        r0 = pl.multiple_of(g * HT, HT)
        best, second = top2
        bits = []
        for n, c in enumerate(range(0, HT, 8)):
            hc = src[pl.ds(c, 8), :]
            if pace is not None:
                z = pace(n)[:8]
                if n >= 3:
                    z = z | pltpu.bitcast(bits[n - 3] & 0xFFFF, _U32)
                hc = _add_zero(hc, z)
            hnb = _layernorm(hc).astype(_BF16)
            hn_s[pl.ds(r0 + c, 8), :] = hnb
            hn = hnb.astype(_F32)
            if pace is not None:
                out_s[pl.ds(r0 + c, 8), :] = (hc + hn).astype(_BF16)
            r = jnp.broadcast_to(jnp.sum(hn * wr, axis=1, keepdims=True), (8, HT))
            rb = pltpu.bitcast(_round_bf16(r) + 0.0, _I32)
            bits.append(rb)
            key = ((jnp.where(rb < 0, rb ^ 0x7FFF0000, rb) >> (16 - _IDX_BITS))
                   + ((_KEY_BIAS + S - 1 - c - r0) - sub8))
            key = pltpu.bitcast(key, _F32)
            if valid is not None:
                key = jnp.where(valid, key, 0.0)
            second = jnp.maximum(second, jnp.minimum(best, key))
            best = jnp.maximum(best, key)
        return best, second

    def prod(rh, t, tiles, z=None):
        KS = 2 * D
        ps = [None] * 7
        for u in _ORDER:
            terms = [_sub(q1, q2) + (s1 * s2,) for q1, s1 in _SA[t] for q2, s2 in _SA[u]]
            fence()
            acc = None
            for k0 in range(0, KO, KS):
                def blk(rb, kb):
                    h0 = (kb * KO + k0) // D
                    return jnp.concatenate(
                        [_as_bf16(ctx_s[h0 + hh, pl.ds(rh + rb * QT // 2, QT // 2), :])
                         for hh in range(KS // D)], axis=1)
                if len(terms) == 1:
                    lhs = blk(terms[0][0], terms[0][1])
                else:
                    lhs = _combine([(blk(rb, kb).astype(_F32), sg)
                                    for rb, kb, sg in terms]).astype(_BF16)
                w = wob_s[7 * t + u, _rows(k0, KS), :]
                if z is not None and k0 == 0 and u == _ORDER[1]:
                    w = _tie(w, {0: jnp.concatenate([z, z], axis=1)})
                d = _dot(lhs, _as_bf16(w))
                tiles.append((d, 0, 0))
                acc = d if acc is None else acc + d
            ps[u] = acc
        c11, c12, c21, c22 = _strassen_c(ps)
        return jnp.concatenate([jnp.concatenate([c11, c12], axis=1),
                                jnp.concatenate([c21, c22], axis=1)], axis=0)

    def o_body(j, top2):
        r0 = pl.multiple_of(j * TQ, TQ)

        @pl.when(j > 1)
        def _():
            out_copy(2 * j - 4).start()

        @pl.when(j > 1)
        def _():
            out_copy(2 * j - 3).start()

        rh = pl.multiple_of(j * (TQ // 2), TQ // 2)
        left, right = pl.ds(0, M // 2), pl.ds(M // 2, M // 2)

        def residual(dst, rows0, cols, att):
            hb = (x_raw[pl.ds(rows0, HT), cols].astype(_F32) + att).astype(_BF16)
            h_s[pl.ds(rows0, HT), cols] = hb
            dst[:, cols] = hb.astype(_F32)

        gp = jnp.maximum(2 * j - 2, 0)
        tl = []
        m3 = prod(rh, 2, tl)
        m4 = prod(rh, 3, tl)
        top2 = epilogue(gp, ht_s, top2, _pacer(tl[:len(tl) * 7 // 8], NPC, 1), j > 0)
        tl = []
        m5 = prod(rh, 4, tl, _zero_of(top2[0]))
        residual(ht_s, r0, right, m3 + m5)
        m1 = prod(rh, 0, tl)
        m7 = prod(rh, 6, tl)
        residual(ht_s, r0, left, m4 - m5 + m1 + m7)
        top2 = epilogue(gp + 1, hb_s, top2, _pacer(tl[:len(tl) * 7 // 8], NPC), j > 0)
        m2 = prod(rh, 1, tl, _zero_of(top2[0]))
        residual(hb_s, r0 + HT, left, m4 + m2)
        m6 = prod(rh, 5, tl)
        residual(hb_s, r0 + HT, right, m3 + m1 - m2 + m6)
        return top2

    for n in range(3):
        ffn_wait(n)
    with jax.named_scope('o_loop'):
        top2 = lax.fori_loop(0, NB, o_body, (jnp.zeros((8, HT), _F32),) * 2)
    rest = ((NG - 2, ht_s), (NG - 1, hb_s))
    out_copy(NG - 4).start()
    out_copy(NG - 3).start()
    for g, src in rest:
        top2 = epilogue(g, src, top2)

    best, second = top2
    k1 = jnp.max(best, axis=0, keepdims=True)
    k2 = jnp.max(jnp.where(best == k1, second, best), axis=0, keepdims=True)

    R = _FIX
    row = lax.broadcasted_iota(_I32, (2 * R, HT), 0)
    idx = S - 1 - (pltpu.bitcast(jnp.where(row < R, k1, k2), _I32) & (2 ** _IDX_BITS - 1))
    i1 = jnp.clip(idx[0, 0], 0, S - 1)
    i2 = jnp.clip(idx[R, 0], 0, S - 1)
    b1 = pl.multiple_of(i1 & -R, R)
    b2 = pl.multiple_of(i2 & -R, R)
    tokr = jnp.where(row < R, b1 + row, b2 + row - R)
    cd = (((pltpu.bitcast(jnp.where(tokr == i1, k1, k2), _I32) - _KEY_BIAS) >> _IDX_BITS) << 16)
    score = pltpu.bitcast(jnp.where(cd < 0, cd ^ 0x7FFF0000, cd), _F32)
    gate = _round_bf16(1.0 / (1.0 + jnp.exp(-score)))
    gate = jnp.concatenate([gate] * (M // HT), axis=1)
    tokr = jnp.concatenate([tokr] * (M // HT), axis=1)

    hnsel = jnp.concatenate([hn_s[pl.ds(b1, R), :].astype(_F32),
                             hn_s[pl.ds(b2, R), :].astype(_F32)], axis=0)
    xs = hnsel.astype(_BF16)
    g = _dot(xs, wg_s[...])
    u = _dot(xs, wu_s[...])
    pace = _pacer([(mat, 0, c0) for mat in (g, u) for c0 in range(0, F, HT)], len(rest) * NPC)
    for k, (gi, src) in enumerate(rest):
        for n, c in enumerate(range(0, HT, 8)):
            rows = pl.ds(gi * HT + c, 8)
            z = pltpu.bitcast(pace(k * NPC + n)[:8], _F32)
            z = jnp.concatenate([z] * (M // HT), axis=1)
            out_s[rows, :] = (src[pl.ds(c, 8), :] + z + hn_s[rows, :].astype(_F32)).astype(_BF16)
        out_copy(gi).start()
    g = _round_bf16(g)
    u = _round_bf16(u)
    g = _round_bf16(g * (1.0 / (1.0 + jnp.exp(-g))))
    act = (g * u).astype(_BF16)
    y = _round_bf16(_round_bf16(_dot(act, wd_s[:, pl.ds(0, M)])) * gate)
    upd = jnp.where(jnp.logical_or(tokr == i1, tokr == i2), y, 0.0)
    hsel = jnp.concatenate([h_s[pl.ds(b1, R), :].astype(_F32),
                            h_s[pl.ds(b2, R), :].astype(_F32)], axis=0)
    fixed = hsel + _round_bf16(hnsel + upd)

    pltpu.make_async_copy(out_s, out_hbm, sem_out.at[0]).wait()

    def fix_copy(b0, k):
        return pltpu.make_async_copy(out_s.at[pl.ds(b0, R), :],
                                     out_hbm.at[pl.ds(b0, R), :], sem_out.at[k])

    out_s[pl.ds(b1, R), :] = fixed[:R].astype(_BF16)
    out_s[pl.ds(b2, R), :] = fixed[R:].astype(_BF16)
    fix_copy(b1, 0).start()

    @pl.when(b2 != b1)
    def _():
        fix_copy(b2, 1).start()
        fix_copy(b2, 1).wait()

    fix_copy(b1, 0).wait()


@jax.jit
def pallas_sequential_preLN__compressed_kv_cla__moe_arch_mod__prompt_kernel(
    A_x: jax.Array,
    A_c_kv: jax.Array,
    A_w_q: jax.Array,
    A_w_uk: jax.Array,
    A_w_uv: jax.Array,
    A_w_o: jax.Array,
    B_x: jax.Array,
    B_w_r: jax.Array,
    B_w_gate: jax.Array,
    B_w_up: jax.Array,
    B_w_down: jax.Array,
):
    B, S, M = A_x.shape
    DC = A_c_kv.shape[2]
    H, D = A_w_q.shape[1], A_w_q.shape[2]
    F = B_w_gate.shape[1]
    assert (B, S, M, DC, H, D) == (1, 8 * _TQ, 1024, 512, 32, _HT) and A_c_kv.shape[1] == S
    assert F % (8 * H) == 0 and S <= 2 ** _IDX_BITS

    scratch = [
        pltpu.VMEM((S, M), _BF16),
        pltpu.VMEM((S, DC), _BF16),
        pltpu.VMEM((S, M), _F32),
        pltpu.VMEM((7, S // 2, DC // 2), _F32),
        pltpu.VMEM((4, S // 2, D), _U32),
        pltpu.VMEM((2, S // 2, D), _U32),
        pltpu.VMEM((2, S // 2, D), _U32),
        pltpu.VMEM((4, M, D), _U32),
        pltpu.VMEM((2, 2, DC, D), _U32),
        pltpu.VMEM((2, 49, M // 8, D), _U32),
        pltpu.VMEM((49, DC // 8, D), _U32),
        pltpu.VMEM((H, S // 2, D), _U32),
        pltpu.VMEM((2, 4, D // 2, M), _BF16),
        pltpu.VMEM((49, H * D // 8, M // 4), _U32),
        pltpu.VMEM((M, F), _BF16),
        pltpu.VMEM((M, F), _BF16),
        pltpu.VMEM((F, M + _WD_PAD), _BF16),
        pltpu.VMEM((_HT, M), _F32),
        pltpu.VMEM((_HT, M), _F32),
        pltpu.VMEM((S, M), _BF16),
        pltpu.VMEM((S, M), _BF16),
        pltpu.VMEM((1024, _HT), _U32),
        pltpu.VMEM((S, M), _BF16),
        pltpu.VMEM((M,), _BF16),
        pltpu.SemaphoreType.DMA((S // _TQ,)),
        pltpu.SemaphoreType.DMA((S // _TQ // 2,)),
        pltpu.SemaphoreType.DMA((2,)),
        pltpu.SemaphoreType.DMA((4,)),
        pltpu.SemaphoreType.DMA((2,)),
        pltpu.SemaphoreType.DMA((4,)),
        pltpu.SemaphoreType.DMA((2,)),
    ]
    any_spec = pl.BlockSpec(memory_space=pl.ANY)
    out = pl.pallas_call(
        functools.partial(_kernel, S=S, M=M, DC=DC, H=H, D=D, F=F),
        in_specs=[any_spec] * 10,
        out_specs=any_spec,
        out_shape=jax.ShapeDtypeStruct((S, M), _BF16),
        scratch_shapes=scratch,
        compiler_params=pltpu.CompilerParams(vmem_limit_bytes=124 * 1024 * 1024,
                                             disable_bounds_checks=True,
                                             disable_semaphore_checks=True),
        name="fused_mla_mod",
    )(A_x.reshape(S, M), A_c_kv.reshape(S, DC), A_w_q, A_w_uk, A_w_uv,
      A_w_o.reshape(H * D, M), B_w_r, B_w_gate, B_w_up, B_w_down)
    return out.reshape(B, S, M)
```

```python
import functools
import math

import jax
import jax.numpy as jnp
from jax import lax
import jax.experimental.pallas as pl
import jax.experimental.pallas.tpu as pltpu

_F32 = jnp.float32
_BF16 = jnp.bfloat16
_U32 = jnp.uint32
_I32 = jnp.int32

_EPS = 1e-5
_NEG = -1e30
_TQ = 256
_HT = 128
_QT = 64
_IDX_BITS = 13
_KEY_BIAS = 0x30000000
_FIX = 8
_PAD = 128


def _dot(a, b):
    return jnp.dot(a, b, preferred_element_type=_F32)


def _dot_nt(a, b):
    return lax.dot_general(a, b, (((1,), (1,)), ((), ())), preferred_element_type=_F32)


def _as_bf16(u):
    return pltpu.bitcast(u, _BF16)


def _pack(x):
    return pltpu.bitcast(x.astype(_BF16), _U32)


def _rows(r0, n):
    if isinstance(r0, int):
        return pl.ds(r0 // 2, n // 2)
    return pl.ds(pl.multiple_of(r0 // 2, 8), n // 2)


def _ld(ref, lead, r0, n):
    return _as_bf16(ref[lead, _rows(r0, n), :])


def _st(ref, lead, r0, x, cols=slice(None)):
    ref[lead, _rows(r0, x.shape[0]), cols] = _pack(x)


def _round_bf16(x):
    return x.astype(_BF16).astype(_F32)


def _zero_of(v):
    return (pltpu.bitcast(v, _U32) >> 16) >> 16


def _lo_hi(w):
    return (pltpu.bitcast(w << 16, _F32), pltpu.bitcast(w & jnp.uint32(0xFFFF0000), _F32))


def _row_stats(x):
    n = x.shape[-1]
    mean = jnp.sum(x, axis=-1, keepdims=True) * (1.0 / n)
    xc = x - mean
    return mean, xc, jnp.sum(xc * xc, axis=-1, keepdims=True) * (1.0 / n)


def _layernorm(x):
    mean, _, var = _row_stats(x)
    den = _round_bf16(jnp.sqrt(_round_bf16(_round_bf16(var) + _EPS)))
    return (x - _round_bf16(mean)) * pl.reciprocal(den, approx=True)


def _layernorm_scaled(x, scale):
    _, xc, var = _row_stats(x)
    return xc * (lax.rsqrt(var + _EPS) * scale)


_SA = (((0, 1), (3, 1)), ((2, 1), (3, 1)), ((0, 1),), ((3, 1),),
       ((0, 1), (1, 1)), ((2, 1), (0, -1)), ((1, 1), (3, -1)))
_SB = (((0, 1), (3, 1)), ((0, 1),), ((1, 1), (3, -1)), ((2, 1), (0, -1)),
       ((3, 1),), ((0, 1), (1, 1)), ((2, 1), (3, 1)))
_ORDER = (2, 4, 3, 1, 0, 6, 5)


def _combine(terms):
    terms = sorted(terms, key=lambda ts: -ts[1])
    assert terms[0][1] > 0
    acc = terms[0][0]
    for v, sg in terms[1:]:
        acc = acc + v if sg > 0 else acc - v
    return acc


def _operands(table, quad):
    return [_combine([(quad[q], sg) for q, sg in terms]) for terms in table]


def _strassen_c(m):
    m1, m2, m3, m4, m5, m6, m7 = m
    return (m4 - m5 + m1 + m7, m3 + m5, m4 + m2, m3 - m2 + m1 + m6)


def _sub(q1, q2):
    return 2 * (q1 // 2) + q2 // 2, 2 * (q1 % 2) + q2 % 2


def _pacer(tiles, total, free=0):
    def zero(n):
        if n < free:
            return jnp.zeros((16, _HT), _U32)
        mat, r, c = tiles[(n - free) * len(tiles) // (total - free)]
        z = _zero_of(mat[r:r + 8, c:c + _HT])
        return jnp.concatenate([z, z], axis=0)
    return zero


def _score_tiles(mats, spans):
    return [(m, t0 % _TQ, (t0 // _TQ) * 4 * _HT)
            for m, (lo, hi) in zip(mats, spans) for t0 in range(lo, hi, 8)]


def _tie(w, ties):
    parts, at = [], 0
    for r in sorted(ties):
        if r > at:
            parts.append(w[at:r])
        parts.append(w[r:r + 8] | ties[r])
        at = r + 8
    if at < w.shape[0]:
        parts.append(w[at:])
    return parts[0] if len(parts) == 1 else jnp.concatenate(parts, axis=0)


def _add_zero(x, z):
    return jnp.concatenate([x[:, :_HT] + pltpu.bitcast(z, _F32), x[:, _HT:]], axis=1)


def _kernel(x_hbm, c_hbm, wq_hbm, wk_hbm, wv_hbm, wo_hbm, wr_hbm, wg_hbm, wu_hbm, wd_hbm,
            out_hbm,
            x_raw, c_raw, xn_s, ca_s, q_s, k_s, v_s,
            wq_p, wkv_p, wqb_s, wkvb_s,
            ctx_s, wo_p, wob_s, wg_s, wu_s, wd_s, ht_s, hb_s, h_s, hn_s, junk_s, out_s, wr_s,
            sem_x, sem_c, sem_w, sem_wq, sem_wo, sem_ffn, sem_out,
            *, S, M, DC, H, D, F):
    TQ, HT, QT = _TQ, _HT, _QT
    NB = S // TQ
    NH = NB // 2
    NG = S // HT
    NP = H // 2
    KQ, MQ = DC // 4, M // 4
    KO, NO = H * D // 4, M // 4
    OS = KO // NP
    qscale = (D ** -0.5) * math.log2(math.e)

    wq32 = wq_hbm.bitcast(_U32)
    wk32 = wk_hbm.bitcast(_U32)
    wv32 = wv_hbm.bitcast(_U32)

    def w_start(pair, slot):
        for k, src in enumerate((wk32, wv32)):
            pltpu.make_async_copy(src.at[:, pair, :], wkv_p.at[slot, k], sem_w.at[slot]).start()

    def w_wait(slot):
        pltpu.make_async_copy(wkv_p.at[slot], wkv_p.at[slot], sem_w.at[slot]).wait()

    def wq_copy(pair):
        return pltpu.make_async_copy(wq32.at[:, pair, :], wq_p.at[pair & 3],
                                     sem_wq.at[pair & 3])

    def wo_start(t, slot):
        r0 = pl.multiple_of(t * OS, OS)
        for k in range(4):
            pltpu.make_async_copy(wo_hbm.at[pl.ds(k * KO + r0, OS), :],
                                  wo_p.at[slot, k], sem_wo.at[slot]).start()

    def wo_wait(slot):
        pltpu.make_async_copy(wo_p.at[slot], wo_p.at[slot], sem_wo.at[slot]).wait()

    def x_copy(n):
        rows = pl.ds(pl.multiple_of(((n + NH) % NB) * TQ, TQ), TQ)
        return pltpu.make_async_copy(x_hbm.at[rows, :], x_raw.at[rows, :], sem_x.at[n])

    def c_copy(i):
        rows = pl.ds(pl.multiple_of(i * 2 * TQ, 2 * TQ), 2 * TQ)
        return pltpu.make_async_copy(c_hbm.at[rows, :], c_raw.at[rows, :], sem_c.at[i])

    ffn = ((wg_hbm, wg_s), (wu_hbm, wu_s), (wd_hbm, wd_s))

    def ffn_start(t):
        for n, (src, dst) in enumerate(ffn):
            rows, cols = src.shape[0] // NP, src.shape[1]
            r0 = pl.multiple_of(t * rows, 16)
            pltpu.make_async_copy(src.at[pl.ds(r0, rows), :],
                                  dst.at[pl.ds(r0, rows), pl.ds(0, cols)],
                                  sem_ffn.at[n]).start()

    def ffn_wait(n):
        src, dst = ffn[n]
        pltpu.make_async_copy(src, dst.at[:, pl.ds(0, src.shape[1])], sem_ffn.at[n]).wait()

    wr_copy = pltpu.make_async_copy(wr_hbm, wr_s, sem_ffn.at[3])

    def out_copy(g):
        rows = pl.ds(pl.multiple_of(g * HT, HT), HT)
        return pltpu.make_async_copy(out_s.at[rows, :], out_hbm.at[rows, :], sem_out.at[0])

    def prep_w4(srcs, dst, kq, rows, pace, sink=None):
        pieces = [(t, r) for t in range(7) for r in rows]
        for n, (t, r) in enumerate(pieces):
            terms = [[] for _ in range(4)]
            for k, (q1, sg) in enumerate(_SB[t]):
                for rb in range(2):
                    w = srcs[q1 % 2][pl.ds((2 * (q1 // 2) + rb) * kq + r, 16), :]
                    if k == 0:
                        w = w | pace(n)
                    lo, hi = _lo_hi(w)
                    terms[2 * rb].append((lo, sg))
                    terms[2 * rb + 1].append((hi, sg))
            z = None
            for u, b in enumerate(_operands(_SB, [_combine(tm) for tm in terms])):
                pk = _pack(b)
                dst[7 * t + u, pl.ds(r // 2, 8), :] = pk
                z = pk if z is None else z | pk
            if sink is not None:
                junk_s[pl.ds(8 * (sink + n), 8), :] = z

    def prep_wq(raw, slot, r, nr, pace, sink=None):
        span = 3 * MQ + nr
        prep_w4((wq_p.at[raw, pl.ds(r, span), :], wq_p.at[raw + 1, pl.ds(r, span), :]),
                wqb_s.at[slot, :, pl.ds(pl.multiple_of(r // 2, 8), nr // 2), :],
                MQ, range(0, nr, 16), pace, sink)

    def prep_wo(slot, src0, nrows, dst0, tiles):
        pieces = [(r, c0, t) for r in range(0, nrows, 16) for c0 in range(0, NO, HT)
                  for t in range(7)]
        pace = _pacer(tiles, len(pieces))
        for n, (r, c0, t) in enumerate(pieces):
            z = pltpu.bitcast(pace(n), _F32)
            sub = []
            for q2 in range(4):
                v = _combine([
                    (wo_p[slot, _sub(q1, q2)[0], pl.ds(src0 + r, 16),
                          pl.ds(_sub(q1, q2)[1] * NO + c0, HT)].astype(_F32), sg)
                    for q1, sg in _SB[t]])
                sub.append(v + z if q2 in (0, 3) else v)
            for u, b in enumerate(_operands(_SB, sub)):
                _st(wob_s, 7 * t + u, dst0 + r, b, pl.ds(c0, HT))

    def fence():
        junk_s[pl.ds(0, 8), :] = jnp.zeros((8, HT), _U32)

    def project4(lhs, w, store, zs=()):
        at = {48 * (k + 1) // len(zs): z for k, z in enumerate(zs)}
        m, tiles = [None] * 7, []
        for nt, t in enumerate(_ORDER):
            ps = [None] * 7
            for nu, u in enumerate(_ORDER):
                fence()
                a = lhs(t, u)
                wt = w[7 * t + u]
                if 7 * nt + nu in at:
                    wt = _tie(wt, {0: at[7 * nt + nu]})
                ps[u] = _dot(a.astype(_BF16), _as_bf16(wt))
                tiles += [(ps[u], r, 0) for r in range(0, QT, QT * D // (2 * a.shape[1]))]
            m[t] = _strassen_c(ps)
        for q2 in range(4):
            for q1, cblk in enumerate(_strassen_c([mt[q2] for mt in m])):
                store(_sub(q1, q2)[1], _sub(q1, q2)[0] * QT, cblk)
        return tiles

    def project_q(xn, wqb, q, r0):
        def lhs(t, u):
            return _combine([
                (xn[pl.ds(r0 + _sub(q1, q2)[0] * QT, QT), pl.ds(_sub(q1, q2)[1] * MQ, MQ)],
                 s1 * s2) for q1, s1 in _SA[t] for q2, s2 in _SA[u]])
        return project4(lhs, wqb, lambda nb, r, val: _st(q, nb, r0 + r, val))

    def project_kv(j, zs=()):
        def lhs(t, u):
            return _combine([
                (ca_s[t, pl.ds(j * HT + (q2 // 2) * QT, QT), pl.ds((q2 % 2) * KQ, KQ)], sg)
                for q2, sg in _SA[u]])
        return project4(lhs, wkvb_s,
                        lambda nb, r, val: _st((k_s, v_s)[nb // 2], nb % 2, j * TQ + r, val), zs)

    def stage_x(r0, xn, x0, pace):
        done = []
        for n, c in enumerate(range(0, TQ, 8)):
            z = pace(n)[:8]
            if n >= 6:
                z = z | done[n - 6]
            y = _layernorm_scaled(_add_zero(x_raw[pl.ds(r0 + c, 8), :].astype(_F32), z), qscale)
            xn[pl.ds(x0 + c, 8), pl.ds(0, M)] = y
            done.append(_zero_of(y[:, :HT]))

    def stage_c(r0, a0, pace):
        kh = DC // 2
        for n, c in enumerate(range(0, HT, 8)):
            top = c_raw[pl.ds(r0 + c, 8), :].astype(_F32)
            bot = c_raw[pl.ds(r0 + HT + c, 8), :].astype(_F32)
            z = pltpu.bitcast(pace(n)[:8], _F32)
            z = jnp.concatenate([z] * (kh // HT), axis=1)
            quad = (top[:, :kh] + z, top[:, kh:], bot[:, :kh], bot[:, kh:] + z)
            for t, a in enumerate(_operands(_SA, quad)):
                ca_s[t, pl.ds(a0 + c, 8), :] = a

    def issue(n, carry):
        @pl.when(n == 0)
        def _():
            w_start(0, 0)

        @pl.when(n < NH)
        def _():
            c_copy(n).start()

        @pl.when(jnp.logical_or(n == NH, n == NH + 2))
        def _():
            wq_copy(n - NH).start()
            wq_copy(n - NH + 1).start()

        @pl.when(n < NB)
        def _():
            x_copy(n).start()

        @pl.when(n == NB)
        def _():
            w_start(1, 1)
            wo_start(0, 0)
        return carry

    lax.fori_loop(0, NB + 1, issue, 0)
    ht_s[...] = jnp.zeros((HT, M), _F32)
    hb_s[...] = jnp.zeros((HT, M), _F32)
    w_wait(0)
    c_copy(0).wait()
    x_copy(0).wait()

    def pro_a(i, carry):
        r0 = pl.multiple_of(i * 2 * TQ, 2 * TQ)
        wkv = jnp.concatenate(_lo_hi(wkv_p[0, 0]) + _lo_hi(wkv_p[0, 1]), axis=1).astype(_BF16)
        kv = _dot(c_raw[pl.ds(r0, 2 * TQ), :], wkv)
        for nb in range(4):
            _st((k_s, v_s)[nb // 2], nb % 2, r0, kv[:, nb * D:(nb + 1) * D])
        tiles = [(kv, r, nb * D) for nb in range(4) for r in range(0, 2 * TQ, 8)]
        nt = len(tiles)
        a0 = pl.multiple_of(i * TQ, TQ)
        stage_c(r0, a0, _pacer(tiles[:nt // 2], HT // 8))
        stage_c(r0 + TQ, a0 + HT, _pacer(tiles[nt // 2:nt * 15 // 16], HT // 8))
        rx = pl.multiple_of((i + NH) * TQ, TQ)
        stage_x(rx, xn_s, rx, _pacer(tiles[:nt * 13 // 16], TQ // 8))

        @pl.when(i + 1 < NH)
        def _():
            c_copy(i + 1).wait()

        x_copy(i + 1).wait()
        return carry

    def pro_b(i, carry):
        r0 = pl.multiple_of(i * TQ, TQ)
        xn = xn_s.at[pl.ds(r0, S // 2 + TQ), :]
        kh = M // 2
        lhs = [xn[pl.ds(S // 2, TQ), pl.ds(k0, kh)].astype(_BF16) for k0 in (0, kh)]
        tiles = []
        for nb in range(4):
            d = [_dot(lhs[k], _lo_hi(wq_p[nb // 2, pl.ds(k * kh, kh), :])[nb % 2].astype(_BF16))
                 for k in range(2)]
            _st(q_s, nb, r0 + S // 2, d[0] + d[1])
            tiles += [(dk, r, 0) for dk in d for r in range(0, TQ, 8)]
        stage_x(r0, xn, 0, _pacer(tiles[:len(tiles) * 13 // 16], TQ // 8))
        nr = MQ // (2 * NH)
        npc = 7 * nr // 16
        pace = _pacer(tiles, 3 * npc)
        for k in range(3):
            u = 3 * i + k
            quad = u // (2 * NH)
            prep_wq(2 * quad, quad, pl.multiple_of((u % (2 * NH)) * nr, nr), nr,
                    lambda n, k=k: pace(k * npc + n))

        @pl.when(i == 1)
        def _():
            wq_copy(2).wait()
            wq_copy(3).wait()

        @pl.when(i + 1 < NH)
        def _():
            x_copy(NH + i + 1).wait()

        return carry

    with jax.named_scope('pro_a'):
        lax.fori_loop(0, NH, pro_a, 0)
    wq_copy(0).wait()
    wq_copy(1).wait()
    with jax.named_scope('pro_b'):
        lax.fori_loop(0, NH, pro_b, 0)

    w_start(2, 0)
    wo_start(1, 1)
    wq_copy(4).start()
    wq_copy(5).start()
    ffn_start(NP - 1)
    wr_copy.start()
    w_wait(1)
    wo_wait(0)

    tri = (lax.broadcasted_iota(_I32, (HT, HT), 1)
           <= lax.broadcasted_iota(_I32, (HT, HT), 0))

    def softmax_rows(parts, group):
        s = parts[0] if len(parts) == 1 else jnp.concatenate(parts, axis=1)
        p = jnp.exp2(s - jnp.max(s, axis=1, keepdims=True))
        nt = p.shape[1] // HT
        tiles, acc, grp = [], None, None
        for j in range(nt):
            pj = p[:, j * HT:(j + 1) * HT]
            grp = pj if grp is None else grp + pj
            if j % group == group - 1 or j == nt - 1:
                if j % group > 0:
                    pj = jnp.minimum(pj, grp)
                acc = grp if acc is None else acc + grp
                grp = None
            tiles.append(pj)
        return (tiles[0] if nt == 1 else jnp.concatenate(tiles, axis=1)), acc

    def scores(q, e, i, zs=()):
        Lm = i * TQ + HT
        ties = {(4 + n * (Lm // HT - 4) // len(zs)) * QT + 8 * n: z for n, z in enumerate(zs)}
        keys = _as_bf16(_tie(k_s[e, pl.ds(0, Lm // 2), :], ties))
        s_main = _dot_nt(_ld(q, e, i * TQ, TQ), keys)
        s_last = _dot_nt(_ld(q, e, i * TQ + HT, HT), _ld(k_s, e, Lm, HT))
        return s_main, s_last

    def context(e, head, i, s_main, s_last, group):
        Lm = i * TQ + HT
        v_main, v_last = _ld(v_s, e, 0, Lm), _ld(v_s, e, Lm, HT)
        top = [jnp.where(tri, s_main[:HT, Lm - HT:], _NEG)]
        if Lm > HT:
            top = [s_main[:HT, :Lm - HT]] + top
        p_top, l_top = softmax_rows(top, group)
        p_bot, l_bot = softmax_rows([s_main[HT:], jnp.where(tri, s_last, _NEG)], group)
        o = _dot(jnp.concatenate([p_top, p_bot[:, :Lm]], axis=0).astype(_BF16), v_main)
        o_last = _dot(p_bot[:, Lm:].astype(_BF16), v_last)
        o = jnp.concatenate([o[:HT], o[HT:] + o_last], axis=0)
        acc = jnp.concatenate([l_top, l_bot], axis=0)

        def normalize(pace=None, n0=0):
            z = None
            for n, g in enumerate(range(0, TQ, 16)):
                a = acc[g:g + 16]
                if pace is not None:
                    a = a + pltpu.bitcast(pace(n0 + n), _F32)
                linv = jnp.broadcast_to(
                    pl.reciprocal(jnp.sum(a, axis=1, keepdims=True), approx=True), (16, D))
                ctx_s.at[head][_rows(i * TQ + g, 16), :] = _pack(o[g:g + 16] * linv)
                bits = pltpu.bitcast(linv, _U32)
                bits = bits[:8] | bits[8:]
                z = bits if z is None else z | bits
            return _zero_of(z)
        return normalize

    def pair_body(s, carry):
        odd = s & 1
        slot = 1 - odd
        wo0 = pl.multiple_of(s * OS, OS)
        q_rd = q_s.at[pl.ds(2 * odd, 2)]
        q_wr = q_s.at[:, pl.ds(pl.multiple_of(odd * (S // 4), S // 4), S // 4), :]
        xn = xn_s.at[pl.ds(pl.multiple_of(odd * (S // 2), S // 2), S // 2), :]
        quad = (s + 1) >> 1
        wqb = wqb_s.at[quad & 1]
        pend, sc = {}, {}

        def norm(i, tiles):
            pace = _pacer(tiles, TQ // 8)
            return [f(pace, k * (TQ // 16)) for k, f in enumerate(pend.pop(i))]

        def qk(i, nrm=None):
            sa = scores(q_rd, 0, i)
            zs = ()
            if nrm is not None:
                zs = norm(nrm, _score_tiles([sa[0]], [(0, (2 * i + 1) * QT * 7 // 8)]))
            sc[i] = (sa, scores(q_rd, 1, i, zs))
            return [sa[0], sc[i][1][0]]

        def pv(i):
            pend[i] = [context(e, 2 * s + e, i, *sc[i][e], 4) for e in range(2)]

        kv = project_kv
        for i in range(7, 3, -1):
            mats = qk(i, i + 2 if i + 2 < NB else None)
            if i == 7:
                prep_w4((wkv_p.at[slot, 0], wkv_p.at[slot, 1]), wkvb_s, KQ, range(0, KQ, 16),
                        _pacer(_score_tiles(mats, [(0, 768), (64, 832)]), 7 * KQ // 16), 1)
            elif i == 6:
                prep_wq(2 * (jnp.minimum(quad + 1, NP // 2 - 1) & 1), (quad + 1) & 1,
                        pl.multiple_of((1 - odd) * (MQ // 2), MQ // 2), MQ // 2,
                        _pacer(_score_tiles(mats, [(0, 704), (96, 672)]), 7 * MQ // 32), 64)
            else:
                r = (5 - i) * (OS // 2)
                prep_wo(odd, r, OS // 2, wo0 + r,
                        _score_tiles(mats, [(0, 512), (128, 576)]))
            project_q(xn, wqb, q_wr, (i - NH) * TQ)
            pv(i)
        qk(3, 5)
        qk(0)
        kv(7)
        pv(3)
        pv(0)
        z = norm(4, kv(6))
        qk(2)
        qk(1)
        kv(5, z)
        pv(2)
        pv(1)
        t = kv(4)
        for j, i in ((3, 3), (2, 0), (1, 2), (0, 1)):
            t = kv(j, norm(i, t[8:]))

        @pl.when(s + 3 < NP)
        def _():
            w_start(s + 3, slot)

        @pl.when(s + 2 < NP)
        def _():
            wo_start(s + 2, odd)

        @pl.when(s + 6 < NP)
        def _():
            wq_copy(s + 6).start()

        ffn_start(s)

        @pl.when(s + 5 < NP)
        def _():
            wq_copy(s + 5).wait()

        @pl.when(s + 2 < NP)
        def _():
            w_wait(odd)

        wo_wait(slot)

        @pl.when(s == 0)
        def _():
            wq_copy(4).wait()

        return carry

    with jax.named_scope('pair_loop'):
        lax.fori_loop(0, NP - 1, pair_body, 0)

    def last_body(e, carry):
        half = OS // 2
        q_rd = q_s.at[pl.ds(2, 2)]
        nxt = scores(q_rd, e, NB - 1)
        prep_wo((NP - 1) % 2, pl.multiple_of(e * half, half), half,
                pl.multiple_of((NP - 1) * OS + e * half, half),
                _score_tiles([nxt[0]], [(0, 768)]))
        pend = []
        for i in range(NB - 1, -1, -1):
            cur = nxt
            if i > 0:
                nxt = scores(q_rd, e, i - 1)
            pend.append(context(e, H - 2 + e, i, *cur, 3))
        for f in pend:
            f()
        return carry

    with jax.named_scope('last_loop'):
        lax.fori_loop(0, 2, last_body, 0)

    wr_copy.wait()
    wr = wr_s[...].astype(_F32).reshape(1, M)
    sub8 = lax.broadcasted_iota(_I32, (8, HT), 0)
    NPC = HT // 8

    def epilogue(g, src, top2, pace=None, valid=None):
        r0 = pl.multiple_of(g * HT, HT)
        best, second = top2
        bits = []
        for n, c in enumerate(range(0, HT, 8)):
            hc = src[pl.ds(c, 8), :]
            if pace is not None:
                z = pace(n)[:8]
                if n >= 3:
                    z = z | pltpu.bitcast(bits[n - 3] & 0xFFFF, _U32)
                hc = _add_zero(hc, z)
            hnb = _layernorm(hc).astype(_BF16)
            hn_s[pl.ds(r0 + c, 8), :] = hnb
            hn = hnb.astype(_F32)
            if pace is not None:
                out_s[pl.ds(r0 + c, 8), :] = (hc + hn).astype(_BF16)
            r = jnp.broadcast_to(jnp.sum(hn * wr, axis=1, keepdims=True), (8, HT))
            rb = pltpu.bitcast(_round_bf16(r) + 0.0, _I32)
            bits.append(rb)
            key = ((jnp.where(rb < 0, rb ^ 0x7FFF0000, rb) >> (16 - _IDX_BITS))
                   + ((_KEY_BIAS + S - 1 - c - r0) - sub8))
            key = pltpu.bitcast(key, _F32)
            if valid is not None:
                key = jnp.where(valid, key, 0.0)
            second = jnp.maximum(second, jnp.minimum(best, key))
            best = jnp.maximum(best, key)
        return best, second

    def prod(rh, t, tiles, z=None):
        KS = 2 * D
        ps = [None] * 7
        for u in _ORDER:
            terms = [_sub(q1, q2) + (s1 * s2,) for q1, s1 in _SA[t] for q2, s2 in _SA[u]]
            fence()
            acc = None
            for k0 in range(0, KO, KS):
                def blk(rb, kb):
                    h0 = (kb * KO + k0) // D
                    return jnp.concatenate(
                        [_as_bf16(ctx_s[h0 + hh, pl.ds(rh + rb * QT // 2, QT // 2), :])
                         for hh in range(KS // D)], axis=1)
                if len(terms) == 1:
                    lhs = blk(terms[0][0], terms[0][1])
                else:
                    lhs = _combine([(blk(rb, kb).astype(_F32), sg)
                                    for rb, kb, sg in terms]).astype(_BF16)
                w = wob_s[7 * t + u, _rows(k0, KS), :]
                if z is not None and k0 == 0 and u == _ORDER[1]:
                    w = _tie(w, {0: jnp.concatenate([z, z], axis=1)})
                d = _dot(lhs, _as_bf16(w))
                tiles.append((d, 0, 0))
                acc = d if acc is None else acc + d
            ps[u] = acc
        c11, c12, c21, c22 = _strassen_c(ps)
        return jnp.concatenate([jnp.concatenate([c11, c12], axis=1),
                                jnp.concatenate([c21, c22], axis=1)], axis=0)

    def o_body(j, top2):
        r0 = pl.multiple_of(j * TQ, TQ)

        @pl.when(j > 1)
        def _():
            out_copy(2 * j - 4).start()

        @pl.when(j > 1)
        def _():
            out_copy(2 * j - 3).start()

        rh = pl.multiple_of(j * (TQ // 2), TQ // 2)
        left, right = pl.ds(0, M // 2), pl.ds(M // 2, M // 2)

        def residual(dst, rows0, cols, att):
            hb = (x_raw[pl.ds(rows0, HT), cols].astype(_F32) + att).astype(_BF16)
            h_s[pl.ds(rows0, HT), cols] = hb
            dst[:, cols] = hb.astype(_F32)

        gp = jnp.maximum(2 * j - 2, 0)
        tl = []
        m3 = prod(rh, 2, tl)
        m4 = prod(rh, 3, tl)
        top2 = epilogue(gp, ht_s, top2, _pacer(tl[:len(tl) * 7 // 8], NPC, 1), j > 0)
        tl = []
        m5 = prod(rh, 4, tl, _zero_of(top2[0]))
        residual(ht_s, r0, right, m3 + m5)
        m1 = prod(rh, 0, tl)
        m7 = prod(rh, 6, tl)
        residual(ht_s, r0, left, m4 - m5 + m1 + m7)
        top2 = epilogue(gp + 1, hb_s, top2, _pacer(tl[:len(tl) * 7 // 8], NPC), j > 0)
        m2 = prod(rh, 1, tl, _zero_of(top2[0]))
        residual(hb_s, r0 + HT, left, m4 + m2)
        m6 = prod(rh, 5, tl)
        residual(hb_s, r0 + HT, right, m3 + m1 - m2 + m6)
        return top2

    for n in range(3):
        ffn_wait(n)
    with jax.named_scope('o_loop'):
        top2 = lax.fori_loop(0, NB, o_body, (jnp.zeros((8, HT), _F32),) * 2)
    rest = ((NG - 2, ht_s), (NG - 1, hb_s))
    out_copy(NG - 4).start()
    out_copy(NG - 3).start()
    for g, src in rest:
        top2 = epilogue(g, src, top2)

    best, second = top2
    k1 = jnp.max(best, axis=0, keepdims=True)
    k2 = jnp.max(jnp.where(best == k1, second, best), axis=0, keepdims=True)

    R = _FIX
    row = lax.broadcasted_iota(_I32, (2 * R, HT), 0)
    idx = S - 1 - (pltpu.bitcast(jnp.where(row < R, k1, k2), _I32) & (2 ** _IDX_BITS - 1))
    i1 = jnp.clip(idx[0, 0], 0, S - 1)
    i2 = jnp.clip(idx[R, 0], 0, S - 1)
    b1 = pl.multiple_of(i1 & -R, R)
    b2 = pl.multiple_of(i2 & -R, R)
    tokr = jnp.where(row < R, b1 + row, b2 + row - R)
    cd = (((pltpu.bitcast(jnp.where(tokr == i1, k1, k2), _I32) - _KEY_BIAS) >> _IDX_BITS) << 16)
    score = pltpu.bitcast(jnp.where(cd < 0, cd ^ 0x7FFF0000, cd), _F32)
    gate = _round_bf16(1.0 / (1.0 + jnp.exp(-score)))
    gate = jnp.concatenate([gate] * (M // HT), axis=1)
    tokr = jnp.concatenate([tokr] * (M // HT), axis=1)

    hnsel = jnp.concatenate([hn_s[pl.ds(b1, R), :].astype(_F32),
                             hn_s[pl.ds(b2, R), :].astype(_F32)], axis=0)
    xs = hnsel.astype(_BF16)
    g = _dot(xs, wg_s[...])
    u = _dot(xs, wu_s[...])
    pace = _pacer([(mat, 0, c0) for mat in (g, u) for c0 in range(0, F, HT)], len(rest) * NPC)
    for k, (gi, src) in enumerate(rest):
        for n, c in enumerate(range(0, HT, 8)):
            rows = pl.ds(gi * HT + c, 8)
            z = pltpu.bitcast(pace(k * NPC + n)[:8], _F32)
            z = jnp.concatenate([z] * (M // HT), axis=1)
            out_s[rows, :] = (src[pl.ds(c, 8), :] + z + hn_s[rows, :].astype(_F32)).astype(_BF16)
        out_copy(gi).start()
    g = _round_bf16(g)
    u = _round_bf16(u)
    g = _round_bf16(g * (1.0 / (1.0 + jnp.exp(-g))))
    act = (g * u).astype(_BF16)
    y = _round_bf16(_round_bf16(_dot(act, wd_s[:, pl.ds(0, M)])) * gate)
    upd = jnp.where(jnp.logical_or(tokr == i1, tokr == i2), y, 0.0)
    hsel = jnp.concatenate([h_s[pl.ds(b1, R), :].astype(_F32),
                            h_s[pl.ds(b2, R), :].astype(_F32)], axis=0)
    fixed = hsel + _round_bf16(hnsel + upd)

    pltpu.make_async_copy(out_s, out_hbm, sem_out.at[0]).wait()

    def fix_copy(b0, k):
        return pltpu.make_async_copy(out_s.at[pl.ds(b0, R), :],
                                     out_hbm.at[pl.ds(b0, R), :], sem_out.at[k])

    out_s[pl.ds(b1, R), :] = fixed[:R].astype(_BF16)
    out_s[pl.ds(b2, R), :] = fixed[R:].astype(_BF16)
    fix_copy(b1, 0).start()

    @pl.when(b2 != b1)
    def _():
        fix_copy(b2, 1).start()
        fix_copy(b2, 1).wait()

    fix_copy(b1, 0).wait()


@jax.jit
def pallas_sequential_preLN__compressed_kv_cla__moe_arch_mod__prompt_kernel(
    A_x: jax.Array,
    A_c_kv: jax.Array,
    A_w_q: jax.Array,
    A_w_uk: jax.Array,
    A_w_uv: jax.Array,
    A_w_o: jax.Array,
    B_x: jax.Array,
    B_w_r: jax.Array,
    B_w_gate: jax.Array,
    B_w_up: jax.Array,
    B_w_down: jax.Array,
):
    B, S, M = A_x.shape
    DC = A_c_kv.shape[2]
    H, D = A_w_q.shape[1], A_w_q.shape[2]
    F = B_w_gate.shape[1]
    assert (B, S, M, DC, H, D) == (1, 8 * _TQ, 1024, 512, 32, _HT) and A_c_kv.shape[1] == S
    assert F % (8 * H) == 0 and S <= 2 ** _IDX_BITS

    scratch = [
        pltpu.VMEM((S, M), _BF16),
        pltpu.VMEM((S, DC), _BF16),
        pltpu.VMEM((S, M + _PAD), _F32),
        pltpu.VMEM((7, S // 2, DC // 2), _F32),
        pltpu.VMEM((4, S // 2, D), _U32),
        pltpu.VMEM((2, S // 2, D), _U32),
        pltpu.VMEM((2, S // 2, D), _U32),
        pltpu.VMEM((4, M, D), _U32),
        pltpu.VMEM((2, 2, DC, D), _U32),
        pltpu.VMEM((2, 49, M // 8, D), _U32),
        pltpu.VMEM((49, DC // 8, D), _U32),
        pltpu.VMEM((H, S // 2, D), _U32),
        pltpu.VMEM((2, 4, D // 2, M), _BF16),
        pltpu.VMEM((49, H * D // 8, M // 4), _U32),
        pltpu.VMEM((M, F), _BF16),
        pltpu.VMEM((M, F), _BF16),
        pltpu.VMEM((F, M + _PAD), _BF16),
        pltpu.VMEM((_HT, M), _F32),
        pltpu.VMEM((_HT, M), _F32),
        pltpu.VMEM((S, M), _BF16),
        pltpu.VMEM((S, M), _BF16),
        pltpu.VMEM((1024, _HT), _U32),
        pltpu.VMEM((S, M), _BF16),
        pltpu.VMEM((M,), _BF16),
        pltpu.SemaphoreType.DMA((S // _TQ,)),
        pltpu.SemaphoreType.DMA((S // _TQ // 2,)),
        pltpu.SemaphoreType.DMA((2,)),
        pltpu.SemaphoreType.DMA((4,)),
        pltpu.SemaphoreType.DMA((2,)),
        pltpu.SemaphoreType.DMA((4,)),
        pltpu.SemaphoreType.DMA((2,)),
    ]
    any_spec = pl.BlockSpec(memory_space=pl.ANY)
    out = pl.pallas_call(
        functools.partial(_kernel, S=S, M=M, DC=DC, H=H, D=D, F=F),
        in_specs=[any_spec] * 10,
        out_specs=any_spec,
        out_shape=jax.ShapeDtypeStruct((S, M), _BF16),
        scratch_shapes=scratch,
        compiler_params=pltpu.CompilerParams(vmem_limit_bytes=124 * 1024 * 1024,
                                             disable_bounds_checks=True,
                                             disable_semaphore_checks=True),
        name="fused_mla_mod",
    )(A_x.reshape(S, M), A_c_kv.reshape(S, DC), A_w_q, A_w_uk, A_w_uv,
      A_w_o.reshape(H * D, M), B_w_r, B_w_gate, B_w_up, B_w_down)
    return out.reshape(B, S, M)
```

```python
import functools
import math

import jax
import jax.numpy as jnp
from jax import lax
import jax.experimental.pallas as pl
import jax.experimental.pallas.tpu as pltpu

_F32 = jnp.float32
_BF16 = jnp.bfloat16
_U32 = jnp.uint32
_I32 = jnp.int32

_EPS = 1e-5
_NEG = -1e30
_TQ = 256
_HT = 128
_QT = 64
_IDX_BITS = 13
_KEY_BIAS = 0x30000000
_FIX = 8
_PAD = 128


def _dot(a, b):
    return jnp.dot(a, b, preferred_element_type=_F32)


def _dot_nt(a, b):
    return lax.dot_general(a, b, (((1,), (1,)), ((), ())), preferred_element_type=_F32)


def _as_bf16(u):
    return pltpu.bitcast(u, _BF16)


def _pack(x):
    return pltpu.bitcast(x.astype(_BF16), _U32)


def _rows(r0, n):
    if isinstance(r0, int):
        return pl.ds(r0 // 2, n // 2)
    return pl.ds(pl.multiple_of(r0 // 2, 8), n // 2)


def _ld(ref, lead, r0, n):
    return _as_bf16(ref[lead, _rows(r0, n), :])


def _st(ref, lead, r0, x, cols=slice(None)):
    ref[lead, _rows(r0, x.shape[0]), cols] = _pack(x)


def _round_bf16(x):
    return x.astype(_BF16).astype(_F32)


def _zero_of(v):
    return (pltpu.bitcast(v, _U32) >> 16) >> 16


def _lo_hi(w):
    return (pltpu.bitcast(w << 16, _F32), pltpu.bitcast(w & jnp.uint32(0xFFFF0000), _F32))


def _row_stats(x):
    n = x.shape[-1]
    mean = jnp.sum(x, axis=-1, keepdims=True) * (1.0 / n)
    xc = x - mean
    return mean, xc, jnp.sum(xc * xc, axis=-1, keepdims=True) * (1.0 / n)


def _layernorm(x):
    mean, _, var = _row_stats(x)
    den = _round_bf16(jnp.sqrt(_round_bf16(_round_bf16(var) + _EPS)))
    return (x - _round_bf16(mean)) * pl.reciprocal(den, approx=True)


def _layernorm_scaled(x, scale):
    _, xc, var = _row_stats(x)
    return xc * (lax.rsqrt(var + _EPS) * scale)


_SA = (((0, 1), (3, 1)), ((2, 1), (3, 1)), ((0, 1),), ((3, 1),),
       ((0, 1), (1, 1)), ((2, 1), (0, -1)), ((1, 1), (3, -1)))
_SB = (((0, 1), (3, 1)), ((0, 1),), ((1, 1), (3, -1)), ((2, 1), (0, -1)),
       ((3, 1),), ((0, 1), (1, 1)), ((2, 1), (3, 1)))
_ORDER = (2, 4, 3, 1, 0, 6, 5)


def _combine(terms):
    terms = sorted(terms, key=lambda ts: -ts[1])
    assert terms[0][1] > 0
    acc = terms[0][0]
    for v, sg in terms[1:]:
        acc = acc + v if sg > 0 else acc - v
    return acc


def _operands(table, quad):
    return [_combine([(quad[q], sg) for q, sg in terms]) for terms in table]


def _strassen_c(m):
    m1, m2, m3, m4, m5, m6, m7 = m
    return (m4 - m5 + m1 + m7, m3 + m5, m4 + m2, m3 - m2 + m1 + m6)


def _sub(q1, q2):
    return 2 * (q1 // 2) + q2 // 2, 2 * (q1 % 2) + q2 % 2


def _pacer(tiles, total, free=0):
    def zero(n):
        if n < free:
            return jnp.zeros((16, _HT), _U32)
        mat, r, c = tiles[(n - free) * len(tiles) // (total - free)]
        z = _zero_of(mat[r:r + 8, c:c + _HT])
        return jnp.concatenate([z, z], axis=0)
    return zero


def _head(tiles, sixteenths):
    return tiles[:len(tiles) * sixteenths // 16]


def _tie(w, ties):
    parts, at = [], 0
    for r in sorted(ties):
        if r > at:
            parts.append(w[at:r])
        parts.append(w[r:r + 8] | ties[r])
        at = r + 8
    if at < w.shape[0]:
        parts.append(w[at:])
    return parts[0] if len(parts) == 1 else jnp.concatenate(parts, axis=0)


def _add_zero(x, z):
    return jnp.concatenate([x[:, :_HT] + pltpu.bitcast(z, _F32), x[:, _HT:]], axis=1)


def _kernel(x_hbm, c_hbm, wq_hbm, wk_hbm, wv_hbm, wo_hbm, wr_hbm, wg_hbm, wu_hbm, wd_hbm,
            out_hbm,
            x_raw, c_raw, xn_s, ca_s, q_s, k_s, v_s, sa_s, sb_s,
            wq_p, wkv_p, wqb_s, wkvb_s,
            ctx_s, wo_p, wob_s, wg_s, wu_s, wd_s, ht_s, hb_s, h_s, hn_s, junk_s, out_s, wr_s,
            sem_x, sem_c, sem_w, sem_wq, sem_wo, sem_ffn, sem_out,
            *, S, M, DC, H, D, F):
    TQ, HT, QT = _TQ, _HT, _QT
    NB = S // TQ
    NH = NB // 2
    NG = S // HT
    NP = H // 2
    KQ, MQ = DC // 4, M // 4
    KO, NO = H * D // 4, M // 4
    OS = KO // NP
    qscale = (D ** -0.5) * math.log2(math.e)

    wq32 = wq_hbm.bitcast(_U32)
    wk32 = wk_hbm.bitcast(_U32)
    wv32 = wv_hbm.bitcast(_U32)

    def w_start(pair, slot):
        for k, src in enumerate((wk32, wv32)):
            pltpu.make_async_copy(src.at[:, pair, :], wkv_p.at[slot, k], sem_w.at[slot]).start()

    def w_wait(slot):
        pltpu.make_async_copy(wkv_p.at[slot], wkv_p.at[slot], sem_w.at[slot]).wait()

    def wq_copy(pair):
        return pltpu.make_async_copy(wq32.at[:, pair, :], wq_p.at[pair & 3],
                                     sem_wq.at[pair & 3])

    def wo_start(t, slot):
        r0 = pl.multiple_of(t * OS, OS)
        for k in range(4):
            pltpu.make_async_copy(wo_hbm.at[pl.ds(k * KO + r0, OS), :],
                                  wo_p.at[slot, k], sem_wo.at[slot]).start()

    def wo_wait(slot):
        pltpu.make_async_copy(wo_p.at[slot], wo_p.at[slot], sem_wo.at[slot]).wait()

    def x_copy(n):
        rows = pl.ds(pl.multiple_of(((n + NH) % NB) * TQ, TQ), TQ)
        return pltpu.make_async_copy(x_hbm.at[rows, :], x_raw.at[rows, :], sem_x.at[n])

    def c_copy(i):
        rows = pl.ds(pl.multiple_of(i * 2 * TQ, 2 * TQ), 2 * TQ)
        return pltpu.make_async_copy(c_hbm.at[rows, :], c_raw.at[rows, :], sem_c.at[i])

    ffn = ((wg_hbm, wg_s), (wu_hbm, wu_s), (wd_hbm, wd_s))

    def ffn_start(t):
        for n, (src, dst) in enumerate(ffn):
            rows, cols = src.shape[0] // NP, src.shape[1]
            r0 = pl.multiple_of(t * rows, 16)
            pltpu.make_async_copy(src.at[pl.ds(r0, rows), :],
                                  dst.at[pl.ds(r0, rows), pl.ds(0, cols)],
                                  sem_ffn.at[n]).start()

    def ffn_wait(n):
        src, dst = ffn[n]
        pltpu.make_async_copy(src, dst.at[:, pl.ds(0, src.shape[1])], sem_ffn.at[n]).wait()

    wr_copy = pltpu.make_async_copy(wr_hbm, wr_s, sem_ffn.at[3])

    def out_copy(g):
        rows = pl.ds(pl.multiple_of(g * HT, HT), HT)
        return pltpu.make_async_copy(out_s.at[rows, :], out_hbm.at[rows, :], sem_out.at[0])

    def prep_w4(srcs, dst, kq, rows, pace, sink=None):
        pieces = [(t, r) for t in range(7) for r in rows]
        for n, (t, r) in enumerate(pieces):
            terms = [[] for _ in range(4)]
            for k, (q1, sg) in enumerate(_SB[t]):
                for rb in range(2):
                    w = srcs[q1 % 2][pl.ds((2 * (q1 // 2) + rb) * kq + r, 16), :]
                    if k == 0:
                        w = w | pace(n)
                    lo, hi = _lo_hi(w)
                    terms[2 * rb].append((lo, sg))
                    terms[2 * rb + 1].append((hi, sg))
            z = None
            for u, b in enumerate(_operands(_SB, [_combine(tm) for tm in terms])):
                pk = _pack(b)
                dst[7 * t + u, pl.ds(r // 2, 8), :] = pk
                z = pk if z is None else z | pk
            if sink is not None:
                junk_s[pl.ds(8 * (sink + n), 8), :] = z

    def prep_wq(raw, slot, r, nr, pace, sink=None):
        span = 3 * MQ + nr
        prep_w4((wq_p.at[raw, pl.ds(r, span), :], wq_p.at[raw + 1, pl.ds(r, span), :]),
                wqb_s.at[slot, :, pl.ds(pl.multiple_of(r // 2, 8), nr // 2), :],
                MQ, range(0, nr, 16), pace, sink)

    def prep_wo(slot, src0, nrows, dst0, tiles):
        pieces = [(r, c0, t) for r in range(0, nrows, 16) for c0 in range(0, NO, HT)
                  for t in range(7)]
        pace = _pacer(tiles, len(pieces))
        for n, (r, c0, t) in enumerate(pieces):
            z = pltpu.bitcast(pace(n), _F32)
            sub = []
            for q2 in range(4):
                v = _combine([
                    (wo_p[slot, _sub(q1, q2)[0], pl.ds(src0 + r, 16),
                          pl.ds(_sub(q1, q2)[1] * NO + c0, HT)].astype(_F32), sg)
                    for q1, sg in _SB[t]])
                sub.append(v + z if q2 in (0, 3) else v)
            for u, b in enumerate(_operands(_SB, sub)):
                _st(wob_s, 7 * t + u, dst0 + r, b, pl.ds(c0, HT))

    def fence():
        junk_s[pl.ds(0, 8), :] = jnp.zeros((8, HT), _U32)

    def project4(lhs, w, store, zs=()):
        at = {48 * (k + 1) // len(zs): z for k, z in enumerate(zs)}
        m, tiles = [None] * 7, []
        for nt, t in enumerate(_ORDER):
            ps = [None] * 7
            for nu, u in enumerate(_ORDER):
                fence()
                a = lhs(t, u)
                wt = w[7 * t + u]
                if 7 * nt + nu in at:
                    wt = _tie(wt, {0: at[7 * nt + nu]})
                ps[u] = _dot(a.astype(_BF16), _as_bf16(wt))
                tiles += [(ps[u], r, 0) for r in range(0, QT, QT * D // (2 * a.shape[1]))]
            m[t] = _strassen_c(ps)
        for q2 in range(4):
            for q1, cblk in enumerate(_strassen_c([mt[q2] for mt in m])):
                store(_sub(q1, q2)[1], _sub(q1, q2)[0] * QT, cblk)
        return tiles

    def project_q(xn, wqb, q, r0):
        def lhs(t, u):
            return _combine([
                (xn[pl.ds(r0 + _sub(q1, q2)[0] * QT, QT), pl.ds(_sub(q1, q2)[1] * MQ, MQ)],
                 s1 * s2) for q1, s1 in _SA[t] for q2, s2 in _SA[u]])
        return project4(lhs, wqb, lambda nb, r, val: _st(q, nb, r0 + r, val))

    def project_kv(j, zs=()):
        def lhs(t, u):
            return _combine([
                (ca_s[t, pl.ds(j * HT + (q2 // 2) * QT, QT), pl.ds((q2 % 2) * KQ, KQ)], sg)
                for q2, sg in _SA[u]])
        return project4(lhs, wkvb_s,
                        lambda nb, r, val: _st((k_s, v_s)[nb // 2], nb % 2, j * TQ + r, val), zs)

    def stage_x(r0, xn, x0, pace):
        done = []
        for n, c in enumerate(range(0, TQ, 8)):
            z = pace(n)[:8]
            if n >= 6:
                z = z | done[n - 6]
            y = _layernorm_scaled(_add_zero(x_raw[pl.ds(r0 + c, 8), :].astype(_F32), z), qscale)
            xn[pl.ds(x0 + c, 8), pl.ds(0, M)] = y
            done.append(_zero_of(y[:, :HT]))

    def stage_c(r0, a0, pace):
        kh = DC // 2
        for n, c in enumerate(range(0, HT, 8)):
            top = c_raw[pl.ds(r0 + c, 8), :].astype(_F32)
            bot = c_raw[pl.ds(r0 + HT + c, 8), :].astype(_F32)
            z = pltpu.bitcast(pace(n)[:8], _F32)
            z = jnp.concatenate([z] * (kh // HT), axis=1)
            quad = (top[:, :kh] + z, top[:, kh:], bot[:, :kh], bot[:, kh:] + z)
            for t, a in enumerate(_operands(_SA, quad)):
                ca_s[t, pl.ds(a0 + c, 8), :] = a

    def issue(n, carry):
        @pl.when(n == 0)
        def _():
            w_start(0, 0)

        @pl.when(n < NH)
        def _():
            c_copy(n).start()

        @pl.when(jnp.logical_or(n == NH, n == NH + 2))
        def _():
            wq_copy(n - NH).start()
            wq_copy(n - NH + 1).start()

        @pl.when(n < NB)
        def _():
            x_copy(n).start()

        @pl.when(n == NB)
        def _():
            w_start(1, 1)
            wo_start(0, 0)
        return carry

    lax.fori_loop(0, NB + 1, issue, 0)
    ht_s[...] = jnp.zeros((HT, M), _F32)
    hb_s[...] = jnp.zeros((HT, M), _F32)
    w_wait(0)
    c_copy(0).wait()
    x_copy(0).wait()

    def pro_a(i, carry):
        r0 = pl.multiple_of(i * 2 * TQ, 2 * TQ)
        wkv = jnp.concatenate(_lo_hi(wkv_p[0, 0]) + _lo_hi(wkv_p[0, 1]), axis=1).astype(_BF16)
        kv = _dot(c_raw[pl.ds(r0, 2 * TQ), :], wkv)
        for nb in range(4):
            _st((k_s, v_s)[nb // 2], nb % 2, r0, kv[:, nb * D:(nb + 1) * D])
        tiles = [(kv, r, nb * D) for nb in range(4) for r in range(0, 2 * TQ, 8)]
        nt = len(tiles)
        a0 = pl.multiple_of(i * TQ, TQ)
        stage_c(r0, a0, _pacer(tiles[:nt // 2], HT // 8))
        stage_c(r0 + TQ, a0 + HT, _pacer(tiles[nt // 2:nt * 15 // 16], HT // 8))
        rx = pl.multiple_of((i + NH) * TQ, TQ)
        stage_x(rx, xn_s, rx, _pacer(tiles[:nt * 13 // 16], TQ // 8))

        @pl.when(i + 1 < NH)
        def _():
            c_copy(i + 1).wait()

        x_copy(i + 1).wait()
        return carry

    def pro_b(i, carry):
        r0 = pl.multiple_of(i * TQ, TQ)
        xn = xn_s.at[pl.ds(r0, S // 2 + TQ), :]
        kh = M // 2
        lhs = [xn[pl.ds(S // 2, TQ), pl.ds(k0, kh)].astype(_BF16) for k0 in (0, kh)]
        tiles = []
        for nb in range(4):
            d = [_dot(lhs[k], _lo_hi(wq_p[nb // 2, pl.ds(k * kh, kh), :])[nb % 2].astype(_BF16))
                 for k in range(2)]
            _st(q_s, nb, r0 + S // 2, d[0] + d[1])
            tiles += [(dk, r, 0) for dk in d for r in range(0, TQ, 8)]
        stage_x(r0, xn, 0, _pacer(tiles[:len(tiles) * 13 // 16], TQ // 8))
        nr = MQ // (2 * NH)
        npc = 7 * nr // 16
        pace = _pacer(tiles, 3 * npc)
        for k in range(3):
            u = 3 * i + k
            quad = u // (2 * NH)
            prep_wq(2 * quad, quad, pl.multiple_of((u % (2 * NH)) * nr, nr), nr,
                    lambda n, k=k: pace(k * npc + n))

        @pl.when(i == 1)
        def _():
            wq_copy(2).wait()
            wq_copy(3).wait()

        @pl.when(i + 1 < NH)
        def _():
            x_copy(NH + i + 1).wait()

        return carry

    with jax.named_scope('pro_a'):
        lax.fori_loop(0, NH, pro_a, 0)
    wq_copy(0).wait()
    wq_copy(1).wait()
    with jax.named_scope('pro_b'):
        lax.fori_loop(0, NH, pro_b, 0)

    w_start(2, 0)
    wo_start(1, 1)
    wq_copy(4).start()
    wq_copy(5).start()
    ffn_start(NP - 1)
    wr_copy.start()
    w_wait(1)
    wo_wait(0)

    col = lax.broadcasted_iota(_I32, (QT, HT), 1)
    tri = col <= lax.broadcasted_iota(_I32, (QT, HT), 0) + QT
    tri0 = col <= lax.broadcasted_iota(_I32, (QT, HT), 0)

    def staging(t):
        off = pl.multiple_of((t >> 8) * 32, 32)
        return [r.at[pl.ds(off, TQ), :] for r in (sa_s, sb_s)]

    def softmax_rows(s, m):
        p = jnp.exp2(s - m)
        nt = p.shape[1] // HT
        tiles, acc, grp = [], None, None
        for j in range(nt):
            pj = p[:, j * HT:(j + 1) * HT]
            grp = pj if grp is None else grp + pj
            if j % 4 == 3 or j == nt - 1:
                if j % 4 > 0:
                    pj = jnp.minimum(pj, grp)
                acc = grp if acc is None else acc + grp
                grp = None
            tiles.append(pj)
        return (tiles[0] if nt == 1 else jnp.concatenate(tiles, axis=1)), acc

    def scores(q, e, i, buf, c0, zs=()):
        L0, Lm = i * TQ, i * TQ + HT

        def q_group(g):
            return _as_bf16(jnp.concatenate([q[e, _rows(L0 + g * QT, QT), :],
                                             q[e, _rows(L0 + HT + g * QT, QT), :]], axis=0))

        main, tiles = [[], []], []
        for g in (1, 0):
            k0, n = (1 - g) * QT, L0 + g * HT
            if n > 0:
                ties = {}
                if g == 0:
                    ties = {(k * (n // HT) // len(zs)) * QT + 8 * k: z for k, z in enumerate(zs)}
                m = _dot_nt(q_group(g), _as_bf16(_tie(k_s[e, _rows(k0, n), :], ties)))
                main[g] = [m]
                tiles += [(m, t0 % HT, (t0 // HT) * 4 * HT) for t0 in range(0, n // 4, 8)]
        left = _dot_nt(_ld(k_s, e, 0, QT), q_group(0))
        left = jnp.concatenate([left, jnp.full((QT, HT), _NEG, _F32)], axis=0).T
        last = [_dot_nt(_ld(q, e, L0 + HT + g * QT, QT), _ld(k_s, e, L0 + QT + g * QT, HT))
                for g in range(2)]
        main[0] = [left] + main[0]
        ms = [None] * 4
        for g, m in enumerate(main):
            sm = m[0] if len(m) == 1 else jnp.concatenate(m, axis=1)
            one = [jnp.where(tri0 if g == 0 and i == 0 else tri, sm[:QT, Lm - HT:], _NEG)]
            if Lm > HT:
                one = [sm[:QT, :Lm - HT]] + one
            for h, parts in enumerate((one, [sm[QT:], jnp.where(tri, last[g], _NEG)])):
                sh = parts[0] if len(parts) == 1 else jnp.concatenate(parts, axis=1)
                buf[pl.ds((2 * g + h) * QT, QT), pl.ds(c0, sh.shape[1])] = sh
                ms[2 * g + h] = jnp.max(sh, axis=1, keepdims=True)
        return (buf, c0, ms), tiles

    def context(e, head, i, buf, c0, ms):
        Lm = i * TQ + HT
        os_, ls = [None] * 4, [None] * 4
        for g in (1, 0):
            if g == 1:
                v_main = v_s[e, _rows(0, Lm), :]
            else:
                v_main = v_s[e, _rows(0, HT), :]
                if i > 0:
                    v_main = jnp.concatenate([v_main, v_s[e, _rows(QT, Lm - HT), :]], axis=0)
            v_last = _ld(v_s, e, Lm - (1 - g) * QT, HT)
            p1, ls[g] = softmax_rows(buf[pl.ds(2 * g * QT, QT), pl.ds(c0, Lm)], ms[2 * g])
            p2, ls[2 + g] = softmax_rows(buf[pl.ds((2 * g + 1) * QT, QT), pl.ds(c0, Lm + HT)],
                                         ms[2 * g + 1])
            o = _dot(jnp.concatenate([p1, p2[:, :Lm]], axis=0).astype(_BF16), _as_bf16(v_main))
            os_[g] = o[:QT]
            os_[2 + g] = o[QT:] + _dot(p2[:, Lm:].astype(_BF16), v_last)
        o = jnp.concatenate(os_, axis=0)
        acc = jnp.concatenate(ls, axis=0)

        def normalize(pace=None, n0=0):
            z = None
            for n, g in enumerate(range(0, TQ, 16)):
                a = acc[g:g + 16]
                if pace is not None:
                    a = a + pltpu.bitcast(pace(n0 + n), _F32)
                linv = jnp.broadcast_to(
                    pl.reciprocal(jnp.sum(a, axis=1, keepdims=True), approx=True), (16, D))
                ctx_s.at[head][_rows(i * TQ + g, 16), :] = _pack(o[g:g + 16] * linv)
                bits = pltpu.bitcast(linv, _U32)
                bits = bits[:8] | bits[8:]
                z = bits if z is None else z | bits
            return _zero_of(z)
        return normalize

    def pair_body(s, carry):
        odd = s & 1
        slot = 1 - odd
        wo0 = pl.multiple_of(s * OS, OS)
        q_rd = q_s.at[pl.ds(2 * odd, 2)]
        q_wr = q_s.at[:, pl.ds(pl.multiple_of(odd * (S // 4), S // 4), S // 4), :]
        xn = xn_s.at[pl.ds(pl.multiple_of(odd * (S // 2), S // 2), S // 2), :]
        quad = (s + 1) >> 1
        wqb = wqb_s.at[quad & 1]
        pend, sc = {}, {}
        bufs = staging(s)

        def norm(i, tiles):
            pace = _pacer(tiles, TQ // 8)
            return [f(pace, k * (TQ // 16)) for k, f in enumerate(pend.pop(i))]

        def qk(i, nrm=None):
            c0 = S // 2 if i < 2 else 0
            sa, ta = scores(q_rd, 0, i, bufs[0], c0)
            zs = ()
            if nrm is not None:
                zs = norm(nrm, _head(ta, 14))
            sb, tb = scores(q_rd, 1, i, bufs[1], c0, zs)
            sc[i] = (sa, sb)
            return [ta, tb]

        def pv(i):
            pend[i] = [context(e, 2 * s + e, i, *sc[i][e]) for e in range(2)]

        kv = project_kv
        tl = {}
        for i in range(7, 3, -1):
            tl[i] = qk(i, i + 2 if i + 2 < NB else None)
            if i == 7:
                prep_wq(2 * (jnp.minimum(quad + 1, NP // 2 - 1) & 1), (quad + 1) & 1,
                        pl.multiple_of((1 - odd) * (MQ // 2), MQ // 2), MQ // 2,
                        _pacer(tl[7][0] + _head(tl[7][1], 14), 7 * MQ // 32), 64)
            project_q(xn, wqb, q_wr, (i - NH) * TQ)
            pv(i)
        prep_w4((wkv_p.at[slot, 0], wkv_p.at[slot, 1]), wkvb_s, KQ, range(0, KQ, 16),
                _pacer(tl[6][0] + _head(tl[6][1], 15), 7 * KQ // 16), 1)
        tl[3] = qk(3, 5)
        qk(0)
        kv(7)
        pv(3)
        pv(0)
        z = norm(4, kv(6))
        qk(2)
        qk(1)
        prep_wo(odd, 0, OS, wo0,
                _head(tl[5][0], 8) + _head(tl[5][1], 15) + tl[4][0] + _head(tl[4][1], 15)
                + tl[3][0] + _head(tl[3][1], 12))
        kv(5, z)
        pv(2)
        pv(1)
        t = kv(4)
        for j, i in ((3, 3), (2, 0), (1, 2), (0, 1)):
            t = kv(j, norm(i, t[8:-8]))

        @pl.when(s + 3 < NP)
        def _():
            w_start(s + 3, slot)

        @pl.when(s + 2 < NP)
        def _():
            wo_start(s + 2, odd)

        @pl.when(s + 6 < NP)
        def _():
            wq_copy(s + 6).start()

        ffn_start(s)

        @pl.when(s + 5 < NP)
        def _():
            wq_copy(s + 5).wait()

        @pl.when(s + 2 < NP)
        def _():
            w_wait(odd)

        wo_wait(slot)

        @pl.when(s == 0)
        def _():
            wq_copy(4).wait()

        return carry

    with jax.named_scope('pair_loop'):
        lax.fori_loop(0, NP - 1, pair_body, 0)

    def last_body(e, carry):
        half = OS // 2
        q_rd = q_s.at[pl.ds(2, 2)]
        bufs = staging(e)
        nxt, tl = scores(q_rd, e, NB - 1, bufs[1], 0)
        prep_wo((NP - 1) % 2, pl.multiple_of(e * half, half), half,
                pl.multiple_of((NP - 1) * OS + e * half, half),
                tl[:96])
        pend = []
        for i in range(NB - 1, -1, -1):
            cur = nxt
            if i > 0:
                nxt, _ = scores(q_rd, e, i - 1, bufs[(i - 1) % 2], 0)
            pend.append(context(e, H - 2 + e, i, *cur))
        for f in pend:
            f()
        return carry

    with jax.named_scope('last_loop'):
        lax.fori_loop(0, 2, last_body, 0)

    wr_copy.wait()
    wr = wr_s[...].astype(_F32).reshape(1, M)
    sub8 = lax.broadcasted_iota(_I32, (8, HT), 0)
    NPC = HT // 8

    def epilogue(g, src, top2, pace=None, valid=None):
        r0 = pl.multiple_of(g * HT, HT)
        best, second = top2
        bits = []
        for n, c in enumerate(range(0, HT, 8)):
            hc = src[pl.ds(c, 8), :]
            if pace is not None:
                z = pace(n)[:8]
                if n >= 3:
                    z = z | pltpu.bitcast(bits[n - 3] & 0xFFFF, _U32)
                hc = _add_zero(hc, z)
            hnb = _layernorm(hc).astype(_BF16)
            hn_s[pl.ds(r0 + c, 8), :] = hnb
            hn = hnb.astype(_F32)
            if pace is not None:
                out_s[pl.ds(r0 + c, 8), :] = (hc + hn).astype(_BF16)
            r = jnp.broadcast_to(jnp.sum(hn * wr, axis=1, keepdims=True), (8, HT))
            rb = pltpu.bitcast(_round_bf16(r) + 0.0, _I32)
            bits.append(rb)
            key = ((jnp.where(rb < 0, rb ^ 0x7FFF0000, rb) >> (16 - _IDX_BITS))
                   + ((_KEY_BIAS + S - 1 - c - r0) - sub8))
            key = pltpu.bitcast(key, _F32)
            if valid is not None:
                key = jnp.where(valid, key, 0.0)
            second = jnp.maximum(second, jnp.minimum(best, key))
            best = jnp.maximum(best, key)
        return best, second

    def prod(rh, t, tiles, z=None):
        KS = 2 * D
        ps = [None] * 7
        for u in _ORDER:
            terms = [_sub(q1, q2) + (s1 * s2,) for q1, s1 in _SA[t] for q2, s2 in _SA[u]]
            fence()
            acc = None
            for k0 in range(0, KO, KS):
                def blk(rb, kb):
                    h0 = (kb * KO + k0) // D
                    return jnp.concatenate(
                        [_as_bf16(ctx_s[h0 + hh, pl.ds(rh + rb * QT // 2, QT // 2), :])
                         for hh in range(KS // D)], axis=1)
                if len(terms) == 1:
                    lhs = blk(terms[0][0], terms[0][1])
                else:
                    lhs = _combine([(blk(rb, kb).astype(_F32), sg)
                                    for rb, kb, sg in terms]).astype(_BF16)
                w = wob_s[7 * t + u, _rows(k0, KS), :]
                if z is not None and k0 == 0 and u == _ORDER[1]:
                    w = _tie(w, {0: jnp.concatenate([z, z], axis=1)})
                d = _dot(lhs, _as_bf16(w))
                tiles.append((d, 0, 0))
                acc = d if acc is None else acc + d
            ps[u] = acc
        c11, c12, c21, c22 = _strassen_c(ps)
        return jnp.concatenate([jnp.concatenate([c11, c12], axis=1),
                                jnp.concatenate([c21, c22], axis=1)], axis=0)

    def o_body(j, top2):
        r0 = pl.multiple_of(j * TQ, TQ)

        @pl.when(j > 1)
        def _():
            out_copy(2 * j - 4).start()

        @pl.when(j > 1)
        def _():
            out_copy(2 * j - 3).start()

        rh = pl.multiple_of(j * (TQ // 2), TQ // 2)
        left, right = pl.ds(0, M // 2), pl.ds(M // 2, M // 2)

        def residual(dst, rows0, cols, att):
            hb = (x_raw[pl.ds(rows0, HT), cols].astype(_F32) + att).astype(_BF16)
            h_s[pl.ds(rows0, HT), cols] = hb
            dst[:, cols] = hb.astype(_F32)

        gp = jnp.maximum(2 * j - 2, 0)
        tl = []
        m3 = prod(rh, 2, tl)
        m4 = prod(rh, 3, tl)
        top2 = epilogue(gp, ht_s, top2, _pacer(tl[:len(tl) * 7 // 8], NPC, 1), j > 0)
        tl = []
        m5 = prod(rh, 4, tl, _zero_of(top2[0]))
        residual(ht_s, r0, right, m3 + m5)
        m1 = prod(rh, 0, tl)
        m7 = prod(rh, 6, tl)
        residual(ht_s, r0, left, m4 - m5 + m1 + m7)
        top2 = epilogue(gp + 1, hb_s, top2, _pacer(tl[:len(tl) * 7 // 8], NPC), j > 0)
        m2 = prod(rh, 1, tl, _zero_of(top2[0]))
        residual(hb_s, r0 + HT, left, m4 + m2)
        m6 = prod(rh, 5, tl)
        residual(hb_s, r0 + HT, right, m3 + m1 - m2 + m6)
        return top2

    for n in range(3):
        ffn_wait(n)
    with jax.named_scope('o_loop'):
        top2 = lax.fori_loop(0, NB, o_body, (jnp.zeros((8, HT), _F32),) * 2)
    rest = ((NG - 2, ht_s), (NG - 1, hb_s))
    out_copy(NG - 4).start()
    out_copy(NG - 3).start()
    for g, src in rest:
        top2 = epilogue(g, src, top2)

    best, second = top2
    k1 = jnp.max(best, axis=0, keepdims=True)
    k2 = jnp.max(jnp.where(best == k1, second, best), axis=0, keepdims=True)

    R = _FIX
    row = lax.broadcasted_iota(_I32, (2 * R, HT), 0)
    idx = S - 1 - (pltpu.bitcast(jnp.where(row < R, k1, k2), _I32) & (2 ** _IDX_BITS - 1))
    i1 = jnp.clip(idx[0, 0], 0, S - 1)
    i2 = jnp.clip(idx[R, 0], 0, S - 1)
    b1 = pl.multiple_of(i1 & -R, R)
    b2 = pl.multiple_of(i2 & -R, R)
    tokr = jnp.where(row < R, b1 + row, b2 + row - R)
    cd = (((pltpu.bitcast(jnp.where(tokr == i1, k1, k2), _I32) - _KEY_BIAS) >> _IDX_BITS) << 16)
    score = pltpu.bitcast(jnp.where(cd < 0, cd ^ 0x7FFF0000, cd), _F32)
    gate = _round_bf16(1.0 / (1.0 + jnp.exp(-score)))
    gate = jnp.concatenate([gate] * (M // HT), axis=1)
    tokr = jnp.concatenate([tokr] * (M // HT), axis=1)

    hnsel = jnp.concatenate([hn_s[pl.ds(b1, R), :].astype(_F32),
                             hn_s[pl.ds(b2, R), :].astype(_F32)], axis=0)
    xs = hnsel.astype(_BF16)
    g = _dot(xs, wg_s[...])
    u = _dot(xs, wu_s[...])
    pace = _pacer([(mat, 0, c0) for mat in (g, u) for c0 in range(0, F, HT)], len(rest) * NPC)
    for k, (gi, src) in enumerate(rest):
        for n, c in enumerate(range(0, HT, 8)):
            rows = pl.ds(gi * HT + c, 8)
            z = pltpu.bitcast(pace(k * NPC + n)[:8], _F32)
            z = jnp.concatenate([z] * (M // HT), axis=1)
            out_s[rows, :] = (src[pl.ds(c, 8), :] + z + hn_s[rows, :].astype(_F32)).astype(_BF16)
        out_copy(gi).start()
    g = _round_bf16(g)
    u = _round_bf16(u)
    g = _round_bf16(g * (1.0 / (1.0 + jnp.exp(-g))))
    act = (g * u).astype(_BF16)
    y = _round_bf16(_round_bf16(_dot(act, wd_s[:, pl.ds(0, M)])) * gate)
    upd = jnp.where(jnp.logical_or(tokr == i1, tokr == i2), y, 0.0)
    hsel = jnp.concatenate([h_s[pl.ds(b1, R), :].astype(_F32),
                            h_s[pl.ds(b2, R), :].astype(_F32)], axis=0)
    fixed = hsel + _round_bf16(hnsel + upd)

    pltpu.make_async_copy(out_s, out_hbm, sem_out.at[0]).wait()

    def fix_copy(b0, k):
        return pltpu.make_async_copy(out_s.at[pl.ds(b0, R), :],
                                     out_hbm.at[pl.ds(b0, R), :], sem_out.at[k])

    out_s[pl.ds(b1, R), :] = fixed[:R].astype(_BF16)
    out_s[pl.ds(b2, R), :] = fixed[R:].astype(_BF16)
    fix_copy(b1, 0).start()

    @pl.when(b2 != b1)
    def _():
        fix_copy(b2, 1).start()
        fix_copy(b2, 1).wait()

    fix_copy(b1, 0).wait()


@jax.jit
def pallas_sequential_preLN__compressed_kv_cla__moe_arch_mod__prompt_kernel(
    A_x: jax.Array,
    A_c_kv: jax.Array,
    A_w_q: jax.Array,
    A_w_uk: jax.Array,
    A_w_uv: jax.Array,
    A_w_o: jax.Array,
    B_x: jax.Array,
    B_w_r: jax.Array,
    B_w_gate: jax.Array,
    B_w_up: jax.Array,
    B_w_down: jax.Array,
):
    B, S, M = A_x.shape
    DC = A_c_kv.shape[2]
    H, D = A_w_q.shape[1], A_w_q.shape[2]
    F = B_w_gate.shape[1]
    assert (B, S, M, DC, H, D) == (1, 8 * _TQ, 1024, 512, 32, _HT) and A_c_kv.shape[1] == S
    assert F % (8 * H) == 0 and S <= 2 ** _IDX_BITS

    scratch = [
        pltpu.VMEM((S, M), _BF16),
        pltpu.VMEM((S, DC), _BF16),
        pltpu.VMEM((S, M + _PAD), _F32),
        pltpu.VMEM((7, S // 2, DC // 2), _F32),
        pltpu.VMEM((4, S // 2, D), _U32),
        pltpu.VMEM((2, S // 2, D), _U32),
        pltpu.VMEM((2, S // 2, D), _U32),
        pltpu.VMEM((_TQ + 32, S + _PAD), _F32),
        pltpu.VMEM((_TQ + 32, S + _PAD), _F32),
        pltpu.VMEM((4, M, D), _U32),
        pltpu.VMEM((2, 2, DC, D), _U32),
        pltpu.VMEM((2, 49, M // 8, D), _U32),
        pltpu.VMEM((49, DC // 8, D), _U32),
        pltpu.VMEM((H, S // 2, D), _U32),
        pltpu.VMEM((2, 4, D // 2, M), _BF16),
        pltpu.VMEM((49, H * D // 8, M // 4), _U32),
        pltpu.VMEM((M, F), _BF16),
        pltpu.VMEM((M, F), _BF16),
        pltpu.VMEM((F, M + _PAD), _BF16),
        pltpu.VMEM((_HT, M), _F32),
        pltpu.VMEM((_HT, M), _F32),
        pltpu.VMEM((S, M), _BF16),
        pltpu.VMEM((S, M), _BF16),
        pltpu.VMEM((1024, _HT), _U32),
        pltpu.VMEM((S, M), _BF16),
        pltpu.VMEM((M,), _BF16),
        pltpu.SemaphoreType.DMA((S // _TQ,)),
        pltpu.SemaphoreType.DMA((S // _TQ // 2,)),
        pltpu.SemaphoreType.DMA((2,)),
        pltpu.SemaphoreType.DMA((4,)),
        pltpu.SemaphoreType.DMA((2,)),
        pltpu.SemaphoreType.DMA((4,)),
        pltpu.SemaphoreType.DMA((2,)),
    ]
    any_spec = pl.BlockSpec(memory_space=pl.ANY)
    out = pl.pallas_call(
        functools.partial(_kernel, S=S, M=M, DC=DC, H=H, D=D, F=F),
        in_specs=[any_spec] * 10,
        out_specs=any_spec,
        out_shape=jax.ShapeDtypeStruct((S, M), _BF16),
        scratch_shapes=scratch,
        compiler_params=pltpu.CompilerParams(vmem_limit_bytes=124 * 1024 * 1024,
                                             disable_bounds_checks=True,
                                             disable_semaphore_checks=True),
        name="fused_mla_mod",
    )(A_x.reshape(S, M), A_c_kv.reshape(S, DC), A_w_q, A_w_uk, A_w_uv,
      A_w_o.reshape(H * D, M), B_w_r, B_w_gate, B_w_up, B_w_down)
    return out.reshape(B, S, M)
```

```python
import functools
import math

import jax
import jax.numpy as jnp
from jax import lax
import jax.experimental.pallas as pl
import jax.experimental.pallas.tpu as pltpu

_F32 = jnp.float32
_BF16 = jnp.bfloat16
_U32 = jnp.uint32
_I32 = jnp.int32

_EPS = 1e-5
_NEG = -1e30
_TQ = 256
_HT = 128
_QT = 64
_IDX_BITS = 13
_KEY_BIAS = 0x30000000
_FIX = 8
_PAD = 128


def _dot(a, b):
    return jnp.dot(a, b, preferred_element_type=_F32)


def _dot_nt(a, b):
    return lax.dot_general(a, b, (((1,), (1,)), ((), ())), preferred_element_type=_F32)


def _as_bf16(u):
    return pltpu.bitcast(u, _BF16)


def _pack(x):
    return pltpu.bitcast(x.astype(_BF16), _U32)


def _rows(r0, n):
    if isinstance(r0, int):
        return pl.ds(r0 // 2, n // 2)
    return pl.ds(pl.multiple_of(r0 // 2, 8), n // 2)


def _ld(ref, lead, r0, n):
    return _as_bf16(ref[lead, _rows(r0, n), :])


def _st(ref, lead, r0, x, cols=slice(None)):
    ref[lead, _rows(r0, x.shape[0]), cols] = _pack(x)


def _round_bf16(x):
    return x.astype(_BF16).astype(_F32)


def _zero_of(v):
    return (pltpu.bitcast(v, _U32) >> 16) >> 16


def _lo_hi(w):
    return (pltpu.bitcast(w << 16, _F32), pltpu.bitcast(w & jnp.uint32(0xFFFF0000), _F32))


def _row_stats(x):
    n = x.shape[-1]
    mean = jnp.sum(x, axis=-1, keepdims=True) * (1.0 / n)
    xc = x - mean
    return mean, xc, jnp.sum(xc * xc, axis=-1, keepdims=True) * (1.0 / n)


def _layernorm(x):
    mean, _, var = _row_stats(x)
    den = _round_bf16(jnp.sqrt(_round_bf16(_round_bf16(var) + _EPS)))
    return (x - _round_bf16(mean)) * pl.reciprocal(den, approx=True)


def _layernorm_scaled(x, scale):
    _, xc, var = _row_stats(x)
    return xc * (lax.rsqrt(var + _EPS) * scale)


_SA = (((0, 1), (3, 1)), ((2, 1), (3, 1)), ((0, 1),), ((3, 1),),
       ((0, 1), (1, 1)), ((2, 1), (0, -1)), ((1, 1), (3, -1)))
_SB = (((0, 1), (3, 1)), ((0, 1),), ((1, 1), (3, -1)), ((2, 1), (0, -1)),
       ((3, 1),), ((0, 1), (1, 1)), ((2, 1), (3, 1)))
_ORDER = (2, 4, 3, 1, 0, 6, 5)


def _combine(terms):
    terms = sorted(terms, key=lambda ts: -ts[1])
    assert terms[0][1] > 0
    acc = terms[0][0]
    for v, sg in terms[1:]:
        acc = acc + v if sg > 0 else acc - v
    return acc


def _operands(table, quad):
    return [_combine([(quad[q], sg) for q, sg in terms]) for terms in table]


def _strassen_c(m):
    m1, m2, m3, m4, m5, m6, m7 = m
    return (m4 - m5 + m1 + m7, m3 + m5, m4 + m2, m3 - m2 + m1 + m6)


def _sub(q1, q2):
    return 2 * (q1 // 2) + q2 // 2, 2 * (q1 % 2) + q2 % 2


def _pacer(tiles, total, free=0):
    def zero(n):
        if n < free:
            return jnp.zeros((16, _HT), _U32)
        mat, r, c = tiles[(n - free) * len(tiles) // (total - free)]
        z = _zero_of(mat[r:r + 8, c:c + _HT])
        return jnp.concatenate([z, z], axis=0)
    return zero


def _head(tiles, sixteenths):
    return tiles[:len(tiles) * sixteenths // 16]


def _tie(w, ties):
    parts, at = [], 0
    for r in sorted(ties):
        if r > at:
            parts.append(w[at:r])
        parts.append(w[r:r + 8] | ties[r])
        at = r + 8
    if at < w.shape[0]:
        parts.append(w[at:])
    return parts[0] if len(parts) == 1 else jnp.concatenate(parts, axis=0)


def _add_zero(x, z):
    return jnp.concatenate([x[:, :_HT] + pltpu.bitcast(z, _F32), x[:, _HT:]], axis=1)


def _kernel(x_hbm, c_hbm, wq_hbm, wk_hbm, wv_hbm, wo_hbm, wr_hbm, wg_hbm, wu_hbm, wd_hbm,
            out_hbm,
            x_raw, c_raw, xn_s, ca_s, q_s, k_s, v_s, sa_s, sb_s,
            wq_p, wkv_p, wqb_s, wkvb_s,
            ctx_s, wo_p, wob_s, wg_s, wu_s, wd_s, ht_s, hb_s, h_s, hn_s, junk_s, out_s, wr_s,
            sem_x, sem_c, sem_w, sem_wq, sem_wo, sem_ffn, sem_out,
            *, S, M, DC, H, D, F):
    TQ, HT, QT = _TQ, _HT, _QT
    NB = S // TQ
    NH = NB // 2
    NG = S // HT
    NP = H // 2
    KQ, MQ = DC // 4, M // 4
    KO, NO = H * D // 4, M // 4
    OS = KO // NP
    qscale = (D ** -0.5) * math.log2(math.e)

    wq32 = wq_hbm.bitcast(_U32)
    wk32 = wk_hbm.bitcast(_U32)
    wv32 = wv_hbm.bitcast(_U32)

    def w_start(pair, slot):
        for k, src in enumerate((wk32, wv32)):
            pltpu.make_async_copy(src.at[:, pair, :], wkv_p.at[slot, k], sem_w.at[slot]).start()

    def w_wait(slot):
        pltpu.make_async_copy(wkv_p.at[slot], wkv_p.at[slot], sem_w.at[slot]).wait()

    def wq_copy(pair):
        return pltpu.make_async_copy(wq32.at[:, pair, :], wq_p.at[pair & 3],
                                     sem_wq.at[pair & 3])

    def wo_start(t, slot):
        r0 = pl.multiple_of(t * OS, OS)
        for k in range(4):
            pltpu.make_async_copy(wo_hbm.at[pl.ds(k * KO + r0, OS), :],
                                  wo_p.at[slot, k], sem_wo.at[slot]).start()

    def wo_wait(slot):
        pltpu.make_async_copy(wo_p.at[slot], wo_p.at[slot], sem_wo.at[slot]).wait()

    def x_copy(n):
        rows = pl.ds(pl.multiple_of(((n + NH) % NB) * TQ, TQ), TQ)
        return pltpu.make_async_copy(x_hbm.at[rows, :], x_raw.at[rows, :], sem_x.at[n])

    def c_copy(i):
        rows = pl.ds(pl.multiple_of(i * 2 * TQ, 2 * TQ), 2 * TQ)
        return pltpu.make_async_copy(c_hbm.at[rows, :], c_raw.at[rows, :], sem_c.at[i])

    ffn = ((wg_hbm, wg_s), (wu_hbm, wu_s), (wd_hbm, wd_s))

    def ffn_start(t):
        for n, (src, dst) in enumerate(ffn):
            rows, cols = src.shape[0] // NP, src.shape[1]
            r0 = pl.multiple_of(t * rows, 16)
            pltpu.make_async_copy(src.at[pl.ds(r0, rows), :],
                                  dst.at[pl.ds(r0, rows), pl.ds(0, cols)],
                                  sem_ffn.at[n]).start()

    def ffn_wait(n):
        src, dst = ffn[n]
        pltpu.make_async_copy(src, dst.at[:, pl.ds(0, src.shape[1])], sem_ffn.at[n]).wait()

    wr_copy = pltpu.make_async_copy(wr_hbm, wr_s, sem_ffn.at[3])

    def out_copy(g):
        rows = pl.ds(pl.multiple_of(g * HT, HT), HT)
        return pltpu.make_async_copy(out_s.at[rows, :], out_hbm.at[rows, :], sem_out.at[0])

    def prep_w4(srcs, dst, kq, rows, pace, sink=None):
        pieces = [(t, r) for t in range(7) for r in rows]
        for n, (t, r) in enumerate(pieces):
            terms = [[] for _ in range(4)]
            for k, (q1, sg) in enumerate(_SB[t]):
                for rb in range(2):
                    w = srcs[q1 % 2][pl.ds((2 * (q1 // 2) + rb) * kq + r, 16), :]
                    if k == 0:
                        w = w | (pace(n) if sink is not None else pace(2 * n + rb))
                    lo, hi = _lo_hi(w)
                    terms[2 * rb].append((lo, sg))
                    terms[2 * rb + 1].append((hi, sg))
            z = None
            for u, b in enumerate(_operands(_SB, [_combine(tm) for tm in terms])):
                pk = _pack(b)
                dst[7 * t + u, pl.ds(r // 2, 8), :] = pk
                z = pk if z is None else z | pk
            if sink is not None:
                junk_s[pl.ds(8 * (sink + n), 8), :] = z

    def prep_wq(raw, slot, r, nr, pace, sink=None):
        span = 3 * MQ + nr
        prep_w4((wq_p.at[raw, pl.ds(r, span), :], wq_p.at[raw + 1, pl.ds(r, span), :]),
                wqb_s.at[slot, :, pl.ds(pl.multiple_of(r // 2, 8), nr // 2), :],
                MQ, range(0, nr, 16), pace, sink)

    def prep_wo(slot, src0, nrows, dst0, tiles):
        pieces = [(r, c0, t) for r in range(0, nrows, 16) for c0 in range(0, NO, HT)
                  for t in range(7)]
        pace = _pacer(tiles, len(pieces))
        for n, (r, c0, t) in enumerate(pieces):
            z = pltpu.bitcast(pace(n), _F32)
            sub = []
            for q2 in range(4):
                v = _combine([
                    (wo_p[slot, _sub(q1, q2)[0], pl.ds(src0 + r, 16),
                          pl.ds(_sub(q1, q2)[1] * NO + c0, HT)].astype(_F32), sg)
                    for q1, sg in _SB[t]])
                sub.append(v + z if q2 in (0, 3) else v)
            for u, b in enumerate(_operands(_SB, sub)):
                _st(wob_s, 7 * t + u, dst0 + r, b, pl.ds(c0, HT))

    def fence():
        junk_s[pl.ds(0, 8), :] = jnp.zeros((8, HT), _U32)

    def project4(lhs, w, store, zs=()):
        at = {48 * (k + 1) // len(zs): z for k, z in enumerate(zs)}
        m, tiles = [None] * 7, []
        for nt, t in enumerate(_ORDER):
            ps = [None] * 7
            for nu, u in enumerate(_ORDER):
                fence()
                a = lhs(t, u)
                wt = w[7 * t + u]
                if 7 * nt + nu in at:
                    wt = _tie(wt, {0: at[7 * nt + nu]})
                ps[u] = _dot(a.astype(_BF16), _as_bf16(wt))
                tiles += [(ps[u], r, 0) for r in range(0, QT, QT * D // (2 * a.shape[1]))]
            m[t] = _strassen_c(ps)
        for q2 in range(4):
            for q1, cblk in enumerate(_strassen_c([mt[q2] for mt in m])):
                store(_sub(q1, q2)[1], _sub(q1, q2)[0] * QT, cblk)
        return tiles

    def project_q(xn, wqb, q, r0):
        def lhs(t, u):
            return _combine([
                (xn[pl.ds(r0 + _sub(q1, q2)[0] * QT, QT), pl.ds(_sub(q1, q2)[1] * MQ, MQ)],
                 s1 * s2) for q1, s1 in _SA[t] for q2, s2 in _SA[u]])
        return project4(lhs, wqb, lambda nb, r, val: _st(q, nb, r0 + r, val))

    def project_kv(j, zs=()):
        def lhs(t, u):
            return _combine([
                (ca_s[t, pl.ds(j * HT + (q2 // 2) * QT, QT), pl.ds((q2 % 2) * KQ, KQ)], sg)
                for q2, sg in _SA[u]])
        return project4(lhs, wkvb_s,
                        lambda nb, r, val: _st((k_s, v_s)[nb // 2], nb % 2, j * TQ + r, val), zs)

    def stage_x(r0, xn, x0, pace):
        done = []
        for n, c in enumerate(range(0, TQ, 8)):
            z = pace(n)[:8]
            if n >= 6:
                z = z | done[n - 6]
            y = _layernorm_scaled(_add_zero(x_raw[pl.ds(r0 + c, 8), :].astype(_F32), z), qscale)
            xn[pl.ds(x0 + c, 8), pl.ds(0, M)] = y
            done.append(_zero_of(y[:, :HT]))

    def stage_c(r0, a0, pace):
        kh = DC // 2
        for n, c in enumerate(range(0, HT, 8)):
            top = c_raw[pl.ds(r0 + c, 8), :].astype(_F32)
            bot = c_raw[pl.ds(r0 + HT + c, 8), :].astype(_F32)
            z = pltpu.bitcast(pace(n)[:8], _F32)
            z = jnp.concatenate([z] * (kh // HT), axis=1)
            quad = (top[:, :kh] + z, top[:, kh:], bot[:, :kh], bot[:, kh:] + z)
            for t, a in enumerate(_operands(_SA, quad)):
                ca_s[t, pl.ds(a0 + c, 8), :] = a

    def issue(n, carry):
        @pl.when(n == 0)
        def _():
            w_start(0, 0)

        @pl.when(n < NH)
        def _():
            c_copy(n).start()

        @pl.when(jnp.logical_or(n == NH, n == NH + 2))
        def _():
            wq_copy(n - NH).start()
            wq_copy(n - NH + 1).start()

        @pl.when(n < NB)
        def _():
            x_copy(n).start()

        @pl.when(n == NB)
        def _():
            w_start(1, 1)
            wo_start(0, 0)
        return carry

    lax.fori_loop(0, NB + 1, issue, 0)
    ht_s[...] = jnp.zeros((HT, M), _F32)
    hb_s[...] = jnp.zeros((HT, M), _F32)
    w_wait(0)
    c_copy(0).wait()
    x_copy(0).wait()

    def pro_a(i, carry):
        r0 = pl.multiple_of(i * 2 * TQ, 2 * TQ)
        wkv = jnp.concatenate(_lo_hi(wkv_p[0, 0]) + _lo_hi(wkv_p[0, 1]), axis=1).astype(_BF16)
        kv = _dot(c_raw[pl.ds(r0, 2 * TQ), :], wkv)
        for nb in range(4):
            _st((k_s, v_s)[nb // 2], nb % 2, r0, kv[:, nb * D:(nb + 1) * D])
        tiles = [(kv, r, nb * D) for nb in range(4) for r in range(0, 2 * TQ, 8)]
        nt = len(tiles)
        a0 = pl.multiple_of(i * TQ, TQ)
        stage_c(r0, a0, _pacer(tiles[:nt // 2], HT // 8))
        stage_c(r0 + TQ, a0 + HT, _pacer(tiles[nt // 2:nt * 15 // 16], HT // 8))
        rx = pl.multiple_of((i + NH) * TQ, TQ)
        stage_x(rx, xn_s, rx, _pacer(tiles[:nt * 13 // 16], TQ // 8))

        @pl.when(i + 1 < NH)
        def _():
            c_copy(i + 1).wait()

        x_copy(i + 1).wait()
        return carry

    def pro_b(i, carry):
        r0 = pl.multiple_of(i * TQ, TQ)
        xn = xn_s.at[pl.ds(r0, S // 2 + TQ), :]
        kh = M // 2
        lhs = [xn[pl.ds(S // 2, TQ), pl.ds(k0, kh)].astype(_BF16) for k0 in (0, kh)]
        tiles = []
        for nb in range(4):
            d = [_dot(lhs[k], _lo_hi(wq_p[nb // 2, pl.ds(k * kh, kh), :])[nb % 2].astype(_BF16))
                 for k in range(2)]
            _st(q_s, nb, r0 + S // 2, d[0] + d[1])
            tiles += [(dk, r, 0) for dk in d for r in range(0, TQ, 8)]
        stage_x(r0, xn, 0, _pacer(tiles[:len(tiles) * 13 // 16], TQ // 8))
        nr = MQ // (2 * NH)
        npc = 7 * nr // 8
        pace = _pacer(tiles, 3 * npc)
        for k in range(3):
            u = 3 * i + k
            quad = u // (2 * NH)
            prep_wq(2 * quad, quad, pl.multiple_of((u % (2 * NH)) * nr, nr), nr,
                    lambda n, k=k: pace(k * npc + n))

        @pl.when(i == 1)
        def _():
            wq_copy(2).wait()
            wq_copy(3).wait()

        @pl.when(i + 1 < NH)
        def _():
            x_copy(NH + i + 1).wait()

        return carry

    with jax.named_scope('pro_a'):
        lax.fori_loop(0, NH, pro_a, 0)
    wq_copy(0).wait()
    wq_copy(1).wait()
    with jax.named_scope('pro_b'):
        lax.fori_loop(0, NH, pro_b, 0)

    w_start(2, 0)
    wo_start(1, 1)
    wq_copy(4).start()
    wq_copy(5).start()
    ffn_start(NP - 1)
    wr_copy.start()
    w_wait(1)
    wo_wait(0)

    col = lax.broadcasted_iota(_I32, (QT, HT), 1)
    tri = col <= lax.broadcasted_iota(_I32, (QT, HT), 0) + QT
    tri0 = col <= lax.broadcasted_iota(_I32, (QT, HT), 0)

    def staging(t):
        off = pl.multiple_of((t >> 8) * 32, 32)
        return [r.at[pl.ds(off, TQ), :] for r in (sa_s, sb_s)]

    def softmax_rows(s, m):
        p = jnp.exp2(s - m)
        nt = p.shape[1] // HT
        tiles, acc, grp = [], None, None
        for j in range(nt):
            pj = p[:, j * HT:(j + 1) * HT]
            grp = pj if grp is None else grp + pj
            if j % 4 == 3 or j == nt - 1:
                if j % 4 > 0:
                    pj = jnp.minimum(pj, grp)
                acc = grp if acc is None else acc + grp
                grp = None
            tiles.append(pj)
        return (tiles[0] if nt == 1 else jnp.concatenate(tiles, axis=1)), acc

    def scores(q, e, i, buf, c0, zs=()):
        L0, Lm = i * TQ, i * TQ + HT

        def q_group(g):
            return _as_bf16(jnp.concatenate([q[e, _rows(L0 + g * QT, QT), :],
                                             q[e, _rows(L0 + HT + g * QT, QT), :]], axis=0))

        main, tiles = [[], []], []
        for g in (1, 0):
            k0, n = (1 - g) * QT, L0 + g * HT
            if n > 0:
                ties = {}
                if g == 0:
                    ties = {(k * (n // HT) // len(zs)) * QT + 8 * k: z for k, z in enumerate(zs)}
                m = _dot_nt(q_group(g), _as_bf16(_tie(k_s[e, _rows(k0, n), :], ties)))
                main[g] = [m]
                tiles += [(m, t0 % HT, (t0 // HT) * 4 * HT) for t0 in range(0, n // 4, 8)]
        left = _dot_nt(_ld(k_s, e, 0, QT), q_group(0))
        left = jnp.concatenate([left, jnp.full((QT, HT), _NEG, _F32)], axis=0).T
        last = [_dot_nt(_ld(q, e, L0 + HT + g * QT, QT), _ld(k_s, e, L0 + QT + g * QT, HT))
                for g in range(2)]
        main[0] = [left] + main[0]
        ms = [None] * 4
        for g, m in enumerate(main):
            sm = m[0] if len(m) == 1 else jnp.concatenate(m, axis=1)
            one = [jnp.where(tri0 if g == 0 and i == 0 else tri, sm[:QT, Lm - HT:], _NEG)]
            if Lm > HT:
                one = [sm[:QT, :Lm - HT]] + one
            for h, parts in enumerate((one, [sm[QT:], jnp.where(tri, last[g], _NEG)])):
                sh = parts[0] if len(parts) == 1 else jnp.concatenate(parts, axis=1)
                buf[pl.ds((2 * g + h) * QT, QT), pl.ds(c0, sh.shape[1])] = sh
                ms[2 * g + h] = jnp.max(sh, axis=1, keepdims=True)
        return (buf, c0, ms), tiles

    def context(e, head, i, buf, c0, ms):
        Lm = i * TQ + HT
        os_, ls = [None] * 4, [None] * 4
        for g in (1, 0):
            if g == 1:
                v_main = v_s[e, _rows(0, Lm), :]
            else:
                v_main = v_s[e, _rows(0, HT), :]
                if i > 0:
                    v_main = jnp.concatenate([v_main, v_s[e, _rows(QT, Lm - HT), :]], axis=0)
            v_last = _ld(v_s, e, Lm - (1 - g) * QT, HT)
            p1, ls[g] = softmax_rows(buf[pl.ds(2 * g * QT, QT), pl.ds(c0, Lm)], ms[2 * g])
            p2, ls[2 + g] = softmax_rows(buf[pl.ds((2 * g + 1) * QT, QT), pl.ds(c0, Lm + HT)],
                                         ms[2 * g + 1])
            o = _dot(jnp.concatenate([p1, p2[:, :Lm]], axis=0).astype(_BF16), _as_bf16(v_main))
            os_[g] = o[:QT]
            os_[2 + g] = o[QT:] + _dot(p2[:, Lm:].astype(_BF16), v_last)
        o = jnp.concatenate(os_, axis=0)
        acc = jnp.concatenate(ls, axis=0)

        def normalize(pace=None, n0=0):
            z = None
            for n, g in enumerate(range(0, TQ, 16)):
                a = acc[g:g + 16]
                if pace is not None:
                    a = a + pltpu.bitcast(pace(n0 + n), _F32)
                linv = jnp.broadcast_to(
                    pl.reciprocal(jnp.sum(a, axis=1, keepdims=True), approx=True), (16, D))
                ctx_s.at[head][_rows(i * TQ + g, 16), :] = _pack(o[g:g + 16] * linv)
                bits = pltpu.bitcast(linv, _U32)
                bits = bits[:8] | bits[8:]
                z = bits if z is None else z | bits
            return _zero_of(z)
        return normalize

    def pair_body(s, carry):
        odd = s & 1
        slot = 1 - odd
        wo0 = pl.multiple_of(s * OS, OS)
        q_rd = q_s.at[pl.ds(2 * odd, 2)]
        q_wr = q_s.at[:, pl.ds(pl.multiple_of(odd * (S // 4), S // 4), S // 4), :]
        xn = xn_s.at[pl.ds(pl.multiple_of(odd * (S // 2), S // 2), S // 2), :]
        quad = (s + 1) >> 1
        wqb = wqb_s.at[quad & 1]
        pend, sc = {}, {}
        bufs = staging(s)

        def norm(i, tiles):
            pace = _pacer(tiles, TQ // 8)
            return [f(pace, k * (TQ // 16)) for k, f in enumerate(pend.pop(i))]

        def qk(i, nrm=None):
            c0 = S // 2 if i < 2 else 0
            sa, ta = scores(q_rd, 0, i, bufs[0], c0)
            zs = ()
            if nrm is not None:
                zs = norm(nrm, _head(ta, 14))
            sb, tb = scores(q_rd, 1, i, bufs[1], c0, zs)
            sc[i] = (sa, sb)
            return [ta, tb]

        def pv(i):
            pend[i] = [context(e, 2 * s + e, i, *sc[i][e]) for e in range(2)]

        kv = project_kv
        tl = {}
        for i in range(7, 3, -1):
            tl[i] = qk(i, i + 2 if i + 2 < NB else None)
            if i == 7:
                prep_wq(2 * (jnp.minimum(quad + 1, NP // 2 - 1) & 1), (quad + 1) & 1,
                        pl.multiple_of((1 - odd) * (MQ // 2), MQ // 2), MQ // 2,
                        _pacer(tl[7][0] + _head(tl[7][1], 14), 7 * MQ // 32), 64)
            project_q(xn, wqb, q_wr, (i - NH) * TQ)
            pv(i)
        prep_w4((wkv_p.at[slot, 0], wkv_p.at[slot, 1]), wkvb_s, KQ, range(0, KQ, 16),
                _pacer(tl[6][0] + _head(tl[6][1], 15), 7 * KQ // 16), 1)
        tl[3] = qk(3, 5)
        qk(0)
        kv(7)
        pv(3)
        pv(0)
        z = norm(4, kv(6))
        qk(2)
        qk(1)
        prep_wo(odd, 0, OS, wo0,
                _head(tl[5][0], 8) + _head(tl[5][1], 15) + tl[4][0] + _head(tl[4][1], 15)
                + tl[3][0] + _head(tl[3][1], 12))
        kv(5, z)
        pv(2)
        pv(1)
        t = kv(4)
        for j, i in ((3, 3), (2, 0), (1, 2), (0, 1)):
            t = kv(j, norm(i, t[8:-8]))

        @pl.when(s + 3 < NP)
        def _():
            w_start(s + 3, slot)

        @pl.when(s + 2 < NP)
        def _():
            wo_start(s + 2, odd)

        @pl.when(s + 6 < NP)
        def _():
            wq_copy(s + 6).start()

        ffn_start(s)

        @pl.when(s + 5 < NP)
        def _():
            wq_copy(s + 5).wait()

        @pl.when(s + 2 < NP)
        def _():
            w_wait(odd)

        wo_wait(slot)

        @pl.when(s == 0)
        def _():
            wq_copy(4).wait()

        return carry

    with jax.named_scope('pair_loop'):
        lax.fori_loop(0, NP - 1, pair_body, 0)

    def last_body(e, carry):
        half = OS // 2
        q_rd = q_s.at[pl.ds(2, 2)]
        bufs = staging(e)
        sc, pend = {}, []
        sc[7], tl = scores(q_rd, e, 7, bufs[1], 0)
        prep_wo((NP - 1) % 2, pl.multiple_of(e * half, half), half,
                pl.multiple_of((NP - 1) * OS + e * half, half), tl[:96])
        for step in "s6 c7 s5 c6 s4 c5 s3 s0 c4 s2 s1 c0 c3 c1 c2".split():
            i = int(step[1])
            if step[0] == "s":
                sc[i], _ = (scores(q_rd, e, i, bufs[i % 2], 0) if i >= 2
                            else scores(q_rd, e, i, bufs[1 - i], S // 2))
            else:
                pend.append(context(e, H - 2 + e, i, *sc[i]))
        for f in pend:
            f()
        return carry

    with jax.named_scope('last_loop'):
        lax.fori_loop(0, 2, last_body, 0)

    wr_copy.wait()
    wr = wr_s[...].astype(_F32).reshape(1, M)
    sub8 = lax.broadcasted_iota(_I32, (8, HT), 0)
    NPC = HT // 8

    def epilogue(g, src, top2, pace=None, valid=None):
        r0 = pl.multiple_of(g * HT, HT)
        best, second = top2
        bits = []
        for n, c in enumerate(range(0, HT, 8)):
            hc = src[pl.ds(c, 8), :]
            if pace is not None:
                z = pace(n)[:8]
                if n >= 3:
                    z = z | pltpu.bitcast(bits[n - 3] & 0xFFFF, _U32)
                hc = _add_zero(hc, z)
            hnb = _layernorm(hc).astype(_BF16)
            hn_s[pl.ds(r0 + c, 8), :] = hnb
            hn = hnb.astype(_F32)
            if pace is not None:
                out_s[pl.ds(r0 + c, 8), :] = (hc + hn).astype(_BF16)
            r = jnp.broadcast_to(jnp.sum(hn * wr, axis=1, keepdims=True), (8, HT))
            rb = pltpu.bitcast(_round_bf16(r) + 0.0, _I32)
            bits.append(rb)
            key = ((jnp.where(rb < 0, rb ^ 0x7FFF0000, rb) >> (16 - _IDX_BITS))
                   + ((_KEY_BIAS + S - 1 - c - r0) - sub8))
            key = pltpu.bitcast(key, _F32)
            if valid is not None:
                key = jnp.where(valid, key, 0.0)
            second = jnp.maximum(second, jnp.minimum(best, key))
            best = jnp.maximum(best, key)
        return best, second

    def prod(rh, t, tiles, z=None):
        KS = 2 * D
        ps = [None] * 7
        for u in _ORDER:
            terms = [_sub(q1, q2) + (s1 * s2,) for q1, s1 in _SA[t] for q2, s2 in _SA[u]]
            fence()
            acc = None
            for k0 in range(0, KO, KS):
                def blk(rb, kb):
                    h0 = (kb * KO + k0) // D
                    return jnp.concatenate(
                        [_as_bf16(ctx_s[h0 + hh, pl.ds(rh + rb * QT // 2, QT // 2), :])
                         for hh in range(KS // D)], axis=1)
                if len(terms) == 1:
                    lhs = blk(terms[0][0], terms[0][1])
                else:
                    lhs = _combine([(blk(rb, kb).astype(_F32), sg)
                                    for rb, kb, sg in terms]).astype(_BF16)
                w = wob_s[7 * t + u, _rows(k0, KS), :]
                if z is not None and k0 == 0 and u == _ORDER[1]:
                    w = _tie(w, {0: jnp.concatenate([z, z], axis=1)})
                d = _dot(lhs, _as_bf16(w))
                tiles.append((d, 0, 0))
                acc = d if acc is None else acc + d
            ps[u] = acc
        c11, c12, c21, c22 = _strassen_c(ps)
        return jnp.concatenate([jnp.concatenate([c11, c12], axis=1),
                                jnp.concatenate([c21, c22], axis=1)], axis=0)

    def o_body(j, top2):
        r0 = pl.multiple_of(j * TQ, TQ)

        @pl.when(j > 1)
        def _():
            out_copy(2 * j - 4).start()

        @pl.when(j > 1)
        def _():
            out_copy(2 * j - 3).start()

        rh = pl.multiple_of(j * (TQ // 2), TQ // 2)
        left, right = pl.ds(0, M // 2), pl.ds(M // 2, M // 2)

        def residual(dst, rows0, cols, att):
            hb = (x_raw[pl.ds(rows0, HT), cols].astype(_F32) + att).astype(_BF16)
            h_s[pl.ds(rows0, HT), cols] = hb
            dst[:, cols] = hb.astype(_F32)

        gp = jnp.maximum(2 * j - 2, 0)
        tl = []
        m3 = prod(rh, 2, tl)
        m4 = prod(rh, 3, tl)
        top2 = epilogue(gp, ht_s, top2, _pacer(tl[:len(tl) * 7 // 8], NPC, 1), j > 0)
        tl = []
        m5 = prod(rh, 4, tl, _zero_of(top2[0]))
        residual(ht_s, r0, right, m3 + m5)
        m1 = prod(rh, 0, tl)
        m7 = prod(rh, 6, tl)
        residual(ht_s, r0, left, m4 - m5 + m1 + m7)
        top2 = epilogue(gp + 1, hb_s, top2, _pacer(tl[:len(tl) * 7 // 8], NPC), j > 0)
        m2 = prod(rh, 1, tl, _zero_of(top2[0]))
        residual(hb_s, r0 + HT, left, m4 + m2)
        m6 = prod(rh, 5, tl)
        residual(hb_s, r0 + HT, right, m3 + m1 - m2 + m6)
        return top2

    for n in range(3):
        ffn_wait(n)
    with jax.named_scope('o_loop'):
        top2 = lax.fori_loop(0, NB, o_body, (jnp.zeros((8, HT), _F32),) * 2)
    rest = ((NG - 2, ht_s), (NG - 1, hb_s))
    out_copy(NG - 4).start()
    out_copy(NG - 3).start()
    for g, src in rest:
        top2 = epilogue(g, src, top2)

    best, second = top2
    k1 = jnp.max(best, axis=0, keepdims=True)
    k2 = jnp.max(jnp.where(best == k1, second, best), axis=0, keepdims=True)

    R = _FIX
    row = lax.broadcasted_iota(_I32, (2 * R, HT), 0)
    idx = S - 1 - (pltpu.bitcast(jnp.where(row < R, k1, k2), _I32) & (2 ** _IDX_BITS - 1))
    i1 = jnp.clip(idx[0, 0], 0, S - 1)
    i2 = jnp.clip(idx[R, 0], 0, S - 1)
    b1 = pl.multiple_of(i1 & -R, R)
    b2 = pl.multiple_of(i2 & -R, R)
    tokr = jnp.where(row < R, b1 + row, b2 + row - R)
    cd = (((pltpu.bitcast(jnp.where(tokr == i1, k1, k2), _I32) - _KEY_BIAS) >> _IDX_BITS) << 16)
    score = pltpu.bitcast(jnp.where(cd < 0, cd ^ 0x7FFF0000, cd), _F32)
    gate = _round_bf16(1.0 / (1.0 + jnp.exp(-score)))
    gate = jnp.concatenate([gate] * (M // HT), axis=1)
    tokr = jnp.concatenate([tokr] * (M // HT), axis=1)

    hnsel = jnp.concatenate([hn_s[pl.ds(b1, R), :].astype(_F32),
                             hn_s[pl.ds(b2, R), :].astype(_F32)], axis=0)
    xs = hnsel.astype(_BF16)
    g = _dot(xs, wg_s[...])
    u = _dot(xs, wu_s[...])
    pace = _pacer([(mat, 0, c0) for mat in (g, u) for c0 in range(0, F, HT)], len(rest) * NPC)
    for k, (gi, src) in enumerate(rest):
        for n, c in enumerate(range(0, HT, 8)):
            rows = pl.ds(gi * HT + c, 8)
            z = pltpu.bitcast(pace(k * NPC + n)[:8], _F32)
            z = jnp.concatenate([z] * (M // HT), axis=1)
            out_s[rows, :] = (src[pl.ds(c, 8), :] + z + hn_s[rows, :].astype(_F32)).astype(_BF16)
        out_copy(gi).start()
    g = _round_bf16(g)
    u = _round_bf16(u)
    g = _round_bf16(g * (1.0 / (1.0 + jnp.exp(-g))))
    act = (g * u).astype(_BF16)
    y = _round_bf16(_round_bf16(_dot(act, wd_s[:, pl.ds(0, M)])) * gate)
    upd = jnp.where(jnp.logical_or(tokr == i1, tokr == i2), y, 0.0)
    hsel = jnp.concatenate([h_s[pl.ds(b1, R), :].astype(_F32),
                            h_s[pl.ds(b2, R), :].astype(_F32)], axis=0)
    fixed = hsel + _round_bf16(hnsel + upd)

    pltpu.make_async_copy(out_s, out_hbm, sem_out.at[0]).wait()

    def fix_copy(b0, k):
        return pltpu.make_async_copy(out_s.at[pl.ds(b0, R), :],
                                     out_hbm.at[pl.ds(b0, R), :], sem_out.at[k])

    out_s[pl.ds(b1, R), :] = fixed[:R].astype(_BF16)
    out_s[pl.ds(b2, R), :] = fixed[R:].astype(_BF16)
    fix_copy(b1, 0).start()

    @pl.when(b2 != b1)
    def _():
        fix_copy(b2, 1).start()
        fix_copy(b2, 1).wait()

    fix_copy(b1, 0).wait()


@jax.jit
def pallas_sequential_preLN__compressed_kv_cla__moe_arch_mod__prompt_kernel(
    A_x: jax.Array,
    A_c_kv: jax.Array,
    A_w_q: jax.Array,
    A_w_uk: jax.Array,
    A_w_uv: jax.Array,
    A_w_o: jax.Array,
    B_x: jax.Array,
    B_w_r: jax.Array,
    B_w_gate: jax.Array,
    B_w_up: jax.Array,
    B_w_down: jax.Array,
):
    B, S, M = A_x.shape
    DC = A_c_kv.shape[2]
    H, D = A_w_q.shape[1], A_w_q.shape[2]
    F = B_w_gate.shape[1]
    assert (B, S, M, DC, H, D) == (1, 8 * _TQ, 1024, 512, 32, _HT) and A_c_kv.shape[1] == S
    assert F % (8 * H) == 0 and S <= 2 ** _IDX_BITS

    scratch = [
        pltpu.VMEM((S, M), _BF16),
        pltpu.VMEM((S, DC), _BF16),
        pltpu.VMEM((S, M + _PAD), _F32),
        pltpu.VMEM((7, S // 2, DC // 2), _F32),
        pltpu.VMEM((4, S // 2, D), _U32),
        pltpu.VMEM((2, S // 2, D), _U32),
        pltpu.VMEM((2, S // 2, D), _U32),
        pltpu.VMEM((_TQ + 32, S + _PAD), _F32),
        pltpu.VMEM((_TQ + 32, S + _PAD), _F32),
        pltpu.VMEM((4, M, D), _U32),
        pltpu.VMEM((2, 2, DC, D), _U32),
        pltpu.VMEM((2, 49, M // 8, D), _U32),
        pltpu.VMEM((49, DC // 8, D), _U32),
        pltpu.VMEM((H, S // 2, D), _U32),
        pltpu.VMEM((2, 4, D // 2, M), _BF16),
        pltpu.VMEM((49, H * D // 8, M // 4), _U32),
        pltpu.VMEM((M, F), _BF16),
        pltpu.VMEM((M, F), _BF16),
        pltpu.VMEM((F, M + _PAD), _BF16),
        pltpu.VMEM((_HT, M), _F32),
        pltpu.VMEM((_HT, M), _F32),
        pltpu.VMEM((S, M), _BF16),
        pltpu.VMEM((S, M), _BF16),
        pltpu.VMEM((1024, _HT), _U32),
        pltpu.VMEM((S, M), _BF16),
        pltpu.VMEM((M,), _BF16),
        pltpu.SemaphoreType.DMA((S // _TQ,)),
        pltpu.SemaphoreType.DMA((S // _TQ // 2,)),
        pltpu.SemaphoreType.DMA((2,)),
        pltpu.SemaphoreType.DMA((4,)),
        pltpu.SemaphoreType.DMA((2,)),
        pltpu.SemaphoreType.DMA((4,)),
        pltpu.SemaphoreType.DMA((2,)),
    ]
    any_spec = pl.BlockSpec(memory_space=pl.ANY)
    out = pl.pallas_call(
        functools.partial(_kernel, S=S, M=M, DC=DC, H=H, D=D, F=F),
        in_specs=[any_spec] * 10,
        out_specs=any_spec,
        out_shape=jax.ShapeDtypeStruct((S, M), _BF16),
        scratch_shapes=scratch,
        compiler_params=pltpu.CompilerParams(vmem_limit_bytes=124 * 1024 * 1024,
                                             disable_bounds_checks=True,
                                             disable_semaphore_checks=True),
        name="fused_mla_mod",
    )(A_x.reshape(S, M), A_c_kv.reshape(S, DC), A_w_q, A_w_uk, A_w_uv,
      A_w_o.reshape(H * D, M), B_w_r, B_w_gate, B_w_up, B_w_down)
    return out.reshape(B, S, M)
```

```python
import functools
import math

import jax
import jax.numpy as jnp
from jax import lax
import jax.experimental.pallas as pl
import jax.experimental.pallas.tpu as pltpu

_F32 = jnp.float32
_BF16 = jnp.bfloat16
_U32 = jnp.uint32
_I32 = jnp.int32

_EPS = 1e-5
_NEG = -1e30
_TQ = 256
_HT = 128
_QT = 64
_IDX_BITS = 13
_KEY_BIAS = 0x30000000
_FIX = 8
_PAD = 128


def _dot(a, b):
    return jnp.dot(a, b, preferred_element_type=_F32)


def _dot_nt(a, b):
    return lax.dot_general(a, b, (((1,), (1,)), ((), ())), preferred_element_type=_F32)


def _as_bf16(u):
    return pltpu.bitcast(u, _BF16)


def _pack(x):
    return pltpu.bitcast(x.astype(_BF16), _U32)


def _rows(r0, n):
    if isinstance(r0, int):
        return pl.ds(r0 // 2, n // 2)
    return pl.ds(pl.multiple_of(r0 // 2, 8), n // 2)


def _ld(ref, lead, r0, n):
    return _as_bf16(ref[lead, _rows(r0, n), :])


def _st(ref, lead, r0, x, cols=slice(None)):
    ref[lead, _rows(r0, x.shape[0]), cols] = _pack(x)


def _round_bf16(x):
    return x.astype(_BF16).astype(_F32)


def _zero_of(v):
    return (pltpu.bitcast(v, _U32) >> 16) >> 16


def _lo_hi(w):
    return (pltpu.bitcast(w << 16, _F32), pltpu.bitcast(w & jnp.uint32(0xFFFF0000), _F32))


def _row_stats(x):
    n = x.shape[-1]
    mean = jnp.sum(x, axis=-1, keepdims=True) * (1.0 / n)
    xc = x - mean
    return mean, xc, jnp.sum(xc * xc, axis=-1, keepdims=True) * (1.0 / n)


def _layernorm(x):
    mean, _, var = _row_stats(x)
    den = _round_bf16(jnp.sqrt(_round_bf16(_round_bf16(var) + _EPS)))
    return (x - _round_bf16(mean)) * pl.reciprocal(den, approx=True)


def _layernorm_scaled(x, scale):
    _, xc, var = _row_stats(x)
    return xc * (lax.rsqrt(var + _EPS) * scale)


_SA = (((0, 1), (3, 1)), ((2, 1), (3, 1)), ((0, 1),), ((3, 1),),
       ((0, 1), (1, 1)), ((2, 1), (0, -1)), ((1, 1), (3, -1)))
_SB = (((0, 1), (3, 1)), ((0, 1),), ((1, 1), (3, -1)), ((2, 1), (0, -1)),
       ((3, 1),), ((0, 1), (1, 1)), ((2, 1), (3, 1)))
_ORDER = (2, 4, 3, 1, 0, 6, 5)


def _combine(terms):
    terms = sorted(terms, key=lambda ts: -ts[1])
    assert terms[0][1] > 0
    acc = terms[0][0]
    for v, sg in terms[1:]:
        acc = acc + v if sg > 0 else acc - v
    return acc


def _operands(table, quad):
    return [_combine([(quad[q], sg) for q, sg in terms]) for terms in table]


def _strassen_c(m):
    m1, m2, m3, m4, m5, m6, m7 = m
    return (m4 - m5 + m1 + m7, m3 + m5, m4 + m2, m3 - m2 + m1 + m6)


def _sub(q1, q2):
    return 2 * (q1 // 2) + q2 // 2, 2 * (q1 % 2) + q2 % 2


def _pacer(tiles, total, free=0):
    def zero(n):
        if n < free:
            return jnp.zeros((16, _HT), _U32)
        mat, r, c = tiles[(n - free) * len(tiles) // (total - free)]
        z = _zero_of(mat[r:r + 8, c:c + _HT])
        return jnp.concatenate([z, z], axis=0)
    return zero


def _head(tiles, sixteenths):
    return tiles[:len(tiles) * sixteenths // 16]


def _tie(w, ties):
    parts, at = [], 0
    for r in sorted(ties):
        if r > at:
            parts.append(w[at:r])
        parts.append(w[r:r + 8] | ties[r])
        at = r + 8
    if at < w.shape[0]:
        parts.append(w[at:])
    return parts[0] if len(parts) == 1 else jnp.concatenate(parts, axis=0)


def _add_zero(x, z):
    return jnp.concatenate([x[:, :_HT] + pltpu.bitcast(z, _F32), x[:, _HT:]], axis=1)


def _kernel(x_hbm, c_hbm, wq_hbm, wk_hbm, wv_hbm, wo_hbm, wr_hbm, wg_hbm, wu_hbm, wd_hbm,
            out_hbm,
            x_raw, c_raw, xn_s, ca_s, q_s, k_s, v_s, sa_s, sb_s,
            wq_p, wkv_p, wqb_s, wkvb_s,
            ctx_s, wo_p, wob_s, wg_s, wu_s, wd_s, ht_s, hb_s, h_s, hn_s, junk_s, out_s, wr_s,
            sem_x, sem_c, sem_w, sem_wq, sem_wo, sem_ffn, sem_out,
            *, S, M, DC, H, D, F):
    TQ, HT, QT = _TQ, _HT, _QT
    NB = S // TQ
    NH = NB // 2
    NG = S // HT
    NP = H // 2
    KQ, MQ = DC // 4, M // 4
    KO, NO = H * D // 4, M // 4
    OS = KO // NP
    qscale = (D ** -0.5) * math.log2(math.e)

    wq32 = wq_hbm.bitcast(_U32)
    wk32 = wk_hbm.bitcast(_U32)
    wv32 = wv_hbm.bitcast(_U32)

    def w_start(pair, slot):
        for k, src in enumerate((wk32, wv32)):
            pltpu.make_async_copy(src.at[:, pair, :], wkv_p.at[slot, k], sem_w.at[slot]).start()

    def w_wait(slot):
        pltpu.make_async_copy(wkv_p.at[slot], wkv_p.at[slot], sem_w.at[slot]).wait()

    def wq_copy(pair):
        return pltpu.make_async_copy(wq32.at[:, pair, :], wq_p.at[pair & 3],
                                     sem_wq.at[pair & 3])

    def wo_start(t, slot):
        r0 = pl.multiple_of(t * OS, OS)
        for k in range(4):
            pltpu.make_async_copy(wo_hbm.at[pl.ds(k * KO + r0, OS), :],
                                  wo_p.at[slot, k], sem_wo.at[slot]).start()

    def wo_wait(slot):
        pltpu.make_async_copy(wo_p.at[slot], wo_p.at[slot], sem_wo.at[slot]).wait()

    def x_chunk(n):
        return jnp.where(n < NH, n + NH, NB - 1 - n)

    def x_copy(n):
        rows = pl.ds(pl.multiple_of(x_chunk(n) * TQ, TQ), TQ)
        return pltpu.make_async_copy(x_hbm.at[rows, :], x_raw.at[rows, :], sem_x.at[n])

    def x0_copy(k):
        rows = pl.ds(pl.multiple_of(k * QT, QT), QT)
        return pltpu.make_async_copy(x_hbm.at[rows, :], x_raw.at[rows, :], sem_x.at[NB - 1 + k])

    def c_copy(i):
        rows = pl.ds(pl.multiple_of(i * 2 * TQ, 2 * TQ), 2 * TQ)
        return pltpu.make_async_copy(c_hbm.at[rows, :], c_raw.at[rows, :], sem_c.at[i])

    ffn = ((wg_hbm, wg_s), (wu_hbm, wu_s), (wd_hbm, wd_s))

    def ffn_start(t):
        for n, (src, dst) in enumerate(ffn):
            rows, cols = src.shape[0] // NP, src.shape[1]
            r0 = pl.multiple_of(t * rows, 16)
            pltpu.make_async_copy(src.at[pl.ds(r0, rows), :],
                                  dst.at[pl.ds(r0, rows), pl.ds(0, cols)],
                                  sem_ffn.at[n]).start()

    def ffn_wait(n):
        src, dst = ffn[n]
        pltpu.make_async_copy(src, dst.at[:, pl.ds(0, src.shape[1])], sem_ffn.at[n]).wait()

    wr_copy = pltpu.make_async_copy(wr_hbm, wr_s, sem_ffn.at[3])

    def out_copy(g):
        rows = pl.ds(pl.multiple_of(g * HT, HT), HT)
        return pltpu.make_async_copy(out_s.at[rows, :], out_hbm.at[rows, :], sem_out.at[0])

    def prep_w4(srcs, dst, kq, rows, pace, sink=None):
        pieces = [(t, r) for t in range(7) for r in rows]
        for n, (t, r) in enumerate(pieces):
            terms = [[] for _ in range(4)]
            for k, (q1, sg) in enumerate(_SB[t]):
                for rb in range(2):
                    w = srcs[q1 % 2][pl.ds((2 * (q1 // 2) + rb) * kq + r, 16), :]
                    if k == 0:
                        w = w | (pace(n) if sink is not None else pace(2 * n + rb))
                    lo, hi = _lo_hi(w)
                    terms[2 * rb].append((lo, sg))
                    terms[2 * rb + 1].append((hi, sg))
            z = None
            for u, b in enumerate(_operands(_SB, [_combine(tm) for tm in terms])):
                pk = _pack(b)
                dst[7 * t + u, pl.ds(r // 2, 8), :] = pk
                z = pk if z is None else z | pk
            if sink is not None:
                junk_s[pl.ds(8 * (sink + n), 8), :] = z

    def prep_wq(raw, slot, r, nr, pace, sink=None):
        span = 3 * MQ + nr
        prep_w4((wq_p.at[raw, pl.ds(r, span), :], wq_p.at[raw + 1, pl.ds(r, span), :]),
                wqb_s.at[slot, :, pl.ds(pl.multiple_of(r // 2, 8), nr // 2), :],
                MQ, range(0, nr, 16), pace, sink)

    def prep_wo(slot, src0, nrows, dst0, tiles):
        pieces = [(r, c0, t) for r in range(0, nrows, 16) for c0 in range(0, NO, HT)
                  for t in range(7)]
        pace = _pacer(tiles, len(pieces))
        for n, (r, c0, t) in enumerate(pieces):
            z = pltpu.bitcast(pace(n), _F32)
            sub = []
            for q2 in range(4):
                v = _combine([
                    (wo_p[slot, _sub(q1, q2)[0], pl.ds(src0 + r, 16),
                          pl.ds(_sub(q1, q2)[1] * NO + c0, HT)].astype(_F32), sg)
                    for q1, sg in _SB[t]])
                sub.append(v + z if q2 in (0, 3) else v)
            for u, b in enumerate(_operands(_SB, sub)):
                _st(wob_s, 7 * t + u, dst0 + r, b, pl.ds(c0, HT))

    def fence():
        junk_s[pl.ds(0, 8), :] = jnp.zeros((8, HT), _U32)

    def project4(lhs, w, store, zs=()):
        at = {48 * (k + 1) // len(zs): z for k, z in enumerate(zs)}
        m, tiles = [None] * 7, []
        for nt, t in enumerate(_ORDER):
            ps = [None] * 7
            for nu, u in enumerate(_ORDER):
                fence()
                a = lhs(t, u)
                wt = w[7 * t + u]
                if 7 * nt + nu in at:
                    wt = _tie(wt, {0: at[7 * nt + nu]})
                ps[u] = _dot(a.astype(_BF16), _as_bf16(wt))
                tiles += [(ps[u], r, 0) for r in range(0, QT, QT * D // (2 * a.shape[1]))]
            m[t] = _strassen_c(ps)
        for q2 in range(4):
            for q1, cblk in enumerate(_strassen_c([mt[q2] for mt in m])):
                store(_sub(q1, q2)[1], _sub(q1, q2)[0] * QT, cblk)
        return tiles

    def project_q(xn, wqb, q, r0):
        def lhs(t, u):
            return _combine([
                (xn[pl.ds(r0 + _sub(q1, q2)[0] * QT, QT), pl.ds(_sub(q1, q2)[1] * MQ, MQ)],
                 s1 * s2) for q1, s1 in _SA[t] for q2, s2 in _SA[u]])
        return project4(lhs, wqb, lambda nb, r, val: _st(q, nb, r0 + r, val))

    def project_kv(j, zs=()):
        def lhs(t, u):
            return _combine([
                (ca_s[t, pl.ds(j * HT + (q2 // 2) * QT, QT), pl.ds((q2 % 2) * KQ, KQ)], sg)
                for q2, sg in _SA[u]])
        return project4(lhs, wkvb_s,
                        lambda nb, r, val: _st((k_s, v_s)[nb // 2], nb % 2, j * TQ + r, val), zs)

    def stage_x(spans, tiles, dist):
        starts = [r0 + c for r0, nrows in spans for c in range(0, nrows, 8)]
        pace = _pacer(tiles, len(starts))
        done = []
        for n, r in enumerate(starts):
            z = pace(n)[:8]
            if n >= dist:
                z = z | done[n - dist]
            y = _layernorm_scaled(_add_zero(x_raw[pl.ds(r, 8), :].astype(_F32), z), qscale)
            xn_s[pl.ds(r, 8), pl.ds(0, M)] = y
            done.append(_zero_of(y[:, :HT]))

    def stage_c(r0, a0, pace):
        kh = DC // 2
        for n, c in enumerate(range(0, HT, 8)):
            top = c_raw[pl.ds(r0 + c, 8), :].astype(_F32)
            bot = c_raw[pl.ds(r0 + HT + c, 8), :].astype(_F32)
            z = pltpu.bitcast(pace(n)[:8], _F32)
            z = jnp.concatenate([z] * (kh // HT), axis=1)
            quad = (top[:, :kh] + z, top[:, kh:], bot[:, :kh], bot[:, kh:] + z)
            for t, a in enumerate(_operands(_SA, quad)):
                ca_s[t, pl.ds(a0 + c, 8), :] = a

    def issue(n, carry):
        @pl.when(n == 0)
        def _():
            w_start(0, 0)

        @pl.when(n < NH)
        def _():
            c_copy(n).start()

        @pl.when(jnp.logical_or(n == NH, n == NH + 2))
        def _():
            wq_copy(n - NH).start()
            wq_copy(n - NH + 1).start()

        @pl.when(n == NB)
        def _():
            w_start(1, 1)
            wo_start(0, 0)

        @pl.when(jnp.logical_and(n > 0, n < NB))
        def _():
            x_copy(n - 1).start()

        @pl.when(jnp.logical_and(n >= NH, n < NB))
        def _():
            x0_copy(n - NH).start()

        return carry

    lax.fori_loop(0, NB + 1, issue, 0)
    ht_s[...] = jnp.zeros((HT, M), _F32)
    hb_s[...] = jnp.zeros((HT, M), _F32)
    x_raw[pl.ds(S, TQ), :] = jnp.zeros((TQ, M), _BF16)
    w_wait(0)
    c_copy(0).wait()

    def pro_a(i, carry):
        r0 = pl.multiple_of(i * 2 * TQ, 2 * TQ)
        wkv = jnp.concatenate(_lo_hi(wkv_p[0, 0]) + _lo_hi(wkv_p[0, 1]), axis=1).astype(_BF16)
        kv = _dot(c_raw[pl.ds(r0, 2 * TQ), :], wkv)
        for nb in range(4):
            _st((k_s, v_s)[nb // 2], nb % 2, r0, kv[:, nb * D:(nb + 1) * D])
        tiles = [(kv, r, nb * D) for nb in range(4) for r in range(0, 2 * TQ, 8)]
        nt = len(tiles)
        a0 = pl.multiple_of(i * TQ, TQ)
        stage_c(r0, a0, _pacer(tiles[:nt // 2], HT // 8))
        stage_c(r0 + TQ, a0 + HT, _pacer(tiles[nt // 2:nt * 15 // 16], HT // 8))
        rx = pl.multiple_of(jnp.where(i == 0, NB, i + NH - 1) * TQ, TQ)
        stage_x([(rx, TQ)], _head(tiles, 13), 6)

        @pl.when(i + 1 < NH)
        def _():
            c_copy(i + 1).wait()

        x_copy(i).wait()
        return carry

    def pro_b(i, carry):
        r0 = pl.multiple_of(i * TQ, TQ)
        kh = M // 2
        lhs = [xn_s[pl.ds(r0 + S // 2, TQ), pl.ds(k0, kh)].astype(_BF16) for k0 in (0, kh)]
        tiles = []
        for nb in range(4):
            d = [_dot(lhs[k], _lo_hi(wq_p[nb // 2, pl.ds(k * kh, kh), :])[nb % 2].astype(_BF16))
                 for k in range(2)]
            _st(q_s, nb, r0 + S // 2, d[0] + d[1])
            tiles += [(dk, r, 0) for dk in d for r in range(0, TQ, 8)]
        rx = pl.multiple_of(x_chunk(NH - 1 + i) * TQ, TQ)
        stage_x([(rx, TQ), (pl.multiple_of(i * QT, QT), QT)],
                _head(tiles, 12), 7)
        nr = MQ // (2 * NH)
        npc = 7 * nr // 8
        pace = _pacer(tiles, 3 * npc)
        for k in range(3):
            u = 3 * i + k
            quad = u // (2 * NH)
            prep_wq(2 * quad, quad, pl.multiple_of((u % (2 * NH)) * nr, nr), nr,
                    lambda n, k=k: pace(k * npc + n))

        @pl.when(i == 1)
        def _():
            wq_copy(2).wait()
            wq_copy(3).wait()

        @pl.when(i + 1 < NH)
        def _():
            x_copy(NH + i).wait()
            x0_copy(i + 1).wait()

        return carry

    with jax.named_scope('pro_a'):
        lax.fori_loop(0, NH, pro_a, 0)
    wq_copy(0).wait()
    wq_copy(1).wait()
    x0_copy(0).wait()
    with jax.named_scope('pro_b'):
        lax.fori_loop(0, NH, pro_b, 0)

    w_start(2, 0)
    wo_start(1, 1)
    wq_copy(4).start()
    wq_copy(5).start()
    ffn_start(NP - 1)
    wr_copy.start()
    w_wait(1)
    wo_wait(0)

    col = lax.broadcasted_iota(_I32, (QT, HT), 1)
    tri = col <= lax.broadcasted_iota(_I32, (QT, HT), 0) + QT
    tri0 = col <= lax.broadcasted_iota(_I32, (QT, HT), 0)

    def staging(t):
        off = pl.multiple_of((t >> 8) * 32, 32)
        return [r.at[pl.ds(off, TQ), :] for r in (sa_s, sb_s)]

    def softmax_rows(s, m):
        p = jnp.exp2(s - m)
        nt = p.shape[1] // HT
        tiles, acc, grp = [], None, None
        for j in range(nt):
            pj = p[:, j * HT:(j + 1) * HT]
            grp = pj if grp is None else grp + pj
            if j % 4 == 3 or j == nt - 1:
                if j % 4 > 0:
                    pj = jnp.minimum(pj, grp)
                acc = grp if acc is None else acc + grp
                grp = None
            tiles.append(pj)
        return (tiles[0] if nt == 1 else jnp.concatenate(tiles, axis=1)), acc

    def scores(q, e, i, buf, c0, zs=()):
        L0, Lm = i * TQ, i * TQ + HT

        def q_group(g):
            return _as_bf16(jnp.concatenate([q[e, _rows(L0 + g * QT, QT), :],
                                             q[e, _rows(L0 + HT + g * QT, QT), :]], axis=0))

        main, tiles = [[], []], []
        for g in (1, 0):
            k0, n = (1 - g) * QT, L0 + g * HT
            if n > 0:
                ties = {}
                if g == 0:
                    ties = {(k * (n // HT) // len(zs)) * QT + 8 * k: z for k, z in enumerate(zs)}
                m = _dot_nt(q_group(g), _as_bf16(_tie(k_s[e, _rows(k0, n), :], ties)))
                main[g] = [m]
                tiles += [(m, t0 % HT, (t0 // HT) * 4 * HT) for t0 in range(0, n // 4, 8)]
        left = _dot_nt(_ld(k_s, e, 0, QT), q_group(0))
        left = jnp.concatenate([left, jnp.full((QT, HT), _NEG, _F32)], axis=0).T
        last = [_dot_nt(_ld(q, e, L0 + HT + g * QT, QT), _ld(k_s, e, L0 + QT + g * QT, HT))
                for g in range(2)]
        main[0] = [left] + main[0]
        ms = [None] * 4
        for g, m in enumerate(main):
            sm = m[0] if len(m) == 1 else jnp.concatenate(m, axis=1)
            one = [jnp.where(tri0 if g == 0 and i == 0 else tri, sm[:QT, Lm - HT:], _NEG)]
            if Lm > HT:
                one = [sm[:QT, :Lm - HT]] + one
            for h, parts in enumerate((one, [sm[QT:], jnp.where(tri, last[g], _NEG)])):
                sh = parts[0] if len(parts) == 1 else jnp.concatenate(parts, axis=1)
                buf[pl.ds((2 * g + h) * QT, QT), pl.ds(c0, sh.shape[1])] = sh
                ms[2 * g + h] = jnp.max(sh, axis=1, keepdims=True)
        return (buf, c0, ms), tiles

    def context(e, head, i, buf, c0, ms):
        Lm = i * TQ + HT
        os_, ls = [None] * 4, [None] * 4
        for g in (1, 0):
            if g == 1:
                v_main = v_s[e, _rows(0, Lm), :]
            else:
                v_main = v_s[e, _rows(0, HT), :]
                if i > 0:
                    v_main = jnp.concatenate([v_main, v_s[e, _rows(QT, Lm - HT), :]], axis=0)
            v_last = _ld(v_s, e, Lm - (1 - g) * QT, HT)
            p1, ls[g] = softmax_rows(buf[pl.ds(2 * g * QT, QT), pl.ds(c0, Lm)], ms[2 * g])
            p2, ls[2 + g] = softmax_rows(buf[pl.ds((2 * g + 1) * QT, QT), pl.ds(c0, Lm + HT)],
                                         ms[2 * g + 1])
            o = _dot(jnp.concatenate([p1, p2[:, :Lm]], axis=0).astype(_BF16), _as_bf16(v_main))
            os_[g] = o[:QT]
            os_[2 + g] = o[QT:] + _dot(p2[:, Lm:].astype(_BF16), v_last)
        o = jnp.concatenate(os_, axis=0)
        acc = jnp.concatenate(ls, axis=0)

        def normalize(pace=None, n0=0):
            z = None
            for n, g in enumerate(range(0, TQ, 16)):
                a = acc[g:g + 16]
                if pace is not None:
                    a = a + pltpu.bitcast(pace(n0 + n), _F32)
                linv = jnp.broadcast_to(
                    pl.reciprocal(jnp.sum(a, axis=1, keepdims=True), approx=True), (16, D))
                ctx_s.at[head][_rows(i * TQ + g, 16), :] = _pack(o[g:g + 16] * linv)
                bits = pltpu.bitcast(linv, _U32)
                bits = bits[:8] | bits[8:]
                z = bits if z is None else z | bits
            return _zero_of(z)
        return normalize

    def pair_body(s, carry):
        odd = s & 1
        slot = 1 - odd
        wo0 = pl.multiple_of(s * OS, OS)
        q_rd = q_s.at[pl.ds(2 * odd, 2)]
        q_wr = q_s.at[:, pl.ds(pl.multiple_of(odd * (S // 4), S // 4), S // 4), :]
        xn = xn_s.at[pl.ds(pl.multiple_of(odd * (S // 2), S // 2), S // 2), :]
        quad = (s + 1) >> 1
        wqb = wqb_s.at[quad & 1]
        pend, sc = {}, {}
        bufs = staging(s)

        def norm(i, tiles):
            pace = _pacer(tiles, TQ // 8)
            return [f(pace, k * (TQ // 16)) for k, f in enumerate(pend.pop(i))]

        def qk(i, nrm=None):
            c0 = S // 2 if i < 2 else 0
            sa, ta = scores(q_rd, 0, i, bufs[0], c0)
            zs = ()
            if nrm is not None:
                zs = norm(nrm, _head(ta, 14))
            sb, tb = scores(q_rd, 1, i, bufs[1], c0, zs)
            sc[i] = (sa, sb)
            return [ta, tb]

        def pv(i):
            pend[i] = [context(e, 2 * s + e, i, *sc[i][e]) for e in range(2)]

        kv = project_kv
        tl = {}
        for i in range(7, 3, -1):
            tl[i] = qk(i, i + 2 if i + 2 < NB else None)
            if i == 7:
                prep_wq(2 * (jnp.minimum(quad + 1, NP // 2 - 1) & 1), (quad + 1) & 1,
                        pl.multiple_of((1 - odd) * (MQ // 2), MQ // 2), MQ // 2,
                        _pacer(tl[7][0] + _head(tl[7][1], 14), 7 * MQ // 32), 64)
            project_q(xn, wqb, q_wr, (i - NH) * TQ)
            pv(i)
        prep_w4((wkv_p.at[slot, 0], wkv_p.at[slot, 1]), wkvb_s, KQ, range(0, KQ, 16),
                _pacer(tl[6][0] + _head(tl[6][1], 15), 7 * KQ // 16), 1)
        tl[3] = qk(3, 5)
        qk(0)
        kv(7)
        pv(3)
        pv(0)
        z = norm(4, kv(6))
        qk(2)
        qk(1)
        prep_wo(odd, 0, OS, wo0,
                _head(tl[5][0], 8) + _head(tl[5][1], 15) + tl[4][0] + _head(tl[4][1], 15)
                + tl[3][0] + _head(tl[3][1], 12))
        kv(5, z)
        pv(2)
        pv(1)
        t = kv(4)
        for j, i in ((3, 3), (2, 0), (1, 2), (0, 1)):
            t = kv(j, norm(i, t[8:-8]))

        @pl.when(s + 3 < NP)
        def _():
            w_start(s + 3, slot)

        @pl.when(s + 2 < NP)
        def _():
            wo_start(s + 2, odd)

        @pl.when(s + 6 < NP)
        def _():
            wq_copy(s + 6).start()

        ffn_start(s)

        @pl.when(s + 5 < NP)
        def _():
            wq_copy(s + 5).wait()

        @pl.when(s + 2 < NP)
        def _():
            w_wait(odd)

        wo_wait(slot)

        @pl.when(s == 0)
        def _():
            wq_copy(4).wait()

        return carry

    with jax.named_scope('pair_loop'):
        lax.fori_loop(0, NP - 1, pair_body, 0)

    def last_body(e, carry):
        half = OS // 2
        q_rd = q_s.at[pl.ds(2, 2)]
        bufs = staging(e)
        sc, pend = {}, []
        sc[7], tl = scores(q_rd, e, 7, bufs[1], 0)
        prep_wo((NP - 1) % 2, pl.multiple_of(e * half, half), half,
                pl.multiple_of((NP - 1) * OS + e * half, half), tl[:96])
        for step in "s6 c7 s5 c6 s4 c5 s3 s0 c4 s2 s1 c0 c3 c1 c2".split():
            i = int(step[1])
            if step[0] == "s":
                sc[i], _ = (scores(q_rd, e, i, bufs[i % 2], 0) if i >= 2
                            else scores(q_rd, e, i, bufs[1 - i], S // 2))
            else:
                pend.append(context(e, H - 2 + e, i, *sc[i]))
        for f in pend:
            f()
        return carry

    with jax.named_scope('last_loop'):
        lax.fori_loop(0, 2, last_body, 0)

    wr_copy.wait()
    wr = wr_s[...].astype(_F32).reshape(1, M)
    sub8 = lax.broadcasted_iota(_I32, (8, HT), 0)
    NPC = HT // 8

    def epilogue(g, src, top2, pace=None, valid=None):
        r0 = pl.multiple_of(g * HT, HT)
        best, second = top2
        bits = []
        for n, c in enumerate(range(0, HT, 8)):
            hc = src[pl.ds(c, 8), :]
            if pace is not None:
                z = pace(n)[:8]
                if n >= 3:
                    z = z | pltpu.bitcast(bits[n - 3] & 0xFFFF, _U32)
                hc = _add_zero(hc, z)
            hnb = _layernorm(hc).astype(_BF16)
            hn_s[pl.ds(r0 + c, 8), :] = hnb
            hn = hnb.astype(_F32)
            if pace is not None:
                out_s[pl.ds(r0 + c, 8), :] = (hc + hn).astype(_BF16)
            r = jnp.broadcast_to(jnp.sum(hn * wr, axis=1, keepdims=True), (8, HT))
            rb = pltpu.bitcast(_round_bf16(r) + 0.0, _I32)
            bits.append(rb)
            key = ((jnp.where(rb < 0, rb ^ 0x7FFF0000, rb) >> (16 - _IDX_BITS))
                   + ((_KEY_BIAS + S - 1 - c - r0) - sub8))
            key = pltpu.bitcast(key, _F32)
            if valid is not None:
                key = jnp.where(valid, key, 0.0)
            second = jnp.maximum(second, jnp.minimum(best, key))
            best = jnp.maximum(best, key)
        return best, second

    def prod(rh, t, tiles, z=None):
        KS = 2 * D
        ps = [None] * 7
        for u in _ORDER:
            terms = [_sub(q1, q2) + (s1 * s2,) for q1, s1 in _SA[t] for q2, s2 in _SA[u]]
            fence()
            acc = None
            for k0 in range(0, KO, KS):
                def blk(rb, kb):
                    h0 = (kb * KO + k0) // D
                    return jnp.concatenate(
                        [_as_bf16(ctx_s[h0 + hh, pl.ds(rh + rb * QT // 2, QT // 2), :])
                         for hh in range(KS // D)], axis=1)
                if len(terms) == 1:
                    lhs = blk(terms[0][0], terms[0][1])
                else:
                    lhs = _combine([(blk(rb, kb).astype(_F32), sg)
                                    for rb, kb, sg in terms]).astype(_BF16)
                w = wob_s[7 * t + u, _rows(k0, KS), :]
                if z is not None and k0 == 0 and u == _ORDER[1]:
                    w = _tie(w, {0: jnp.concatenate([z, z], axis=1)})
                d = _dot(lhs, _as_bf16(w))
                tiles.append((d, 0, 0))
                acc = d if acc is None else acc + d
            ps[u] = acc
        c11, c12, c21, c22 = _strassen_c(ps)
        return jnp.concatenate([jnp.concatenate([c11, c12], axis=1),
                                jnp.concatenate([c21, c22], axis=1)], axis=0)

    def o_body(j, top2):
        r0 = pl.multiple_of(j * TQ, TQ)

        @pl.when(j > 1)
        def _():
            out_copy(2 * j - 4).start()

        @pl.when(j > 1)
        def _():
            out_copy(2 * j - 3).start()

        rh = pl.multiple_of(j * (TQ // 2), TQ // 2)
        left, right = pl.ds(0, M // 2), pl.ds(M // 2, M // 2)

        def residual(dst, rows0, cols, att):
            hb = (x_raw[pl.ds(rows0, HT), cols].astype(_F32) + att).astype(_BF16)
            h_s[pl.ds(rows0, HT), cols] = hb
            dst[:, cols] = hb.astype(_F32)

        gp = jnp.maximum(2 * j - 2, 0)
        tl = []
        m3 = prod(rh, 2, tl)
        m4 = prod(rh, 3, tl)
        top2 = epilogue(gp, ht_s, top2, _pacer(tl[:len(tl) * 7 // 8], NPC, 1), j > 0)
        tl = []
        m5 = prod(rh, 4, tl, _zero_of(top2[0]))
        residual(ht_s, r0, right, m3 + m5)
        m1 = prod(rh, 0, tl)
        m7 = prod(rh, 6, tl)
        residual(ht_s, r0, left, m4 - m5 + m1 + m7)
        top2 = epilogue(gp + 1, hb_s, top2, _pacer(tl[:len(tl) * 7 // 8], NPC), j > 0)
        m2 = prod(rh, 1, tl, _zero_of(top2[0]))
        residual(hb_s, r0 + HT, left, m4 + m2)
        m6 = prod(rh, 5, tl)
        residual(hb_s, r0 + HT, right, m3 + m1 - m2 + m6)
        return top2

    for n in range(3):
        ffn_wait(n)
    with jax.named_scope('o_loop'):
        top2 = lax.fori_loop(0, NB, o_body, (jnp.zeros((8, HT), _F32),) * 2)
    rest = ((NG - 2, ht_s), (NG - 1, hb_s))
    out_copy(NG - 4).start()
    out_copy(NG - 3).start()
    for g, src in rest:
        top2 = epilogue(g, src, top2)

    best, second = top2
    k1 = jnp.max(best, axis=0, keepdims=True)
    k2 = jnp.max(jnp.where(best == k1, second, best), axis=0, keepdims=True)

    R = _FIX
    row = lax.broadcasted_iota(_I32, (2 * R, HT), 0)
    idx = S - 1 - (pltpu.bitcast(jnp.where(row < R, k1, k2), _I32) & (2 ** _IDX_BITS - 1))
    i1 = jnp.clip(idx[0, 0], 0, S - 1)
    i2 = jnp.clip(idx[R, 0], 0, S - 1)
    b1 = pl.multiple_of(i1 & -R, R)
    b2 = pl.multiple_of(i2 & -R, R)
    tokr = jnp.where(row < R, b1 + row, b2 + row - R)
    cd = (((pltpu.bitcast(jnp.where(tokr == i1, k1, k2), _I32) - _KEY_BIAS) >> _IDX_BITS) << 16)
    score = pltpu.bitcast(jnp.where(cd < 0, cd ^ 0x7FFF0000, cd), _F32)
    gate = _round_bf16(1.0 / (1.0 + jnp.exp(-score)))
    gate = jnp.concatenate([gate] * (M // HT), axis=1)
    tokr = jnp.concatenate([tokr] * (M // HT), axis=1)

    hnsel = jnp.concatenate([hn_s[pl.ds(b1, R), :].astype(_F32),
                             hn_s[pl.ds(b2, R), :].astype(_F32)], axis=0)
    xs = hnsel.astype(_BF16)
    g = _dot(xs, wg_s[...])
    u = _dot(xs, wu_s[...])
    pace = _pacer([(mat, 0, c0) for mat in (g, u) for c0 in range(0, F, HT)], len(rest) * NPC)
    for k, (gi, src) in enumerate(rest):
        for n, c in enumerate(range(0, HT, 8)):
            rows = pl.ds(gi * HT + c, 8)
            z = pltpu.bitcast(pace(k * NPC + n)[:8], _F32)
            z = jnp.concatenate([z] * (M // HT), axis=1)
            out_s[rows, :] = (src[pl.ds(c, 8), :] + z + hn_s[rows, :].astype(_F32)).astype(_BF16)
        out_copy(gi).start()
    g = _round_bf16(g)
    u = _round_bf16(u)
    g = _round_bf16(g * (1.0 / (1.0 + jnp.exp(-g))))
    act = (g * u).astype(_BF16)
    y = _round_bf16(_round_bf16(_dot(act, wd_s[:, pl.ds(0, M)])) * gate)
    upd = jnp.where(jnp.logical_or(tokr == i1, tokr == i2), y, 0.0)
    hsel = jnp.concatenate([h_s[pl.ds(b1, R), :].astype(_F32),
                            h_s[pl.ds(b2, R), :].astype(_F32)], axis=0)
    fixed = hsel + _round_bf16(hnsel + upd)

    pltpu.make_async_copy(out_s, out_hbm, sem_out.at[0]).wait()

    def fix_copy(b0, k):
        return pltpu.make_async_copy(out_s.at[pl.ds(b0, R), :],
                                     out_hbm.at[pl.ds(b0, R), :], sem_out.at[k])

    out_s[pl.ds(b1, R), :] = fixed[:R].astype(_BF16)
    out_s[pl.ds(b2, R), :] = fixed[R:].astype(_BF16)
    fix_copy(b1, 0).start()

    @pl.when(b2 != b1)
    def _():
        fix_copy(b2, 1).start()
        fix_copy(b2, 1).wait()

    fix_copy(b1, 0).wait()


@jax.jit
def pallas_sequential_preLN__compressed_kv_cla__moe_arch_mod__prompt_kernel(
    A_x: jax.Array,
    A_c_kv: jax.Array,
    A_w_q: jax.Array,
    A_w_uk: jax.Array,
    A_w_uv: jax.Array,
    A_w_o: jax.Array,
    B_x: jax.Array,
    B_w_r: jax.Array,
    B_w_gate: jax.Array,
    B_w_up: jax.Array,
    B_w_down: jax.Array,
):
    B, S, M = A_x.shape
    DC = A_c_kv.shape[2]
    H, D = A_w_q.shape[1], A_w_q.shape[2]
    F = B_w_gate.shape[1]
    assert (B, S, M, DC, H, D) == (1, 8 * _TQ, 1024, 512, 32, _HT) and A_c_kv.shape[1] == S
    assert F % (8 * H) == 0 and S <= 2 ** _IDX_BITS

    scratch = [
        pltpu.VMEM((S + _TQ, M), _BF16),
        pltpu.VMEM((S, DC), _BF16),
        pltpu.VMEM((S + _TQ, M + _PAD), _F32),
        pltpu.VMEM((7, S // 2, DC // 2), _F32),
        pltpu.VMEM((4, S // 2, D), _U32),
        pltpu.VMEM((2, S // 2, D), _U32),
        pltpu.VMEM((2, S // 2, D), _U32),
        pltpu.VMEM((_TQ + 32, S + _PAD), _F32),
        pltpu.VMEM((_TQ + 32, S + _PAD), _F32),
        pltpu.VMEM((4, M, D), _U32),
        pltpu.VMEM((2, 2, DC, D), _U32),
        pltpu.VMEM((2, 49, M // 8, D), _U32),
        pltpu.VMEM((49, DC // 8, D), _U32),
        pltpu.VMEM((H, S // 2, D), _U32),
        pltpu.VMEM((2, 4, D // 2, M), _BF16),
        pltpu.VMEM((49, H * D // 8, M // 4), _U32),
        pltpu.VMEM((M, F), _BF16),
        pltpu.VMEM((M, F), _BF16),
        pltpu.VMEM((F, M + _PAD), _BF16),
        pltpu.VMEM((_HT, M), _F32),
        pltpu.VMEM((_HT, M), _F32),
        pltpu.VMEM((S, M), _BF16),
        pltpu.VMEM((S, M), _BF16),
        pltpu.VMEM((1024, _HT), _U32),
        pltpu.VMEM((S, M), _BF16),
        pltpu.VMEM((M,), _BF16),
        pltpu.SemaphoreType.DMA((S // _TQ + 3,)),
        pltpu.SemaphoreType.DMA((S // _TQ // 2,)),
        pltpu.SemaphoreType.DMA((2,)),
        pltpu.SemaphoreType.DMA((4,)),
        pltpu.SemaphoreType.DMA((2,)),
        pltpu.SemaphoreType.DMA((4,)),
        pltpu.SemaphoreType.DMA((2,)),
    ]
    any_spec = pl.BlockSpec(memory_space=pl.ANY)
    out = pl.pallas_call(
        functools.partial(_kernel, S=S, M=M, DC=DC, H=H, D=D, F=F),
        in_specs=[any_spec] * 10,
        out_specs=any_spec,
        out_shape=jax.ShapeDtypeStruct((S, M), _BF16),
        scratch_shapes=scratch,
        compiler_params=pltpu.CompilerParams(vmem_limit_bytes=124 * 1024 * 1024,
                                             disable_bounds_checks=True,
                                             disable_semaphore_checks=True),
        name="fused_mla_mod",
    )(A_x.reshape(S, M), A_c_kv.reshape(S, DC), A_w_q, A_w_uk, A_w_uv,
      A_w_o.reshape(H * D, M), B_w_r, B_w_gate, B_w_up, B_w_down)
    return out.reshape(B, S, M)
```

```python
import functools
import math

import jax
import jax.numpy as jnp
from jax import lax
import jax.experimental.pallas as pl
import jax.experimental.pallas.tpu as pltpu

_F32 = jnp.float32
_BF16 = jnp.bfloat16
_U32 = jnp.uint32
_I32 = jnp.int32

_EPS = 1e-5
_NEG = -1e30
_TQ = 256
_HT = 128
_QT = 64
_IDX_BITS = 13
_KEY_BIAS = 0x30000000
_FIX = 8
_PAD = 128


def _dot(a, b):
    return jnp.dot(a, b, preferred_element_type=_F32)


def _dot_nt(a, b):
    return lax.dot_general(a, b, (((1,), (1,)), ((), ())), preferred_element_type=_F32)


def _as_bf16(u):
    return pltpu.bitcast(u, _BF16)


def _pack(x):
    return pltpu.bitcast(x.astype(_BF16), _U32)


def _pack_all(xs):
    y = _pack(jnp.concatenate(xs, axis=1))
    return [y[:, k * _HT:(k + 1) * _HT] for k in range(len(xs))]


def _rows(r0, n):
    if isinstance(r0, int):
        return pl.ds(r0 // 2, n // 2)
    return pl.ds(pl.multiple_of(r0 // 2, 8), n // 2)


def _ld(ref, lead, r0, n):
    return _as_bf16(ref[lead, _rows(r0, n), :])


def _st(ref, lead, r0, x, cols=slice(None)):
    ref[lead, _rows(r0, x.shape[0]), cols] = _pack(x)


def _round_bf16(x):
    return x.astype(_BF16).astype(_F32)


def _zero_of(v):
    return (pltpu.bitcast(v, _U32) >> 16) >> 16


def _lo_hi(w):
    return (pltpu.bitcast(w << 16, _F32), pltpu.bitcast(w & jnp.uint32(0xFFFF0000), _F32))


def _row_stats(x):
    n = x.shape[-1]
    mean = jnp.sum(x, axis=-1, keepdims=True) * (1.0 / n)
    xc = x - mean
    return mean, xc, jnp.sum(xc * xc, axis=-1, keepdims=True) * (1.0 / n)


def _layernorm(x):
    mean, _, var = _row_stats(x)
    den = _round_bf16(jnp.sqrt(_round_bf16(_round_bf16(var) + _EPS)))
    return (x - _round_bf16(mean)) * pl.reciprocal(den, approx=True)


def _layernorm_scaled(x, scale):
    _, xc, var = _row_stats(x)
    return xc * (lax.rsqrt(var + _EPS) * scale)


_SA = (((0, 1), (3, 1)), ((2, 1), (3, 1)), ((0, 1),), ((3, 1),),
       ((0, 1), (1, 1)), ((2, 1), (0, -1)), ((1, 1), (3, -1)))
_SB = (((0, 1), (3, 1)), ((0, 1),), ((1, 1), (3, -1)), ((2, 1), (0, -1)),
       ((3, 1),), ((0, 1), (1, 1)), ((2, 1), (3, 1)))
_ORDER = (2, 4, 3, 1, 0, 6, 5)


def _combine(terms):
    terms = sorted(terms, key=lambda ts: -ts[1])
    assert terms[0][1] > 0
    acc = terms[0][0]
    for v, sg in terms[1:]:
        acc = acc + v if sg > 0 else acc - v
    return acc


def _operands(table, quad):
    return [_combine([(quad[q], sg) for q, sg in terms]) for terms in table]


def _strassen_c(m):
    m1, m2, m3, m4, m5, m6, m7 = m
    return (m4 - m5 + m1 + m7, m3 + m5, m4 + m2, m3 - m2 + m1 + m6)


def _sub(q1, q2):
    return 2 * (q1 // 2) + q2 // 2, 2 * (q1 % 2) + q2 % 2


def _pacer(tiles, total, free=0):
    def zero(n):
        if n < free:
            return jnp.zeros((16, _HT), _U32)
        mat, r, c = tiles[(n - free) * len(tiles) // (total - free)]
        z = _zero_of(mat[r:r + 8, c:c + _HT])
        return jnp.concatenate([z, z], axis=0)
    return zero


def _head(tiles, sixteenths):
    return tiles[:len(tiles) * sixteenths // 16]


def _tie(w, ties):
    parts, at = [], 0
    for r in sorted(ties):
        if r > at:
            parts.append(w[at:r])
        parts.append(w[r:r + 8] | ties[r])
        at = r + 8
    if at < w.shape[0]:
        parts.append(w[at:])
    return parts[0] if len(parts) == 1 else jnp.concatenate(parts, axis=0)


def _add_zero(x, z):
    return jnp.concatenate([x[:, :_HT] + pltpu.bitcast(z, _F32), x[:, _HT:]], axis=1)


def _kernel(x_hbm, c_hbm, wq_hbm, wk_hbm, wv_hbm, wo_hbm, wr_hbm, wg_hbm, wu_hbm, wd_hbm,
            out_hbm,
            x_raw, c_raw, xn_s, ca_s, q_s, k_s, v_s, sa_s, sb_s,
            wq_p, wkv_p, wqb_s, wkvb_s,
            ctx_s, wo_p, wob_s, wg_s, wu_s, wd_s, ht_s, hb_s, h_s, hn_s, junk_s, out_s, wr_s,
            sem_x, sem_c, sem_w, sem_wq, sem_wo, sem_ffn, sem_out,
            *, S, M, DC, H, D, F):
    TQ, HT, QT = _TQ, _HT, _QT
    NB = S // TQ
    NH = NB // 2
    NG = S // HT
    NP = H // 2
    KQ, MQ = DC // 4, M // 4
    KO, NO = H * D // 4, M // 4
    OS = KO // NP
    qscale = (D ** -0.5) * math.log2(math.e)

    wq32 = wq_hbm.bitcast(_U32)
    wk32 = wk_hbm.bitcast(_U32)
    wv32 = wv_hbm.bitcast(_U32)

    def w_start(pair, slot):
        for k, src in enumerate((wk32, wv32)):
            pltpu.make_async_copy(src.at[:, pair, :], wkv_p.at[slot, k], sem_w.at[slot]).start()

    def w_wait(slot):
        pltpu.make_async_copy(wkv_p.at[slot], wkv_p.at[slot], sem_w.at[slot]).wait()

    def wq_copy(pair):
        return pltpu.make_async_copy(wq32.at[:, pair, :], wq_p.at[pair & 3],
                                     sem_wq.at[pair & 3])

    def wo_start(t, slot):
        r0 = pl.multiple_of(t * OS, OS)
        for k in range(4):
            pltpu.make_async_copy(wo_hbm.at[pl.ds(k * KO + r0, OS), :],
                                  wo_p.at[slot, k], sem_wo.at[slot]).start()

    def wo_wait(slot):
        pltpu.make_async_copy(wo_p.at[slot], wo_p.at[slot], sem_wo.at[slot]).wait()

    def x_chunk(n):
        return jnp.where(n < NH, n + NH, NB - 1 - n)

    def x_copy(n):
        rows = pl.ds(pl.multiple_of(x_chunk(n) * TQ, TQ), TQ)
        return pltpu.make_async_copy(x_hbm.at[rows, :], x_raw.at[rows, :], sem_x.at[n])

    def x0_copy(k):
        rows = pl.ds(pl.multiple_of(k * QT, QT), QT)
        return pltpu.make_async_copy(x_hbm.at[rows, :], x_raw.at[rows, :], sem_x.at[NB - 1 + k])

    def c_copy(i):
        rows = pl.ds(pl.multiple_of(i * 2 * TQ, 2 * TQ), 2 * TQ)
        return pltpu.make_async_copy(c_hbm.at[rows, :], c_raw.at[rows, :], sem_c.at[i])

    ffn = ((wg_hbm, wg_s), (wu_hbm, wu_s), (wd_hbm, wd_s))

    def ffn_start(t):
        for n, (src, dst) in enumerate(ffn):
            rows, cols = src.shape[0] // NP, src.shape[1]
            r0 = pl.multiple_of(t * rows, 16)
            pltpu.make_async_copy(src.at[pl.ds(r0, rows), :],
                                  dst.at[pl.ds(r0, rows), pl.ds(0, cols)],
                                  sem_ffn.at[n]).start()

    def ffn_wait(n):
        src, dst = ffn[n]
        pltpu.make_async_copy(src, dst.at[:, pl.ds(0, src.shape[1])], sem_ffn.at[n]).wait()

    wr_copy = pltpu.make_async_copy(wr_hbm, wr_s, sem_ffn.at[3])

    def out_copy(g):
        rows = pl.ds(pl.multiple_of(g * HT, HT), HT)
        return pltpu.make_async_copy(out_s.at[rows, :], out_hbm.at[rows, :], sem_out.at[0])

    def prep_w4(srcs, dst, kq, rows, pace, sink=None):
        pieces = [(t, r) for t in range(7) for r in rows]
        for n, (t, r) in enumerate(pieces):
            terms = [[] for _ in range(4)]
            for k, (q1, sg) in enumerate(_SB[t]):
                for rb in range(2):
                    w = srcs[q1 % 2][pl.ds((2 * (q1 // 2) + rb) * kq + r, 16), :]
                    if k == 0:
                        w = w | (pace(n) if sink is not None else pace(2 * n + rb))
                    lo, hi = _lo_hi(w)
                    terms[2 * rb].append((lo, sg))
                    terms[2 * rb + 1].append((hi, sg))
            z = None
            for u, pk in enumerate(_pack_all(_operands(_SB, [_combine(tm) for tm in terms]))):
                dst[7 * t + u, pl.ds(r // 2, 8), :] = pk
                z = pk if z is None else z | pk
            if sink is not None:
                junk_s[pl.ds(8 * (sink + n), 8), :] = z

    def prep_wq(raw, slot, r, nr, pace, sink=None):
        span = 3 * MQ + nr
        prep_w4((wq_p.at[raw, pl.ds(r, span), :], wq_p.at[raw + 1, pl.ds(r, span), :]),
                wqb_s.at[slot, :, pl.ds(pl.multiple_of(r // 2, 8), nr // 2), :],
                MQ, range(0, nr, 16), pace, sink)

    def prep_wo(slot, src0, nrows, dst0, tiles):
        pieces = [(r, c0, t) for r in range(0, nrows, 16) for c0 in range(0, NO, HT)
                  for t in range(7)]
        pace = _pacer(tiles, len(pieces))
        for n, (r, c0, t) in enumerate(pieces):
            z = pltpu.bitcast(pace(n), _F32)
            sub = []
            for q2 in range(4):
                v = _combine([
                    (wo_p[slot, _sub(q1, q2)[0], pl.ds(src0 + r, 16),
                          pl.ds(_sub(q1, q2)[1] * NO + c0, HT)].astype(_F32), sg)
                    for q1, sg in _SB[t]])
                sub.append(v + z if q2 in (0, 3) else v)
            for u, pk in enumerate(_pack_all(_operands(_SB, sub))):
                wob_s[7 * t + u, _rows(dst0 + r, 16), pl.ds(c0, HT)] = pk

    def fence():
        junk_s[pl.ds(0, 8), :] = jnp.zeros((8, HT), _U32)

    def project4(lhs, w, store, zs=()):
        at = {46 * (k + 1) // len(zs): z for k, z in enumerate(zs)}
        m, tiles = [None] * 7, []
        for nt, t in enumerate(_ORDER):
            ps = [None] * 7
            for nu, u in enumerate(_ORDER):
                fence()
                a = lhs(t, u)
                wt = w[7 * t + u]
                if 7 * nt + nu in at:
                    wt = _tie(wt, {0: at[7 * nt + nu]})
                ps[u] = _dot(a.astype(_BF16), _as_bf16(wt))
                tiles += [(ps[u], r, 0) for r in range(0, QT, QT * D // (2 * a.shape[1]))]
            m[t] = _strassen_c(ps)
        for q2 in range(4):
            for q1, cblk in enumerate(_strassen_c([mt[q2] for mt in m])):
                store(_sub(q1, q2)[1], _sub(q1, q2)[0] * QT, cblk)
        return tiles

    def project_q(xn, wqb, q, r0):
        def lhs(t, u):
            return _combine([
                (xn[pl.ds(r0 + _sub(q1, q2)[0] * QT, QT), pl.ds(_sub(q1, q2)[1] * MQ, MQ)],
                 s1 * s2) for q1, s1 in _SA[t] for q2, s2 in _SA[u]])
        return project4(lhs, wqb, lambda nb, r, val: _st(q, nb, r0 + r, val))

    def project_kv(j, zs=()):
        def lhs(t, u):
            return _combine([
                (ca_s[t, pl.ds(j * HT + (q2 // 2) * QT, QT), pl.ds((q2 % 2) * KQ, KQ)], sg)
                for q2, sg in _SA[u]])
        return project4(lhs, wkvb_s,
                        lambda nb, r, val: _st((k_s, v_s)[nb // 2], nb % 2, j * TQ + r, val), zs)

    def stage_x(spans, tiles, dist):
        starts = [r0 + c for r0, nrows in spans for c in range(0, nrows, 8)]
        pace = _pacer(tiles, len(starts))
        done = []
        for n, r in enumerate(starts):
            z = pace(n)[:8]
            if n >= dist:
                z = z | done[n - dist]
            y = _layernorm_scaled(_add_zero(x_raw[pl.ds(r, 8), :].astype(_F32), z), qscale)
            xn_s[pl.ds(r, 8), pl.ds(0, M)] = y
            done.append(_zero_of(y[:, :HT]))

    def stage_c(r0, a0, pace):
        kh = DC // 2
        for n, c in enumerate(range(0, HT, 8)):
            top = c_raw[pl.ds(r0 + c, 8), :].astype(_F32)
            bot = c_raw[pl.ds(r0 + HT + c, 8), :].astype(_F32)
            z = pltpu.bitcast(pace(n)[:8], _F32)
            z = jnp.concatenate([z] * (kh // HT), axis=1)
            quad = (top[:, :kh] + z, top[:, kh:], bot[:, :kh], bot[:, kh:] + z)
            for t, a in enumerate(_operands(_SA, quad)):
                ca_s[t, pl.ds(a0 + c, 8), :] = a

    def issue(n, carry):
        @pl.when(n == 0)
        def _():
            w_start(0, 0)

        @pl.when(n < NH)
        def _():
            c_copy(n).start()

        @pl.when(jnp.logical_or(n == NH, n == NH + 2))
        def _():
            wq_copy(n - NH).start()
            wq_copy(n - NH + 1).start()

        @pl.when(n == NB)
        def _():
            w_start(1, 1)
            wo_start(0, 0)

        @pl.when(jnp.logical_and(n > 0, n < NB))
        def _():
            x_copy(n - 1).start()

        @pl.when(jnp.logical_and(n >= NH, n < NB))
        def _():
            x0_copy(n - NH).start()

        return carry

    lax.fori_loop(0, NB + 1, issue, 0)
    ht_s[...] = jnp.zeros((HT, M), _F32)
    hb_s[...] = jnp.zeros((HT, M), _F32)
    x_raw[pl.ds(S, TQ), :] = jnp.zeros((TQ, M), _BF16)
    w_wait(0)
    c_copy(0).wait()

    def pro_a(i, carry):
        r0 = pl.multiple_of(i * 2 * TQ, 2 * TQ)
        wkv = jnp.concatenate(_lo_hi(wkv_p[0, 0]) + _lo_hi(wkv_p[0, 1]), axis=1).astype(_BF16)
        kv = _dot(c_raw[pl.ds(r0, 2 * TQ), :], wkv)
        for nb in range(4):
            _st((k_s, v_s)[nb // 2], nb % 2, r0, kv[:, nb * D:(nb + 1) * D])
        tiles = [(kv, r, nb * D) for nb in range(4) for r in range(0, 2 * TQ, 8)]
        nt = len(tiles)
        a0 = pl.multiple_of(i * TQ, TQ)
        stage_c(r0, a0, _pacer(tiles[:nt // 2], HT // 8))
        stage_c(r0 + TQ, a0 + HT, _pacer(tiles[nt // 2:nt * 15 // 16], HT // 8))
        rx = pl.multiple_of(jnp.where(i == 0, NB, i + NH - 1) * TQ, TQ)
        stage_x([(rx, TQ)], _head(tiles, 13), 6)

        @pl.when(i + 1 < NH)
        def _():
            c_copy(i + 1).wait()

        x_copy(i).wait()
        return carry

    def pro_b(i, carry):
        r0 = pl.multiple_of(i * TQ, TQ)
        kh = M // 2
        lhs = [xn_s[pl.ds(r0 + S // 2, TQ), pl.ds(k0, kh)].astype(_BF16) for k0 in (0, kh)]
        tiles = []
        for nb in range(4):
            d = [_dot(lhs[k], _lo_hi(wq_p[nb // 2, pl.ds(k * kh, kh), :])[nb % 2].astype(_BF16))
                 for k in range(2)]
            _st(q_s, nb, r0 + S // 2, d[0] + d[1])
            tiles += [(dk, r, 0) for dk in d for r in range(0, TQ, 8)]
        rx = pl.multiple_of(x_chunk(NH - 1 + i) * TQ, TQ)
        stage_x([(rx, TQ), (pl.multiple_of(i * QT, QT), QT)],
                _head(tiles, 12), 7)
        nr = MQ // (2 * NH)
        npc = 7 * nr // 8
        pace = _pacer(tiles, 3 * npc)
        for k in range(3):
            u = 3 * i + k
            quad = u // (2 * NH)
            prep_wq(2 * quad, quad, pl.multiple_of((u % (2 * NH)) * nr, nr), nr,
                    lambda n, k=k: pace(k * npc + n))

        @pl.when(i == 1)
        def _():
            wq_copy(2).wait()
            wq_copy(3).wait()

        @pl.when(i + 1 < NH)
        def _():
            x_copy(NH + i).wait()
            x0_copy(i + 1).wait()

        return carry

    with jax.named_scope('pro_a'):
        lax.fori_loop(0, NH, pro_a, 0)
    wq_copy(0).wait()
    wq_copy(1).wait()
    x0_copy(0).wait()
    with jax.named_scope('pro_b'):
        lax.fori_loop(0, NH, pro_b, 0)

    w_start(2, 0)
    wo_start(1, 1)
    wq_copy(4).start()
    wq_copy(5).start()
    ffn_start(NP - 1)
    wr_copy.start()
    w_wait(1)
    wo_wait(0)

    col = lax.broadcasted_iota(_I32, (QT, HT), 1)
    tri = col <= lax.broadcasted_iota(_I32, (QT, HT), 0) + QT
    tri0 = col <= lax.broadcasted_iota(_I32, (QT, HT), 0)

    def staging(t):
        off = pl.multiple_of((t >> 8) * 32, 32)
        return [r.at[pl.ds(off, TQ), :] for r in (sa_s, sb_s)]

    def softmax_rows(s, m):
        p = jnp.exp2(s - m)
        nt = p.shape[1] // HT
        tiles, acc, grp = [], None, None
        for j in range(nt):
            pj = p[:, j * HT:(j + 1) * HT]
            grp = pj if grp is None else grp + pj
            if j % 4 == 3 or j == nt - 1:
                if j % 4 > 0:
                    pj = jnp.minimum(pj, grp)
                acc = grp if acc is None else acc + grp
                grp = None
            tiles.append(pj)
        return (tiles[0] if nt == 1 else jnp.concatenate(tiles, axis=1)), acc

    def scores(q, e, i, buf, c0, zs=()):
        L0, Lm = i * TQ, i * TQ + HT

        def q_group(g):
            return _as_bf16(jnp.concatenate([q[e, _rows(L0 + g * QT, QT), :],
                                             q[e, _rows(L0 + HT + g * QT, QT), :]], axis=0))

        main, tiles = [[], []], []
        for g in (1, 0):
            k0, n = (1 - g) * QT, L0 + g * HT
            if n > 0:
                ties = {}
                if g == 0:
                    ties = {(k * (n // HT) // len(zs)) * QT + 8 * k: z for k, z in enumerate(zs)}
                m = _dot_nt(q_group(g), _as_bf16(_tie(k_s[e, _rows(k0, n), :], ties)))
                main[g] = [m]
                tiles += [(m, t0 % HT, (t0 // HT) * 4 * HT) for t0 in range(0, n // 4, 8)]
        left = _dot_nt(_ld(k_s, e, 0, QT), q_group(0))
        left = jnp.concatenate([left, jnp.full((QT, HT), _NEG, _F32)], axis=0).T
        last = [_dot_nt(_ld(q, e, L0 + HT + g * QT, QT), _ld(k_s, e, L0 + QT + g * QT, HT))
                for g in range(2)]
        main[0] = [left] + main[0]
        ms = [None] * 4
        for g, m in enumerate(main):
            sm = m[0] if len(m) == 1 else jnp.concatenate(m, axis=1)
            one = [jnp.where(tri0 if g == 0 and i == 0 else tri, sm[:QT, Lm - HT:], _NEG)]
            if Lm > HT:
                one = [sm[:QT, :Lm - HT]] + one
            for h, parts in enumerate((one, [sm[QT:], jnp.where(tri, last[g], _NEG)])):
                sh = parts[0] if len(parts) == 1 else jnp.concatenate(parts, axis=1)
                buf[pl.ds((2 * g + h) * QT, QT), pl.ds(c0, sh.shape[1])] = sh
                ms[2 * g + h] = jnp.max(sh, axis=1, keepdims=True)
        return (buf, c0, ms), tiles

    def context(e, head, i, buf, c0, ms):
        Lm = i * TQ + HT
        os_, ls = [None] * 4, [None] * 4
        for g in (1, 0):
            if g == 1:
                v_main = v_s[e, _rows(0, Lm), :]
            else:
                v_main = v_s[e, _rows(0, HT), :]
                if i > 0:
                    v_main = jnp.concatenate([v_main, v_s[e, _rows(QT, Lm - HT), :]], axis=0)
            v_last = _ld(v_s, e, Lm - (1 - g) * QT, HT)
            p1, ls[g] = softmax_rows(buf[pl.ds(2 * g * QT, QT), pl.ds(c0, Lm)], ms[2 * g])
            p2, ls[2 + g] = softmax_rows(buf[pl.ds((2 * g + 1) * QT, QT), pl.ds(c0, Lm + HT)],
                                         ms[2 * g + 1])
            o = _dot(jnp.concatenate([p1, p2[:, :Lm]], axis=0).astype(_BF16), _as_bf16(v_main))
            os_[g] = o[:QT]
            os_[2 + g] = o[QT:] + _dot(p2[:, Lm:].astype(_BF16), v_last)
        o = jnp.concatenate(os_, axis=0)
        acc = jnp.concatenate(ls, axis=0)

        def normalize(pace=None, n0=0):
            z = None
            for n, g in enumerate(range(0, TQ, 16)):
                a = acc[g:g + 16]
                if pace is not None:
                    a = a + pltpu.bitcast(pace(n0 + n), _F32)
                linv = jnp.broadcast_to(
                    pl.reciprocal(jnp.sum(a, axis=1, keepdims=True), approx=True), (16, D))
                ctx_s.at[head][_rows(i * TQ + g, 16), :] = _pack(o[g:g + 16] * linv)
                bits = pltpu.bitcast(linv, _U32)
                bits = bits[:8] | bits[8:]
                z = bits if z is None else z | bits
            return _zero_of(z)
        return normalize

    def pair_body(s, carry):
        odd = s & 1
        slot = 1 - odd
        wo0 = pl.multiple_of(s * OS, OS)
        q_rd = q_s.at[pl.ds(2 * odd, 2)]
        q_wr = q_s.at[:, pl.ds(pl.multiple_of(odd * (S // 4), S // 4), S // 4), :]
        xn = xn_s.at[pl.ds(pl.multiple_of(odd * (S // 2), S // 2), S // 2), :]
        quad = (s + 1) >> 1
        wqb = wqb_s.at[quad & 1]
        pend, sc = {}, {}
        bufs = staging(s)

        def norm(i, tiles):
            pace = _pacer(tiles, TQ // 8)
            return [f(pace, k * (TQ // 16)) for k, f in enumerate(pend.pop(i))]

        def qk(i, nrm=None):
            c0 = S // 2 if i < 2 else 0
            sa, ta = scores(q_rd, 0, i, bufs[0], c0)
            zs = ()
            if nrm is not None:
                zs = norm(nrm, _head(ta, 14))
            sb, tb = scores(q_rd, 1, i, bufs[1], c0, zs)
            sc[i] = (sa, sb)
            return [ta, tb]

        def pv(i):
            pend[i] = [context(e, 2 * s + e, i, *sc[i][e]) for e in range(2)]

        kv = project_kv
        tl = {}
        for i in range(7, 3, -1):
            tl[i] = qk(i, i + 2 if i + 2 < NB else None)
            if i == 7:
                prep_wq(2 * (jnp.minimum(quad + 1, NP // 2 - 1) & 1), (quad + 1) & 1,
                        pl.multiple_of((1 - odd) * (MQ // 2), MQ // 2), MQ // 2,
                        _pacer(tl[7][0] + _head(tl[7][1], 15), 7 * MQ // 32), 64)
            project_q(xn, wqb, q_wr, (i - NH) * TQ)
            pv(i)
        prep_w4((wkv_p.at[slot, 0], wkv_p.at[slot, 1]), wkvb_s, KQ, range(0, KQ, 16),
                _pacer(tl[6][0] + tl[6][1], 7 * KQ // 16), 1)
        tl[3] = qk(3, 5)
        qk(0)
        kv(7)
        pv(3)
        pv(0)
        z = norm(4, kv(6))
        qk(2)
        qk(1)
        prep_wo(odd, 0, OS, wo0,
                _head(tl[5][0], 8) + _head(tl[5][1], 14) + _head(tl[4][0], 12)
                + _head(tl[4][1], 15) + tl[3][0] + _head(tl[3][1], 12))
        kv(5, z)
        pv(2)
        pv(1)
        t = kv(4)
        for j, i in ((3, 3), (2, 0), (1, 2), (0, 1)):
            t = kv(j, norm(i, t[8:-12]))

        @pl.when(s + 3 < NP)
        def _():
            w_start(s + 3, slot)

        @pl.when(s + 2 < NP)
        def _():
            wo_start(s + 2, odd)

        @pl.when(s + 6 < NP)
        def _():
            wq_copy(s + 6).start()

        ffn_start(s)

        @pl.when(s + 5 < NP)
        def _():
            wq_copy(s + 5).wait()

        @pl.when(s + 2 < NP)
        def _():
            w_wait(odd)

        wo_wait(slot)

        @pl.when(s == 0)
        def _():
            wq_copy(4).wait()

        return carry

    with jax.named_scope('pair_loop'):
        lax.fori_loop(0, NP - 1, pair_body, 0)

    def last_body(e, carry):
        half = OS // 2
        q_rd = q_s.at[pl.ds(2, 2)]
        bufs = staging(e)
        sc, pend = {}, []
        sc[7], tl = scores(q_rd, e, 7, bufs[1], 0)
        prep_wo((NP - 1) % 2, pl.multiple_of(e * half, half), half,
                pl.multiple_of((NP - 1) * OS + e * half, half), tl[:96])
        for step in "s6 c7 s5 c6 s4 c5 s3 s0 c4 s2 s1 c0 c3 c1 c2".split():
            i = int(step[1])
            if step[0] == "s":
                sc[i], _ = (scores(q_rd, e, i, bufs[i % 2], 0) if i >= 2
                            else scores(q_rd, e, i, bufs[1 - i], S // 2))
            else:
                pend.append(context(e, H - 2 + e, i, *sc[i]))
        for f in pend:
            f()
        return carry

    with jax.named_scope('last_loop'):
        lax.fori_loop(0, 2, last_body, 0)

    wr_copy.wait()
    wr = wr_s[...].astype(_F32).reshape(1, M)
    sub8 = lax.broadcasted_iota(_I32, (8, HT), 0)
    NPC = HT // 8

    def epilogue(g, src, top2, pace=None, valid=None):
        r0 = pl.multiple_of(g * HT, HT)
        best, second = top2
        bits = []
        for n, c in enumerate(range(0, HT, 8)):
            hc = src[pl.ds(c, 8), :]
            if pace is not None:
                z = pace(n)[:8]
                if n >= 3:
                    z = z | pltpu.bitcast(bits[n - 3] & 0xFFFF, _U32)
                hc = _add_zero(hc, z)
            hnb = _layernorm(hc).astype(_BF16)
            hn_s[pl.ds(r0 + c, 8), :] = hnb
            hn = hnb.astype(_F32)
            if pace is not None:
                out_s[pl.ds(r0 + c, 8), :] = (hc + hn).astype(_BF16)
            r = jnp.broadcast_to(jnp.sum(hn * wr, axis=1, keepdims=True), (8, HT))
            rb = pltpu.bitcast(_round_bf16(r) + 0.0, _I32)
            bits.append(rb)
            key = ((jnp.where(rb < 0, rb ^ 0x7FFF0000, rb) >> (16 - _IDX_BITS))
                   + ((_KEY_BIAS + S - 1 - c - r0) - sub8))
            key = pltpu.bitcast(key, _F32)
            if valid is not None:
                key = jnp.where(valid, key, 0.0)
            second = jnp.maximum(second, jnp.minimum(best, key))
            best = jnp.maximum(best, key)
        return best, second

    def prod(rh, t, tiles, z=None):
        KS = 2 * D
        ps = [None] * 7
        for u in _ORDER:
            terms = [_sub(q1, q2) + (s1 * s2,) for q1, s1 in _SA[t] for q2, s2 in _SA[u]]
            fence()
            acc = None
            for k0 in range(0, KO, KS):
                def blk(rb, kb):
                    h0 = (kb * KO + k0) // D
                    return jnp.concatenate(
                        [_as_bf16(ctx_s[h0 + hh, pl.ds(rh + rb * QT // 2, QT // 2), :])
                         for hh in range(KS // D)], axis=1)
                if len(terms) == 1:
                    lhs = blk(terms[0][0], terms[0][1])
                else:
                    lhs = _combine([(blk(rb, kb).astype(_F32), sg)
                                    for rb, kb, sg in terms]).astype(_BF16)
                w = wob_s[7 * t + u, _rows(k0, KS), :]
                if z is not None and k0 == 0 and u == _ORDER[1]:
                    w = _tie(w, {0: jnp.concatenate([z, z], axis=1)})
                d = _dot(lhs, _as_bf16(w))
                tiles.append((d, 0, 0))
                acc = d if acc is None else acc + d
            ps[u] = acc
        c11, c12, c21, c22 = _strassen_c(ps)
        return jnp.concatenate([jnp.concatenate([c11, c12], axis=1),
                                jnp.concatenate([c21, c22], axis=1)], axis=0)

    def o_body(j, top2):
        r0 = pl.multiple_of(j * TQ, TQ)

        @pl.when(j > 1)
        def _():
            out_copy(2 * j - 4).start()

        @pl.when(j > 1)
        def _():
            out_copy(2 * j - 3).start()

        rh = pl.multiple_of(j * (TQ // 2), TQ // 2)
        left, right = pl.ds(0, M // 2), pl.ds(M // 2, M // 2)

        def residual(dst, rows0, cols, att):
            hb = (x_raw[pl.ds(rows0, HT), cols].astype(_F32) + att).astype(_BF16)
            h_s[pl.ds(rows0, HT), cols] = hb
            dst[:, cols] = hb.astype(_F32)

        gp = jnp.maximum(2 * j - 2, 0)
        tl = []
        m3 = prod(rh, 2, tl)
        m4 = prod(rh, 3, tl)
        top2 = epilogue(gp, ht_s, top2, _pacer(tl[:len(tl) * 7 // 8], NPC, 1), j > 0)
        tl = []
        m5 = prod(rh, 4, tl, _zero_of(top2[0]))
        residual(ht_s, r0, right, m3 + m5)
        m1 = prod(rh, 0, tl)
        m7 = prod(rh, 6, tl)
        residual(ht_s, r0, left, m4 - m5 + m1 + m7)
        top2 = epilogue(gp + 1, hb_s, top2, _pacer(tl[:len(tl) * 7 // 8], NPC), j > 0)
        m2 = prod(rh, 1, tl, _zero_of(top2[0]))
        residual(hb_s, r0 + HT, left, m4 + m2)
        m6 = prod(rh, 5, tl)
        residual(hb_s, r0 + HT, right, m3 + m1 - m2 + m6)
        return top2

    for n in range(3):
        ffn_wait(n)
    with jax.named_scope('o_loop'):
        top2 = lax.fori_loop(0, NB, o_body, (jnp.zeros((8, HT), _F32),) * 2)
    rest = ((NG - 2, ht_s), (NG - 1, hb_s))
    out_copy(NG - 4).start()
    out_copy(NG - 3).start()
    for g, src in rest:
        top2 = epilogue(g, src, top2)

    best, second = top2
    k1 = jnp.max(best, axis=0, keepdims=True)
    k2 = jnp.max(jnp.where(best == k1, second, best), axis=0, keepdims=True)

    R = _FIX
    row = lax.broadcasted_iota(_I32, (2 * R, HT), 0)
    idx = S - 1 - (pltpu.bitcast(jnp.where(row < R, k1, k2), _I32) & (2 ** _IDX_BITS - 1))
    i1 = jnp.clip(idx[0, 0], 0, S - 1)
    i2 = jnp.clip(idx[R, 0], 0, S - 1)
    b1 = pl.multiple_of(i1 & -R, R)
    b2 = pl.multiple_of(i2 & -R, R)
    tokr = jnp.where(row < R, b1 + row, b2 + row - R)
    cd = (((pltpu.bitcast(jnp.where(tokr == i1, k1, k2), _I32) - _KEY_BIAS) >> _IDX_BITS) << 16)
    score = pltpu.bitcast(jnp.where(cd < 0, cd ^ 0x7FFF0000, cd), _F32)
    gate = _round_bf16(1.0 / (1.0 + jnp.exp(-score)))
    gate = jnp.concatenate([gate] * (M // HT), axis=1)
    tokr = jnp.concatenate([tokr] * (M // HT), axis=1)

    hnsel = jnp.concatenate([hn_s[pl.ds(b1, R), :].astype(_F32),
                             hn_s[pl.ds(b2, R), :].astype(_F32)], axis=0)
    xs = hnsel.astype(_BF16)
    g = _dot(xs, wg_s[...])
    u = _dot(xs, wu_s[...])
    pace = _pacer([(mat, 0, c0) for mat in (g, u) for c0 in range(0, F, HT)], len(rest) * NPC)
    for k, (gi, src) in enumerate(rest):
        for n, c in enumerate(range(0, HT, 8)):
            rows = pl.ds(gi * HT + c, 8)
            z = pltpu.bitcast(pace(k * NPC + n)[:8], _F32)
            z = jnp.concatenate([z] * (M // HT), axis=1)
            out_s[rows, :] = (src[pl.ds(c, 8), :] + z + hn_s[rows, :].astype(_F32)).astype(_BF16)
        out_copy(gi).start()
    g = _round_bf16(g)
    u = _round_bf16(u)
    g = _round_bf16(g * (1.0 / (1.0 + jnp.exp(-g))))
    act = (g * u).astype(_BF16)
    y = _round_bf16(_round_bf16(_dot(act, wd_s[:, pl.ds(0, M)])) * gate)
    upd = jnp.where(jnp.logical_or(tokr == i1, tokr == i2), y, 0.0)
    hsel = jnp.concatenate([h_s[pl.ds(b1, R), :].astype(_F32),
                            h_s[pl.ds(b2, R), :].astype(_F32)], axis=0)
    fixed = hsel + _round_bf16(hnsel + upd)

    pltpu.make_async_copy(out_s, out_hbm, sem_out.at[0]).wait()

    def fix_copy(b0, k):
        return pltpu.make_async_copy(out_s.at[pl.ds(b0, R), :],
                                     out_hbm.at[pl.ds(b0, R), :], sem_out.at[k])

    out_s[pl.ds(b1, R), :] = fixed[:R].astype(_BF16)
    out_s[pl.ds(b2, R), :] = fixed[R:].astype(_BF16)
    fix_copy(b1, 0).start()

    @pl.when(b2 != b1)
    def _():
        fix_copy(b2, 1).start()
        fix_copy(b2, 1).wait()

    fix_copy(b1, 0).wait()


@jax.jit
def pallas_sequential_preLN__compressed_kv_cla__moe_arch_mod__prompt_kernel(
    A_x: jax.Array,
    A_c_kv: jax.Array,
    A_w_q: jax.Array,
    A_w_uk: jax.Array,
    A_w_uv: jax.Array,
    A_w_o: jax.Array,
    B_x: jax.Array,
    B_w_r: jax.Array,
    B_w_gate: jax.Array,
    B_w_up: jax.Array,
    B_w_down: jax.Array,
):
    B, S, M = A_x.shape
    DC = A_c_kv.shape[2]
    H, D = A_w_q.shape[1], A_w_q.shape[2]
    F = B_w_gate.shape[1]
    assert (B, S, M, DC, H, D) == (1, 8 * _TQ, 1024, 512, 32, _HT) and A_c_kv.shape[1] == S
    assert F % (8 * H) == 0 and S <= 2 ** _IDX_BITS

    scratch = [
        pltpu.VMEM((S + _TQ, M), _BF16),
        pltpu.VMEM((S, DC), _BF16),
        pltpu.VMEM((S + _TQ, M + _PAD), _F32),
        pltpu.VMEM((7, S // 2, DC // 2), _F32),
        pltpu.VMEM((4, S // 2, D), _U32),
        pltpu.VMEM((2, S // 2, D), _U32),
        pltpu.VMEM((2, S // 2, D), _U32),
        pltpu.VMEM((_TQ + 32, S + _PAD), _F32),
        pltpu.VMEM((_TQ + 32, S + _PAD), _F32),
        pltpu.VMEM((4, M, D), _U32),
        pltpu.VMEM((2, 2, DC, D), _U32),
        pltpu.VMEM((2, 49, M // 8, D), _U32),
        pltpu.VMEM((49, DC // 8, D), _U32),
        pltpu.VMEM((H, S // 2, D), _U32),
        pltpu.VMEM((2, 4, D // 2, M), _BF16),
        pltpu.VMEM((49, H * D // 8, M // 4), _U32),
        pltpu.VMEM((M, F), _BF16),
        pltpu.VMEM((M, F), _BF16),
        pltpu.VMEM((F, M + _PAD), _BF16),
        pltpu.VMEM((_HT, M), _F32),
        pltpu.VMEM((_HT, M), _F32),
        pltpu.VMEM((S, M), _BF16),
        pltpu.VMEM((S, M), _BF16),
        pltpu.VMEM((1024, _HT), _U32),
        pltpu.VMEM((S, M), _BF16),
        pltpu.VMEM((M,), _BF16),
        pltpu.SemaphoreType.DMA((S // _TQ + 3,)),
        pltpu.SemaphoreType.DMA((S // _TQ // 2,)),
        pltpu.SemaphoreType.DMA((2,)),
        pltpu.SemaphoreType.DMA((4,)),
        pltpu.SemaphoreType.DMA((2,)),
        pltpu.SemaphoreType.DMA((4,)),
        pltpu.SemaphoreType.DMA((2,)),
    ]
    any_spec = pl.BlockSpec(memory_space=pl.ANY)
    out = pl.pallas_call(
        functools.partial(_kernel, S=S, M=M, DC=DC, H=H, D=D, F=F),
        in_specs=[any_spec] * 10,
        out_specs=any_spec,
        out_shape=jax.ShapeDtypeStruct((S, M), _BF16),
        scratch_shapes=scratch,
        compiler_params=pltpu.CompilerParams(vmem_limit_bytes=124 * 1024 * 1024,
                                             disable_bounds_checks=True,
                                             disable_semaphore_checks=True),
        name="fused_mla_mod",
    )(A_x.reshape(S, M), A_c_kv.reshape(S, DC), A_w_q, A_w_uk, A_w_uv,
      A_w_o.reshape(H * D, M), B_w_r, B_w_gate, B_w_up, B_w_down)
    return out.reshape(B, S, M)
```
